```python
import jax
import jax.numpy as jnp

def _softmax(x, axis=-1):
    return jax.nn.softmax(x, axis=axis)
def _gelu(x):
    return jax.nn.gelu(x, approximate=True)
def _silu(x):
    return jax.nn.silu(x)
def _sigmoid(x):
    return jax.nn.sigmoid(x)
def _layernorm(x, axis=-1, eps=1e-5):
    m = jnp.mean(x, axis=axis, keepdims=True)
    v = jnp.var(x, axis=axis, keepdims=True)
    return (x - m) / jnp.sqrt(v + eps)
def _scatter_add(tgt, idx, src, axis=0):
    return tgt.at[idx].add(src)
def _segment_sum(src, seg, n):
    return jax.ops.segment_sum(src, seg, n)
class _Rng:
    def __init__(self, key):
        self._k = key
    def _next(self):
        self._k, sub = jax.random.split(self._k)
        return sub
    def normal(self, shape):
        return jax.random.normal(self._next(), shape, dtype=jnp.bfloat16)
    def randint(self, lo, hi, shape):
        return jax.random.randint(self._next(), shape, lo, hi, dtype=jnp.int32)
    def uniform(self, shape, lo=0.0, hi=1.0):
        return jax.random.uniform(self._next(), shape, jnp.bfloat16, lo, hi)
    def permutation(self, n):
        return jax.random.permutation(self._next(), n)


kernel_name = 'interleave_layers__sliding_local_dilated__glu_gated_geglu__prompt'

def setup_inputs():
    _rng = _Rng(jax.random.key(int.from_bytes(__import__("os").urandom(4), "little")))
    _w = (lambda a: (lambda t: t.astype(jnp.bfloat16) if jnp.issubdtype(t.dtype, jnp.floating) else t)(jnp.asarray(a)))
    def _A_setup():
        B, S, D = 1, 2048, 576
        return {
            "x": _w((lambda *s: _rng.normal(s) * 0.05)(B, S, D)),
            "wqkv": _w((lambda *s: _rng.normal(s) * 0.05)(D, 3 * D)),
            "wo": _w((lambda *s: _rng.normal(s) * 0.05)(D, D)),
        }
    _A_in = _A_setup()

    def _B_setup():
        B, S, Dm, Df = 1, 2048, 576, 4608
        return {
            "x": _w((lambda *s: _rng.normal(s) * 0.05)(B, S, Dm)),
            "w_gate": _w((lambda *s: _rng.normal(s) * 0.05)(Dm, Df) * (Dm ** -0.5)),
            "w_up": _w((lambda *s: _rng.normal(s) * 0.05)(Dm, Df) * (Dm ** -0.5)),
            "w_down": _w((lambda *s: _rng.normal(s) * 0.05)(Df, Dm) * (Df ** -0.5)),
        }
    _B_in = _B_setup()

    return {
        "A_x": _A_in["x"],
        "A_wqkv": _A_in["wqkv"],
        "A_wo": _A_in["wo"],
        "B_x": _B_in["x"],
        "B_w_gate": _B_in["w_gate"],
        "B_w_up": _B_in["w_up"],
        "B_w_down": _B_in["w_down"],
    }

def reference(A_x, A_wqkv, A_wo, B_x, B_w_gate, B_w_up, B_w_down):
    def _A_ref(x, wqkv, wo):
        B, S, D = x.shape
        H = 32; Dh = D // H
        W, dil = 8, 2
        qkv = (lambda x, *d: x.transpose(*d))((x @ wqkv).reshape(B, S, 3, H, Dh), 2, 0, 3, 1, 4)
        q, k, v = qkv[0], qkv[1], qkv[2]
        scale = Dh ** -0.5
        pos = jnp.arange(S)
        off = jnp.arange(W) * dil
        idx = pos[:, None] - off[None, :]
        mask = idx >= 0
        idx_c = jnp.where(mask, idx, 0).reshape(-1)
        kg = k[:, :, idx_c, :].reshape(B, H, S, W, Dh)
        vg = v[:, :, idx_c, :].reshape(B, H, S, W, Dh)
        logits = jnp.einsum("bhsd,bhswd->bhsw", q, kg) * scale
        logits = jnp.where(mask[None, None, :, :], logits, -1e9)
        attn = _softmax(logits, axis=-1)
        o = jnp.einsum("bhsw,bhswd->bhsd", attn, vg)
        return (lambda x, *d: x.transpose(*d))(o, 0, 2, 1, 3).reshape(B, S, D) @ wo

    def _B_ref(x, w_gate, w_up, w_down):
        g = jnp.einsum("bsd,df->bsf", x, w_gate)
        u = jnp.einsum("bsd,df->bsf", x, w_up)
        h = _gelu(g) * u
        return jnp.einsum("bsf,fd->bsd", h, w_down)

    x = A_x
    x = x + _A_ref(_layernorm(x, axis=-1), A_wqkv, A_wo)
    x = x + _B_ref(_layernorm(x, axis=-1), B_w_gate, B_w_up, B_w_down)
    x = x + _A_ref(_layernorm(x, axis=-1), A_wqkv, A_wo)
    x = x + _B_ref(_layernorm(x, axis=-1), B_w_gate, B_w_up, B_w_down)
    return x
```

```python
import functools

import jax
import jax.numpy as jnp
import jax.experimental.pallas as pl
import jax.experimental.pallas.tpu as pltpu
from jax import lax

H = 32
W = 8
DIL = 2
EPS = 1e-5
LANES = 128

F32 = jnp.float32
BF16 = jnp.bfloat16
U32 = jnp.uint32

_NT = (((1,), (1,)), ((), ()))


def _ln_t(x):
    d = x.shape[0]
    m = jnp.sum(x, axis=0, keepdims=True) * (1.0 / d)
    xc = x - m
    v = jnp.sum(xc * xc, axis=0, keepdims=True) * (1.0 / d)
    return xc * lax.rsqrt(v + EPS)


def _gelu_mul(g, u):
    c0 = 0.7978845608028654
    c1 = c0 * 0.044715
    t = jnp.tanh(g * (c0 + c1 * (g * g)))
    return (g * u) * (0.5 + 0.5 * t)


def _lo(x):
    return lax.bitcast_convert_type(x << 16, F32)


def _hi(x):
    return lax.bitcast_convert_type(x & jnp.uint32(0xFFFF0000), F32)


def _make_kernel(S, D, F, TM, P, parts):
    NB = S // TM
    NT = TM // LANES
    DH = D // H
    DP = DH // 2
    RP = D // 2
    scale = float(DH) ** -0.5
    NU = 2 * NB

    def kernel(x_hbm, wqkv_hbm, wo_hbm, wg_hbm, wu_hbm, wdt_hbm, out_hbm,
               x_v, wqkv_v, wo_v, wg_v, wu_v, wdt_v, wqkvt_s, wot_s,
               xin_s, xmid_s, xn2_s, qkv_s, o_s, out_s, sem_x, sem_w, sem_o):

        def x_copy(b):
            return pltpu.make_async_copy(
                x_hbm.at[:, pl.ds(b * TM, TM)], x_v.at[b], sem_x.at[b])

        def out_copy(b):
            off = b * TM
            if not isinstance(b, int):
                off = pl.multiple_of(off, TM)
            return pltpu.make_async_copy(
                out_s.at[b], out_hbm.at[:, pl.ds(off, TM)], sem_o.at[b])

        w_copies = [
            pltpu.make_async_copy(src, dst, sem_w.at[i])
            for i, (src, dst) in enumerate([
                (wqkv_hbm, wqkv_v), (wo_hbm, wo_v), (wg_hbm, wg_v),
                (wu_hbm, wu_v), (wdt_hbm, wdt_v)])]

        lane = lax.broadcasted_iota(jnp.int32, (8, LANES), 1)

        def front(blk, x):
            xn = _ln_t(x).astype(BF16)
            qkv = jnp.dot(wqkvt_s[...], xn, preferred_element_type=F32)
            pk = pltpu.bitcast(qkv.astype(BF16), U32)
            for c in range(NT):
                qkv_s[1 + blk * NT + c] = pk[:, c * LANES:(c + 1) * LANES]

        def shifted(cur, prev, w):
            if w == 0:
                return cur
            sh = DIL * w
            return pltpu.roll(jnp.where(lane < LANES - sh, cur, prev), sh, axis=1)

        def attention(blk, slot):
            for c in range(NT):
                cur = qkv_s.at[1 + blk * NT + c]
                prev = qkv_s.at[blk * NT + c]
                o_t = o_s.at[slot, c]
                for hg in range(H // 8):
                    base = hg * 8 * DP
                    logits = [None] * W
                    for dd in range(DP):
                        q = cur[pl.ds(base + dd, 8, stride=DP), :]
                        kc = cur[pl.ds(RP + base + dd, 8, stride=DP), :]
                        kp = prev[pl.ds(RP + base + dd, 8, stride=DP), :]
                        q0, q1 = _lo(q), _hi(q)
                        for w in range(W):
                            ks = shifted(kc, kp, w)
                            t = q0 * _lo(ks) + q1 * _hi(ks)
                            logits[w] = t if logits[w] is None else logits[w] + t
                    logits = [l * scale for l in logits]
                    if c == 0:
                        pos = lane + blk * TM
                        logits = [l if w == 0 else jnp.where(pos >= DIL * w, l, -1e9)
                                  for w, l in enumerate(logits)]
                    m = functools.reduce(jnp.maximum, logits)
                    e = [jnp.exp(l - m) for l in logits]
                    r = 1.0 / functools.reduce(lambda a, b: a + b, e)
                    p = [x * r for x in e]
                    for dd in range(DP):
                        vc = cur[pl.ds(2 * RP + base + dd, 8, stride=DP), :]
                        vp = prev[pl.ds(2 * RP + base + dd, 8, stride=DP), :]
                        o0 = o1 = None
                        for w in range(W):
                            vs = shifted(vc, vp, w)
                            t0, t1 = p[w] * _lo(vs), p[w] * _hi(vs)
                            o0 = t0 if o0 is None else o0 + t0
                            o1 = t1 if o1 is None else o1 + t1
                        o_t[pl.ds(hg * 8 * DH + 2 * dd, 8, stride=DH), :] = o0
                        o_t[pl.ds(hg * 8 * DH + 2 * dd + 1, 8, stride=DH), :] = o1

        def back(blk, slot):
            attention(blk, slot)
            o = jnp.concatenate([o_s[slot, c] for c in range(NT)], axis=1)
            y = jnp.dot(wot_s[...], o.astype(BF16), preferred_element_type=F32)
            xm = xin_s[blk] + y
            xmid_s[blk] = xm
            xn2_s[blk] = _ln_t(xm).astype(BF16).T

        def ffn_part(xn, lo, hi):
            g = jnp.dot(xn, wg_v[:, lo:hi], preferred_element_type=F32)
            u = jnp.dot(xn, wu_v[:, lo:hi], preferred_element_type=F32)
            h = _gelu_mul(g, u).astype(BF16)
            return lax.dot_general(wdt_v[:, lo:hi], h, _NT, preferred_element_type=F32)

        x_copy(0).start()
        w_copies[0].start()
        qkv_s[0] = jnp.zeros(qkv_s.shape[1:], U32)
        x_copy(0).wait()
        w_copies[0].wait()
        w_copies[1].start()
        for b in range(1, NB):
            x_copy(b).start()
        for cp in w_copies[2:]:
            cp.start()

        wqkvt_s[...] = wqkv_v[...].T
        x0 = x_v[0].astype(F32)
        xin_s[0] = x0
        front(0, x0)

        w_copies[1].wait()
        for b in range(1, NB):
            x_copy(b).wait()
        wot_s[...] = wo_v[...].T
        for b in range(P):
            if b + 1 < P:
                xb = x_v[b + 1].astype(F32)
                xin_s[b + 1] = xb
                front(b + 1, xb)
            back(b, b % 2)
        for b in range(P, NB):
            xin_s[b] = x_v[b].astype(F32)

        for cp in w_copies[2:]:
            cp.wait()

        def body1(u, carry):
            bu = lax.rem(u, NB)
            ba = lax.rem(u + P, NB)
            xn = xn2_s[bu]
            acc = ffn_part(xn, parts[0], parts[1])
            front(ba, xin_s[ba])
            acc = acc + ffn_part(xn, parts[1], parts[2])
            back(ba, 0)
            acc = acc + ffn_part(xn, parts[2], parts[3])
            xo = xmid_s[bu] + acc
            xin_s[bu] = xo
            out_s[bu] = xo.astype(BF16)

            @pl.when(u >= NB)
            def _():
                out_copy(bu).start()
            return carry

        lax.fori_loop(0, NU - P, body1, 0)

        def body2(u, carry):
            bu = u - NB
            acc = ffn_part(xn2_s[bu], 0, F)
            out_s[bu] = (xmid_s[bu] + acc).astype(BF16)
            out_copy(bu).start()
            return carry

        lax.fori_loop(NU - P, NU, body2, 0)

        for b in range(NB):
            out_copy(b).wait()

    scratch = [
        pltpu.VMEM((NB, D, TM), BF16),
        pltpu.VMEM((D, 3 * D), BF16),
        pltpu.VMEM((D, D), BF16),
        pltpu.VMEM((D, F), BF16),
        pltpu.VMEM((D, F), BF16),
        pltpu.VMEM((D, F), BF16),
        pltpu.VMEM((3 * D, D), BF16),
        pltpu.VMEM((D, D), BF16),
        pltpu.VMEM((NB, D, TM), F32),
        pltpu.VMEM((NB, D, TM), F32),
        pltpu.VMEM((NB, TM, D), BF16),
        pltpu.VMEM((S // LANES + 1, 3 * RP, LANES), U32),
        pltpu.VMEM((2, NT, D, LANES), F32),
        pltpu.VMEM((NB, D, TM), BF16),
        pltpu.SemaphoreType.DMA((NB,)),
        pltpu.SemaphoreType.DMA((5,)),
        pltpu.SemaphoreType.DMA((NB,)),
    ]
    return kernel, scratch


def _run(A_x, A_wqkv, A_wo, B_w_gate, B_w_up, B_w_down, *, TM=256, P=7,
         parts=(0, 1536, 3072, 4608)):
    _, S, D = A_x.shape
    F = B_w_gate.shape[1]
    kernel, scratch = _make_kernel(S, D, F, TM, P, parts)
    hbm = pl.BlockSpec(memory_space=pl.ANY)
    out_t = pl.pallas_call(
        kernel,
        in_specs=[hbm] * 6,
        out_specs=hbm,
        out_shape=jax.ShapeDtypeStruct((D, S), A_x.dtype),
        scratch_shapes=scratch,
        compiler_params=pltpu.CompilerParams(vmem_limit_bytes=110 * 1024 * 1024),
    )(A_x[0].T, A_wqkv, A_wo, B_w_gate, B_w_up, B_w_down.T)
    return out_t.T[None]


@jax.jit
def pallas_interleave_layers__sliding_local_dilated__glu_gated_geglu__prompt_kernel(
    A_x: jax.Array,
    A_wqkv: jax.Array,
    A_wo: jax.Array,
    B_x: jax.Array,
    B_w_gate: jax.Array,
    B_w_up: jax.Array,
    B_w_down: jax.Array,
):
    del B_x
    return _run(A_x, A_wqkv, A_wo, B_w_gate, B_w_up, B_w_down)
```

```python
import functools

import jax
import jax.numpy as jnp
import jax.experimental.pallas as pl
import jax.experimental.pallas.tpu as pltpu
from jax import lax

H = 32
W = 8
DIL = 2
EPS = 1e-5
LANES = 128

F32 = jnp.float32
BF16 = jnp.bfloat16
U32 = jnp.uint32

_NT = (((1,), (1,)), ((), ()))


def _ln_t(x):
    d = x.shape[0]
    m = jnp.sum(x, axis=0, keepdims=True) * (1.0 / d)
    xc = x - m
    v = jnp.sum(xc * xc, axis=0, keepdims=True) * (1.0 / d)
    return xc * lax.rsqrt(v + EPS)


def _gelu_mul(g, u):
    c0 = 0.7978845608028654
    c1 = c0 * 0.044715
    t = jnp.tanh(g * (c0 + c1 * (g * g)))
    return (g * u) * (0.5 + 0.5 * t)


def _lo(x):
    return lax.bitcast_convert_type(x << 16, F32)


def _hi(x):
    return lax.bitcast_convert_type(x & jnp.uint32(0xFFFF0000), F32)


def _dot(a, b):
    return jnp.dot(a, b, preferred_element_type=F32)


def _dot_nt(a, b):
    return lax.dot_general(a, b, _NT, preferred_element_type=F32)


def _a_ops(a11, a12, a21, a22):
    return [a11 + a22, a21 + a22, a11, a22, a11 + a12, a21 - a11, a12 - a22]


def _b_ops(b11, b12, b21, b22):
    return [b11 + b22, b11, b12 - b22, b21 - b11, b22, b11 + b12, b21 + b22]


def _combine(m):
    return (m[0] + m[3] - m[4] + m[6], m[2] + m[4], m[1] + m[3],
            m[0] - m[1] + m[2] + m[5])


_A_SUMS = (0, 1, 4, 5, 6)
_B_SUMS = (0, 2, 3, 5, 6)


def _make_kernel(S, D, F, TM, bounds, bounds0):
    NB = S // TM
    NT = TM // LANES
    DH = D // H
    DP = DH // 2
    RP = D // 2
    scale = float(DH) ** -0.5
    NU = 2 * NB
    TH = TM // 2
    FH = F // 2
    D2 = D // 2
    KH = (D // (2 * LANES)) * LANES
    KT = D - 2 * KH
    NC0 = len(bounds0) - 1

    def kernel(x_hbm, wqkv_hbm, wo_hbm, wg_hbm, wu_hbm, wdt_hbm, out_hbm,
               x_v, wqkv_v, wo_v, wg_v, wu_v, wdt_v, wqkvt_s, wot_s,
               gs_s, us_s, ds_s,
               xin_s, xmid_s, a_s, at_s, qkv_s, o_s, out_s,
               sem_x, sem_w, sem_f, sem_o):

        def x_copy(b):
            return pltpu.make_async_copy(
                x_hbm.at[:, pl.ds(b * TM, TM)], x_v.at[b], sem_x.at[b])

        def out_copy(b):
            off = b * TM
            if not isinstance(b, int):
                off = pl.multiple_of(off, TM)
            return pltpu.make_async_copy(
                out_s.at[b], out_hbm.at[:, pl.ds(off, TM)], sem_o.at[b])

        wqkv_copy = pltpu.make_async_copy(wqkv_hbm, wqkv_v, sem_w.at[0])
        wo_copy = pltpu.make_async_copy(wo_hbm, wo_v, sem_w.at[1])

        def ffn_copies(c):
            lo, n = bounds0[c], bounds0[c + 1] - bounds0[c]
            cps = []
            for i, (src, dst) in enumerate(
                    [(wg_hbm, wg_v), (wu_hbm, wu_v), (wdt_hbm, wdt_v)]):
                for j in range(2):
                    sl = pl.ds(j * FH + lo, n)
                    cps.append(pltpu.make_async_copy(
                        src.at[:, sl], dst.at[:, sl], sem_f.at[6 * c + 2 * i + j]))
            return cps

        lane = lax.broadcasted_iota(jnp.int32, (8, LANES), 1)

        def qkv_mm(blk, xn):
            hr = 3 * D // 2
            for r in range(2):
                qkv = _dot(wqkvt_s[r * hr:(r + 1) * hr, :], xn)
                pk = pltpu.bitcast(qkv.astype(BF16), U32)
                for c in range(NT):
                    qkv_s[1 + blk * NT + c, r * hr // 2:(r + 1) * hr // 2, :] = (
                        pk[:, c * LANES:(c + 1) * LANES])

        def shifted(cur, prev, w):
            if w == 0:
                return cur
            sh = DIL * w
            return pltpu.roll(jnp.where(lane < LANES - sh, cur, prev), sh, axis=1)

        def attention(blk):
            for c in range(NT):
                cur = qkv_s.at[1 + blk * NT + c]
                prev = qkv_s.at[blk * NT + c]
                o_t = o_s.at[c]
                for hg in range(H // 8):
                    base = hg * 8 * DP
                    logits = [None] * W
                    for dd in range(DP):
                        q = cur[pl.ds(base + dd, 8, stride=DP), :]
                        kc = cur[pl.ds(RP + base + dd, 8, stride=DP), :]
                        kp = prev[pl.ds(RP + base + dd, 8, stride=DP), :]
                        q0, q1 = _lo(q), _hi(q)
                        for w in range(W):
                            ks = shifted(kc, kp, w)
                            t = q0 * _lo(ks) + q1 * _hi(ks)
                            logits[w] = t if logits[w] is None else logits[w] + t
                    logits = [l * scale for l in logits]
                    if c == 0:
                        pos = lane + blk * TM
                        logits = [l if w == 0 else jnp.where(pos >= DIL * w, l, -1e9)
                                  for w, l in enumerate(logits)]
                    m = functools.reduce(jnp.maximum, logits)
                    e = [jnp.exp(l - m) for l in logits]
                    r = 1.0 / functools.reduce(lambda a, b: a + b, e)
                    p = [x * r for x in e]
                    for dd in range(DP):
                        vc = cur[pl.ds(2 * RP + base + dd, 8, stride=DP), :]
                        vp = prev[pl.ds(2 * RP + base + dd, 8, stride=DP), :]
                        o0 = o1 = None
                        for w in range(W):
                            vs = shifted(vc, vp, w)
                            t0, t1 = p[w] * _lo(vs), p[w] * _hi(vs)
                            o0 = t0 if o0 is None else o0 + t0
                            o1 = t1 if o1 is None else o1 + t1
                        o_t[pl.ds(hg * 8 * DH + 2 * dd, 8, stride=DH), :] = o0
                        o_t[pl.ds(hg * 8 * DH + 2 * dd + 1, 8, stride=DH), :] = o1

        def wo_mm(blk):
            o = jnp.concatenate([o_s[c] for c in range(NT)], axis=1).astype(BF16)
            y = jnp.concatenate([_dot(wot_s[:D2, :], o), _dot(wot_s[D2:, :], o)], axis=0)
            xm = xin_s[blk] + y
            xmid_s[blk] = xm
            xn = _ln_t(xm)
            ops = _a_ops(xn[:KH, :TH], xn[KH:2 * KH, :TH], xn[:KH, TH:], xn[KH:2 * KH, TH:])
            for i in range(7):
                a_s[blk, i] = ops[i].astype(BF16).T
            at_s[blk] = xn[2 * KH:, :].astype(BF16).T

        def prep(lo, hi):
            for w_v, s_s in ((wg_v, gs_s), (wu_v, us_s)):
                ops = _b_ops(w_v[:KH, lo:hi].astype(F32),
                             w_v[:KH, FH + lo:FH + hi].astype(F32),
                             w_v[KH:2 * KH, lo:hi].astype(F32),
                             w_v[KH:2 * KH, FH + lo:FH + hi].astype(F32))
                for j, i in enumerate(_B_SUMS):
                    s_s[j, :, lo:hi] = ops[i].astype(BF16)
            ops = _a_ops(wdt_v[:D2, lo:hi].astype(F32),
                         wdt_v[:D2, FH + lo:FH + hi].astype(F32),
                         wdt_v[D2:, lo:hi].astype(F32),
                         wdt_v[D2:, FH + lo:FH + hi].astype(F32))
            for j, i in enumerate(_A_SUMS):
                ds_s[j, :, lo:hi] = ops[i].astype(BF16)

        def load_lhs(blk):
            return [a_s[blk, i] for i in range(7)], at_s[blk]

        def gu_mm(lhs, lo, hi):
            a, at = lhs

            def proj(w_v, s_s):
                t1 = _dot(at, w_v[2 * KH:, lo:hi])
                t2 = _dot(at, w_v[2 * KH:, FH + lo:FH + hi])
                m = [None] * 7
                m[1] = _dot(a[1], w_v[:KH, lo:hi])
                m[4] = _dot(a[4], w_v[KH:2 * KH, FH + lo:FH + hi])
                for j, i in enumerate(_B_SUMS):
                    m[i] = _dot(a[i], s_s[j, :, lo:hi])
                c11, c12, c21, c22 = _combine(m)
                return c11 + t1[:TH], c12 + t2[:TH], c21 + t1[TH:], c22 + t2[TH:]

            return proj(wg_v, gs_s), proj(wu_v, us_s)

        def act(gu):
            h = [_gelu_mul(g, u) for g, u in zip(*gu)]
            return [b.astype(BF16) for b in _b_ops(h[0], h[2], h[1], h[3])]

        def down_mm(acc, b, lo, hi):
            p = [None] * 7
            p[2] = _dot_nt(wdt_v[:D2, lo:hi], b[2])
            p[3] = _dot_nt(wdt_v[D2:, FH + lo:FH + hi], b[3])
            for j, i in enumerate(_A_SUMS):
                p[i] = _dot_nt(ds_s[j, :, lo:hi], b[i])
            return p if acc is None else [x + y for x, y in zip(acc, p)]

        def finish(blk, acc, keep):
            c11, c12, c21, c22 = _combine(acc)
            y = jnp.concatenate([jnp.concatenate([c11, c12], axis=1),
                                 jnp.concatenate([c21, c22], axis=1)], axis=0)
            xo = xmid_s[blk] + y
            if keep:
                xin_s[blk] = xo
            out_s[blk] = xo.astype(BF16)

        def unit(bu, ba, bf, keep):
            lhs = load_lhs(bu)
            xn1 = None if bf is None else _ln_t(xin_s[bf]).astype(BF16)
            if ba is not None:
                attention(ba)
            n = len(bounds) - 1
            acc, pend = None, None
            for c in range(n):
                b = act(gu_mm(lhs, bounds[c], bounds[c + 1]))
                if pend is not None:
                    acc = down_mm(acc, *pend)
                pend = (b, bounds[c], bounds[c + 1])
                if c == 1 and ba is not None:
                    wo_mm(ba)
            acc = down_mm(acc, *pend)
            finish(bu, acc, keep)
            if bf is not None:
                qkv_mm(bf, xn1)

        x_copy(0).start()
        wqkv_copy.start()
        x_copy(1).start()
        wo_copy.start()
        qkv_s[0] = jnp.zeros(qkv_s.shape[1:], U32)
        x_copy(0).wait()
        wqkv_copy.wait()
        for c in range(NC0):
            for cp in ffn_copies(c):
                cp.start()
            if c == 1:
                for b in range(2, NB):
                    x_copy(b).start()

        wqkvt_s[...] = wqkv_v[...].T
        x0 = x_v[0].astype(F32)
        xin_s[0] = x0
        qkv_mm(0, _ln_t(x0).astype(BF16))

        x_copy(1).wait()
        wo_copy.wait()
        wot_s[...] = wo_v[...].T
        x1 = x_v[1].astype(F32)
        xin_s[1] = x1
        attention(0)
        qkv_mm(1, _ln_t(x1).astype(BF16))
        wo_mm(0)

        acc, gu, pend = None, None, None
        for c in range(NC0):
            lo, hi = bounds0[c], bounds0[c + 1]
            for cp in ffn_copies(c):
                cp.wait()
            if c == 2:
                for b in range(2, NB):
                    x_copy(b).wait()
            lhs = load_lhs(0)
            prep(lo, hi)
            if c == NC0 - 2:
                attention(1)
            if c == NC0 - 1:
                for b in range(2, NB):
                    xin_s[b] = x_v[b].astype(F32)
                xn1 = _ln_t(x_v[2].astype(F32)).astype(BF16)
                wo_mm(1)
            if gu is not None:
                pend = (act(gu), bounds0[c - 1], lo)
            gu = gu_mm(lhs, lo, hi)
            if pend is not None:
                acc = down_mm(acc, *pend)
        b = act(gu)
        qkv_mm(2, xn1)
        acc = down_mm(acc, b, bounds0[-2], bounds0[-1])
        finish(0, acc, True)

        def body(u, carry):
            bu = lax.rem(u, NB)
            unit(bu, lax.rem(u + 1, NB), lax.rem(u + 2, NB), True)

            @pl.when(u >= NB)
            def _():
                out_copy(bu).start()
            return carry

        lax.fori_loop(1, NU - 2, body, 0)

        unit(NB - 2, NB - 1, None, False)
        out_copy(NB - 2).start()
        unit(NB - 1, None, None, False)
        out_copy(NB - 1).start()
        for b in range(NB):
            out_copy(b).wait()

    scratch = [
        pltpu.VMEM((NB, D, TM), BF16),
        pltpu.VMEM((D, 3 * D), BF16),
        pltpu.VMEM((D, D), BF16),
        pltpu.VMEM((D, F), BF16),
        pltpu.VMEM((D, F), BF16),
        pltpu.VMEM((D, F), BF16),
        pltpu.VMEM((3 * D, D), BF16),
        pltpu.VMEM((D, D), BF16),
        pltpu.VMEM((5, KH, FH), BF16),
        pltpu.VMEM((5, KH, FH), BF16),
        pltpu.VMEM((5, D2, FH), BF16),
        pltpu.VMEM((NB, D, TM), F32),
        pltpu.VMEM((NB, D, TM), F32),
        pltpu.VMEM((NB, 7, TH, KH), BF16),
        pltpu.VMEM((NB, TM, KT), BF16),
        pltpu.VMEM((S // LANES + 1, 3 * RP, LANES), U32),
        pltpu.VMEM((NT, D, LANES), F32),
        pltpu.VMEM((NB, D, TM), BF16),
        pltpu.SemaphoreType.DMA((NB,)),
        pltpu.SemaphoreType.DMA((2,)),
        pltpu.SemaphoreType.DMA((6 * NC0,)),
        pltpu.SemaphoreType.DMA((NB,)),
    ]
    return kernel, scratch


def _run(A_x, A_wqkv, A_wo, B_w_gate, B_w_up, B_w_down, *, TM=256,
         bounds=(0, 768, 1536, 2304), bounds0=(0, 256, 768, 1536, 2304)):
    _, S, D = A_x.shape
    F = B_w_gate.shape[1]
    kernel, scratch = _make_kernel(S, D, F, TM, bounds, bounds0)
    hbm = pl.BlockSpec(memory_space=pl.ANY)
    out_t = pl.pallas_call(
        kernel,
        in_specs=[hbm] * 6,
        out_specs=hbm,
        out_shape=jax.ShapeDtypeStruct((D, S), A_x.dtype),
        scratch_shapes=scratch,
        compiler_params=pltpu.CompilerParams(vmem_limit_bytes=110 * 1024 * 1024),
    )(A_x[0].T, A_wqkv, A_wo, B_w_gate, B_w_up, B_w_down.T)
    return out_t.T[None]


@jax.jit
def pallas_interleave_layers__sliding_local_dilated__glu_gated_geglu__prompt_kernel(
    A_x: jax.Array,
    A_wqkv: jax.Array,
    A_wo: jax.Array,
    B_x: jax.Array,
    B_w_gate: jax.Array,
    B_w_up: jax.Array,
    B_w_down: jax.Array,
):
    del B_x
    return _run(A_x, A_wqkv, A_wo, B_w_gate, B_w_up, B_w_down)
```

```python
import functools

import jax
import jax.numpy as jnp
import jax.experimental.pallas as pl
import jax.experimental.pallas.tpu as pltpu
from jax import lax

H = 32
W = 8
DIL = 2
EPS = 1e-5
LANES = 128

F32 = jnp.float32
BF16 = jnp.bfloat16
U32 = jnp.uint32

_NT = (((1,), (1,)), ((), ()))


def _sum0(x):
    parts = [x[i:i + 8] for i in range(0, x.shape[0], 8)]
    while len(parts) > 1:
        nxt = [parts[i] + parts[i + 1] for i in range(0, len(parts) - 1, 2)]
        if len(parts) % 2:
            nxt.append(parts[-1])
        parts = nxt
    return jnp.sum(parts[0], axis=0, keepdims=True)


def _ln_t(x):
    d = x.shape[0]
    m = _sum0(x) * (1.0 / d)
    xc = x - m
    v = _sum0(xc * xc) * (1.0 / d)
    return xc * lax.rsqrt(v + EPS)


def _zero_like_dep(v):
    return (lax.bitcast_convert_type(v, U32) >> 31) >> 1


def _tie(x, anchor):
    if anchor is None:
        return x
    z = lax.bitcast_convert_type(_zero_like_dep(anchor), F32)
    z = jnp.concatenate([z] * (x.shape[1] // LANES), axis=1)
    if x.shape[0] == 8:
        return x + z
    return jnp.concatenate([x[:8] + z, x[8:]], axis=0)


def _gelu_mul(g, u):
    c0 = 0.7978845608028654
    c1 = c0 * 0.044715
    t = jnp.tanh(g * (c0 + c1 * (g * g)))
    return (g * u) * (0.5 + 0.5 * t)


def _lo(x):
    return lax.bitcast_convert_type(x << 16, F32)


def _hi(x):
    return lax.bitcast_convert_type(x & jnp.uint32(0xFFFF0000), F32)


def _dot(a, b):
    return jnp.dot(a, b, preferred_element_type=F32)


def _dot_nt(a, b):
    return lax.dot_general(a, b, _NT, preferred_element_type=F32)


def _a_ops(a11, a12, a21, a22):
    return [a11 + a22, a21 + a22, a11, a22, a11 + a12, a21 - a11, a12 - a22]


def _b_ops(b11, b12, b21, b22):
    return [b11 + b22, b11, b12 - b22, b21 - b11, b22, b11 + b12, b21 + b22]


def _combine(m):
    return (m[0] + m[3] - m[4] + m[6], m[2] + m[4], m[1] + m[3],
            m[0] - m[1] + m[2] + m[5])


_A_SUMS = (0, 1, 4, 5, 6)
_B_SUMS = (0, 2, 3, 5, 6)


def _make_kernel(S, D, F, TM, bounds, bounds0, att_ix, scopes):
    NB = S // TM
    NT = TM // LANES
    DH = D // H
    DP = DH // 2
    RP = D // 2
    scale = float(DH) ** -0.5
    NU = 2 * NB
    TH = TM // 2
    FH = F // 2
    D2 = D // 2
    KH = (D // (2 * LANES)) * LANES
    KT = D - 2 * KH
    NC0 = len(bounds0) - 1
    NQ = 6
    QR = 3 * D // NQ
    WQ = (0, 640, 1152, 3 * D)

    def kernel(x_hbm, wqkv_hbm, wo_hbm, wg_hbm, wu_hbm, wdt_hbm, out_hbm,
               xio_s, wqkv_v, wo_v, wg_v, wu_v, wdt_v, wqkvt_s, wot_s,
               gs_s, us_s, ds_s, xmid_s, a_s, at_s, qkv_s, o_s,
               sem_i, sem_o):

        def scope(name):
            return jax.named_scope(name)

        n_sem = [0]

        def in_copy(src, dst):
            cp = pltpu.make_async_copy(src, dst, sem_i.at[n_sem[0]])
            n_sem[0] += 1
            return cp

        def wait(name, cps):
            if scopes:
                with scope(name):
                    for cp in cps:
                        cp.wait()
            else:
                for cp in cps:
                    cp.wait()

        def out_copy(b):
            off = b * TM
            if not isinstance(b, int):
                off = pl.multiple_of(off, TM)
            return pltpu.make_async_copy(
                xio_s.at[b], out_hbm.at[:, pl.ds(off, TM)], sem_o.at[b])

        x_cp = [in_copy(x_hbm.at[:, pl.ds(b * TM, TM)], xio_s.at[b]) for b in range(NB)]
        wq_cp = [in_copy(wqkv_hbm.at[:, pl.ds(a, b - a)], wqkv_v.at[:, pl.ds(a, b - a)])
                 for a, b in zip(WQ[:-1], WQ[1:])]
        wo_cp = in_copy(wo_hbm, wo_v)

        def col_copies(src, dst, lo, hi):
            return [in_copy(src.at[:, pl.ds(j * FH + lo, hi - lo)],
                            dst.at[:, pl.ds(j * FH + lo, hi - lo)]) for j in range(2)]

        ffn_cp = []
        for c in range(NC0):
            lo, hi = bounds0[c], bounds0[c + 1]
            cps = col_copies(wg_hbm, wg_v, lo, hi) + col_copies(wu_hbm, wu_v, lo, hi)
            if c > 0:
                cps += col_copies(wdt_hbm, wdt_v, bounds0[c - 1],
                                  hi if c == NC0 - 1 else lo)
            ffn_cp.append(cps)

        lane = lax.broadcasted_iota(jnp.int32, (8, LANES), 1)

        def ln1(blk, anchor):
            return _ln_t(_tie(xio_s[blk].astype(F32), anchor)).astype(BF16)

        def qkv_mm(blk, xn, chunks, anchors):
            for r in chunks:
                qkv = _dot(wqkvt_s[r * QR:(r + 1) * QR, :], xn)
                anchors.append(qkv[:8, :LANES])
                anchors.append(qkv[QR - 8:, TM - LANES:])
                pk = pltpu.bitcast(qkv.astype(BF16), U32)
                for c in range(NT):
                    qkv_s[1 + blk * NT + c, r * QR // 2:(r + 1) * QR // 2, :] = (
                        pk[:, c * LANES:(c + 1) * LANES])

        def shifted(ln, cur, prev, w):
            if w == 0:
                return cur
            sh = DIL * w
            return pltpu.roll(jnp.where(ln < LANES - sh, cur, prev), sh, axis=1)

        def attention(blk, anchors):
            for c in range(NT):
                cur = qkv_s.at[1 + blk * NT + c]
                prev = qkv_s.at[blk * NT + c]
                o_t = o_s.at[c]
                for hg in range(H // 8):
                    anchor = anchors[c * (H // 8) + hg]
                    ln = lane + _zero_like_dep(anchor).astype(jnp.int32)
                    base = hg * 8 * DP
                    logits = [None] * W
                    for dd in range(DP):
                        q = cur[pl.ds(base + dd, 8, stride=DP), :]
                        kc = cur[pl.ds(RP + base + dd, 8, stride=DP), :]
                        kp = prev[pl.ds(RP + base + dd, 8, stride=DP), :]
                        q0, q1 = _lo(q), _hi(q)
                        for w in range(W):
                            ks = shifted(ln, kc, kp, w)
                            t = q0 * _lo(ks) + q1 * _hi(ks)
                            logits[w] = t if logits[w] is None else logits[w] + t
                    logits = [l * scale for l in logits]
                    if c == 0:
                        pos = lane + blk * TM
                        logits = [l if w == 0 else jnp.where(pos >= DIL * w, l, -1e9)
                                  for w, l in enumerate(logits)]
                    m = functools.reduce(jnp.maximum, logits)
                    ln = lane + _zero_like_dep(m).astype(jnp.int32)
                    e = [jnp.exp(l - m) for l in logits]
                    r = 1.0 / functools.reduce(lambda a, b: a + b, e)
                    p = [x * r for x in e]
                    for dd in range(DP):
                        vc = cur[pl.ds(2 * RP + base + dd, 8, stride=DP), :]
                        vp = prev[pl.ds(2 * RP + base + dd, 8, stride=DP), :]
                        o0 = o1 = None
                        for w in range(W):
                            vs = shifted(ln, vc, vp, w)
                            t0, t1 = p[w] * _lo(vs), p[w] * _hi(vs)
                            o0 = t0 if o0 is None else o0 + t0
                            o1 = t1 if o1 is None else o1 + t1
                        o_t[pl.ds(hg * 8 * DH + 2 * dd, 8, stride=DH), :] = o0
                        o_t[pl.ds(hg * 8 * DH + 2 * dd + 1, 8, stride=DH), :] = o1

        def wo_mm(blk):
            o = jnp.concatenate([o_s[c] for c in range(NT)], axis=1).astype(BF16)
            y = jnp.concatenate([_dot(wot_s[:D2, :], o), _dot(wot_s[D2:, :], o)], axis=0)
            xm = xio_s[blk].astype(F32) + y
            xmid_s[blk] = xm
            xn = _ln_t(xm)
            ops = _a_ops(xn[:KH, :TH], xn[KH:2 * KH, :TH], xn[:KH, TH:], xn[KH:2 * KH, TH:])
            for i in range(7):
                a_s[blk, i] = ops[i].astype(BF16).T
            at_s[blk] = xn[2 * KH:, :].astype(BF16).T

        def prep(w_v, s_s, half, ops_fn, keep, lo, hi, anchors):
            PR, PC = 16, 256
            patches = [(r, c) for c in range(lo, hi, PC) for r in range(0, half, PR)]
            for n, (r, c) in enumerate(patches):
                anchor = anchors[n * len(anchors) // len(patches)]
                blk = lambda r0, c0: w_v[r0:r0 + PR, c0:c0 + PC].astype(F32)
                ops = ops_fn(_tie(blk(r, c), anchor), blk(r, FH + c),
                             blk(half + r, c), blk(half + r, FH + c))
                for j, i in enumerate(keep):
                    s_s[j, r:r + PR, c:c + PC] = ops[i].astype(BF16)

        def load_lhs(blk):
            return [a_s[blk, i] for i in range(7)], at_s[blk]

        def spread(y, anchors):
            for j in range(y.shape[1] // LANES):
                anchors.append(y[:8, j * LANES:(j + 1) * LANES])
            return y

        def proj_raw(lhs, w_v, lo, hi, anchors):
            a, at = lhs
            t1 = spread(_dot(at, w_v[2 * KH:, lo:hi]), anchors)
            t2 = spread(_dot(at, w_v[2 * KH:, FH + lo:FH + hi]), anchors)
            m1 = spread(_dot(a[1], w_v[:KH, lo:hi]), anchors)
            m4 = spread(_dot(a[4], w_v[KH:2 * KH, FH + lo:FH + hi]), anchors)
            return t1, t2, m1, m4

        def proj_sum(lhs, raw, s_s, lo, hi, anchors):
            a, _ = lhs
            t1, t2, m1, m4 = raw
            m = [None] * 7
            m[1], m[4] = m1, m4
            for j, i in enumerate(_B_SUMS):
                m[i] = spread(_dot(a[i], s_s[j, :, lo:hi]), anchors)
            c11, c12, c21, c22 = _combine(m)
            return c11 + t1[:TH], c12 + t2[:TH], c21 + t1[TH:], c22 + t2[TH:]

        def gu_mm(lhs, lo, hi, anchors):
            g = proj_sum(lhs, proj_raw(lhs, wg_v, lo, hi, anchors), gs_s, lo, hi, anchors)
            u = proj_sum(lhs, proj_raw(lhs, wu_v, lo, hi, anchors), us_s, lo, hi, anchors)
            return g, u

        def act(gu):
            h = [_gelu_mul(g, u) for g, u in zip(*gu)]
            return [b.astype(BF16) for b in _b_ops(h[0], h[2], h[1], h[3])]

        def down_mm(acc, b, lo, hi):
            p = [None] * 7
            p[2] = _dot_nt(wdt_v[:D2, lo:hi], b[2])
            p[3] = _dot_nt(wdt_v[D2:, FH + lo:FH + hi], b[3])
            for j, i in enumerate(_A_SUMS):
                p[i] = _dot_nt(ds_s[j, :, lo:hi], b[i])
            return p if acc is None else [x + y for x, y in zip(acc, p)]

        def finish(blk, acc):
            c11, c12, c21, c22 = _combine(acc)
            y = jnp.concatenate([jnp.concatenate([c11, c12], axis=1),
                                 jnp.concatenate([c21, c22], axis=1)], axis=0)
            xio_s[blk] = (xmid_s[blk] + y).astype(BF16)

        def pick(anchors, fracs):
            return [anchors[min(int(f * len(anchors)), len(anchors) - 1)] for f in fracs]

        def unit(bu, ba, bf):
            lhs = load_lhs(bu)
            n = len(bounds) - 1
            acc, pend, xn1 = None, None, None
            for c in range(n):
                anchors = []
                b = act(gu_mm(lhs, bounds[c], bounds[c + 1], anchors))
                if c == 0 and ba is not None:
                    attention(ba, pick(anchors, att_ix))
                if c == n - 1 and bf is not None:
                    xn1 = ln1(bf, pick(anchors, [0.4])[0])
                if pend is not None:
                    acc = down_mm(acc, *pend)
                pend = (b, bounds[c], bounds[c + 1])
                if c == 1 and ba is not None:
                    wo_mm(ba)
            acc = down_mm(acc, *pend)
            finish(bu, acc)
            if bf is not None:
                qkv_mm(bf, xn1, range(NQ), [])

        order = ([x_cp[0]] + wq_cp + [x_cp[1], wo_cp, x_cp[2]]
                 + [cp for cps in ffn_cp for cp in cps] + x_cp[3:])
        for cp in order:
            cp.start()
        qkv_s[0] = jnp.zeros(qkv_s.shape[1:], U32)
        wait('WX0', [x_cp[0]])
        xn0 = ln1(0, None)
        done = 0
        for i in range(3):
            wait('WQ%d' % i, [wq_cp[i]] + ([x_cp[1], wo_cp, x_cp[2]] if i == 2 else []))
            wqkvt_s[WQ[i]:WQ[i + 1], :] = wqkv_v[:, WQ[i]:WQ[i + 1]].T
            anchors = []
            qkv_mm(0, xn0, range(done, WQ[i + 1] // QR), anchors)
            done = WQ[i + 1] // QR
        xn1 = ln1(1, anchors[0])
        wot_s[...] = wo_v[...].T
        an1 = [anchors[-1]]
        qkv_mm(1, xn1, range(NQ), an1)
        attention(0, [an1[i] for i in (0, 0, 2, 3, 4, 6, 7, 8)])
        xn2 = ln1(2, an1[10])
        wo_mm(0)
        qkv_mm(2, xn2, range(2), [])

        acc, pend = None, None
        for c in range(NC0):
            lo, hi = bounds0[c], bounds0[c + 1]
            wait('WF%d' % c, ffn_cp[c])
            lhs = load_lhs(0)
            an_g, an_u, an_s = [], [], []
            raw_g = proj_raw(lhs, wg_v, lo, hi, an_g)
            raw_u = proj_raw(lhs, wu_v, lo, hi, an_u)
            prep(wg_v, gs_s, KH, _b_ops, _B_SUMS, lo, hi, an_g)
            prep(wu_v, us_s, KH, _b_ops, _B_SUMS, lo, hi, an_u)
            g = proj_sum(lhs, raw_g, gs_s, lo, hi, an_s)
            u = proj_sum(lhs, raw_u, us_s, lo, hi, an_s)
            if c == 0:
                attention(1, pick(an_u + an_s, [0.1 * i for i in range(8)]))
            else:
                prep(wdt_v, ds_s, D2, _a_ops, _A_SUMS, bounds0[c - 1],
                     hi if c == NC0 - 1 else lo, an_s[:len(an_s) * 3 // 4])
            b = act((g, u))
            if c == 0:
                wo_mm(1)
                qkv_mm(2, xn2, range(2, NQ), [])
            else:
                acc = down_mm(acc, *pend)
            pend = (b, lo, hi)
        acc = down_mm(acc, *pend)
        finish(0, acc)
        wait('WX', x_cp[3:])

        def body(u, carry):
            bu = lax.rem(u, NB)
            unit(bu, lax.rem(u + 1, NB), lax.rem(u + 2, NB))

            @pl.when(u >= NB)
            def _():
                out_copy(bu).start()
            return carry

        if scopes:
            with scope('LOOP'):
                lax.fori_loop(1, NU - 2, body, 0)
        else:
            lax.fori_loop(1, NU - 2, body, 0)

        unit(NB - 2, NB - 1, None)
        out_copy(NB - 2).start()
        unit(NB - 1, None, None)
        out_copy(NB - 1).start()
        wait('WOUT', [out_copy(b) for b in range(NB)])

    n_in = NB + 3 + 1 + 4 * NC0 + 2 * (NC0 - 1)
    scratch = [
        pltpu.VMEM((NB, D, TM), BF16),
        pltpu.VMEM((D, 3 * D), BF16),
        pltpu.VMEM((D, D), BF16),
        pltpu.VMEM((D, F), BF16),
        pltpu.VMEM((D, F), BF16),
        pltpu.VMEM((D, F), BF16),
        pltpu.VMEM((3 * D, D), BF16),
        pltpu.VMEM((D, D), BF16),
        pltpu.VMEM((5, KH, FH), BF16),
        pltpu.VMEM((5, KH, FH), BF16),
        pltpu.VMEM((5, D2, FH), BF16),
        pltpu.VMEM((NB, D, TM), F32),
        pltpu.VMEM((NB, 7, TH, KH), BF16),
        pltpu.VMEM((NB, TM, KT), BF16),
        pltpu.VMEM((S // LANES + 1, 3 * RP, LANES), U32),
        pltpu.VMEM((NT, D, LANES), F32),
        pltpu.SemaphoreType.DMA((n_in,)),
        pltpu.SemaphoreType.DMA((NB,)),
    ]
    return kernel, scratch


def _run(A_x, A_wqkv, A_wo, B_w_gate, B_w_up, B_w_down, *, TM=256,
         bounds=(0, 768, 1536, 2304), bounds0=(0, 768, 1792, 2304),
         att_ix=tuple(0.08 * i for i in range(8)), scopes=False):
    _, S, D = A_x.shape
    F = B_w_gate.shape[1]
    kernel, scratch = _make_kernel(S, D, F, TM, bounds, bounds0, att_ix, scopes)
    hbm = pl.BlockSpec(memory_space=pl.ANY)
    out_t = pl.pallas_call(
        kernel,
        in_specs=[hbm] * 6,
        out_specs=hbm,
        out_shape=jax.ShapeDtypeStruct((D, S), A_x.dtype),
        scratch_shapes=scratch,
        compiler_params=pltpu.CompilerParams(vmem_limit_bytes=110 * 1024 * 1024),
    )(A_x[0].T, A_wqkv, A_wo, B_w_gate, B_w_up, B_w_down.T)
    return out_t.T[None]


@jax.jit
def pallas_interleave_layers__sliding_local_dilated__glu_gated_geglu__prompt_kernel(
    A_x: jax.Array,
    A_wqkv: jax.Array,
    A_wo: jax.Array,
    B_x: jax.Array,
    B_w_gate: jax.Array,
    B_w_up: jax.Array,
    B_w_down: jax.Array,
):
    del B_x
    return _run(A_x, A_wqkv, A_wo, B_w_gate, B_w_up, B_w_down)
```

```python
import functools

import jax
import jax.numpy as jnp
import jax.experimental.pallas as pl
import jax.experimental.pallas.tpu as pltpu
from jax import lax

H = 32
W = 8
DIL = 2
EPS = 1e-5
LANES = 128

F32 = jnp.float32
BF16 = jnp.bfloat16
U32 = jnp.uint32

_NT = (((1,), (1,)), ((), ()))


def _tree_sum(parts):
    while len(parts) > 1:
        nxt = [parts[i] + parts[i + 1] for i in range(0, len(parts) - 1, 2)]
        if len(parts) % 2:
            nxt.append(parts[-1])
        parts = nxt
    return parts[0]


def _ln_stats(slabs, d):
    n_acc = 4
    s1, s2, pilot = [None] * n_acc, [None] * n_acc, None
    for i, x in enumerate(slabs):
        if pilot is None:
            pilot = x[0:1, :]
        dx = x - pilot
        j = i % n_acc
        s1[j] = dx if s1[j] is None else s1[j] + dx
        s2[j] = dx * dx if s2[j] is None else s2[j] + dx * dx
    e1 = jnp.sum(_tree_sum(s1), axis=0, keepdims=True) * (1.0 / d)
    e2 = jnp.sum(_tree_sum(s2), axis=0, keepdims=True) * (1.0 / d)
    var = jnp.maximum(e2 - e1 * e1, 0.0)
    return pilot + e1, lax.rsqrt(var + EPS)


def _zero_like_dep(v):
    return (lax.bitcast_convert_type(v, U32) >> 31) >> 1


def _tie(x, anchor):
    if anchor is None:
        return x
    z = lax.bitcast_convert_type(_zero_like_dep(anchor), F32)
    z = jnp.concatenate([z] * (x.shape[1] // LANES), axis=1)
    if x.shape[0] == 8:
        return x + z
    return jnp.concatenate([x[:8] + z, x[8:]], axis=0)


def _gelu_mul(g, u):
    c0 = 0.7978845608028654
    c1 = c0 * 0.044715
    t = jnp.tanh(g * (c0 + c1 * (g * g)))
    return (g * u) * (0.5 + 0.5 * t)


def _lo(x):
    return lax.bitcast_convert_type(x << 16, F32)


def _hi(x):
    return lax.bitcast_convert_type(x & jnp.uint32(0xFFFF0000), F32)


def _pk(x):
    return pltpu.bitcast(x.astype(BF16), U32)


def _upk(x):
    return pltpu.bitcast(x, BF16)


def _dot(a, b):
    return jnp.dot(a, b, preferred_element_type=F32)


def _dot_nt(a, b):
    return lax.dot_general(a, b, _NT, preferred_element_type=F32)


def _a_ops(a11, a12, a21, a22):
    return [a11 + a22, a21 + a22, a11, a22, a11 + a12, a21 - a11, a12 - a22]


def _b_ops(b11, b12, b21, b22):
    return [b11 + b22, b11, b12 - b22, b21 - b11, b22, b11 + b12, b21 + b22]


def _combine(m):
    return (m[0] + m[3] - m[4] + m[6], m[2] + m[4], m[1] + m[3],
            m[0] - m[1] + m[2] + m[5])


_A_SUMS = (0, 1, 4, 5, 6)
_B_SUMS = (0, 2, 3, 5, 6)


def _make_kernel(S, D, F, TM, cfg):
    NB = S // TM
    NT = TM // LANES
    DH = D // H
    DP = DH // 2
    RP = D // 2
    NG = H // 8
    scale = float(DH) ** -0.5
    NU = 2 * NB
    TH = TM // 2
    FH = F // 2
    D2 = D // 2
    KH = (D // (2 * LANES)) * LANES
    KT = D - 2 * KH
    NQ = 6
    QR = 3 * D // NQ
    WQ = (0, 640, 1152, 3 * D)
    PW = 256
    NP = FH // PW
    CW = cfg['cw']
    scopes = cfg['scopes']
    SEM_GU = NB + 4
    SEM_D = SEM_GU + 4 * NP

    def kernel(x_hbm, wqkv_hbm, wo_hbm, wg_hbm, wu_hbm, wdt_hbm, out_hbm,
               xio_s, wqkv_v, wo_v, wg_v, wu_v, wdt_v, wqkvt_s, wot_s,
               gs_s, us_s, ds_s, xmid_s, a_s, at_s, qkv_s, o_s, acc_s, b_s,
               sem_i, sem_o):

        def wait(name, cps):
            if scopes:
                with jax.named_scope(name):
                    for cp in cps:
                        cp.wait()
            else:
                for cp in cps:
                    cp.wait()

        def cols(lo, n):
            if not isinstance(lo, int):
                lo = pl.multiple_of(lo, LANES)
            return pl.ds(lo, n)

        def out_copy(b):
            return pltpu.make_async_copy(
                xio_s.at[b], out_hbm.at[:, cols(b * TM, TM)], sem_o.at[b])

        x_cp = [pltpu.make_async_copy(x_hbm.at[:, cols(b * TM, TM)], xio_s.at[b],
                                      sem_i.at[b]) for b in range(NB)]
        wq_cp = [pltpu.make_async_copy(wqkv_hbm.at[:, cols(a, b - a)],
                                       wqkv_v.at[:, cols(a, b - a)], sem_i.at[NB + i])
                 for i, (a, b) in enumerate(zip(WQ[:-1], WQ[1:]))]
        wo_cp = pltpu.make_async_copy(wo_hbm, wo_v, sem_i.at[NB + 3])

        def piece_cp(src, dst, p, sem0):
            return [pltpu.make_async_copy(src.at[:, cols(j * FH + p * PW, PW)],
                                          dst.at[:, cols(j * FH + p * PW, PW)],
                                          sem_i.at[sem0 + j]) for j in range(2)]

        def gu_cp(p):
            return (piece_cp(wg_hbm, wg_v, p, SEM_GU + 4 * p)
                    + piece_cp(wu_hbm, wu_v, p, SEM_GU + 4 * p + 2))

        def d_cp(p):
            return piece_cp(wdt_hbm, wdt_v, p, SEM_D + 2 * p)

        lane = lax.broadcasted_iota(jnp.int32, (8, LANES), 1)

        def pick(anchors, fracs):
            return [anchors[min(int(f * len(anchors)), len(anchors) - 1)] for f in fracs]

        def ln1(blk, anchor):
            def slabs():
                for r in range(0, D, 8):
                    x = xio_s[blk, r:r + 8, :].astype(F32)
                    yield _tie(x, anchor) if r == 0 else x
            m, rs = _ln_stats(slabs(), D)
            return ((xio_s[blk].astype(F32) - m) * rs).astype(BF16)

        def qkv_mm(blk, xn, chunks, anchors):
            for r in chunks:
                rows = slice(r * QR // 2, (r + 1) * QR // 2)
                qkv = _dot(_upk(wqkvt_s[rows, :]), xn)
                anchors.append(qkv[:8, :LANES])
                anchors.append(qkv[QR - 8:, TM - LANES:])
                pk = _pk(qkv)
                for c in range(NT):
                    qkv_s[1 + blk * NT + c, rows, :] = pk[:, c * LANES:(c + 1) * LANES]

        def shifted(ln, cur, prev, w):
            if w == 0:
                return cur
            sh = DIL * w
            return pltpu.roll(jnp.where(ln < LANES - sh, cur, prev), sh, axis=1)

        def att_group(blk, c, hg, anchor):
            tile = blk * NT + c
            base = hg * 8 * DP
            if isinstance(hg, int):
                cur, prev, o_t = qkv_s.at[1 + tile], qkv_s.at[tile], o_s.at[c]
                obase = hg * 8 * DH
            else:
                n = 2 * RP + 8 * DP
                base = pl.multiple_of(base, 8)
                cur = qkv_s.at[1 + tile, pl.ds(base, n)]
                prev = qkv_s.at[tile, pl.ds(base, n)]
                o_t = o_s.at[c, pl.ds(pl.multiple_of(hg * 8 * DH, 8), 8 * DH)]
                base, obase = 0, 0
            ln = lane + _zero_like_dep(anchor).astype(jnp.int32)
            logits = [None] * W
            for dd in range(DP):
                q = cur[pl.ds(base + dd, 8, stride=DP), :]
                kc = cur[pl.ds(RP + base + dd, 8, stride=DP), :]
                kp = prev[pl.ds(RP + base + dd, 8, stride=DP), :]
                q0, q1 = _lo(q), _hi(q)
                for w in range(W):
                    ks = shifted(ln, kc, kp, w)
                    t = q0 * _lo(ks) + q1 * _hi(ks)
                    logits[w] = t if logits[w] is None else logits[w] + t
            logits = [l * scale for l in logits]
            if not (isinstance(c, int) and c > 0):
                pos = lane + tile * LANES
                logits = [l if w == 0 else jnp.where(pos >= DIL * w, l, -1e9)
                          for w, l in enumerate(logits)]
            m = functools.reduce(jnp.maximum, logits)
            ln = lane + _zero_like_dep(m).astype(jnp.int32)
            e = [jnp.exp(l - m) for l in logits]
            r = 1.0 / functools.reduce(lambda a, b: a + b, e)
            p = [x * r for x in e]
            for dd in range(DP):
                vc = cur[pl.ds(2 * RP + base + dd, 8, stride=DP), :]
                vp = prev[pl.ds(2 * RP + base + dd, 8, stride=DP), :]
                o0 = o1 = None
                for w in range(W):
                    vs = shifted(ln, vc, vp, w)
                    t0, t1 = p[w] * _lo(vs), p[w] * _hi(vs)
                    o0 = t0 if o0 is None else o0 + t0
                    o1 = t1 if o1 is None else o1 + t1
                o_t[pl.ds(obase + 2 * dd, 8, stride=DH), :] = o0
                o_t[pl.ds(obase + 2 * dd + 1, 8, stride=DH), :] = o1

        def attention(blk, anchors):
            for c in range(NT):
                for hg in range(NG):
                    att_group(blk, c, hg, anchors[c * NG + hg])

        def wo_mm(blk, anchors):
            o = jnp.concatenate([o_s[c] for c in range(NT)], axis=1).astype(BF16)
            ys = [_dot(_upk(wot_s[:D2 // 2, :]), o), _dot(_upk(wot_s[D2 // 2:, :]), o)]
            for y in ys:
                anchors.append(y[:8, :LANES])
                anchors.append(y[D2 - 8:, TM - LANES:])
            xm = xio_s[blk].astype(F32) + jnp.concatenate(ys, axis=0)
            xmid_s[blk] = xm
            return _ln_stats((xm[r:r + 8] for r in range(0, D, 8)), D)

        def ffn_lhs(blk, stats, anchors):
            m, rs = stats

            def xn(r0, n, anchor=None):
                return (_tie(xmid_s[blk, r0:r0 + n, :], anchor) - m) * rs

            for j, r in enumerate(range(0, KH, LANES)):
                lo, hi = xn(r, LANES, anchors[j]), xn(KH + r, LANES)
                ops = _a_ops(lo[:, :TH], hi[:, :TH], lo[:, TH:], hi[:, TH:])
                for i in range(7):
                    a_s[blk, i, :, r:r + LANES] = _pk(ops[i].astype(BF16).T)
            at_s[blk] = _pk(xn(2 * KH, KT, anchors[-1]).astype(BF16).T)

        def prep(w_v, s_s, half, ops_fn, keep, lo, anchors):
            PR = 16
            rows = range(0, half, PR)
            for n, r in enumerate(rows):
                anchor = anchors[n * len(anchors) // len(rows)]
                blk = lambda r0, c0: w_v[r0:r0 + PR, cols(c0, PW)].astype(F32)
                ops = ops_fn(_tie(blk(r, lo), anchor), blk(r, FH + lo),
                             blk(half + r, lo), blk(half + r, FH + lo))
                for j, i in enumerate(keep):
                    s_s[j, r // 2:(r + PR) // 2, cols(lo, PW)] = _pk(ops[i])

        def load_lhs(blk):
            return [_upk(a_s[blk, i]) for i in range(7)], _upk(at_s[blk])

        def spread(y, anchors):
            for j in range(y.shape[1] // LANES):
                anchors.append(y[:8, j * LANES:(j + 1) * LANES])
            return y

        def proj_raw(lhs, w_v, lo, n, anchors):
            a, at = lhs
            t1 = spread(_dot(at, w_v[2 * KH:, cols(lo, n)]), anchors)
            t2 = spread(_dot(at, w_v[2 * KH:, cols(FH + lo, n)]), anchors)
            m1 = spread(_dot(a[1], w_v[:KH, cols(lo, n)]), anchors)
            m4 = spread(_dot(a[4], w_v[KH:2 * KH, cols(FH + lo, n)]), anchors)
            return t1, t2, m1, m4

        def proj_sum(lhs, raw, s_s, lo, n, anchors):
            a, _ = lhs
            t1, t2, m1, m4 = raw
            m = [None] * 7
            m[1], m[4] = m1, m4
            for j, i in enumerate(_B_SUMS):
                m[i] = spread(_dot(a[i], _upk(s_s[j, :, cols(lo, n)])), anchors)
            c11, c12, c21, c22 = _combine(m)
            return c11 + t1[:TH], c12 + t2[:TH], c21 + t1[TH:], c22 + t2[TH:]

        def act(g, u):
            h = [_gelu_mul(a, b) for a, b in zip(g, u)]
            return [b.astype(BF16) for b in _b_ops(h[0], h[2], h[1], h[3])]

        def gu_act(lhs, lo, n, anchors):
            g = proj_sum(lhs, proj_raw(lhs, wg_v, lo, n, anchors), gs_s, lo, n, anchors)
            u = proj_sum(lhs, proj_raw(lhs, wu_v, lo, n, anchors), us_s, lo, n, anchors)
            return act(g, u)

        def gu_act_prep(lhs, lo, anchors):
            an_g, an_u = [], []
            raw_g = proj_raw(lhs, wg_v, lo, PW, an_g)
            raw_u = proj_raw(lhs, wu_v, lo, PW, an_u)
            prep(wg_v, gs_s, KH, _b_ops, _B_SUMS, lo, an_g)
            prep(wu_v, us_s, KH, _b_ops, _B_SUMS, lo, an_u)
            g = proj_sum(lhs, raw_g, gs_s, lo, PW, anchors)
            u = proj_sum(lhs, raw_u, us_s, lo, PW, anchors)
            return act(g, u)

        def down_mm(acc, b, lo, n, anchors):
            p = [None] * 7
            p[2] = _dot_nt(wdt_v[:D2, cols(lo, n)], b[2])
            p[3] = _dot_nt(wdt_v[D2:, cols(FH + lo, n)], b[3])
            for j, i in enumerate(_A_SUMS):
                p[i] = _dot_nt(_upk(ds_s[j, :, cols(lo, n)]), b[i])
            p = p if acc is None else [x + y for x, y in zip(acc, p)]
            anchors.extend(p[i][:8] for i in (2, 3) + _A_SUMS)
            return p

        def finish(blk, acc):
            c11, c12, c21, c22 = _combine(acc)
            y = jnp.concatenate([jnp.concatenate([c11, c12], axis=1),
                                 jnp.concatenate([c21, c22], axis=1)], axis=0)
            xio_s[blk] = (xmid_s[blk] + y).astype(BF16)

        def load_acc():
            return [acc_s[i] for i in range(7)]

        def store_acc(acc):
            for i in range(7):
                acc_s[i] = acc[i]

        order = [x_cp[0], wq_cp[0], wq_cp[1], x_cp[1], wq_cp[2], wo_cp] + gu_cp(0)
        for p in range(1, NP):
            order += gu_cp(p) + d_cp(p - 1)
        order += d_cp(NP - 1) + x_cp[2:]
        for cp in order:
            cp.start()
        qkv_s[0] = jnp.zeros(qkv_s.shape[1:], U32)
        acc_s[...] = jnp.zeros(acc_s.shape, F32)
        wait('WX0', [x_cp[0]])
        xn0 = ln1(0, None)
        done = 0
        for i in range(3):
            wait('WQ%d' % i, [wq_cp[i]] + ([x_cp[1]] if i == 2 else []))
            wqkvt_s[WQ[i] // 2:WQ[i + 1] // 2, :] = _pk(wqkv_v[:, WQ[i]:WQ[i + 1]].T)
            anchors = []
            qkv_mm(0, xn0, range(done, WQ[i + 1] // QR), anchors)
            done = WQ[i + 1] // QR
        xn1 = ln1(1, anchors[0])
        an1 = [anchors[-1]]
        qkv_mm(1, xn1, range(4), an1)
        attention(0, [an1[i] for i in cfg['att0']])
        wait('WO', [wo_cp] + gu_cp(0))
        wot_s[...] = _pk(wo_v[...].T)
        stats = wo_mm(0, [])
        qkv_mm(1, xn1, [4], [])
        ffn_lhs(0, stats, [None, None, None])
        b = gu_act_prep(load_lhs(0), 0, [])
        qkv_mm(1, xn1, [5], [])
        for i in range(7):
            b_s[i] = _pk(b[i])

        def piece(p, carry):
            wait('WP', gu_cp(p) + d_cp(p - 1))
            lhs = load_lhs(0)
            b_prev = [_upk(b_s[i]) for i in range(7)]
            an = []
            b = gu_act_prep(lhs, p * PW, an)
            prep(wdt_v, ds_s, D2, _a_ops, _A_SUMS, (p - 1) * PW, an[:len(an) * 3 // 4])
            g = p - 1
            att_group(1, g // NG, lax.rem(g, NG), an[0])
            store_acc(down_mm(load_acc(), b_prev, (p - 1) * PW, PW, []))
            for i in range(7):
                b_s[i] = _pk(b[i])
            return carry

        lax.fori_loop(1, NP, piece, 0)

        wait('WD', d_cp(NP - 1) + x_cp[2:])
        an = []
        stats = wo_mm(1, an)
        prep(wdt_v, ds_s, D2, _a_ops, _A_SUMS, (NP - 1) * PW, an[:2])
        acc = down_mm(load_acc(), [_upk(b_s[i]) for i in range(7)], (NP - 1) * PW, PW, [])
        ffn_lhs(1, stats, [None, None, None])
        finish(0, acc)

        def body(u, carry):
            bu = lax.rem(u, NB)
            ba = lax.rem(u + 1, NB)
            lhs = load_lhs(bu)
            an = []
            b0 = gu_act(lhs, 0, CW, an)
            xn = ln1(ba, pick(an, [cfg['ln1']])[0])
            qkv_mm(ba, xn, range(NQ), [])
            an = []
            b1 = gu_act(lhs, CW, CW, an)
            attention(ba, pick(an, cfg['att']))
            acc = down_mm(None, b0, 0, CW, [])
            stats = wo_mm(ba, [])
            an = []
            b2 = gu_act(lhs, 2 * CW, CW, an)
            ffn_lhs(ba, stats, pick(an, cfg['lhs']))
            acc = down_mm(acc, b1, CW, CW, [])
            acc = down_mm(acc, b2, 2 * CW, CW, [])
            finish(bu, acc)

            @pl.when(u >= NB)
            def _():
                out_copy(bu).start()
            return carry

        if scopes:
            with jax.named_scope('LOOP'):
                lax.fori_loop(1, NU - 1, body, 0)
        else:
            lax.fori_loop(1, NU - 1, body, 0)

        acc_s[...] = jnp.zeros(acc_s.shape, F32)

        def last(c, carry):
            lhs = load_lhs(NB - 1)
            acc, pend = load_acc(), None
            for j in range(CW // PW):
                lo = c * CW + j * PW
                b = gu_act(lhs, lo, PW, [])
                if pend is not None:
                    acc = down_mm(acc, *pend, PW, [])
                pend = (b, lo)
            store_acc(down_mm(acc, *pend, PW, []))
            return carry

        lax.fori_loop(0, FH // CW, last, 0)
        finish(NB - 1, load_acc())
        out_copy(NB - 1).start()
        wait('WOUT', [out_copy(b) for b in range(NB)])

    scratch = [
        pltpu.VMEM((NB, D, TM), BF16),
        pltpu.VMEM((D, 3 * D), BF16),
        pltpu.VMEM((D, D), BF16),
        pltpu.VMEM((D, F), BF16),
        pltpu.VMEM((D, F), BF16),
        pltpu.VMEM((D, F), BF16),
        pltpu.VMEM((3 * D // 2, D), U32),
        pltpu.VMEM((D // 2, D), U32),
        pltpu.VMEM((5, KH // 2, FH), U32),
        pltpu.VMEM((5, KH // 2, FH), U32),
        pltpu.VMEM((5, D2 // 2, FH), U32),
        pltpu.VMEM((NB, D, TM), F32),
        pltpu.VMEM((NB, 7, TH // 2, KH), U32),
        pltpu.VMEM((NB, TM // 2, KT), U32),
        pltpu.VMEM((S // LANES + 1, 3 * RP, LANES), U32),
        pltpu.VMEM((NT, D, LANES), F32),
        pltpu.VMEM((7, D2, TH), F32),
        pltpu.VMEM((7, TH // 2, PW), U32),
        pltpu.SemaphoreType.DMA((SEM_D + 2 * NP,)),
        pltpu.SemaphoreType.DMA((NB,)),
    ]
    return kernel, scratch


_CFG = dict(cw=768, scopes=False, ln1=0.3, att=tuple(0.08 * i for i in range(8)),
            lhs=(0.1, 0.2, 0.3), att0=(0, 0, 1, 2, 3, 4, 5, 6))


def _run(A_x, A_wqkv, A_wo, B_w_gate, B_w_up, B_w_down, **kw):
    _, S, D = A_x.shape
    F = B_w_gate.shape[1]
    kernel, scratch = _make_kernel(S, D, F, 256, {**_CFG, **kw})
    hbm = pl.BlockSpec(memory_space=pl.ANY)
    out_t = pl.pallas_call(
        kernel,
        in_specs=[hbm] * 6,
        out_specs=hbm,
        out_shape=jax.ShapeDtypeStruct((D, S), A_x.dtype),
        scratch_shapes=scratch,
        compiler_params=pltpu.CompilerParams(vmem_limit_bytes=110 * 1024 * 1024),
    )(A_x[0].T, A_wqkv, A_wo, B_w_gate, B_w_up, B_w_down.T)
    return out_t.T[None]


@jax.jit
def pallas_interleave_layers__sliding_local_dilated__glu_gated_geglu__prompt_kernel(
    A_x: jax.Array,
    A_wqkv: jax.Array,
    A_wo: jax.Array,
    B_x: jax.Array,
    B_w_gate: jax.Array,
    B_w_up: jax.Array,
    B_w_down: jax.Array,
):
    del B_x
    return _run(A_x, A_wqkv, A_wo, B_w_gate, B_w_up, B_w_down)
```

```python
import functools

import jax
import jax.numpy as jnp
import jax.experimental.pallas as pl
import jax.experimental.pallas.tpu as pltpu
from jax import lax

H = 32
W = 8
DIL = 2
EPS = 1e-5
LANES = 128

F32 = jnp.float32
BF16 = jnp.bfloat16
U32 = jnp.uint32

_NT = (((1,), (1,)), ((), ()))


def _tree_sum(parts):
    while len(parts) > 1:
        nxt = [parts[i] + parts[i + 1] for i in range(0, len(parts) - 1, 2)]
        if len(parts) % 2:
            nxt.append(parts[-1])
        parts = nxt
    return parts[0]


def _ln_stats(slabs, d):
    n_acc = 4
    s1, s2, pilot = [None] * n_acc, [None] * n_acc, None
    for i, x in enumerate(slabs):
        if pilot is None:
            pilot = x[0:1, :]
        dx = x - pilot
        j = i % n_acc
        s1[j] = dx if s1[j] is None else s1[j] + dx
        s2[j] = dx * dx if s2[j] is None else s2[j] + dx * dx
    e1 = jnp.sum(_tree_sum(s1), axis=0, keepdims=True) * (1.0 / d)
    e2 = jnp.sum(_tree_sum(s2), axis=0, keepdims=True) * (1.0 / d)
    var = jnp.maximum(e2 - e1 * e1, 0.0)
    return pilot + e1, lax.rsqrt(var + EPS)


def _zero_like_dep(v):
    return (lax.bitcast_convert_type(v, U32) >> 31) >> 1


def _tie(x, anchor):
    if anchor is None:
        return x
    z = lax.bitcast_convert_type(_zero_like_dep(anchor), F32)
    z = jnp.concatenate([z] * (x.shape[1] // LANES), axis=1)
    if x.shape[0] == 8:
        return x + z
    return jnp.concatenate([x[:8] + z, x[8:]], axis=0)


def _gelu_mul(g, u):
    c0 = 0.7978845608028654
    c1 = c0 * 0.044715
    t = jnp.tanh(g * (c0 + c1 * (g * g)))
    return (g * u) * (0.5 + 0.5 * t)


def _lo(x):
    return lax.bitcast_convert_type(x << 16, F32)


def _hi(x):
    return lax.bitcast_convert_type(x & jnp.uint32(0xFFFF0000), F32)


def _pk(x):
    return pltpu.bitcast(x.astype(BF16), U32)


def _upk(x):
    return pltpu.bitcast(x, BF16)


def _dot(a, b):
    return jnp.dot(a, b, preferred_element_type=F32)


def _dot_nt(a, b):
    return lax.dot_general(a, b, _NT, preferred_element_type=F32)


def _a_ops(a11, a12, a21, a22):
    return [a11 + a22, a21 + a22, a11, a22, a11 + a12, a21 - a11, a12 - a22]


def _b_ops(b11, b12, b21, b22):
    return [b11 + b22, b11, b12 - b22, b21 - b11, b22, b11 + b12, b21 + b22]


def _combine(m):
    return (m[0] + m[3] - m[4] + m[6], m[2] + m[4], m[1] + m[3],
            m[0] - m[1] + m[2] + m[5])


def _c17(r):
    p2, p5, p3, p4, ra, rb, e11, e12, e21, e22 = r
    return (ra + p4 - p5 + e11, rb + p3 + p5 + e12,
            rb + p2 + p4 + e21, ra - p2 + p3 + e22)


_A_SUMS = (0, 1, 4, 5, 6)
_B_SUMS = (0, 2, 3, 5, 6)


def _make_kernel(S, D, F, TM, cfg):
    NB = S // TM
    NT = TM // LANES
    DH = D // H
    DP = DH // 2
    RP = D // 2
    NG = H // 8
    scale = float(DH) ** -0.5
    NU = 2 * NB
    TH = TM // 2
    FH = F // 2
    D2 = D // 2
    KU = D // 9
    KA, KB = slice(0, 3 * KU), slice(3 * KU, 6 * KU)
    KC, KD, KE = (slice(6 * KU, 7 * KU), slice(7 * KU, 8 * KU), slice(8 * KU, 9 * KU))
    KS = 4 * KU
    LW = (KS, KS, KS, KS, 3 * KU, KU, KS, 2 * KU, 2 * KU, KS)
    LO = [0]
    for w_ in LW:
        LO.append(LO[-1] + -(-w_ // LANES) * LANES)
    NQ = 6
    QR = 3 * D // NQ
    WQ = (0, 640, 1152, 3 * D)
    PW = 256
    NP = FH // PW
    CW = cfg['cw']
    scopes = cfg['scopes']
    SEM_GU = NB + 4
    SEM_D = SEM_GU + 4 * NP

    def kernel(x_hbm, wqkv_hbm, wo_hbm, wg_hbm, wu_hbm, wdt_hbm, out_hbm,
               xio_s, wqkv_v, wo_v, wg_v, wu_v, wdt_v, wqkvt_s, wot_s,
               gs_s, us_s, ds_s, xmid_s, a_s, qkv_s, o_s, acc_s, b_s,
               sem_i, sem_o):

        def wait(name, cps):
            if scopes:
                with jax.named_scope(name):
                    for cp in cps:
                        cp.wait()
            else:
                for cp in cps:
                    cp.wait()

        def cols(lo, n):
            if not isinstance(lo, int):
                lo = pl.multiple_of(lo, LANES)
            return pl.ds(lo, n)

        def out_copy(b):
            return pltpu.make_async_copy(
                xio_s.at[b], out_hbm.at[:, cols(b * TM, TM)], sem_o.at[b])

        x_cp = [pltpu.make_async_copy(x_hbm.at[:, cols(b * TM, TM)], xio_s.at[b],
                                      sem_i.at[b]) for b in range(NB)]
        wq_cp = [pltpu.make_async_copy(wqkv_hbm.at[:, cols(a, b - a)],
                                       wqkv_v.at[:, cols(a, b - a)], sem_i.at[NB + i])
                 for i, (a, b) in enumerate(zip(WQ[:-1], WQ[1:]))]
        wo_cp = pltpu.make_async_copy(wo_hbm, wo_v, sem_i.at[NB + 3])

        def piece_cp(src, dst, p, sem0):
            return [pltpu.make_async_copy(src.at[:, cols(j * FH + p * PW, PW)],
                                          dst.at[:, cols(j * FH + p * PW, PW)],
                                          sem_i.at[sem0 + j]) for j in range(2)]

        def gu_cp(p):
            return (piece_cp(wg_hbm, wg_v, p, SEM_GU + 4 * p)
                    + piece_cp(wu_hbm, wu_v, p, SEM_GU + 4 * p + 2))

        def d_cp(p):
            return piece_cp(wdt_hbm, wdt_v, p, SEM_D + 2 * p)

        lane = lax.broadcasted_iota(jnp.int32, (8, LANES), 1)

        def pick(anchors, fracs):
            return [anchors[min(int(f * len(anchors)), len(anchors) - 1)] for f in fracs]

        def ln1(blk, anchor):
            def slabs():
                for r in range(0, D, 8):
                    x = xio_s[blk, r:r + 8, :].astype(F32)
                    yield _tie(x, anchor) if r == 0 else x
            m, rs = _ln_stats(slabs(), D)
            return ((xio_s[blk].astype(F32) - m) * rs).astype(BF16)

        def qkv_mm(blk, xn, chunks, anchors):
            for r in chunks:
                rows = slice(r * QR // 2, (r + 1) * QR // 2)
                qkv = _dot(_upk(wqkvt_s[rows, :]), xn)
                anchors.append(qkv[:8, :LANES])
                anchors.append(qkv[QR - 8:, TM - LANES:])
                pk = _pk(qkv)
                for c in range(NT):
                    qkv_s[1 + blk * NT + c, rows, :] = pk[:, c * LANES:(c + 1) * LANES]

        def shifted(ln, cur, prev, w):
            if w == 0:
                return cur
            sh = DIL * w
            return pltpu.roll(jnp.where(ln < LANES - sh, cur, prev), sh, axis=1)

        def att_group(blk, c, hg, anchor, win):
            tile = blk * NT + c
            base = hg * 8 * DP
            if isinstance(hg, int):
                cur, prev, o_t = qkv_s.at[1 + tile], qkv_s.at[tile], o_s.at[c]
                obase = hg * 8 * DH
            else:
                n = 2 * RP + 8 * DP
                base = pl.multiple_of(base, 8)
                cur = qkv_s.at[1 + tile, pl.ds(base, n)]
                prev = qkv_s.at[tile, pl.ds(base, n)]
                o_t = o_s.at[c, pl.ds(pl.multiple_of(hg * 8 * DH, 8), 8 * DH)]
                base, obase = 0, 0
            ln = lane + _zero_like_dep(anchor).astype(jnp.int32)
            logits = [None] * W
            done = []
            for dd in range(DP):
                q = cur[pl.ds(base + dd, 8, stride=DP), :]
                kc = cur[pl.ds(RP + base + dd, 8, stride=DP), :]
                if dd >= win:
                    kc = kc | _zero_like_dep(done[dd - win])
                kp = prev[pl.ds(RP + base + dd, 8, stride=DP), :]
                q0, q1 = _lo(q), _hi(q)
                for w in range(W):
                    ks = shifted(ln, kc, kp, w)
                    t = q0 * _lo(ks) + q1 * _hi(ks)
                    logits[w] = t if logits[w] is None else logits[w] + t
                done.append(ks)
            logits = [l * scale for l in logits]
            if not (isinstance(c, int) and c > 0):
                pos = lane + tile * LANES
                logits = [l if w == 0 else jnp.where(pos >= DIL * w, l, -1e9)
                          for w, l in enumerate(logits)]
            m = functools.reduce(jnp.maximum, logits)
            ln = lane + _zero_like_dep(m).astype(jnp.int32)
            e = [jnp.exp(l - m) for l in logits]
            r = 1.0 / functools.reduce(lambda a, b: a + b, e)
            p = [x * r for x in e]
            done = []
            for dd in range(DP):
                vc = cur[pl.ds(2 * RP + base + dd, 8, stride=DP), :]
                if dd >= win:
                    vc = vc | _zero_like_dep(done[dd - win])
                vp = prev[pl.ds(2 * RP + base + dd, 8, stride=DP), :]
                o0 = o1 = None
                for w in range(W):
                    vs = shifted(ln, vc, vp, w)
                    t0, t1 = p[w] * _lo(vs), p[w] * _hi(vs)
                    o0 = t0 if o0 is None else o0 + t0
                    o1 = t1 if o1 is None else o1 + t1
                done.append(vs)
                o_t[pl.ds(obase + 2 * dd, 8, stride=DH), :] = o0
                o_t[pl.ds(obase + 2 * dd + 1, 8, stride=DH), :] = o1

        def attention(blk, anchors, win):
            for c in range(NT):
                for hg in range(NG):
                    att_group(blk, c, hg, anchors[c * NG + hg], win)

        def wo_mm(blk, anchors):
            o = jnp.concatenate([o_s[c] for c in range(NT)], axis=1).astype(BF16)
            ys = [_dot(_upk(wot_s[:D2 // 2, :]), o), _dot(_upk(wot_s[D2 // 2:, :]), o)]
            for y in ys:
                anchors.append(y[:8, :LANES])
                anchors.append(y[D2 - 8:, TM - LANES:])
            xm = xio_s[blk].astype(F32) + jnp.concatenate(ys, axis=0)
            xmid_s[blk] = xm
            return _ln_stats((xm[r:r + 8] for r in range(0, D, 8)), D)

        def ffn_lhs(blk, stats, anchors):
            m, rs = stats

            def x(half, k, anchor=None):
                t = slice(half * TH, (half + 1) * TH)
                return (_tie(xmid_s[blk, k, t], anchor) - m[:, t]) * rs[:, t]

            def put(i, parts):
                v = parts[0] if len(parts) == 1 else jnp.concatenate(parts, axis=0)
                a_s[blk, :, LO[i]:LO[i] + LW[i]] = _pk(v.astype(BF16).T)

            an = list(anchors) + [None] * 4
            c11, c12, c21, c22 = x(0, KC, an[0]), x(0, KD), x(1, KC), x(1, KD)
            e1, e2 = x(0, KE), x(1, KE)
            put(5, [c11 + c22])
            put(7, [c12 - c22, e1])
            put(8, [c21 - c11, e2])
            a11, a22 = x(0, KA, an[1]), x(1, KB)
            put(2, [a11, c22])
            put(3, [a22, c11])
            put(4, [a11 + a22])
            a12 = x(0, KB, an[2])
            put(1, [a11 + a12, -(c11 + c12)])
            put(6, [a12 - a22, e1])
            a21 = x(1, KA, an[3])
            put(0, [a21 + a22, -(c21 + c22)])
            put(9, [a21 - a11, e2])

        def prep_gu(w_v, s_s, lo, anchors):
            PR = 16
            rows = range(0, KS, PR)
            for n, r in enumerate(rows):
                anchor = anchors[n * len(anchors) // len(rows)]
                blk = lambda r0, c0: w_v[r0:r0 + PR, cols(c0, PW)].astype(F32)
                if r < 3 * KU:
                    r1, r2 = KA.start + r, KB.start + r
                else:
                    r1, r2 = KC.start + r - 3 * KU, KD.start + r - 3 * KU
                b11, b12 = _tie(blk(r1, lo), anchor), blk(r1, FH + lo)
                b21, b22 = blk(r2, lo), blk(r2, FH + lo)
                if r < 3 * KU:
                    ops = [b12 - b22, b21 - b11, b11 + b22, b21 + b22, b11 + b12]
                else:
                    ops = [b22 - b12, b11 - b21, b12 + b21, b21 + b22, b11 + b12]
                for j in range(5):
                    s_s.at[j][r // 2:(r + PR) // 2, cols(lo, PW)] = _pk(ops[j])

        def prep(w_v, s_s, half, ops_fn, keep, lo, anchors):
            PR = 16
            rows = range(0, half, PR)
            for n, r in enumerate(rows):
                anchor = anchors[n * len(anchors) // len(rows)]
                blk = lambda r0, c0: w_v[r0:r0 + PR, cols(c0, PW)].astype(F32)
                ops = ops_fn(_tie(blk(r, lo), anchor), blk(r, FH + lo),
                             blk(half + r, lo), blk(half + r, FH + lo))
                for j, i in enumerate(keep):
                    s_s.at[j][r // 2:(r + PR) // 2, cols(lo, PW)] = _pk(ops[i])

        def load_lhs(blk):
            return [_upk(a_s[blk, :, LO[i]:LO[i] + LW[i]]) for i in range(10)]

        def spread(y, anchors):
            for j in range(y.shape[1] // LANES):
                anchors.append(y[:8, j * LANES:(j + 1) * LANES])
            return y

        def proj_raw(lhs, w_v, lo, n, anchors):
            f1, f2 = cols(lo, n), cols(FH + lo, n)
            cat = lambda u, v: jnp.concatenate([u, v], axis=0)
            p2 = spread(_dot(lhs[0], cat(w_v[KA, f1], w_v[KC, f2])), anchors)
            p5 = spread(_dot(lhs[1], cat(w_v[KB, f2], w_v[KD, f1])), anchors)
            return [p2, p5]

        def proj_sum(lhs, raw, w_v, s_s, lo, n, anchors):
            f1, f2 = cols(lo, n), cols(FH + lo, n)
            cat = lambda u, v: jnp.concatenate([u, v], axis=0)
            h = 3 * KU // 2
            top = lambda j: _upk(s_s[j, :h, f1])
            bot = lambda j: _upk(s_s[j, h:, f1])
            rhs = [_upk(s_s[0, :, f1]), _upk(s_s[1, :, f1]), top(2), bot(2),
                   cat(top(3), w_v[KE, f1]), cat(bot(3), w_v[KE, f2]),
                   cat(bot(4), w_v[KE, f1]), cat(top(4), w_v[KE, f2])]
            r = raw + [spread(_dot(lhs[2 + i], rhs[i]), anchors) for i in range(8)]
            return _c17(r)

        def act(g, u):
            h = [_gelu_mul(a, b) for a, b in zip(g, u)]
            return [b.astype(BF16) for b in _b_ops(h[0], h[2], h[1], h[3])]

        def gu_act(lhs, lo, n, anchors):
            g = proj_sum(lhs, proj_raw(lhs, wg_v, lo, n, anchors), wg_v, gs_s, lo, n, anchors)
            u = proj_sum(lhs, proj_raw(lhs, wu_v, lo, n, anchors), wu_v, us_s, lo, n, anchors)
            return act(g, u)

        def gu_act_prep(lhs, lo, anchors):
            an_r, an_g = [], []
            raw_g = proj_raw(lhs, wg_v, lo, PW, an_r)
            raw_u = proj_raw(lhs, wu_v, lo, PW, an_r)
            prep_gu(wg_v, gs_s, lo, an_r[:4])
            g = proj_sum(lhs, raw_g, wg_v, gs_s, lo, PW, an_g)
            prep_gu(wu_v, us_s, lo, an_r[4:] + an_g[:8])
            anchors.extend(an_g[8:])
            u = proj_sum(lhs, raw_u, wu_v, us_s, lo, PW, anchors)
            return act(g, u)

        def down_mm(acc, b, lo, n, anchors):
            p = [None] * 7
            p[2] = _dot_nt(wdt_v[:D2, cols(lo, n)], b[2])
            p[3] = _dot_nt(wdt_v[D2:, cols(FH + lo, n)], b[3])
            for j, i in enumerate(_A_SUMS):
                p[i] = _dot_nt(_upk(ds_s[j, :, cols(lo, n)]), b[i])
            p = p if acc is None else [x + y for x, y in zip(acc, p)]
            anchors.extend(p[i][:8] for i in (2, 3) + _A_SUMS)
            return p

        def finish(blk, acc):
            c11, c12, c21, c22 = _combine(acc)
            y = jnp.concatenate([jnp.concatenate([c11, c12], axis=1),
                                 jnp.concatenate([c21, c22], axis=1)], axis=0)
            xio_s[blk] = (xmid_s[blk] + y).astype(BF16)

        def load_acc():
            return [acc_s[i] for i in range(7)]

        def store_acc(acc):
            for i in range(7):
                acc_s[i] = acc[i]

        order = [x_cp[0], wq_cp[0], wq_cp[1], x_cp[1], wq_cp[2], wo_cp] + gu_cp(0)
        for p in range(1, NP):
            order += gu_cp(p) + d_cp(p - 1)
        order += d_cp(NP - 1) + x_cp[2:]
        for cp in order:
            cp.start()
        qkv_s[0] = jnp.zeros(qkv_s.shape[1:], U32)
        acc_s[...] = jnp.zeros(acc_s.shape, F32)
        wait('WX0', [x_cp[0]])
        xn0 = ln1(0, None)
        done = 0
        for i in range(3):
            wait('WQ%d' % i, [wq_cp[i]] + ([x_cp[1]] if i == 2 else []))
            wqkvt_s[WQ[i] // 2:WQ[i + 1] // 2, :] = _pk(wqkv_v[:, WQ[i]:WQ[i + 1]].T)
            anchors = []
            qkv_mm(0, xn0, range(done, WQ[i + 1] // QR), anchors)
            done = WQ[i + 1] // QR
        xn1 = ln1(1, anchors[0])
        an1 = [anchors[-1]]
        qkv_mm(1, xn1, range(4), an1)
        attention(0, [an1[i] for i in cfg['att0']], cfg['win0'])
        wait('WO', [wo_cp] + gu_cp(0))
        wot_s[...] = _pk(wo_v[...].T)
        stats = wo_mm(0, [])
        qkv_mm(1, xn1, [4], [])
        ffn_lhs(0, stats, [])
        b = gu_act_prep(load_lhs(0), 0, [])
        qkv_mm(1, xn1, [5], [])
        for i in range(7):
            b_s[i * TH // 2:(i + 1) * TH // 2, :] = _pk(b[i])

        def piece(p, carry):
            wait('WP', gu_cp(p) + d_cp(p - 1))
            lhs = load_lhs(0)
            b_prev = [_upk(b_s[i * TH // 2:(i + 1) * TH // 2, :]) for i in range(7)]
            an = []
            b = gu_act_prep(lhs, p * PW, an)
            prep(wdt_v, ds_s, D2, _a_ops, _A_SUMS, (p - 1) * PW, an[:len(an) * 3 // 4])
            g = p - 1
            att_group(1, g // NG, lax.rem(g, NG), an[0], cfg['winp'])
            store_acc(down_mm(load_acc(), b_prev, (p - 1) * PW, PW, []))
            for i in range(7):
                b_s[i * TH // 2:(i + 1) * TH // 2, :] = _pk(b[i])
            return carry

        lax.fori_loop(1, NP, piece, 0)

        wait('WD', d_cp(NP - 1) + x_cp[2:])
        an = []
        stats = wo_mm(1, an)
        prep(wdt_v, ds_s, D2, _a_ops, _A_SUMS, (NP - 1) * PW, an[:2])
        acc = down_mm(load_acc(), [_upk(b_s[i * TH // 2:(i + 1) * TH // 2, :]) for i in range(7)], (NP - 1) * PW, PW, [])
        ffn_lhs(1, stats, [])
        finish(0, acc)

        def body(u, carry):
            bu = lax.rem(u, NB)
            ba = lax.rem(u + 1, NB)
            lhs = load_lhs(bu)
            an = []
            b0 = gu_act(lhs, 0, CW, an)
            xn = ln1(ba, pick(an, [cfg['ln1']])[0])
            qkv_mm(ba, xn, range(NQ), [])
            if cfg['order'] == 0:
                an = []
                b1 = gu_act(lhs, CW, CW, an)
                attention(ba, pick(an, cfg['att']), cfg['win'])
                acc = down_mm(None, b0, 0, CW, [])
                stats = wo_mm(ba, [])
                an = []
                b2 = gu_act(lhs, 2 * CW, CW, an)
                ffn_lhs(ba, stats, pick(an, cfg['lhs']))
                acc = down_mm(acc, b1, CW, CW, [])
                acc = down_mm(acc, b2, 2 * CW, CW, [])
            else:
                b1 = gu_act(lhs, CW, CW, [])
                b2 = gu_act(lhs, 2 * CW, CW, [])
                an = []
                acc = down_mm(None, b0, 0, CW, an)
                acc = down_mm(acc, b1, CW, CW, an)
                attention(ba, [an[i] for i in cfg['attd']], cfg['win'])
                stats = wo_mm(ba, [])
                an = []
                acc = down_mm(acc, b2, 2 * CW, CW, an)
                ffn_lhs(ba, stats, [an[i] for i in cfg['lhsd']])
            finish(bu, acc)

            @pl.when(u >= NB)
            def _():
                out_copy(bu).start()
            return carry

        if scopes:
            with jax.named_scope('LOOP'):
                lax.fori_loop(1, NU - 1, body, 0)
        else:
            lax.fori_loop(1, NU - 1, body, 0)

        acc_s[...] = jnp.zeros(acc_s.shape, F32)

        def last(c, carry):
            lhs = load_lhs(NB - 1)
            acc, pend = load_acc(), None
            for j in range(CW // PW):
                lo = c * CW + j * PW
                b = gu_act(lhs, lo, PW, [])
                if pend is not None:
                    acc = down_mm(acc, *pend, PW, [])
                pend = (b, lo)
            store_acc(down_mm(acc, *pend, PW, []))
            return carry

        lax.fori_loop(0, FH // CW, last, 0)
        finish(NB - 1, load_acc())
        out_copy(NB - 1).start()
        wait('WOUT', [out_copy(b) for b in range(NB)])

    scratch = [
        pltpu.VMEM((NB, D, TM), BF16),
        pltpu.VMEM((D, 3 * D), BF16),
        pltpu.VMEM((D, D), BF16),
        pltpu.VMEM((D, F), BF16),
        pltpu.VMEM((D, F), BF16),
        pltpu.VMEM((D, F), BF16),
        pltpu.VMEM((3 * D // 2, D), U32),
        pltpu.VMEM((D // 2, D), U32),
        pltpu.VMEM((5, KS // 2, FH), U32),
        pltpu.VMEM((5, KS // 2, FH), U32),
        pltpu.VMEM((5, D2 // 2, FH), U32),
        pltpu.VMEM((NB, D, TM), F32),
        pltpu.VMEM((NB, TH // 2, LO[-1]), U32),
        pltpu.VMEM((S // LANES + 1, 3 * RP, LANES), U32),
        pltpu.VMEM((NT, D, LANES), F32),
        pltpu.VMEM((7, D2, TH), F32),
        pltpu.VMEM((7 * TH // 2, PW), U32),
        pltpu.SemaphoreType.DMA((SEM_D + 2 * NP,)),
        pltpu.SemaphoreType.DMA((NB,)),
    ]
    return kernel, scratch


_CFG = dict(order=0, win0=9, winp=9, win=9, attd=(2, 3, 5, 6, 8, 9, 10, 11), lhsd=(0, 1, 2), cw=768, scopes=False, ln1=0.3, att=tuple(0.08 * i for i in range(8)),
            lhs=(0.05, 0.12, 0.2, 0.28), att0=(0, 0, 1, 2, 3, 4, 5, 6))


def _run(A_x, A_wqkv, A_wo, B_w_gate, B_w_up, B_w_down, **kw):
    _, S, D = A_x.shape
    F = B_w_gate.shape[1]
    kernel, scratch = _make_kernel(S, D, F, 256, {**_CFG, **kw})
    hbm = pl.BlockSpec(memory_space=pl.ANY)
    out_t = pl.pallas_call(
        kernel,
        in_specs=[hbm] * 6,
        out_specs=hbm,
        out_shape=jax.ShapeDtypeStruct((D, S), A_x.dtype),
        scratch_shapes=scratch,
        compiler_params=pltpu.CompilerParams(vmem_limit_bytes=110 * 1024 * 1024),
    )(A_x[0].T, A_wqkv, A_wo, B_w_gate, B_w_up, B_w_down.T)
    return out_t.T[None]


@jax.jit
def pallas_interleave_layers__sliding_local_dilated__glu_gated_geglu__prompt_kernel(
    A_x: jax.Array,
    A_wqkv: jax.Array,
    A_wo: jax.Array,
    B_x: jax.Array,
    B_w_gate: jax.Array,
    B_w_up: jax.Array,
    B_w_down: jax.Array,
):
    del B_x
    return _run(A_x, A_wqkv, A_wo, B_w_gate, B_w_up, B_w_down)
```

```python
import functools

import jax
import jax.numpy as jnp
import jax.experimental.pallas as pl
import jax.experimental.pallas.tpu as pltpu
from jax import lax

H = 32
W = 8
DIL = 2
EPS = 1e-5
LANES = 128

F32 = jnp.float32
BF16 = jnp.bfloat16
U32 = jnp.uint32

_NT = (((1,), (1,)), ((), ()))


def _tree_sum(parts):
    while len(parts) > 1:
        nxt = [parts[i] + parts[i + 1] for i in range(0, len(parts) - 1, 2)]
        if len(parts) % 2:
            nxt.append(parts[-1])
        parts = nxt
    return parts[0]


def _ln_stats(slabs, d):
    n_acc = 4
    s1, s2, pilot = [None] * n_acc, [None] * n_acc, None
    for i, x in enumerate(slabs):
        if pilot is None:
            pilot = x[0:1, :]
        dx = x - pilot
        j = i % n_acc
        s1[j] = dx if s1[j] is None else s1[j] + dx
        s2[j] = dx * dx if s2[j] is None else s2[j] + dx * dx
    e1 = jnp.sum(_tree_sum(s1), axis=0, keepdims=True) * (1.0 / d)
    e2 = jnp.sum(_tree_sum(s2), axis=0, keepdims=True) * (1.0 / d)
    var = jnp.maximum(e2 - e1 * e1, 0.0)
    return pilot + e1, lax.rsqrt(var + EPS)


def _zero_like_dep(v):
    return (lax.bitcast_convert_type(v, U32) >> 31) >> 1


def _tie(x, anchor):
    if anchor is None:
        return x
    z = lax.bitcast_convert_type(_zero_like_dep(anchor), F32)
    z = jnp.concatenate([z] * (x.shape[1] // LANES), axis=1)
    if x.shape[0] == 8:
        return x + z
    return jnp.concatenate([x[:8] + z, x[8:]], axis=0)


def _gelu_mul(g, u):
    c0 = 0.7978845608028654
    c1 = c0 * 0.044715
    t = jnp.tanh(g * (c0 + c1 * (g * g)))
    return (g * u) * (0.5 + 0.5 * t)


def _lo(x):
    return lax.bitcast_convert_type(x << 16, F32)


def _hi(x):
    return lax.bitcast_convert_type(x & jnp.uint32(0xFFFF0000), F32)


def _pk(x):
    return pltpu.bitcast(x.astype(BF16), U32)


def _upk(x):
    return pltpu.bitcast(x, BF16)


def _dot(a, b):
    return jnp.dot(a, b, preferred_element_type=F32)


def _dot_nt(a, b):
    return lax.dot_general(a, b, _NT, preferred_element_type=F32)


def _a_ops(a11, a12, a21, a22):
    return [a11 + a22, a21 + a22, a11, a22, a11 + a12, a21 - a11, a12 - a22]


def _b_ops(b11, b12, b21, b22):
    return [b11 + b22, b11, b12 - b22, b21 - b11, b22, b11 + b12, b21 + b22]


def _combine(m):
    return (m[0] + m[3] - m[4] + m[6], m[2] + m[4], m[1] + m[3],
            m[0] - m[1] + m[2] + m[5])


def _c17(r):
    p2, p5, p3, p4, ra, rb, e11, e12, e21, e22 = r
    return (ra + p4 - p5 + e11, rb + p3 + p5 + e12,
            rb + p2 + p4 + e21, ra - p2 + p3 + e22)


_A_SUMS = (0, 1, 4, 5, 6)
_B_SUMS = (0, 2, 3, 5, 6)


def _make_kernel(S, D, F, TM, cfg):
    NB = S // TM
    NT = TM // LANES
    DH = D // H
    DP = DH // 2
    RP = D // 2
    NG = H // 8
    scale = float(DH) ** -0.5
    NU = 2 * NB
    TH = TM // 2
    FH = F // 2
    D2 = D // 2
    KU = D // 9
    KA, KB = slice(0, 3 * KU), slice(3 * KU, 6 * KU)
    KC, KD, KE = (slice(6 * KU, 7 * KU), slice(7 * KU, 8 * KU), slice(8 * KU, 9 * KU))
    KS = 4 * KU
    LW = (KS, KS, KS, KS, 3 * KU, KU, KS, 2 * KU, 2 * KU, KS)
    LO = [0]
    for w_ in LW:
        LO.append(LO[-1] + -(-w_ // LANES) * LANES)
    NQ = 6
    QR = 3 * D // NQ
    WQ = (0, 640, 1152, 3 * D)
    PW = 256
    NP = FH // PW
    CW = cfg['cw']
    scopes = cfg['scopes']
    SEM_GU = NB + 4
    SEM_D = SEM_GU + 4 * NP

    def kernel(x_hbm, wqkv_hbm, wo_hbm, wg_hbm, wu_hbm, wdt_hbm, out_hbm,
               xio_s, wqkv_v, wo_v, wg_v, wu_v, wdt_v, wt_s, wl_s,
               gs_s, us_s, ds_s, xmid_s, a_s, qkv_s, o_s, acc_s, b_s,
               sem_i, sem_o):

        def wait(name, cps):
            if scopes:
                with jax.named_scope(name):
                    for cp in cps:
                        cp.wait()
            else:
                for cp in cps:
                    cp.wait()

        def cols(lo, n):
            if not isinstance(lo, int):
                lo = pl.multiple_of(lo, LANES)
            return pl.ds(lo, n)

        def out_copy(b):
            return pltpu.make_async_copy(
                xio_s.at[b], out_hbm.at[:, cols(b * TM, TM)], sem_o.at[b])

        x_cp = [pltpu.make_async_copy(x_hbm.at[:, cols(b * TM, TM)], xio_s.at[b],
                                      sem_i.at[b]) for b in range(NB)]
        wq_cp = [pltpu.make_async_copy(wqkv_hbm.at[:, cols(a, b - a)],
                                       wqkv_v.at[:, cols(a, b - a)], sem_i.at[NB + i])
                 for i, (a, b) in enumerate(zip(WQ[:-1], WQ[1:]))]
        wo_cp = pltpu.make_async_copy(wo_hbm, wo_v, sem_i.at[NB + 3])

        def piece_cp(src, dst, p, sem0):
            return [pltpu.make_async_copy(src.at[:, cols(j * FH + p * PW, PW)],
                                          dst.at[:, cols(j * FH + p * PW, PW)],
                                          sem_i.at[sem0 + j]) for j in range(2)]

        def gu_cp(p):
            return (piece_cp(wg_hbm, wg_v, p, SEM_GU + 4 * p)
                    + piece_cp(wu_hbm, wu_v, p, SEM_GU + 4 * p + 2))

        def d_cp(p):
            return piece_cp(wdt_hbm, wdt_v, p, SEM_D + 2 * p)

        lane = lax.broadcasted_iota(jnp.int32, (8, LANES), 1)

        def pick(anchors, fracs):
            return [anchors[min(int(f * len(anchors)), len(anchors) - 1)] for f in fracs]

        def ln1(blk, anchor):
            def slabs():
                for r in range(0, D, 8):
                    x = xio_s[blk, r:r + 8, :].astype(F32)
                    yield _tie(x, anchor) if r == 0 else x
            m, rs = _ln_stats(slabs(), D)
            return (xio_s[blk].astype(F32) - m) * rs

        def qkv_mm(blk, xn, chunks, anchors):
            for r in chunks:
                rows = slice(r * QR // 2, (r + 1) * QR // 2)
                qkv = _dot(_upk(wt_s[rows, :]), xn)
                anchors.append(qkv[:8, :LANES])
                anchors.append(qkv[QR - 8:, TM - LANES:])
                pk = _pk(qkv)
                for c in range(NT):
                    qkv_s[1 + blk * NT + c, rows, :] = pk[:, c * LANES:(c + 1) * LANES]

        def prep_att(row0, anchor):
            q = D2 // 2
            src0 = row0 + (row0 // q) * q
            ld = lambda r: _upk(wt_s[pl.ds(pl.multiple_of(r, 8), 8), :]).astype(F32)
            w1, w2 = ld(src0), ld(src0 + q)
            w1 = jnp.concatenate([_tie(w1[:, :LANES], anchor), w1[:, LANES:]], axis=1)
            t = lambda w, j: w[:, j * LANES:(j + 1) * LANES]
            mix = lambda u, v: jnp.concatenate([u[:, :KU], v[:, KU:]], axis=1)
            cat = lambda u, v: jnp.concatenate([u[:, :KU], v], axis=1)
            e1, e2 = w1[:, 4 * LANES:], w2[:, 4 * LANES:]
            d2, d3 = t(w2, 2) - t(w1, 2), t(w1, 3) - t(w2, 3)
            tiles = [t(w2, 0) + t(w2, 1), t(w2, 2) + t(w2, 3),
                     t(w1, 0) + t(w1, 1), t(w1, 2) + t(w1, 3),
                     mix(t(w1, 2), t(w2, 3)), mix(t(w2, 3), t(w1, 2)),
                     t(w1, 0) + t(w2, 1), t(w1, 2) + t(w2, 3),
                     t(w1, 1) - t(w2, 1), cat(d3, e1),
                     cat(e1, d3[:, KU:]), cat(e2, d2[:, KU:]),
                     t(w2, 0) - t(w1, 0), cat(d2, e2)]
            wl_s[pl.ds(pl.multiple_of(row0, 8), 8), :] = _pk(jnp.concatenate(tiles, axis=1))

        def att_rhs(x):
            x1, x2 = x[:, :TH], x[:, TH:]
            L2, L3 = 2 * LANES, 3 * LANES
            ka = lambda v: jnp.concatenate([v[:LANES], v[L2:L2 + KU]], axis=0)
            kb = lambda v: jnp.concatenate([v[LANES:L2], v[L3:L3 + KU]], axis=0)
            kc = lambda v: v[L2 + KU:L3]
            kd = lambda v: v[L3 + KU:4 * LANES]
            ke = lambda v: v[4 * LANES:]
            cat = lambda u, v: jnp.concatenate([u, v], axis=0)
            ops = [cat(ka(x1), -kc(x2)), cat(kb(x2), -kd(x1)),
                   cat(ka(x2) - kb(x2), kd(x2) - kc(x2)),
                   cat(kb(x1) - ka(x1), kc(x1) - kd(x1)),
                   ka(x1) + kb(x2),
                   cat(jnp.zeros((KU, TH), F32), kc(x2) + kd(x1)),
                   cat(kb(x1) + kb(x2), ke(x1)), cat(ke(x2), kd(x1) + kd(x2)),
                   cat(ke(x1), kc(x1) + kc(x2)), cat(ka(x1) + ka(x2), ke(x2))]
            return [v.astype(BF16) for v in ops]

        def att_mm(sec, rhs, anchors):
            q = D2 // 2
            tl = lambda j, n: _upk(wl_s[sec * q:(sec + 1) * q, j * LANES:j * LANES + n])
            raw = lambda h, j: _upk(wt_s[(2 * sec + h) * q:(2 * sec + h + 1) * q,
                                         j * LANES:(j + 1) * LANES])
            cat = lambda u, v: jnp.concatenate([u, v], axis=1)
            lhs = [tl(0, KS), tl(2, KS), cat(raw(0, 0), tl(4, LANES)),
                   cat(raw(1, 1), tl(5, LANES)), tl(6, 3 * KU), tl(7, LANES),
                   tl(8, KS), tl(10, LANES), tl(11, LANES), tl(12, KS)]
            r = [_dot(lhs[i], rhs[i]) for i in range(10)]
            anchors.extend(v[:8] for v in r)
            c11, c12, c21, c22 = _c17(r)
            return jnp.concatenate([cat(c11, c12), cat(c21, c22)], axis=0)

        def qkv_fast(blk, xn, anchors):
            rhs = att_rhs(xn)
            for sec in range(3):
                pk = _pk(att_mm(sec, rhs, anchors))
                for c in range(NT):
                    qkv_s[1 + blk * NT + c, sec * RP:(sec + 1) * RP, :] = (
                        pk[:, c * LANES:(c + 1) * LANES])

        def shifted(ln, cur, prev, w):
            if w == 0:
                return cur
            sh = DIL * w
            return pltpu.roll(jnp.where(ln < LANES - sh, cur, prev), sh, axis=1)

        def att_group(blk, c, hg, anchor, win):
            tile = blk * NT + c
            base = hg * 8 * DP
            if isinstance(hg, int):
                cur, prev, o_t = qkv_s.at[1 + tile], qkv_s.at[tile], o_s.at[c]
                obase = hg * 8 * DH
            else:
                n = 2 * RP + 8 * DP
                base = pl.multiple_of(base, 8)
                cur = qkv_s.at[1 + tile, pl.ds(base, n)]
                prev = qkv_s.at[tile, pl.ds(base, n)]
                o_t = o_s.at[c, pl.ds(pl.multiple_of(hg * 8 * DH, 8), 8 * DH)]
                base, obase = 0, 0
            ln = lane + _zero_like_dep(anchor).astype(jnp.int32)
            logits = [None] * W
            done = []
            for dd in range(DP):
                q = cur[pl.ds(base + dd, 8, stride=DP), :]
                kc = cur[pl.ds(RP + base + dd, 8, stride=DP), :]
                if dd >= win:
                    kc = kc | _zero_like_dep(done[dd - win])
                kp = prev[pl.ds(RP + base + dd, 8, stride=DP), :]
                q0, q1 = _lo(q), _hi(q)
                for w in range(W):
                    ks = shifted(ln, kc, kp, w)
                    t = q0 * _lo(ks) + q1 * _hi(ks)
                    logits[w] = t if logits[w] is None else logits[w] + t
                done.append(ks)
            logits = [l * scale for l in logits]
            if not (isinstance(c, int) and c > 0):
                pos = lane + tile * LANES
                logits = [l if w == 0 else jnp.where(pos >= DIL * w, l, -1e9)
                          for w, l in enumerate(logits)]
            m = functools.reduce(jnp.maximum, logits)
            ln = lane + _zero_like_dep(m).astype(jnp.int32)
            e = [jnp.exp(l - m) for l in logits]
            r = 1.0 / functools.reduce(lambda a, b: a + b, e)
            p = [x * r for x in e]
            done = []
            for dd in range(DP):
                vc = cur[pl.ds(2 * RP + base + dd, 8, stride=DP), :]
                if dd >= win:
                    vc = vc | _zero_like_dep(done[dd - win])
                vp = prev[pl.ds(2 * RP + base + dd, 8, stride=DP), :]
                o0 = o1 = None
                for w in range(W):
                    vs = shifted(ln, vc, vp, w)
                    t0, t1 = p[w] * _lo(vs), p[w] * _hi(vs)
                    o0 = t0 if o0 is None else o0 + t0
                    o1 = t1 if o1 is None else o1 + t1
                done.append(vs)
                o_t[pl.ds(obase + 2 * dd, 8, stride=DH), :] = o0
                o_t[pl.ds(obase + 2 * dd + 1, 8, stride=DH), :] = o1

        def attention(blk, anchors, win):
            for c in range(NT):
                for hg in range(NG):
                    att_group(blk, c, hg, anchors[c * NG + hg], win)

        def wo_mm(blk, anchors, fast=False):
            o = jnp.concatenate([o_s[c] for c in range(NT)], axis=1)
            if fast:
                ys = [att_mm(3, att_rhs(o), anchors)]
            else:
                o = o.astype(BF16)
                q = D2 // 2
                ys = [_dot(_upk(wt_s[6 * q:7 * q, :]), o), _dot(_upk(wt_s[7 * q:, :]), o)]
                for y in ys:
                    anchors.append(y[:8, :LANES])
                    anchors.append(y[D2 - 8:, TM - LANES:])
            xm = xio_s[blk].astype(F32) + jnp.concatenate(ys, axis=0)
            xmid_s[blk] = xm
            return _ln_stats((xm[r:r + 8] for r in range(0, D, 8)), D)

        def ffn_lhs(blk, stats, anchors):
            m, rs = stats

            def x(half, k, anchor=None):
                t = slice(half * TH, (half + 1) * TH)
                return (_tie(xmid_s[blk, k, t], anchor) - m[:, t]) * rs[:, t]

            def put(i, parts):
                v = parts[0] if len(parts) == 1 else jnp.concatenate(parts, axis=0)
                a_s[blk, :, LO[i]:LO[i] + LW[i]] = _pk(v.astype(BF16).T)

            an = list(anchors) + [None] * 4
            c11, c12, c21, c22 = x(0, KC, an[0]), x(0, KD), x(1, KC), x(1, KD)
            e1, e2 = x(0, KE), x(1, KE)
            put(5, [c11 + c22])
            put(7, [c12 - c22, e1])
            put(8, [c21 - c11, e2])
            a11, a22 = x(0, KA, an[1]), x(1, KB)
            put(2, [a11, c22])
            put(3, [a22, c11])
            put(4, [a11 + a22])
            a12 = x(0, KB, an[2])
            put(1, [a11 + a12, -(c11 + c12)])
            put(6, [a12 - a22, e1])
            a21 = x(1, KA, an[3])
            put(0, [a21 + a22, -(c21 + c22)])
            put(9, [a21 - a11, e2])

        def prep_gu(w_v, s_s, lo, anchors):
            PR = 16
            rows = range(0, KS, PR)
            for n, r in enumerate(rows):
                anchor = anchors[n * len(anchors) // len(rows)]
                blk = lambda r0, c0: w_v[r0:r0 + PR, cols(c0, PW)].astype(F32)
                if r < 3 * KU:
                    r1, r2 = KA.start + r, KB.start + r
                else:
                    r1, r2 = KC.start + r - 3 * KU, KD.start + r - 3 * KU
                b11, b12 = _tie(blk(r1, lo), anchor), blk(r1, FH + lo)
                b21, b22 = blk(r2, lo), blk(r2, FH + lo)
                if r < 3 * KU:
                    ops = [b12 - b22, b21 - b11, b11 + b22, b21 + b22, b11 + b12]
                else:
                    ops = [b22 - b12, b11 - b21, b12 + b21, b21 + b22, b11 + b12]
                for j in range(5):
                    s_s.at[j][r // 2:(r + PR) // 2, cols(lo, PW)] = _pk(ops[j])

        def prep(w_v, s_s, half, ops_fn, keep, lo, anchors):
            PR = 16
            rows = range(0, half, PR)
            for n, r in enumerate(rows):
                anchor = anchors[n * len(anchors) // len(rows)]
                blk = lambda r0, c0: w_v[r0:r0 + PR, cols(c0, PW)].astype(F32)
                ops = ops_fn(_tie(blk(r, lo), anchor), blk(r, FH + lo),
                             blk(half + r, lo), blk(half + r, FH + lo))
                for j, i in enumerate(keep):
                    s_s.at[j][r // 2:(r + PR) // 2, cols(lo, PW)] = _pk(ops[i])

        def load_lhs(blk):
            return [_upk(a_s[blk, :, LO[i]:LO[i] + LW[i]]) for i in range(10)]

        def spread(y, anchors):
            for j in range(y.shape[1] // LANES):
                anchors.append(y[:8, j * LANES:(j + 1) * LANES])
            return y

        def proj_raw(lhs, w_v, lo, n, anchors):
            f1, f2 = cols(lo, n), cols(FH + lo, n)
            cat = lambda u, v: jnp.concatenate([u, v], axis=0)
            p2 = spread(_dot(lhs[0], cat(w_v[KA, f1], w_v[KC, f2])), anchors)
            p5 = spread(_dot(lhs[1], cat(w_v[KB, f2], w_v[KD, f1])), anchors)
            return [p2, p5]

        def proj_sum(lhs, raw, w_v, s_s, lo, n, anchors):
            f1, f2 = cols(lo, n), cols(FH + lo, n)
            cat = lambda u, v: jnp.concatenate([u, v], axis=0)
            h = 3 * KU // 2
            top = lambda j: _upk(s_s[j, :h, f1])
            bot = lambda j: _upk(s_s[j, h:, f1])
            rhs = [_upk(s_s[0, :, f1]), _upk(s_s[1, :, f1]), top(2), bot(2),
                   cat(top(3), w_v[KE, f1]), cat(bot(3), w_v[KE, f2]),
                   cat(bot(4), w_v[KE, f1]), cat(top(4), w_v[KE, f2])]
            r = raw + [spread(_dot(lhs[2 + i], rhs[i]), anchors) for i in range(8)]
            return _c17(r)

        def act(g, u):
            h = [_gelu_mul(a, b) for a, b in zip(g, u)]
            return [b.astype(BF16) for b in _b_ops(h[0], h[2], h[1], h[3])]

        def gu_act(lhs, lo, n, anchors):
            g = proj_sum(lhs, proj_raw(lhs, wg_v, lo, n, anchors), wg_v, gs_s, lo, n, anchors)
            u = proj_sum(lhs, proj_raw(lhs, wu_v, lo, n, anchors), wu_v, us_s, lo, n, anchors)
            return act(g, u)

        def gu_act_prep(lhs, lo, anchors):
            an_r, an_g = [], []
            raw_g = proj_raw(lhs, wg_v, lo, PW, an_r)
            raw_u = proj_raw(lhs, wu_v, lo, PW, an_r)
            prep_gu(wg_v, gs_s, lo, an_r[:4])
            g = proj_sum(lhs, raw_g, wg_v, gs_s, lo, PW, an_g)
            prep_gu(wu_v, us_s, lo, an_r[4:] + an_g[:8])
            anchors.extend(an_g[8:])
            u = proj_sum(lhs, raw_u, wu_v, us_s, lo, PW, anchors)
            return act(g, u)

        def down_mm(acc, b, lo, n, anchors):
            p = [None] * 7
            p[2] = _dot_nt(wdt_v[:D2, cols(lo, n)], b[2])
            p[3] = _dot_nt(wdt_v[D2:, cols(FH + lo, n)], b[3])
            for j, i in enumerate(_A_SUMS):
                p[i] = _dot_nt(_upk(ds_s[j, :, cols(lo, n)]), b[i])
            p = p if acc is None else [x + y for x, y in zip(acc, p)]
            anchors.extend(p[i][:8] for i in (2, 3) + _A_SUMS)
            return p

        def finish(blk, acc):
            c11, c12, c21, c22 = _combine(acc)
            y = jnp.concatenate([jnp.concatenate([c11, c12], axis=1),
                                 jnp.concatenate([c21, c22], axis=1)], axis=0)
            xio_s[blk] = (xmid_s[blk] + y).astype(BF16)

        def load_acc():
            return [acc_s[i] for i in range(7)]

        def store_acc(acc):
            for i in range(7):
                acc_s[i] = acc[i]

        order = [x_cp[0], wq_cp[0], wq_cp[1], x_cp[1], wq_cp[2], wo_cp] + gu_cp(0)
        for p in range(1, NP):
            order += gu_cp(p) + d_cp(p - 1)
        order += d_cp(NP - 1) + x_cp[2:]
        for cp in order:
            cp.start()
        qkv_s[0] = jnp.zeros(qkv_s.shape[1:], U32)
        acc_s[...] = jnp.zeros(acc_s.shape, F32)
        wait('WX0', [x_cp[0]])
        xn0 = ln1(0, None).astype(BF16)
        done = 0
        for i in range(3):
            wait('WQ%d' % i, [wq_cp[i]] + ([x_cp[1]] if i == 2 else []))
            wt_s[WQ[i] // 2:WQ[i + 1] // 2, :] = _pk(wqkv_v[:, WQ[i]:WQ[i + 1]].T)
            anchors = []
            qkv_mm(0, xn0, range(done, WQ[i + 1] // QR), anchors)
            done = WQ[i + 1] // QR
        xn1 = ln1(1, anchors[0]).astype(BF16)
        an1 = [anchors[-1]]
        qkv_mm(1, xn1, range(4), an1)
        attention(0, [an1[i] for i in cfg['att0']], cfg['win0'])
        wait('WO', [wo_cp] + gu_cp(0))
        wt_s[3 * RP:, :] = _pk(wo_v[...].T)
        stats = wo_mm(0, [])
        qkv_mm(1, xn1, [4], [])
        ffn_lhs(0, stats, [])
        b = gu_act_prep(load_lhs(0), 0, [])
        qkv_mm(1, xn1, [5], [])
        for i in range(7):
            b_s[i * TH // 2:(i + 1) * TH // 2, :] = _pk(b[i])

        def piece(p, carry):
            wait('WP', gu_cp(p) + d_cp(p - 1))
            lhs = load_lhs(0)
            b_prev = [_upk(b_s[i * TH // 2:(i + 1) * TH // 2, :]) for i in range(7)]
            an = []
            b = gu_act_prep(lhs, p * PW, an)
            prep(wdt_v, ds_s, D2, _a_ops, _A_SUMS, (p - 1) * PW, an[:len(an) * 3 // 4])
            g = p - 1
            att_group(1, g // NG, lax.rem(g, NG), an[0], cfg['winp'])
            an_d = []
            store_acc(down_mm(load_acc(), b_prev, (p - 1) * PW, PW, an_d))
            npat = D // 8 // (NP - 1)
            for i in range(npat):
                prep_att((g * npat + i) * 8, an_d[i * 5 // npat])
            for i in range(7):
                b_s[i * TH // 2:(i + 1) * TH // 2, :] = _pk(b[i])
            return carry

        lax.fori_loop(1, NP, piece, 0)

        wait('WD', d_cp(NP - 1) + x_cp[2:])
        an = []
        stats = wo_mm(1, an)
        prep(wdt_v, ds_s, D2, _a_ops, _A_SUMS, (NP - 1) * PW, an[:2])
        acc = down_mm(load_acc(), [_upk(b_s[i * TH // 2:(i + 1) * TH // 2, :]) for i in range(7)], (NP - 1) * PW, PW, [])
        ffn_lhs(1, stats, [])
        finish(0, acc)

        def body(u, carry):
            bu = lax.rem(u, NB)
            ba = lax.rem(u + 1, NB)
            lhs = load_lhs(bu)
            an = []
            b0 = gu_act(lhs, 0, CW, an)
            xn = ln1(ba, pick(an, [cfg['ln1']])[0])
            qkv_fast(ba, xn, [])
            if cfg['order'] == 0:
                an = []
                b1 = gu_act(lhs, CW, CW, an)
                attention(ba, [an[i] for i in cfg['att']], cfg['win'])
                acc = down_mm(None, b0, 0, CW, [])
                stats = wo_mm(ba, [], True)
                an = []
                b2 = gu_act(lhs, 2 * CW, CW, an)
                ffn_lhs(ba, stats, pick(an, cfg['lhs']))
                acc = down_mm(acc, b1, CW, CW, [])
                acc = down_mm(acc, b2, 2 * CW, CW, [])
            else:
                an = []
                b1 = gu_act(lhs, CW, CW, an)
                b2 = gu_act(lhs, 2 * CW, CW, an)
                attention(ba, [an[i] for i in cfg['att2']], cfg['win'])
                stats = wo_mm(ba, [], True)
                an = []
                acc = down_mm(None, b0, 0, CW, an)
                acc = down_mm(acc, b1, CW, CW, an)
                acc = down_mm(acc, b2, 2 * CW, CW, an)
                ffn_lhs(ba, stats, [an[i] for i in cfg['lhsd']])
            finish(bu, acc)

            @pl.when(u >= NB)
            def _():
                out_copy(bu).start()
            return carry

        if scopes:
            with jax.named_scope('LOOP'):
                lax.fori_loop(1, NU - 1, body, 0)
        else:
            lax.fori_loop(1, NU - 1, body, 0)

        acc_s[...] = jnp.zeros(acc_s.shape, F32)

        def last(c, carry):
            lhs = load_lhs(NB - 1)
            acc, pend = load_acc(), None
            for j in range(CW // PW):
                lo = c * CW + j * PW
                b = gu_act(lhs, lo, PW, [])
                if pend is not None:
                    acc = down_mm(acc, *pend, PW, [])
                pend = (b, lo)
            store_acc(down_mm(acc, *pend, PW, []))
            return carry

        lax.fori_loop(0, FH // CW, last, 0)
        finish(NB - 1, load_acc())
        out_copy(NB - 1).start()
        wait('WOUT', [out_copy(b) for b in range(NB)])

    scratch = [
        pltpu.VMEM((NB, D, TM), BF16),
        pltpu.VMEM((D, 3 * D), BF16),
        pltpu.VMEM((D, D), BF16),
        pltpu.VMEM((D, F), BF16),
        pltpu.VMEM((D, F), BF16),
        pltpu.VMEM((D, F), BF16),
        pltpu.VMEM((2 * D, D), U32),
        pltpu.VMEM((D, 14 * LANES), U32),
        pltpu.VMEM((5, KS // 2, FH), U32),
        pltpu.VMEM((5, KS // 2, FH), U32),
        pltpu.VMEM((5, D2 // 2, FH), U32),
        pltpu.VMEM((NB, D, TM), F32),
        pltpu.VMEM((NB, TH // 2, LO[-1]), U32),
        pltpu.VMEM((S // LANES + 1, 3 * RP, LANES), U32),
        pltpu.VMEM((NT, D, LANES), F32),
        pltpu.VMEM((7, D2, TH), F32),
        pltpu.VMEM((7 * TH // 2, PW), U32),
        pltpu.SemaphoreType.DMA((SEM_D + 2 * NP,)),
        pltpu.SemaphoreType.DMA((NB,)),
    ]
    return kernel, scratch


_CFG = dict(order=0, win0=9, winp=9, win=9, attd=(2, 3, 5, 6, 8, 9, 10, 11), lhsd=(2, 4, 6, 8), cw=768, scopes=False, ln1=0.3, att=(0, 7, 15, 22, 62, 69, 77, 84), att2=(0, 12, 66, 78, 132, 142, 186, 198),
            lhs=(0.05, 0.12, 0.2, 0.28), att0=(0, 0, 1, 2, 3, 4, 5, 6))


def _run(A_x, A_wqkv, A_wo, B_w_gate, B_w_up, B_w_down, **kw):
    _, S, D = A_x.shape
    F = B_w_gate.shape[1]
    kernel, scratch = _make_kernel(S, D, F, 256, {**_CFG, **kw})
    hbm = pl.BlockSpec(memory_space=pl.ANY)
    out_t = pl.pallas_call(
        kernel,
        in_specs=[hbm] * 6,
        out_specs=hbm,
        out_shape=jax.ShapeDtypeStruct((D, S), A_x.dtype),
        scratch_shapes=scratch,
        compiler_params=pltpu.CompilerParams(vmem_limit_bytes=110 * 1024 * 1024),
    )(A_x[0].T, A_wqkv, A_wo, B_w_gate, B_w_up, B_w_down.T)
    return out_t.T[None]


@jax.jit
def pallas_interleave_layers__sliding_local_dilated__glu_gated_geglu__prompt_kernel(
    A_x: jax.Array,
    A_wqkv: jax.Array,
    A_wo: jax.Array,
    B_x: jax.Array,
    B_w_gate: jax.Array,
    B_w_up: jax.Array,
    B_w_down: jax.Array,
):
    del B_x
    return _run(A_x, A_wqkv, A_wo, B_w_gate, B_w_up, B_w_down)
```

```python
import functools

import jax
import jax.numpy as jnp
import jax.experimental.pallas as pl
import jax.experimental.pallas.tpu as pltpu
from jax import lax

H = 32
W = 8
DIL = 2
EPS = 1e-5
LANES = 128

F32 = jnp.float32
BF16 = jnp.bfloat16
U32 = jnp.uint32

_NT = (((1,), (1,)), ((), ()))


def _tree_sum(parts):
    while len(parts) > 1:
        nxt = [parts[i] + parts[i + 1] for i in range(0, len(parts) - 1, 2)]
        if len(parts) % 2:
            nxt.append(parts[-1])
        parts = nxt
    return parts[0]


def _ln_stats(slabs, d):
    n_acc = 4
    s1, s2, pilot = [None] * n_acc, [None] * n_acc, None
    for i, x in enumerate(slabs):
        if pilot is None:
            pilot = x[0:1, :]
        dx = x - pilot
        j = i % n_acc
        s1[j] = dx if s1[j] is None else s1[j] + dx
        s2[j] = dx * dx if s2[j] is None else s2[j] + dx * dx
    e1 = jnp.sum(_tree_sum(s1), axis=0, keepdims=True) * (1.0 / d)
    e2 = jnp.sum(_tree_sum(s2), axis=0, keepdims=True) * (1.0 / d)
    var = jnp.maximum(e2 - e1 * e1, 0.0)
    return pilot + e1, lax.rsqrt(var + EPS)


def _zero_like_dep(v):
    return (lax.bitcast_convert_type(v, U32) >> 31) >> 1


def _tie(x, anchor):
    if anchor is None:
        return x
    z = lax.bitcast_convert_type(_zero_like_dep(anchor), F32)
    z = jnp.concatenate([z] * (x.shape[1] // LANES), axis=1)
    if x.shape[0] == 8:
        return x + z
    return jnp.concatenate([x[:8] + z, x[8:]], axis=0)


def _gelu_mul(g, u):
    c0 = 0.7978845608028654
    c1 = c0 * 0.044715
    t = jnp.tanh(g * (c0 + c1 * (g * g)))
    return (g * u) * (0.5 + 0.5 * t)


def _lo(x):
    return lax.bitcast_convert_type(x << 16, F32)


def _hi(x):
    return lax.bitcast_convert_type(x & jnp.uint32(0xFFFF0000), F32)


def _pk(x):
    return pltpu.bitcast(x.astype(BF16), U32)


def _upk(x):
    return pltpu.bitcast(x, BF16)


def _dot(a, b):
    return jnp.dot(a, b, preferred_element_type=F32)


def _dot_nt(a, b):
    return lax.dot_general(a, b, _NT, preferred_element_type=F32)


def _a_ops(a11, a12, a21, a22):
    return [a11 + a22, a21 + a22, a11, a22, a11 + a12, a21 - a11, a12 - a22]


def _b_ops(b11, b12, b21, b22):
    return [b11 + b22, b11, b12 - b22, b21 - b11, b22, b11 + b12, b21 + b22]


def _combine(m):
    return (m[0] + m[3] - m[4] + m[6], m[2] + m[4], m[1] + m[3],
            m[0] - m[1] + m[2] + m[5])


def _c17(r):
    p2, p5, p3, p4, ra, rb, e11, e12, e21, e22 = r
    return (ra + p4 - p5 + e11, rb + p3 + p5 + e12,
            rb + p2 + p4 + e21, ra - p2 + p3 + e22)


_A_SUMS = (0, 1, 4, 5, 6)
_B_SUMS = (0, 2, 3, 5, 6)


def _make_kernel(S, D, F, TM, cfg):
    NB = S // TM
    NT = TM // LANES
    DH = D // H
    DP = DH // 2
    RP = D // 2
    NG = H // 8
    scale = float(DH) ** -0.5
    NU = 2 * NB
    TH = TM // 2
    FH = F // 2
    D2 = D // 2
    KU = D // 9
    KA, KB = slice(0, 3 * KU), slice(3 * KU, 6 * KU)
    KC, KD, KE = (slice(6 * KU, 7 * KU), slice(7 * KU, 8 * KU), slice(8 * KU, 9 * KU))
    KS = 4 * KU
    LW = (KS, KS, KS, KS, 3 * KU, KU, KS, 2 * KU, 2 * KU, KS)
    LO = [0]
    for w_ in LW:
        LO.append(LO[-1] + -(-w_ // LANES) * LANES)
    NQ = 6
    QR = 3 * D // NQ
    WQ = (0, 640, 1152, 3 * D)
    PW = 256
    NP = FH // PW
    CW = cfg['cw']
    scopes = cfg['scopes']
    SEM_GU = NB + 4
    SEM_D = SEM_GU + 4 * NP

    def kernel(x_hbm, wqkv_hbm, wo_hbm, wg_hbm, wu_hbm, wdt_hbm, out_hbm,
               xio_s, wqkv_v, wo_v, wg_v, wu_v, wdt_v, wt_s, wl_s,
               gs_s, us_s, ds_s, xmid_s, a_s, qkv_s, o_s, acc_s, b_s, r_s,
               sem_i, sem_o):

        def wait(name, cps):
            if scopes:
                with jax.named_scope(name):
                    for cp in cps:
                        cp.wait()
            else:
                for cp in cps:
                    cp.wait()

        def cols(lo, n):
            if not isinstance(lo, int):
                lo = pl.multiple_of(lo, LANES)
            return pl.ds(lo, n)

        def out_copy(b):
            return pltpu.make_async_copy(
                xio_s.at[b], out_hbm.at[:, cols(b * TM, TM)], sem_o.at[b])

        x_cp = [pltpu.make_async_copy(x_hbm.at[:, cols(b * TM, TM)], xio_s.at[b],
                                      sem_i.at[b]) for b in range(NB)]
        wq_cp = [pltpu.make_async_copy(wqkv_hbm.at[:, cols(a, b - a)],
                                       wqkv_v.at[:, cols(a, b - a)], sem_i.at[NB + i])
                 for i, (a, b) in enumerate(zip(WQ[:-1], WQ[1:]))]
        wo_cp = pltpu.make_async_copy(wo_hbm, wo_v, sem_i.at[NB + 3])

        def piece_cp(src, dst, p, sem0):
            return [pltpu.make_async_copy(src.at[:, cols(j * FH + p * PW, PW)],
                                          dst.at[:, cols(j * FH + p * PW, PW)],
                                          sem_i.at[sem0 + j]) for j in range(2)]

        def gu_cp(p):
            return (piece_cp(wg_hbm, wg_v, p, SEM_GU + 4 * p)
                    + piece_cp(wu_hbm, wu_v, p, SEM_GU + 4 * p + 2))

        def d_cp(p):
            return piece_cp(wdt_hbm, wdt_v, p, SEM_D + 2 * p)

        lane = lax.broadcasted_iota(jnp.int32, (8, LANES), 1)

        def pick(anchors, fracs):
            return [anchors[min(int(f * len(anchors)), len(anchors) - 1)] for f in fracs]

        def ln1(blk, anchor):
            def slabs():
                for r in range(0, D, 8):
                    x = xio_s[blk, r:r + 8, :].astype(F32)
                    yield _tie(x, anchor) if r == 0 else x
            m, rs = _ln_stats(slabs(), D)
            return (xio_s[blk].astype(F32) - m) * rs

        def qkv_mm(blk, xn, chunks, anchors):
            for r in chunks:
                rows = slice(r * QR // 2, (r + 1) * QR // 2)
                qkv = _dot(_upk(wt_s[rows, :]), xn)
                anchors.append(qkv[:8, :LANES])
                anchors.append(qkv[QR - 8:, TM - LANES:])
                pk = _pk(qkv)
                for c in range(NT):
                    qkv_s[1 + blk * NT + c, rows, :] = pk[:, c * LANES:(c + 1) * LANES]

        def prep_att(row0, anchor):
            q = D2 // 2
            src0 = row0 + (row0 // q) * q
            ld = lambda r: _upk(wt_s[pl.ds(pl.multiple_of(r, 8), 8), :]).astype(F32)
            w1, w2 = ld(src0), ld(src0 + q)
            w1 = jnp.concatenate([_tie(w1[:, :LANES], anchor), w1[:, LANES:]], axis=1)
            t = lambda w, j: w[:, j * LANES:(j + 1) * LANES]
            mix = lambda u, v: jnp.concatenate([u[:, :KU], v[:, KU:]], axis=1)
            cat = lambda u, v: jnp.concatenate([u[:, :KU], v], axis=1)
            e1, e2 = w1[:, 4 * LANES:], w2[:, 4 * LANES:]
            d2, d3 = t(w2, 2) - t(w1, 2), t(w1, 3) - t(w2, 3)
            tiles = [t(w2, 0) + t(w2, 1), t(w2, 2) + t(w2, 3),
                     t(w1, 0) + t(w1, 1), t(w1, 2) + t(w1, 3),
                     mix(t(w1, 2), t(w2, 3)), mix(t(w2, 3), t(w1, 2)),
                     t(w1, 0) + t(w2, 1), t(w1, 2) + t(w2, 3),
                     t(w1, 1) - t(w2, 1), cat(d3, e1),
                     cat(e1, d3[:, KU:]), cat(e2, d2[:, KU:]),
                     t(w2, 0) - t(w1, 0), cat(d2, e2)]
            wl_s[pl.ds(pl.multiple_of(row0, 8), 8), :] = _pk(jnp.concatenate(tiles, axis=1))

        def att_rhs(x):
            x1, x2 = x[:, :TH], x[:, TH:]
            L2, L3 = 2 * LANES, 3 * LANES
            ka = lambda v: jnp.concatenate([v[:LANES], v[L2:L2 + KU]], axis=0)
            kb = lambda v: jnp.concatenate([v[LANES:L2], v[L3:L3 + KU]], axis=0)
            kc = lambda v: v[L2 + KU:L3]
            kd = lambda v: v[L3 + KU:4 * LANES]
            ke = lambda v: v[4 * LANES:]
            cat = lambda u, v: jnp.concatenate([u, v], axis=0)
            ops = [cat(ka(x1), -kc(x2)), cat(kb(x2), -kd(x1)),
                   cat(ka(x2) - kb(x2), kd(x2) - kc(x2)),
                   cat(kb(x1) - ka(x1), kc(x1) - kd(x1)),
                   ka(x1) + kb(x2),
                   cat(jnp.zeros((KU, TH), F32), kc(x2) + kd(x1)),
                   cat(kb(x1) + kb(x2), ke(x1)), cat(ke(x2), kd(x1) + kd(x2)),
                   cat(ke(x1), kc(x1) + kc(x2)), cat(ka(x1) + ka(x2), ke(x2))]
            return [v.astype(BF16) for v in ops]

        def att_mm(sec, rhs, anchors, rb=None):
            q = D2 // 2
            tl = lambda j, n: _upk(wl_s[sec * q:(sec + 1) * q, j * LANES:j * LANES + n])
            raw = lambda h, j: _upk(wt_s[(2 * sec + h) * q:(2 * sec + h + 1) * q,
                                         j * LANES:(j + 1) * LANES])
            cat = lambda u, v: jnp.concatenate([u, v], axis=1)
            lhs = [tl(0, KS), tl(2, KS), cat(raw(0, 0), tl(4, LANES)),
                   cat(raw(1, 1), tl(5, LANES)), tl(6, 3 * KU), tl(7, LANES),
                   tl(8, KS), tl(10, LANES), tl(11, LANES), tl(12, KS)]
            r = [rb if i == 5 and rb is not None else _dot(lhs[i], rhs[i])
                 for i in range(10)]
            anchors.extend(v[:8] for v in r)
            c11, c12, c21, c22 = _c17(r)
            return jnp.concatenate([cat(c11, c12), cat(c21, c22)], axis=0)

        RW = (KS, KS, KS, KS, 3 * KU, 2 * KU, KS, 2 * KU, 2 * KU, KS)
        RO = [sum(RW[:i]) // 2 for i in range(11)]

        def stash_rhs(rhs):
            for i in range(10):
                r_s[RO[i]:RO[i + 1], :] = _pk(rhs[i])
            return [_upk(r_s[RO[i]:RO[i + 1], :]) for i in range(10)]

        def rb_mm(rhs, cuts):
            return jnp.concatenate(
                [_dot(_upk(wl_s[a:b, 7 * LANES:8 * LANES]), rhs[5])
                 for a, b in zip(cuts[:-1], cuts[1:])], axis=0)

        def qkv_fast(blk, rhs, anchors):
            rb = rb_mm(rhs, (0, 112, 224, 328, 432))
            for sec in range(3):
                pk = _pk(att_mm(sec, rhs, anchors, rb[sec * D2:(sec + 1) * D2]))
                for c in range(NT):
                    qkv_s[1 + blk * NT + c, sec * RP:(sec + 1) * RP, :] = (
                        pk[:, c * LANES:(c + 1) * LANES])

        def shifted(ln, cur, prev, w):
            if w == 0:
                return cur
            sh = DIL * w
            return pltpu.roll(jnp.where(ln < LANES - sh, cur, prev), sh, axis=1)

        def att_group(blk, c, hg, anchor, win):
            tile = blk * NT + c
            base = hg * 8 * DP
            if isinstance(hg, int):
                cur, prev, o_t = qkv_s.at[1 + tile], qkv_s.at[tile], o_s.at[c]
                obase = hg * 8 * DH
            else:
                n = 2 * RP + 8 * DP
                base = pl.multiple_of(base, 8)
                cur = qkv_s.at[1 + tile, pl.ds(base, n)]
                prev = qkv_s.at[tile, pl.ds(base, n)]
                o_t = o_s.at[c, pl.ds(pl.multiple_of(hg * 8 * DH, 8), 8 * DH)]
                base, obase = 0, 0
            ln = lane + _zero_like_dep(anchor).astype(jnp.int32)
            logits = [None] * W
            done = []
            for dd in range(DP):
                q = cur[pl.ds(base + dd, 8, stride=DP), :]
                kc = cur[pl.ds(RP + base + dd, 8, stride=DP), :]
                if dd >= win:
                    kc = kc | _zero_like_dep(done[dd - win])
                kp = prev[pl.ds(RP + base + dd, 8, stride=DP), :]
                q0, q1 = _lo(q), _hi(q)
                for w in range(W):
                    ks = shifted(ln, kc, kp, w)
                    t = q0 * _lo(ks) + q1 * _hi(ks)
                    logits[w] = t if logits[w] is None else logits[w] + t
                done.append(ks)
            logits = [l * scale for l in logits]
            if not (isinstance(c, int) and c > 0):
                pos = lane + tile * LANES
                logits = [l if w == 0 else jnp.where(pos >= DIL * w, l, -1e9)
                          for w, l in enumerate(logits)]
            m = functools.reduce(jnp.maximum, logits)
            ln = lane + _zero_like_dep(m).astype(jnp.int32)
            e = [jnp.exp(l - m) for l in logits]
            r = 1.0 / functools.reduce(lambda a, b: a + b, e)
            p = [x * r for x in e]
            done = []
            for dd in range(DP):
                vc = cur[pl.ds(2 * RP + base + dd, 8, stride=DP), :]
                if dd >= win:
                    vc = vc | _zero_like_dep(done[dd - win])
                vp = prev[pl.ds(2 * RP + base + dd, 8, stride=DP), :]
                o0 = o1 = None
                for w in range(W):
                    vs = shifted(ln, vc, vp, w)
                    t0, t1 = p[w] * _lo(vs), p[w] * _hi(vs)
                    o0 = t0 if o0 is None else o0 + t0
                    o1 = t1 if o1 is None else o1 + t1
                done.append(vs)
                o_t[pl.ds(obase + 2 * dd, 8, stride=DH), :] = o0
                o_t[pl.ds(obase + 2 * dd + 1, 8, stride=DH), :] = o1

        def attention(blk, anchors, win):
            for c in range(NT):
                for hg in range(NG):
                    att_group(blk, c, hg, anchors[c * NG + hg], win)

        def wo_mm(blk, anchors, fast=False):
            o = jnp.concatenate([o_s[c] for c in range(NT)], axis=1)
            if fast:
                rhs = att_rhs(o)
                ys = [att_mm(3, rhs, anchors, rb_mm(rhs, (432, 464, 496, 536, 576)))]
            else:
                o = o.astype(BF16)
                q = D2 // 2
                ys = [_dot(_upk(wt_s[6 * q:7 * q, :]), o), _dot(_upk(wt_s[7 * q:, :]), o)]
                for y in ys:
                    anchors.append(y[:8, :LANES])
                    anchors.append(y[D2 - 8:, TM - LANES:])
            xm = xio_s[blk].astype(F32) + jnp.concatenate(ys, axis=0)
            xmid_s[blk] = xm
            return _ln_stats((xm[r:r + 8] for r in range(0, D, 8)), D)

        def ffn_lhs(blk, stats, anchors):
            m, rs = stats

            def x(half, k, anchor=None):
                t = slice(half * TH, (half + 1) * TH)
                return (_tie(xmid_s[blk, k, t], anchor) - m[:, t]) * rs[:, t]

            def put(i, parts):
                v = parts[0] if len(parts) == 1 else jnp.concatenate(parts, axis=0)
                a_s[blk, :, LO[i]:LO[i] + LW[i]] = _pk(v.astype(BF16).T)

            an = list(anchors) + [None] * 4
            c11, c12, c21, c22 = x(0, KC, an[0]), x(0, KD), x(1, KC), x(1, KD)
            e1, e2 = x(0, KE), x(1, KE)
            put(5, [c11 + c22])
            put(7, [c12 - c22, e1])
            put(8, [c21 - c11, e2])
            a11, a22 = x(0, KA, an[1]), x(1, KB)
            put(2, [a11, c22])
            put(3, [a22, c11])
            put(4, [a11 + a22])
            a12 = x(0, KB, an[2])
            put(1, [a11 + a12, -(c11 + c12)])
            put(6, [a12 - a22, e1])
            a21 = x(1, KA, an[3])
            put(0, [a21 + a22, -(c21 + c22)])
            put(9, [a21 - a11, e2])

        def prep_gu(w_v, s_s, lo, anchors):
            PR = 16
            rows = range(0, KS, PR)
            for n, r in enumerate(rows):
                anchor = anchors[n * len(anchors) // len(rows)]
                blk = lambda r0, c0: w_v[r0:r0 + PR, cols(c0, PW)].astype(F32)
                if r < 3 * KU:
                    r1, r2 = KA.start + r, KB.start + r
                else:
                    r1, r2 = KC.start + r - 3 * KU, KD.start + r - 3 * KU
                b11, b12 = _tie(blk(r1, lo), anchor), blk(r1, FH + lo)
                b21, b22 = blk(r2, lo), blk(r2, FH + lo)
                if r < 3 * KU:
                    ops = [b12 - b22, b21 - b11, b11 + b22, b21 + b22, b11 + b12]
                else:
                    ops = [b22 - b12, b11 - b21, b12 + b21, b21 + b22, b11 + b12]
                for j in range(5):
                    s_s.at[j][r // 2:(r + PR) // 2, cols(lo, PW)] = _pk(ops[j])

        def prep(w_v, s_s, half, ops_fn, keep, lo, anchors):
            PR = 16
            rows = range(0, half, PR)
            for n, r in enumerate(rows):
                anchor = anchors[n * len(anchors) // len(rows)]
                blk = lambda r0, c0: w_v[r0:r0 + PR, cols(c0, PW)].astype(F32)
                ops = ops_fn(_tie(blk(r, lo), anchor), blk(r, FH + lo),
                             blk(half + r, lo), blk(half + r, FH + lo))
                for j, i in enumerate(keep):
                    s_s.at[j][r // 2:(r + PR) // 2, cols(lo, PW)] = _pk(ops[i])

        def load_lhs(blk):
            return [_upk(a_s[blk, :, LO[i]:LO[i] + LW[i]]) for i in range(10)]

        def spread(y, anchors):
            for j in range(y.shape[1] // LANES):
                anchors.append(y[:8, j * LANES:(j + 1) * LANES])
            return y

        def proj_raw(lhs, w_v, lo, n, anchors):
            f1, f2 = cols(lo, n), cols(FH + lo, n)
            cat = lambda u, v: jnp.concatenate([u, v], axis=0)
            p2 = spread(_dot(lhs[0], cat(w_v[KA, f1], w_v[KC, f2])), anchors)
            p5 = spread(_dot(lhs[1], cat(w_v[KB, f2], w_v[KD, f1])), anchors)
            return [p2, p5]

        def proj_sum(lhs, raw, w_v, s_s, lo, n, anchors):
            f1, f2 = cols(lo, n), cols(FH + lo, n)
            cat = lambda u, v: jnp.concatenate([u, v], axis=0)
            h = 3 * KU // 2
            top = lambda j: _upk(s_s[j, :h, f1])
            bot = lambda j: _upk(s_s[j, h:, f1])
            rhs = [_upk(s_s[0, :, f1]), _upk(s_s[1, :, f1]), top(2), bot(2),
                   cat(top(3), w_v[KE, f1]), cat(bot(3), w_v[KE, f2]),
                   cat(bot(4), w_v[KE, f1]), cat(top(4), w_v[KE, f2])]
            r = raw + [spread(_dot(lhs[2 + i], rhs[i]), anchors) for i in range(8)]
            return _c17(r)

        def act(g, u):
            h = [_gelu_mul(a, b) for a, b in zip(g, u)]
            return [b.astype(BF16) for b in _b_ops(h[0], h[2], h[1], h[3])]

        def gu_act(lhs, lo, n, anchors):
            g = proj_sum(lhs, proj_raw(lhs, wg_v, lo, n, anchors), wg_v, gs_s, lo, n, anchors)
            u = proj_sum(lhs, proj_raw(lhs, wu_v, lo, n, anchors), wu_v, us_s, lo, n, anchors)
            return act(g, u)

        def gu_act_prep(lhs, lo, anchors):
            an_r, an_g = [], []
            raw_g = proj_raw(lhs, wg_v, lo, PW, an_r)
            raw_u = proj_raw(lhs, wu_v, lo, PW, an_r)
            prep_gu(wg_v, gs_s, lo, an_r[:4])
            g = proj_sum(lhs, raw_g, wg_v, gs_s, lo, PW, an_g)
            prep_gu(wu_v, us_s, lo, an_r[4:] + an_g[:8])
            anchors.extend(an_g[8:])
            u = proj_sum(lhs, raw_u, wu_v, us_s, lo, PW, anchors)
            return act(g, u)

        def down_mm(acc, b, lo, n, anchors, even=False):
            p = [None] * 7
            p[2] = _dot_nt(wdt_v[:D2, cols(lo, n)], b[2])
            p[3] = _dot_nt(wdt_v[D2:, cols(FH + lo, n)], b[3])
            for j, i in enumerate(_A_SUMS):
                if even and j == 4:
                    m, q = n - 2 * LANES, D2 // 4
                    p[i] = jnp.concatenate(
                        [_dot_nt(_upk(ds_s[j, h * q:(h + 1) * q, cols(lo + m, 2 * LANES)]),
                                 b[i][:, m:]) for h in range(2)], axis=0)
                    if m:
                        p[i] = _dot_nt(_upk(ds_s[j, :, cols(lo, m)]), b[i][:, :m]) + p[i]
                else:
                    p[i] = _dot_nt(_upk(ds_s[j, :, cols(lo, n)]), b[i])
            p = p if acc is None else [x + y for x, y in zip(acc, p)]
            anchors.extend(p[i][:8] for i in (2, 3) + _A_SUMS)
            return p

        def finish(blk, acc):
            c11, c12, c21, c22 = _combine(acc)
            y = jnp.concatenate([jnp.concatenate([c11, c12], axis=1),
                                 jnp.concatenate([c21, c22], axis=1)], axis=0)
            xio_s[blk] = (xmid_s[blk] + y).astype(BF16)

        def load_acc():
            return [acc_s[i] for i in range(7)]

        def store_acc(acc):
            for i in range(7):
                acc_s[i] = acc[i]

        order = [x_cp[0], wq_cp[0], wq_cp[1], x_cp[1], wq_cp[2], wo_cp] + gu_cp(0)
        for p in range(1, NP):
            order += gu_cp(p) + d_cp(p - 1)
        order += d_cp(NP - 1) + x_cp[2:]
        for cp in order:
            cp.start()
        qkv_s[0] = jnp.zeros(qkv_s.shape[1:], U32)
        acc_s[...] = jnp.zeros(acc_s.shape, F32)
        wait('WX0', [x_cp[0]])
        xn0 = ln1(0, None).astype(BF16)
        done = 0
        for i in range(3):
            wait('WQ%d' % i, [wq_cp[i]] + ([x_cp[1]] if i == 2 else []))
            wt_s[WQ[i] // 2:WQ[i + 1] // 2, :] = _pk(wqkv_v[:, WQ[i]:WQ[i + 1]].T)
            anchors = []
            qkv_mm(0, xn0, range(done, WQ[i + 1] // QR), anchors)
            done = WQ[i + 1] // QR
        xn1 = ln1(1, anchors[0]).astype(BF16)
        an1 = [anchors[-1]]
        qkv_mm(1, xn1, range(4), an1)
        attention(0, [an1[i] for i in cfg['att0']], cfg['win0'])
        wait('WO', [wo_cp] + gu_cp(0))
        wt_s[3 * RP:, :] = _pk(wo_v[...].T)
        stats = wo_mm(0, [])
        qkv_mm(1, xn1, [4], [])
        ffn_lhs(0, stats, [])
        b = gu_act_prep(load_lhs(0), 0, [])
        qkv_mm(1, xn1, [5], [])
        for i in range(7):
            b_s[i * TH // 2:(i + 1) * TH // 2, :] = _pk(b[i])

        def piece(p, carry):
            wait('WP', gu_cp(p) + d_cp(p - 1))
            lhs = load_lhs(0)
            b_prev = [_upk(b_s[i * TH // 2:(i + 1) * TH // 2, :]) for i in range(7)]
            an = []
            b = gu_act_prep(lhs, p * PW, an)
            prep(wdt_v, ds_s, D2, _a_ops, _A_SUMS, (p - 1) * PW, an[:len(an) * 3 // 4])
            g = p - 1
            att_group(1, g // NG, lax.rem(g, NG), an[0], cfg['winp'])
            an_d = []
            store_acc(down_mm(load_acc(), b_prev, (p - 1) * PW, PW, an_d, True))
            npat = D // 8 // (NP - 1)
            for i in range(npat):
                prep_att((g * npat + i) * 8, an_d[i * 5 // npat])
            for i in range(7):
                b_s[i * TH // 2:(i + 1) * TH // 2, :] = _pk(b[i])
            return carry

        lax.fori_loop(1, NP, piece, 0)

        wait('WD', d_cp(NP - 1) + x_cp[2:])
        an = []
        stats = wo_mm(1, an)
        prep(wdt_v, ds_s, D2, _a_ops, _A_SUMS, (NP - 1) * PW, an[:2])
        acc = down_mm(load_acc(), [_upk(b_s[i * TH // 2:(i + 1) * TH // 2, :]) for i in range(7)], (NP - 1) * PW, PW, [], True)
        ffn_lhs(1, stats, [])
        finish(0, acc)

        def body(u, carry):
            bu = lax.rem(u, NB)
            ba = lax.rem(u + 1, NB)
            lhs = load_lhs(bu)
            an = []
            b0 = gu_act(lhs, 0, CW, an)
            xn = ln1(ba, pick(an, [cfg['ln1']])[0])
            rhs = att_rhs(xn)
            if cfg['stash']:
                rhs = stash_rhs(rhs)
            qkv_fast(ba, rhs, [])
            if cfg['order'] == 0:
                an = []
                b1 = gu_act(lhs, CW, CW, an)
                attention(ba, [an[i] for i in cfg['att']], cfg['win'])
                acc = down_mm(None, b0, 0, CW, [])
                stats = wo_mm(ba, [], True)
                an = []
                b2 = gu_act(lhs, 2 * CW, CW, an)
                ffn_lhs(ba, stats, pick(an, cfg['lhs']))
                acc = down_mm(acc, b1, CW, CW, [])
                acc = down_mm(acc, b2, 2 * CW, CW, [], True)
            else:
                an = []
                b1 = gu_act(lhs, CW, CW, an)
                b2 = gu_act(lhs, 2 * CW, CW, an)
                attention(ba, [an[i] for i in cfg['att2']], cfg['win'])
                stats = wo_mm(ba, [], True)
                an = []
                acc = down_mm(None, b0, 0, CW, an)
                acc = down_mm(acc, b1, CW, CW, an)
                acc = down_mm(acc, b2, 2 * CW, CW, an, True)
                ffn_lhs(ba, stats, [an[i] for i in cfg['lhsd']])
            finish(bu, acc)

            @pl.when(u >= NB)
            def _():
                out_copy(bu).start()
            return carry

        if scopes:
            with jax.named_scope('LOOP'):
                lax.fori_loop(1, NU - 1, body, 0)
        else:
            lax.fori_loop(1, NU - 1, body, 0)

        acc_s[...] = jnp.zeros(acc_s.shape, F32)

        def last(c, carry):
            lhs = load_lhs(NB - 1)
            acc, pend = load_acc(), None
            for j in range(CW // PW):
                lo = c * CW + j * PW
                b = gu_act(lhs, lo, PW, [])
                if pend is not None:
                    acc = down_mm(acc, *pend, PW, [])
                pend = (b, lo)
            store_acc(down_mm(acc, *pend, PW, [], True))
            return carry

        lax.fori_loop(0, FH // CW, last, 0)
        finish(NB - 1, load_acc())
        out_copy(NB - 1).start()
        wait('WOUT', [out_copy(b) for b in range(NB)])

    scratch = [
        pltpu.VMEM((NB, D, TM), BF16),
        pltpu.VMEM((D, 3 * D), BF16),
        pltpu.VMEM((D, D), BF16),
        pltpu.VMEM((D, F), BF16),
        pltpu.VMEM((D, F), BF16),
        pltpu.VMEM((D, F), BF16),
        pltpu.VMEM((2 * D, D), U32),
        pltpu.VMEM((D, 14 * LANES), U32),
        pltpu.VMEM((5, KS // 2, FH), U32),
        pltpu.VMEM((5, KS // 2, FH), U32),
        pltpu.VMEM((5, D2 // 2, FH), U32),
        pltpu.VMEM((NB, D, TM), F32),
        pltpu.VMEM((NB, TH // 2, LO[-1]), U32),
        pltpu.VMEM((S // LANES + 1, 3 * RP, LANES), U32),
        pltpu.VMEM((NT, D, LANES), F32),
        pltpu.VMEM((7, D2, TH), F32),
        pltpu.VMEM((7 * TH // 2, PW), U32),
        pltpu.VMEM((33 * D // 18, TH), U32),
        pltpu.SemaphoreType.DMA((SEM_D + 2 * NP,)),
        pltpu.SemaphoreType.DMA((NB,)),
    ]
    return kernel, scratch


_CFG = dict(order=1, stash=True, win0=9, winp=9, win=9, attd=(2, 3, 5, 6, 8, 9, 10, 11), lhsd=(2, 4, 6, 8), cw=768, scopes=False, ln1=0.3, att=(0, 7, 15, 22, 62, 69, 77, 84), att2=(0, 12, 66, 78, 132, 142, 186, 198),
            lhs=(0.05, 0.12, 0.2, 0.28), att0=(0, 0, 1, 2, 3, 4, 5, 6))


def _run(A_x, A_wqkv, A_wo, B_w_gate, B_w_up, B_w_down, **kw):
    _, S, D = A_x.shape
    F = B_w_gate.shape[1]
    kernel, scratch = _make_kernel(S, D, F, 256, {**_CFG, **kw})
    hbm = pl.BlockSpec(memory_space=pl.ANY)
    out_t = pl.pallas_call(
        kernel,
        in_specs=[hbm] * 6,
        out_specs=hbm,
        out_shape=jax.ShapeDtypeStruct((D, S), A_x.dtype),
        scratch_shapes=scratch,
        compiler_params=pltpu.CompilerParams(vmem_limit_bytes=110 * 1024 * 1024),
    )(A_x[0].T, A_wqkv, A_wo, B_w_gate, B_w_up, B_w_down.T)
    return out_t.T[None]


@jax.jit
def pallas_interleave_layers__sliding_local_dilated__glu_gated_geglu__prompt_kernel(
    A_x: jax.Array,
    A_wqkv: jax.Array,
    A_wo: jax.Array,
    B_x: jax.Array,
    B_w_gate: jax.Array,
    B_w_up: jax.Array,
    B_w_down: jax.Array,
):
    del B_x
    return _run(A_x, A_wqkv, A_wo, B_w_gate, B_w_up, B_w_down)
```

```python
import functools

import jax
import jax.numpy as jnp
import jax.experimental.pallas as pl
import jax.experimental.pallas.tpu as pltpu
from jax import lax

H = 32
W = 8
DIL = 2
EPS = 1e-5
LANES = 128

F32 = jnp.float32
BF16 = jnp.bfloat16
U32 = jnp.uint32

_NT = (((1,), (1,)), ((), ()))


def _tree_sum(parts):
    while len(parts) > 1:
        nxt = [parts[i] + parts[i + 1] for i in range(0, len(parts) - 1, 2)]
        if len(parts) % 2:
            nxt.append(parts[-1])
        parts = nxt
    return parts[0]


def _ln_stats(slabs, d, anchors=()):
    n_acc = 4
    s1, s2, pilot = [None] * n_acc, [None] * n_acc, None
    for i, x in enumerate(slabs):
        if pilot is None:
            pilot = x[0:1, :]
            pil = jnp.broadcast_to(pilot, x.shape)
            pils = [_tie(pil, a) for a in anchors] or [pil]
        dx = x - pils[i * len(pils) // (d // 8)]
        j = i % n_acc
        s1[j] = dx if s1[j] is None else s1[j] + dx
        s2[j] = dx * dx if s2[j] is None else s2[j] + dx * dx
    e1 = jnp.sum(_tree_sum(s1), axis=0, keepdims=True) * (1.0 / d)
    e2 = jnp.sum(_tree_sum(s2), axis=0, keepdims=True) * (1.0 / d)
    var = jnp.maximum(e2 - e1 * e1, 0.0)
    return pilot + e1, lax.rsqrt(var + EPS)


def _zero_like_dep(v):
    return (lax.bitcast_convert_type(v, U32) >> 31) >> 1


def _tie(x, anchor):
    if anchor is None:
        return x
    z = lax.bitcast_convert_type(_zero_like_dep(anchor), F32)
    z = jnp.concatenate([z] * (x.shape[1] // LANES), axis=1)
    if x.shape[0] == 8:
        return x + z
    return jnp.concatenate([x[:8] + z, x[8:]], axis=0)


def _gelu_mul(g, u):
    c0 = 0.7978845608028654
    c1 = c0 * 0.044715
    t = jnp.tanh(g * (c0 + c1 * (g * g)))
    return (g * u) * (0.5 + 0.5 * t)


def _lo(x):
    return lax.bitcast_convert_type(x << 16, F32)


def _hi(x):
    return lax.bitcast_convert_type(x & jnp.uint32(0xFFFF0000), F32)


def _pk(x):
    return pltpu.bitcast(x.astype(BF16), U32)


def _upk(x):
    return pltpu.bitcast(x, BF16)


def _dot(a, b):
    return jnp.dot(a, b, preferred_element_type=F32)


def _dot_nt(a, b):
    return lax.dot_general(a, b, _NT, preferred_element_type=F32)


def _a_ops(a11, a12, a21, a22):
    return [a11 + a22, a21 + a22, a11, a22, a11 + a12, a21 - a11, a12 - a22]


def _b_ops(b11, b12, b21, b22):
    return [b11 + b22, b11, b12 - b22, b21 - b11, b22, b11 + b12, b21 + b22]


def _combine(m):
    return (m[0] + m[3] - m[4] + m[6], m[2] + m[4], m[1] + m[3],
            m[0] - m[1] + m[2] + m[5])


def _c17(r):
    p2, p5, p3, p4, ra, rb, e11, e12, e21, e22 = r
    return (ra + p4 - p5 + e11, rb + p3 + p5 + e12,
            rb + p2 + p4 + e21, ra - p2 + p3 + e22)


_A_SUMS = (0, 1, 4, 5, 6)
_B_SUMS = (0, 2, 3, 5, 6)


def _make_kernel(S, D, F, TM, cfg):
    NB = S // TM
    NT = TM // LANES
    DH = D // H
    DP = DH // 2
    RP = D // 2
    NG = H // 8
    scale = float(DH) ** -0.5
    NU = 2 * NB
    TH = TM // 2
    FH = F // 2
    D2 = D // 2
    KU = D // 9
    KA, KB = slice(0, 3 * KU), slice(3 * KU, 6 * KU)
    KC, KD, KE = (slice(6 * KU, 7 * KU), slice(7 * KU, 8 * KU), slice(8 * KU, 9 * KU))
    KS = 4 * KU
    LW = (KS, KS, KS, KS, 3 * KU, KU, KS, 2 * KU, 2 * KU, KS)
    LO = [0]
    for w_ in LW:
        LO.append(LO[-1] + -(-w_ // LANES) * LANES)
    NQ = 6
    QR = 3 * D // NQ
    WQ = (0, 640, 1152, 3 * D)
    PW = 256
    NP = FH // PW
    CW = cfg['cw']
    scopes = cfg['scopes']
    SEM_GU = NB + 4
    SEM_D = SEM_GU + 4 * NP

    def kernel(x_hbm, wqkv_hbm, wo_hbm, wg_hbm, wu_hbm, wdt_hbm, out_hbm,
               xio_s, wqkv_v, wo_v, wg_v, wu_v, wdt_v, wt_s, wl_s,
               gs_s, us_s, ds_s, xmid_s, a_s, qkv_s, o_s, acc_s, b_s, r_s,
               sem_i, sem_o):

        def wait(name, cps):
            if scopes:
                with jax.named_scope(name):
                    for cp in cps:
                        cp.wait()
            else:
                for cp in cps:
                    cp.wait()

        def cols(lo, n):
            if not isinstance(lo, int):
                lo = pl.multiple_of(lo, LANES)
            return pl.ds(lo, n)

        def out_copy(b):
            return pltpu.make_async_copy(
                xio_s.at[b], out_hbm.at[:, cols(b * TM, TM)], sem_o.at[b])

        x_cp = [pltpu.make_async_copy(x_hbm.at[:, cols(b * TM, TM)], xio_s.at[b],
                                      sem_i.at[b]) for b in range(NB)]
        wq_cp = [pltpu.make_async_copy(wqkv_hbm.at[:, cols(a, b - a)],
                                       wqkv_v.at[:, cols(a, b - a)], sem_i.at[NB + i])
                 for i, (a, b) in enumerate(zip(WQ[:-1], WQ[1:]))]
        wo_cp = pltpu.make_async_copy(wo_hbm, wo_v, sem_i.at[NB + 3])

        def piece_cp(src, dst, p, sem0):
            return [pltpu.make_async_copy(src.at[:, cols(j * FH + p * PW, PW)],
                                          dst.at[:, cols(j * FH + p * PW, PW)],
                                          sem_i.at[sem0 + j]) for j in range(2)]

        def gu_cp(p):
            return (piece_cp(wg_hbm, wg_v, p, SEM_GU + 4 * p)
                    + piece_cp(wu_hbm, wu_v, p, SEM_GU + 4 * p + 2))

        def d_cp(p):
            return piece_cp(wdt_hbm, wdt_v, p, SEM_D + 2 * p)

        lane = lax.broadcasted_iota(jnp.int32, (8, LANES), 1)

        def pick(anchors, fracs):
            return [anchors[min(int(f * len(anchors)), len(anchors) - 1)] for f in fracs]

        def ln1(blk, anchors1, anchors2=()):
            slabs = (xio_s[blk, r:r + 8, :].astype(F32) for r in range(0, D, 8))
            m, rs = _ln_stats(slabs, D, anchors1)
            if not anchors2:
                return (xio_s[blk].astype(F32) - m) * rs
            m8 = jnp.broadcast_to(m, (8, TM))
            ms = [jnp.concatenate([_tie(m8, a)] * (KU // 8), axis=0) for a in anchors2]
            order = (0, 2, 1, 3, 4, 6, 5, 7, 8)
            out = [None] * 9
            for n, k in enumerate(order):
                x = xio_s[blk, k * KU:(k + 1) * KU, :].astype(F32)
                out[k] = (x - ms[n * len(ms) // 9]) * rs
            return jnp.concatenate(out, axis=0)

        def qkv_mm(blk, xn, chunks, anchors):
            for r in chunks:
                rows = slice(r * QR // 2, (r + 1) * QR // 2)
                qkv = _dot(_upk(wt_s[rows, :]), xn)
                anchors.append(qkv[:8, :LANES])
                anchors.append(qkv[QR - 8:, TM - LANES:])
                pk = _pk(qkv)
                for c in range(NT):
                    qkv_s[1 + blk * NT + c, rows, :] = pk[:, c * LANES:(c + 1) * LANES]

        def prep_att(row0, anchor):
            q = D2 // 2
            src0 = row0 + (row0 // q) * q
            ld = lambda r: _upk(wt_s[pl.ds(pl.multiple_of(r, 8), 8), :]).astype(F32)
            w1, w2 = ld(src0), ld(src0 + q)
            w1 = jnp.concatenate([_tie(w1[:, :LANES], anchor), w1[:, LANES:]], axis=1)
            t = lambda w, j: w[:, j * LANES:(j + 1) * LANES]
            mix = lambda u, v: jnp.concatenate([u[:, :KU], v[:, KU:]], axis=1)
            cat = lambda u, v: jnp.concatenate([u[:, :KU], v], axis=1)
            e1, e2 = w1[:, 4 * LANES:], w2[:, 4 * LANES:]
            d2, d3 = t(w2, 2) - t(w1, 2), t(w1, 3) - t(w2, 3)
            tiles = [t(w2, 0) + t(w2, 1), t(w2, 2) + t(w2, 3),
                     t(w1, 0) + t(w1, 1), t(w1, 2) + t(w1, 3),
                     mix(t(w1, 2), t(w2, 3)), mix(t(w2, 3), t(w1, 2)),
                     t(w1, 0) + t(w2, 1), t(w1, 2) + t(w2, 3),
                     t(w1, 1) - t(w2, 1), cat(d3, e1),
                     cat(e1, d3[:, KU:]), cat(e2, d2[:, KU:]),
                     t(w2, 0) - t(w1, 0), cat(d2, e2)]
            wl_s[pl.ds(pl.multiple_of(row0, 8), 8), :] = _pk(jnp.concatenate(tiles, axis=1))

        def att_rhs(x):
            x1, x2 = x[:, :TH], x[:, TH:]
            L2, L3 = 2 * LANES, 3 * LANES
            ka = lambda v: jnp.concatenate([v[:LANES], v[L2:L2 + KU]], axis=0)
            kb = lambda v: jnp.concatenate([v[LANES:L2], v[L3:L3 + KU]], axis=0)
            kc = lambda v: v[L2 + KU:L3]
            kd = lambda v: v[L3 + KU:4 * LANES]
            ke = lambda v: v[4 * LANES:]
            cat = lambda u, v: jnp.concatenate([u, v], axis=0)
            ops = [cat(ka(x1), -kc(x2)), cat(kb(x2), -kd(x1)),
                   cat(ka(x2) - kb(x2), kd(x2) - kc(x2)),
                   cat(kb(x1) - ka(x1), kc(x1) - kd(x1)),
                   ka(x1) + kb(x2),
                   cat(jnp.zeros((KU, TH), F32), kc(x2) + kd(x1)),
                   cat(kb(x1) + kb(x2), ke(x1)), cat(ke(x2), kd(x1) + kd(x2)),
                   cat(ke(x1), kc(x1) + kc(x2)), cat(ka(x1) + ka(x2), ke(x2))]
            return [v.astype(BF16) for v in ops]

        def att_mm(sec, rhs, anchors, rb=None):
            q = D2 // 2
            tl = lambda j, n: _upk(wl_s[sec * q:(sec + 1) * q, j * LANES:j * LANES + n])
            raw = lambda h, j: _upk(wt_s[(2 * sec + h) * q:(2 * sec + h + 1) * q,
                                         j * LANES:(j + 1) * LANES])
            cat = lambda u, v: jnp.concatenate([u, v], axis=1)
            lhs = [tl(0, KS), tl(2, KS), cat(raw(0, 0), tl(4, LANES)),
                   cat(raw(1, 1), tl(5, LANES)), tl(6, 3 * KU), tl(7, LANES),
                   tl(8, KS), tl(10, LANES), tl(11, LANES), tl(12, KS)]
            r = [rb if i == 5 and rb is not None else _dot(lhs[i], rhs[i])
                 for i in range(10)]
            anchors.extend(v[:8] for v in r)
            c11, c12, c21, c22 = _c17(r)
            return jnp.concatenate([cat(c11, c12), cat(c21, c22)], axis=0)

        RW = (KS, KS, KS, KS, 3 * KU, 2 * KU, KS, 2 * KU, 2 * KU, KS)
        RO = [sum(RW[:i]) // 2 for i in range(11)]

        def stash_rhs(rhs):
            for i in range(10):
                r_s[RO[i]:RO[i + 1], :] = _pk(rhs[i])
            return [_upk(r_s[RO[i]:RO[i + 1], :]) for i in range(10)]

        def rb_mm(rhs, cuts):
            return jnp.concatenate(
                [_dot(_upk(wl_s[a:b, 7 * LANES:8 * LANES]), rhs[5])
                 for a, b in zip(cuts[:-1], cuts[1:])], axis=0)

        def qkv_fast(blk, rhs, anchors):
            rb = rb_mm(rhs, (0, 112, 224, 328, 432))
            for sec in range(3):
                pk = _pk(att_mm(sec, rhs, anchors, rb[sec * D2:(sec + 1) * D2]))
                for c in range(NT):
                    qkv_s[1 + blk * NT + c, sec * RP:(sec + 1) * RP, :] = (
                        pk[:, c * LANES:(c + 1) * LANES])

        def shifted(ln, cur, prev, w):
            if w == 0:
                return cur
            sh = DIL * w
            return pltpu.roll(jnp.where(ln < LANES - sh, cur, prev), sh, axis=1)

        def att_group(blk, c, hg, anchor, win):
            tile = blk * NT + c
            base = hg * 8 * DP
            if isinstance(hg, int):
                cur, prev, o_t = qkv_s.at[1 + tile], qkv_s.at[tile], o_s.at[c]
                obase = hg * 8 * DH
            else:
                n = 2 * RP + 8 * DP
                base = pl.multiple_of(base, 8)
                cur = qkv_s.at[1 + tile, pl.ds(base, n)]
                prev = qkv_s.at[tile, pl.ds(base, n)]
                o_t = o_s.at[c, pl.ds(pl.multiple_of(hg * 8 * DH, 8), 8 * DH)]
                base, obase = 0, 0
            ln = lane + _zero_like_dep(anchor).astype(jnp.int32)
            logits = [None] * W
            done = []
            for dd in range(DP):
                q = cur[pl.ds(base + dd, 8, stride=DP), :]
                kc = cur[pl.ds(RP + base + dd, 8, stride=DP), :]
                if dd >= win:
                    kc = kc | _zero_like_dep(done[dd - win])
                kp = prev[pl.ds(RP + base + dd, 8, stride=DP), :]
                q0, q1 = _lo(q), _hi(q)
                for w in range(W):
                    ks = shifted(ln, kc, kp, w)
                    t = q0 * _lo(ks) + q1 * _hi(ks)
                    logits[w] = t if logits[w] is None else logits[w] + t
                done.append(ks)
            logits = [l * scale for l in logits]
            if not (isinstance(c, int) and c > 0):
                pos = lane + tile * LANES
                logits = [l if w == 0 else jnp.where(pos >= DIL * w, l, -1e9)
                          for w, l in enumerate(logits)]
            m = functools.reduce(jnp.maximum, logits)
            ln = lane + _zero_like_dep(m).astype(jnp.int32)
            e = [jnp.exp(l - m) for l in logits]
            r = 1.0 / functools.reduce(lambda a, b: a + b, e)
            p = [x * r for x in e]
            done = []
            for dd in range(DP):
                vc = cur[pl.ds(2 * RP + base + dd, 8, stride=DP), :]
                if dd >= win:
                    vc = vc | _zero_like_dep(done[dd - win])
                vp = prev[pl.ds(2 * RP + base + dd, 8, stride=DP), :]
                o0 = o1 = None
                for w in range(W):
                    vs = shifted(ln, vc, vp, w)
                    t0, t1 = p[w] * _lo(vs), p[w] * _hi(vs)
                    o0 = t0 if o0 is None else o0 + t0
                    o1 = t1 if o1 is None else o1 + t1
                done.append(vs)
                o_t[pl.ds(obase + 2 * dd, 8, stride=DH), :] = o0
                o_t[pl.ds(obase + 2 * dd + 1, 8, stride=DH), :] = o1

        def attention(blk, anchors, win):
            for c in range(NT):
                for hg in range(NG):
                    att_group(blk, c, hg, anchors[c * NG + hg], win)

        def wo_mm(blk, anchors, fast=False):
            o = jnp.concatenate([o_s[c] for c in range(NT)], axis=1)
            if fast:
                rhs = att_rhs(o)
                ys = [att_mm(3, rhs, anchors, rb_mm(rhs, (432, 464, 496, 536, 576)))]
            else:
                o = o.astype(BF16)
                q = D2 // 2
                ys = [_dot(_upk(wt_s[6 * q:7 * q, :]), o), _dot(_upk(wt_s[7 * q:, :]), o)]
                for y in ys:
                    anchors.append(y[:8, :LANES])
                    anchors.append(y[D2 - 8:, TM - LANES:])
            xm = xio_s[blk].astype(F32) + jnp.concatenate(ys, axis=0)
            xmid_s[blk] = xm
            return _ln_stats((xm[r:r + 8] for r in range(0, D, 8)), D)

        def ffn_lhs(blk, stats, anchors):
            m, rs = stats

            def x(half, k, anchor=None):
                t = slice(half * TH, (half + 1) * TH)
                return (_tie(xmid_s[blk, k, t], anchor) - m[:, t]) * rs[:, t]

            def put(i, parts):
                v = parts[0] if len(parts) == 1 else jnp.concatenate(parts, axis=0)
                a_s[blk, :, LO[i]:LO[i] + LW[i]] = _pk(v.astype(BF16).T)

            an = list(anchors) + [None] * 4
            c11, c12, c21, c22 = x(0, KC, an[0]), x(0, KD), x(1, KC), x(1, KD)
            e1, e2 = x(0, KE), x(1, KE)
            put(5, [c11 + c22])
            put(7, [c12 - c22, e1])
            put(8, [c21 - c11, e2])
            a11, a22 = x(0, KA, an[1]), x(1, KB)
            put(2, [a11, c22])
            put(3, [a22, c11])
            put(4, [a11 + a22])
            a12 = x(0, KB, an[2])
            put(1, [a11 + a12, -(c11 + c12)])
            put(6, [a12 - a22, e1])
            a21 = x(1, KA, an[3])
            put(0, [a21 + a22, -(c21 + c22)])
            put(9, [a21 - a11, e2])

        def prep_gu(w_v, s_s, lo, anchors):
            PR = 16
            rows = range(0, KS, PR)
            for n, r in enumerate(rows):
                anchor = anchors[n * len(anchors) // len(rows)]
                blk = lambda r0, c0: w_v[r0:r0 + PR, cols(c0, PW)].astype(F32)
                if r < 3 * KU:
                    r1, r2 = KA.start + r, KB.start + r
                else:
                    r1, r2 = KC.start + r - 3 * KU, KD.start + r - 3 * KU
                b11, b12 = _tie(blk(r1, lo), anchor), blk(r1, FH + lo)
                b21, b22 = blk(r2, lo), blk(r2, FH + lo)
                if r < 3 * KU:
                    ops = [b12 - b22, b21 - b11, b11 + b22, b21 + b22, b11 + b12]
                else:
                    ops = [b22 - b12, b11 - b21, b12 + b21, b21 + b22, b11 + b12]
                for j in range(5):
                    s_s.at[j][r // 2:(r + PR) // 2, cols(lo, PW)] = _pk(ops[j])

        def prep(w_v, s_s, half, ops_fn, keep, lo, anchors):
            PR = 16
            rows = range(0, half, PR)
            for n, r in enumerate(rows):
                anchor = anchors[n * len(anchors) // len(rows)]
                blk = lambda r0, c0: w_v[r0:r0 + PR, cols(c0, PW)].astype(F32)
                ops = ops_fn(_tie(blk(r, lo), anchor), blk(r, FH + lo),
                             blk(half + r, lo), blk(half + r, FH + lo))
                for j, i in enumerate(keep):
                    s_s.at[j][r // 2:(r + PR) // 2, cols(lo, PW)] = _pk(ops[i])

        def load_lhs(blk):
            return [_upk(a_s[blk, :, LO[i]:LO[i] + LW[i]]) for i in range(10)]

        def spread(y, anchors):
            for j in range(y.shape[1] // LANES):
                anchors.append(y[:8, j * LANES:(j + 1) * LANES])
            return y

        def proj_raw(lhs, w_v, lo, n, anchors):
            f1, f2 = cols(lo, n), cols(FH + lo, n)
            cat = lambda u, v: jnp.concatenate([u, v], axis=0)
            p2 = spread(_dot(lhs[0], cat(w_v[KA, f1], w_v[KC, f2])), anchors)
            p5 = spread(_dot(lhs[1], cat(w_v[KB, f2], w_v[KD, f1])), anchors)
            return [p2, p5]

        def proj_sum(lhs, raw, w_v, s_s, lo, n, anchors):
            f1, f2 = cols(lo, n), cols(FH + lo, n)
            cat = lambda u, v: jnp.concatenate([u, v], axis=0)
            h = 3 * KU // 2
            top = lambda j: _upk(s_s[j, :h, f1])
            bot = lambda j: _upk(s_s[j, h:, f1])
            rhs = [_upk(s_s[0, :, f1]), _upk(s_s[1, :, f1]), top(2), bot(2),
                   cat(top(3), w_v[KE, f1]), cat(bot(3), w_v[KE, f2]),
                   cat(bot(4), w_v[KE, f1]), cat(top(4), w_v[KE, f2])]
            r = raw + [spread(_dot(lhs[2 + i], rhs[i]), anchors) for i in range(8)]
            return _c17(r)

        def act(g, u):
            h = [_gelu_mul(a, b) for a, b in zip(g, u)]
            return [b.astype(BF16) for b in _b_ops(h[0], h[2], h[1], h[3])]

        def gu_act(lhs, lo, n, anchors):
            g = proj_sum(lhs, proj_raw(lhs, wg_v, lo, n, anchors), wg_v, gs_s, lo, n, anchors)
            u = proj_sum(lhs, proj_raw(lhs, wu_v, lo, n, anchors), wu_v, us_s, lo, n, anchors)
            return act(g, u)

        def gu_rhs(w_v, s_s, lo, n, i):
            f1, f2 = cols(lo, n), cols(FH + lo, n)
            cat = lambda u, v: jnp.concatenate([u, v], axis=0)
            h = 3 * KU // 2
            top = lambda j: _upk(s_s[j, :h, f1])
            bot = lambda j: _upk(s_s[j, h:, f1])
            return [lambda: cat(w_v[KA, f1], w_v[KC, f2]),
                    lambda: cat(w_v[KB, f2], w_v[KD, f1]),
                    lambda: _upk(s_s[0, :, f1]), lambda: _upk(s_s[1, :, f1]),
                    lambda: top(2), lambda: bot(2),
                    lambda: cat(top(3), w_v[KE, f1]), lambda: cat(bot(3), w_v[KE, f2]),
                    lambda: cat(bot(4), w_v[KE, f1]), lambda: cat(top(4), w_v[KE, f2])][i]()

        def gu_shared(lhs, lo, n, anchors):
            return [[spread(_dot(lhs[i], gu_rhs(w_v, s_s, lo, n, i)), anchors)
                     for i in range(6)] for w_v, s_s in ((wg_v, gs_s), (wu_v, us_s))]

        def gu_final(lhs, sh, lo, n, anchors):
            rg, ru = list(sh[0]), list(sh[1])
            for i in range(6, 10):
                rg.append(spread(_dot(lhs[i], gu_rhs(wg_v, gs_s, lo, n, i)), anchors))
                ru.append(spread(_dot(lhs[i], gu_rhs(wu_v, us_s, lo, n, i)), anchors))
            return act(_c17(rg), _c17(ru))

        def gu_act_prep(lhs, lo, anchors):
            an_r, an_g = [], []
            raw_g = proj_raw(lhs, wg_v, lo, PW, an_r)
            raw_u = proj_raw(lhs, wu_v, lo, PW, an_r)
            prep_gu(wg_v, gs_s, lo, an_r[:4])
            g = proj_sum(lhs, raw_g, wg_v, gs_s, lo, PW, an_g)
            prep_gu(wu_v, us_s, lo, an_r[4:] + an_g[:8])
            anchors.extend(an_g[8:])
            u = proj_sum(lhs, raw_u, wu_v, us_s, lo, PW, anchors)
            return act(g, u)

        def down_mm(acc, b, lo, n, anchors, even=False):
            p = [None] * 7
            p[2] = _dot_nt(wdt_v[:D2, cols(lo, n)], b[2])
            p[3] = _dot_nt(wdt_v[D2:, cols(FH + lo, n)], b[3])
            for j, i in enumerate(_A_SUMS):
                if even and j == 4:
                    m, q = n - 2 * LANES, D2 // 4
                    p[i] = jnp.concatenate(
                        [_dot_nt(_upk(ds_s[j, h * q:(h + 1) * q, cols(lo + m, 2 * LANES)]),
                                 b[i][:, m:]) for h in range(2)], axis=0)
                    if m:
                        p[i] = _dot_nt(_upk(ds_s[j, :, cols(lo, m)]), b[i][:, :m]) + p[i]
                else:
                    p[i] = _dot_nt(_upk(ds_s[j, :, cols(lo, n)]), b[i])
            p = p if acc is None else [x + y for x, y in zip(acc, p)]
            anchors.extend(p[i][:8] for i in (2, 3) + _A_SUMS)
            return p

        def finish(blk, acc):
            c11, c12, c21, c22 = _combine(acc)
            y = jnp.concatenate([jnp.concatenate([c11, c12], axis=1),
                                 jnp.concatenate([c21, c22], axis=1)], axis=0)
            xio_s[blk] = (xmid_s[blk] + y).astype(BF16)

        def load_acc():
            return [acc_s[i] for i in range(7)]

        def store_acc(acc):
            for i in range(7):
                acc_s[i] = acc[i]

        order = [x_cp[0], wq_cp[0], wq_cp[1], x_cp[1], wq_cp[2], wo_cp] + gu_cp(0)
        for p in range(1, NP):
            order += gu_cp(p) + d_cp(p - 1)
        order += d_cp(NP - 1) + x_cp[2:]
        for cp in order:
            cp.start()
        qkv_s[0] = jnp.zeros(qkv_s.shape[1:], U32)
        acc_s[...] = jnp.zeros(acc_s.shape, F32)
        wait('WX0', [x_cp[0]])
        xn0 = ln1(0, ()).astype(BF16)
        done = 0
        for i in range(3):
            wait('WQ%d' % i, [wq_cp[i]] + ([x_cp[1]] if i == 2 else []))
            wt_s[WQ[i] // 2:WQ[i + 1] // 2, :] = _pk(wqkv_v[:, WQ[i]:WQ[i + 1]].T)
            anchors = []
            qkv_mm(0, xn0, range(done, WQ[i + 1] // QR), anchors)
            done = WQ[i + 1] // QR
        xn1 = ln1(1, anchors[:1]).astype(BF16)
        an1 = [anchors[-1]]
        qkv_mm(1, xn1, range(4), an1)
        attention(0, [an1[i] for i in cfg['att0']], cfg['win0'])
        wait('WO', [wo_cp] + gu_cp(0))
        wt_s[3 * RP:, :] = _pk(wo_v[...].T)
        stats = wo_mm(0, [])
        qkv_mm(1, xn1, [4], [])
        ffn_lhs(0, stats, [])
        b = gu_act_prep(load_lhs(0), 0, [])
        qkv_mm(1, xn1, [5], [])
        for i in range(7):
            b_s[i * TH // 2:(i + 1) * TH // 2, :] = _pk(b[i])

        def piece(p, carry):
            wait('WP', gu_cp(p) + d_cp(p - 1))
            lhs = load_lhs(0)
            b_prev = [_upk(b_s[i * TH // 2:(i + 1) * TH // 2, :]) for i in range(7)]
            an = []
            b = gu_act_prep(lhs, p * PW, an)
            prep(wdt_v, ds_s, D2, _a_ops, _A_SUMS, (p - 1) * PW, an[:len(an) * 3 // 4])
            g = p - 1
            att_group(1, g // NG, lax.rem(g, NG), an[0], cfg['winp'])
            an_d = []
            store_acc(down_mm(load_acc(), b_prev, (p - 1) * PW, PW, an_d, True))
            npat = D // 8 // (NP - 1)
            for i in range(npat):
                prep_att((g * npat + i) * 8, an_d[i * 5 // npat])
            for i in range(7):
                b_s[i * TH // 2:(i + 1) * TH // 2, :] = _pk(b[i])
            return carry

        lax.fori_loop(1, NP, piece, 0)

        wait('WD', d_cp(NP - 1) + x_cp[2:])
        an = []
        stats = wo_mm(1, an)
        prep(wdt_v, ds_s, D2, _a_ops, _A_SUMS, (NP - 1) * PW, an[:2])
        acc = down_mm(load_acc(), [_upk(b_s[i * TH // 2:(i + 1) * TH // 2, :]) for i in range(7)], (NP - 1) * PW, PW, [], True)
        ffn_lhs(1, stats, [])
        finish(0, acc)

        def body(u, carry):
            bu = lax.rem(u, NB)
            ba = lax.rem(u + 1, NB)
            lhs = load_lhs(bu)
            acc, pend, stats, an = None, None, None, {}
            MW = cfg['mw']
            nm = FH // MW
            for j in range(nm):
                an[j] = []
                sh = gu_shared(lhs, j * MW, MW, an[j])
                if j == cfg['qkv_at']:
                    xn = ln1(ba, [an[ji][ii] for ji, ii in cfg['ln1']],
                             [an[ji][ii] for ji, ii in cfg['ln1b']])
                    qkv_fast(ba, att_rhs(xn), [])
                if j == cfg['wo_at']:
                    attention(ba, [an[ji][ii] for ji, ii in cfg['att']], cfg['win'])
                    stats = wo_mm(ba, [], True)
                b = gu_final(lhs, sh, j * MW, MW, an[j])
                if pend is not None:
                    acc = down_mm(acc, *pend, MW, an[j], cfg['even_all'])
                pend = (b, j * MW)
            ffn_lhs(ba, stats, [an[ji][ii] for ji, ii in cfg['lhs']])
            acc = down_mm(acc, *pend, MW, [], True)
            finish(bu, acc)

            @pl.when(u >= NB)
            def _():
                out_copy(bu).start()
            return carry

        if scopes:
            with jax.named_scope('LOOP'):
                lax.fori_loop(1, NU - 1, body, 0)
        else:
            lax.fori_loop(1, NU - 1, body, 0)

        acc_s[...] = jnp.zeros(acc_s.shape, F32)

        def last(c, carry):
            lhs = load_lhs(NB - 1)
            acc, pend = load_acc(), None
            for j in range(CW // PW):
                lo = c * CW + j * PW
                b = gu_final(lhs, gu_shared(lhs, lo, PW, []), lo, PW, [])
                if pend is not None:
                    acc = down_mm(acc, *pend, PW, [])
                pend = (b, lo)
            store_acc(down_mm(acc, *pend, PW, [], True))
            return carry

        lax.fori_loop(0, FH // CW, last, 0)
        finish(NB - 1, load_acc())
        out_copy(NB - 1).start()
        wait('WOUT', [out_copy(b) for b in range(NB)])

    scratch = [
        pltpu.VMEM((NB, D, TM), BF16),
        pltpu.VMEM((D, 3 * D), BF16),
        pltpu.VMEM((D, D), BF16),
        pltpu.VMEM((D, F), BF16),
        pltpu.VMEM((D, F), BF16),
        pltpu.VMEM((D, F), BF16),
        pltpu.VMEM((2 * D, D), U32),
        pltpu.VMEM((D, 14 * LANES), U32),
        pltpu.VMEM((5, KS // 2, FH), U32),
        pltpu.VMEM((5, KS // 2, FH), U32),
        pltpu.VMEM((5, D2 // 2, FH), U32),
        pltpu.VMEM((NB, D, TM), F32),
        pltpu.VMEM((NB, TH // 2, LO[-1]), U32),
        pltpu.VMEM((S // LANES + 1, 3 * RP, LANES), U32),
        pltpu.VMEM((NT, D, LANES), F32),
        pltpu.VMEM((7, D2, TH), F32),
        pltpu.VMEM((7 * TH // 2, PW), U32),
        pltpu.VMEM((33 * D // 18, TH), U32),
        pltpu.SemaphoreType.DMA((SEM_D + 2 * NP,)),
        pltpu.SemaphoreType.DMA((NB,)),
    ]
    return kernel, scratch


_CFG = dict(win0=9, winp=9, win=9, cw=768, mw=256, scopes=False, even_all=True,
            qkv_at=1, ln1=tuple((0, i) for i in range(2, 20, 2)),
            ln1b=tuple((1, i) for i in (4, 4, 8, 8, 12, 12, 16, 16, 18)), wo_at=6,
            att=((2, 6), (2, 42), (3, 6), (3, 42), (4, 6), (4, 42), (5, 6), (5, 42)),
            lhs=((7, 4), (7, 12), (8, 4), (8, 12)),
            att0=(0, 0, 1, 2, 3, 4, 5, 6))


def _run(A_x, A_wqkv, A_wo, B_w_gate, B_w_up, B_w_down, **kw):
    _, S, D = A_x.shape
    F = B_w_gate.shape[1]
    kernel, scratch = _make_kernel(S, D, F, 256, {**_CFG, **kw})
    hbm = pl.BlockSpec(memory_space=pl.ANY)
    out_t = pl.pallas_call(
        kernel,
        in_specs=[hbm] * 6,
        out_specs=hbm,
        out_shape=jax.ShapeDtypeStruct((D, S), A_x.dtype),
        scratch_shapes=scratch,
        compiler_params=pltpu.CompilerParams(vmem_limit_bytes=110 * 1024 * 1024),
    )(A_x[0].T, A_wqkv, A_wo, B_w_gate, B_w_up, B_w_down.T)
    return out_t.T[None]


@jax.jit
def pallas_interleave_layers__sliding_local_dilated__glu_gated_geglu__prompt_kernel(
    A_x: jax.Array,
    A_wqkv: jax.Array,
    A_wo: jax.Array,
    B_x: jax.Array,
    B_w_gate: jax.Array,
    B_w_up: jax.Array,
    B_w_down: jax.Array,
):
    del B_x
    return _run(A_x, A_wqkv, A_wo, B_w_gate, B_w_up, B_w_down)
```

```python
import functools

import jax
import jax.numpy as jnp
import jax.experimental.pallas as pl
import jax.experimental.pallas.tpu as pltpu
from jax import lax

H = 32
W = 8
DIL = 2
EPS = 1e-5
LANES = 128

F32 = jnp.float32
BF16 = jnp.bfloat16
U32 = jnp.uint32

_NT = (((1,), (1,)), ((), ()))


def _tree_sum(parts):
    while len(parts) > 1:
        nxt = [parts[i] + parts[i + 1] for i in range(0, len(parts) - 1, 2)]
        if len(parts) % 2:
            nxt.append(parts[-1])
        parts = nxt
    return parts[0]


def _ln_stats(slabs, d, anchors=()):
    n_acc = 4
    s1, s2, pilot = [None] * n_acc, [None] * n_acc, None
    for i, x in enumerate(slabs):
        if pilot is None:
            pilot = x[0:1, :]
            pil = jnp.broadcast_to(pilot, x.shape)
            pils = [_tie(pil, a) for a in anchors] or [pil]
        dx = x - pils[i * len(pils) // (d // 8)]
        j = i % n_acc
        s1[j] = dx if s1[j] is None else s1[j] + dx
        s2[j] = dx * dx if s2[j] is None else s2[j] + dx * dx
    e1 = jnp.sum(_tree_sum(s1), axis=0, keepdims=True) * (1.0 / d)
    e2 = jnp.sum(_tree_sum(s2), axis=0, keepdims=True) * (1.0 / d)
    var = jnp.maximum(e2 - e1 * e1, 0.0)
    return pilot + e1, lax.rsqrt(var + EPS)


def _zero_like_dep(v):
    return (lax.bitcast_convert_type(v, U32) >> 31) >> 1


def _tie(x, anchor):
    if anchor is None:
        return x
    z = lax.bitcast_convert_type(_zero_like_dep(anchor), F32)
    z = jnp.concatenate([z] * (x.shape[1] // LANES), axis=1)
    if x.shape[0] == 8:
        return x + z
    return jnp.concatenate([x[:8] + z, x[8:]], axis=0)


def _gelu_mul(g, u):
    c0 = 0.7978845608028654
    c1 = c0 * 0.044715
    t = jnp.tanh(g * (c0 + c1 * (g * g)))
    return (g * u) * (0.5 + 0.5 * t)


def _lo(x):
    return lax.bitcast_convert_type(x << 16, F32)


def _hi(x):
    return lax.bitcast_convert_type(x & jnp.uint32(0xFFFF0000), F32)


def _pk(x):
    return pltpu.bitcast(x.astype(BF16), U32)


def _upk(x):
    return pltpu.bitcast(x, BF16)


def _dot(a, b):
    return jnp.dot(a, b, preferred_element_type=F32)


def _dot_nt(a, b):
    return lax.dot_general(a, b, _NT, preferred_element_type=F32)


def _x_ops(x1, x2):
    d = [a - b for a, b in zip(x1, x2)]
    return [x1[0] + x2[1], x2[0] + x2[1], x1[0] + x1[1],
            d[1] + x1[2], x1[1] + x1[2], d[1] + d[2],
            d[0] - x2[2], d[0] + d[2], x2[0] + x2[2],
            x1[0], d[0], x2[1], d[1], x1[2], x2[2]]


def _x_rem(x1, x2):
    a, b, c = 0, 1, 2
    cat = lambda u, v: jnp.concatenate([u, v], axis=0)
    return [cat(x1[c], x2[b]), cat(x1[a], x1[b] - x2[b]), cat(x2[a], x2[c] - x1[c])]


def _w_sums(w):
    return [w[0][1] + w[1][0], w[1][2] + w[2][1], w[0][2] + w[2][0],
            w[0][0] + w[0][2] - w[1][0], w[2][0] - w[0][0] - w[0][1],
            w[1][1] + w[1][2] - w[0][1], w[1][0] + w[1][1] - w[2][1],
            w[2][0] + w[2][2] - w[1][2], w[2][1] + w[2][2] - w[0][2]]


_W_SUM = {0: 0, 3: 1, 6: 2, 9: 3, 10: 4, 11: 5, 12: 6, 13: 7, 14: 8}
_W_RAW = {1: (0, 1), 2: (1, 0), 4: (1, 2), 5: (2, 1), 7: (2, 0), 8: (0, 2)}
_PAIR_ORDER = (1, 2, 4, 5, 7, 8, 0, 3, 6)
_DIAG = {(0, 0): 9, (2, 0): 10, (0, 1): 11, (1, 1): 12, (1, 2): 13, (2, 2): 14}
_PAIR = {(0, 0): ((6, -1), (8, -1)), (1, 0): ((2, 1), (7, 1)), (2, 0): ((0, 1), (1, -1)),
         (0, 1): ((3, 1), (4, -1)), (1, 1): ((0, 1), (2, -1)), (2, 1): ((1, 1), (5, -1)),
         (0, 2): ((4, 1), (8, 1)), (1, 2): ((6, 1), (7, -1)), (2, 2): ((5, 1), (3, -1))}


def _column(t, base, j):
    s = []
    for k in range(3):
        v = base[k]
        for i, sg in _PAIR[k, j]:
            v = t[i] if v is None else (v + t[i] if sg > 0 else v - t[i])
        s.append(v)
    return s[1] + s[0], s[2] + s[0]


def _make_kernel(S, D, F, TM, cfg):
    NB = S // TM
    NT = TM // LANES
    DH = D // H
    DP = DH // 2
    RP = D // 2
    NG = H // 8
    scale = float(DH) ** -0.5
    NU = 2 * NB
    TH = TM // 2
    FT = F // 3
    D2 = D // 2
    D3 = D // 3
    Q3 = D3 // 2
    KU = D // 9
    KR = 3 * LANES
    NQ = 6
    QR = 3 * D // NQ
    WQ = (0, 640, 1152, 3 * D)
    PW = 256
    NP = FT // PW
    scopes = cfg['scopes']
    SEM_P = 4

    def kernel(x_hbm, wqkv_hbm, wo_hbm, wg_hbm, wu_hbm, wdt_hbm, out_hbm,
               xio_s, wqkv_v, wo_v, wg_v, wu_v, wdt_v, wt_s, wl_s,
               gs_s, us_s, ds_s, xmid_s, a_s, qkv_s, o_s, acc_s, b_s,
               sem_i, sem_o):

        def wait(name, cps):
            if scopes:
                with jax.named_scope(name):
                    for cp in cps:
                        cp.wait()
            else:
                for cp in cps:
                    cp.wait()

        def cols(lo, n):
            if not isinstance(lo, int):
                lo = pl.multiple_of(lo, LANES)
            return pl.ds(lo, n)

        def rows8(lo, n=8):
            if not isinstance(lo, int):
                lo = pl.multiple_of(lo, 8)
            return pl.ds(lo, n)

        def out_copy(b):
            return pltpu.make_async_copy(
                xio_s.at[b], out_hbm.at[:, cols(b * TM, TM)], sem_o.at[0])

        def x_cp(b, sem):
            return pltpu.make_async_copy(x_hbm.at[:, cols(b * TM, TM)], xio_s.at[b],
                                         sem_i.at[sem])

        def wq_cp(i):
            sl = cols(WQ[i], WQ[i + 1] - WQ[i])
            return pltpu.make_async_copy(wqkv_hbm.at[:, sl], wqkv_v.at[:, sl],
                                         sem_i.at[1 + i])

        def piece_cp(src, dst, p, sem):
            return [pltpu.make_async_copy(src.at[:, cols(j * FT + p * PW, PW)],
                                          dst.at[:, cols(j * FT + p * PW, PW)],
                                          sem_i.at[sem]) for j in range(3)]

        def group_cp(p):
            sem = SEM_P + p
            cps = []
            if isinstance(p, int) and p == 0:
                cps.append(pltpu.make_async_copy(wo_hbm, wo_v, sem_i.at[sem]))
            if not (isinstance(p, int) and p == NP):
                cps += piece_cp(wg_hbm, wg_v, p, sem) + piece_cp(wu_hbm, wu_v, p, sem)
            if not (isinstance(p, int) and p == 0):
                cps += piece_cp(wdt_hbm, wdt_v, p - 1, sem)
            if isinstance(p, int) and p == NP:
                cps += [x_cp(b, sem) for b in range(2, NB)]
            return cps

        lane = lax.broadcasted_iota(jnp.int32, (8, LANES), 1)
        cat0 = lambda *v: jnp.concatenate(v, axis=0)
        cat1 = lambda *v: jnp.concatenate(v, axis=1)

        def spread_over(anchors, n, total):
            return anchors[n * len(anchors) // total] if anchors else None

        def ln1(blk, anchors1, anchors2=()):
            slabs = (xio_s[blk, r:r + 8, :].astype(F32) for r in range(0, D, 8))
            m, rs = _ln_stats(slabs, D, anchors1)
            if not anchors2:
                return (xio_s[blk].astype(F32) - m) * rs
            m8 = jnp.broadcast_to(m, (8, TM))
            ms = [cat0(*[_tie(m8, a)] * (KU // 8)) for a in anchors2]
            out = [None] * 9
            for n, k in enumerate((0, 2, 4, 1, 3, 5, 6, 7, 8)):
                x = xio_s[blk, k * KU:(k + 1) * KU, :].astype(F32)
                out[k] = (x - spread_over(ms, n, 9)) * rs
            return cat0(*out)

        def put_qkv(blk, rows, y):
            pk = _pk(y)
            for c in range(NT):
                qkv_s[1 + blk * NT + c, rows, :] = pk[:, c * LANES:(c + 1) * LANES]

        def qkv_mm(blk, xn, chunks, anchors):
            for r in chunks:
                rows = slice(r * QR // 2, (r + 1) * QR // 2)
                qkv = _dot(_upk(wt_s[rows, :]), xn)
                anchors.append(qkv[:8, :LANES])
                anchors.append(qkv[QR - 8:, TM - LANES:])
                put_qkv(blk, rows, qkv)

        def split_k(x):
            hs = (x[:, :TH], x[:, TH:])
            blocks = [[h[k * LANES:(k + 1) * LANES] for k in range(3)] for h in hs]
            units = [[h[KR + k * KU:KR + (k + 1) * KU] for k in range(3)] for h in hs]
            return blocks, units

        def prep_att(row0, anchor):
            src0 = row0 + (row0 // Q3) * (2 * Q3)
            w = [_upk(wt_s[rows8(src0 + j * Q3), :]).astype(F32) for j in range(3)]
            w[0] = cat1(_tie(w[0][:, :LANES], anchor), w[0][:, LANES:])
            tiles = _w_sums([[w[j][:, k * LANES:(k + 1) * LANES] for j in range(3)]
                             for k in range(3)])
            for j in range(3):
                a, b, c = (w[j][:, KR + k * KU:KR + (k + 1) * KU] for k in range(3))
                tiles += [cat1(c, b), cat1(a, c)]
            wl_s[rows8(row0), :] = _pk(cat1(*tiles))

        def att_rhs(x):
            blocks, units = split_k(x)
            return [v.astype(BF16) for v in _x_ops(*blocks) + _x_rem(*units)]

        def att_mm(sec, rhs, anchors):
            tl = lambda i: _upk(wl_s[sec * Q3:(sec + 1) * Q3, i * LANES:(i + 1) * LANES])
            raw = lambda k, j: _upk(wt_s[(3 * sec + j) * Q3:(3 * sec + j + 1) * Q3,
                                         k * LANES:(k + 1) * LANES])
            t = {}
            for i in _PAIR_ORDER:
                t[i] = _dot(raw(*_W_RAW[i]) if i in _W_RAW else tl(_W_SUM[i]), rhs[i])
                anchors.append(t[i][:8])
            out = []
            for j in range(3):
                base = []
                for s in range(3):
                    lhs = raw(3, j) if s == 1 else tl(9 + 2 * j + s // 2)
                    r = rhs[15 + s]
                    if (s, j) in _DIAG:
                        i = _DIAG[s, j]
                        lhs, r = cat1(tl(_W_SUM[i]), lhs), cat0(rhs[i], r)
                    base.append(_dot(lhs, r))
                    anchors.append(base[-1][:8])
                out.append(cat1(*_column(t, base, j)))
            return cat0(*out)

        def qkv_fast(blk, rhs, anchors):
            for sec in range(3):
                put_qkv(blk, slice(sec * RP, (sec + 1) * RP), att_mm(sec, rhs, anchors))

        def shifted(ln, cur, prev, w):
            if w == 0:
                return cur
            sh = DIL * w
            return pltpu.roll(jnp.where(ln < LANES - sh, cur, prev), sh, axis=1)

        def att_group(blk, c, hg, anchor, win):
            tile = blk * NT + c
            base = hg * 8 * DP
            if isinstance(hg, int):
                cur, prev, o_t = qkv_s.at[1 + tile], qkv_s.at[tile], o_s.at[c]
                obase = hg * 8 * DH
            else:
                n = 2 * RP + 8 * DP
                base = pl.multiple_of(base, 8)
                cur = qkv_s.at[1 + tile, pl.ds(base, n)]
                prev = qkv_s.at[tile, pl.ds(base, n)]
                o_t = o_s.at[c, pl.ds(pl.multiple_of(hg * 8 * DH, 8), 8 * DH)]
                base, obase = 0, 0
            ln = lane + _zero_like_dep(anchor).astype(jnp.int32)
            logits = [None] * W
            done = []
            for dd in range(DP):
                q = cur[pl.ds(base + dd, 8, stride=DP), :]
                kc = cur[pl.ds(RP + base + dd, 8, stride=DP), :]
                if dd >= win:
                    kc = kc | _zero_like_dep(done[dd - win])
                kp = prev[pl.ds(RP + base + dd, 8, stride=DP), :]
                q0, q1 = _lo(q), _hi(q)
                for w in range(W):
                    ks = shifted(ln, kc, kp, w)
                    t = q0 * _lo(ks) + q1 * _hi(ks)
                    logits[w] = t if logits[w] is None else logits[w] + t
                done.append(ks)
            logits = [l * scale for l in logits]
            if not (isinstance(c, int) and c > 0):
                pos = lane + tile * LANES
                logits = [l if w == 0 else jnp.where(pos >= DIL * w, l, -1e9)
                          for w, l in enumerate(logits)]
            m = functools.reduce(jnp.maximum, logits)
            ln = lane + _zero_like_dep(m).astype(jnp.int32)
            e = [jnp.exp(l - m) for l in logits]
            r = 1.0 / functools.reduce(lambda a, b: a + b, e)
            p = [x * r for x in e]
            done = []
            for dd in range(DP):
                vc = cur[pl.ds(2 * RP + base + dd, 8, stride=DP), :]
                if dd >= win:
                    vc = vc | _zero_like_dep(done[dd - win])
                vp = prev[pl.ds(2 * RP + base + dd, 8, stride=DP), :]
                o0 = o1 = None
                for w in range(W):
                    vs = shifted(ln, vc, vp, w)
                    t0, t1 = p[w] * _lo(vs), p[w] * _hi(vs)
                    o0 = t0 if o0 is None else o0 + t0
                    o1 = t1 if o1 is None else o1 + t1
                done.append(vs)
                o_t[pl.ds(obase + 2 * dd, 8, stride=DH), :] = o0
                o_t[pl.ds(obase + 2 * dd + 1, 8, stride=DH), :] = o1

        def attention(blk, anchors, win):
            for c in range(NT):
                for hg in range(NG):
                    att_group(blk, c, hg, anchors[c * NG + hg], win)

        def wo_mm(blk, anchors, fast):
            o = cat1(*[o_s[c] for c in range(NT)])
            if fast:
                y = att_mm(3, att_rhs(o), anchors)
            else:
                o = o.astype(BF16)
                q = D2 // 2
                ys = [_dot(_upk(wt_s[6 * q:7 * q, :]), o), _dot(_upk(wt_s[7 * q:, :]), o)]
                for y in ys:
                    anchors.append(y[:8, :LANES])
                    anchors.append(y[D2 - 8:, TM - LANES:])
                y = cat0(*ys)
            xm = xio_s[blk].astype(F32) + y
            xmid_s[blk] = xm
            return _ln_stats((xm[r:r + 8] for r in range(0, D, 8)), D)

        def ffn_lhs(blk, stats, anchors):
            m, rs = stats
            m8 = jnp.broadcast_to(m, (8, TM))
            parts = []
            for n, (r0, nr) in enumerate(((0, LANES), (LANES, LANES), (2 * LANES, LANES),
                                          (KR, 3 * KU))):
                mt = cat0(*[_tie(m8, spread_over(anchors, n, 4))] * (nr // 8))
                parts.append((xmid_s[blk, r0:r0 + nr, :] - mt) * rs)
            blocks, units = split_k(cat0(*parts))
            for i, v in enumerate(_x_ops(*blocks) + _x_rem(*units)):
                a_s[blk, :, i * LANES:(i + 1) * LANES] = _pk(v.astype(BF16).T)

        def prep(w_v, s_s, nrow, blk_of, lo, anchors):
            PR = 16
            for n in range(nrow // PR):
                r = n * PR
                w = [[None] * 3 for _ in range(3)]
                for k in range(3):
                    for j in range(3):
                        rb, cb = blk_of(k, j)
                        w[k][j] = w_v[rb * nrow + r:rb * nrow + r + PR,
                                      cols(cb * FT + lo, PW)].astype(F32)
                w[0][1] = _tie(w[0][1], spread_over(anchors, n, nrow // PR))
                for i, v in enumerate(_w_sums(w)):
                    s_s.at[i][r // 2:(r + PR) // 2, cols(lo, PW)] = _pk(v)

        def prep_gu(w_v, s_s, lo, anchors):
            prep(w_v, s_s, LANES, lambda k, j: (k, j), lo, anchors)

        def prep_d(lo, anchors):
            prep(wdt_v, ds_s, D3, lambda k, j: (j, k), lo, anchors)

        def load_lhs(blk):
            return [_upk(a_s[blk, :, i * LANES:(i + 1) * LANES]) for i in range(18)]

        def spread(y, anchors):
            for j in range(y.shape[1] // LANES):
                anchors.append(y[:8, j * LANES:(j + 1) * LANES])
            return y

        GU = ((wg_v, gs_s), (wu_v, us_s))

        def gu_pair(lhs, m, lo, which, t, anchors):
            w_v, s_s = GU[m]
            for i in which:
                if i in _W_RAW:
                    k, j = _W_RAW[i]
                    r = w_v[k * LANES:(k + 1) * LANES, cols(j * FT + lo, PW)]
                else:
                    r = _upk(s_s[_W_SUM[i], :, cols(lo, PW)])
                t[i] = spread(_dot(lhs[i], r), anchors)

        def gu_base(lhs, m, lo, j, anchors):
            w_v, s_s = GU[m]
            u = lambda k, n=1: w_v[KR + k * KU:KR + (k + n) * KU, cols(j * FT + lo, PW)]
            base = []
            for s in range(3):
                l, r = lhs[15 + s], (cat0(u(2), u(1)), u(0, 2), cat0(u(0), u(2)))[s]
                if (s, j) in _DIAG:
                    i = _DIAG[s, j]
                    l, r = cat1(lhs[i], l), cat0(_upk(s_s[_W_SUM[i], :, cols(lo, PW)]), r)
                base.append(spread(_dot(l, r), anchors))
            return base

        def gu_shared(lhs, lo, anchors):
            t = ({}, {})
            for m in range(2):
                gu_pair(lhs, m, lo, _PAIR_ORDER, t[m], anchors)
            return t

        def gu_shared_prep(lhs, lo, anchors):
            t, an = ({}, {}), []
            for m in range(2):
                gu_pair(lhs, m, lo, _PAIR_ORDER[:6], t[m], an)
            prep_gu(wg_v, gs_s, lo, an[:10])
            prep_gu(wu_v, us_s, lo, an[10:22])
            for m in range(2):
                gu_pair(lhs, m, lo, _PAIR_ORDER[6:], t[m], anchors)
            return t

        def gu_final(lhs, t, lo, anchors):
            h = ([], [])
            for j in range(3):
                g = _column(t[0], gu_base(lhs, 0, lo, j, anchors), j)
                u = _column(t[1], gu_base(lhs, 1, lo, j, anchors), j)
                for i in range(2):
                    h[i].append(_gelu_mul(g[i], u[i]))
            return [v.astype(BF16) for v in _x_ops(*h)]

        D_ORDER = _PAIR_ORDER + (9, 10, 11, 12, 13, 14)

        def down_mm(acc, b, lo, anchors, even=False):
            n = b[0].shape[1]
            p = [None] * 15
            for i in D_ORDER:
                if i in _W_RAW:
                    k, j = _W_RAW[i]
                    p[i] = _dot_nt(wdt_v[j * D3:(j + 1) * D3, cols(k * FT + lo, n)], b[i])
                elif even and i == 14:
                    p[i] = cat0(*[_dot_nt(_upk(ds_s[_W_SUM[i], h * Q3 // 2:(h + 1) * Q3 // 2,
                                                    cols(lo, n)]), b[i]) for h in range(2)])
                else:
                    p[i] = _dot_nt(_upk(ds_s[_W_SUM[i], :, cols(lo, n)]), b[i])
                if acc is not None:
                    p[i] = acc[i] + p[i]
                anchors.append(p[i][:8])
            return p

        def finish(blk, acc):
            y = [cat1(*_column(acc, [acc[_DIAG[s, j]] if (s, j) in _DIAG else None
                                     for s in range(3)], j)) for j in range(3)]
            xio_s[blk] = (xmid_s[blk] + cat0(*y)).astype(BF16)

        def load_acc(k):
            return [acc_s[k, i] for i in range(15)]

        def store_acc(k, acc):
            for i in range(15):
                acc_s[k, i] = acc[i]

        def load_b():
            return [_upk(b_s[i * TH // 2:(i + 1) * TH // 2, :]) for i in range(15)]

        def store_b(b):
            for i in range(15):
                b_s[i * TH // 2:(i + 1) * TH // 2, :] = _pk(b[i])

        x0_cp, x1_cp = x_cp(0, 0), x_cp(1, 3)
        order = [x0_cp, wq_cp(0), wq_cp(1), x1_cp, wq_cp(2)]
        for p in range(NP + 1):
            order += group_cp(p)
        for cp in order:
            cp.start()
        qkv_s[0] = jnp.zeros(qkv_s.shape[1:], U32)
        acc_s[...] = jnp.zeros(acc_s.shape, F32)
        wait('WX0', [x0_cp])
        xn0 = ln1(0, ()).astype(BF16)
        done = 0
        for i in range(3):
            wait('WQ%d' % i, [wq_cp(i)] + ([x1_cp] if i == 2 else []))
            wt_s[WQ[i] // 2:WQ[i + 1] // 2, :] = _pk(wqkv_v[:, WQ[i]:WQ[i + 1]].T)
            anchors = []
            qkv_mm(0, xn0, range(done, WQ[i + 1] // QR), anchors)
            done = WQ[i + 1] // QR
        xn1 = ln1(1, anchors[:1]).astype(BF16)
        qkv_mm(1, xn1, range(4), anchors)
        attention(0, [anchors[i] for i in cfg['att0']], 9)
        wait('WO', group_cp(0))
        wt_s[3 * RP:, :] = _pk(wo_v[...].T)
        stats = wo_mm(0, [], False)
        qkv_mm(1, xn1, [4], [])
        ffn_lhs(0, stats, [])
        lhs = load_lhs(0)
        b = gu_final(lhs, gu_shared_prep(lhs, 0, []), 0, [])
        qkv_mm(1, xn1, [5], [])
        store_b(b)

        def piece(p, carry):
            wait('WP', group_cp(p))
            lhs = load_lhs(0)
            b_prev = load_b()
            an, an_d = [], []
            t = gu_shared_prep(lhs, p * PW, an)
            b = gu_final(lhs, t, p * PW, an)
            prep_d((p - 1) * PW, [an[i] for i in cfg['p_d']])
            store_acc(0, down_mm(load_acc(0), b_prev, (p - 1) * PW, an_d, True))
            an += an_d
            for i in range(2):
                g = jnp.minimum(2 * (p - 1) + i, NT * NG - 1)
                att_group(1, g // NG, lax.rem(g, NG), an[cfg['p_att'][i]], 9)
            npat = len(cfg['p_w'])
            for i in range(npat):
                r = jnp.minimum((p - 1) * npat + i, 4 * Q3 // 8 - 1)
                prep_att(r * 8, an[cfg['p_w'][i]])
            store_b(b)
            return carry

        lax.fori_loop(1, NP, piece, 0)

        wait('WD', group_cp(NP))
        an = []
        stats = wo_mm(1, an, True)
        prep_d((NP - 1) * PW, an[:12])
        acc = down_mm(load_acc(0), load_b(), (NP - 1) * PW, [], True)
        ffn_lhs(1, stats, [])
        finish(0, acc)

        def body(u, carry):
            bu = lax.rem(u, NB)
            ba = lax.rem(u + 1, NB)
            lhs = load_lhs(bu)
            acc, stats, an, b = None, None, {}, {}
            get = lambda name: [an[k][i] for k, i in cfg[name]]
            for step in cfg['body']:
                an[step] = []
                if step == 'Q':
                    qkv_fast(ba, att_rhs(ln1(ba, get('ln1'), get('ln1b'))), an[step])
                elif step == 'W':
                    attention(ba, get('att'), 9)
                    stats = wo_mm(ba, an[step], True)
                elif step == 'L':
                    ffn_lhs(ba, stats, get('lhs'))
                elif step[0] == 'S':
                    b[step] = gu_shared(lhs, int(step[1]) * PW, an[step])
                elif step[0] == 'F':
                    j = int(step[1])
                    b[j] = gu_final(lhs, b['S' + step[1]], j * PW, an[step])
                else:
                    js = [int(c) for c in step[1:]]
                    bb = [cat1(*[b[j][i] for j in js]) for i in range(15)]
                    acc = down_mm(acc, bb, js[0] * PW, an[step], len(js) % 2 == 1)
            finish(bu, acc)

            @pl.when(u >= NB)
            def _():
                out_copy(bu).start()
            return carry

        if scopes:
            with jax.named_scope('LOOP'):
                lax.fori_loop(1, NU - 1, body, 0)
        else:
            lax.fori_loop(1, NU - 1, body, 0)

        def last(c, carry):
            lhs = load_lhs(NB - 1)
            los = [(2 * c + j) * PW for j in range(2)]
            b = [gu_final(lhs, gu_shared(lhs, lo, []), lo, []) for lo in los]
            acc = load_acc(1)
            for j in range(2):
                acc = down_mm(acc, b[j], los[j], [])
            store_acc(1, acc)
            return carry

        lax.fori_loop(0, NP // 2, last, 0)
        finish(NB - 1, load_acc(1))
        out_copy(NB - 1).start()
        wait('WOUT', [out_copy(b) for b in range(NB)])

    scratch = [
        pltpu.VMEM((NB, D, TM), BF16),
        pltpu.VMEM((D, 3 * D), BF16),
        pltpu.VMEM((D, D), BF16),
        pltpu.VMEM((D, F), BF16),
        pltpu.VMEM((D, F), BF16),
        pltpu.VMEM((D, F), BF16),
        pltpu.VMEM((2 * D, D), U32),
        pltpu.VMEM((4 * Q3, 15 * LANES), U32),
        pltpu.VMEM((9, LANES // 2, FT), U32),
        pltpu.VMEM((9, LANES // 2, FT), U32),
        pltpu.VMEM((9, Q3, FT), U32),
        pltpu.VMEM((NB, D, TM), F32),
        pltpu.VMEM((NB, TH // 2, 18 * LANES), U32),
        pltpu.VMEM((S // LANES + 1, 3 * RP, LANES), U32),
        pltpu.VMEM((NT, D, LANES), F32),
        pltpu.VMEM((2, 15, D3, TH), F32),
        pltpu.VMEM((15 * TH // 2, PW), U32),
        pltpu.SemaphoreType.DMA((SEM_P + NP + 1,)),
        pltpu.SemaphoreType.DMA((1,)),
    ]
    return kernel, scratch


_CFG = dict(
    scopes=False,
    body=('S0', 'F0', 'S1', 'Q', 'F1', 'S2', 'F2', 'D01', 'S3', 'F3', 'S4', 'W', 'F4',
          'S5', 'L', 'F5', 'D23', 'D45'),
    ln1=tuple(('S0', i) for i in range(2, 36, 4)),
    ln1b=tuple(('S1', i) for i in (8, 16, 24)),
    att=(('S2', 8), ('S2', 22), ('D01', 2), ('D01', 5), ('D01', 8), ('D01', 11),
         ('S3', 4), ('S3', 18)),
    lhs=(('S5', 4), ('S5', 12), ('S5', 20), ('S5', 28)),
    att0=(1, 2, 3, 4, 5, 6, 7, 8),
    p_d=tuple(range(0, 36, 3)), p_att=(0, 50), p_w=(48, 49, 50, 52, 53, 54, 56, 57, 58, 59))


def _run(A_x, A_wqkv, A_wo, B_w_gate, B_w_up, B_w_down, **kw):
    _, S, D = A_x.shape
    F = B_w_gate.shape[1]
    kernel, scratch = _make_kernel(S, D, F, 256, {**_CFG, **kw})
    hbm = pl.BlockSpec(memory_space=pl.ANY)
    out_t = pl.pallas_call(
        kernel,
        in_specs=[hbm] * 6,
        out_specs=hbm,
        out_shape=jax.ShapeDtypeStruct((D, S), A_x.dtype),
        scratch_shapes=scratch,
        compiler_params=pltpu.CompilerParams(vmem_limit_bytes=110 * 1024 * 1024),
    )(A_x[0].T, A_wqkv, A_wo, B_w_gate, B_w_up, B_w_down.T)
    return out_t.T[None]


@jax.jit
def pallas_interleave_layers__sliding_local_dilated__glu_gated_geglu__prompt_kernel(
    A_x: jax.Array,
    A_wqkv: jax.Array,
    A_wo: jax.Array,
    B_x: jax.Array,
    B_w_gate: jax.Array,
    B_w_up: jax.Array,
    B_w_down: jax.Array,
):
    del B_x
    return _run(A_x, A_wqkv, A_wo, B_w_gate, B_w_up, B_w_down)
```

```python
import functools

import jax
import jax.numpy as jnp
import jax.experimental.pallas as pl
import jax.experimental.pallas.tpu as pltpu
from jax import lax

H = 32
W = 8
DIL = 2
EPS = 1e-5
LANES = 128

F32 = jnp.float32
BF16 = jnp.bfloat16
U32 = jnp.uint32

_NT = (((1,), (1,)), ((), ()))


def _tree_sum(parts):
    while len(parts) > 1:
        nxt = [parts[i] + parts[i + 1] for i in range(0, len(parts) - 1, 2)]
        if len(parts) % 2:
            nxt.append(parts[-1])
        parts = nxt
    return parts[0]


def _ln_stats(slabs, d, anchors=()):
    n_acc = 4
    s1, s2, pilot = [None] * n_acc, [None] * n_acc, None
    for i, x in enumerate(slabs):
        if pilot is None:
            pilot = x[0:1, :]
            pil = jnp.broadcast_to(pilot, x.shape)
            pils = [_tie(pil, a) for a in anchors] or [pil]
        dx = x - pils[i * len(pils) // (d // 8)]
        j = i % n_acc
        s1[j] = dx if s1[j] is None else s1[j] + dx
        s2[j] = dx * dx if s2[j] is None else s2[j] + dx * dx
    e1 = jnp.sum(_tree_sum(s1), axis=0, keepdims=True) * (1.0 / d)
    e2 = jnp.sum(_tree_sum(s2), axis=0, keepdims=True) * (1.0 / d)
    var = jnp.maximum(e2 - e1 * e1, 0.0)
    return pilot + e1, lax.rsqrt(var + EPS)


def _zero_like_dep(v):
    return (lax.bitcast_convert_type(v, U32) >> 31) >> 1


def _tie(x, anchor):
    if anchor is None:
        return x
    z = lax.bitcast_convert_type(_zero_like_dep(anchor), F32)
    z = jnp.concatenate([z] * (x.shape[1] // LANES), axis=1)
    if x.shape[0] == 8:
        return x + z
    return jnp.concatenate([x[:8] + z, x[8:]], axis=0)


def _gelu_mul2(g, u):
    c0 = 0.7978845608028654
    c1 = c0 * 0.044715
    t = jnp.tanh(g * (c0 + c1 * (g * g)))
    return (g * u) * (1.0 + t)


def _lo(x):
    return lax.bitcast_convert_type(x << 16, F32)


def _hi(x):
    return lax.bitcast_convert_type(x & jnp.uint32(0xFFFF0000), F32)


def _pk(x):
    return pltpu.bitcast(x.astype(BF16), U32)


def _upk(x):
    return pltpu.bitcast(x, BF16)


def _dot(a, b):
    return jnp.dot(a, b, preferred_element_type=F32)


def _dot_nt(a, b):
    return lax.dot_general(a, b, _NT, preferred_element_type=F32)


def _x_ops(x1, x2):
    d = [a - b for a, b in zip(x1, x2)]
    return [x1[0] + x2[1], x2[0] + x2[1], x1[0] + x1[1],
            d[1] + x1[2], x1[1] + x1[2], d[1] + d[2],
            d[0] - x2[2], d[0] + d[2], x2[0] + x2[2],
            x1[0], d[0], x2[1], d[1], x1[2], x2[2]]


def _x_rem(x1, x2):
    a, b, c = 0, 1, 2
    cat = lambda u, v: jnp.concatenate([u, v], axis=0)
    return [cat(x1[c], x2[b]), cat(x1[a], x1[b] - x2[b]), cat(x2[a], x2[c] - x1[c])]


def _w_sums(w):
    return [w[0][1] + w[1][0], w[1][2] + w[2][1], w[0][2] + w[2][0],
            w[0][0] + w[0][2] - w[1][0], w[2][0] - w[0][0] - w[0][1],
            w[1][1] + w[1][2] - w[0][1], w[1][0] + w[1][1] - w[2][1],
            w[2][0] + w[2][2] - w[1][2], w[2][1] + w[2][2] - w[0][2]]


_W_SUM = {0: 0, 3: 1, 6: 2, 9: 3, 10: 4, 11: 5, 12: 6, 13: 7, 14: 8}
_W_RAW = {1: (0, 1), 2: (1, 0), 4: (1, 2), 5: (2, 1), 7: (2, 0), 8: (0, 2)}
_PAIR_ORDER = (1, 2, 4, 5, 7, 8, 0, 3, 6)
_DIAG = {(0, 0): 9, (2, 0): 10, (0, 1): 11, (1, 1): 12, (1, 2): 13, (2, 2): 14}
_PAIR = {(0, 0): ((6, -1), (8, -1)), (1, 0): ((2, 1), (7, 1)), (2, 0): ((0, 1), (1, -1)),
         (0, 1): ((3, 1), (4, -1)), (1, 1): ((0, 1), (2, -1)), (2, 1): ((1, 1), (5, -1)),
         (0, 2): ((4, 1), (8, 1)), (1, 2): ((6, 1), (7, -1)), (2, 2): ((5, 1), (3, -1))}


def _column(t, base, j):
    s = []
    for k in range(3):
        v = base[k]
        for i, sg in _PAIR[k, j]:
            v = t[i] if v is None else (v + t[i] if sg > 0 else v - t[i])
        s.append(v)
    return s[1] + s[0], s[2] + s[0]


def _make_kernel(S, D, F, TM, cfg):
    NB = S // TM
    NT = TM // LANES
    DH = D // H
    DP = DH // 2
    RP = D // 2
    NG = H // 8
    scale = float(DH) ** -0.5
    NU = 2 * NB
    TH = TM // 2
    FT = F // 3
    D2 = D // 2
    D3 = D // 3
    Q3 = D3 // 2
    KU = D // 9
    KR = 3 * LANES
    NQ = 6
    QR = 3 * D // NQ
    WQ = (0, 640, 1152, 3 * D)
    PW = 256
    NP = FT // PW
    scopes = cfg['scopes']
    assert NG == 4 and NB & (NB - 1) == 0
    SEM_P = 4

    def kernel(x_hbm, wqkv_hbm, wo_hbm, wg_hbm, wu_hbm, wdt_hbm, out_hbm,
               xio_s, wqkv_v, wo_v, wg_v, wu_v, wdt_v, wt_s, wl_s,
               gs_s, us_s, ds_s, xmid_s, a_s, qkv_s, o_s, acc_s, b_s,
               sem_i, sem_o):

        def wait(name, cps):
            if scopes:
                with jax.named_scope(name):
                    for cp in cps:
                        cp.wait()
            else:
                for cp in cps:
                    cp.wait()

        def cols(lo, n):
            if not isinstance(lo, int):
                lo = pl.multiple_of(lo, LANES)
            return pl.ds(lo, n)

        def rows8(lo, n=8):
            if not isinstance(lo, int):
                lo = pl.multiple_of(lo, 8)
            return pl.ds(lo, n)

        def out_copy(b):
            return pltpu.make_async_copy(
                xio_s.at[b], out_hbm.at[:, cols(b * TM, TM)], sem_o.at[0])

        def x_cp(b, sem):
            return pltpu.make_async_copy(x_hbm.at[:, cols(b * TM, TM)], xio_s.at[b],
                                         sem_i.at[sem])

        def wq_cp(i):
            sl = cols(WQ[i], WQ[i + 1] - WQ[i])
            return pltpu.make_async_copy(wqkv_hbm.at[:, sl], wqkv_v.at[:, sl],
                                         sem_i.at[1 + i])

        def piece_cp(src, dst, p, sem):
            return [pltpu.make_async_copy(src.at[:, cols(j * FT + p * PW, PW)],
                                          dst.at[:, cols(j * FT + p * PW, PW)],
                                          sem_i.at[sem]) for j in range(3)]

        def group_cp(p):
            sem = SEM_P + p
            cps = []
            if isinstance(p, int) and p == 0:
                cps.append(pltpu.make_async_copy(wo_hbm, wo_v, sem_i.at[sem]))
            if not (isinstance(p, int) and p == NP):
                cps += piece_cp(wg_hbm, wg_v, p, sem) + piece_cp(wu_hbm, wu_v, p, sem)
            if not (isinstance(p, int) and p == 0):
                cps += piece_cp(wdt_hbm, wdt_v, p - 1, sem)
            return cps

        lane = lax.broadcasted_iota(jnp.int32, (8, LANES), 1)
        cat0 = lambda *v: jnp.concatenate(v, axis=0)
        cat1 = lambda *v: jnp.concatenate(v, axis=1)

        def spread_over(anchors, n, total):
            return anchors[n * len(anchors) // total] if anchors else None

        def ln1(blk, anchors1, anchors2=()):
            slabs = (xio_s[blk, r:r + 8, :].astype(F32) for r in range(0, D, 8))
            m, rs = _ln_stats(slabs, D, anchors1)
            if not anchors2:
                return (xio_s[blk].astype(F32) - m) * rs
            m8 = jnp.broadcast_to(m, (8, TM))
            ms = [cat0(*[_tie(m8, a)] * (KU // 8)) for a in anchors2]
            out = [None] * 9
            for n, k in enumerate((0, 2, 4, 1, 3, 5, 6, 7, 8)):
                x = xio_s[blk, k * KU:(k + 1) * KU, :].astype(F32)
                out[k] = (x - spread_over(ms, n, 9)) * rs
            return cat0(*out)

        def put_qkv(blk, rows, y):
            pk = _pk(y)
            for c in range(NT):
                qkv_s[1 + blk * NT + c, rows, :] = pk[:, c * LANES:(c + 1) * LANES]

        def qkv_mm(blk, xn, chunks, anchors):
            for r in chunks:
                rows = slice(r * QR // 2, (r + 1) * QR // 2)
                qkv = _dot(_upk(wt_s[rows, :]), xn)
                anchors.append(qkv[:8, :LANES])
                anchors.append(qkv[QR - 8:, TM - LANES:])
                put_qkv(blk, rows, qkv)

        def split_k(x):
            hs = (x[:, :TH], x[:, TH:])
            blocks = [[h[k * LANES:(k + 1) * LANES] for k in range(3)] for h in hs]
            units = [[h[KR + k * KU:KR + (k + 1) * KU] for k in range(3)] for h in hs]
            return blocks, units

        def prep_att(pat, anchor):
            assert Q3 == 96
            row0 = pat * 8
            src0 = row0 + ((pat * 43) >> 9) * (2 * Q3)
            w = [_upk(wt_s[rows8(src0 + j * Q3), :]).astype(F32) for j in range(3)]
            w[0] = cat1(_tie(w[0][:, :LANES], anchor), w[0][:, LANES:])
            tiles = _w_sums([[w[j][:, k * LANES:(k + 1) * LANES] for j in range(3)]
                             for k in range(3)])
            for j in range(3):
                a, b, c = (w[j][:, KR + k * KU:KR + (k + 1) * KU] for k in range(3))
                tiles += [cat1(c, b), cat1(a, c)]
            wl_s[rows8(row0), :] = _pk(cat1(*tiles))

        def att_rhs(x):
            blocks, units = split_k(x)
            return [v.astype(BF16) for v in _x_ops(*blocks) + _x_rem(*units)]

        def att_mm(sec, rhs, anchors):
            tl = lambda i: _upk(wl_s[sec * Q3:(sec + 1) * Q3, i * LANES:(i + 1) * LANES])
            raw = lambda k, j: _upk(wt_s[(3 * sec + j) * Q3:(3 * sec + j + 1) * Q3,
                                         k * LANES:(k + 1) * LANES])
            t = {}
            for i in _PAIR_ORDER:
                t[i] = _dot(raw(*_W_RAW[i]) if i in _W_RAW else tl(_W_SUM[i]), rhs[i])
                anchors.append(t[i][:8])
            out = []
            for j in range(3):
                base = []
                for s in range(3):
                    v = _dot(raw(3, j) if s == 1 else tl(9 + 2 * j + s // 2), rhs[15 + s])
                    if (s, j) in _DIAG:
                        i = _DIAG[s, j]
                        v = _dot(tl(_W_SUM[i]), rhs[i]) + v
                    base.append(v)
                    anchors.append(base[-1][:8])
                out.append(cat1(*_column(t, base, j)))
            return cat0(*out)

        def qkv_fast(blk, rhs, anchors):
            for sec in range(3):
                put_qkv(blk, slice(sec * RP, (sec + 1) * RP), att_mm(sec, rhs, anchors))

        def shifted(ln, cur, prev, w):
            if w == 0:
                return cur
            sh = DIL * w
            return pltpu.roll(jnp.where(ln < LANES - sh, cur, prev), sh, axis=1)

        def att_group(blk, c, hg, anchor, win):
            tile = blk * NT + c
            base = hg * 8 * DP
            if isinstance(hg, int):
                cur, prev, o_t = qkv_s.at[1 + tile], qkv_s.at[tile], o_s.at[c]
                obase = hg * 8 * DH
            else:
                n = 2 * RP + 8 * DP
                base = pl.multiple_of(base, 8)
                cur = qkv_s.at[1 + tile, pl.ds(base, n)]
                prev = qkv_s.at[tile, pl.ds(base, n)]
                o_t = o_s.at[c, pl.ds(pl.multiple_of(hg * 8 * DH, 8), 8 * DH)]
                base, obase = 0, 0
            ln = lane + _zero_like_dep(anchor).astype(jnp.int32)
            logits = [None] * W
            done = []
            for dd in range(DP):
                q = cur[pl.ds(base + dd, 8, stride=DP), :]
                kc = cur[pl.ds(RP + base + dd, 8, stride=DP), :]
                if dd >= win:
                    kc = kc | _zero_like_dep(done[dd - win])
                kp = prev[pl.ds(RP + base + dd, 8, stride=DP), :]
                q0, q1 = _lo(q), _hi(q)
                for w in range(W):
                    ks = shifted(ln, kc, kp, w)
                    t = q0 * _lo(ks) + q1 * _hi(ks)
                    logits[w] = t if logits[w] is None else logits[w] + t
                done.append(ks)
            logits = [l * scale for l in logits]
            if not (isinstance(c, int) and c > 0):
                pos = lane + tile * LANES
                logits = [l if w == 0 else jnp.where(pos >= DIL * w, l, -1e9)
                          for w, l in enumerate(logits)]
            m = functools.reduce(jnp.maximum, logits)
            ln = lane + _zero_like_dep(m).astype(jnp.int32)
            e = [jnp.exp(l - m) for l in logits]
            r = 1.0 / functools.reduce(lambda a, b: a + b, e)
            p = [x * r for x in e]
            done = []
            for dd in range(DP):
                vc = cur[pl.ds(2 * RP + base + dd, 8, stride=DP), :]
                if dd >= win:
                    vc = vc | _zero_like_dep(done[dd - win])
                vp = prev[pl.ds(2 * RP + base + dd, 8, stride=DP), :]
                o0 = o1 = None
                for w in range(W):
                    vs = shifted(ln, vc, vp, w)
                    t0, t1 = p[w] * _lo(vs), p[w] * _hi(vs)
                    o0 = t0 if o0 is None else o0 + t0
                    o1 = t1 if o1 is None else o1 + t1
                done.append(vs)
                o_t[pl.ds(obase + 2 * dd, 8, stride=DH), :] = o0
                o_t[pl.ds(obase + 2 * dd + 1, 8, stride=DH), :] = o1

        def attention(blk, anchors, win):
            for c in range(NT):
                for hg in range(NG):
                    att_group(blk, c, hg, anchors[c * NG + hg], win)

        def wo_mm(blk, anchors, fast):
            o = cat1(*[o_s[c] for c in range(NT)])
            if fast:
                y = att_mm(3, att_rhs(o), anchors)
            else:
                o = o.astype(BF16)
                q = D2 // 2
                ys = [_dot(_upk(wt_s[6 * q:7 * q, :]), o), _dot(_upk(wt_s[7 * q:, :]), o)]
                for y in ys:
                    anchors.append(y[:8, :LANES])
                    anchors.append(y[D2 - 8:, TM - LANES:])
                y = cat0(*ys)
            xm = xio_s[blk].astype(F32) + y
            xmid_s[blk] = xm
            return _ln_stats((xm[r:r + 8] for r in range(0, D, 8)), D)

        def ffn_lhs(blk, stats, anchors):
            m, rs = stats
            m8 = jnp.broadcast_to(m, (8, TM))
            parts = []
            for n, (r0, nr) in enumerate(((0, LANES), (LANES, LANES), (2 * LANES, LANES),
                                          (KR, 3 * KU))):
                mt = cat0(*[_tie(m8, spread_over(anchors, n, 4))] * (nr // 8))
                parts.append((xmid_s[blk, r0:r0 + nr, :] - mt) * rs)
            blocks, units = split_k(cat0(*parts))
            for i, v in enumerate(_x_ops(*blocks) + _x_rem(*units)):
                a_s[blk, :, i * LANES:(i + 1) * LANES] = _pk(v.astype(BF16).T)

        def prep(w_v, s_s, nrow, blk_of, lo, anchors):
            PR = 16
            for n in range(nrow // PR):
                r = n * PR
                w = [[None] * 3 for _ in range(3)]
                for k in range(3):
                    for j in range(3):
                        rb, cb = blk_of(k, j)
                        w[k][j] = w_v[rb * nrow + r:rb * nrow + r + PR,
                                      cols(cb * FT + lo, PW)].astype(F32)
                w[0][1] = _tie(w[0][1], spread_over(anchors, n, nrow // PR))
                for i, v in enumerate(_w_sums(w)):
                    s_s.at[i][r // 2:(r + PR) // 2, cols(lo, PW)] = _pk(v)

        def prep_gu(w_v, s_s, lo, anchors):
            prep(w_v, s_s, LANES, lambda k, j: (k, j), lo, anchors)

        def prep_d(lo, anchors):
            prep(wdt_v, ds_s, D3, lambda k, j: (j, k), lo, anchors)

        def load_lhs(blk):
            return [_upk(a_s[blk, :, i * LANES:(i + 1) * LANES]) for i in range(18)]

        def spread(y, anchors):
            for j in range(y.shape[1] // LANES):
                anchors.append(y[:8, j * LANES:(j + 1) * LANES])
            return y

        GU = ((wg_v, gs_s), (wu_v, us_s))

        def gu_pair(lhs, m, lo, which, t, anchors):
            w_v, s_s = GU[m]
            for i in which:
                if i in _W_RAW:
                    k, j = _W_RAW[i]
                    r = w_v[k * LANES:(k + 1) * LANES, cols(j * FT + lo, PW)]
                else:
                    r = _upk(s_s[_W_SUM[i], :, cols(lo, PW)])
                t[i] = spread(_dot(lhs[i], r), anchors)

        def base_rhs(m, lo, n, j, s):
            w_v, s_s = GU[m]
            u = lambda k, c=1: w_v[KR + k * KU:KR + (k + c) * KU, cols(j * FT + lo, n)]
            r = cat0(u(2), u(1)) if s == 0 else u(0, 2) if s == 1 else cat0(u(0), u(2))
            if (s, j) in _DIAG:
                r = cat0(_upk(s_s[_W_SUM[_DIAG[s, j]], :, cols(lo, n)]), r)
            return r

        def gu_base(lhs, lo, j, anchors):
            base = ([], [])
            ls = [cat1(lhs[_DIAG[s, j]], lhs[15 + s]) if (s, j) in _DIAG else lhs[15 + s]
                  for s in range(3)]
            if cfg['guil'] == 0:
                for m in range(2):
                    for s in range(3):
                        base[m].append(spread(_dot(ls[s], base_rhs(m, lo, PW, j, s)), anchors))
            elif cfg['guil'] == 1:
                for s in range(3):
                    for m in range(2):
                        base[m].append(spread(_dot(ls[s], base_rhs(m, lo, PW, j, s)), anchors))
            else:
                for s in range(3):
                    r = cat1(*[base_rhs(m, lo + n * LANES, LANES, j, s)
                               for n in range(PW // LANES) for m in range(2)])
                    y = spread(_dot(ls[s], r), anchors)
                    for m in range(2):
                        base[m].append(cat1(*[y[:, (2 * n + m) * LANES:(2 * n + m + 1) * LANES]
                                              for n in range(PW // LANES)]))
            return base

        def gu_shared(lhs, lo, anchors):
            t = ({}, {})
            for m in range(2):
                gu_pair(lhs, m, lo, _PAIR_ORDER, t[m], anchors)
            return t

        def gu_shared_prep(lhs, lo, anchors):
            t, an = ({}, {}), []
            for m in range(2):
                gu_pair(lhs, m, lo, _PAIR_ORDER[:6], t[m], an)
            prep_gu(wg_v, gs_s, lo, [an[i] for i in cfg['p_g']])
            prep_gu(wu_v, us_s, lo, [an[i] for i in cfg['p_u']])
            for m in range(2):
                gu_pair(lhs, m, lo, _PAIR_ORDER[6:], t[m], anchors)
            return t

        def gu_col(lhs, t, lo, j, anchors):
            base = gu_base(lhs, lo, j, anchors)
            g, u = _column(t[0], base[0], j), _column(t[1], base[1], j)
            return [_gelu_mul2(g[i], u[i]) for i in range(2)]

        def h_ops(h):
            return [v.astype(BF16) for v in _x_ops(*[[h[j][i] for j in range(3)]
                                                     for i in range(2)])]

        def gu_final(lhs, t, lo, anchors):
            return h_ops({j: gu_col(lhs, t, lo, j, anchors) for j in range(3)})

        D_ORDER = _PAIR_ORDER + (9, 10, 11, 12, 13, 14)

        def down_mm(acc, bs, lo, anchors):
            p = [None] * 15
            for i in D_ORDER:
                for n, b in enumerate(bs):
                    c0 = lo + n * PW
                    if i in _W_RAW:
                        k, j = _W_RAW[i]
                        v = _dot_nt(wdt_v[j * D3:(j + 1) * D3, cols(k * FT + c0, PW)], b[i])
                    elif len(bs) % 2 and i == 14 and n == 0:
                        v = cat0(*[_dot_nt(_upk(ds_s[_W_SUM[i], h * Q3 // 2:(h + 1) * Q3 // 2,
                                                     cols(c0, PW)]), b[i]) for h in range(2)])
                    else:
                        v = _dot_nt(_upk(ds_s[_W_SUM[i], :, cols(c0, PW)]), b[i])
                    p[i] = v if p[i] is None else p[i] + v
                if acc is not None:
                    p[i] = acc[i] + p[i]
                anchors.append(p[i][:8])
            return p

        def finish(blk, acc):
            y = [cat1(*_column(acc, [acc[_DIAG[s, j]] if (s, j) in _DIAG else None
                                     for s in range(3)], j)) for j in range(3)]
            xio_s[blk] = (xmid_s[blk] + 0.5 * cat0(*y)).astype(BF16)

        def load_acc(k):
            return [acc_s[k, i] for i in range(15)]

        def store_acc(k, acc):
            for i in range(15):
                acc_s[k, i] = acc[i]

        def load_b():
            return [_upk(b_s[i * TH // 2:(i + 1) * TH // 2, :]) for i in range(15)]

        def store_b(b):
            for i in range(15):
                b_s[i * TH // 2:(i + 1) * TH // 2, :] = _pk(b[i])

        def pre_phase():
            x0_cp, x1_cp = x_cp(0, 0), x_cp(1, 3)
            order = [x0_cp, wq_cp(0), wq_cp(1), x1_cp, wq_cp(2)]
            for p in range(NP + 1):
                order += group_cp(p)
            xr_cp = [x_cp(b, SEM_P + NP + 1) for b in range(2, NB)]
            order += xr_cp
            for cp in order:
                cp.start()
            qkv_s[0] = jnp.zeros(qkv_s.shape[1:], U32)
            acc_s[...] = jnp.zeros(acc_s.shape, F32)
            wait('WX0', [x0_cp])
            xn0 = ln1(0, ()).astype(BF16)
            done = 0
            for i in range(3):
                wait('WQ%d' % i, [wq_cp(i)] + ([x1_cp] if i == 2 else []))
                wt_s[WQ[i] // 2:WQ[i + 1] // 2, :] = _pk(wqkv_v[:, WQ[i]:WQ[i + 1]].T)
                anchors = []
                qkv_mm(0, xn0, range(done, WQ[i + 1] // QR), anchors)
                done = WQ[i + 1] // QR
            xn1 = ln1(1, anchors[:1]).astype(BF16)
            qkv_mm(1, xn1, range(4), anchors)
            attention(0, [anchors[i] for i in cfg['att0']], 9)
            wait('WO', group_cp(0))
            wt_s[3 * RP:, :] = _pk(wo_v[...].T)
            stats = wo_mm(0, [], False)
            qkv_mm(1, xn1, [4], [])
            ffn_lhs(0, stats, [])
            lhs = load_lhs(0)
            b = gu_final(lhs, gu_shared_prep(lhs, 0, []), 0, [])
            qkv_mm(1, xn1, [5], [])
            store_b(b)

            def piece(p, carry):
                wait('WP', group_cp(p))
                lhs = load_lhs(0)
                b_prev = load_b()
                an, an_d = [], []
                t = gu_shared_prep(lhs, p * PW, an)
                b = gu_final(lhs, t, p * PW, an)
                prep_d((p - 1) * PW, [an[i] for i in cfg['p_d']])
                store_acc(0, down_mm(load_acc(0), [b_prev], (p - 1) * PW, an_d))
                an += an_d
                for i in range(2):
                    g = jnp.minimum(2 * (p - 1) + i, NT * NG - 1)
                    att_group(1, g >> 2, g & (NG - 1), an[cfg['p_att'][i]], 9)
                npat = len(cfg['p_w'])
                for i in range(npat):
                    r = jnp.minimum((p - 1) * npat + i, 4 * Q3 // 8 - 1)
                    prep_att(r, an[cfg['p_w'][i]])
                store_b(b)
                return carry

            lax.fori_loop(1, NP, piece, 0)

            wait('WD', group_cp(NP))
            an = []
            stats = wo_mm(1, an, True)
            prep_d((NP - 1) * PW, [an[i] for i in cfg['t_d']])
            acc = down_mm(load_acc(0), [load_b()], (NP - 1) * PW, [])
            ffn_lhs(1, stats, [])
            finish(0, acc)
            wait('WX', xr_cp)

        if 'pre' in cfg['phases']:
            pre_phase()

        def body(u, carry):
            bu = u & (NB - 1)
            ba = (u + 1) & (NB - 1)
            lhs = load_lhs(bu)
            acc, stats, an, b = None, None, {}, {}
            get = lambda name: [an[k][i] for k, i in cfg[name]]
            for step in cfg['body']:
                an[step] = []
                if step == 'Q':
                    qkv_fast(ba, att_rhs(ln1(ba, get('ln1'), get('ln1b'))), an[step])
                elif step == 'W':
                    attention(ba, get('att'), 9)
                    stats = wo_mm(ba, an[step], True)
                elif step == 'L':
                    ffn_lhs(ba, stats, get('lhs'))
                elif step[0] == 'S':
                    t = b.setdefault(step[:2], ({}, {}))
                    which = _PAIR_ORDER
                    if len(step) > 2:
                        which = cfg['sparts'][int(step[2])]
                    for m in range(2):
                        gu_pair(lhs, m, int(step[1]) * PW, which, t[m], an[step])
                elif step[0] == 'F':
                    j = int(step[1])
                    h = b.setdefault(step[:2], {})
                    for c in ([int(step[2])] if len(step) > 2 else range(3)):
                        h[c] = gu_col(lhs, b['S' + step[1]], j * PW, c, an[step])
                    if len(h) == 3:
                        b[j] = h_ops(h)
                else:
                    js = [int(c) for c in step[1:]]
                    acc = down_mm(acc, [b[j] for j in js], js[0] * PW, an[step])
            finish(bu, acc)

            @pl.when(u >= NB)
            def _():
                out_copy(bu).start()
            return carry

        if scopes:
            with jax.named_scope('LOOP'):
                lax.fori_loop(1, NU - 1, body, 0)
        elif 'main' in cfg['phases']:
            lax.fori_loop(1, NU - 1, body, 0)

        def last(c, carry):
            lhs = load_lhs(NB - 1)
            los = [(2 * c + j) * PW for j in range(2)]
            b = [gu_final(lhs, gu_shared(lhs, lo, []), lo, []) for lo in los]
            acc = load_acc(1)
            for j in range(2):
                acc = down_mm(acc, [b[j]], los[j], [])
            store_acc(1, acc)
            return carry

        if 'last' in cfg['phases']:
            lax.fori_loop(0, NP // 2, last, 0)
        finish(NB - 1, load_acc(1))
        out_copy(NB - 1).start()
        wait('WOUT', [out_copy(b) for b in range(NB)])

    scratch = [
        pltpu.VMEM((NB, D, TM), BF16),
        pltpu.VMEM((D, 3 * D), BF16),
        pltpu.VMEM((D, D), BF16),
        pltpu.VMEM((D, F), BF16),
        pltpu.VMEM((D, F), BF16),
        pltpu.VMEM((D, F), BF16),
        pltpu.VMEM((2 * D, D), U32),
        pltpu.VMEM((4 * Q3, 15 * LANES), U32),
        pltpu.VMEM((9, LANES // 2, FT), U32),
        pltpu.VMEM((9, LANES // 2, FT), U32),
        pltpu.VMEM((9, Q3, FT), U32),
        pltpu.VMEM((NB, D, TM), F32),
        pltpu.VMEM((NB, TH // 2, 18 * LANES), U32),
        pltpu.VMEM((S // LANES + 1, 3 * RP, LANES), U32),
        pltpu.VMEM((NT, D, LANES), F32),
        pltpu.VMEM((2, 15, D3, TH), F32),
        pltpu.VMEM((15 * TH // 2, PW), U32),
        pltpu.SemaphoreType.DMA((SEM_P + NP + 2,)),
        pltpu.SemaphoreType.DMA((1,)),
    ]
    return kernel, scratch


_CFG = dict(
    scopes=False,
    phases=('pre', 'main', 'last'),
    sparts=((0, 1, 2), (6, 7, 8), (3, 4, 5)),
    guil=2,
    body=('S0', 'F0', 'S3', 'S2', 'Q', 'S1', 'F2', 'F3', 'F1', 'D2', 'S4', 'D01', 'F4',
        'W', 'S5', 'L', 'F5', 'D3', 'D4', 'D5'),
    ln1=(('S0', 2), ('S0', 6), ('S0', 10), ('S0', 14), ('S0', 18), ('S0', 22), ('S0',
        26), ('S0', 30), ('S0', 34)),
    ln1b=(('S3', 30), ('S2', 7), ('S2', 15)),
    att=(('S1', 6), ('S1', 18), ('D2', 5), ('S4', 12), ('D01', 7), ('D01', 8), ('D01',
        9), ('D01', 12)),
    lhs=(('S5', 12), ('S5', 14), ('S5', 20), ('S5', 24)),
    att0=(0, 1, 2, 3, 3, 4, 6, 8),
    p_g=(0, 1, 2, 3, 5, 6, 7, 8),
    p_u=(10, 11, 13, 14, 16, 17, 20, 20),
    t_d=(1, 2, 3, 4, 5, 6, 6, 8, 9, 10, 11, 13),
    p_d=(0, 3, 6, 9, 15, 18, 21, 22, 24, 27, 30, 33),
    p_att=(0, 52),
    p_w=(43, 45, 49, 51, 53, 55, 57, 59, 60, 62),
)


def _run(A_x, A_wqkv, A_wo, B_w_gate, B_w_up, B_w_down, **kw):
    _, S, D = A_x.shape
    F = B_w_gate.shape[1]
    kernel, scratch = _make_kernel(S, D, F, 256, {**_CFG, **kw})
    hbm = pl.BlockSpec(memory_space=pl.ANY)
    out_t = pl.pallas_call(
        kernel,
        in_specs=[hbm] * 6,
        out_specs=hbm,
        out_shape=jax.ShapeDtypeStruct((D, S), A_x.dtype),
        scratch_shapes=scratch,
        compiler_params=pltpu.CompilerParams(vmem_limit_bytes=110 * 1024 * 1024),
    )(A_x[0].T, A_wqkv, A_wo, B_w_gate, B_w_up, B_w_down.T)
    return out_t.T[None]


@jax.jit
def pallas_interleave_layers__sliding_local_dilated__glu_gated_geglu__prompt_kernel(
    A_x: jax.Array,
    A_wqkv: jax.Array,
    A_wo: jax.Array,
    B_x: jax.Array,
    B_w_gate: jax.Array,
    B_w_up: jax.Array,
    B_w_down: jax.Array,
):
    del B_x
    return _run(A_x, A_wqkv, A_wo, B_w_gate, B_w_up, B_w_down)
```

```python
import functools

import jax
import jax.numpy as jnp
import jax.experimental.pallas as pl
import jax.experimental.pallas.tpu as pltpu
from jax import lax

H = 32
W = 8
DIL = 2
EPS = 1e-5
LANES = 128

F32 = jnp.float32
BF16 = jnp.bfloat16
U32 = jnp.uint32

_NT = (((1,), (1,)), ((), ()))


def _tree_sum(parts):
    while len(parts) > 1:
        nxt = [parts[i] + parts[i + 1] for i in range(0, len(parts) - 1, 2)]
        if len(parts) % 2:
            nxt.append(parts[-1])
        parts = nxt
    return parts[0]


def _ln_stats(slabs, d, anchors=()):
    n_acc = 4
    s1, s2, pilot = [None] * n_acc, [None] * n_acc, None
    for i, x in enumerate(slabs):
        if pilot is None:
            pilot = x[0:1, :]
            pil = jnp.broadcast_to(pilot, x.shape)
            pils = [_tie(pil, a) for a in anchors] or [pil]
        dx = x - pils[i * len(pils) // (d // 8)]
        j = i % n_acc
        s1[j] = dx if s1[j] is None else s1[j] + dx
        s2[j] = dx * dx if s2[j] is None else s2[j] + dx * dx
    e1 = jnp.sum(_tree_sum(s1), axis=0, keepdims=True) * (1.0 / d)
    e2 = jnp.sum(_tree_sum(s2), axis=0, keepdims=True) * (1.0 / d)
    var = jnp.maximum(e2 - e1 * e1, 0.0)
    return pilot + e1, lax.rsqrt(var + EPS)


def _zero_like_dep(v):
    return (lax.bitcast_convert_type(v, U32) >> 31) >> 1


def _tie(x, anchor):
    if anchor is None:
        return x
    z = lax.bitcast_convert_type(_zero_like_dep(anchor), F32)
    z = jnp.concatenate([z] * (x.shape[1] // LANES), axis=1)
    if x.shape[0] == 8:
        return x + z
    return jnp.concatenate([x[:8] + z, x[8:]], axis=0)


def _gelu_mul2(g, u):
    c0 = 0.7978845608028654
    c1 = c0 * 0.044715
    t = jnp.tanh(g * (c0 + c1 * (g * g)))
    return (g * u) * (1.0 + t)


def _lo(x):
    return lax.bitcast_convert_type(x << 16, F32)


def _hi(x):
    return lax.bitcast_convert_type(x & jnp.uint32(0xFFFF0000), F32)


def _pk(x):
    return pltpu.bitcast(x.astype(BF16), U32)


def _upk(x):
    return pltpu.bitcast(x, BF16)


def _dot(a, b):
    return jnp.dot(a, b, preferred_element_type=F32)


def _dot_nt(a, b):
    return lax.dot_general(a, b, _NT, preferred_element_type=F32)


def _x_ops(x1, x2):
    d = [a - b for a, b in zip(x1, x2)]
    return [x1[0] + x2[1], x2[0] + x2[1], x1[0] + x1[1],
            d[1] + x1[2], x1[1] + x1[2], d[1] + d[2],
            d[0] - x2[2], d[0] + d[2], x2[0] + x2[2],
            x1[0], d[0], x2[1], d[1], x1[2], x2[2]]


def _x_rem(x1, x2):
    a, b, c = 0, 1, 2
    cat = lambda u, v: jnp.concatenate([u, v], axis=0)
    return [cat(x1[c], x2[b]), cat(x1[a], x1[b] - x2[b]), cat(x2[a], x2[c] - x1[c])]


def _w_sums(w):
    return [w[0][1] + w[1][0], w[1][2] + w[2][1], w[0][2] + w[2][0],
            w[0][0] + w[0][2] - w[1][0], w[2][0] - w[0][0] - w[0][1],
            w[1][1] + w[1][2] - w[0][1], w[1][0] + w[1][1] - w[2][1],
            w[2][0] + w[2][2] - w[1][2], w[2][1] + w[2][2] - w[0][2]]


_W_SUM = {0: 0, 3: 1, 6: 2, 9: 3, 10: 4, 11: 5, 12: 6, 13: 7, 14: 8}
_W_RAW = {1: (0, 1), 2: (1, 0), 4: (1, 2), 5: (2, 1), 7: (2, 0), 8: (0, 2)}
_PAIR_ORDER = (1, 2, 4, 5, 7, 8, 0, 3, 6)
_DIAG = {(0, 0): 9, (2, 0): 10, (0, 1): 11, (1, 1): 12, (1, 2): 13, (2, 2): 14}
_PAIR = {(0, 0): ((6, -1), (8, -1)), (1, 0): ((2, 1), (7, 1)), (2, 0): ((0, 1), (1, -1)),
         (0, 1): ((3, 1), (4, -1)), (1, 1): ((0, 1), (2, -1)), (2, 1): ((1, 1), (5, -1)),
         (0, 2): ((4, 1), (8, 1)), (1, 2): ((6, 1), (7, -1)), (2, 2): ((5, 1), (3, -1))}


def _column(t, base, j):
    s = []
    for k in range(3):
        v = base[k]
        for i, sg in _PAIR[k, j]:
            v = t[i] if v is None else (v + t[i] if sg > 0 else v - t[i])
        s.append(v)
    return s[1] + s[0], s[2] + s[0]


def _make_kernel(S, D, F, TM, cfg):
    NB = S // TM
    NT = TM // LANES
    DH = D // H
    DP = DH // 2
    RP = D // 2
    NG = H // 8
    scale = float(DH) ** -0.5
    NU = 2 * NB
    TH = TM // 2
    FT = F // 3
    D2 = D // 2
    D3 = D // 3
    Q3 = D3 // 2
    KU = D // 9
    KR = 3 * LANES
    NQ = 6
    QR = 3 * D // NQ
    WQ = (0, 640, 1152, 3 * D)
    PW = 256
    NP = FT // PW
    scopes = cfg['scopes']
    assert NG == 4 and NB & (NB - 1) == 0
    SEM_P = 4

    def kernel(x_hbm, wqkv_hbm, wo_hbm, wg_hbm, wu_hbm, wdt_hbm, out_hbm,
               xio_s, wqkv_v, wo_v, wg_v, wu_v, wdt_v, wt_s, wl_s,
               gs_s, us_s, ds_s, xmid_s, a_s, qkv_s, o_s, acc_s, b_s,
               sem_i, sem_o):

        def wait(name, cps):
            if scopes:
                with jax.named_scope(name):
                    for cp in cps:
                        cp.wait()
            else:
                for cp in cps:
                    cp.wait()

        def cols(lo, n):
            if not isinstance(lo, int):
                lo = pl.multiple_of(lo, LANES)
            return pl.ds(lo, n)

        def rows8(lo, n=8):
            if not isinstance(lo, int):
                lo = pl.multiple_of(lo, 8)
            return pl.ds(lo, n)

        def out_copy(b):
            return pltpu.make_async_copy(
                xio_s.at[b], out_hbm.at[:, cols(b * TM, TM)], sem_o.at[0])

        def x_cp(b, sem):
            return pltpu.make_async_copy(x_hbm.at[:, cols(b * TM, TM)], xio_s.at[b],
                                         sem_i.at[sem])

        def wq_cp(i):
            sl = cols(WQ[i], WQ[i + 1] - WQ[i])
            return pltpu.make_async_copy(wqkv_hbm.at[:, sl], wqkv_v.at[:, sl],
                                         sem_i.at[1 + i])

        def piece_cp(src, dst, p, sem):
            return [pltpu.make_async_copy(src.at[:, cols(j * FT + p * PW, PW)],
                                          dst.at[p, j],
                                          sem_i.at[sem]) for j in range(3)]

        def group_cp(p):
            sem = SEM_P + p
            cps = []
            if isinstance(p, int) and p == 0:
                cps.append(pltpu.make_async_copy(wo_hbm, wo_v, sem_i.at[sem]))
            if not (isinstance(p, int) and p == NP):
                cps += piece_cp(wg_hbm, wg_v, p, sem) + piece_cp(wu_hbm, wu_v, p, sem)
            if not (isinstance(p, int) and p == 0):
                cps += piece_cp(wdt_hbm, wdt_v, p - 1, sem)
            return cps

        lane = lax.broadcasted_iota(jnp.int32, (8, LANES), 1)
        cat0 = lambda *v: jnp.concatenate(v, axis=0)
        cat1 = lambda *v: jnp.concatenate(v, axis=1)

        def spread_over(anchors, n, total):
            return anchors[n * len(anchors) // total] if anchors else None

        def ln1(blk, anchors1, anchors2=()):
            slabs = (xio_s[blk, r:r + 8, :].astype(F32) for r in range(0, D, 8))
            m, rs = _ln_stats(slabs, D, anchors1)
            if not anchors2:
                return (xio_s[blk].astype(F32) - m) * rs
            m8 = jnp.broadcast_to(m, (8, TM))
            ms = [cat0(*[_tie(m8, a)] * (KU // 8)) for a in anchors2]
            out = [None] * 9
            for n, k in enumerate((0, 2, 4, 1, 3, 5, 6, 7, 8)):
                x = xio_s[blk, k * KU:(k + 1) * KU, :].astype(F32)
                out[k] = (x - spread_over(ms, n, 9)) * rs
            return cat0(*out)

        def put_qkv(blk, rows, y):
            pk = _pk(y)
            for c in range(NT):
                qkv_s[1 + blk * NT + c, rows, :] = pk[:, c * LANES:(c + 1) * LANES]

        def qkv_mm(blk, xn, chunks, anchors):
            for r in chunks:
                rows = slice(r * QR // 2, (r + 1) * QR // 2)
                qkv = _dot(_upk(wt_s[rows, :]), xn)
                anchors.append(qkv[:8, :LANES])
                anchors.append(qkv[QR - 8:, TM - LANES:])
                put_qkv(blk, rows, qkv)

        def split_k(x):
            hs = (x[:, :TH], x[:, TH:])
            blocks = [[h[k * LANES:(k + 1) * LANES] for k in range(3)] for h in hs]
            units = [[h[KR + k * KU:KR + (k + 1) * KU] for k in range(3)] for h in hs]
            return blocks, units

        def prep_att(pat, anchor):
            assert Q3 == 96
            row0 = pat * 8
            src0 = row0 + ((pat * 43) >> 9) * (2 * Q3)
            w = [_upk(wt_s[rows8(src0 + j * Q3), :]).astype(F32) for j in range(3)]
            w[0] = cat1(_tie(w[0][:, :LANES], anchor), w[0][:, LANES:])
            tiles = _w_sums([[w[j][:, k * LANES:(k + 1) * LANES] for j in range(3)]
                             for k in range(3)])
            for j in range(3):
                a, b, c = (w[j][:, KR + k * KU:KR + (k + 1) * KU] for k in range(3))
                tiles += [cat1(c, b), cat1(a, c)]
            wl_s[rows8(row0), :] = _pk(cat1(*tiles))

        def att_rhs(x):
            blocks, units = split_k(x)
            return [v.astype(BF16) for v in _x_ops(*blocks) + _x_rem(*units)]

        def att_mm(sec, rhs, anchors):
            tl = lambda i: _upk(wl_s[sec * Q3:(sec + 1) * Q3, i * LANES:(i + 1) * LANES])
            raw = lambda k, j: _upk(wt_s[(3 * sec + j) * Q3:(3 * sec + j + 1) * Q3,
                                         k * LANES:(k + 1) * LANES])
            t = {}
            for i in _PAIR_ORDER:
                t[i] = _dot(raw(*_W_RAW[i]) if i in _W_RAW else tl(_W_SUM[i]), rhs[i])
                anchors.append(t[i][:8])
            out = []
            for j in range(3):
                base = []
                for s in range(3):
                    v = _dot(raw(3, j) if s == 1 else tl(9 + 2 * j + s // 2), rhs[15 + s])
                    if (s, j) in _DIAG:
                        i = _DIAG[s, j]
                        v = _dot(tl(_W_SUM[i]), rhs[i]) + v
                    base.append(v)
                    anchors.append(base[-1][:8])
                out.append(cat1(*_column(t, base, j)))
            return cat0(*out)

        def qkv_fast(blk, rhs, anchors):
            for sec in range(3):
                put_qkv(blk, slice(sec * RP, (sec + 1) * RP), att_mm(sec, rhs, anchors))

        def shifted(ln, cur, prev, w):
            if w == 0:
                return cur
            sh = DIL * w
            return pltpu.roll(jnp.where(ln < LANES - sh, cur, prev), sh, axis=1)

        def att_group(blk, c, hg, anchor, win):
            tile = blk * NT + c
            base = hg * 8 * DP
            if isinstance(hg, int):
                cur, prev, o_t = qkv_s.at[1 + tile], qkv_s.at[tile], o_s.at[c]
                obase = hg * 8 * DH
            else:
                n = 2 * RP + 8 * DP
                base = pl.multiple_of(base, 8)
                cur = qkv_s.at[1 + tile, pl.ds(base, n)]
                prev = qkv_s.at[tile, pl.ds(base, n)]
                o_t = o_s.at[c, pl.ds(pl.multiple_of(hg * 8 * DH, 8), 8 * DH)]
                base, obase = 0, 0
            ln = lane + _zero_like_dep(anchor).astype(jnp.int32)
            logits = [None] * W
            done = []
            for dd in range(DP):
                q = cur[pl.ds(base + dd, 8, stride=DP), :]
                kc = cur[pl.ds(RP + base + dd, 8, stride=DP), :]
                if dd >= win:
                    kc = kc | _zero_like_dep(done[dd - win])
                kp = prev[pl.ds(RP + base + dd, 8, stride=DP), :]
                q0, q1 = _lo(q), _hi(q)
                for w in range(W):
                    ks = shifted(ln, kc, kp, w)
                    t = q0 * _lo(ks) + q1 * _hi(ks)
                    logits[w] = t if logits[w] is None else logits[w] + t
                done.append(ks)
            logits = [l * scale for l in logits]
            if not (isinstance(c, int) and c > 0):
                pos = lane + tile * LANES
                logits = [l if w == 0 else jnp.where(pos >= DIL * w, l, -1e9)
                          for w, l in enumerate(logits)]
            m = functools.reduce(jnp.maximum, logits)
            ln = lane + _zero_like_dep(m).astype(jnp.int32)
            e = [jnp.exp(l - m) for l in logits]
            r = 1.0 / functools.reduce(lambda a, b: a + b, e)
            p = [x * r for x in e]
            done = []
            for dd in range(DP):
                vc = cur[pl.ds(2 * RP + base + dd, 8, stride=DP), :]
                if dd >= win:
                    vc = vc | _zero_like_dep(done[dd - win])
                vp = prev[pl.ds(2 * RP + base + dd, 8, stride=DP), :]
                o0 = o1 = None
                for w in range(W):
                    vs = shifted(ln, vc, vp, w)
                    t0, t1 = p[w] * _lo(vs), p[w] * _hi(vs)
                    o0 = t0 if o0 is None else o0 + t0
                    o1 = t1 if o1 is None else o1 + t1
                done.append(vs)
                o_t[pl.ds(obase + 2 * dd, 8, stride=DH), :] = o0
                o_t[pl.ds(obase + 2 * dd + 1, 8, stride=DH), :] = o1

        def attention(blk, anchors, win):
            for c in range(NT):
                for hg in range(NG):
                    att_group(blk, c, hg, anchors[c * NG + hg], win)

        def wo_mm(blk, anchors, fast):
            o = cat1(*[o_s[c] for c in range(NT)])
            if fast:
                y = att_mm(3, att_rhs(o), anchors)
            else:
                o = o.astype(BF16)
                q = D2 // 2
                ys = [_dot(_upk(wt_s[6 * q:7 * q, :]), o), _dot(_upk(wt_s[7 * q:, :]), o)]
                for y in ys:
                    anchors.append(y[:8, :LANES])
                    anchors.append(y[D2 - 8:, TM - LANES:])
                y = cat0(*ys)
            xm = xio_s[blk].astype(F32) + y
            xmid_s[blk] = xm
            return _ln_stats((xm[r:r + 8] for r in range(0, D, 8)), D)

        def ffn_lhs(blk, stats, anchors):
            m, rs = stats
            m8 = jnp.broadcast_to(m, (8, TM))
            parts = []
            for n, (r0, nr) in enumerate(((0, LANES), (LANES, LANES), (2 * LANES, LANES),
                                          (KR, 3 * KU))):
                mt = cat0(*[_tie(m8, spread_over(anchors, n, 4))] * (nr // 8))
                parts.append((xmid_s[blk, r0:r0 + nr, :] - mt) * rs)
            blocks, units = split_k(cat0(*parts))
            for i, v in enumerate(_x_ops(*blocks) + _x_rem(*units)):
                a_s[blk, :, i * LANES:(i + 1) * LANES] = _pk(v.astype(BF16).T)

        def prep(w_v, s_s, nrow, blk_of, p, anchors):
            PR = 16
            for n in range(nrow // PR):
                r = n * PR
                w = [[None] * 3 for _ in range(3)]
                for k in range(3):
                    for j in range(3):
                        rb, cb = blk_of(k, j)
                        w[k][j] = w_v[p, cb, rb * nrow + r:rb * nrow + r + PR, :].astype(F32)
                w[0][1] = _tie(w[0][1], spread_over(anchors, n, nrow // PR))
                for i, v in enumerate(_w_sums(w)):
                    s_s.at[p, i][r // 2:(r + PR) // 2, :] = _pk(v)

        def prep_gu(w_v, s_s, p, anchors):
            prep(w_v, s_s, LANES, lambda k, j: (k, j), p, anchors)

        def prep_d(p, anchors):
            prep(wdt_v, ds_s, D3, lambda k, j: (j, k), p, anchors)

        def load_lhs(blk):
            return [_upk(a_s[blk, :, i * LANES:(i + 1) * LANES]) for i in range(18)]

        def spread(y, anchors):
            for j in range(y.shape[1] // LANES):
                anchors.append(y[:8, j * LANES:(j + 1) * LANES])
            return y

        GU = ((wg_v, gs_s), (wu_v, us_s))

        def gu_pair(lhs, m, p, which, t, anchors):
            w_v, s_s = GU[m]
            for i in which:
                if i in _W_RAW:
                    k, j = _W_RAW[i]
                    r = w_v[p, j, k * LANES:(k + 1) * LANES, :]
                else:
                    r = _upk(s_s[p, _W_SUM[i]])
                t[i] = spread(_dot(lhs[i], r), anchors)

        def base_rhs(m, p, n, j, s):
            w_v, s_s = GU[m]
            cs = slice(n * LANES, (n + 1) * LANES)
            u = lambda k, c=1: w_v[p, j, KR + k * KU:KR + (k + c) * KU, cs]
            r = cat0(u(2), u(1)) if s == 0 else u(0, 2) if s == 1 else cat0(u(0), u(2))
            if (s, j) in _DIAG:
                r = cat0(_upk(s_s[p, _W_SUM[_DIAG[s, j]], :, cs]), r)
            return r

        def gu_base(lhs, p, j, anchors):
            base = ([], [])
            for s in range(3):
                l = cat1(lhs[_DIAG[s, j]], lhs[15 + s]) if (s, j) in _DIAG else lhs[15 + s]
                r = cat1(*[base_rhs(m, p, n, j, s)
                           for n in range(PW // LANES) for m in range(2)])
                y = spread(_dot(l, r), anchors)
                for m in range(2):
                    base[m].append(cat1(*[y[:, (2 * n + m) * LANES:(2 * n + m + 1) * LANES]
                                          for n in range(PW // LANES)]))
            return base

        def gu_shared(lhs, lo, anchors):
            t = ({}, {})
            for m in range(2):
                gu_pair(lhs, m, lo, _PAIR_ORDER, t[m], anchors)
            return t

        def gu_shared_prep(lhs, lo, anchors):
            t, an = ({}, {}), []
            for m in range(2):
                gu_pair(lhs, m, lo, _PAIR_ORDER[:6], t[m], an)
            prep_gu(wg_v, gs_s, lo, [an[i] for i in cfg['p_g']])
            prep_gu(wu_v, us_s, lo, [an[i] for i in cfg['p_u']])
            for m in range(2):
                gu_pair(lhs, m, lo, _PAIR_ORDER[6:], t[m], anchors)
            return t

        def gu_col(lhs, t, lo, j, anchors):
            base = gu_base(lhs, lo, j, anchors)
            g, u = _column(t[0], base[0], j), _column(t[1], base[1], j)
            return [_gelu_mul2(g[i], u[i]) for i in range(2)]

        def h_ops(h):
            return [v.astype(BF16) for v in _x_ops(*[[h[j][i] for j in range(3)]
                                                     for i in range(2)])]

        def gu_final(lhs, t, lo, anchors):
            return h_ops({j: gu_col(lhs, t, lo, j, anchors) for j in range(3)})

        D_ORDER = _PAIR_ORDER + (9, 10, 11, 12, 13, 14)

        def down_mm(acc, bs, lo, anchors):
            p = [None] * 15
            for i in D_ORDER:
                for n, b in enumerate(bs):
                    if i in _W_RAW:
                        k, j = _W_RAW[i]
                        v = _dot_nt(wdt_v[lo + n, k, j * D3:(j + 1) * D3, :], b[i])
                    elif len(bs) % 2 and i == 14 and n == 0:
                        v = cat0(*[_dot_nt(_upk(ds_s[lo, _W_SUM[i],
                                                     h * Q3 // 2:(h + 1) * Q3 // 2, :]), b[i])
                                   for h in range(2)])
                    else:
                        v = _dot_nt(_upk(ds_s[lo + n, _W_SUM[i]]), b[i])
                    p[i] = v if p[i] is None else p[i] + v
                if acc is not None:
                    p[i] = acc[i] + p[i]
                anchors.append(p[i][:8])
            return p

        def finish(blk, acc):
            y = [cat1(*_column(acc, [acc[_DIAG[s, j]] if (s, j) in _DIAG else None
                                     for s in range(3)], j)) for j in range(3)]
            xio_s[blk] = (xmid_s[blk] + 0.5 * cat0(*y)).astype(BF16)

        def load_acc(k):
            return [acc_s[k, i] for i in range(15)]

        def store_acc(k, acc):
            for i in range(15):
                acc_s[k, i] = acc[i]

        def load_b():
            return [_upk(b_s[i * TH // 2:(i + 1) * TH // 2, :]) for i in range(15)]

        def store_b(b):
            for i in range(15):
                b_s[i * TH // 2:(i + 1) * TH // 2, :] = _pk(b[i])

        def pre_phase():
            x0_cp, x1_cp = x_cp(0, 0), x_cp(1, 3)
            order = [x0_cp, wq_cp(0), wq_cp(1), x1_cp, wq_cp(2)]
            for p in range(NP + 1):
                order += group_cp(p)
            xr_cp = [x_cp(b, SEM_P + NP + 1) for b in range(2, NB)]
            order += xr_cp
            for cp in order:
                cp.start()
            qkv_s[0] = jnp.zeros(qkv_s.shape[1:], U32)
            acc_s[...] = jnp.zeros(acc_s.shape, F32)
            wait('WX0', [x0_cp])
            xn0 = ln1(0, ()).astype(BF16)
            done = 0
            for i in range(3):
                wait('WQ%d' % i, [wq_cp(i)] + ([x1_cp] if i == 2 else []))
                wt_s[WQ[i] // 2:WQ[i + 1] // 2, :] = _pk(wqkv_v[:, WQ[i]:WQ[i + 1]].T)
                anchors = []
                qkv_mm(0, xn0, range(done, WQ[i + 1] // QR), anchors)
                done = WQ[i + 1] // QR
            xn1 = ln1(1, anchors[:1]).astype(BF16)
            qkv_mm(1, xn1, range(4), anchors)
            attention(0, [anchors[i] for i in cfg['att0']], 9)
            wait('WO', group_cp(0))
            wt_s[3 * RP:, :] = _pk(wo_v[...].T)
            stats = wo_mm(0, [], False)
            qkv_mm(1, xn1, [4], [])
            ffn_lhs(0, stats, [])
            lhs = load_lhs(0)
            b = gu_final(lhs, gu_shared_prep(lhs, 0, []), 0, [])
            qkv_mm(1, xn1, [5], [])
            store_b(b)

            def piece(p, carry):
                wait('WP', group_cp(p))
                lhs = load_lhs(0)
                b_prev = load_b()
                an, an_d = [], []
                t = gu_shared_prep(lhs, p, an)
                b = gu_final(lhs, t, p, an)
                prep_d(p - 1, [an[i] for i in cfg['p_d']])
                store_acc(0, down_mm(load_acc(0), [b_prev], p - 1, an_d))
                an += an_d
                for i in range(2):
                    g = jnp.minimum(2 * (p - 1) + i, NT * NG - 1)
                    att_group(1, g >> 2, g & (NG - 1), an[cfg['p_att'][i]], 9)
                npat = len(cfg['p_w'])
                for i in range(npat):
                    r = jnp.minimum((p - 1) * npat + i, 4 * Q3 // 8 - 1)
                    prep_att(r, an[cfg['p_w'][i]])
                store_b(b)
                return carry

            lax.fori_loop(1, NP, piece, 0)

            wait('WD', group_cp(NP))
            an = []
            stats = wo_mm(1, an, True)
            prep_d(NP - 1, [an[i] for i in cfg['t_d']])
            acc = down_mm(load_acc(0), [load_b()], NP - 1, [])
            ffn_lhs(1, stats, [])
            finish(0, acc)
            wait('WX', xr_cp)

        if 'pre' in cfg['phases']:
            pre_phase()

        def body(u, carry):
            bu = u & (NB - 1)
            ba = (u + 1) & (NB - 1)
            lhs = load_lhs(bu)
            acc, stats, an, b = None, None, {}, {}
            get = lambda name: [an[k][i] for k, i in cfg[name]]
            for step in cfg['body']:
                an[step] = []
                if step == 'Q':
                    qkv_fast(ba, att_rhs(ln1(ba, get('ln1'), get('ln1b'))), an[step])
                elif step == 'W':
                    attention(ba, get('att'), 9)
                    stats = wo_mm(ba, an[step], True)
                elif step == 'L':
                    ffn_lhs(ba, stats, get('lhs'))
                elif step[0] == 'S':
                    t = b.setdefault(step[:2], ({}, {}))
                    which = _PAIR_ORDER
                    if len(step) > 2:
                        which = cfg['sparts'][int(step[2])]
                    for m in range(2):
                        gu_pair(lhs, m, int(step[1]), which, t[m], an[step])
                elif step[0] == 'F':
                    j = int(step[1])
                    h = b.setdefault(step[:2], {})
                    for c in ([int(step[2])] if len(step) > 2 else range(3)):
                        h[c] = gu_col(lhs, b['S' + step[1]], j, c, an[step])
                    if len(h) == 3:
                        b[j] = h_ops(h)
                else:
                    js = [int(c) for c in step[1:]]
                    acc = down_mm(acc, [b[j] for j in js], js[0], an[step])
            finish(bu, acc)

            @pl.when(u >= NB)
            def _():
                out_copy(bu).start()
            return carry

        if scopes:
            with jax.named_scope('LOOP'):
                lax.fori_loop(1, NU - 1, body, 0)
        elif 'main' in cfg['phases']:
            lax.fori_loop(1, NU - 1, body, 0)

        def last(c, carry):
            lhs = load_lhs(NB - 1)
            los = [2 * c + j for j in range(2)]
            b = [gu_final(lhs, gu_shared(lhs, lo, []), lo, []) for lo in los]
            acc = load_acc(1)
            for j in range(2):
                acc = down_mm(acc, [b[j]], los[j], [])
            store_acc(1, acc)
            return carry

        if 'last' in cfg['phases']:
            lax.fori_loop(0, NP // 2, last, 0)
        finish(NB - 1, load_acc(1))
        out_copy(NB - 1).start()
        wait('WOUT', [out_copy(b) for b in range(NB)])

    scratch = [
        pltpu.VMEM((NB, D, TM), BF16),
        pltpu.VMEM((D, 3 * D), BF16),
        pltpu.VMEM((D, D), BF16),
        pltpu.VMEM((NP, 3, D, PW), BF16),
        pltpu.VMEM((NP, 3, D, PW), BF16),
        pltpu.VMEM((NP, 3, D, PW), BF16),
        pltpu.VMEM((2 * D, D), U32),
        pltpu.VMEM((4 * Q3, 15 * LANES), U32),
        pltpu.VMEM((NP, 9, LANES // 2, PW), U32),
        pltpu.VMEM((NP, 9, LANES // 2, PW), U32),
        pltpu.VMEM((NP, 9, Q3, PW), U32),
        pltpu.VMEM((NB, D, TM), F32),
        pltpu.VMEM((NB, TH // 2, 18 * LANES), U32),
        pltpu.VMEM((S // LANES + 1, 3 * RP, LANES), U32),
        pltpu.VMEM((NT, D, LANES), F32),
        pltpu.VMEM((2, 15, D3, TH), F32),
        pltpu.VMEM((15 * TH // 2, PW), U32),
        pltpu.SemaphoreType.DMA((SEM_P + NP + 2,)),
        pltpu.SemaphoreType.DMA((1,)),
    ]
    return kernel, scratch


_CFG = dict(
    scopes=False,
    phases=('pre', 'main', 'last'),
    sparts=((0, 1, 2), (6, 7, 8), (3, 4, 5)),
    guil=2,
    body=('S0', 'F0', 'S3', 'S2', 'Q', 'S1', 'F2', 'F3', 'F1', 'D2', 'S4', 'D01', 'F4',
        'W', 'S5', 'L', 'F5', 'D3', 'D4', 'D5'),
    ln1=(('S0', 2), ('S0', 6), ('S0', 10), ('S0', 14), ('S0', 18), ('S0', 22), ('S0',
        26), ('S0', 30), ('S0', 34)),
    ln1b=(('S3', 30), ('S2', 7), ('S2', 15)),
    att=(('S1', 6), ('S1', 18), ('D2', 5), ('S4', 12), ('D01', 7), ('D01', 8), ('D01',
        9), ('D01', 12)),
    lhs=(('S5', 12), ('S5', 14), ('S5', 20), ('S5', 24)),
    att0=(0, 1, 2, 3, 3, 4, 6, 8),
    p_g=(0, 1, 2, 3, 5, 6, 7, 8),
    p_u=(10, 11, 13, 14, 16, 17, 20, 20),
    t_d=(1, 2, 3, 4, 5, 6, 6, 8, 9, 10, 11, 13),
    p_d=(0, 3, 6, 9, 15, 18, 21, 22, 24, 27, 30, 33),
    p_att=(0, 52),
    p_w=(43, 45, 49, 51, 53, 55, 57, 59, 60, 62),
)


def _run(A_x, A_wqkv, A_wo, B_w_gate, B_w_up, B_w_down, **kw):
    _, S, D = A_x.shape
    F = B_w_gate.shape[1]
    kernel, scratch = _make_kernel(S, D, F, 256, {**_CFG, **kw})
    hbm = pl.BlockSpec(memory_space=pl.ANY)
    out_t = pl.pallas_call(
        kernel,
        in_specs=[hbm] * 6,
        out_specs=hbm,
        out_shape=jax.ShapeDtypeStruct((D, S), A_x.dtype),
        scratch_shapes=scratch,
        compiler_params=pltpu.CompilerParams(vmem_limit_bytes=110 * 1024 * 1024),
    )(A_x[0].T, A_wqkv, A_wo, B_w_gate, B_w_up, B_w_down.T)
    return out_t.T[None]


@jax.jit
def pallas_interleave_layers__sliding_local_dilated__glu_gated_geglu__prompt_kernel(
    A_x: jax.Array,
    A_wqkv: jax.Array,
    A_wo: jax.Array,
    B_x: jax.Array,
    B_w_gate: jax.Array,
    B_w_up: jax.Array,
    B_w_down: jax.Array,
):
    del B_x
    return _run(A_x, A_wqkv, A_wo, B_w_gate, B_w_up, B_w_down)
```

```python
import functools

import jax
import jax.numpy as jnp
import jax.experimental.pallas as pl
import jax.experimental.pallas.tpu as pltpu
from jax import lax

H = 32
W = 8
DIL = 2
EPS = 1e-5
LANES = 128

F32 = jnp.float32
BF16 = jnp.bfloat16
U32 = jnp.uint32

_NT = (((1,), (1,)), ((), ()))


def _tree_sum(parts):
    while len(parts) > 1:
        nxt = [parts[i] + parts[i + 1] for i in range(0, len(parts) - 1, 2)]
        if len(parts) % 2:
            nxt.append(parts[-1])
        parts = nxt
    return parts[0]


def _ln_stats(slabs, d, anchors=()):
    n_acc = 4
    s1, s2, pilot = [None] * n_acc, [None] * n_acc, None
    for i, x in enumerate(slabs):
        if pilot is None:
            pilot = x[0:1, :]
            pil = jnp.broadcast_to(pilot, x.shape)
            pils = [_tie(pil, a) for a in anchors] or [pil]
        dx = x - pils[i * len(pils) // (d // 8)]
        j = i % n_acc
        s1[j] = dx if s1[j] is None else s1[j] + dx
        s2[j] = dx * dx if s2[j] is None else s2[j] + dx * dx
    e1 = jnp.sum(_tree_sum(s1), axis=0, keepdims=True) * (1.0 / d)
    e2 = jnp.sum(_tree_sum(s2), axis=0, keepdims=True) * (1.0 / d)
    var = jnp.maximum(e2 - e1 * e1, 0.0)
    return pilot + e1, lax.rsqrt(var + EPS)


def _zero_like_dep(v):
    return (lax.bitcast_convert_type(v, U32) >> 31) >> 1


def _tie(x, anchor):
    if anchor is None:
        return x
    z = lax.bitcast_convert_type(_zero_like_dep(anchor), F32)
    z = jnp.concatenate([z] * (x.shape[1] // LANES), axis=1)
    if x.shape[0] == 8:
        return x + z
    return jnp.concatenate([x[:8] + z, x[8:]], axis=0)


def _gelu_mul2(g, u):
    c0 = 0.7978845608028654
    c1 = c0 * 0.044715
    t = jnp.tanh(g * (c0 + c1 * (g * g)))
    return (g * u) * (1.0 + t)


def _lo(x):
    return lax.bitcast_convert_type(x << 16, F32)


def _hi(x):
    return lax.bitcast_convert_type(x & jnp.uint32(0xFFFF0000), F32)


def _pk(x):
    return pltpu.bitcast(x.astype(BF16), U32)


def _upk(x):
    return pltpu.bitcast(x, BF16)


def _dot(a, b):
    return jnp.dot(a, b, preferred_element_type=F32)


def _dot_nt(a, b):
    return lax.dot_general(a, b, _NT, preferred_element_type=F32)


def _x_ops(x1, x2):
    d = [a - b for a, b in zip(x1, x2)]
    return [x1[0] + x2[1], x2[0] + x2[1], x1[0] + x1[1],
            d[1] + x1[2], x1[1] + x1[2], d[1] + d[2],
            d[0] - x2[2], d[0] + d[2], x2[0] + x2[2],
            x1[0], d[0], x2[1], d[1], x1[2], x2[2]]


def _x_rem(x1, x2):
    a, b, c = 0, 1, 2
    cat = lambda u, v: jnp.concatenate([u, v], axis=0)
    return [cat(x1[c], x2[b]), cat(x1[a], x1[b] - x2[b]), cat(x2[a], x2[c] - x1[c])]


def _w_sums(w):
    return [w[0][1] + w[1][0], w[1][2] + w[2][1], w[0][2] + w[2][0],
            w[0][0] + w[0][2] - w[1][0], w[2][0] - w[0][0] - w[0][1],
            w[1][1] + w[1][2] - w[0][1], w[1][0] + w[1][1] - w[2][1],
            w[2][0] + w[2][2] - w[1][2], w[2][1] + w[2][2] - w[0][2]]


_W_TERMS = {0: ((0, 1, 1), (1, 0, 1)), 3: ((1, 2, 1), (2, 1, 1)), 6: ((0, 2, 1), (2, 0, 1)),
            9: ((0, 0, 1), (0, 2, 1), (1, 0, -1)), 10: ((2, 0, 1), (0, 0, -1), (0, 1, -1)),
            11: ((1, 1, 1), (1, 2, 1), (0, 1, -1)), 12: ((1, 0, 1), (1, 1, 1), (2, 1, -1)),
            13: ((2, 0, 1), (2, 2, 1), (1, 2, -1)), 14: ((2, 1, 1), (2, 2, 1), (0, 2, -1)),
            1: ((0, 1, 1),), 2: ((1, 0, 1),), 4: ((1, 2, 1),), 5: ((2, 1, 1),),
            7: ((2, 0, 1),), 8: ((0, 2, 1),)}
_PARTS = ((1, 2, 0), (7, 8, 6), (4, 5, 3), (9, 10, 11, 12, 13, 14))
_W_SUM = {0: 0, 3: 1, 6: 2, 9: 3, 10: 4, 11: 5, 12: 6, 13: 7, 14: 8}
_W_RAW = {1: (0, 1), 2: (1, 0), 4: (1, 2), 5: (2, 1), 7: (2, 0), 8: (0, 2)}
_PAIR_ORDER = (1, 2, 4, 5, 7, 8, 0, 3, 6)
_DIAG = {(0, 0): 9, (2, 0): 10, (0, 1): 11, (1, 1): 12, (1, 2): 13, (2, 2): 14}
_PAIR = {(0, 0): ((6, -1), (8, -1)), (1, 0): ((2, 1), (7, 1)), (2, 0): ((0, 1), (1, -1)),
         (0, 1): ((3, 1), (4, -1)), (1, 1): ((0, 1), (2, -1)), (2, 1): ((1, 1), (5, -1)),
         (0, 2): ((4, 1), (8, 1)), (1, 2): ((6, 1), (7, -1)), (2, 2): ((5, 1), (3, -1))}


def _column(t, base, j):
    s = []
    for k in range(3):
        v = base[k]
        for i, sg in _PAIR[k, j]:
            v = t[i] if v is None else (v + t[i] if sg > 0 else v - t[i])
        s.append(v)
    return s[1] + s[0], s[2] + s[0]


def _make_kernel(S, D, F, TM, cfg):
    NB = S // TM
    NT = TM // LANES
    DH = D // H
    DP = DH // 2
    RP = D // 2
    NG = H // 8
    scale = float(DH) ** -0.5
    NU = 2 * NB
    TH = TM // 2
    FT = F // 3
    D2 = D // 2
    D3 = D // 3
    Q3 = D3 // 2
    KU = D // 9
    KR = 3 * LANES
    NQ = 6
    QR = 3 * D // NQ
    WQ = (0, 640, 1152, 3 * D)
    PW = 256
    NP = FT // PW
    scopes = cfg['scopes']
    assert NG == 4 and NB & (NB - 1) == 0
    SEM_P = 4

    def kernel(x_hbm, wqkv_hbm, wo_hbm, wg_hbm, wu_hbm, wdt_hbm, out_hbm,
               xio_s, wqkv_v, wo_v, wg_v, wu_v, wdt_v, wt_s, wl_s,
               gs_s, us_s, ds_s, xmid_s, a_s, qkv_s, o_s, acc_s, b_s,
               sem_i, sem_o):

        def wait(name, cps):
            if scopes:
                with jax.named_scope(name):
                    for cp in cps:
                        cp.wait()
            else:
                for cp in cps:
                    cp.wait()

        def cols(lo, n):
            if not isinstance(lo, int):
                lo = pl.multiple_of(lo, LANES)
            return pl.ds(lo, n)

        def rows8(lo, n=8):
            if not isinstance(lo, int):
                lo = pl.multiple_of(lo, 8)
            return pl.ds(lo, n)

        def out_copy(b):
            return pltpu.make_async_copy(
                xio_s.at[b], out_hbm.at[:, cols(b * TM, TM)], sem_o.at[0])

        def x_cp(b, sem):
            return pltpu.make_async_copy(x_hbm.at[:, cols(b * TM, TM)], xio_s.at[b],
                                         sem_i.at[sem])

        def wq_cp(i):
            sl = cols(WQ[i], WQ[i + 1] - WQ[i])
            return pltpu.make_async_copy(wqkv_hbm.at[:, sl], wqkv_v.at[:, sl],
                                         sem_i.at[1 + i])

        def piece_cp(src, dst, p, sem):
            return [pltpu.make_async_copy(src.at[:, cols(j * FT + p * PW, PW)],
                                          dst.at[p, j],
                                          sem_i.at[sem]) for j in range(3)]

        def group_cp(p):
            sem = SEM_P + p
            cps = []
            if isinstance(p, int) and p == 0:
                cps.append(pltpu.make_async_copy(wo_hbm, wo_v, sem_i.at[sem]))
            if not (isinstance(p, int) and p == NP):
                cps += piece_cp(wg_hbm, wg_v, p, sem) + piece_cp(wu_hbm, wu_v, p, sem)
            if not (isinstance(p, int) and p == 0):
                cps += piece_cp(wdt_hbm, wdt_v, p - 1, sem)
            return cps

        lane = lax.broadcasted_iota(jnp.int32, (8, LANES), 1)
        cat0 = lambda *v: jnp.concatenate(v, axis=0)
        cat1 = lambda *v: jnp.concatenate(v, axis=1)

        def spread_over(anchors, n, total):
            return anchors[n * len(anchors) // total] if anchors else None

        def slab_group(r):
            return (r % LANES) // 16 if r < KR else 8 + ((r - KR) % KU) // 16

        def ln1(blk, anchors1, anchors2=()):
            slabs = (xio_s[blk, r:r + 8, :].astype(F32) for r in range(0, D, 8))
            m, rs = _ln_stats(slabs, D, anchors1)
            if not anchors2:
                return (xio_s[blk].astype(F32) - m) * rs
            m8 = jnp.broadcast_to(m, (8, TM))
            ms = [_tie(m8, a) for a in anchors2]
            ms = [spread_over(ms, slab_group(r), 12) for r in range(0, D, 8)]
            return (xio_s[blk].astype(F32) - cat0(*ms)) * rs

        def put_qkv(blk, rows, y):
            pk = _pk(y)
            for c in range(NT):
                qkv_s[1 + blk * NT + c, rows, :] = pk[:, c * LANES:(c + 1) * LANES]

        def qkv_mm(blk, xn, chunks, anchors):
            for r in chunks:
                rows = slice(r * QR // 2, (r + 1) * QR // 2)
                qkv = _dot(_upk(wt_s[rows, :]), xn)
                anchors.append(qkv[:8, :LANES])
                anchors.append(qkv[QR - 8:, TM - LANES:])
                put_qkv(blk, rows, qkv)

        def split_k(x):
            hs = (x[:, :TH], x[:, TH:])
            blocks = [[h[k * LANES:(k + 1) * LANES] for k in range(3)] for h in hs]
            units = [[h[KR + k * KU:KR + (k + 1) * KU] for k in range(3)] for h in hs]
            return blocks, units

        def prep_att(pat, anchor):
            assert Q3 == 96
            row0 = pat * 8
            src0 = row0 + ((pat * 43) >> 9) * (2 * Q3)
            w = [_upk(wt_s[rows8(src0 + j * Q3), :]).astype(F32) for j in range(3)]
            w[0] = cat1(_tie(w[0][:, :LANES], anchor), w[0][:, LANES:])
            tiles = _w_sums([[w[j][:, k * LANES:(k + 1) * LANES] for j in range(3)]
                             for k in range(3)])
            for j in range(3):
                a, b, c = (w[j][:, KR + k * KU:KR + (k + 1) * KU] for k in range(3))
                tiles += [cat1(c, b), cat1(a, c)]
            wl_s[rows8(row0), :] = _pk(cat1(*tiles))

        def att_rhs(x):
            blocks, units = split_k(x)
            return [v.astype(BF16) for v in _x_ops(*blocks) + _x_rem(*units)]

        def att_mm(sec, rhs, anchors):
            tl = lambda i: _upk(wl_s[sec * Q3:(sec + 1) * Q3, i * LANES:(i + 1) * LANES])
            raw = lambda k, j: _upk(wt_s[(3 * sec + j) * Q3:(3 * sec + j + 1) * Q3,
                                         k * LANES:(k + 1) * LANES])
            t = {}
            for i in _PAIR_ORDER:
                t[i] = _dot(raw(*_W_RAW[i]) if i in _W_RAW else tl(_W_SUM[i]), rhs[i])
                anchors.append(t[i][:8])
            out = []
            for j in range(3):
                base = []
                for s in range(3):
                    v = _dot(raw(3, j) if s == 1 else tl(9 + 2 * j + s // 2), rhs[15 + s])
                    if (s, j) in _DIAG:
                        i = _DIAG[s, j]
                        v = _dot(tl(_W_SUM[i]), rhs[i]) + v
                    base.append(v)
                    anchors.append(base[-1][:8])
                out.append(cat1(*_column(t, base, j)))
            return cat0(*out)

        def qkv_fast(blk, rhs, anchors):
            for sec in range(3):
                put_qkv(blk, slice(sec * RP, (sec + 1) * RP), att_mm(sec, rhs, anchors))

        def shifted(ln, cur, prev, w):
            if w == 0:
                return cur
            sh = DIL * w
            return pltpu.roll(jnp.where(ln < LANES - sh, cur, prev), sh, axis=1)

        def att_group(blk, c, hg, anchor, win):
            tile = blk * NT + c
            base = hg * 8 * DP
            if isinstance(hg, int):
                cur, prev, o_t = qkv_s.at[1 + tile], qkv_s.at[tile], o_s.at[c]
                obase = hg * 8 * DH
            else:
                n = 2 * RP + 8 * DP
                base = pl.multiple_of(base, 8)
                cur = qkv_s.at[1 + tile, pl.ds(base, n)]
                prev = qkv_s.at[tile, pl.ds(base, n)]
                o_t = o_s.at[c, pl.ds(pl.multiple_of(hg * 8 * DH, 8), 8 * DH)]
                base, obase = 0, 0
            ln = lane + _zero_like_dep(anchor).astype(jnp.int32)
            logits = [None] * W
            done = []
            for dd in range(DP):
                q = cur[pl.ds(base + dd, 8, stride=DP), :]
                kc = cur[pl.ds(RP + base + dd, 8, stride=DP), :]
                if dd >= win:
                    kc = kc | _zero_like_dep(done[dd - win])
                kp = prev[pl.ds(RP + base + dd, 8, stride=DP), :]
                q0, q1 = _lo(q), _hi(q)
                for w in range(W):
                    ks = shifted(ln, kc, kp, w)
                    t = q0 * _lo(ks) + q1 * _hi(ks)
                    logits[w] = t if logits[w] is None else logits[w] + t
                done.append(ks)
            logits = [l * scale for l in logits]
            if not (isinstance(c, int) and c > 0):
                pos = lane + tile * LANES
                logits = [l if w == 0 else jnp.where(pos >= DIL * w, l, -1e9)
                          for w, l in enumerate(logits)]
            m = functools.reduce(jnp.maximum, logits)
            ln = lane + _zero_like_dep(m).astype(jnp.int32)
            e = [jnp.exp(l - m) for l in logits]
            r = 1.0 / functools.reduce(lambda a, b: a + b, e)
            p = [x * r for x in e]
            done = []
            for dd in range(DP):
                vc = cur[pl.ds(2 * RP + base + dd, 8, stride=DP), :]
                if dd >= win:
                    vc = vc | _zero_like_dep(done[dd - win])
                vp = prev[pl.ds(2 * RP + base + dd, 8, stride=DP), :]
                o0 = o1 = None
                for w in range(W):
                    vs = shifted(ln, vc, vp, w)
                    t0, t1 = p[w] * _lo(vs), p[w] * _hi(vs)
                    o0 = t0 if o0 is None else o0 + t0
                    o1 = t1 if o1 is None else o1 + t1
                done.append(vs)
                o_t[pl.ds(obase + 2 * dd, 8, stride=DH), :] = o0
                o_t[pl.ds(obase + 2 * dd + 1, 8, stride=DH), :] = o1

        def attention(blk, anchors, win):
            for c in range(NT):
                for hg in range(NG):
                    att_group(blk, c, hg, anchors[c * NG + hg], win)

        def wo_mm(blk, anchors, fast, anchors_in=()):
            o = cat1(*[o_s[c] for c in range(NT)])
            if anchors_in:
                o = cat0(*[_tie(o[r:r + 8], spread_over(anchors_in, slab_group(r), 12))
                           for r in range(0, D, 8)])
            if fast:
                y = att_mm(3, att_rhs(o), anchors)
            else:
                o = o.astype(BF16)
                q = D2 // 2
                ys = [_dot(_upk(wt_s[6 * q:7 * q, :]), o), _dot(_upk(wt_s[7 * q:, :]), o)]
                for y in ys:
                    anchors.append(y[:8, :LANES])
                    anchors.append(y[D2 - 8:, TM - LANES:])
                y = cat0(*ys)
            xm = xio_s[blk].astype(F32) + y
            xmid_s[blk] = xm
            return _ln_stats((xm[r:r + 8] for r in range(0, D, 8)), D)

        def ffn_lhs(blk, stats, anchors):
            m, rs = stats
            m8 = jnp.broadcast_to(m, (8, TM))
            xs = []
            for k in range(3):
                mt = cat0(*[_tie(m8, spread_over(anchors, k, 3))] * (D3 // 8))
                xs.append((xmid_s[blk, k * D3:(k + 1) * D3, :] - mt) * rs)
            ops = _x_ops([x[:, :TH] for x in xs], [x[:, TH:] for x in xs])
            for i, v in enumerate(ops):
                for s, t in enumerate((v[KU:], v[:2 * KU], cat0(v[:KU], v[2 * KU:]))):
                    a_s[3 * i + s] = _pk(t.astype(BF16).T)

        def prep(w_v, s_s, nrow, blk_of, p, anchors):
            PR = 16
            for n in range(nrow // PR):
                r = n * PR
                w = [[None] * 3 for _ in range(3)]
                for k in range(3):
                    for j in range(3):
                        rb, cb = blk_of(k, j)
                        w[k][j] = w_v[p, cb, rb * nrow + r:rb * nrow + r + PR, :].astype(F32)
                w[0][1] = _tie(w[0][1], spread_over(anchors, n, nrow // PR))
                for i, v in enumerate(_w_sums(w)):
                    s_s.at[p, i][r // 2:(r + PR) // 2, :] = _pk(v)

        GU = ((wg_v, gs_s), (wu_v, us_s))

        def prep_gu(p, part, anchors):
            PR = 16
            nr = D3 // PR
            for n in range(2 * nr):
                (w_v, s_s), r = GU[n % 2], (n // 2) * PR
                cache = {}

                def w(k, j):
                    if (k, j) not in cache:
                        v = w_v[p, j, k * D3 + r:k * D3 + r + PR, :].astype(F32)
                        if not cache:
                            v = _tie(v, spread_over(anchors, n, 2 * nr))
                        l, h = v[:, :LANES], v[:, LANES:]
                        cache[k, j] = (v, cat1(l - h, h), cat1(l, h - l))[r // KU]
                    return cache[k, j]

                for i in _PARTS[part]:
                    v = None
                    for k, j, sg in _W_TERMS[i]:
                        v = w(k, j) if v is None else (v + w(k, j) if sg > 0 else v - w(k, j))
                    s_s.at[p, i][r // 2:(r + PR) // 2, :] = _pk(v)

        def prep_d(p, anchors):
            prep(wdt_v, ds_s, D3, lambda k, j: (j, k), p, anchors)

        def gu_prod(p, i, t, anchors, even=False):
            u = KU // 2

            def rhs(s, s_s):
                if s == 1:
                    return s_s[p, i, :2 * u, :LANES]
                if s == 0:
                    return cat0(s_s[p, i, u:2 * u, LANES:], s_s[p, i, 2 * u:, :LANES])
                return cat0(s_s[p, i, :u, LANES:], s_s[p, i, 2 * u:, LANES:])

            ns = cfg['msplit']
            q = TH // 2 // ns
            y1, y2 = [], []
            for h in range(ns):
                y = []
                for s in range(3):
                    r = _upk(cat1(rhs(s, gs_s), rhs(s, us_s)))
                    if even and s == 2 and ns == 1:
                        y.append(cat0(*[_dot(_upk(a_s[3 * i + s, k * q // 2:(k + 1) * q // 2]), r)
                                        for k in range(2)]))
                    else:
                        y.append(_dot(_upk(a_s[3 * i + s, h * q:(h + 1) * q]), r))
                    if (3 * h + s) % ns == 0:
                        anchors.append(y[-1][:8, :LANES])
                y1.append(y[1] + y[0])
                y2.append(y[2] + y[0])
            y1, y2 = cat0(*y1), cat0(*y2)
            for m in range(2):
                cs = slice(m * LANES, (m + 1) * LANES)
                t[m][i] = cat1(y1[:, cs], y2[:, cs])

        def gu_col(t, p, j, anchors, even=False):
            ids = [_DIAG.get((s, j)) for s in range(3)]
            for i in ids:
                if i is not None:
                    gu_prod(p, i, t, anchors, even and i == 14)
            g, u = [_column(t[m], [None if i is None else t[m][i] for i in ids], j)
                    for m in range(2)]
            return [_gelu_mul2(g[i], u[i]) for i in range(2)]

        def h_ops(h):
            return [v.astype(BF16) for v in _x_ops(*[[h[j][i] for j in range(3)]
                                                     for i in range(2)])]

        def gu_piece(p, order, anchors, even=False):
            t, h = ({}, {}), {}
            for step in order:
                if step[0] == 'S':
                    for i in _PARTS[int(step[1])]:
                        gu_prod(p, i, t, anchors)
                else:
                    h[int(step[1])] = gu_col(t, p, int(step[1]), anchors, even)
            return h_ops(h)

        D_ORDER = _PAIR_ORDER + (9, 10, 11, 12, 13, 14)

        def down_mm(acc, bs, lo, anchors, which=D_ORDER):
            p = [None] * 15 if acc is None else list(acc)
            for i in which:
                y = None
                for n, b in enumerate(bs):
                    if i in _W_RAW:
                        k, j = _W_RAW[i]
                        v = _dot_nt(wdt_v[lo + n, k, j * D3:(j + 1) * D3, :], b[i])
                    elif len(bs) % 2 and i == 14 and n == 0:
                        v = cat0(*[_dot_nt(_upk(ds_s[lo, _W_SUM[i],
                                                     h * Q3 // 2:(h + 1) * Q3 // 2, :]), b[i])
                                   for h in range(2)])
                    else:
                        v = _dot_nt(_upk(ds_s[lo + n, _W_SUM[i]]), b[i])
                    y = v if y is None else y + v
                p[i] = y if p[i] is None else p[i] + y
                anchors.append(p[i][:8])
            return p

        def finish(blk, acc):
            y = [cat1(*_column(acc, [acc[_DIAG[s, j]] if (s, j) in _DIAG else None
                                     for s in range(3)], j)) for j in range(3)]
            xio_s[blk] = (xmid_s[blk] + 0.5 * cat0(*y)).astype(BF16)

        def load_acc(k):
            return [acc_s[k, i] for i in range(15)]

        def store_acc(k, acc):
            for i in range(15):
                acc_s[k, i] = acc[i]

        def load_b():
            return [_upk(b_s[i * TH // 2:(i + 1) * TH // 2, :]) for i in range(15)]

        def store_b(b):
            for i in range(15):
                b_s[i * TH // 2:(i + 1) * TH // 2, :] = _pk(b[i])

        def pre_phase():
            x0_cp, x1_cp = x_cp(0, 0), x_cp(1, 3)
            order = [x0_cp, wq_cp(0), wq_cp(1), x1_cp, wq_cp(2)]
            for p in range(NP + 1):
                order += group_cp(p)
            xr_cp = [x_cp(b, SEM_P + NP + 1) for b in range(2, NB)]
            order += xr_cp
            for cp in order:
                cp.start()
            qkv_s[0] = jnp.zeros(qkv_s.shape[1:], U32)
            acc_s[...] = jnp.zeros(acc_s.shape, F32)
            wait('WX0', [x0_cp])
            xn0 = ln1(0, ()).astype(BF16)
            done = 0
            for i in range(3):
                wait('WQ%d' % i, [wq_cp(i)] + ([x1_cp] if i == 2 else []))
                wt_s[WQ[i] // 2:WQ[i + 1] // 2, :] = _pk(wqkv_v[:, WQ[i]:WQ[i + 1]].T)
                anchors = []
                qkv_mm(0, xn0, range(done, WQ[i + 1] // QR), anchors)
                done = WQ[i + 1] // QR
            xn1 = ln1(1, anchors[:1]).astype(BF16)
            qkv_mm(1, xn1, range(4), anchors)
            attention(0, [anchors[i] for i in cfg['att0']], 9)
            wait('WO', group_cp(0))
            wt_s[3 * RP:, :] = _pk(wo_v[...].T)
            an = []
            stats = wo_mm(0, an, False)
            qkv_mm(1, xn1, [4], an)
            for part in range(4):
                prep_gu(0, part, [an[i] for i in cfg['z_g'][part]])
            ffn_lhs(0, stats, [])
            b = gu_piece(0, cfg['order'], [], True)
            qkv_mm(1, xn1, [5], [])
            store_b(b)

            def piece(p, carry):
                wait('WP', group_cp(p))
                b_prev = load_b()
                an, t = [], ({}, {})
                acc = down_mm(load_acc(0), [b_prev], p - 1, an, D_ORDER[:6])
                for part in range(3):
                    prep_gu(p, part, [an[i] for i in cfg['p_g'][part]])
                    for i in _PARTS[part]:
                        gu_prod(p, i, t, an)
                prep_gu(p, 3, [an[i] for i in cfg['p_g'][3]])
                b = h_ops({j: gu_col(t, p, j, an, True) for j in range(3)})
                prep_d(p - 1, [an[i] for i in cfg['p_d']])
                store_acc(0, down_mm(acc, [b_prev], p - 1, an, D_ORDER[6:]))
                for i in range(2):
                    g = jnp.minimum(2 * (p - 1) + i, NT * NG - 1)
                    att_group(1, g >> 2, g & (NG - 1), an[cfg['p_att'][i]], 9)
                npat = len(cfg['p_w'])
                for i in range(npat):
                    r = jnp.minimum((p - 1) * npat + i, 4 * Q3 // 8 - 1)
                    prep_att(r, an[cfg['p_w'][i]])
                store_b(b)
                return carry

            lax.fori_loop(1, NP, piece, 0)

            wait('WD', group_cp(NP))
            an = []
            stats = wo_mm(1, an, True)
            prep_d(NP - 1, [an[i] for i in cfg['t_d']])
            acc = down_mm(load_acc(0), [load_b()], NP - 1, [])
            ffn_lhs(1, stats, [])
            finish(0, acc)
            wait('WX', xr_cp)

        if 'pre' in cfg['phases']:
            pre_phase()

        def body(u, carry):
            bu = u & (NB - 1)
            ba = (u + 1) & (NB - 1)
            acc, stats, an, b = None, None, {}, {}
            get = lambda name: [an[k][i] for k, i in cfg[name]]
            for step in cfg['body']:
                an[step] = []
                if step == 'Q':
                    qkv_fast(ba, att_rhs(ln1(ba, get('ln1'), get('ln1b'))), an[step])
                elif step == 'W':
                    attention(ba, get('att'), 9)
                    stats = wo_mm(ba, an[step], True, get('orhs'))
                elif step == 'L':
                    ffn_lhs(ba, stats, get('lhs'))
                elif step[0] == 'S':
                    t = b.setdefault(step[:2], ({}, {}))
                    for i in _PARTS[int(step[2])]:
                        gu_prod(int(step[1]), i, t, an[step])
                elif step[0] == 'F':
                    j, c = int(step[1]), int(step[2])
                    h = b.setdefault(step[:2], {})
                    h[c] = gu_col(b['S' + step[1]], j, c, an[step])
                    if len(h) == 3:
                        b[j] = h_ops(h)
                else:
                    js = [int(c) for c in step[1:]]
                    acc = down_mm(acc, [b[j] for j in js], js[0], an[step])
            finish(bu, acc)

            @pl.when(u >= NB)
            def _():
                out_copy(bu).start()
            return carry

        if scopes:
            with jax.named_scope('LOOP'):
                lax.fori_loop(1, NU - 1, body, 0)
        elif 'main' in cfg['phases']:
            lax.fori_loop(1, NU - 1, body, 0)

        def last(c, carry):
            los = [2 * c + j for j in range(2)]
            b = [gu_piece(lo, cfg['order'], []) for lo in los]
            acc = load_acc(1)
            for j in range(2):
                acc = down_mm(acc, [b[j]], los[j], [])
            store_acc(1, acc)
            return carry

        if 'last' in cfg['phases']:
            lax.fori_loop(0, NP // 2, last, 0)
        finish(NB - 1, load_acc(1))
        out_copy(NB - 1).start()
        wait('WOUT', [out_copy(b) for b in range(NB)])

    scratch = [
        pltpu.VMEM((NB, D, TM), BF16),
        pltpu.VMEM((D, 3 * D), BF16),
        pltpu.VMEM((D, D), BF16),
        pltpu.VMEM((NP, 3, D, PW), BF16),
        pltpu.VMEM((NP, 3, D, PW), BF16),
        pltpu.VMEM((NP, 3, D, PW), BF16),
        pltpu.VMEM((2 * D, D), U32),
        pltpu.VMEM((4 * Q3, 15 * LANES), U32),
        pltpu.VMEM((NP, 15, Q3, PW), U32),
        pltpu.VMEM((NP, 15, Q3, PW), U32),
        pltpu.VMEM((NP, 9, Q3, PW), U32),
        pltpu.VMEM((NB, D, TM), F32),
        pltpu.VMEM((45, TH // 2, LANES), U32),
        pltpu.VMEM((S // LANES + 1, 3 * RP, LANES), U32),
        pltpu.VMEM((NT, D, LANES), F32),
        pltpu.VMEM((2, 15, D3, TH), F32),
        pltpu.VMEM((15 * TH // 2, PW), U32),
        pltpu.SemaphoreType.DMA((SEM_P + NP + 2,)),
        pltpu.SemaphoreType.DMA((1,)),
    ]
    return kernel, scratch


_CFG = dict(
    scopes=False,
    orhs=(),
    msplit=2,
    phases=('pre', 'main', 'last'),
    order=('S0', 'S1', 'F0', 'S2', 'F1', 'F2'),
    body=('S00', 'S01', 'F00', 'S02', 'F01', 'F02', 'S10', 'S11', 'Q', 'F10', 'S12',
        'F11', 'F12', 'S20', 'S21', 'F20', 'S22', 'F22', 'F21', 'S30', 'S41', 'S31',
        'D01', 'F30', 'S32', 'F31', 'F32', 'S40', 'F40', 'S42', 'F42', 'S50', 'D23',
        'F41', 'S51', 'W', 'F50', 'S52', 'F51', 'F52', 'D4', 'L', 'D5'),
    ln1=(('S00', 0), ('S00', 1), ('S00', 2), ('S00', 3), ('S00', 4), ('S00', 5), ('S00',
        6), ('S00', 7), ('S00', 8)),
    ln1b=(('S10', 5), ('S10', 6), ('S10', 7), ('S10', 8), ('S11', 0), ('S11', 1),
        ('S11', 2), ('S11', 3), ('S11', 4), ('S11', 5), ('S11', 6), ('S11', 7)),
    att=(('S41', 0), ('D01', 0), ('D01', 5), ('D01', 6), ('D01', 9), ('D23', 4), ('D23',
        5), ('D23', 10)),
    lhs=(('D4', 7), ('D4', 9), ('D4', 14)),
    att0=(0, 1, 2, 3, 3, 4, 6, 8),
    z_g=((0,), (1,), (2,), (3, 4)),
    p_g=((0, 1), (2, 3, 4), (5, 6, 7, 8), (10, 11, 12, 13, 14, 15, 16, 17, 18, 19, 20,
        21, 22, 23, 24, 25, 26, 27)),
    t_d=(0, 1, 2, 3, 4, 5, 6, 7, 8, 9, 10, 11),
    p_d=(24, 26, 28, 30, 32, 34, 36, 38, 40, 42, 44, 46),
    p_att=(8, 52),
    p_w=(12, 15, 18, 21, 24, 27, 30, 53, 55, 57),
)


def _run(A_x, A_wqkv, A_wo, B_w_gate, B_w_up, B_w_down, **kw):
    _, S, D = A_x.shape
    F = B_w_gate.shape[1]
    kernel, scratch = _make_kernel(S, D, F, 256, {**_CFG, **kw})
    hbm = pl.BlockSpec(memory_space=pl.ANY)
    out_t = pl.pallas_call(
        kernel,
        in_specs=[hbm] * 6,
        out_specs=hbm,
        out_shape=jax.ShapeDtypeStruct((D, S), A_x.dtype),
        scratch_shapes=scratch,
        compiler_params=pltpu.CompilerParams(vmem_limit_bytes=110 * 1024 * 1024),
    )(A_x[0].T, A_wqkv, A_wo, B_w_gate, B_w_up, B_w_down.T)
    return out_t.T[None]


@jax.jit
def pallas_interleave_layers__sliding_local_dilated__glu_gated_geglu__prompt_kernel(
    A_x: jax.Array,
    A_wqkv: jax.Array,
    A_wo: jax.Array,
    B_x: jax.Array,
    B_w_gate: jax.Array,
    B_w_up: jax.Array,
    B_w_down: jax.Array,
):
    del B_x
    return _run(A_x, A_wqkv, A_wo, B_w_gate, B_w_up, B_w_down)
```

```python
import functools

import jax
import jax.numpy as jnp
import jax.experimental.pallas as pl
import jax.experimental.pallas.tpu as pltpu
from jax import lax

H = 32
W = 8
DIL = 2
EPS = 1e-5
LANES = 128

F32 = jnp.float32
BF16 = jnp.bfloat16
U32 = jnp.uint32

_NT = (((1,), (1,)), ((), ()))


def _tree_sum(parts):
    while len(parts) > 1:
        nxt = [parts[i] + parts[i + 1] for i in range(0, len(parts) - 1, 2)]
        if len(parts) % 2:
            nxt.append(parts[-1])
        parts = nxt
    return parts[0]


def _ln_stats(slabs, d, anchors=()):
    n_acc = 4
    s1, s2, pilot = [None] * n_acc, [None] * n_acc, None
    for i, x in enumerate(slabs):
        if pilot is None:
            pilot = x[0:1, :]
            pil = jnp.broadcast_to(pilot, x.shape)
            pils = [_tie(pil, a) for a in anchors] or [pil]
        dx = x - pils[i * len(pils) // (d // 8)]
        j = i % n_acc
        s1[j] = dx if s1[j] is None else s1[j] + dx
        s2[j] = dx * dx if s2[j] is None else s2[j] + dx * dx
    e1 = jnp.sum(_tree_sum(s1), axis=0, keepdims=True) * (1.0 / d)
    e2 = jnp.sum(_tree_sum(s2), axis=0, keepdims=True) * (1.0 / d)
    var = jnp.maximum(e2 - e1 * e1, 0.0)
    return pilot + e1, lax.rsqrt(var + EPS)


def _zero_like_dep(v):
    return (lax.bitcast_convert_type(v, U32) >> 31) >> 1


def _tie(x, anchor):
    if anchor is None:
        return x
    z = lax.bitcast_convert_type(_zero_like_dep(anchor), F32)
    z = jnp.concatenate([z] * (x.shape[1] // LANES), axis=1)
    if x.shape[0] == 8:
        return x + z
    return jnp.concatenate([x[:8] + z, x[8:]], axis=0)


def _gelu_mul2(g, u):
    c0 = 0.7978845608028654
    c1 = c0 * 0.044715
    t = jnp.tanh(g * (c0 + c1 * (g * g)))
    return (g * u) * (1.0 + t)


def _lo(x):
    return lax.bitcast_convert_type(x << 16, F32)


def _hi(x):
    return lax.bitcast_convert_type(x & jnp.uint32(0xFFFF0000), F32)


def _pk(x):
    return pltpu.bitcast(x.astype(BF16), U32)


def _upk(x):
    return pltpu.bitcast(x, BF16)


def _dot(a, b):
    return jnp.dot(a, b, preferred_element_type=F32)


def _dot_nt(a, b):
    return lax.dot_general(a, b, _NT, preferred_element_type=F32)


def _x_ops(x1, x2):
    d = [a - b for a, b in zip(x1, x2)]
    return [x1[0] + x2[1], x2[0] + x2[1], x1[0] + x1[1],
            d[1] + x1[2], x1[1] + x1[2], d[1] + d[2],
            d[0] - x2[2], d[0] + d[2], x2[0] + x2[2],
            x1[0], d[0], x2[1], d[1], x1[2], x2[2]]


def _x_rem(x1, x2):
    a, b, c = 0, 1, 2
    cat = lambda u, v: jnp.concatenate([u, v], axis=0)
    return [cat(x1[c], x2[b]), cat(x1[a], x1[b] - x2[b]), cat(x2[a], x2[c] - x1[c])]


def _w_sums(w):
    return [w[0][1] + w[1][0], w[1][2] + w[2][1], w[0][2] + w[2][0],
            w[0][0] + w[0][2] - w[1][0], w[2][0] - w[0][0] - w[0][1],
            w[1][1] + w[1][2] - w[0][1], w[1][0] + w[1][1] - w[2][1],
            w[2][0] + w[2][2] - w[1][2], w[2][1] + w[2][2] - w[0][2]]


_W_TERMS = {0: ((0, 1, 1), (1, 0, 1)), 3: ((1, 2, 1), (2, 1, 1)), 6: ((0, 2, 1), (2, 0, 1)),
            9: ((0, 0, 1), (0, 2, 1), (1, 0, -1)), 10: ((2, 0, 1), (0, 0, -1), (0, 1, -1)),
            11: ((1, 1, 1), (1, 2, 1), (0, 1, -1)), 12: ((1, 0, 1), (1, 1, 1), (2, 1, -1)),
            13: ((2, 0, 1), (2, 2, 1), (1, 2, -1)), 14: ((2, 1, 1), (2, 2, 1), (0, 2, -1)),
            1: ((0, 1, 1),), 2: ((1, 0, 1),), 4: ((1, 2, 1),), 5: ((2, 1, 1),),
            7: ((2, 0, 1),), 8: ((0, 2, 1),)}
_PARTS = ((1, 2, 0), (7, 8, 6), (4, 5, 3), (9, 10, 11, 12, 13, 14))
_W_SUM = {0: 0, 3: 1, 6: 2, 9: 3, 10: 4, 11: 5, 12: 6, 13: 7, 14: 8}
_W_RAW = {1: (0, 1), 2: (1, 0), 4: (1, 2), 5: (2, 1), 7: (2, 0), 8: (0, 2)}
_PAIR_ORDER = (1, 2, 4, 5, 7, 8, 0, 3, 6)
_DIAG = {(0, 0): 9, (2, 0): 10, (0, 1): 11, (1, 1): 12, (1, 2): 13, (2, 2): 14}
_PAIR = {(0, 0): ((6, -1), (8, -1)), (1, 0): ((2, 1), (7, 1)), (2, 0): ((0, 1), (1, -1)),
         (0, 1): ((3, 1), (4, -1)), (1, 1): ((0, 1), (2, -1)), (2, 1): ((1, 1), (5, -1)),
         (0, 2): ((4, 1), (8, 1)), (1, 2): ((6, 1), (7, -1)), (2, 2): ((5, 1), (3, -1))}


def _column(t, base, j):
    s = []
    for k in range(3):
        v = base[k]
        for i, sg in _PAIR[k, j]:
            v = t[i] if v is None else (v + t[i] if sg > 0 else v - t[i])
        s.append(v)
    return s[1] + s[0], s[2] + s[0]


def _make_kernel(S, D, F, TM, cfg):
    NB = S // TM
    NT = TM // LANES
    DH = D // H
    DP = DH // 2
    RP = D // 2
    NG = H // 8
    scale = float(DH) ** -0.5
    NU = 2 * NB
    TH = TM // 2
    FT = F // 3
    D2 = D // 2
    D3 = D // 3
    Q3 = D3 // 2
    KU = D // 9
    KR = 3 * LANES
    NQ = 6
    QR = 3 * D // NQ
    WQ = (0, 640, 1152, 3 * D)
    PW = 256
    NP = FT // PW
    scopes = cfg['scopes']
    assert NG == 4 and NB & (NB - 1) == 0
    SEM_P = 4

    def kernel(x_hbm, wqkv_hbm, wo_hbm, wg_hbm, wu_hbm, wdt_hbm, out_hbm,
               xio_s, wqkv_v, wo_v, wg_v, wu_v, wdt_v, wt_s, wl_s,
               gs_s, us_s, ds_s, xmid_s, a_s, qkv_s, o_s, acc_s, b_s,
               sem_i, sem_o):

        def wait(name, cps):
            if scopes:
                with jax.named_scope(name):
                    for cp in cps:
                        cp.wait()
            else:
                for cp in cps:
                    cp.wait()

        def cols(lo, n):
            if not isinstance(lo, int):
                lo = pl.multiple_of(lo, LANES)
            return pl.ds(lo, n)

        def rows8(lo, n=8):
            if not isinstance(lo, int):
                lo = pl.multiple_of(lo, 8)
            return pl.ds(lo, n)

        def out_copy(b):
            return pltpu.make_async_copy(
                xio_s.at[b], out_hbm.at[:, cols(b * TM, TM)], sem_o.at[0])

        def x_cp(b, sem):
            return pltpu.make_async_copy(x_hbm.at[:, cols(b * TM, TM)], xio_s.at[b],
                                         sem_i.at[sem])

        def wq_cp(i):
            sl = cols(WQ[i], WQ[i + 1] - WQ[i])
            return pltpu.make_async_copy(wqkv_hbm.at[:, sl], wqkv_v.at[:, sl],
                                         sem_i.at[1 + i])

        def piece_cp(src, dst, p, sem):
            return [pltpu.make_async_copy(src.at[:, cols(j * FT + p * PW, PW)],
                                          dst.at[p, j],
                                          sem_i.at[sem]) for j in range(3)]

        def group_cp(p):
            sem = SEM_P + p
            cps = []
            if isinstance(p, int) and p == 0:
                cps.append(pltpu.make_async_copy(wo_hbm, wo_v, sem_i.at[sem]))
            if not (isinstance(p, int) and p == NP):
                cps += piece_cp(wg_hbm, wg_v, p, sem) + piece_cp(wu_hbm, wu_v, p, sem)
            if not (isinstance(p, int) and p == 0):
                cps += piece_cp(wdt_hbm, wdt_v, p - 1, sem)
            return cps

        lane = lax.broadcasted_iota(jnp.int32, (8, LANES), 1)
        cat0 = lambda *v: jnp.concatenate(v, axis=0)
        cat1 = lambda *v: jnp.concatenate(v, axis=1)

        def spread_over(anchors, n, total):
            return anchors[n * len(anchors) // total] if anchors else None

        def slab_group(r):
            return (r % LANES) // 16 if r < KR else 8 + ((r - KR) % KU) // 16

        def ln1(blk, anchors1, anchors2=()):
            slabs = (xio_s[blk, r:r + 8, :].astype(F32) for r in range(0, D, 8))
            m, rs = _ln_stats(slabs, D, anchors1)
            if not anchors2:
                return (xio_s[blk].astype(F32) - m) * rs
            m8 = jnp.broadcast_to(m, (8, TM))
            ms = [_tie(m8, a) for a in anchors2]
            ms = [spread_over(ms, slab_group(r), 12) for r in range(0, D, 8)]
            return (xio_s[blk].astype(F32) - cat0(*ms)) * rs

        def dot_k(rows, x, anchors):
            y = None
            for n, k in enumerate(range(0, D, LANES)):
                ks = slice(k, min(k + LANES, D))
                v = _dot(_upk(wt_s[rows, ks]), x[ks])
                anchors.extend(v[r:r + 8, :LANES] for r in ((0, 144) if n % 2 else (72, 216)))
                y = v if y is None else y + v
            return y

        def put_qkv(blk, rows, y):
            pk = _pk(y)
            for c in range(NT):
                qkv_s[1 + blk * NT + c, rows, :] = pk[:, c * LANES:(c + 1) * LANES]

        def qkv_mm(blk, xn, chunks, anchors):
            for r in chunks:
                rows = slice(r * QR // 2, (r + 1) * QR // 2)
                put_qkv(blk, rows, dot_k(rows, xn, anchors))

        def split_k(x):
            hs = (x[:, :TH], x[:, TH:])
            blocks = [[h[k * LANES:(k + 1) * LANES] for k in range(3)] for h in hs]
            units = [[h[KR + k * KU:KR + (k + 1) * KU] for k in range(3)] for h in hs]
            return blocks, units

        def prep_att(pat, anchor):
            assert Q3 == 96
            row0 = pat * 8
            src0 = row0 + ((pat * 43) >> 9) * (2 * Q3)
            w = [_upk(wt_s[rows8(src0 + j * Q3), :]).astype(F32) for j in range(3)]
            w[0] = cat1(_tie(w[0][:, :LANES], anchor), w[0][:, LANES:])
            tiles = _w_sums([[w[j][:, k * LANES:(k + 1) * LANES] for j in range(3)]
                             for k in range(3)])
            for j in range(3):
                a, b, c = (w[j][:, KR + k * KU:KR + (k + 1) * KU] for k in range(3))
                tiles += [cat1(c, b), cat1(a, c)]
            wl_s[rows8(row0), :] = _pk(cat1(*tiles))

        def att_rhs(x):
            blocks, units = split_k(x)
            return [v.astype(BF16) for v in _x_ops(*blocks) + _x_rem(*units)]

        def att_mm(sec, rhs, anchors):
            tl = lambda i: _upk(wl_s[sec * Q3:(sec + 1) * Q3, i * LANES:(i + 1) * LANES])
            raw = lambda k, j: _upk(wt_s[(3 * sec + j) * Q3:(3 * sec + j + 1) * Q3,
                                         k * LANES:(k + 1) * LANES])
            t = {}
            for i in _PAIR_ORDER:
                t[i] = _dot(raw(*_W_RAW[i]) if i in _W_RAW else tl(_W_SUM[i]), rhs[i])
                anchors.append(t[i][:8])
            out = []
            for j in range(3):
                base = []
                for s in range(3):
                    v = _dot(raw(3, j) if s == 1 else tl(9 + 2 * j + s // 2), rhs[15 + s])
                    if (s, j) in _DIAG:
                        i = _DIAG[s, j]
                        v = _dot(tl(_W_SUM[i]), rhs[i]) + v
                    base.append(v)
                    anchors.append(base[-1][:8])
                out.append(cat1(*_column(t, base, j)))
            return cat0(*out)

        def qkv_fast(blk, rhs, anchors):
            for sec in range(3):
                put_qkv(blk, slice(sec * RP, (sec + 1) * RP), att_mm(sec, rhs, anchors))

        def shifted(ln, cur, prev, w):
            if w == 0:
                return cur
            sh = DIL * w
            return pltpu.roll(jnp.where(ln < LANES - sh, cur, prev), sh, axis=1)

        def att_group(blk, c, hg, anchor, win):
            tile = blk * NT + c
            base = hg * 8 * DP
            if isinstance(hg, int):
                cur, prev, o_t = qkv_s.at[1 + tile], qkv_s.at[tile], o_s.at[c]
                obase = hg * 8 * DH
            else:
                n = 2 * RP + 8 * DP
                base = pl.multiple_of(base, 8)
                cur = qkv_s.at[1 + tile, pl.ds(base, n)]
                prev = qkv_s.at[tile, pl.ds(base, n)]
                o_t = o_s.at[c, pl.ds(pl.multiple_of(hg * 8 * DH, 8), 8 * DH)]
                base, obase = 0, 0
            ln = lane + _zero_like_dep(anchor).astype(jnp.int32)
            logits = [None] * W
            done = []
            for dd in range(DP):
                q = cur[pl.ds(base + dd, 8, stride=DP), :]
                kc = cur[pl.ds(RP + base + dd, 8, stride=DP), :]
                if dd >= win:
                    kc = kc | _zero_like_dep(done[dd - win])
                kp = prev[pl.ds(RP + base + dd, 8, stride=DP), :]
                q0, q1 = _lo(q), _hi(q)
                for w in range(W):
                    ks = shifted(ln, kc, kp, w)
                    t = q0 * _lo(ks) + q1 * _hi(ks)
                    logits[w] = t if logits[w] is None else logits[w] + t
                done.append(ks)
            logits = [l * scale for l in logits]
            if not (isinstance(c, int) and c > 0):
                pos = lane + tile * LANES
                logits = [l if w == 0 else jnp.where(pos >= DIL * w, l, -1e9)
                          for w, l in enumerate(logits)]
            m = functools.reduce(jnp.maximum, logits)
            ln = lane + _zero_like_dep(m).astype(jnp.int32)
            e = [jnp.exp(l - m) for l in logits]
            r = 1.0 / functools.reduce(lambda a, b: a + b, e)
            p = [x * r for x in e]
            done = []
            for dd in range(DP):
                vc = cur[pl.ds(2 * RP + base + dd, 8, stride=DP), :]
                if dd >= win:
                    vc = vc | _zero_like_dep(done[dd - win])
                vp = prev[pl.ds(2 * RP + base + dd, 8, stride=DP), :]
                o0 = o1 = None
                for w in range(W):
                    vs = shifted(ln, vc, vp, w)
                    t0, t1 = p[w] * _lo(vs), p[w] * _hi(vs)
                    o0 = t0 if o0 is None else o0 + t0
                    o1 = t1 if o1 is None else o1 + t1
                done.append(vs)
                o_t[pl.ds(obase + 2 * dd, 8, stride=DH), :] = o0
                o_t[pl.ds(obase + 2 * dd + 1, 8, stride=DH), :] = o1

        def attention(blk, anchors, win):
            for c in range(NT):
                for hg in range(NG):
                    att_group(blk, c, hg, anchors[c * NG + hg], win)

        def wo_mm(blk, anchors, fast, anchors_in=()):
            o = cat1(*[o_s[c] for c in range(NT)])
            if anchors_in:
                o = cat0(*[_tie(o[r:r + 8], spread_over(anchors_in, slab_group(r), 12))
                           for r in range(0, D, 8)])
            if fast:
                y = att_mm(3, att_rhs(o), anchors)
            else:
                o = o.astype(BF16)
                q = D2 // 2
                y = cat0(*[dot_k(slice(h * q, (h + 1) * q), o, anchors) for h in (6, 7)])
            xm = xio_s[blk].astype(F32) + y
            xmid_s[blk] = xm
            return _ln_stats((xm[r:r + 8] for r in range(0, D, 8)), D)

        def ffn_lhs(blk, stats, anchors):
            m, rs = stats
            m8 = jnp.broadcast_to(m, (8, TM))
            xs = []
            for k in range(3):
                mt = cat0(*[_tie(m8, spread_over(anchors, k, 3))] * (D3 // 8))
                xs.append((xmid_s[blk, k * D3:(k + 1) * D3, :] - mt) * rs)
            ops = _x_ops([x[:, :TH] for x in xs], [x[:, TH:] for x in xs])
            for i, v in enumerate(ops):
                for s, t in enumerate((v[KU:], v[:2 * KU], cat0(v[:KU], v[2 * KU:]))):
                    a_s[3 * i + s] = _pk(t.astype(BF16).T)

        def plain_lhs(blk, stats):
            m, rs = stats
            blocks, units = split_k((xmid_s[blk] - m) * rs)
            for i, v in enumerate(blocks[0] + blocks[1] + _x_rem(*units)):
                a_s[i] = _pk(v.astype(BF16).T)

        def plain_piece(p, anchors):
            h = {}
            for j in range(3):
                hs = []
                for n in range(PW // LANES):
                    cs = slice(n * LANES, (n + 1) * LANES)
                    w = lambda r0, r1: cat1(wg_v[p, j, r0:r1, cs], wu_v[p, j, r0:r1, cs])
                    u = lambda k: w(KR + k * KU, KR + (k + 1) * KU)
                    tl = lambda *i: _upk(cat1(*[a_s[k] for k in i]))
                    y0 = _dot(tl(6), cat0(u(2), u(1)))
                    y1 = _dot(tl(0, 1, 2, 7), w(0, KR + 2 * KU))
                    y2 = _dot(tl(3, 4, 5, 8), cat0(w(0, KR + KU), u(2)))
                    for y in (y0, y1, y2):
                        anchors.extend(y[r:r + 8, c:c + LANES]
                                       for c in ((0,) if y is y0 else (0, LANES))
                                       for r in ((0,) if y is y0 else (0, TH // 2)))
                    hs.append([_gelu_mul2(*[(y + y0)[:, c:c + LANES] for c in (0, LANES)])
                               for y in (y1, y2)])
                h[j] = [cat1(*[v[i] for v in hs]) for i in range(2)]
            return h_ops(h)

        def prep_d(p, anchors):
            PR = 16
            for n in range(2 * D3 // PR):
                r, cs = (n // 2) * PR, slice((n % 2) * LANES, (n % 2 + 1) * LANES)
                w = [[wdt_v[p, k, j * D3 + r:j * D3 + r + PR, cs].astype(F32)
                      for j in range(3)] for k in range(3)]
                w[0][1] = _tie(w[0][1], spread_over(anchors, n, 2 * D3 // PR))
                for i, v in enumerate(_w_sums(w)):
                    ds_s.at[p, i][r // 2:(r + PR) // 2, cs] = _pk(v)

        GU = ((wg_v, gs_s), (wu_v, us_s))

        def prep_gu(p, anchors):
            PR = 16
            nr = D3 // PR
            for n in range(4 * nr):
                c, (w_v, s_s), r = n % 2, GU[(n // 2) % 2], (n // 4) * PR
                cache = {}

                def w(k, j):
                    if (k, j) not in cache:
                        ld = lambda c: w_v[p, j, k * D3 + r:k * D3 + r + PR,
                                           c * LANES:(c + 1) * LANES].astype(F32)
                        v = ld(c)
                        if k != j:
                            v = _tie(v, spread_over(anchors, n, 4 * nr))
                        cache[k, j] = v - ld(1 - c) if r // KU == 1 + c else v
                    return cache[k, j]

                for i in range(15):
                    v = None
                    for k, j, sg in _W_TERMS[i]:
                        v = w(k, j) if v is None else (v + w(k, j) if sg > 0 else v - w(k, j))
                    s_s.at[p, i][r // 2:(r + PR) // 2, c * LANES:(c + 1) * LANES] = _pk(v)

        def gu_prod(p, i, t, anchors, even=False):
            u = KU // 2

            def rhs(s, s_s):
                if s == 1:
                    return s_s[p, i, :2 * u, :LANES]
                if s == 0:
                    return cat0(s_s[p, i, u:2 * u, LANES:], s_s[p, i, 2 * u:, :LANES])
                return cat0(s_s[p, i, :u, LANES:], s_s[p, i, 2 * u:, LANES:])

            ns = cfg['msplit']
            q = TH // 2 // ns
            y1, y2 = [], []
            for h in range(ns):
                y = []
                for s in range(3):
                    r = _upk(cat1(rhs(s, gs_s), rhs(s, us_s)))
                    if even and s == 2 and ns == 1:
                        y.append(cat0(*[_dot(_upk(a_s[3 * i + s, k * q // 2:(k + 1) * q // 2]), r)
                                        for k in range(2)]))
                    else:
                        y.append(_dot(_upk(a_s[3 * i + s, h * q:(h + 1) * q]), r))
                    if (3 * h + s) % ns == 0:
                        anchors.append(y[-1][:8, :LANES])
                y1.append(y[1] + y[0])
                y2.append(y[2] + y[0])
            y1, y2 = cat0(*y1), cat0(*y2)
            for m in range(2):
                cs = slice(m * LANES, (m + 1) * LANES)
                t[m][i] = cat1(y1[:, cs], y2[:, cs])

        def gu_col(t, p, j, anchors, even=False):
            ids = [_DIAG.get((s, j)) for s in range(3)]
            for i in ids:
                if i is not None:
                    gu_prod(p, i, t, anchors, even and i == 14)
            g, u = [_column(t[m], [None if i is None else t[m][i] for i in ids], j)
                    for m in range(2)]
            return [_gelu_mul2(g[i], u[i]) for i in range(2)]

        def h_ops(h):
            return [v.astype(BF16) for v in _x_ops(*[[h[j][i] for j in range(3)]
                                                     for i in range(2)])]

        def gu_piece(p, order, anchors, even=False):
            t, h = ({}, {}), {}
            for step in order:
                if step[0] == 'S':
                    for i in _PARTS[int(step[1])]:
                        gu_prod(p, i, t, anchors)
                else:
                    h[int(step[1])] = gu_col(t, p, int(step[1]), anchors, even)
            return h_ops(h)

        D_ORDER = _PAIR_ORDER + (9, 10, 11, 12, 13, 14)

        def down_mm(acc, bs, lo, anchors, which=D_ORDER, fine=False):
            p = [None] * 15 if acc is None else list(acc)
            for i in which:
                y = None
                for n, b in enumerate(bs):
                    if i in _W_RAW:
                        k, j = _W_RAW[i]
                        v = _dot_nt(wdt_v[lo + n, k, j * D3:(j + 1) * D3, :], b[i])
                    elif len(bs) % 2 and i == 14 and n == 0:
                        v = cat0(*[_dot_nt(_upk(ds_s[lo, _W_SUM[i],
                                                     h * Q3 // 2:(h + 1) * Q3 // 2, :]), b[i])
                                   for h in range(2)])
                    else:
                        v = _dot_nt(_upk(ds_s[lo + n, _W_SUM[i]]), b[i])
                    y = v if y is None else y + v
                p[i] = y if p[i] is None else p[i] + y
                anchors.append(p[i][:8])
                if fine:
                    anchors.append(p[i][D3 // 2:D3 // 2 + 8])
            return p

        def finish(blk, acc):
            y = [cat1(*_column(acc, [acc[_DIAG[s, j]] if (s, j) in _DIAG else None
                                     for s in range(3)], j)) for j in range(3)]
            xio_s[blk] = (xmid_s[blk] + 0.5 * cat0(*y)).astype(BF16)

        def load_acc(k):
            return [acc_s[k, i] for i in range(15)]

        def store_acc(k, acc):
            for i in range(15):
                acc_s[k, i] = acc[i]

        def load_b():
            return [_upk(b_s[i * TH // 2:(i + 1) * TH // 2, :]) for i in range(15)]

        def store_b(b):
            for i in range(15):
                b_s[i * TH // 2:(i + 1) * TH // 2, :] = _pk(b[i])

        def pre_phase():
            x0_cp, x1_cp = x_cp(0, 0), x_cp(1, 3)
            order = [x0_cp, wq_cp(0), wq_cp(1), x1_cp, wq_cp(2)]
            for p in range(NP + 1):
                order += group_cp(p)
            xr_cp = [x_cp(b, SEM_P + NP + 1) for b in range(2, NB)]
            order += xr_cp
            for cp in order:
                cp.start()
            get = lambda an, name: [an[min(i, len(an) - 1)] for i in cfg[name]]
            e_grp = lambda e: ((e >> 1) & 1, ((e >> 2) << 1) | (e & 1))
            if 'a' in cfg['sub']:
                pre_a(x0_cp, x1_cp, get, e_grp)
            if 'b' in cfg['sub']:
                pre_b(get, e_grp)
            if 'c' in cfg['sub']:
                pre_c(get)
            wait('WX', xr_cp)

        def pre_a(x0_cp, x1_cp, get, e_grp):
            qkv_s[0] = jnp.zeros(qkv_s.shape[1:], U32)
            acc_s[...] = jnp.zeros(acc_s.shape, F32)
            wait('WX0', [x0_cp])
            xn0 = ln1(0, ()).astype(BF16)
            done = 0
            for i in range(3):
                wait('WQ%d' % i, [wq_cp(i)] + ([x1_cp] if i == 2 else []))
                wt = _pk(wqkv_v[:, WQ[i]:WQ[i + 1]].T)
                wt_s[WQ[i] // 2:WQ[i + 1] // 2, :] = wt
                anchors = []
                qkv_mm(0, xn0, range(done, WQ[i + 1] // QR), anchors)
                done = WQ[i + 1] // QR
                if i > 0:
                    for n, a in enumerate(get(anchors, 'a_w%d' % i)):
                        prep_att(12 * (i - 1) + n, a)
            xn1 = ln1(1, get(anchors, 'a_ln'), get(anchors, 'a_lnb')).astype(BF16)
            qkv_mm(1, xn1, (0, 2, 4, 1), anchors)
            for e in range(8):
                att_group(0, *e_grp(e), anchors[cfg['att0'][e]], 9)
            wait('WO', group_cp(0))
            wt = _pk(wo_v[...].T)
            wt_s[3 * RP:, :] = wt
            an = []
            stats = wo_mm(0, an, False)
            qkv_mm(1, xn1, [3], an)
            plain_lhs(0, stats)
            b = plain_piece(0, an)
            qkv_mm(1, xn1, [5], an)
            prep_gu(0, get(an, 'z_g'))
            for e in range(3):
                att_group(1, *e_grp(e), an[cfg['z_att'][e]], 9)
            store_b(b)

        def pre_b(get, e_grp):
            def piece(p, carry):
                wait('WP', group_cp(p))
                b_prev = load_b()
                an = []
                b = plain_piece(p, an)
                prep_d(p - 1, get(an, 'p_d'))
                store_acc(0, down_mm(load_acc(0), [b_prev], p - 1, an))
                prep_gu(p, get(an, 'p_g'))
                att_group(1, *e_grp(p + 2), an[cfg['p_att'][0]], 9)
                for i, a in enumerate(get(an, 'p_w')):
                    prep_att(jnp.minimum(24 + (p - 1) * 5 + i, 47), a)
                store_b(b)
                return carry

            lax.fori_loop(1, NP, piece, 0)

        def pre_c(get):
            wait('WD', group_cp(NP))
            an = []
            stats = wo_mm(1, an, True)
            prep_d(NP - 1, get(an, 't_d'))
            acc = down_mm(load_acc(0), [load_b()], NP - 1, [])
            ffn_lhs(1, stats, [])
            finish(0, acc)

        if 'pre' in cfg['phases']:
            pre_phase()

        def body(u, carry):
            bu = u & (NB - 1)
            ba = (u + 1) & (NB - 1)
            acc, stats, an, b = None, None, {}, {}
            get = lambda name: [an[k][i] for k, i in cfg[name]]
            for step in cfg['body']:
                an[step] = []
                if step == 'Q':
                    qkv_fast(ba, att_rhs(ln1(ba, get('ln1'), get('ln1b'))), an[step])
                elif step == 'W':
                    attention(ba, get('att'), 9)
                    stats = wo_mm(ba, an[step], True, get('orhs'))
                elif step == 'L':
                    ffn_lhs(ba, stats, get('lhs'))
                elif step[0] == 'S':
                    t = b.setdefault(step[:2], ({}, {}))
                    for i in _PARTS[int(step[2])]:
                        gu_prod(int(step[1]), i, t, an[step])
                elif step[0] == 'F':
                    j, c = int(step[1]), int(step[2])
                    h = b.setdefault(step[:2], {})
                    h[c] = gu_col(b['S' + step[1]], j, c, an[step])
                    if len(h) == 3:
                        b[j] = h_ops(h)
                else:
                    js = [int(c) for c in step[1:]]
                    acc = down_mm(acc, [b[j] for j in js], js[0], an[step])
            finish(bu, acc)

            @pl.when(u >= NB)
            def _():
                out_copy(bu).start()
            return carry

        if scopes:
            with jax.named_scope('LOOP'):
                lax.fori_loop(1, NU - 1, body, 0)
        elif 'main' in cfg['phases']:
            lax.fori_loop(1, NU - 1, body, 0)

        def last(c, carry):
            los = [2 * c + j for j in range(2)]
            b = [gu_piece(lo, cfg['order'], []) for lo in los]
            acc = load_acc(1)
            for j in range(2):
                acc = down_mm(acc, [b[j]], los[j], [])
            store_acc(1, acc)
            return carry

        if 'last' in cfg['phases']:
            lax.fori_loop(0, NP // 2, last, 0)
        if len(cfg['phases']) < 3:
            def keep(i, c):
                v = (gs_s[i, i, :8, :LANES] + us_s[i, i, :8, :LANES] + ds_s[i, i, :8, :LANES]
                     + wl_s[rows8(i * 8), :LANES] + a_s[i, :8] + qkv_s[i, :8]
                     + b_s[rows8(i * 8), :LANES] + wt_s[rows8(i * 8), :LANES])
                acc_s[1, 0, :8] = (lax.bitcast_convert_type(v, F32) + o_s[i, :8]
                                   + acc_s[i, i, :8])
                return c
            lax.fori_loop(0, 2, keep, 0)
        finish(NB - 1, load_acc(1))
        out_copy(NB - 1).start()
        wait('WOUT', [out_copy(b) for b in range(NB)])

    scratch = [
        pltpu.VMEM((NB, D, TM), BF16),
        pltpu.VMEM((D, 3 * D), BF16),
        pltpu.VMEM((D, D), BF16),
        pltpu.VMEM((NP, 3, D, PW), BF16),
        pltpu.VMEM((NP, 3, D, PW), BF16),
        pltpu.VMEM((NP, 3, D, PW), BF16),
        pltpu.VMEM((2 * D, D), U32),
        pltpu.VMEM((4 * Q3, 15 * LANES), U32),
        pltpu.VMEM((NP, 15, Q3, PW), U32),
        pltpu.VMEM((NP, 15, Q3, PW), U32),
        pltpu.VMEM((NP, 9, Q3, PW), U32),
        pltpu.VMEM((NB, D, TM), F32),
        pltpu.VMEM((45, TH // 2, LANES), U32),
        pltpu.VMEM((S // LANES + 1, 3 * RP, LANES), U32),
        pltpu.VMEM((NT, D, LANES), F32),
        pltpu.VMEM((2, 15, D3, TH), F32),
        pltpu.VMEM((15 * TH // 2, PW), U32),
        pltpu.SemaphoreType.DMA((SEM_P + NP + 2,)),
        pltpu.SemaphoreType.DMA((1,)),
    ]
    return kernel, scratch


_CFG = dict(
    scopes=False,
    sub='abc',
    orhs=(),
    msplit=2,
    phases=('pre', 'main', 'last'),
    order=('S0', 'S1', 'F0', 'S2', 'F1', 'F2'),
    body=('S00', 'S01', 'F00', 'S02', 'F01', 'F02', 'S10', 'S11', 'Q', 'F10', 'S12',
        'F11', 'F12', 'S20', 'S21', 'F20', 'S22', 'F22', 'F21', 'S30', 'S41', 'S31',
        'D01', 'F30', 'S32', 'F31', 'F32', 'S40', 'F40', 'S42', 'F42', 'S50', 'D23',
        'F41', 'S51', 'W', 'F50', 'S52', 'F51', 'F52', 'D4', 'L', 'D5'),
    ln1=(('S00', 0), ('S00', 1), ('S00', 2), ('S00', 3), ('S00', 4), ('S00', 5), ('S00',
        6), ('S00', 7), ('S00', 8)),
    ln1b=(('S10', 5), ('S10', 6), ('S10', 7), ('S10', 8), ('S11', 0), ('S11', 1),
        ('S11', 2), ('S11', 3), ('S11', 4), ('S11', 5), ('S11', 6), ('S11', 7)),
    att=(('S41', 0), ('D01', 0), ('D01', 5), ('D01', 6), ('D01', 9), ('D23', 4), ('D23',
        5), ('D23', 10)),
    lhs=(('D4', 7), ('D4', 9), ('D4', 14)),
    att0=(15, 18, 21, 24, 27, 30, 33, 37),
    order0=('S0', 'S1', 'S2', 'F0', 'F1', 'F2'),
    order1=('S0', 'S1', 'S2', 'F0', 'F1', 'F2'),
    a_w1=(0, 1, 2, 3, 5, 5, 8, 9, 10, 11, 12, 14),
    a_w2=(0, 0, 2, 3, 4, 4, 6, 6, 8, 9, 11, 16),
    a_ln=(0, 3, 7),
    a_lnb=(6, 6, 8),
    z_g=(3, 4, 5, 6, 8, 9, 10, 12, 13, 14, 15, 17, 18, 19, 21, 22, 23, 25, 26, 27, 28,
        30, 31, 32, 34, 35, 36, 38, 39, 40, 41, 43, 44, 45, 47, 48, 49, 51, 52, 53, 54,
        56, 57, 58, 60, 61, 62, 64),
    z_att=(72, 75, 78),
    p_g0=(0, 1, 2, 3, 4, 5),
    p_g1=(6, 7, 8, 9, 10, 10),
    p_g2=(12, 13, 14, 15, 16, 17),
    p_g3=(14, 16, 18, 20, 22, 24, 26, 28, 30, 32, 34, 36),
    t_d=(0, 0, 1, 1, 2, 3, 3, 4, 5, 6, 6, 7, 8, 9, 9, 9, 10, 11, 11, 12, 13, 14, 15,
        16),
    p_d=(0, 2, 6, 8, 10, 12, 14, 16, 18, 20, 22, 24, 26, 28, 30, 32, 34, 36, 38, 40, 40,
        42, 44, 46),
    p_att=(52,),
    p_w=(10, 19, 30, 44, 48),
    p_g=(0, 1, 2, 3, 4, 5, 6, 7, 9, 10, 11, 12, 13, 14, 15, 16, 18, 19, 20, 21, 22, 23,
        24, 25, 27, 28, 29, 30, 31, 32, 33, 34, 36, 37, 38, 39, 40, 41, 42, 43, 45, 46,
        47, 48, 49, 50, 51, 53),
)


def _run(A_x, A_wqkv, A_wo, B_w_gate, B_w_up, B_w_down, **kw):
    _, S, D = A_x.shape
    F = B_w_gate.shape[1]
    kernel, scratch = _make_kernel(S, D, F, 256, {**_CFG, **kw})
    hbm = pl.BlockSpec(memory_space=pl.ANY)
    out_t = pl.pallas_call(
        kernel,
        in_specs=[hbm] * 6,
        out_specs=hbm,
        out_shape=jax.ShapeDtypeStruct((D, S), A_x.dtype),
        scratch_shapes=scratch,
        compiler_params=pltpu.CompilerParams(vmem_limit_bytes=110 * 1024 * 1024),
    )(A_x[0].T, A_wqkv, A_wo, B_w_gate, B_w_up, B_w_down.T)
    return out_t.T[None]


@jax.jit
def pallas_interleave_layers__sliding_local_dilated__glu_gated_geglu__prompt_kernel(
    A_x: jax.Array,
    A_wqkv: jax.Array,
    A_wo: jax.Array,
    B_x: jax.Array,
    B_w_gate: jax.Array,
    B_w_up: jax.Array,
    B_w_down: jax.Array,
):
    del B_x
    return _run(A_x, A_wqkv, A_wo, B_w_gate, B_w_up, B_w_down)
```

```python
import functools

import jax
import jax.numpy as jnp
import jax.experimental.pallas as pl
import jax.experimental.pallas.tpu as pltpu
from jax import lax

H = 32
W = 8
DIL = 2
EPS = 1e-5
LANES = 128

F32 = jnp.float32
BF16 = jnp.bfloat16
U32 = jnp.uint32

_NT = (((1,), (1,)), ((), ()))


def _tree_sum(parts, op=jnp.add):
    while len(parts) > 1:
        nxt = [op(parts[i], parts[i + 1]) for i in range(0, len(parts) - 1, 2)]
        if len(parts) % 2:
            nxt.append(parts[-1])
        parts = nxt
    return parts[0]


def _ln_stats(slabs, d, anchors=()):
    n_acc = 4
    s1, s2, pilot = [None] * n_acc, [None] * n_acc, None
    for i, x in enumerate(slabs):
        if pilot is None:
            pilot = x[0:1, :]
            pil = jnp.broadcast_to(pilot, x.shape)
            pils = [_tie(pil, a) for a in anchors] or [pil]
        dx = x - pils[i * len(pils) // (d // 8)]
        j = i % n_acc
        s1[j] = dx if s1[j] is None else s1[j] + dx
        s2[j] = dx * dx if s2[j] is None else s2[j] + dx * dx
    e1 = jnp.sum(_tree_sum(s1), axis=0, keepdims=True) * (1.0 / d)
    e2 = jnp.sum(_tree_sum(s2), axis=0, keepdims=True) * (1.0 / d)
    var = jnp.maximum(e2 - e1 * e1, 0.0)
    return pilot + e1, lax.rsqrt(var + EPS)


def _zero_like_dep(v):
    return (lax.bitcast_convert_type(v, U32) >> 31) >> 1


def _tie(x, anchor):
    if anchor is None:
        return x
    z = lax.bitcast_convert_type(_zero_like_dep(anchor), F32)
    z = jnp.concatenate([z] * (x.shape[1] // LANES), axis=1)
    if x.shape[0] == 8:
        return x + z
    return jnp.concatenate([x[:8] + z, x[8:]], axis=0)


def _gelu_mul2(g, u):
    c0 = 0.7978845608028654
    c1 = c0 * 0.044715
    t = jnp.tanh(g * (c0 + c1 * (g * g)))
    return (g * u) * (1.0 + t)


def _lo(x):
    return lax.bitcast_convert_type(x << 16, F32)


def _hi(x):
    return lax.bitcast_convert_type(x & jnp.uint32(0xFFFF0000), F32)


def _pk(x):
    return pltpu.bitcast(x.astype(BF16), U32)


def _upk(x):
    return pltpu.bitcast(x, BF16)


def _dot(a, b):
    return jnp.dot(a, b, preferred_element_type=F32)


def _dot_nt(a, b):
    return lax.dot_general(a, b, _NT, preferred_element_type=F32)


def _x_ops(x1, x2):
    d = [a - b for a, b in zip(x1, x2)]
    return [x1[0] + x2[1], x2[0] + x2[1], x1[0] + x1[1],
            d[1] + x1[2], x1[1] + x1[2], d[1] + d[2],
            d[0] - x2[2], d[0] + d[2], x2[0] + x2[2],
            x1[0], d[0], x2[1], d[1], x1[2], x2[2]]


def _x_rem(x1, x2):
    a, b, c = 0, 1, 2
    cat = lambda u, v: jnp.concatenate([u, v], axis=0)
    return [cat(x1[c], x2[b]), cat(x1[a], x1[b] - x2[b]), cat(x2[a], x2[c] - x1[c])]


def _w_sums(w):
    return [w[0][1] + w[1][0], w[1][2] + w[2][1], w[0][2] + w[2][0],
            w[0][0] + w[0][2] - w[1][0], w[2][0] - w[0][0] - w[0][1],
            w[1][1] + w[1][2] - w[0][1], w[1][0] + w[1][1] - w[2][1],
            w[2][0] + w[2][2] - w[1][2], w[2][1] + w[2][2] - w[0][2]]


_W_TERMS = {0: ((0, 1, 1), (1, 0, 1)), 3: ((1, 2, 1), (2, 1, 1)), 6: ((0, 2, 1), (2, 0, 1)),
            9: ((0, 0, 1), (0, 2, 1), (1, 0, -1)), 10: ((2, 0, 1), (0, 0, -1), (0, 1, -1)),
            11: ((1, 1, 1), (1, 2, 1), (0, 1, -1)), 12: ((1, 0, 1), (1, 1, 1), (2, 1, -1)),
            13: ((2, 0, 1), (2, 2, 1), (1, 2, -1)), 14: ((2, 1, 1), (2, 2, 1), (0, 2, -1)),
            1: ((0, 1, 1),), 2: ((1, 0, 1),), 4: ((1, 2, 1),), 5: ((2, 1, 1),),
            7: ((2, 0, 1),), 8: ((0, 2, 1),)}
_PARTS = ((1, 2, 0), (7, 8, 6), (4, 5, 3), (9, 10, 11, 12, 13, 14))
_W_SUM = {0: 0, 3: 1, 6: 2, 9: 3, 10: 4, 11: 5, 12: 6, 13: 7, 14: 8}
_W_RAW = {1: (0, 1), 2: (1, 0), 4: (1, 2), 5: (2, 1), 7: (2, 0), 8: (0, 2)}
_PAIR_ORDER = (1, 2, 4, 5, 7, 8, 0, 3, 6)
_DIAG = {(0, 0): 9, (2, 0): 10, (0, 1): 11, (1, 1): 12, (1, 2): 13, (2, 2): 14}
_PAIR = {(0, 0): ((6, -1), (8, -1)), (1, 0): ((2, 1), (7, 1)), (2, 0): ((0, 1), (1, -1)),
         (0, 1): ((3, 1), (4, -1)), (1, 1): ((0, 1), (2, -1)), (2, 1): ((1, 1), (5, -1)),
         (0, 2): ((4, 1), (8, 1)), (1, 2): ((6, 1), (7, -1)), (2, 2): ((5, 1), (3, -1))}


def _column(t, base, j):
    s = []
    for k in range(3):
        v = base[k]
        for i, sg in _PAIR[k, j]:
            ti = t[i]() if callable(t[i]) else t[i]
            v = ti if v is None else (v + ti if sg > 0 else v - ti)
        s.append(v)
    return s[1] + s[0], s[2] + s[0]


def _make_kernel(S, D, F, TM, cfg):
    NB = S // TM
    NT = TM // LANES
    DH = D // H
    DP = DH // 2
    RP = D // 2
    NG = H // 8
    scale = float(DH) ** -0.5
    NU = 2 * NB
    TH = TM // 2
    FT = F // 3
    D2 = D // 2
    D3 = D // 3
    Q3 = D3 // 2
    KU = D // 9
    KR = 3 * LANES
    NQ = 6
    QR = 3 * D // NQ
    WQ = (0, 640, 1152, 3 * D)
    PW = 256
    NP = FT // PW
    scopes = cfg['scopes']
    assert NG == 4 and NB & (NB - 1) == 0
    SEM_P = 4

    def kernel(x_hbm, wqkv_hbm, wo_hbm, wg_hbm, wu_hbm, wdt_hbm, out_hbm,
               xio_s, wqkv_v, wo_v, wg_v, wu_v, wdt_v, wt_s, wl_s,
               gs_s, us_s, ds_s, xmid_s, a_s, qkv_s, o_s, acc_s, b_s, r_s, t_s,
               sem_i, sem_o):

        def wait(name, cps):
            if scopes:
                with jax.named_scope(name):
                    for cp in cps:
                        cp.wait()
            else:
                for cp in cps:
                    cp.wait()

        def cols(lo, n):
            if not isinstance(lo, int):
                lo = pl.multiple_of(lo, LANES)
            return pl.ds(lo, n)

        def rows8(lo, n=8):
            if not isinstance(lo, int):
                lo = pl.multiple_of(lo, 8)
            return pl.ds(lo, n)

        def out_copy(b):
            return pltpu.make_async_copy(
                xio_s.at[b], out_hbm.at[:, cols(b * TM, TM)], sem_o.at[0])

        def x_cp(b, sem):
            return pltpu.make_async_copy(x_hbm.at[:, cols(b * TM, TM)], xio_s.at[b],
                                         sem_i.at[sem])

        def wq_cp(i):
            sl = cols(WQ[i], WQ[i + 1] - WQ[i])
            return pltpu.make_async_copy(wqkv_hbm.at[:, sl], wqkv_v.at[:, sl],
                                         sem_i.at[1 + i])

        def piece_cp(src, dst, p, sem):
            return [pltpu.make_async_copy(src.at[:, cols(j * FT + p * PW, PW)],
                                          dst.at[p, j],
                                          sem_i.at[sem]) for j in range(3)]

        def group_cp(p):
            sem = SEM_P + p
            cps = []
            if isinstance(p, int) and p == 0:
                cps.append(pltpu.make_async_copy(wo_hbm, wo_v, sem_i.at[sem]))
            if not (isinstance(p, int) and p == NP):
                cps += piece_cp(wg_hbm, wg_v, p, sem) + piece_cp(wu_hbm, wu_v, p, sem)
            if not (isinstance(p, int) and p == 0):
                cps += piece_cp(wdt_hbm, wdt_v, p - 1, sem)
            return cps

        lane = lax.broadcasted_iota(jnp.int32, (8, LANES), 1)
        cat0 = lambda *v: jnp.concatenate(v, axis=0)
        cat1 = lambda *v: jnp.concatenate(v, axis=1)

        def spread_over(anchors, n, total):
            return anchors[n * len(anchors) // total] if anchors else None

        def slab_group(r):
            return (r % LANES) // 16 if r < KR else 8 + ((r - KR) % KU) // 16

        def ln1(blk, anchors1, anchors2=()):
            slabs = (xio_s[blk, r:r + 8, :].astype(F32) for r in range(0, D, 8))
            m, rs = _ln_stats(slabs, D, anchors1)
            if not anchors2:
                return (xio_s[blk].astype(F32) - m) * rs
            m8 = jnp.broadcast_to(m, (8, TM))
            ms = [_tie(m8, a) for a in anchors2]
            ms = [spread_over(ms, slab_group(r), 12) for r in range(0, D, 8)]
            return (xio_s[blk].astype(F32) - cat0(*ms)) * rs

        def dot_k(rows, x, anchors):
            y = None
            for n, k in enumerate(range(0, D, LANES)):
                ks = slice(k, min(k + LANES, D))
                v = _dot(_upk(wt_s[rows, ks]), x[ks])
                anchors.extend(v[r:r + 8, :LANES] for r in ((0, 144) if n % 2 else (72, 216)))
                y = v if y is None else y + v
            return y

        def put_qkv(blk, rows, y):
            pk = _pk(y)
            for c in range(NT):
                qkv_s[1 + blk * NT + c, rows, :] = pk[:, c * LANES:(c + 1) * LANES]

        def qkv_mm(blk, xn, chunks, anchors):
            for r in chunks:
                rows = slice(r * QR // 2, (r + 1) * QR // 2)
                put_qkv(blk, rows, dot_k(rows, xn, anchors))

        def split_k(x):
            hs = (x[:, :TH], x[:, TH:])
            blocks = [[h[k * LANES:(k + 1) * LANES] for k in range(3)] for h in hs]
            units = [[h[KR + k * KU:KR + (k + 1) * KU] for k in range(3)] for h in hs]
            return blocks, units

        def prep_att(pat, anchor):
            assert Q3 == 96
            row0 = pat * 8
            src0 = row0 + ((pat * 43) >> 9) * (2 * Q3)
            w = [_upk(wt_s[rows8(src0 + j * Q3), :]).astype(F32) for j in range(3)]
            w[0] = cat1(_tie(w[0][:, :LANES], anchor), w[0][:, LANES:])
            tiles = _w_sums([[w[j][:, k * LANES:(k + 1) * LANES] for j in range(3)]
                             for k in range(3)])
            for j in range(3):
                a, b, c = (w[j][:, KR + k * KU:KR + (k + 1) * KU] for k in range(3))
                tiles += [cat1(c, b), cat1(a, c)]
            wl_s[rows8(row0), :] = _pk(cat1(*tiles))

        def att_rhs(x, stash=None):
            blocks, units = split_k(x)
            ops = _x_ops(*blocks) + _x_rem(*units)
            if stash is None:
                return [v.astype(BF16) for v in ops]
            loc = lambda i, r0, n: (slice((i // 2) * 64 + r0, (i // 2) * 64 + r0 + n),
                                    slice((i % 2) * LANES, (i % 2 + 1) * LANES))
            for r in range(0, LANES, 16):
                for i, v in enumerate(ops):
                    r_s.at[0][loc(i, r // 2, 8)] = _pk(v[r:r + 16])
            return [_upk(r_s.at[stash][loc(i, 0, 64)]) for i in range(18)]

        def att_mm(sec, rhs, anchors):
            tl = lambda i: _upk(wl_s[sec * Q3:(sec + 1) * Q3, i * LANES:(i + 1) * LANES])
            raw = lambda k, j: _upk(wt_s[(3 * sec + j) * Q3:(3 * sec + j + 1) * Q3,
                                         k * LANES:(k + 1) * LANES])
            t = {}
            for i in _PAIR_ORDER:
                t[i] = _dot(raw(*_W_RAW[i]) if i in _W_RAW else tl(_W_SUM[i]), rhs[i])
                anchors.append(t[i][:8])
            out = []
            for j in range(3):
                base = []
                for s in range(3):
                    v = _dot(raw(3, j) if s == 1 else tl(9 + 2 * j + s // 2), rhs[15 + s])
                    if (s, j) in _DIAG:
                        i = _DIAG[s, j]
                        v = _dot(tl(_W_SUM[i]), rhs[i]) + v
                    base.append(v)
                    anchors.append(base[-1][:8])
                out.append(cat1(*_column(t, base, j)))
            return cat0(*out)

        def qkv_fast(blk, rhs, anchors):
            for sec in range(3):
                put_qkv(blk, slice(sec * RP, (sec + 1) * RP), att_mm(sec, rhs, anchors))

        def shifted(ln, cur, prev, w):
            if w == 0:
                return cur
            sh = DIL * w
            return pltpu.roll(jnp.where(ln < LANES - sh, cur, prev), sh, axis=1)

        def att_group(blk, c, hg, anchor, win):
            tile = blk * NT + c
            base = hg * 8 * DP
            if isinstance(hg, int):
                cur, prev, o_t = qkv_s.at[1 + tile], qkv_s.at[tile], o_s.at[c]
                obase = hg * 8 * DH
            else:
                n = 2 * RP + 8 * DP
                base = pl.multiple_of(base, 8)
                cur = qkv_s.at[1 + tile, pl.ds(base, n)]
                prev = qkv_s.at[tile, pl.ds(base, n)]
                o_t = o_s.at[c, pl.ds(pl.multiple_of(hg * 8 * DH, 8), 8 * DH)]
                base, obase = 0, 0
            ln = lane + _zero_like_dep(anchor).astype(jnp.int32)
            logits = [None] * W
            done = []
            for dd in range(DP):
                q = cur[pl.ds(base + dd, 8, stride=DP), :]
                kc = cur[pl.ds(RP + base + dd, 8, stride=DP), :]
                if dd >= win:
                    kc = kc | _zero_like_dep(done[dd - win])
                kp = prev[pl.ds(RP + base + dd, 8, stride=DP), :]
                q0, q1 = _lo(q), _hi(q)
                for w in range(W):
                    ks = shifted(ln, kc, kp, w)
                    t = q0 * _lo(ks) + q1 * _hi(ks)
                    logits[w] = t if logits[w] is None else logits[w] + t
                done.append(ks)
            logits = [l * scale for l in logits]
            if not (isinstance(c, int) and c > 0):
                pos = lane + tile * LANES
                logits = [l if w == 0 else jnp.where(pos >= DIL * w, l, -1e9)
                          for w, l in enumerate(logits)]
            m = _tree_sum(logits, jnp.maximum)
            ln = lane + _zero_like_dep(m).astype(jnp.int32)
            e = [jnp.exp(l - m) for l in logits]
            den = _tree_sum(e)
            if cfg['rcp']:
                r = pl.reciprocal(den, approx=True)
                r = r * (2.0 - den * r)
            else:
                r = 1.0 / den
            p = e if cfg['late'] else [x * r for x in e]
            done = []
            for dd in range(DP):
                vc = cur[pl.ds(2 * RP + base + dd, 8, stride=DP), :]
                if dd >= win:
                    vc = vc | _zero_like_dep(done[dd - win])
                vp = prev[pl.ds(2 * RP + base + dd, 8, stride=DP), :]
                o0 = o1 = None
                for w in range(W):
                    vs = shifted(ln, vc, vp, w)
                    t0, t1 = p[w] * _lo(vs), p[w] * _hi(vs)
                    o0 = t0 if o0 is None else o0 + t0
                    o1 = t1 if o1 is None else o1 + t1
                done.append(vs)
                if cfg['late']:
                    o0, o1 = o0 * r, o1 * r
                o_t[pl.ds(obase + 2 * dd, 8, stride=DH), :] = o0
                o_t[pl.ds(obase + 2 * dd + 1, 8, stride=DH), :] = o1

        def attention(blk, anchors, win):
            for c in range(NT):
                for hg in range(NG):
                    att_group(blk, c, hg, anchors[c * NG + hg], win)

        def wo_mm(blk, anchors, fast, anchors_in=(), stash=None):
            o = cat1(*[o_s[c] for c in range(NT)])
            if anchors_in:
                o = cat0(*[_tie(o[r:r + 8], spread_over(anchors_in, slab_group(r), 12))
                           for r in range(0, D, 8)])
            if fast:
                y = att_mm(3, att_rhs(o, stash), anchors)
            else:
                o = o.astype(BF16)
                q = D2 // 2
                y = cat0(*[dot_k(slice(h * q, (h + 1) * q), o, anchors) for h in (6, 7)])
            xm = xio_s[blk].astype(F32) + y
            xmid_s[blk] = xm
            return _ln_stats((xm[r:r + 8] for r in range(0, D, 8)), D)

        def ffn_lhs(blk, stats, anchors):
            m, rs = stats
            m8 = jnp.broadcast_to(m, (8, TM))
            xs = []
            for k in range(3):
                mt = cat0(*[_tie(m8, spread_over(anchors, k, 3))] * (D3 // 8))
                xs.append((xmid_s[blk, k * D3:(k + 1) * D3, :] - mt) * rs)
            ops = _x_ops([x[:, :TH] for x in xs], [x[:, TH:] for x in xs])
            for i, v in enumerate(ops):
                for s, t in enumerate((v[KU:], v[:2 * KU], cat0(v[:KU], v[2 * KU:]))):
                    a_s[3 * i + s] = _pk(t.astype(BF16).T)

        def plain_lhs(blk, stats):
            m, rs = stats
            blocks, units = split_k((xmid_s[blk] - m) * rs)
            for i, v in enumerate(blocks[0] + blocks[1] + _x_rem(*units)):
                a_s[i] = _pk(v.astype(BF16).T)

        def plain_piece(p, anchors):
            h = {}
            for j in range(3):
                hs = []
                for n in range(PW // LANES):
                    cs = slice(n * LANES, (n + 1) * LANES)
                    w = lambda r0, r1: cat1(wg_v[p, j, r0:r1, cs], wu_v[p, j, r0:r1, cs])
                    u = lambda k: w(KR + k * KU, KR + (k + 1) * KU)
                    tl = lambda *i: _upk(cat1(*[a_s[k] for k in i]))
                    y0 = _dot(tl(6), cat0(u(2), u(1)))
                    y1 = _dot(tl(0, 1, 2, 7), w(0, KR + 2 * KU))
                    y2 = _dot(tl(3, 4, 5, 8), cat0(w(0, KR + KU), u(2)))
                    for y in (y0, y1, y2):
                        anchors.extend(y[r:r + 8, c:c + LANES]
                                       for c in ((0,) if y is y0 else (0, LANES))
                                       for r in ((0,) if y is y0 else (0, TH // 2)))
                    hs.append([_gelu_mul2(*[(y + y0)[:, c:c + LANES] for c in (0, LANES)])
                               for y in (y1, y2)])
                h[j] = [cat1(*[v[i] for v in hs]) for i in range(2)]
            return h_ops(h)

        def prep_d(p, anchors):
            PR = 16
            for n in range(2 * D3 // PR):
                r, cs = (n // 2) * PR, slice((n % 2) * LANES, (n % 2 + 1) * LANES)
                w = [[wdt_v[p, k, j * D3 + r:j * D3 + r + PR, cs].astype(F32)
                      for j in range(3)] for k in range(3)]
                w[0][1] = _tie(w[0][1], spread_over(anchors, n, 2 * D3 // PR))
                for i, v in enumerate(_w_sums(w)):
                    ds_s.at[p, i][r // 2:(r + PR) // 2, cs] = _pk(v)

        GU = ((wg_v, gs_s), (wu_v, us_s))

        def prep_gu(p, anchors):
            PR = 16
            nr = D3 // PR
            for n in range(4 * nr):
                c, (w_v, s_s), r = n % 2, GU[(n // 2) % 2], (n // 4) * PR
                cache = {}

                def w(k, j):
                    if (k, j) not in cache:
                        ld = lambda c: w_v[p, j, k * D3 + r:k * D3 + r + PR,
                                           c * LANES:(c + 1) * LANES].astype(F32)
                        v = ld(c)
                        if k != j:
                            v = _tie(v, spread_over(anchors, n, 4 * nr))
                        cache[k, j] = v - ld(1 - c) if r // KU == 1 + c else v
                    return cache[k, j]

                for i in range(15):
                    v = None
                    for k, j, sg in _W_TERMS[i]:
                        v = w(k, j) if v is None else (v + w(k, j) if sg > 0 else v - w(k, j))
                    s_s.at[p, i][r // 2:(r + PR) // 2, c * LANES:(c + 1) * LANES] = _pk(v)

        NS = cfg['msplit']

        def gu_prod(p, i, t, anchors, slabs, slot=0):
            u = KU // 2

            def rhs(s, s_s):
                if s == 1:
                    return s_s[p, i, :2 * u, :LANES]
                if s == 0:
                    return cat0(s_s[p, i, u:2 * u, LANES:], s_s[p, i, 2 * u:, :LANES])
                return cat0(s_s[p, i, :u, LANES:], s_s[p, i, 2 * u:, LANES:])

            q = TH // 2 // NS
            for n, h in enumerate(slabs):
                y = []
                for s in range(3):
                    r = _upk(cat1(rhs(s, gs_s), rhs(s, us_s)))
                    y.append(_dot(_upk(a_s[3 * i + s, h * q:(h + 1) * q]), r))
                    if (3 * n + s) % len(slabs) == 0:
                        anchors.append(y[-1][:8, :LANES])
                y1, y2 = y[1] + y[0], y[2] + y[0]
                for m in range(2):
                    cs = slice(m * LANES, (m + 1) * LANES)
                    v = cat1(y1[:, cs], y2[:, cs])
                    if i < 9 and 't' in cfg['stash']:
                        k = p if isinstance(p, int) else slot
                        t_s[k, m, i, 2 * h * q:2 * (h + 1) * q] = v
                        v = lambda k=k, m=m, h=h: t_s[k, m, i, 2 * h * q:2 * (h + 1) * q]
                    t.setdefault((m, h), {})[i] = v

        def gu_col(t, hv, p, j, anchors, slabs):
            ids = [_DIAG.get((s, j)) for s in range(3)]
            if cfg['fslab']:
                for h in slabs:
                    for i in ids:
                        if i is not None:
                            gu_prod(p, i, t, anchors if h == slabs[0] else [], [h])
            else:
                for i in ids:
                    if i is not None:
                        gu_prod(p, i, t, anchors, slabs)
            for h in slabs:
                g, u = [_column(t[m, h], [None if i is None else t[m, h][i] for i in ids], j)
                        for m in range(2)]
                hv[j, h] = [_gelu_mul2(g[i], u[i]) for i in range(2)]

        def h_ops(h):
            return [v.astype(BF16) for v in _x_ops(*[[h[j][i] for j in range(3)]
                                                     for i in range(2)])]

        def h_join(hv):
            return h_ops({j: [cat0(*[hv[j, h][i] for h in range(NS)]) for i in range(2)]
                          for j in range(3)})

        def gu_piece(p, order, anchors, slot):
            t, hv = {}, {}
            for slabs in ([[h] for h in range(NS)] if cfg['slab'] else [list(range(NS))]):
                for step in order:
                    if step[0] == 'S':
                        for i in _PARTS[int(step[1])]:
                            gu_prod(p, i, t, anchors, slabs, slot)
                    else:
                        gu_col(t, hv, p, int(step[1]), anchors, slabs)
            return h_join(hv)

        D_ORDER = _PAIR_ORDER + (9, 10, 11, 12, 13, 14)

        def down_mm(acc, bs, lo, anchors, which=D_ORDER, fine=False):
            p = [None] * 15 if acc is None else list(acc)
            for i in which:
                y = None
                for n, b in enumerate(bs):
                    if i in _W_RAW:
                        k, j = _W_RAW[i]
                        v = _dot_nt(wdt_v[lo + n, k, j * D3:(j + 1) * D3, :], b[i])
                    elif len(bs) % 2 and i == 14 and n == 0:
                        v = cat0(*[_dot_nt(_upk(ds_s[lo, _W_SUM[i],
                                                     h * Q3 // 2:(h + 1) * Q3 // 2, :]), b[i])
                                   for h in range(2)])
                    else:
                        v = _dot_nt(_upk(ds_s[lo + n, _W_SUM[i]]), b[i])
                    y = v if y is None else y + v
                p[i] = y if p[i] is None else p[i] + y
                anchors.append(p[i][:8])
                if fine:
                    anchors.append(p[i][D3 // 2:D3 // 2 + 8])
            return p

        def finish(blk, acc):
            y = [cat1(*_column(acc, [acc[_DIAG[s, j]] if (s, j) in _DIAG else None
                                     for s in range(3)], j)) for j in range(3)]
            xio_s[blk] = (xmid_s[blk] + 0.5 * cat0(*y)).astype(BF16)

        def load_acc(k):
            return [acc_s[k, i] for i in range(15)]

        def store_acc(k, acc):
            for i in range(15):
                acc_s[k, i] = acc[i]

        def load_b(k=0):
            return [_upk(b_s[i * TH // 2:(i + 1) * TH // 2, :])
                    for i in range(15 * k, 15 * k + 15)]

        def store_b(b, k=0):
            for i in range(15):
                b_s[(15 * k + i) * TH // 2:(15 * k + i + 1) * TH // 2, :] = _pk(b[i])

        def pre_phase():
            x0_cp, x1_cp = x_cp(0, 0), x_cp(1, 3)
            order = [x0_cp, wq_cp(0), wq_cp(1), x1_cp, wq_cp(2)]
            for p in range(NP + 1):
                order += group_cp(p)
            xr_cp = [x_cp(b, SEM_P + NP + 1) for b in range(2, NB)]
            order += xr_cp
            for cp in order:
                cp.start()
            get = lambda an, name: [an[min(i, len(an) - 1)] for i in cfg[name]]
            e_grp = lambda e: ((e >> 1) & 1, ((e >> 2) << 1) | (e & 1))
            if 'a' in cfg['sub']:
                pre_a(x0_cp, x1_cp, get, e_grp)
            if 'b' in cfg['sub']:
                pre_b(get, e_grp)
            if 'c' in cfg['sub']:
                pre_c(get)
            wait('WX', xr_cp)

        def pre_a(x0_cp, x1_cp, get, e_grp):
            qkv_s[0] = jnp.zeros(qkv_s.shape[1:], U32)
            acc_s[...] = jnp.zeros(acc_s.shape, F32)
            wait('WX0', [x0_cp])
            xn0 = ln1(0, ()).astype(BF16)
            done = 0
            for i in range(3):
                wait('WQ%d' % i, [wq_cp(i)] + ([x1_cp] if i == 2 else []))
                wt = _pk(wqkv_v[:, WQ[i]:WQ[i + 1]].T)
                wt_s[WQ[i] // 2:WQ[i + 1] // 2, :] = wt
                anchors = []
                qkv_mm(0, xn0, range(done, WQ[i + 1] // QR), anchors)
                done = WQ[i + 1] // QR
                if i > 0:
                    for n, a in enumerate(get(anchors, 'a_w%d' % i)):
                        prep_att(12 * (i - 1) + n, a)
            xn1 = ln1(1, get(anchors, 'a_ln'), get(anchors, 'a_lnb')).astype(BF16)
            qkv_mm(1, xn1, (0, 2, 4, 1), anchors)
            for e in range(8):
                att_group(0, *e_grp(e), anchors[cfg['att0'][e]], 9)
            wait('WO', group_cp(0))
            wt = _pk(wo_v[...].T)
            wt_s[3 * RP:, :] = wt
            an = []
            stats = wo_mm(0, an, False)
            qkv_mm(1, xn1, [3], an)
            plain_lhs(0, stats)
            b = plain_piece(0, an)
            qkv_mm(1, xn1, [5], an)
            prep_gu(0, get(an, 'z_g'))
            for e in range(3):
                att_group(1, *e_grp(e), an[cfg['z_att'][e]], 9)
            store_b(b)

        def pre_b(get, e_grp):
            def piece(p, carry):
                wait('WP', group_cp(p))
                b_prev = load_b()
                an = []
                b = plain_piece(p, an)
                prep_d(p - 1, get(an, 'p_d'))
                store_acc(0, down_mm(load_acc(0), [b_prev], p - 1, an))
                prep_gu(p, get(an, 'p_g'))
                att_group(1, *e_grp(p + 2), an[cfg['p_att'][0]], 9)
                for i, a in enumerate(get(an, 'p_w')):
                    prep_att(jnp.minimum(24 + (p - 1) * 5 + i, 47), a)
                store_b(b)
                return carry

            lax.fori_loop(1, NP, piece, 0)

        def pre_c(get):
            wait('WD', group_cp(NP))
            an = []
            stats = wo_mm(1, an, True)
            prep_d(NP - 1, get(an, 't_d'))
            acc = down_mm(load_acc(0), [load_b()], NP - 1, [])
            ffn_lhs(1, stats, [])
            finish(0, acc)

        if 'pre' in cfg['phases']:
            pre_phase()

        def body(u, carry):
            bu = u & (NB - 1)
            ba = (u + 1) & (NB - 1)
            acc, stats, an, b = None, None, {}, {}
            get = lambda name: [an[k][i] for k, i in cfg[name]]
            for step in cfg['body']:
                an[step] = []
                if step == 'Q':
                    qkv_fast(ba, att_rhs(ln1(ba, get('ln1'), get('ln1b')), u >> 8 if 'q' in cfg['stash'] else None),
                             an[step])
                elif step == 'W':
                    attention(ba, get('att'), cfg['win'])
                    stats = wo_mm(ba, an[step], True, get('orhs'),
                                  u >> 8 if 'w' in cfg['stash'] else None)
                elif step == 'L':
                    ffn_lhs(ba, stats, get('lhs'))
                elif step[0] == 'S':
                    slabs = [int(step[3])] if len(step) > 3 else list(range(NS))
                    for i in _PARTS[int(step[2])]:
                        gu_prod(int(step[1]), i, b.setdefault(step[:2], {}), an[step], slabs)
                elif step[0] == 'F':
                    j, c = int(step[1]), int(step[2])
                    slabs = [int(step[3])] if len(step) > 3 else list(range(NS))
                    hv = b.setdefault(step[:2], {})
                    gu_col(b['S' + step[1]], hv, j, c, an[step], slabs)
                    if len(hv) == 3 * NS:
                        b[j] = h_join(hv)
                        if 'b' in cfg['stash']:
                            store_b(b[j], j)
                            b[j] = load_b(j)
                else:
                    js = [int(c) for c in step[1:]]
                    acc = down_mm(acc, [b[j] for j in js], js[0], an[step])
            finish(bu, acc)

            @pl.when(u >= NB)
            def _():
                out_copy(bu).start()
            return carry

        if scopes:
            with jax.named_scope('LOOP'):
                lax.fori_loop(1, NU - 1, body, 0)
        elif 'main' in cfg['phases']:
            lax.fori_loop(1, NU - 1, body, 0)

        def last(c, carry):
            los = [2 * c + j for j in range(2)]
            b = [gu_piece(lo, cfg['order'], [], j) for j, lo in enumerate(los)]
            acc = load_acc(1)
            for j in range(2):
                acc = down_mm(acc, [b[j]], los[j], [])
            store_acc(1, acc)
            return carry

        if 'last' in cfg['phases']:
            lax.fori_loop(0, NP // 2, last, 0)
        if len(cfg['phases']) < 3:
            def keep(i, c):
                v = (gs_s[i, i, :8, :LANES] + us_s[i, i, :8, :LANES] + ds_s[i, i, :8, :LANES]
                     + wl_s[rows8(i * 8), :LANES] + a_s[i, :8] + qkv_s[i, :8]
                     + b_s[rows8(i * 8), :LANES] + wt_s[rows8(i * 8), :LANES])
                acc_s[1, 0, :8] = (lax.bitcast_convert_type(v, F32) + o_s[i, :8]
                                   + acc_s[i, i, :8])
                return c
            lax.fori_loop(0, 2, keep, 0)
        finish(NB - 1, load_acc(1))
        out_copy(NB - 1).start()
        wait('WOUT', [out_copy(b) for b in range(NB)])

    scratch = [
        pltpu.VMEM((NB, D, TM), BF16),
        pltpu.VMEM((D, 3 * D), BF16),
        pltpu.VMEM((D, D), BF16),
        pltpu.VMEM((NP, 3, D, PW), BF16),
        pltpu.VMEM((NP, 3, D, PW), BF16),
        pltpu.VMEM((NP, 3, D, PW), BF16),
        pltpu.VMEM((2 * D, D), U32),
        pltpu.VMEM((4 * Q3, 15 * LANES), U32),
        pltpu.VMEM((NP, 15, Q3, PW), U32),
        pltpu.VMEM((NP, 15, Q3, PW), U32),
        pltpu.VMEM((NP, 9, Q3, PW), U32),
        pltpu.VMEM((NB, D, TM), F32),
        pltpu.VMEM((45, TH // 2, LANES), U32),
        pltpu.VMEM((S // LANES + 1, 3 * RP, LANES), U32),
        pltpu.VMEM((NT, D, LANES), F32),
        pltpu.VMEM((2, 15, D3, TH), F32),
        pltpu.VMEM((NP * 15 * TH // 2, PW), U32),
        pltpu.VMEM((1, 9 * 64, 2 * LANES), U32),
        pltpu.VMEM((NP, 2, 9, TH, PW), F32),
        pltpu.SemaphoreType.DMA((SEM_P + NP + 2,)),
        pltpu.SemaphoreType.DMA((1,)),
    ]
    return kernel, scratch


_CFG = dict(
    scopes=False,
    rcp=False,
    late=True,
    stash='qw',
    slab=True,
    fslab=False,
    win=9,
    sub='abc',
    orhs=(),
    msplit=2,
    phases=('pre', 'main', 'last'),
    order=('S0', 'S1', 'F0', 'S2', 'F1', 'F2'),
    body=('S010', 'S000', 'F000', 'S020', 'F010', 'F020', 'S001', 'S011', 'F001',
        'S021', 'F011', 'F021', 'S100', 'S110', 'F100', 'S120', 'S101', 'F110', 'Q',
        'F120', 'S111', 'F101', 'S121', 'F111', 'F121', 'S200', 'S210', 'F200', 'S220',
        'F210', 'F220', 'S300', 'S201', 'S211', 'F201', 'S221', 'F211', 'F221', 'S310',
        'D01', 'F300', 'S320', 'S301', 'F310', 'S311', 'F301', 'S321', 'F311', 'F321',
        'S400', 'F320', 'S420', 'F410', 'S410', 'F400', 'S401', 'F420', 'S411', 'S421',
        'F411', 'F401', 'F421', 'S500', 'S501', 'S510', 'D23', 'F500', 'S520', 'W',
        'F520', 'S511', 'F510', 'F501', 'S521', 'F511', 'F521', 'D4', 'D5', 'L'),
    ln1=(('S010', 4), ('S010', 5), ('S010', 6), ('S010', 7), ('S010', 8), ('S000', 0),
        ('S000', 1), ('S000', 2), ('S000', 3)),
    ln1b=(('S110', 0), ('S110', 1), ('S110', 3), ('S110', 4), ('S110', 6), ('S110', 7),
        ('F100', 0), ('F100', 1), ('F100', 3), ('F100', 4), ('S120', 0), ('S120', 1)),
    att=(('S300', 6), ('D01', 0), ('D01', 6), ('D01', 8), ('D01', 9), ('D23', 0),
        ('D23', 6), ('D23', 10)),
    lhs=(('S511', 1), ('D5', 1), ('D5', 4)),
    att0=(15, 18, 21, 24, 27, 30, 33, 37),
    order0=('S0', 'S1', 'S2', 'F0', 'F1', 'F2'),
    order1=('S0', 'S1', 'S2', 'F0', 'F1', 'F2'),
    a_w1=(0, 1, 2, 3, 5, 5, 8, 9, 10, 11, 12, 14),
    a_w2=(0, 0, 2, 3, 4, 4, 6, 6, 8, 9, 11, 16),
    a_ln=(0, 3, 7),
    a_lnb=(6, 6, 8),
    z_g=(3, 4, 5, 6, 8, 9, 10, 12, 13, 14, 15, 17, 18, 19, 21, 22, 23, 25, 26, 27, 28,
        30, 31, 32, 34, 35, 36, 38, 39, 40, 41, 43, 44, 45, 47, 48, 49, 51, 52, 53, 54,
        56, 57, 58, 60, 61, 62, 64),
    z_att=(72, 75, 78),
    p_g0=(0, 1, 2, 3, 4, 5),
    p_g1=(6, 7, 8, 9, 10, 10),
    p_g2=(12, 13, 14, 15, 16, 17),
    p_g3=(14, 16, 18, 20, 22, 24, 26, 28, 30, 32, 34, 36),
    t_d=(0, 0, 1, 1, 2, 3, 3, 4, 5, 6, 6, 7, 8, 9, 9, 9, 10, 11, 11, 12, 13, 14, 15,
        16),
    p_d=(0, 2, 6, 8, 10, 12, 14, 16, 18, 20, 22, 24, 26, 28, 30, 32, 34, 36, 38, 40, 40,
        42, 44, 46),
    p_att=(52,),
    p_w=(10, 19, 30, 44, 48),
    p_g=(0, 1, 2, 3, 4, 5, 6, 7, 9, 10, 11, 12, 13, 14, 15, 16, 18, 19, 20, 21, 22, 23,
        24, 25, 27, 28, 29, 30, 31, 32, 33, 34, 36, 37, 38, 39, 40, 41, 42, 43, 45, 46,
        47, 48, 49, 50, 51, 53),
)


def _run(A_x, A_wqkv, A_wo, B_w_gate, B_w_up, B_w_down, **kw):
    _, S, D = A_x.shape
    F = B_w_gate.shape[1]
    kernel, scratch = _make_kernel(S, D, F, 256, {**_CFG, **kw})
    hbm = pl.BlockSpec(memory_space=pl.ANY)
    out_t = pl.pallas_call(
        kernel,
        in_specs=[hbm] * 6,
        out_specs=hbm,
        out_shape=jax.ShapeDtypeStruct((D, S), A_x.dtype),
        scratch_shapes=scratch,
        compiler_params=pltpu.CompilerParams(vmem_limit_bytes=110 * 1024 * 1024),
    )(A_x.reshape(S, D).T, A_wqkv, A_wo, B_w_gate, B_w_up, B_w_down.T)
    return out_t.T.reshape(A_x.shape)


@jax.jit
def pallas_interleave_layers__sliding_local_dilated__glu_gated_geglu__prompt_kernel(
    A_x: jax.Array,
    A_wqkv: jax.Array,
    A_wo: jax.Array,
    B_x: jax.Array,
    B_w_gate: jax.Array,
    B_w_up: jax.Array,
    B_w_down: jax.Array,
):
    del B_x
    return _run(A_x, A_wqkv, A_wo, B_w_gate, B_w_up, B_w_down)
```

```python
import functools

import jax
import jax.numpy as jnp
import jax.experimental.pallas as pl
import jax.experimental.pallas.tpu as pltpu
from jax import lax

H = 32
W = 8
DIL = 2
EPS = 1e-5
LANES = 128

F32 = jnp.float32
BF16 = jnp.bfloat16
U32 = jnp.uint32

_NT = (((1,), (1,)), ((), ()))


def _tree_sum(parts, op=jnp.add):
    while len(parts) > 1:
        nxt = [op(parts[i], parts[i + 1]) for i in range(0, len(parts) - 1, 2)]
        if len(parts) % 2:
            nxt.append(parts[-1])
        parts = nxt
    return parts[0]


def _ln_stats(slabs, d, anchors=()):
    n_acc = 4
    s1, s2, pilot = [None] * n_acc, [None] * n_acc, None
    for i, x in enumerate(slabs):
        if pilot is None:
            pilot = x[0:1, :]
            pil = jnp.broadcast_to(pilot, x.shape)
            pils = [_tie(pil, a) for a in anchors] or [pil]
        dx = x - pils[i * len(pils) // (d // 8)]
        j = i % n_acc
        s1[j] = dx if s1[j] is None else s1[j] + dx
        s2[j] = dx * dx if s2[j] is None else s2[j] + dx * dx
    e1 = jnp.sum(_tree_sum(s1), axis=0, keepdims=True) * (1.0 / d)
    e2 = jnp.sum(_tree_sum(s2), axis=0, keepdims=True) * (1.0 / d)
    var = jnp.maximum(e2 - e1 * e1, 0.0)
    return pilot + e1, lax.rsqrt(var + EPS)


def _zero_like_dep(v):
    return (lax.bitcast_convert_type(v, U32) >> 31) >> 1


def _tie(x, anchor):
    if anchor is None:
        return x
    z = lax.bitcast_convert_type(_zero_like_dep(anchor), F32)
    z = jnp.concatenate([z] * (x.shape[1] // LANES), axis=1)
    if x.shape[0] == 8:
        return x + z
    return jnp.concatenate([x[:8] + z, x[8:]], axis=0)


def _gelu_mul2(g, u):
    c0 = 0.7978845608028654
    c1 = c0 * 0.044715
    t = jnp.tanh(g * (c0 + c1 * (g * g)))
    return (g * u) * (1.0 + t)


def _lo(x):
    return lax.bitcast_convert_type(x << 16, F32)


def _hi(x):
    return lax.bitcast_convert_type(x & jnp.uint32(0xFFFF0000), F32)


def _pk(x):
    return pltpu.bitcast(x.astype(BF16), U32)


def _upk(x):
    return pltpu.bitcast(x, BF16)


def _dot(a, b):
    return jnp.dot(a, b, preferred_element_type=F32)


def _dot_nt(a, b):
    return lax.dot_general(a, b, _NT, preferred_element_type=F32)


def _x_ops(x1, x2):
    d = [a - b for a, b in zip(x1, x2)]
    return [x1[0] + x2[1], x2[0] + x2[1], x1[0] + x1[1],
            d[1] + x1[2], x1[1] + x1[2], d[1] + d[2],
            d[0] - x2[2], d[0] + d[2], x2[0] + x2[2],
            x1[0], d[0], x2[1], d[1], x1[2], x2[2]]


def _x_rem(x1, x2):
    a, b, c = 0, 1, 2
    cat = lambda u, v: jnp.concatenate([u, v], axis=0)
    return [cat(x1[c], x2[b]), cat(x1[a], x1[b] - x2[b]), cat(x2[a], x2[c] - x1[c])]


def _w_sums(w):
    return [w[0][1] + w[1][0], w[1][2] + w[2][1], w[0][2] + w[2][0],
            w[0][0] + w[0][2] - w[1][0], w[2][0] - w[0][0] - w[0][1],
            w[1][1] + w[1][2] - w[0][1], w[1][0] + w[1][1] - w[2][1],
            w[2][0] + w[2][2] - w[1][2], w[2][1] + w[2][2] - w[0][2]]


_W_TERMS = {0: ((0, 1, 1), (1, 0, 1)), 3: ((1, 2, 1), (2, 1, 1)), 6: ((0, 2, 1), (2, 0, 1)),
            9: ((0, 0, 1), (0, 2, 1), (1, 0, -1)), 10: ((2, 0, 1), (0, 0, -1), (0, 1, -1)),
            11: ((1, 1, 1), (1, 2, 1), (0, 1, -1)), 12: ((1, 0, 1), (1, 1, 1), (2, 1, -1)),
            13: ((2, 0, 1), (2, 2, 1), (1, 2, -1)), 14: ((2, 1, 1), (2, 2, 1), (0, 2, -1)),
            1: ((0, 1, 1),), 2: ((1, 0, 1),), 4: ((1, 2, 1),), 5: ((2, 1, 1),),
            7: ((2, 0, 1),), 8: ((0, 2, 1),)}
_PARTS = ((1, 2, 0), (7, 8, 6), (4, 5, 3), (9, 10, 11, 12, 13, 14))
_W_SUM = {0: 0, 3: 1, 6: 2, 9: 3, 10: 4, 11: 5, 12: 6, 13: 7, 14: 8}
_W_RAW = {1: (0, 1), 2: (1, 0), 4: (1, 2), 5: (2, 1), 7: (2, 0), 8: (0, 2)}
_PAIR_ORDER = (1, 2, 4, 5, 7, 8, 0, 3, 6)
_DIAG = {(0, 0): 9, (2, 0): 10, (0, 1): 11, (1, 1): 12, (1, 2): 13, (2, 2): 14}
_PAIR = {(0, 0): ((6, -1), (8, -1)), (1, 0): ((2, 1), (7, 1)), (2, 0): ((0, 1), (1, -1)),
         (0, 1): ((3, 1), (4, -1)), (1, 1): ((0, 1), (2, -1)), (2, 1): ((1, 1), (5, -1)),
         (0, 2): ((4, 1), (8, 1)), (1, 2): ((6, 1), (7, -1)), (2, 2): ((5, 1), (3, -1))}


def _column(t, base, j):
    s = []
    for k in range(3):
        v = base[k]
        for i, sg in _PAIR[k, j]:
            ti = t[i]() if callable(t[i]) else t[i]
            v = ti if v is None else (v + ti if sg > 0 else v - ti)
        s.append(v)
    return s[1] + s[0], s[2] + s[0]


def _make_kernel(S, D, F, TM, cfg):
    NB = S // TM
    NT = TM // LANES
    DH = D // H
    DP = DH // 2
    RP = D // 2
    NG = H // 8
    scale = float(DH) ** -0.5
    NU = 2 * NB
    TH = TM // 2
    FT = F // 3
    D2 = D // 2
    D3 = D // 3
    Q3 = D3 // 2
    KU = D // 9
    KR = 3 * LANES
    NQ = 6
    QR = 3 * D // NQ
    WQ = (0, 640, 1152, 3 * D)
    PW = 256
    NP = FT // PW
    scopes = cfg['scopes']
    assert NG == 4 and NB & (NB - 1) == 0
    SEM_P = 4

    def kernel(x_hbm, wqkv_hbm, wo_hbm, wg_hbm, wu_hbm, wdt_hbm, out_hbm,
               xio_s, wqkv_v, wo_v, wg_v, wu_v, wdt_v, wt_s, wl_s,
               gs_s, us_s, ds_s, xmid_s, a_s, qkv_s, o_s, acc_s, b_s, r_s, t_s,
               sem_i, sem_o):

        def wait(name, cps):
            if scopes:
                with jax.named_scope(name):
                    for cp in cps:
                        cp.wait()
            else:
                for cp in cps:
                    cp.wait()

        def cols(lo, n):
            if not isinstance(lo, int):
                lo = pl.multiple_of(lo, LANES)
            return pl.ds(lo, n)

        def rows8(lo, n=8):
            if not isinstance(lo, int):
                lo = pl.multiple_of(lo, 8)
            return pl.ds(lo, n)

        def out_copy(b):
            return pltpu.make_async_copy(
                xio_s.at[b], out_hbm.at[:, cols(b * TM, TM)], sem_o.at[0])

        def x_cp(b, sem):
            return pltpu.make_async_copy(x_hbm.at[:, cols(b * TM, TM)], xio_s.at[b],
                                         sem_i.at[sem])

        def wq_cp(i):
            sl = cols(WQ[i], WQ[i + 1] - WQ[i])
            return pltpu.make_async_copy(wqkv_hbm.at[:, sl], wqkv_v.at[:, sl],
                                         sem_i.at[1 + i])

        def piece_cp(src, dst, p, sem):
            return [pltpu.make_async_copy(src.at[:, cols(j * FT + p * PW, PW)],
                                          dst.at[p, j],
                                          sem_i.at[sem]) for j in range(3)]

        def group_cp(p):
            sem = SEM_P + p
            cps = []
            if isinstance(p, int) and p == 0:
                cps.append(pltpu.make_async_copy(wo_hbm, wo_v, sem_i.at[sem]))
            if not (isinstance(p, int) and p == NP):
                cps += piece_cp(wg_hbm, wg_v, p, sem) + piece_cp(wu_hbm, wu_v, p, sem)
            if not (isinstance(p, int) and p == 0):
                cps += piece_cp(wdt_hbm, wdt_v, p - 1, sem)
            return cps

        lane = lax.broadcasted_iota(jnp.int32, (8, LANES), 1)
        cat0 = lambda *v: jnp.concatenate(v, axis=0)
        cat1 = lambda *v: jnp.concatenate(v, axis=1)

        def spread_over(anchors, n, total):
            return anchors[n * len(anchors) // total] if anchors else None

        def slab_group(r):
            return (r % LANES) // 16 if r < KR else 8 + ((r - KR) % KU) // 16

        def ln1(blk, anchors1, anchors2=()):
            slabs = (xio_s[blk, r:r + 8, :].astype(F32) for r in range(0, D, 8))
            m, rs = _ln_stats(slabs, D, anchors1)
            if not anchors2:
                return (xio_s[blk].astype(F32) - m) * rs
            m8 = jnp.broadcast_to(m, (8, TM))
            ms = [_tie(m8, a) for a in anchors2]
            ms = [spread_over(ms, slab_group(r), 12) for r in range(0, D, 8)]
            return (xio_s[blk].astype(F32) - cat0(*ms)) * rs

        def dot_k(rows, x, anchors):
            y = None
            for n, k in enumerate(range(0, D, LANES)):
                ks = slice(k, min(k + LANES, D))
                v = _dot(_upk(wt_s[rows, ks]), x[ks])
                anchors.extend(v[r:r + 8, :LANES] for r in ((0, 144) if n % 2 else (72, 216)))
                y = v if y is None else y + v
            return y

        def put_qkv(blk, rows, y):
            pk = _pk(y)
            for c in range(NT):
                qkv_s[1 + blk * NT + c, rows, :] = pk[:, c * LANES:(c + 1) * LANES]

        def qkv_mm(blk, xn, chunks, anchors):
            for r in chunks:
                rows = slice(r * QR // 2, (r + 1) * QR // 2)
                put_qkv(blk, rows, dot_k(rows, xn, anchors))

        def split_k(x):
            hs = (x[:, :TH], x[:, TH:])
            blocks = [[h[k * LANES:(k + 1) * LANES] for k in range(3)] for h in hs]
            units = [[h[KR + k * KU:KR + (k + 1) * KU] for k in range(3)] for h in hs]
            return blocks, units

        def prep_att(pat, anchor):
            assert Q3 == 96
            row0 = pat * 8
            src0 = row0 + ((pat * 43) >> 9) * (2 * Q3)
            w = [_upk(wt_s[rows8(src0 + j * Q3), :]).astype(F32) for j in range(3)]
            w[0] = cat1(_tie(w[0][:, :LANES], anchor), w[0][:, LANES:])
            tiles = _w_sums([[w[j][:, k * LANES:(k + 1) * LANES] for j in range(3)]
                             for k in range(3)])
            for j in range(3):
                a, b, c = (w[j][:, KR + k * KU:KR + (k + 1) * KU] for k in range(3))
                tiles += [cat1(c, b), cat1(a, c)]
            wl_s[rows8(row0), :] = _pk(cat1(*tiles))

        def att_rhs(x, stash=None):
            blocks, units = split_k(x)
            ops = _x_ops(*blocks) + _x_rem(*units)
            if stash is None:
                return [v.astype(BF16) for v in ops]
            loc = lambda i, r0, n: (slice((i // 2) * 64 + r0, (i // 2) * 64 + r0 + n),
                                    slice((i % 2) * LANES, (i % 2 + 1) * LANES))
            for r in range(0, LANES, 16):
                for i, v in enumerate(ops):
                    r_s.at[0][loc(i, r // 2, 8)] = _pk(v[r:r + 16])
            return [_upk(r_s.at[stash][loc(i, 0, 64)]) for i in range(18)]

        def att_mm(sec, rhs, anchors):
            tl = lambda i: _upk(wl_s[sec * Q3:(sec + 1) * Q3, i * LANES:(i + 1) * LANES])
            raw = lambda k, j: _upk(wt_s[(3 * sec + j) * Q3:(3 * sec + j + 1) * Q3,
                                         k * LANES:(k + 1) * LANES])
            t = {}
            for i in _PAIR_ORDER:
                t[i] = _dot(raw(*_W_RAW[i]) if i in _W_RAW else tl(_W_SUM[i]), rhs[i])
                anchors.append(t[i][:8])
            out = []
            for j in range(3):
                base = []
                for s in range(3):
                    v = _dot(raw(3, j) if s == 1 else tl(9 + 2 * j + s // 2), rhs[15 + s])
                    if (s, j) in _DIAG:
                        i = _DIAG[s, j]
                        v = _dot(tl(_W_SUM[i]), rhs[i]) + v
                    base.append(v)
                    anchors.append(base[-1][:8])
                out.append(cat1(*_column(t, base, j)))
            return cat0(*out)

        def qkv_fast(blk, rhs, anchors):
            for sec in range(3):
                put_qkv(blk, slice(sec * RP, (sec + 1) * RP), att_mm(sec, rhs, anchors))

        def shifted(ln, cur, prev, w):
            if w == 0:
                return cur
            sh = DIL * w
            return pltpu.roll(jnp.where(ln < LANES - sh, cur, prev), sh, axis=1)

        def att_group(blk, c, hg, anchor, win):
            tile = blk * NT + c
            base = hg * 8 * DP
            if isinstance(hg, int):
                cur, prev, o_t = qkv_s.at[1 + tile], qkv_s.at[tile], o_s.at[c]
            else:
                n = 2 * RP + 8 * DP
                base = pl.multiple_of(base, 8)
                cur = qkv_s.at[1 + tile, pl.ds(base, n)]
                prev = qkv_s.at[tile, pl.ds(base, n)]
                o_t = o_s.at[c, pl.ds(base, RP + 8 * DP)]
                base = 0
            ln = lane + _zero_like_dep(anchor).astype(jnp.int32)
            logits = [None] * W
            done = []
            for dd in range(DP):
                q = cur[pl.ds(base + dd, 8, stride=DP), :]
                kc = cur[pl.ds(RP + base + dd, 8, stride=DP), :]
                if dd >= win:
                    kc = kc | _zero_like_dep(done[dd - win])
                kp = prev[pl.ds(RP + base + dd, 8, stride=DP), :]
                q0, q1 = _lo(q), _hi(q)
                for w in range(W):
                    ks = shifted(ln, kc, kp, w)
                    t = q0 * _lo(ks) + q1 * _hi(ks)
                    logits[w] = t if logits[w] is None else logits[w] + t
                done.append(ks)
            logits = [l * scale for l in logits]
            if not (isinstance(c, int) and c > 0):
                pos = lane + tile * LANES
                logits = [l if w == 0 else jnp.where(pos >= DIL * w, l, -1e9)
                          for w, l in enumerate(logits)]
            m = _tree_sum(logits, jnp.maximum)
            ln = lane + _zero_like_dep(m).astype(jnp.int32)
            e = [jnp.exp(l - m) for l in logits]
            den = _tree_sum(e)
            if cfg['rcp']:
                r = pl.reciprocal(den, approx=True)
                r = r * (2.0 - den * r)
            else:
                r = 1.0 / den
            p = e if cfg['late'] else [x * r for x in e]
            done = []
            for dd in range(DP):
                vc = cur[pl.ds(2 * RP + base + dd, 8, stride=DP), :]
                if dd >= win:
                    vc = vc | _zero_like_dep(done[dd - win])
                vp = prev[pl.ds(2 * RP + base + dd, 8, stride=DP), :]
                o0 = o1 = None
                for w in range(W):
                    vs = shifted(ln, vc, vp, w)
                    t0, t1 = p[w] * _lo(vs), p[w] * _hi(vs)
                    o0 = t0 if o0 is None else o0 + t0
                    o1 = t1 if o1 is None else o1 + t1
                done.append(vs)
                if cfg['late']:
                    o0, o1 = o0 * r, o1 * r
                o_t[pl.ds(base + dd, 8, stride=DP), :] = o0
                o_t[pl.ds(RP + base + dd, 8, stride=DP), :] = o1

        def attention(blk, anchors, win):
            for c in range(NT):
                for hg in range(NG):
                    att_group(blk, c, hg, anchors[c * NG + hg], win)

        def wo_mm(blk, anchors, fast, anchors_in=(), stash=None):
            o = cat1(*[o_s[c] for c in range(NT)])
            if anchors_in:
                o = cat0(*[_tie(o[r:r + 8], spread_over(anchors_in, slab_group(r), 12))
                           for r in range(0, D, 8)])
            if fast:
                y = att_mm(3, att_rhs(o, stash), anchors)
            else:
                o = o.astype(BF16)
                q = D2 // 2
                y = cat0(*[dot_k(slice(h * q, (h + 1) * q), o, anchors) for h in (6, 7)])
            xm = xio_s[blk].astype(F32) + y
            xmid_s[blk] = xm
            return _ln_stats((xm[r:r + 8] for r in range(0, D, 8)), D)

        def ffn_lhs(blk, stats, anchors):
            m, rs = stats
            m8 = jnp.broadcast_to(m, (8, TM))
            xs = []
            for k in range(3):
                mt = cat0(*[_tie(m8, spread_over(anchors, k, 3))] * (D3 // 8))
                xs.append((xmid_s[blk, k * D3:(k + 1) * D3, :] - mt) * rs)
            ops = _x_ops([x[:, :TH] for x in xs], [x[:, TH:] for x in xs])
            for i, v in enumerate(ops):
                for s, t in enumerate((v[KU:], v[:2 * KU], cat0(v[:KU], v[2 * KU:]))):
                    a_s[3 * i + s] = _pk(t.astype(BF16).T)

        def plain_lhs(blk, stats):
            m, rs = stats
            blocks, units = split_k((xmid_s[blk] - m) * rs)
            for i, v in enumerate(blocks[0] + blocks[1] + _x_rem(*units)):
                a_s[i] = _pk(v.astype(BF16).T)

        def plain_piece(p, anchors):
            h = {}
            for j in range(3):
                hs = []
                for n in range(PW // LANES):
                    cs = slice(n * LANES, (n + 1) * LANES)
                    w = lambda r0, r1: cat1(wg_v[p, j, r0:r1, cs], wu_v[p, j, r0:r1, cs])
                    u = lambda k: w(KR + k * KU, KR + (k + 1) * KU)
                    tl = lambda *i: _upk(cat1(*[a_s[k] for k in i]))
                    y0 = _dot(tl(6), cat0(u(2), u(1)))
                    y1 = _dot(tl(0, 1, 2, 7), w(0, KR + 2 * KU))
                    y2 = _dot(tl(3, 4, 5, 8), cat0(w(0, KR + KU), u(2)))
                    for y in (y0, y1, y2):
                        anchors.extend(y[r:r + 8, c:c + LANES]
                                       for c in ((0,) if y is y0 else (0, LANES))
                                       for r in ((0,) if y is y0 else (0, TH // 2)))
                    hs.append([_gelu_mul2(*[(y + y0)[:, c:c + LANES] for c in (0, LANES)])
                               for y in (y1, y2)])
                h[j] = [cat1(*[v[i] for v in hs]) for i in range(2)]
            return h_ops(h)

        def prep_d(p, anchors):
            PR = 16
            for n in range(2 * D3 // PR):
                r, cs = (n // 2) * PR, slice((n % 2) * LANES, (n % 2 + 1) * LANES)
                w = [[wdt_v[p, k, j * D3 + r:j * D3 + r + PR, cs].astype(F32)
                      for j in range(3)] for k in range(3)]
                w[0][1] = _tie(w[0][1], spread_over(anchors, n, 2 * D3 // PR))
                for i, v in enumerate(_w_sums(w)):
                    ds_s.at[p, i][r // 2:(r + PR) // 2, cs] = _pk(v)

        GU = ((wg_v, gs_s), (wu_v, us_s))

        def prep_gu(p, anchors):
            PR = 16
            nr = D3 // PR
            for n in range(4 * nr):
                c, (w_v, s_s), r = n % 2, GU[(n // 2) % 2], (n // 4) * PR
                cache = {}

                def w(k, j):
                    if (k, j) not in cache:
                        ld = lambda c: w_v[p, j, k * D3 + r:k * D3 + r + PR,
                                           c * LANES:(c + 1) * LANES].astype(F32)
                        v = ld(c)
                        if k != j:
                            v = _tie(v, spread_over(anchors, n, 4 * nr))
                        cache[k, j] = v - ld(1 - c) if r // KU == 1 + c else v
                    return cache[k, j]

                for i in range(15):
                    v = None
                    for k, j, sg in _W_TERMS[i]:
                        v = w(k, j) if v is None else (v + w(k, j) if sg > 0 else v - w(k, j))
                    s_s.at[p, i][r // 2:(r + PR) // 2, c * LANES:(c + 1) * LANES] = _pk(v)

        NS = cfg['msplit']

        def gu_prod(p, i, t, anchors, slabs, slot=0):
            u = KU // 2

            def rhs(s, s_s):
                if s == 1:
                    return s_s[p, i, :2 * u, :LANES]
                if s == 0:
                    return cat0(s_s[p, i, u:2 * u, LANES:], s_s[p, i, 2 * u:, :LANES])
                return cat0(s_s[p, i, :u, LANES:], s_s[p, i, 2 * u:, LANES:])

            q = TH // 2 // NS
            for n, h in enumerate(slabs):
                y = []
                for s in range(3):
                    r = _upk(cat1(rhs(s, gs_s), rhs(s, us_s)))
                    y.append(_dot(_upk(a_s[3 * i + s, h * q:(h + 1) * q]), r))
                    if (3 * n + s) % len(slabs) == 0:
                        anchors.append(y[-1][:8, :LANES])
                y1, y2 = y[1] + y[0], y[2] + y[0]
                for m in range(2):
                    cs = slice(m * LANES, (m + 1) * LANES)
                    v = cat1(y1[:, cs], y2[:, cs])
                    if i < 9 and 't' in cfg['stash']:
                        k = p if isinstance(p, int) else slot
                        t_s[k, m, i, 2 * h * q:2 * (h + 1) * q] = v
                        v = lambda k=k, m=m, h=h: t_s[k, m, i, 2 * h * q:2 * (h + 1) * q]
                    t.setdefault((m, h), {})[i] = v

        def gu_col(t, hv, p, j, anchors, slabs):
            ids = [_DIAG.get((s, j)) for s in range(3)]
            if cfg['fslab']:
                for h in slabs:
                    for i in ids:
                        if i is not None:
                            gu_prod(p, i, t, anchors if h == slabs[0] else [], [h])
            else:
                for i in ids:
                    if i is not None:
                        gu_prod(p, i, t, anchors, slabs)
            for h in slabs:
                g, u = [_column(t[m, h], [None if i is None else t[m, h][i] for i in ids], j)
                        for m in range(2)]
                hv[j, h] = [_gelu_mul2(g[i], u[i]) for i in range(2)]

        def h_ops(h):
            return [v.astype(BF16) for v in _x_ops(*[[h[j][i] for j in range(3)]
                                                     for i in range(2)])]

        def h_join(hv):
            return h_ops({j: [cat0(*[hv[j, h][i] for h in range(NS)]) for i in range(2)]
                          for j in range(3)})

        def gu_piece(p, order, anchors, slot):
            t, hv = {}, {}
            for slabs in ([[h] for h in range(NS)] if cfg['slab'] else [list(range(NS))]):
                for step in order:
                    if step[0] == 'S':
                        for i in _PARTS[int(step[1])]:
                            gu_prod(p, i, t, anchors, slabs, slot)
                    else:
                        gu_col(t, hv, p, int(step[1]), anchors, slabs)
            return h_join(hv)

        D_ORDER = _PAIR_ORDER + (9, 10, 11, 12, 13, 14)

        def down_mm(acc, bs, lo, anchors, which=D_ORDER, fine=False):
            p = [None] * 15 if acc is None else list(acc)
            for i in which:
                y = None
                for n, b in enumerate(bs):
                    if i in _W_RAW:
                        k, j = _W_RAW[i]
                        v = _dot_nt(wdt_v[lo + n, k, j * D3:(j + 1) * D3, :], b[i])
                    elif len(bs) % 2 and i == 14 and n == 0:
                        v = cat0(*[_dot_nt(_upk(ds_s[lo, _W_SUM[i],
                                                     h * Q3 // 2:(h + 1) * Q3 // 2, :]), b[i])
                                   for h in range(2)])
                    else:
                        v = _dot_nt(_upk(ds_s[lo + n, _W_SUM[i]]), b[i])
                    y = v if y is None else y + v
                p[i] = y if p[i] is None else p[i] + y
                anchors.append(p[i][:8])
                if fine:
                    anchors.append(p[i][D3 // 2:D3 // 2 + 8])
            return p

        def finish(blk, acc):
            y = [cat1(*_column(acc, [acc[_DIAG[s, j]] if (s, j) in _DIAG else None
                                     for s in range(3)], j)) for j in range(3)]
            xio_s[blk] = (xmid_s[blk] + 0.5 * cat0(*y)).astype(BF16)

        def load_acc(k):
            return [acc_s[k, i] for i in range(15)]

        def store_acc(k, acc):
            for i in range(15):
                acc_s[k, i] = acc[i]

        def load_b(k=0):
            return [_upk(b_s[i * TH // 2:(i + 1) * TH // 2, :])
                    for i in range(15 * k, 15 * k + 15)]

        def store_b(b, k=0):
            for i in range(15):
                b_s[(15 * k + i) * TH // 2:(15 * k + i + 1) * TH // 2, :] = _pk(b[i])

        def pre_phase():
            x0_cp, x1_cp = x_cp(0, 0), x_cp(1, 3)
            order = [x0_cp, wq_cp(0), wq_cp(1), x1_cp, wq_cp(2)]
            for p in range(NP + 1):
                order += group_cp(p)
            xr_cp = [x_cp(b, SEM_P + NP + 1) for b in range(2, NB)]
            order += xr_cp
            for cp in order:
                cp.start()
            get = lambda an, name: [an[min(i, len(an) - 1)] for i in cfg[name]]
            e_grp = lambda e: ((e >> 1) & 1, ((e >> 2) << 1) | (e & 1))
            if 'a' in cfg['sub']:
                pre_a(x0_cp, x1_cp, get, e_grp)
            if 'b' in cfg['sub']:
                pre_b(get, e_grp)
            if 'c' in cfg['sub']:
                pre_c(get)
            wait('WX', xr_cp)

        def pre_a(x0_cp, x1_cp, get, e_grp):
            qkv_s[0] = jnp.zeros(qkv_s.shape[1:], U32)
            acc_s[...] = jnp.zeros(acc_s.shape, F32)
            wait('WX0', [x0_cp])
            xn0 = ln1(0, ()).astype(BF16)
            done = 0
            for i in range(3):
                wait('WQ%d' % i, [wq_cp(i)] + ([x1_cp] if i == 2 else []))
                wt = _pk(wqkv_v[:, WQ[i]:WQ[i + 1]].T)
                wt_s[WQ[i] // 2:WQ[i + 1] // 2, :] = wt
                anchors = []
                qkv_mm(0, xn0, range(done, WQ[i + 1] // QR), anchors)
                done = WQ[i + 1] // QR
                if i > 0:
                    for n, a in enumerate(get(anchors, 'a_w%d' % i)):
                        prep_att(12 * (i - 1) + n, a)
            xn1 = ln1(1, get(anchors, 'a_ln'), get(anchors, 'a_lnb')).astype(BF16)
            qkv_mm(1, xn1, (0, 2, 4, 1), anchors)
            for e in range(8):
                att_group(0, *e_grp(e), anchors[cfg['att0'][e]], 9)
            wait('WO', group_cp(0))
            wo = pltpu.bitcast(wo_v[...], U32)
            wt_s[3 * RP:, :] = _pk(cat0(_lo(wo), _hi(wo)).astype(BF16).T)
            an = []
            stats = wo_mm(0, an, False)
            qkv_mm(1, xn1, [3], an)
            plain_lhs(0, stats)
            b = plain_piece(0, an)
            qkv_mm(1, xn1, [5], an)
            prep_gu(0, get(an, 'z_g'))
            for e in range(3):
                att_group(1, *e_grp(e), an[cfg['z_att'][e]], 9)
            store_b(b)

        def pre_b(get, e_grp):
            def piece(p, carry):
                wait('WP', group_cp(p))
                b_prev = load_b()
                an = []
                b = plain_piece(p, an)
                prep_d(p - 1, get(an, 'p_d'))
                store_acc(0, down_mm(load_acc(0), [b_prev], p - 1, an))
                prep_gu(p, get(an, 'p_g'))
                att_group(1, *e_grp(p + 2), an[cfg['p_att'][0]], 9)
                for i, a in enumerate(get(an, 'p_w')):
                    prep_att(jnp.minimum(24 + (p - 1) * 5 + i, 47), a)
                store_b(b)
                return carry

            lax.fori_loop(1, NP, piece, 0)

        def pre_c(get):
            wait('WD', group_cp(NP))
            an = []
            stats = wo_mm(1, an, True)
            prep_d(NP - 1, get(an, 't_d'))
            acc = down_mm(load_acc(0), [load_b()], NP - 1, [])
            ffn_lhs(1, stats, [])
            finish(0, acc)

        if 'pre' in cfg['phases']:
            pre_phase()

        def body(u, carry):
            bu = u & (NB - 1)
            ba = (u + 1) & (NB - 1)
            acc, stats, an, b = None, None, {}, {}
            get = lambda name: [an[k][i] for k, i in cfg[name]]
            for step in cfg['body']:
                an[step] = []
                if step == 'Q':
                    qkv_fast(ba, att_rhs(ln1(ba, get('ln1'), get('ln1b')), u >> 8 if 'q' in cfg['stash'] else None),
                             an[step])
                elif step == 'W':
                    attention(ba, get('att'), cfg['win'])
                    stats = wo_mm(ba, an[step], True, get('orhs'),
                                  u >> 8 if 'w' in cfg['stash'] else None)
                elif step == 'L':
                    ffn_lhs(ba, stats, get('lhs'))
                elif step[0] == 'S':
                    slabs = [int(step[3])] if len(step) > 3 else list(range(NS))
                    for i in _PARTS[int(step[2])]:
                        gu_prod(int(step[1]), i, b.setdefault(step[:2], {}), an[step], slabs)
                elif step[0] == 'F':
                    j, c = int(step[1]), int(step[2])
                    slabs = [int(step[3])] if len(step) > 3 else list(range(NS))
                    hv = b.setdefault(step[:2], {})
                    gu_col(b['S' + step[1]], hv, j, c, an[step], slabs)
                    if len(hv) == 3 * NS:
                        b[j] = h_join(hv)
                        if 'b' in cfg['stash']:
                            store_b(b[j], j)
                            b[j] = load_b(j)
                else:
                    js = [int(c) for c in step[1:]]
                    acc = down_mm(acc, [b[j] for j in js], js[0], an[step])
            finish(bu, acc)

            @pl.when(u >= NB)
            def _():
                out_copy(bu).start()
            return carry

        if scopes:
            with jax.named_scope('LOOP'):
                lax.fori_loop(1, NU - 1, body, 0)
        elif 'main' in cfg['phases']:
            lax.fori_loop(1, NU - 1, body, 0)

        def last(c, carry):
            los = [2 * c + j for j in range(2)]
            b = [gu_piece(lo, cfg['order'], [], j) for j, lo in enumerate(los)]
            acc = load_acc(1)
            for j in range(2):
                acc = down_mm(acc, [b[j]], los[j], [])
            store_acc(1, acc)
            return carry

        if 'last' in cfg['phases']:
            lax.fori_loop(0, NP // 2, last, 0)
        if len(cfg['phases']) < 3:
            def keep(i, c):
                v = (gs_s[i, i, :8, :LANES] + us_s[i, i, :8, :LANES] + ds_s[i, i, :8, :LANES]
                     + wl_s[rows8(i * 8), :LANES] + a_s[i, :8] + qkv_s[i, :8]
                     + b_s[rows8(i * 8), :LANES] + wt_s[rows8(i * 8), :LANES])
                acc_s[1, 0, :8] = (lax.bitcast_convert_type(v, F32) + o_s[i, :8]
                                   + acc_s[i, i, :8])
                return c
            lax.fori_loop(0, 2, keep, 0)
        finish(NB - 1, load_acc(1))
        out_copy(NB - 1).start()
        wait('WOUT', [out_copy(b) for b in range(NB)])

    scratch = [
        pltpu.VMEM((NB, D, TM), BF16),
        pltpu.VMEM((D, 3 * D), BF16),
        pltpu.VMEM((D, D), BF16),
        pltpu.VMEM((NP, 3, D, PW), BF16),
        pltpu.VMEM((NP, 3, D, PW), BF16),
        pltpu.VMEM((NP, 3, D, PW), BF16),
        pltpu.VMEM((2 * D, D), U32),
        pltpu.VMEM((4 * Q3, 15 * LANES), U32),
        pltpu.VMEM((NP, 15, Q3, PW), U32),
        pltpu.VMEM((NP, 15, Q3, PW), U32),
        pltpu.VMEM((NP, 9, Q3, PW), U32),
        pltpu.VMEM((NB, D, TM), F32),
        pltpu.VMEM((45, TH // 2, LANES), U32),
        pltpu.VMEM((S // LANES + 1, 3 * RP, LANES), U32),
        pltpu.VMEM((NT, D, LANES), F32),
        pltpu.VMEM((2, 15, D3, TH), F32),
        pltpu.VMEM((NP * 15 * TH // 2, PW), U32),
        pltpu.VMEM((1, 9 * 64, 2 * LANES), U32),
        pltpu.VMEM((NP, 2, 9, TH, PW), F32),
        pltpu.SemaphoreType.DMA((SEM_P + NP + 2,)),
        pltpu.SemaphoreType.DMA((1,)),
    ]
    return kernel, scratch


_CFG = dict(
    scopes=False,
    rcp=False,
    late=True,
    stash='qw',
    slab=True,
    fslab=False,
    win=9,
    sub='abc',
    orhs=(),
    msplit=2,
    phases=('pre', 'main', 'last'),
    order=('S0', 'S1', 'F0', 'S2', 'F1', 'F2'),
    body=('S010', 'S000', 'F000', 'S020', 'F010', 'F020', 'S001', 'S011', 'F001',
        'S021', 'F011', 'F021', 'S100', 'S110', 'F100', 'S120', 'S101', 'F110', 'Q',
        'F120', 'S111', 'F101', 'S121', 'F111', 'F121', 'S200', 'S210', 'F200', 'S220',
        'F210', 'F220', 'S300', 'S201', 'S211', 'F201', 'S221', 'F211', 'F221', 'S310',
        'D01', 'F300', 'S320', 'S301', 'F310', 'S311', 'F301', 'S321', 'F311', 'F321',
        'S400', 'F320', 'S420', 'F410', 'S410', 'F400', 'S401', 'F420', 'S411', 'S421',
        'F411', 'F401', 'F421', 'S500', 'S501', 'S510', 'D23', 'F500', 'S520', 'W',
        'F520', 'S511', 'F510', 'F501', 'S521', 'F511', 'F521', 'D4', 'D5', 'L'),
    ln1=(('S010', 4), ('S010', 5), ('S010', 6), ('S010', 7), ('S010', 8), ('S000', 0),
        ('S000', 1), ('S000', 2), ('S000', 3)),
    ln1b=(('S110', 0), ('S110', 1), ('S110', 3), ('S110', 4), ('S110', 6), ('S110', 7),
        ('F100', 0), ('F100', 1), ('F100', 3), ('F100', 4), ('S120', 0), ('S120', 1)),
    att=(('S300', 6), ('D01', 0), ('D01', 6), ('D01', 8), ('D01', 9), ('D23', 0),
        ('D23', 6), ('D23', 10)),
    lhs=(('S511', 1), ('D5', 1), ('D5', 4)),
    att0=(15, 18, 21, 24, 27, 30, 33, 37),
    order0=('S0', 'S1', 'S2', 'F0', 'F1', 'F2'),
    order1=('S0', 'S1', 'S2', 'F0', 'F1', 'F2'),
    a_w1=(0, 1, 2, 3, 5, 5, 8, 9, 10, 11, 12, 14),
    a_w2=(0, 0, 2, 3, 4, 4, 6, 6, 8, 9, 11, 16),
    a_ln=(0, 3, 7),
    a_lnb=(6, 6, 8),
    z_g=(3, 4, 5, 6, 8, 9, 10, 12, 13, 14, 15, 17, 18, 19, 21, 22, 23, 25, 26, 27, 28,
        30, 31, 32, 34, 35, 36, 38, 39, 40, 41, 43, 44, 45, 47, 48, 49, 51, 52, 53, 54,
        56, 57, 58, 60, 61, 62, 64),
    z_att=(72, 75, 78),
    p_g0=(0, 1, 2, 3, 4, 5),
    p_g1=(6, 7, 8, 9, 10, 10),
    p_g2=(12, 13, 14, 15, 16, 17),
    p_g3=(14, 16, 18, 20, 22, 24, 26, 28, 30, 32, 34, 36),
    t_d=(0, 0, 1, 1, 2, 3, 3, 4, 5, 6, 6, 7, 8, 9, 9, 9, 10, 11, 11, 12, 13, 14, 15,
        16),
    p_d=(0, 2, 6, 8, 10, 12, 14, 16, 18, 20, 22, 24, 26, 28, 30, 32, 34, 36, 38, 40, 40,
        42, 44, 46),
    p_att=(52,),
    p_w=(10, 19, 30, 44, 48),
    p_g=(0, 1, 2, 3, 4, 5, 6, 7, 9, 10, 11, 12, 13, 14, 15, 16, 18, 19, 20, 21, 22, 23,
        24, 25, 27, 28, 29, 30, 31, 32, 33, 34, 36, 37, 38, 39, 40, 41, 42, 43, 45, 46,
        47, 48, 49, 50, 51, 53),
)


def _run(A_x, A_wqkv, A_wo, B_w_gate, B_w_up, B_w_down, **kw):
    _, S, D = A_x.shape
    F = B_w_gate.shape[1]
    kernel, scratch = _make_kernel(S, D, F, 256, {**_CFG, **kw})
    hbm = pl.BlockSpec(memory_space=pl.ANY)
    out_t = pl.pallas_call(
        kernel,
        in_specs=[hbm] * 6,
        out_specs=hbm,
        out_shape=jax.ShapeDtypeStruct((D, S), A_x.dtype),
        scratch_shapes=scratch,
        compiler_params=pltpu.CompilerParams(vmem_limit_bytes=110 * 1024 * 1024),
    )(A_x.reshape(S, D).T, A_wqkv, A_wo, B_w_gate, B_w_up, B_w_down.T)
    return out_t.T.reshape(A_x.shape)


@jax.jit
def pallas_interleave_layers__sliding_local_dilated__glu_gated_geglu__prompt_kernel(
    A_x: jax.Array,
    A_wqkv: jax.Array,
    A_wo: jax.Array,
    B_x: jax.Array,
    B_w_gate: jax.Array,
    B_w_up: jax.Array,
    B_w_down: jax.Array,
):
    del B_x
    return _run(A_x, A_wqkv, A_wo, B_w_gate, B_w_up, B_w_down)
```

```python
import functools

import jax
import jax.numpy as jnp
import jax.experimental.pallas as pl
import jax.experimental.pallas.tpu as pltpu
from jax import lax

H = 32
W = 8
DIL = 2
EPS = 1e-5
LANES = 128

F32 = jnp.float32
BF16 = jnp.bfloat16
U32 = jnp.uint32

_NT = (((1,), (1,)), ((), ()))


def _tree_sum(parts, op=jnp.add):
    while len(parts) > 1:
        nxt = [op(parts[i], parts[i + 1]) for i in range(0, len(parts) - 1, 2)]
        if len(parts) % 2:
            nxt.append(parts[-1])
        parts = nxt
    return parts[0]


def _ln_stats(slabs, d, anchors=()):
    n_acc = 4
    s1, s2, pilot = [None] * n_acc, [None] * n_acc, None
    for i, x in enumerate(slabs):
        if pilot is None:
            pilot = x[0:1, :]
            pil = jnp.broadcast_to(pilot, x.shape)
            pils = [_tie(pil, a) for a in anchors] or [pil]
        dx = x - pils[i * len(pils) // (d // 8)]
        j = i % n_acc
        s1[j] = dx if s1[j] is None else s1[j] + dx
        s2[j] = dx * dx if s2[j] is None else s2[j] + dx * dx
    e1 = jnp.sum(_tree_sum(s1), axis=0, keepdims=True) * (1.0 / d)
    e2 = jnp.sum(_tree_sum(s2), axis=0, keepdims=True) * (1.0 / d)
    var = jnp.maximum(e2 - e1 * e1, 0.0)
    return pilot + e1, lax.rsqrt(var + EPS)


def _zero_like_dep(v):
    return (lax.bitcast_convert_type(v, U32) >> 31) >> 1


def _tie(x, anchor):
    if anchor is None:
        return x
    z = lax.bitcast_convert_type(_zero_like_dep(anchor), F32)
    z = jnp.concatenate([z] * (x.shape[1] // LANES), axis=1)
    if x.shape[0] == 8:
        return x + z
    return jnp.concatenate([x[:8] + z, x[8:]], axis=0)


def _gelu_mul2(g, u):
    c0 = 0.7978845608028654
    c1 = c0 * 0.044715
    t = jnp.tanh(g * (c0 + c1 * (g * g)))
    return (g * u) * (1.0 + t)


def _lo(x):
    return lax.bitcast_convert_type(x << 16, F32)


def _hi(x):
    return lax.bitcast_convert_type(x & jnp.uint32(0xFFFF0000), F32)


def _pk(x):
    return pltpu.bitcast(x.astype(BF16), U32)


def _upk(x):
    return pltpu.bitcast(x, BF16)


def _dot(a, b):
    return jnp.dot(a, b, preferred_element_type=F32)


def _dot_nt(a, b):
    return lax.dot_general(a, b, _NT, preferred_element_type=F32)


def _x_ops(x1, x2):
    d = [a - b for a, b in zip(x1, x2)]
    return [x1[0] + x2[1], x2[0] + x2[1], x1[0] + x1[1],
            d[1] + x1[2], x1[1] + x1[2], d[1] + d[2],
            d[0] - x2[2], d[0] + d[2], x2[0] + x2[2],
            x1[0], d[0], x2[1], d[1], x1[2], x2[2]]


def _x_rem(x1, x2):
    a, b, c = 0, 1, 2
    cat = lambda u, v: jnp.concatenate([u, v], axis=0)
    return [cat(x1[c], x2[b]), cat(x1[a], x1[b] - x2[b]), cat(x2[a], x2[c] - x1[c])]


def _w_sums(w):
    return [w[0][1] + w[1][0], w[1][2] + w[2][1], w[0][2] + w[2][0],
            w[0][0] + w[0][2] - w[1][0], w[2][0] - w[0][0] - w[0][1],
            w[1][1] + w[1][2] - w[0][1], w[1][0] + w[1][1] - w[2][1],
            w[2][0] + w[2][2] - w[1][2], w[2][1] + w[2][2] - w[0][2]]


_W_TERMS = {0: ((0, 1, 1), (1, 0, 1)), 3: ((1, 2, 1), (2, 1, 1)), 6: ((0, 2, 1), (2, 0, 1)),
            9: ((0, 0, 1), (0, 2, 1), (1, 0, -1)), 10: ((2, 0, 1), (0, 0, -1), (0, 1, -1)),
            11: ((1, 1, 1), (1, 2, 1), (0, 1, -1)), 12: ((1, 0, 1), (1, 1, 1), (2, 1, -1)),
            13: ((2, 0, 1), (2, 2, 1), (1, 2, -1)), 14: ((2, 1, 1), (2, 2, 1), (0, 2, -1)),
            1: ((0, 1, 1),), 2: ((1, 0, 1),), 4: ((1, 2, 1),), 5: ((2, 1, 1),),
            7: ((2, 0, 1),), 8: ((0, 2, 1),)}
_PARTS = ((1, 2, 0), (7, 8, 6), (4, 5, 3), (9, 10, 11, 12, 13, 14))
_W_SUM = {0: 0, 3: 1, 6: 2, 9: 3, 10: 4, 11: 5, 12: 6, 13: 7, 14: 8}
_W_RAW = {1: (0, 1), 2: (1, 0), 4: (1, 2), 5: (2, 1), 7: (2, 0), 8: (0, 2)}
_PAIR_ORDER = (1, 2, 4, 5, 7, 8, 0, 3, 6)
_DIAG = {(0, 0): 9, (2, 0): 10, (0, 1): 11, (1, 1): 12, (1, 2): 13, (2, 2): 14}
_PAIR = {(0, 0): ((6, -1), (8, -1)), (1, 0): ((2, 1), (7, 1)), (2, 0): ((0, 1), (1, -1)),
         (0, 1): ((3, 1), (4, -1)), (1, 1): ((0, 1), (2, -1)), (2, 1): ((1, 1), (5, -1)),
         (0, 2): ((4, 1), (8, 1)), (1, 2): ((6, 1), (7, -1)), (2, 2): ((5, 1), (3, -1))}


def _column(t, base, j):
    s = []
    for k in range(3):
        v = base[k]
        for i, sg in _PAIR[k, j]:
            ti = t[i]() if callable(t[i]) else t[i]
            v = ti if v is None else (v + ti if sg > 0 else v - ti)
        s.append(v)
    return s[1] + s[0], s[2] + s[0]


def _make_kernel(S, D, F, TM, cfg):
    NB = S // TM
    NT = TM // LANES
    DH = D // H
    DP = DH // 2
    RP = D // 2
    NG = H // 8
    scale = float(DH) ** -0.5
    NU = 2 * NB
    TH = TM // 2
    FT = F // 3
    D2 = D // 2
    D3 = D // 3
    Q3 = D3 // 2
    KU = D // 9
    KR = 3 * LANES
    NQ = 6
    QR = 3 * D // NQ
    WQ = (0, 640, 1152, 3 * D)
    PW = 256
    NP = FT // PW
    scopes = cfg['scopes']
    assert NG == 4 and NB & (NB - 1) == 0
    SEM_P = 4

    def kernel(x_hbm, wqkv_hbm, wo_hbm, wg_hbm, wu_hbm, wdt_hbm, out_hbm,
               xio_s, wqkv_v, wo_v, wg_v, wu_v, wdt_v, wt_s, wl_s,
               gs_s, us_s, ds_s, xmid_s, a_s, qkv_s, o_s, acc_s, b_s, r_s, t_s,
               sem_i, sem_o):

        def wait(name, cps):
            if scopes:
                with jax.named_scope(name):
                    for cp in cps:
                        cp.wait()
            else:
                for cp in cps:
                    cp.wait()

        def cols(lo, n):
            if not isinstance(lo, int):
                lo = pl.multiple_of(lo, LANES)
            return pl.ds(lo, n)

        def rows8(lo, n=8):
            if not isinstance(lo, int):
                lo = pl.multiple_of(lo, 8)
            return pl.ds(lo, n)

        def out_copy(b):
            return pltpu.make_async_copy(
                xio_s.at[b], out_hbm.at[:, cols(b * TM, TM)], sem_o.at[0])

        def x_cp(b, sem):
            return pltpu.make_async_copy(x_hbm.at[:, cols(b * TM, TM)], xio_s.at[b],
                                         sem_i.at[sem])

        def wq_cp(i):
            sl = cols(WQ[i], WQ[i + 1] - WQ[i])
            return pltpu.make_async_copy(wqkv_hbm.at[:, sl], wqkv_v.at[:, sl],
                                         sem_i.at[1 + i])

        def piece_cp(src, dst, p, sem):
            return [pltpu.make_async_copy(src.at[:, cols(j * FT + p * PW, PW)],
                                          dst.at[p, j],
                                          sem_i.at[sem]) for j in range(3)]

        def group_cp(p):
            sem = SEM_P + p
            cps = []
            if isinstance(p, int) and p == 0:
                cps.append(pltpu.make_async_copy(wo_hbm, wo_v, sem_i.at[sem]))
            if not (isinstance(p, int) and p == NP):
                cps += piece_cp(wg_hbm, wg_v, p, sem) + piece_cp(wu_hbm, wu_v, p, sem)
            if not (isinstance(p, int) and p == 0):
                cps += piece_cp(wdt_hbm, wdt_v, p - 1, sem)
            return cps

        lane = lax.broadcasted_iota(jnp.int32, (8, LANES), 1)
        cat0 = lambda *v: jnp.concatenate(v, axis=0)
        cat1 = lambda *v: jnp.concatenate(v, axis=1)

        def spread_over(anchors, n, total):
            return anchors[n * len(anchors) // total] if anchors else None

        def slab_group(r):
            return (r % LANES) // 16 if r < KR else 8 + ((r - KR) % KU) // 16

        def ln1(blk, anchors1, anchors2=()):
            slabs = (xio_s[blk, r:r + 8, :].astype(F32) for r in range(0, D, 8))
            m, rs = _ln_stats(slabs, D, anchors1)
            if not anchors2:
                return (xio_s[blk].astype(F32) - m) * rs
            m8 = jnp.broadcast_to(m, (8, TM))
            ms = [_tie(m8, a) for a in anchors2]
            ms = [spread_over(ms, slab_group(r), 12) for r in range(0, D, 8)]
            return (xio_s[blk].astype(F32) - cat0(*ms)) * rs

        def dot_k(rows, x, anchors):
            y = None
            for n, k in enumerate(range(0, D, LANES)):
                ks = slice(k, min(k + LANES, D))
                v = _dot(_upk(wt_s[rows, ks]), x[ks])
                anchors.extend(v[r:r + 8, :LANES] for r in ((0, 144) if n % 2 else (72, 216)))
                y = v if y is None else y + v
            return y

        def put_qkv(blk, rows, y):
            pk = _pk(y)
            for c in range(NT):
                qkv_s[1 + blk * NT + c, rows, :] = pk[:, c * LANES:(c + 1) * LANES]

        def qkv_mm(blk, xn, chunks, anchors):
            for r in chunks:
                rows = slice(r * QR // 2, (r + 1) * QR // 2)
                put_qkv(blk, rows, dot_k(rows, xn, anchors))

        def split_k(x):
            hs = (x[:, :TH], x[:, TH:])
            blocks = [[h[k * LANES:(k + 1) * LANES] for k in range(3)] for h in hs]
            units = [[h[KR + k * KU:KR + (k + 1) * KU] for k in range(3)] for h in hs]
            return blocks, units

        def prep_att(pat, anchor):
            assert Q3 == 96
            row0 = pat * 8
            src0 = row0 + ((pat * 43) >> 9) * (2 * Q3)
            w = [_upk(wt_s[rows8(src0 + j * Q3), :D]).astype(F32) for j in range(3)]
            w[0] = cat1(_tie(w[0][:, :LANES], anchor), w[0][:, LANES:])
            tiles = _w_sums([[w[j][:, k * LANES:(k + 1) * LANES] for j in range(3)]
                             for k in range(3)])
            for j in range(3):
                a, b, c = (w[j][:, KR + k * KU:KR + (k + 1) * KU] for k in range(3))
                tiles += [cat1(c, b), cat1(a, c)]
            wl_s[rows8(row0), :15 * LANES] = _pk(cat1(*tiles))

        def att_rhs(x, stash=None):
            blocks, units = split_k(x)
            ops = _x_ops(*blocks) + _x_rem(*units)
            if stash is None:
                return [v.astype(BF16) for v in ops]
            loc = lambda i, r0, n: (slice((i // 2) * 64 + r0, (i // 2) * 64 + r0 + n),
                                    slice((i % 2) * LANES, (i % 2 + 1) * LANES))
            for r in range(0, LANES, 16):
                for i, v in enumerate(ops):
                    r_s.at[0][loc(i, r // 2, 8)] = _pk(v[r:r + 16])
            return [_upk(r_s.at[stash][loc(i, 0, 64)]) for i in range(18)]

        def att_mm(sec, rhs, anchors):
            tl = lambda i: _upk(wl_s[sec * Q3:(sec + 1) * Q3, i * LANES:(i + 1) * LANES])
            raw = lambda k, j: _upk(wt_s[(3 * sec + j) * Q3:(3 * sec + j + 1) * Q3,
                                         k * LANES:(k + 1) * LANES])
            t = {}
            for i in _PAIR_ORDER:
                t[i] = _dot(raw(*_W_RAW[i]) if i in _W_RAW else tl(_W_SUM[i]), rhs[i])
                anchors.append(t[i][:8])
            out = []
            for j in range(3):
                base = []
                for s in range(3):
                    v = _dot(raw(3, j) if s == 1 else tl(9 + 2 * j + s // 2), rhs[15 + s])
                    if (s, j) in _DIAG:
                        i = _DIAG[s, j]
                        v = _dot(tl(_W_SUM[i]), rhs[i]) + v
                    base.append(v)
                    anchors.append(base[-1][:8])
                out.append(cat1(*_column(t, base, j)))
            return cat0(*out)

        def qkv_fast(blk, rhs, anchors):
            for sec in range(3):
                put_qkv(blk, slice(sec * RP, (sec + 1) * RP), att_mm(sec, rhs, anchors))

        def shifted(ln, cur, prev, w):
            if w == 0:
                return cur
            sh = DIL * w
            return pltpu.roll(jnp.where(ln < LANES - sh, cur, prev), sh, axis=1)

        def att_group(blk, c, hg, anchor, win):
            tile = blk * NT + c
            base = hg * 8 * DP
            if isinstance(hg, int):
                cur, prev, o_t = qkv_s.at[1 + tile], qkv_s.at[tile], o_s.at[c]
            else:
                n = 2 * RP + 8 * DP
                base = pl.multiple_of(base, 8)
                cur = qkv_s.at[1 + tile, pl.ds(base, n)]
                prev = qkv_s.at[tile, pl.ds(base, n)]
                o_t = o_s.at[c, pl.ds(base, RP + 8 * DP)]
                base = 0
            ln = lane + _zero_like_dep(anchor).astype(jnp.int32)
            logits = [None] * W
            done = []
            for dd in range(DP):
                q = cur[pl.ds(base + dd, 8, stride=DP), :]
                kc = cur[pl.ds(RP + base + dd, 8, stride=DP), :]
                if dd >= win:
                    kc = kc | _zero_like_dep(done[dd - win])
                kp = prev[pl.ds(RP + base + dd, 8, stride=DP), :]
                q0, q1 = _lo(q), _hi(q)
                for w in range(W):
                    ks = shifted(ln, kc, kp, w)
                    t = q0 * _lo(ks) + q1 * _hi(ks)
                    logits[w] = t if logits[w] is None else logits[w] + t
                done.append(ks)
            logits = [l * scale for l in logits]
            if not (isinstance(c, int) and c > 0):
                pos = lane + tile * LANES
                logits = [l if w == 0 else jnp.where(pos >= DIL * w, l, -1e9)
                          for w, l in enumerate(logits)]
            m = _tree_sum(logits, jnp.maximum)
            ln = lane + _zero_like_dep(m).astype(jnp.int32)
            e = [jnp.exp(l - m) for l in logits]
            den = _tree_sum(e)
            if cfg['rcp']:
                r = pl.reciprocal(den, approx=True)
                r = r * (2.0 - den * r)
            else:
                r = 1.0 / den
            p = e if cfg['late'] else [x * r for x in e]
            done = []
            for dd in range(DP):
                vc = cur[pl.ds(2 * RP + base + dd, 8, stride=DP), :]
                if dd >= win:
                    vc = vc | _zero_like_dep(done[dd - win])
                vp = prev[pl.ds(2 * RP + base + dd, 8, stride=DP), :]
                o0 = o1 = None
                for w in range(W):
                    vs = shifted(ln, vc, vp, w)
                    t0, t1 = p[w] * _lo(vs), p[w] * _hi(vs)
                    o0 = t0 if o0 is None else o0 + t0
                    o1 = t1 if o1 is None else o1 + t1
                done.append(vs)
                if cfg['late']:
                    o0, o1 = o0 * r, o1 * r
                o_t[pl.ds(base + dd, 8, stride=DP), :] = o0
                o_t[pl.ds(RP + base + dd, 8, stride=DP), :] = o1

        def attention(blk, anchors, win):
            for c in range(NT):
                for hg in range(NG):
                    att_group(blk, c, hg, anchors[c * NG + hg], win)

        def wo_mm(blk, anchors, fast, anchors_in=(), stash=None):
            o = cat1(*[o_s[c] for c in range(NT)])
            if anchors_in:
                o = cat0(*[_tie(o[r:r + 8], spread_over(anchors_in, slab_group(r), 12))
                           for r in range(0, D, 8)])
            if fast:
                y = att_mm(3, att_rhs(o, stash), anchors)
            else:
                o = o.astype(BF16)
                q = D2 // 2
                y = cat0(*[dot_k(slice(h * q, (h + 1) * q), o, anchors) for h in (6, 7)])
            xm = xio_s[blk].astype(F32) + y
            xmid_s[blk] = xm
            return _ln_stats((xm[r:r + 8] for r in range(0, D, 8)), D)

        def ffn_lhs(blk, stats, anchors):
            m, rs = stats
            m8 = jnp.broadcast_to(m, (8, TM))
            xs = []
            for k in range(3):
                mt = cat0(*[_tie(m8, spread_over(anchors, k, 3))] * (D3 // 8))
                xs.append((xmid_s[blk, k * D3:(k + 1) * D3, :] - mt) * rs)
            ops = _x_ops([x[:, :TH] for x in xs], [x[:, TH:] for x in xs])
            for i, v in enumerate(ops):
                for s, t in enumerate((v[KU:], v[:2 * KU], cat0(v[:KU], v[2 * KU:]))):
                    a_s[3 * i + s] = _pk(t.astype(BF16).T)

        def plain_lhs(blk, stats):
            m, rs = stats
            blocks, units = split_k((xmid_s[blk] - m) * rs)
            for i, v in enumerate(blocks[0] + blocks[1] + _x_rem(*units)):
                a_s[i] = _pk(v.astype(BF16).T)

        def plain_piece(p, anchors):
            h = {}
            for j in range(3):
                hs = []
                for n in range(PW // LANES):
                    cs = slice(n * LANES, (n + 1) * LANES)
                    w = lambda r0, r1: cat1(wg_v[p, j, r0:r1, cs], wu_v[p, j, r0:r1, cs])
                    u = lambda k: w(KR + k * KU, KR + (k + 1) * KU)
                    tl = lambda *i: _upk(cat1(*[a_s[k] for k in i]))
                    y0 = _dot(tl(6), cat0(u(2), u(1)))
                    y1 = _dot(tl(0, 1, 2, 7), w(0, KR + 2 * KU))
                    y2 = _dot(tl(3, 4, 5, 8), cat0(w(0, KR + KU), u(2)))
                    for y in (y0, y1, y2):
                        anchors.extend(y[r:r + 8, c:c + LANES]
                                       for c in ((0,) if y is y0 else (0, LANES))
                                       for r in ((0,) if y is y0 else (0, TH // 2)))
                    hs.append([_gelu_mul2(*[(y + y0)[:, c:c + LANES] for c in (0, LANES)])
                               for y in (y1, y2)])
                h[j] = [cat1(*[v[i] for v in hs]) for i in range(2)]
            return h_ops(h)

        def prep_d(p, anchors):
            PR = 16
            for n in range(2 * D3 // PR):
                r, cs = (n // 2) * PR, slice((n % 2) * LANES, (n % 2 + 1) * LANES)
                w = [[wdt_v[p, k, j * D3 + r:j * D3 + r + PR, cs].astype(F32)
                      for j in range(3)] for k in range(3)]
                w[0][1] = _tie(w[0][1], spread_over(anchors, n, 2 * D3 // PR))
                for i, v in enumerate(_w_sums(w)):
                    ds_s.at[p, i][r // 2:(r + PR) // 2, cs] = _pk(v)

        GU = ((wg_v, gs_s), (wu_v, us_s))

        def prep_gu(p, anchors):
            PR = 16
            nr = D3 // PR
            for n in range(4 * nr):
                c, (w_v, s_s), r = n % 2, GU[(n // 2) % 2], (n // 4) * PR
                cache = {}

                def w(k, j):
                    if (k, j) not in cache:
                        ld = lambda c: w_v[p, j, k * D3 + r:k * D3 + r + PR,
                                           c * LANES:(c + 1) * LANES].astype(F32)
                        v = ld(c)
                        if k != j:
                            v = _tie(v, spread_over(anchors, n, 4 * nr))
                        cache[k, j] = v - ld(1 - c) if r // KU == 1 + c else v
                    return cache[k, j]

                for i in range(15):
                    v = None
                    for k, j, sg in _W_TERMS[i]:
                        v = w(k, j) if v is None else (v + w(k, j) if sg > 0 else v - w(k, j))
                    s_s.at[p, i][r // 2:(r + PR) // 2, c * LANES:(c + 1) * LANES] = _pk(v)

        NS = cfg['msplit']

        def gu_prod(p, i, t, anchors, slabs, slot=0):
            u = KU // 2

            def rhs(s, s_s):
                if s == 1:
                    return s_s[p, i, :2 * u, :LANES]
                if s == 0:
                    return cat0(s_s[p, i, u:2 * u, LANES:], s_s[p, i, 2 * u:, :LANES])
                return cat0(s_s[p, i, :u, LANES:], s_s[p, i, 2 * u:, LANES:])

            q = TH // 2 // NS
            for n, h in enumerate(slabs):
                y = []
                for s in range(3):
                    r = _upk(cat1(rhs(s, gs_s), rhs(s, us_s)))
                    y.append(_dot(_upk(a_s[3 * i + s, h * q:(h + 1) * q]), r))
                    if (3 * n + s) % len(slabs) == 0:
                        anchors.append(y[-1][:8, :LANES])
                y1, y2 = y[1] + y[0], y[2] + y[0]
                for m in range(2):
                    cs = slice(m * LANES, (m + 1) * LANES)
                    v = cat1(y1[:, cs], y2[:, cs])
                    if i < 9 and 't' in cfg['stash']:
                        k = p if isinstance(p, int) else slot
                        t_s[k, m, i, 2 * h * q:2 * (h + 1) * q] = v
                        v = lambda k=k, m=m, h=h: t_s[k, m, i, 2 * h * q:2 * (h + 1) * q]
                    t.setdefault((m, h), {})[i] = v

        def gu_col(t, hv, p, j, anchors, slabs):
            ids = [_DIAG.get((s, j)) for s in range(3)]
            if cfg['fslab']:
                for h in slabs:
                    for i in ids:
                        if i is not None:
                            gu_prod(p, i, t, anchors if h == slabs[0] else [], [h])
            else:
                for i in ids:
                    if i is not None:
                        gu_prod(p, i, t, anchors, slabs)
            for h in slabs:
                g, u = [_column(t[m, h], [None if i is None else t[m, h][i] for i in ids], j)
                        for m in range(2)]
                hv[j, h] = [_gelu_mul2(g[i], u[i]) for i in range(2)]

        def h_ops(h):
            return [v.astype(BF16) for v in _x_ops(*[[h[j][i] for j in range(3)]
                                                     for i in range(2)])]

        def h_join(hv):
            return h_ops({j: [cat0(*[hv[j, h][i] for h in range(NS)]) for i in range(2)]
                          for j in range(3)})

        def gu_piece(p, order, anchors, slot):
            t, hv = {}, {}
            for slabs in ([[h] for h in range(NS)] if cfg['slab'] else [list(range(NS))]):
                for step in order:
                    if step[0] == 'S':
                        for i in _PARTS[int(step[1])]:
                            gu_prod(p, i, t, anchors, slabs, slot)
                    else:
                        gu_col(t, hv, p, int(step[1]), anchors, slabs)
            return h_join(hv)

        D_ORDER = _PAIR_ORDER + (9, 10, 11, 12, 13, 14)

        def down_mm(acc, bs, lo, anchors, which=D_ORDER, fine=False):
            p = [None] * 15 if acc is None else list(acc)
            for i in which:
                y = None
                for n, b in enumerate(bs):
                    if i in _W_RAW:
                        k, j = _W_RAW[i]
                        v = _dot_nt(wdt_v[lo + n, k, j * D3:(j + 1) * D3, :], b[i])
                    elif len(bs) % 2 and i == 14 and n == 0:
                        v = cat0(*[_dot_nt(_upk(ds_s[lo, _W_SUM[i],
                                                     h * Q3 // 2:(h + 1) * Q3 // 2, :]), b[i])
                                   for h in range(2)])
                    else:
                        v = _dot_nt(_upk(ds_s[lo + n, _W_SUM[i]]), b[i])
                    y = v if y is None else y + v
                p[i] = y if p[i] is None else p[i] + y
                anchors.append(p[i][:8])
                if fine:
                    anchors.append(p[i][D3 // 2:D3 // 2 + 8])
            return p

        def finish(blk, acc):
            y = [cat1(*_column(acc, [acc[_DIAG[s, j]] if (s, j) in _DIAG else None
                                     for s in range(3)], j)) for j in range(3)]
            xio_s[blk] = (xmid_s[blk] + 0.5 * cat0(*y)).astype(BF16)

        def load_acc(k):
            return [acc_s[k, i] for i in range(15)]

        def store_acc(k, acc):
            for i in range(15):
                acc_s[k, i] = acc[i]

        def load_b(k=0):
            return [_upk(b_s[i * TH // 2:(i + 1) * TH // 2, :])
                    for i in range(15 * k, 15 * k + 15)]

        def store_b(b, k=0):
            for i in range(15):
                b_s[(15 * k + i) * TH // 2:(15 * k + i + 1) * TH // 2, :] = _pk(b[i])

        def pre_phase():
            x0_cp, x1_cp = x_cp(0, 0), x_cp(1, 3)
            order = [x0_cp, wq_cp(0), wq_cp(1), x1_cp, wq_cp(2)]
            for p in range(NP + 1):
                order += group_cp(p)
            xr_cp = [x_cp(b, SEM_P + NP + 1) for b in range(2, NB)]
            order += xr_cp
            for cp in order:
                cp.start()
            get = lambda an, name: [an[min(i, len(an) - 1)] for i in cfg[name]]
            e_grp = lambda e: ((e >> 1) & 1, ((e >> 2) << 1) | (e & 1))
            if 'a' in cfg['sub']:
                pre_a(x0_cp, x1_cp, get, e_grp)
            if 'b' in cfg['sub']:
                pre_b(get, e_grp)
            if 'c' in cfg['sub']:
                pre_c(get)
            wait('WX', xr_cp)

        def pre_a(x0_cp, x1_cp, get, e_grp):
            qkv_s[0] = jnp.zeros(qkv_s.shape[1:], U32)
            acc_s[...] = jnp.zeros(acc_s.shape, F32)
            wait('WX0', [x0_cp])
            xn0 = ln1(0, ()).astype(BF16)
            done = 0
            for i in range(3):
                wait('WQ%d' % i, [wq_cp(i)] + ([x1_cp] if i == 2 else []))
                wt = _pk(wqkv_v[:, WQ[i]:WQ[i + 1]].T)
                wt_s[WQ[i] // 2:WQ[i + 1] // 2, :D] = wt
                anchors = []
                qkv_mm(0, xn0, range(done, WQ[i + 1] // QR), anchors)
                done = WQ[i + 1] // QR
                if i > 0:
                    for n, a in enumerate(get(anchors, 'a_w%d' % i)):
                        prep_att(12 * (i - 1) + n, a)
            xn1 = ln1(1, get(anchors, 'a_ln'), get(anchors, 'a_lnb')).astype(BF16)
            qkv_mm(1, xn1, (0, 2, 4, 1), anchors)
            for e in range(8):
                att_group(0, *e_grp(e), anchors[cfg['att0'][e]], 9)
            wait('WO', group_cp(0))
            wo = pltpu.bitcast(wo_v[...], U32)
            wt_s[3 * RP:, :D] = _pk(cat0(_lo(wo), _hi(wo)).astype(BF16).T)
            an = []
            stats = wo_mm(0, an, False)
            qkv_mm(1, xn1, [3], an)
            plain_lhs(0, stats)
            b = plain_piece(0, an)
            qkv_mm(1, xn1, [5], an)
            prep_gu(0, get(an, 'z_g'))
            for e in range(3):
                att_group(1, *e_grp(e), an[cfg['z_att'][e]], 9)
            store_b(b)

        def pre_b(get, e_grp):
            def piece(p, carry):
                wait('WP', group_cp(p))
                b_prev = load_b()
                an = []
                b = plain_piece(p, an)
                prep_d(p - 1, get(an, 'p_d'))
                store_acc(0, down_mm(load_acc(0), [b_prev], p - 1, an))
                prep_gu(p, get(an, 'p_g'))
                att_group(1, *e_grp(p + 2), an[cfg['p_att'][0]], 9)
                for i, a in enumerate(get(an, 'p_w')):
                    prep_att(jnp.minimum(24 + (p - 1) * 5 + i, 47), a)
                store_b(b)
                return carry

            lax.fori_loop(1, NP, piece, 0)

        def pre_c(get):
            wait('WD', group_cp(NP))
            an = []
            stats = wo_mm(1, an, True)
            prep_d(NP - 1, get(an, 't_d'))
            acc = down_mm(load_acc(0), [load_b()], NP - 1, [])
            ffn_lhs(1, stats, [])
            finish(0, acc)

        if 'pre' in cfg['phases']:
            pre_phase()

        def body(u, carry):
            bu = u & (NB - 1)
            ba = (u + 1) & (NB - 1)
            acc, stats, an, b = None, None, {}, {}
            get = lambda name: [an[k][i] for k, i in cfg[name]]
            for step in cfg['body']:
                an[step] = []
                if step == 'Q':
                    qkv_fast(ba, att_rhs(ln1(ba, get('ln1'), get('ln1b')), u >> 8 if 'q' in cfg['stash'] else None),
                             an[step])
                elif step == 'W':
                    attention(ba, get('att'), cfg['win'])
                    stats = wo_mm(ba, an[step], True, get('orhs'),
                                  u >> 8 if 'w' in cfg['stash'] else None)
                elif step == 'L':
                    ffn_lhs(ba, stats, get('lhs'))
                elif step[0] == 'S':
                    slabs = [int(step[3])] if len(step) > 3 else list(range(NS))
                    for i in _PARTS[int(step[2])]:
                        gu_prod(int(step[1]), i, b.setdefault(step[:2], {}), an[step], slabs)
                elif step[0] == 'F':
                    j, c = int(step[1]), int(step[2])
                    slabs = [int(step[3])] if len(step) > 3 else list(range(NS))
                    hv = b.setdefault(step[:2], {})
                    gu_col(b['S' + step[1]], hv, j, c, an[step], slabs)
                    if len(hv) == 3 * NS:
                        b[j] = h_join(hv)
                        if 'b' in cfg['stash']:
                            store_b(b[j], j)
                            b[j] = load_b(j)
                else:
                    js = [int(c) for c in step[1:]]
                    acc = down_mm(acc, [b[j] for j in js], js[0], an[step])
            finish(bu, acc)

            @pl.when(u >= NB)
            def _():
                out_copy(bu).start()
            return carry

        if scopes:
            with jax.named_scope('LOOP'):
                lax.fori_loop(1, NU - 1, body, 0)
        elif 'main' in cfg['phases']:
            lax.fori_loop(1, NU - 1, body, 0)

        def last(c, carry):
            los = [2 * c + j for j in range(2)]
            b = [gu_piece(lo, cfg['order'], [], j) for j, lo in enumerate(los)]
            acc = load_acc(1)
            for j in range(2):
                acc = down_mm(acc, [b[j]], los[j], [])
            store_acc(1, acc)
            return carry

        if 'last' in cfg['phases']:
            lax.fori_loop(0, NP // 2, last, 0)
        if len(cfg['phases']) < 3:
            def keep(i, c):
                v = (gs_s[i, i, :8, :LANES] + us_s[i, i, :8, :LANES] + ds_s[i, i, :8, :LANES]
                     + wl_s[rows8(i * 8), :LANES] + a_s[i, :8] + qkv_s[i, :8]
                     + b_s[rows8(i * 8), :LANES] + wt_s[rows8(i * 8), :LANES])
                acc_s[1, 0, :8] = (lax.bitcast_convert_type(v, F32) + o_s[i, :8]
                                   + acc_s[i, i, :8])
                return c
            lax.fori_loop(0, 2, keep, 0)
        finish(NB - 1, load_acc(1))
        out_copy(NB - 1).start()
        wait('WOUT', [out_copy(b) for b in range(NB)])

    scratch = [
        pltpu.VMEM((NB, D, TM), BF16),
        pltpu.VMEM((D, 3 * D), BF16),
        pltpu.VMEM((D, D), BF16),
        pltpu.VMEM((NP, 3, D, PW), BF16),
        pltpu.VMEM((NP, 3, D, PW), BF16),
        pltpu.VMEM((NP, 3, D, PW), BF16),
        pltpu.VMEM((2 * D, 8 * LANES), U32),
        pltpu.VMEM((4 * Q3, 16 * LANES), U32),
        pltpu.VMEM((NP, 15, Q3, PW), U32),
        pltpu.VMEM((NP, 15, Q3, PW), U32),
        pltpu.VMEM((NP, 9, Q3, PW), U32),
        pltpu.VMEM((NB, D, TM), F32),
        pltpu.VMEM((45, TH // 2, LANES), U32),
        pltpu.VMEM((S // LANES + 1, 3 * RP, LANES), U32),
        pltpu.VMEM((NT, D, LANES), F32),
        pltpu.VMEM((2, 15, D3, TH), F32),
        pltpu.VMEM((NP * 15 * TH // 2, PW), U32),
        pltpu.VMEM((1, 9 * 64, 2 * LANES), U32),
        pltpu.VMEM((NP, 2, 9, TH, PW), F32),
        pltpu.SemaphoreType.DMA((SEM_P + NP + 2,)),
        pltpu.SemaphoreType.DMA((1,)),
    ]
    return kernel, scratch


_CFG = dict(
    scopes=False,
    rcp=False,
    late=True,
    stash='qw',
    slab=True,
    fslab=False,
    win=9,
    sub='abc',
    orhs=(),
    msplit=2,
    phases=('pre', 'main', 'last'),
    order=('S0', 'S1', 'F0', 'S2', 'F1', 'F2'),
    body=('S010', 'S000', 'F000', 'S020', 'F010', 'F020', 'S001', 'S011', 'F001',
        'S021', 'F011', 'F021', 'S100', 'S110', 'F100', 'S120', 'S101', 'F110', 'Q',
        'F120', 'S111', 'F101', 'S121', 'F111', 'F121', 'S200', 'S210', 'F200', 'S220',
        'F210', 'F220', 'S300', 'S201', 'S211', 'F201', 'S221', 'F211', 'F221', 'S310',
        'D01', 'F300', 'S320', 'S301', 'F310', 'S311', 'F301', 'S321', 'F311', 'F321',
        'S400', 'F320', 'S420', 'F410', 'S410', 'F400', 'S401', 'F420', 'S411', 'S421',
        'F411', 'F401', 'F421', 'S500', 'S501', 'S510', 'D23', 'F500', 'S520', 'W',
        'F520', 'S511', 'F510', 'F501', 'S521', 'F511', 'F521', 'D4', 'D5', 'L'),
    ln1=(('S010', 4), ('S010', 5), ('S010', 6), ('S010', 7), ('S010', 8), ('S000', 0),
        ('S000', 1), ('S000', 2), ('S000', 3)),
    ln1b=(('S110', 0), ('S110', 1), ('S110', 3), ('S110', 4), ('S110', 6), ('S110', 7),
        ('F100', 0), ('F100', 1), ('F100', 3), ('F100', 4), ('S120', 0), ('S120', 1)),
    att=(('S300', 6), ('D01', 0), ('D01', 6), ('D01', 8), ('D01', 9), ('D23', 0),
        ('D23', 6), ('D23', 10)),
    lhs=(('S511', 1), ('D5', 1), ('D5', 4)),
    att0=(15, 18, 21, 24, 27, 30, 33, 37),
    order0=('S0', 'S1', 'S2', 'F0', 'F1', 'F2'),
    order1=('S0', 'S1', 'S2', 'F0', 'F1', 'F2'),
    a_w1=(0, 1, 2, 3, 5, 5, 8, 9, 10, 11, 12, 14),
    a_w2=(0, 0, 2, 3, 4, 4, 6, 6, 8, 9, 11, 16),
    a_ln=(0, 3, 7),
    a_lnb=(6, 6, 8),
    z_g=(3, 4, 5, 6, 8, 9, 10, 12, 13, 14, 15, 17, 18, 19, 21, 22, 23, 25, 26, 27, 28,
        30, 31, 32, 34, 35, 36, 38, 39, 40, 41, 43, 44, 45, 47, 48, 49, 51, 52, 53, 54,
        56, 57, 58, 60, 61, 62, 64),
    z_att=(72, 75, 78),
    p_g0=(0, 1, 2, 3, 4, 5),
    p_g1=(6, 7, 8, 9, 10, 10),
    p_g2=(12, 13, 14, 15, 16, 17),
    p_g3=(14, 16, 18, 20, 22, 24, 26, 28, 30, 32, 34, 36),
    t_d=(0, 0, 1, 1, 2, 3, 3, 4, 5, 6, 6, 7, 8, 9, 9, 9, 10, 11, 11, 12, 13, 14, 15,
        16),
    p_d=(0, 2, 6, 8, 10, 12, 14, 16, 18, 20, 22, 24, 26, 28, 30, 32, 34, 36, 38, 40, 40,
        42, 44, 46),
    p_att=(52,),
    p_w=(10, 19, 30, 44, 48),
    p_g=(0, 1, 2, 3, 4, 5, 6, 7, 9, 10, 11, 12, 13, 14, 15, 16, 18, 19, 20, 21, 22, 23,
        24, 25, 27, 28, 29, 30, 31, 32, 33, 34, 36, 37, 38, 39, 40, 41, 42, 43, 45, 46,
        47, 48, 49, 50, 51, 53),
)


def _run(A_x, A_wqkv, A_wo, B_w_gate, B_w_up, B_w_down, **kw):
    _, S, D = A_x.shape
    F = B_w_gate.shape[1]
    kernel, scratch = _make_kernel(S, D, F, 256, {**_CFG, **kw})
    hbm = pl.BlockSpec(memory_space=pl.ANY)
    out_t = pl.pallas_call(
        kernel,
        in_specs=[hbm] * 6,
        out_specs=hbm,
        out_shape=jax.ShapeDtypeStruct((D, S), A_x.dtype),
        scratch_shapes=scratch,
        compiler_params=pltpu.CompilerParams(vmem_limit_bytes=110 * 1024 * 1024),
    )(A_x.reshape(S, D).T, A_wqkv, A_wo, B_w_gate, B_w_up, B_w_down.T)
    return out_t.T.reshape(A_x.shape)


@jax.jit
def pallas_interleave_layers__sliding_local_dilated__glu_gated_geglu__prompt_kernel(
    A_x: jax.Array,
    A_wqkv: jax.Array,
    A_wo: jax.Array,
    B_x: jax.Array,
    B_w_gate: jax.Array,
    B_w_up: jax.Array,
    B_w_down: jax.Array,
):
    del B_x
    return _run(A_x, A_wqkv, A_wo, B_w_gate, B_w_up, B_w_down)
```

```python
import functools

import jax
import jax.numpy as jnp
import jax.experimental.pallas as pl
import jax.experimental.pallas.tpu as pltpu
from jax import lax

H = 32
W = 8
DIL = 2
EPS = 1e-5
LANES = 128

F32 = jnp.float32
BF16 = jnp.bfloat16
U32 = jnp.uint32

_NT = (((1,), (1,)), ((), ()))


def _tree_sum(parts, op=jnp.add):
    while len(parts) > 1:
        nxt = [op(parts[i], parts[i + 1]) for i in range(0, len(parts) - 1, 2)]
        if len(parts) % 2:
            nxt.append(parts[-1])
        parts = nxt
    return parts[0]


def _ln_stats(slabs, d, anchors=()):
    n_acc = 4
    s1, s2, pilot = [None] * n_acc, [None] * n_acc, None
    for i, x in enumerate(slabs):
        if pilot is None:
            pilot = x[0:1, :]
            pil = jnp.broadcast_to(pilot, x.shape)
            pils = [_tie(pil, a) for a in anchors] or [pil]
        dx = x - pils[i * len(pils) // (d // 8)]
        j = i % n_acc
        s1[j] = dx if s1[j] is None else s1[j] + dx
        s2[j] = dx * dx if s2[j] is None else s2[j] + dx * dx
    e1 = jnp.sum(_tree_sum(s1), axis=0, keepdims=True) * (1.0 / d)
    e2 = jnp.sum(_tree_sum(s2), axis=0, keepdims=True) * (1.0 / d)
    var = jnp.maximum(e2 - e1 * e1, 0.0)
    return pilot + e1, lax.rsqrt(var + EPS)


def _zero_like_dep(v):
    return (lax.bitcast_convert_type(v, U32) >> 31) >> 1


def _tie(x, anchor):
    if anchor is None:
        return x
    z = lax.bitcast_convert_type(_zero_like_dep(anchor), F32)
    z = jnp.concatenate([z] * (x.shape[1] // LANES), axis=1)
    if x.shape[0] == 8:
        return x + z
    return jnp.concatenate([x[:8] + z, x[8:]], axis=0)


def _gelu_mul2(g, u):
    c0 = 0.7978845608028654
    c1 = c0 * 0.044715
    t = jnp.tanh(g * (c0 + c1 * (g * g)))
    return (g * u) * (1.0 + t)


def _lo(x):
    return lax.bitcast_convert_type(x << 16, F32)


def _hi(x):
    return lax.bitcast_convert_type(x & jnp.uint32(0xFFFF0000), F32)


def _pk(x):
    return pltpu.bitcast(x.astype(BF16), U32)


def _upk(x):
    return pltpu.bitcast(x, BF16)


def _dot(a, b):
    return jnp.dot(a, b, preferred_element_type=F32)


def _dot_nt(a, b):
    return lax.dot_general(a, b, _NT, preferred_element_type=F32)


def _x_ops(x1, x2):
    d = [a - b for a, b in zip(x1, x2)]
    return [x1[0] + x2[1], x2[0] + x2[1], x1[0] + x1[1],
            d[1] + x1[2], x1[1] + x1[2], d[1] + d[2],
            d[0] - x2[2], d[0] + d[2], x2[0] + x2[2],
            x1[0], d[0], x2[1], d[1], x1[2], x2[2]]


def _x_rem(x1, x2):
    a, b, c = 0, 1, 2
    cat = lambda u, v: jnp.concatenate([u, v], axis=0)
    return [cat(x1[c], x2[b]), cat(x1[a], x1[b] - x2[b]), cat(x2[a], x2[c] - x1[c])]


def _w_sums(w):
    return [w[0][1] + w[1][0], w[1][2] + w[2][1], w[0][2] + w[2][0],
            w[0][0] + w[0][2] - w[1][0], w[2][0] - w[0][0] - w[0][1],
            w[1][1] + w[1][2] - w[0][1], w[1][0] + w[1][1] - w[2][1],
            w[2][0] + w[2][2] - w[1][2], w[2][1] + w[2][2] - w[0][2]]


_W_TERMS = {0: ((0, 1, 1), (1, 0, 1)), 3: ((1, 2, 1), (2, 1, 1)), 6: ((0, 2, 1), (2, 0, 1)),
            9: ((0, 0, 1), (0, 2, 1), (1, 0, -1)), 10: ((2, 0, 1), (0, 0, -1), (0, 1, -1)),
            11: ((1, 1, 1), (1, 2, 1), (0, 1, -1)), 12: ((1, 0, 1), (1, 1, 1), (2, 1, -1)),
            13: ((2, 0, 1), (2, 2, 1), (1, 2, -1)), 14: ((2, 1, 1), (2, 2, 1), (0, 2, -1)),
            1: ((0, 1, 1),), 2: ((1, 0, 1),), 4: ((1, 2, 1),), 5: ((2, 1, 1),),
            7: ((2, 0, 1),), 8: ((0, 2, 1),)}
_PARTS = ((1, 2, 0), (7, 8, 6), (4, 5, 3), (9, 10, 11, 12, 13, 14))
_W_SUM = {0: 0, 3: 1, 6: 2, 9: 3, 10: 4, 11: 5, 12: 6, 13: 7, 14: 8}
_W_RAW = {1: (0, 1), 2: (1, 0), 4: (1, 2), 5: (2, 1), 7: (2, 0), 8: (0, 2)}
_PAIR_ORDER = (1, 2, 4, 5, 7, 8, 0, 3, 6)
_DIAG = {(0, 0): 9, (2, 0): 10, (0, 1): 11, (1, 1): 12, (1, 2): 13, (2, 2): 14}
_PAIR = {(0, 0): ((6, -1), (8, -1)), (1, 0): ((2, 1), (7, 1)), (2, 0): ((0, 1), (1, -1)),
         (0, 1): ((3, 1), (4, -1)), (1, 1): ((0, 1), (2, -1)), (2, 1): ((1, 1), (5, -1)),
         (0, 2): ((4, 1), (8, 1)), (1, 2): ((6, 1), (7, -1)), (2, 2): ((5, 1), (3, -1))}


def _column(t, base, j):
    s = []
    for k in range(3):
        v = base[k]
        for i, sg in _PAIR[k, j]:
            ti = t[i]() if callable(t[i]) else t[i]
            v = ti if v is None else (v + ti if sg > 0 else v - ti)
        s.append(v)
    return s[1] + s[0], s[2] + s[0]


def _make_kernel(S, D, F, TM, cfg):
    NB = S // TM
    NT = TM // LANES
    DH = D // H
    DP = DH // 2
    RP = D // 2
    NG = H // 8
    scale = float(DH) ** -0.5
    NU = 2 * NB
    TH = TM // 2
    FT = F // 3
    D2 = D // 2
    D3 = D // 3
    Q3 = D3 // 2
    KU = D // 9
    KR = 3 * LANES
    NQ = 6
    QR = 3 * D // NQ
    WQ = (0, 640, 1152, 3 * D)
    PW = 256
    NP = FT // PW
    scopes = cfg['scopes']
    assert NG == 4 and NB & (NB - 1) == 0
    SEM_P = 4

    def kernel(x_hbm, wqkv_hbm, wo_hbm, wg_hbm, wu_hbm, wdt_hbm, out_hbm,
               xio_s, wqkv_v, wo_v, wg_v, wu_v, wdt_v, wt_s, wl_s,
               gs_s, us_s, ds_s, xmid_s, a_s, qkv_s, o_s, acc_s, b_s, r_s, t_s,
               sem_i, sem_o):

        def wait(name, cps):
            if scopes:
                with jax.named_scope(name):
                    for cp in cps:
                        cp.wait()
            else:
                for cp in cps:
                    cp.wait()

        def cols(lo, n):
            if not isinstance(lo, int):
                lo = pl.multiple_of(lo, LANES)
            return pl.ds(lo, n)

        def rows8(lo, n=8):
            if not isinstance(lo, int):
                lo = pl.multiple_of(lo, 8)
            return pl.ds(lo, n)

        def out_copy(b):
            return pltpu.make_async_copy(
                xio_s.at[b], out_hbm.at[:, cols(b * TM, TM)], sem_o.at[0])

        def x_cp(b, sem):
            return pltpu.make_async_copy(x_hbm.at[:, cols(b * TM, TM)], xio_s.at[b],
                                         sem_i.at[sem])

        def wq_cp(i):
            sl = cols(WQ[i], WQ[i + 1] - WQ[i])
            return pltpu.make_async_copy(wqkv_hbm.at[:, sl], wqkv_v.at[:, sl],
                                         sem_i.at[1 + i])

        def piece_cp(src, dst, p, sem):
            return [pltpu.make_async_copy(src.at[:, cols(j * FT + p * PW, PW)],
                                          dst.at[p, j],
                                          sem_i.at[sem]) for j in range(3)]

        def group_cp(p):
            sem = SEM_P + p
            cps = []
            if isinstance(p, int) and p == 0:
                cps.append(pltpu.make_async_copy(wo_hbm, wo_v, sem_i.at[sem]))
            if not (isinstance(p, int) and p == NP):
                cps += piece_cp(wg_hbm, wg_v, p, sem) + piece_cp(wu_hbm, wu_v, p, sem)
            if not (isinstance(p, int) and p == 0):
                cps += piece_cp(wdt_hbm, wdt_v, p - 1, sem)
            return cps

        lane = lax.broadcasted_iota(jnp.int32, (8, LANES), 1)
        cat0 = lambda *v: jnp.concatenate(v, axis=0)
        cat1 = lambda *v: jnp.concatenate(v, axis=1)

        def spread_over(anchors, n, total):
            return anchors[n * len(anchors) // total] if anchors else None

        def slab_group(r):
            return (r % LANES) // 16 if r < KR else 8 + ((r - KR) % KU) // 16

        def ln1(blk, anchors1, anchors2=()):
            slabs = (xio_s[blk, r:r + 8, :].astype(F32) for r in range(0, D, 8))
            m, rs = _ln_stats(slabs, D, anchors1)
            if not anchors2:
                return (xio_s[blk].astype(F32) - m) * rs
            m8 = jnp.broadcast_to(m, (8, TM))
            ms = [_tie(m8, a) for a in anchors2]
            ms = [spread_over(ms, slab_group(r), 12) for r in range(0, D, 8)]
            return (xio_s[blk].astype(F32) - cat0(*ms)) * rs

        def dot_k(rows, x, anchors):
            y = None
            for n, k in enumerate(range(0, D, LANES)):
                ks = slice(k, min(k + LANES, D))
                v = _dot(_upk(wt_s[rows, ks]), x[ks])
                anchors.extend(v[r:r + 8, :LANES] for r in ((0, 144) if n % 2 else (72, 216)))
                y = v if y is None else y + v
            return y

        def put_qkv(blk, rows, y):
            pk = _pk(y)
            for c in range(NT):
                qkv_s[1 + blk * NT + c, rows, :] = pk[:, c * LANES:(c + 1) * LANES]

        def qkv_mm(blk, xn, chunks, anchors):
            for r in chunks:
                rows = slice(r * QR // 2, (r + 1) * QR // 2)
                put_qkv(blk, rows, dot_k(rows, xn, anchors))

        def split_k(x):
            hs = (x[:, :TH], x[:, TH:])
            blocks = [[h[k * LANES:(k + 1) * LANES] for k in range(3)] for h in hs]
            units = [[h[KR + k * KU:KR + (k + 1) * KU] for k in range(3)] for h in hs]
            return blocks, units

        def prep_att(pat, anchor):
            assert Q3 == 96
            row0 = pat * 8
            src0 = row0 + ((pat * 43) >> 9) * (2 * Q3)
            w = [_upk(wt_s[rows8(src0 + j * Q3), :D]).astype(F32) for j in range(3)]
            w[0] = cat1(_tie(w[0][:, :LANES], anchor), w[0][:, LANES:])
            tiles = _w_sums([[w[j][:, k * LANES:(k + 1) * LANES] for j in range(3)]
                             for k in range(3)])
            for j in range(3):
                a, b, c = (w[j][:, KR + k * KU:KR + (k + 1) * KU] for k in range(3))
                tiles += [cat1(c, b), cat1(a, c)]
            wl_s[rows8(row0), :15 * LANES] = _pk(cat1(*tiles))

        def att_rhs(x, stash=None):
            blocks, units = split_k(x)
            ops = _x_ops(*blocks) + _x_rem(*units)
            if stash is None:
                return [v.astype(BF16) for v in ops]
            loc = lambda i, r0, n: (slice((i // 2) * 64 + r0, (i // 2) * 64 + r0 + n),
                                    slice((i % 2) * LANES, (i % 2 + 1) * LANES))
            for r in range(0, LANES, 16):
                for i, v in enumerate(ops):
                    r_s.at[0][loc(i, r // 2, 8)] = _pk(v[r:r + 16])
            return [_upk(r_s.at[stash][loc(i, 0, 64)]) for i in range(18)]

        def att_mm(sec, rhs, anchors):
            tl = lambda i: _upk(wl_s[sec * Q3:(sec + 1) * Q3, i * LANES:(i + 1) * LANES])
            raw = lambda k, j: _upk(wt_s[(3 * sec + j) * Q3:(3 * sec + j + 1) * Q3,
                                         k * LANES:(k + 1) * LANES])
            t = {}
            for i in _PAIR_ORDER:
                t[i] = _dot(raw(*_W_RAW[i]) if i in _W_RAW else tl(_W_SUM[i]), rhs[i])
                anchors.append(t[i][:8])
            out = []
            for j in range(3):
                base = []
                for s in range(3):
                    v = _dot(raw(3, j) if s == 1 else tl(9 + 2 * j + s // 2), rhs[15 + s])
                    if (s, j) in _DIAG:
                        i = _DIAG[s, j]
                        v = _dot(tl(_W_SUM[i]), rhs[i]) + v
                    base.append(v)
                    anchors.append(base[-1][:8])
                out.append(cat1(*_column(t, base, j)))
            return cat0(*out)

        def qkv_fast(blk, rhs, anchors):
            for sec in range(3):
                put_qkv(blk, slice(sec * RP, (sec + 1) * RP), att_mm(sec, rhs, anchors))

        def shifted(ln, cur, prev, w):
            if w == 0:
                return cur
            sh = DIL * w
            return pltpu.roll(jnp.where(ln < LANES - sh, cur, prev), sh, axis=1)

        def att_group(blk, c, hg, anchor, win):
            tile = blk * NT + c
            base = hg * 8 * DP
            if isinstance(hg, int):
                cur, prev, o_t = qkv_s.at[1 + tile], qkv_s.at[tile], o_s.at[c]
            else:
                n = 2 * RP + 8 * DP
                base = pl.multiple_of(base, 8)
                cur = qkv_s.at[1 + tile, pl.ds(base, n)]
                prev = qkv_s.at[tile, pl.ds(base, n)]
                o_t = o_s.at[c, pl.ds(base, RP + 8 * DP)]
                base = 0
            ln = lane + _zero_like_dep(anchor).astype(jnp.int32)
            logits = [None] * W
            done = []
            for dd in range(DP):
                q = cur[pl.ds(base + dd, 8, stride=DP), :]
                kc = cur[pl.ds(RP + base + dd, 8, stride=DP), :]
                if dd >= win:
                    kc = kc | _zero_like_dep(done[dd - win])
                kp = prev[pl.ds(RP + base + dd, 8, stride=DP), :]
                q0, q1 = _lo(q), _hi(q)
                for w in range(W):
                    ks = shifted(ln, kc, kp, w)
                    t = q0 * _lo(ks) + q1 * _hi(ks)
                    logits[w] = t if logits[w] is None else logits[w] + t
                done.append(ks)
            logits = [l * scale for l in logits]
            if not (isinstance(c, int) and c > 0):
                pos = lane + tile * LANES
                logits = [l if w == 0 else jnp.where(pos >= DIL * w, l, -1e9)
                          for w, l in enumerate(logits)]
            m = _tree_sum(logits, jnp.maximum)
            ln = lane + _zero_like_dep(m).astype(jnp.int32)
            e = [jnp.exp(l - m) for l in logits]
            den = _tree_sum(e)
            if cfg['rcp']:
                r = pl.reciprocal(den, approx=True)
                r = r * (2.0 - den * r)
            else:
                r = 1.0 / den
            p = e if cfg['late'] else [x * r for x in e]
            done = []
            for dd in range(DP):
                vc = cur[pl.ds(2 * RP + base + dd, 8, stride=DP), :]
                if dd >= win:
                    vc = vc | _zero_like_dep(done[dd - win])
                vp = prev[pl.ds(2 * RP + base + dd, 8, stride=DP), :]
                o0 = o1 = None
                for w in range(W):
                    vs = shifted(ln, vc, vp, w)
                    t0, t1 = p[w] * _lo(vs), p[w] * _hi(vs)
                    o0 = t0 if o0 is None else o0 + t0
                    o1 = t1 if o1 is None else o1 + t1
                done.append(vs)
                if cfg['late']:
                    o0, o1 = o0 * r, o1 * r
                o_t[pl.ds(base + dd, 8, stride=DP), :] = o0
                o_t[pl.ds(RP + base + dd, 8, stride=DP), :] = o1

        def attention(blk, anchors, win):
            for c in range(NT):
                for hg in range(NG):
                    att_group(blk, c, hg, anchors[c * NG + hg], win)

        def wo_mm(blk, anchors, fast, anchors_in=(), stash=None):
            o = cat1(*[o_s[c] for c in range(NT)])
            if anchors_in:
                o = cat0(*[_tie(o[r:r + 8], spread_over(anchors_in, slab_group(r), 12))
                           for r in range(0, D, 8)])
            if fast:
                y = att_mm(3, att_rhs(o, stash), anchors)
            else:
                o = o.astype(BF16)
                q = D2 // 2
                y = cat0(*[dot_k(slice(h * q, (h + 1) * q), o, anchors) for h in (6, 7)])
            xm = xio_s[blk].astype(F32) + y
            xmid_s[blk] = xm
            return _ln_stats((xm[r:r + 8] for r in range(0, D, 8)), D)

        def ffn_lhs(blk, stats, anchors):
            m, rs = stats
            m8 = jnp.broadcast_to(m, (8, TM))
            xs = []
            for k in range(3):
                mt = cat0(*[_tie(m8, spread_over(anchors, k, 3))] * (D3 // 8))
                xs.append((xmid_s[blk, k * D3:(k + 1) * D3, :] - mt) * rs)
            ops = _x_ops([x[:, :TH] for x in xs], [x[:, TH:] for x in xs])
            for i, v in enumerate(ops):
                for s, t in enumerate((v[KU:], v[:2 * KU], cat0(v[:KU], v[2 * KU:]))):
                    a_s[3 * i + s] = _pk(t.astype(BF16).T)

        def plain_lhs(blk, stats):
            m, rs = stats
            blocks, units = split_k((xmid_s[blk] - m) * rs)
            for i, v in enumerate(blocks[0] + blocks[1] + _x_rem(*units)):
                a_s[i] = _pk(v.astype(BF16).T)

        def plain_piece(p, anchors):
            h = {}
            for j in range(3):
                hs = []
                for n in range(PW // LANES):
                    cs = slice(n * LANES, (n + 1) * LANES)
                    w = lambda r0, r1: cat1(wg_v[p, j, r0:r1, cs], wu_v[p, j, r0:r1, cs])
                    u = lambda k: w(KR + k * KU, KR + (k + 1) * KU)
                    tl = lambda *i: _upk(cat1(*[a_s[k] for k in i]))
                    y0 = _dot(tl(6), cat0(u(2), u(1)))
                    y1 = _dot(tl(0, 1, 2, 7), w(0, KR + 2 * KU))
                    y2 = _dot(tl(3, 4, 5, 8), cat0(w(0, KR + KU), u(2)))
                    for y in (y0, y1, y2):
                        anchors.extend(y[r:r + 8, c:c + LANES]
                                       for c in ((0,) if y is y0 else (0, LANES))
                                       for r in ((0,) if y is y0 else (0, TH // 2)))
                    hs.append([_gelu_mul2(*[(y + y0)[:, c:c + LANES] for c in (0, LANES)])
                               for y in (y1, y2)])
                h[j] = [cat1(*[v[i] for v in hs]) for i in range(2)]
            return h_ops(h)

        def prep_d(p, anchors):
            PR = 16
            for n in range(2 * D3 // PR):
                r, cs = (n // 2) * PR, slice((n % 2) * LANES, (n % 2 + 1) * LANES)
                w = [[wdt_v[p, k, j * D3 + r:j * D3 + r + PR, cs].astype(F32)
                      for j in range(3)] for k in range(3)]
                w[0][1] = _tie(w[0][1], spread_over(anchors, n, 2 * D3 // PR))
                for i, v in enumerate(_w_sums(w)):
                    ds_s.at[p, i][r // 2:(r + PR) // 2, cs] = _pk(v)

        GU = ((wg_v, gs_s), (wu_v, us_s))

        def prep_gu(p, anchors):
            PR = 16
            nr = D3 // PR
            for n in range(4 * nr):
                c, (w_v, s_s), r = n % 2, GU[(n // 2) % 2], (n // 4) * PR
                cache = {}

                def w(k, j):
                    if (k, j) not in cache:
                        ld = lambda c: w_v[p, j, k * D3 + r:k * D3 + r + PR,
                                           c * LANES:(c + 1) * LANES].astype(F32)
                        v = ld(c)
                        if k != j:
                            v = _tie(v, spread_over(anchors, n, 4 * nr))
                        cache[k, j] = v - ld(1 - c) if r // KU == 1 + c else v
                    return cache[k, j]

                for i in range(15):
                    v = None
                    for k, j, sg in _W_TERMS[i]:
                        v = w(k, j) if v is None else (v + w(k, j) if sg > 0 else v - w(k, j))
                    s_s.at[p, i][r // 2:(r + PR) // 2, c * LANES:(c + 1) * LANES] = _pk(v)

        NS = cfg['msplit']

        def gu_prod(p, i, t, anchors, slabs, slot=0):
            u = KU // 2

            def rhs(s, s_s):
                if s == 1:
                    return s_s[p, i, :2 * u, :LANES]
                if s == 0:
                    return cat0(s_s[p, i, u:2 * u, LANES:], s_s[p, i, 2 * u:, :LANES])
                return cat0(s_s[p, i, :u, LANES:], s_s[p, i, 2 * u:, LANES:])

            q = TH // 2 // NS
            for n, h in enumerate(slabs):
                y = []
                for s in range(3):
                    r = _upk(cat1(rhs(s, gs_s), rhs(s, us_s)))
                    y.append(_dot(_upk(a_s[3 * i + s, h * q:(h + 1) * q]), r))
                    if (3 * n + s) % len(slabs) == 0:
                        anchors.append(y[-1][:8, :LANES])
                y1, y2 = y[1] + y[0], y[2] + y[0]
                for m in range(2):
                    cs = slice(m * LANES, (m + 1) * LANES)
                    v = cat1(y1[:, cs], y2[:, cs])
                    if i < 9 and 't' in cfg['stash']:
                        k = p if isinstance(p, int) else slot
                        t_s[k, m, i, 2 * h * q:2 * (h + 1) * q] = v
                        v = lambda k=k, m=m, h=h: t_s[k, m, i, 2 * h * q:2 * (h + 1) * q]
                    t.setdefault((m, h), {})[i] = v

        def gu_col(t, hv, p, j, anchors, slabs):
            ids = [_DIAG.get((s, j)) for s in range(3)]
            if cfg['fslab']:
                for h in slabs:
                    for i in ids:
                        if i is not None:
                            gu_prod(p, i, t, anchors if h == slabs[0] else [], [h])
            else:
                for i in ids:
                    if i is not None:
                        gu_prod(p, i, t, anchors, slabs)
            for h in slabs:
                g, u = [_column(t[m, h], [None if i is None else t[m, h][i] for i in ids], j)
                        for m in range(2)]
                hv[j, h] = [_gelu_mul2(g[i], u[i]) for i in range(2)]

        def h_ops(h):
            return [v.astype(BF16) for v in _x_ops(*[[h[j][i] for j in range(3)]
                                                     for i in range(2)])]

        def h_join(hv):
            return h_ops({j: [cat0(*[hv[j, h][i] for h in range(NS)]) for i in range(2)]
                          for j in range(3)})

        def gu_piece(p, order, anchors, slot):
            t, hv = {}, {}
            for slabs in ([[h] for h in range(NS)] if cfg['slab'] else [list(range(NS))]):
                for step in order:
                    if step[0] == 'S':
                        for i in _PARTS[int(step[1])]:
                            gu_prod(p, i, t, anchors, slabs, slot)
                    else:
                        gu_col(t, hv, p, int(step[1]), anchors, slabs)
            return h_join(hv)

        D_ORDER = _PAIR_ORDER + (9, 10, 11, 12, 13, 14)

        def down_mm(acc, bs, lo, anchors, which=D_ORDER, fine=False):
            p = [None] * 15 if acc is None else list(acc)
            for i in which:
                y = None
                for n, b in enumerate(bs):
                    if i in _W_RAW:
                        k, j = _W_RAW[i]
                        v = _dot_nt(wdt_v[lo + n, k, j * D3:(j + 1) * D3, :], b[i])
                    elif len(bs) % 2 and i == 14 and n == 0:
                        v = cat0(*[_dot_nt(_upk(ds_s[lo, _W_SUM[i],
                                                     h * Q3 // 2:(h + 1) * Q3 // 2, :]), b[i])
                                   for h in range(2)])
                    else:
                        v = _dot_nt(_upk(ds_s[lo + n, _W_SUM[i]]), b[i])
                    y = v if y is None else y + v
                p[i] = y if p[i] is None else p[i] + y
                anchors.append(p[i][:8])
                if fine:
                    anchors.append(p[i][D3 // 2:D3 // 2 + 8])
            return p

        def finish(blk, acc):
            y = [cat1(*_column(acc, [acc[_DIAG[s, j]] if (s, j) in _DIAG else None
                                     for s in range(3)], j)) for j in range(3)]
            xio_s[blk] = (xmid_s[blk] + 0.5 * cat0(*y)).astype(BF16)

        def load_acc(k):
            return [acc_s[k, i] for i in range(15)]

        def store_acc(k, acc):
            for i in range(15):
                acc_s[k, i] = acc[i]

        def load_b(k=0):
            return [_upk(b_s[i * TH // 2:(i + 1) * TH // 2, :])
                    for i in range(15 * k, 15 * k + 15)]

        def store_b(b, k=0):
            for i in range(15):
                b_s[(15 * k + i) * TH // 2:(15 * k + i + 1) * TH // 2, :] = _pk(b[i])

        def pre_phase():
            x0_cp, x1_cp = x_cp(0, 0), x_cp(1, 3)
            order = [x0_cp, wq_cp(0), wq_cp(1), x1_cp, wq_cp(2)]
            for p in range(NP + 1):
                order += group_cp(p)
            xr_cp = [x_cp(b, SEM_P + NP + 1) for b in range(2, NB)]
            order += xr_cp
            for cp in order:
                cp.start()
            get = lambda an, name: [an[min(i, len(an) - 1)] for i in cfg[name]]
            e_grp = lambda e: ((e >> 1) & 1, ((e >> 2) << 1) | (e & 1))
            if 'a' in cfg['sub']:
                pre_a(x0_cp, x1_cp, get, e_grp)
            if 'b' in cfg['sub']:
                pre_b(get, e_grp)
            if 'c' in cfg['sub']:
                pre_c(get)
            wait('WX', xr_cp)

        def pre_a(x0_cp, x1_cp, get, e_grp):
            qkv_s[0] = jnp.zeros(qkv_s.shape[1:], U32)
            acc_s[...] = jnp.zeros(acc_s.shape, F32)
            wait('WX0', [x0_cp])
            xn0 = ln1(0, ()).astype(BF16)
            done = 0
            for i in range(3):
                wait('WQ%d' % i, [wq_cp(i)] + ([x1_cp] if i == 2 else []))
                wt = _pk(wqkv_v[:, WQ[i]:WQ[i + 1]].T)
                wt_s[WQ[i] // 2:WQ[i + 1] // 2, :D] = wt
                anchors = []
                qkv_mm(0, xn0, range(done, WQ[i + 1] // QR), anchors)
                done = WQ[i + 1] // QR
                if i > 0:
                    for n, a in enumerate(get(anchors, 'a_w%d' % i)):
                        prep_att(12 * (i - 1) + n, a)
            xn1 = ln1(1, get(anchors, 'a_ln'), get(anchors, 'a_lnb')).astype(BF16)
            qkv_mm(1, xn1, (0, 2, 4, 1), anchors)
            for e in range(8):
                att_group(0, *e_grp(e), anchors[cfg['att0'][e]], 9)
            wait('WO', group_cp(0))
            wo = pltpu.bitcast(wo_v[...], U32)
            wt_s[3 * RP:, :D] = _pk(cat0(_lo(wo), _hi(wo)).astype(BF16).T)
            an = []
            stats = wo_mm(0, an, False)
            qkv_mm(1, xn1, [3], an)
            plain_lhs(0, stats)
            b = plain_piece(0, an)
            qkv_mm(1, xn1, [5], an)
            prep_gu(0, get(an, 'z_g'))
            for e in range(3):
                att_group(1, *e_grp(e), an[cfg['z_att'][e]], 9)
            store_b(b)

        def pre_b(get, e_grp):
            def piece(p, carry):
                wait('WP', group_cp(p))
                b_prev = load_b()
                an = []
                b = plain_piece(p, an)
                prep_d(p - 1, get(an, 'p_d'))
                store_acc(0, down_mm(load_acc(0), [b_prev], p - 1, an))
                prep_gu(p, get(an, 'p_g'))
                att_group(1, *e_grp(p + 2), an[cfg['p_att'][0]], 9)
                for i, a in enumerate(get(an, 'p_w')):
                    prep_att(jnp.minimum(24 + (p - 1) * 5 + i, 47), a)
                store_b(b)
                return carry

            lax.fori_loop(1, NP, piece, 0)

        def pre_c(get):
            wait('WD', group_cp(NP))
            an = []
            stats = wo_mm(1, an, True)
            prep_d(NP - 1, get(an, 't_d'))
            acc = down_mm(load_acc(0), [load_b()], NP - 1, [])
            ffn_lhs(1, stats, [])
            finish(0, acc)

        if 'pre' in cfg['phases']:
            pre_phase()

        def body(u, carry):
            bu = u & (NB - 1)
            ba = (u + 1) & (NB - 1)
            acc, stats, an, b = None, None, {}, {}
            get = lambda name: [an[k][i] for k, i in cfg[name]]
            for step in cfg['body']:
                an[step] = []
                if step == 'Q':
                    qkv_fast(ba, att_rhs(ln1(ba, get('ln1'), get('ln1b')), u >> 8 if 'q' in cfg['stash'] else None),
                             an[step])
                elif step == 'W':
                    attention(ba, get('att'), cfg['win'])
                    stats = wo_mm(ba, an[step], True, get('orhs'),
                                  u >> 8 if 'w' in cfg['stash'] else None)
                elif step == 'L':
                    ffn_lhs(ba, stats, get('lhs'))
                elif step[0] == 'S':
                    slabs = [int(step[3])] if len(step) > 3 else list(range(NS))
                    for i in _PARTS[int(step[2])]:
                        gu_prod(int(step[1]), i, b.setdefault(step[:2], {}), an[step], slabs)
                elif step[0] == 'F':
                    j, c = int(step[1]), int(step[2])
                    slabs = [int(step[3])] if len(step) > 3 else list(range(NS))
                    hv = b.setdefault(step[:2], {})
                    gu_col(b['S' + step[1]], hv, j, c, an[step], slabs)
                    if len(hv) == 3 * NS:
                        b[j] = h_join(hv)
                        if 'b' in cfg['stash']:
                            store_b(b[j], j)
                            b[j] = load_b(j)
                else:
                    js = [int(c) for c in step[1:]]
                    acc = down_mm(acc, [b[j] for j in js], js[0], an[step])
            finish(bu, acc)

            @pl.when(u >= NB)
            def _():
                out_copy(bu).start()
            return carry

        if scopes:
            with jax.named_scope('LOOP'):
                lax.fori_loop(1, NU - 1, body, 0)
        elif 'main' in cfg['phases']:
            lax.fori_loop(1, NU - 1, body, 0)

        def last(c, carry):
            los = [2 * c + j for j in range(2)]
            b = [gu_piece(lo, cfg['order'], [], j) for j, lo in enumerate(los)]
            acc = load_acc(1)
            for j in range(2):
                acc = down_mm(acc, [b[j]], los[j], [])
            store_acc(1, acc)
            return carry

        if 'last' in cfg['phases']:
            lax.fori_loop(0, NP // 2, last, 0)
        if len(cfg['phases']) < 3:
            def keep(i, c):
                v = (gs_s[i, i, :8, :LANES] + us_s[i, i, :8, :LANES] + ds_s[i, i, :8, :LANES]
                     + wl_s[rows8(i * 8), :LANES] + a_s[i, :8] + qkv_s[i, :8]
                     + b_s[rows8(i * 8), :LANES] + wt_s[rows8(i * 8), :LANES])
                acc_s[1, 0, :8] = (lax.bitcast_convert_type(v, F32) + o_s[i, :8]
                                   + acc_s[i, i, :8])
                return c
            lax.fori_loop(0, 2, keep, 0)
        finish(NB - 1, load_acc(1))
        out_copy(NB - 1).start()
        wait('WOUT', [out_copy(b) for b in range(NB)])

    scratch = [
        pltpu.VMEM((NB, D, TM), BF16),
        pltpu.VMEM((D, 3 * D), BF16),
        pltpu.VMEM((D, D), BF16),
        pltpu.VMEM((NP, 3, D, PW), BF16),
        pltpu.VMEM((NP, 3, D, PW), BF16),
        pltpu.VMEM((NP, 3, D, PW), BF16),
        pltpu.VMEM((2 * D, 8 * LANES), U32),
        pltpu.VMEM((4 * Q3, 16 * LANES), U32),
        pltpu.VMEM((NP, 15, Q3, PW), U32),
        pltpu.VMEM((NP, 15, Q3, PW), U32),
        pltpu.VMEM((NP, 9, Q3, PW), U32),
        pltpu.VMEM((NB, D, TM), F32),
        pltpu.VMEM((45, TH // 2, LANES), U32),
        pltpu.VMEM((S // LANES + 1, 3 * RP, LANES), U32),
        pltpu.VMEM((NT, D, LANES), F32),
        pltpu.VMEM((2, 15, D3, TH), F32),
        pltpu.VMEM((NP * 15 * TH // 2, PW), U32),
        pltpu.VMEM((1, 9 * 64, 2 * LANES), U32),
        pltpu.VMEM((NP, 2, 9, TH, PW), F32),
        pltpu.SemaphoreType.DMA((SEM_P + NP + 2,)),
        pltpu.SemaphoreType.DMA((1,)),
    ]
    return kernel, scratch


_CFG = dict(
    scopes=False,
    rcp=False,
    late=True,
    stash='qw',
    slab=True,
    fslab=False,
    win=9,
    sub='abc',
    orhs=(),
    msplit=2,
    phases=('pre', 'main', 'last'),
    order=('S0', 'S1', 'F0', 'S2', 'F1', 'F2'),
    body=('S010', 'S000', 'F000', 'S020', 'F010', 'F020', 'S001', 'S011', 'F001',
        'S110', 'S021', 'F021', 'S100', 'F100', 'S120', 'S101', 'F110', 'F011', 'Q',
        'F120', 'S111', 'F101', 'S121', 'F111', 'F121', 'S200', 'S210', 'F200', 'S220',
        'F210', 'F220', 'S300', 'S201', 'S211', 'F201', 'S320', 'S221', 'F211', 'F221',
        'S310', 'D01', 'F300', 'S301', 'S311', 'F301', 'S321', 'F311', 'F321', 'S400',
        'F310', 'F320', 'S420', 'F410', 'S410', 'S401', 'F420', 'S411', 'F400', 'S421',
        'F411', 'F421', 'S500', 'F401', 'S501', 'S510', 'D23', 'F500', 'S520', 'W',
        'F520', 'S511', 'F510', 'S521', 'F501', 'F511', 'F521', 'D4', 'D5', 'L'),
    ln1=(('S010', 4), ('S010', 5), ('S010', 6), ('S010', 7), ('S010', 8), ('S000', 0),
        ('S000', 1), ('S000', 2), ('S000', 3)),
    ln1b=(('S110', 2), ('S110', 3), ('S110', 5), ('S110', 6), ('S110', 8), ('S021', 0),
        ('S021', 2), ('S021', 3), ('S021', 5), ('S021', 6), ('S021', 8), ('F021', 0)),
    att=(('S300', 8), ('D01', 1), ('D01', 7), ('D01', 8), ('D01', 10), ('F300', 4),
        ('D23', 5), ('D23', 9)),
    lhs=(('D4', 3), ('D5', 1), ('D5', 4)),
    att0=(15, 18, 21, 24, 27, 30, 33, 37),
    order0=('S0', 'S1', 'S2', 'F0', 'F1', 'F2'),
    order1=('S0', 'S1', 'S2', 'F0', 'F1', 'F2'),
    a_w1=(0, 1, 2, 3, 5, 5, 8, 9, 10, 11, 12, 14),
    a_w2=(0, 0, 2, 3, 4, 4, 6, 6, 8, 9, 11, 16),
    a_ln=(0, 3, 7),
    a_lnb=(6, 6, 8),
    z_g=(3, 4, 5, 6, 8, 9, 10, 12, 13, 14, 15, 17, 18, 19, 21, 22, 23, 25, 26, 27, 28,
        30, 31, 32, 34, 35, 36, 38, 39, 40, 41, 43, 44, 45, 47, 48, 49, 51, 52, 53, 54,
        56, 57, 58, 60, 61, 62, 64),
    z_att=(72, 75, 78),
    p_g0=(0, 1, 2, 3, 4, 5),
    p_g1=(6, 7, 8, 9, 10, 10),
    p_g2=(12, 13, 14, 15, 16, 17),
    p_g3=(14, 16, 18, 20, 22, 24, 26, 28, 30, 32, 34, 36),
    t_d=(0, 0, 1, 1, 2, 3, 3, 4, 5, 6, 6, 7, 8, 9, 9, 9, 10, 11, 11, 12, 13, 14, 15,
        16),
    p_d=(0, 2, 6, 8, 10, 12, 14, 16, 18, 20, 22, 24, 26, 28, 30, 32, 34, 36, 38, 40, 40,
        42, 44, 46),
    p_att=(52,),
    p_w=(10, 19, 30, 44, 48),
    p_g=(0, 1, 2, 3, 4, 5, 6, 7, 9, 10, 11, 12, 13, 14, 15, 16, 18, 19, 20, 21, 22, 23,
        24, 25, 27, 28, 29, 30, 31, 32, 33, 34, 36, 37, 38, 39, 40, 41, 42, 43, 45, 46,
        47, 48, 49, 50, 51, 53),
)


def _run(A_x, A_wqkv, A_wo, B_w_gate, B_w_up, B_w_down, **kw):
    _, S, D = A_x.shape
    F = B_w_gate.shape[1]
    kernel, scratch = _make_kernel(S, D, F, 256, {**_CFG, **kw})
    hbm = pl.BlockSpec(memory_space=pl.ANY)
    out_t = pl.pallas_call(
        kernel,
        in_specs=[hbm] * 6,
        out_specs=hbm,
        out_shape=jax.ShapeDtypeStruct((D, S), A_x.dtype),
        scratch_shapes=scratch,
        compiler_params=pltpu.CompilerParams(vmem_limit_bytes=110 * 1024 * 1024),
    )(A_x.reshape(S, D).T, A_wqkv, A_wo, B_w_gate, B_w_up, B_w_down.T)
    return out_t.T.reshape(A_x.shape)


@jax.jit
def pallas_interleave_layers__sliding_local_dilated__glu_gated_geglu__prompt_kernel(
    A_x: jax.Array,
    A_wqkv: jax.Array,
    A_wo: jax.Array,
    B_x: jax.Array,
    B_w_gate: jax.Array,
    B_w_up: jax.Array,
    B_w_down: jax.Array,
):
    del B_x
    return _run(A_x, A_wqkv, A_wo, B_w_gate, B_w_up, B_w_down)
```

```python
import functools

import jax
import jax.numpy as jnp
import jax.experimental.pallas as pl
import jax.experimental.pallas.tpu as pltpu
from jax import lax

H = 32
W = 8
DIL = 2
EPS = 1e-5
LANES = 128

F32 = jnp.float32
BF16 = jnp.bfloat16
U32 = jnp.uint32

_NT = (((1,), (1,)), ((), ()))


def _tree_sum(parts, op=jnp.add):
    while len(parts) > 1:
        nxt = [op(parts[i], parts[i + 1]) for i in range(0, len(parts) - 1, 2)]
        if len(parts) % 2:
            nxt.append(parts[-1])
        parts = nxt
    return parts[0]


def _ln_stats(slabs, d, anchors=()):
    n_acc = 4
    s1, s2, pilot = [None] * n_acc, [None] * n_acc, None
    for i, x in enumerate(slabs):
        if pilot is None:
            pilot = x[0:1, :]
            pil = jnp.broadcast_to(pilot, x.shape)
            pils = [_tie(pil, a) for a in anchors] or [pil]
        dx = x - pils[i * len(pils) // (d // 8)]
        j = i % n_acc
        s1[j] = dx if s1[j] is None else s1[j] + dx
        s2[j] = dx * dx if s2[j] is None else s2[j] + dx * dx
    e1 = jnp.sum(_tree_sum(s1), axis=0, keepdims=True) * (1.0 / d)
    e2 = jnp.sum(_tree_sum(s2), axis=0, keepdims=True) * (1.0 / d)
    var = jnp.maximum(e2 - e1 * e1, 0.0)
    return pilot + e1, lax.rsqrt(var + EPS)


def _zero_like_dep(v):
    return (lax.bitcast_convert_type(v, U32) >> 31) >> 1


def _tie(x, anchor):
    if anchor is None:
        return x
    z = lax.bitcast_convert_type(_zero_like_dep(anchor), F32)
    z = jnp.concatenate([z] * (x.shape[1] // LANES), axis=1)
    if x.shape[0] == 8:
        return x + z
    return jnp.concatenate([x[:8] + z, x[8:]], axis=0)


def _gelu_mul2(g, u):
    c0 = 0.7978845608028654
    c1 = c0 * 0.044715
    t = jnp.tanh(g * (c0 + c1 * (g * g)))
    return (g * u) * (1.0 + t)


def _lo(x):
    return lax.bitcast_convert_type(x << 16, F32)


def _hi(x):
    return lax.bitcast_convert_type(x & jnp.uint32(0xFFFF0000), F32)


def _pk(x):
    return pltpu.bitcast(x.astype(BF16), U32)


def _upk(x):
    return pltpu.bitcast(x, BF16)


def _dot(a, b):
    return jnp.dot(a, b, preferred_element_type=F32)


def _dot_nt(a, b):
    return lax.dot_general(a, b, _NT, preferred_element_type=F32)


def _x_ops(x1, x2):
    d = [a - b for a, b in zip(x1, x2)]
    return [x1[0] + x2[1], x2[0] + x2[1], x1[0] + x1[1],
            d[1] + x1[2], x1[1] + x1[2], d[1] + d[2],
            d[0] - x2[2], d[0] + d[2], x2[0] + x2[2],
            x1[0], d[0], x2[1], d[1], x1[2], x2[2]]


def _x_rem(x1, x2):
    a, b, c = 0, 1, 2
    cat = lambda u, v: jnp.concatenate([u, v], axis=0)
    return [cat(x1[c], x2[b]), cat(x1[a], x1[b] - x2[b]), cat(x2[a], x2[c] - x1[c])]


def _w_sums(w):
    return [w[0][1] + w[1][0], w[1][2] + w[2][1], w[0][2] + w[2][0],
            w[0][0] + w[0][2] - w[1][0], w[2][0] - w[0][0] - w[0][1],
            w[1][1] + w[1][2] - w[0][1], w[1][0] + w[1][1] - w[2][1],
            w[2][0] + w[2][2] - w[1][2], w[2][1] + w[2][2] - w[0][2]]


_W_TERMS = {0: ((0, 1, 1), (1, 0, 1)), 3: ((1, 2, 1), (2, 1, 1)), 6: ((0, 2, 1), (2, 0, 1)),
            9: ((0, 0, 1), (0, 2, 1), (1, 0, -1)), 10: ((2, 0, 1), (0, 0, -1), (0, 1, -1)),
            11: ((1, 1, 1), (1, 2, 1), (0, 1, -1)), 12: ((1, 0, 1), (1, 1, 1), (2, 1, -1)),
            13: ((2, 0, 1), (2, 2, 1), (1, 2, -1)), 14: ((2, 1, 1), (2, 2, 1), (0, 2, -1)),
            1: ((0, 1, 1),), 2: ((1, 0, 1),), 4: ((1, 2, 1),), 5: ((2, 1, 1),),
            7: ((2, 0, 1),), 8: ((0, 2, 1),)}
_PARTS = ((1, 2, 0), (7, 8, 6), (4, 5, 3), (9, 10, 11, 12, 13, 14))
_W_SUM = {0: 0, 3: 1, 6: 2, 9: 3, 10: 4, 11: 5, 12: 6, 13: 7, 14: 8}
_W_RAW = {1: (0, 1), 2: (1, 0), 4: (1, 2), 5: (2, 1), 7: (2, 0), 8: (0, 2)}
_PAIR_ORDER = (1, 2, 4, 5, 7, 8, 0, 3, 6)
_DIAG = {(0, 0): 9, (2, 0): 10, (0, 1): 11, (1, 1): 12, (1, 2): 13, (2, 2): 14}
_PAIR = {(0, 0): ((6, -1), (8, -1)), (1, 0): ((2, 1), (7, 1)), (2, 0): ((0, 1), (1, -1)),
         (0, 1): ((3, 1), (4, -1)), (1, 1): ((0, 1), (2, -1)), (2, 1): ((1, 1), (5, -1)),
         (0, 2): ((4, 1), (8, 1)), (1, 2): ((6, 1), (7, -1)), (2, 2): ((5, 1), (3, -1))}


def _column(t, base, j):
    s = []
    for k in range(3):
        v = base[k]
        for i, sg in _PAIR[k, j]:
            ti = t[i]() if callable(t[i]) else t[i]
            v = ti if v is None else (v + ti if sg > 0 else v - ti)
        s.append(v)
    return s[1] + s[0], s[2] + s[0]


def _make_kernel(S, D, F, TM, cfg):
    NB = S // TM
    NT = TM // LANES
    DH = D // H
    DP = DH // 2
    RP = D // 2
    NG = H // 8
    scale = float(DH) ** -0.5
    NU = 2 * NB
    TH = TM // 2
    FT = F // 3
    D2 = D // 2
    D3 = D // 3
    Q3 = D3 // 2
    KU = D // 9
    KR = 3 * LANES
    NQ = 6
    QR = 3 * D // NQ
    WQ = (0, 640, 1152, 3 * D)
    PW = 256
    NP = FT // PW
    scopes = cfg['scopes']
    assert NG == 4 and NB & (NB - 1) == 0
    SEM_P = 4

    def kernel(x_hbm, wqkv_hbm, wo_hbm, wg_hbm, wu_hbm, wdt_hbm, out_hbm,
               xio_s, wqkv_v, wo_v, wg_v, wu_v, wdt_v, wt_s, wl_s,
               gs_s, us_s, ds_s, xmid_s, a_s, qkv_s, o_s, acc_s, b_s, r_s, t_s,
               sem_i, sem_o):

        def wait(name, cps):
            if scopes:
                with jax.named_scope(name):
                    for cp in cps:
                        cp.wait()
            else:
                for cp in cps:
                    cp.wait()

        def cols(lo, n):
            if not isinstance(lo, int):
                lo = pl.multiple_of(lo, LANES)
            return pl.ds(lo, n)

        def rows8(lo, n=8):
            if not isinstance(lo, int):
                lo = pl.multiple_of(lo, 8)
            return pl.ds(lo, n)

        def out_copy(b):
            return pltpu.make_async_copy(
                xio_s.at[b], out_hbm.at[:, cols(b * TM, TM)], sem_o.at[0])

        def x_cp(b, sem):
            return pltpu.make_async_copy(x_hbm.at[:, cols(b * TM, TM)], xio_s.at[b],
                                         sem_i.at[sem])

        def wq_cp(i):
            sl = cols(WQ[i], WQ[i + 1] - WQ[i])
            return pltpu.make_async_copy(wqkv_hbm.at[:, sl], wqkv_v.at[:, sl],
                                         sem_i.at[1 + i])

        def piece_cp(src, dst, p, sem):
            return [pltpu.make_async_copy(src.at[:, cols(j * FT + p * PW, PW)],
                                          dst.at[p, j],
                                          sem_i.at[sem]) for j in range(3)]

        def group_cp(p):
            sem = SEM_P + p
            cps = []
            if isinstance(p, int) and p == 0:
                cps.append(pltpu.make_async_copy(wo_hbm, wo_v, sem_i.at[sem]))
            if not (isinstance(p, int) and p == NP):
                cps += piece_cp(wg_hbm, wg_v, p, sem) + piece_cp(wu_hbm, wu_v, p, sem)
            if not (isinstance(p, int) and p == 0):
                cps += piece_cp(wdt_hbm, wdt_v, p - 1, sem)
            return cps

        lane = lax.broadcasted_iota(jnp.int32, (8, LANES), 1)
        cat0 = lambda *v: jnp.concatenate(v, axis=0)
        cat1 = lambda *v: jnp.concatenate(v, axis=1)

        def spread_over(anchors, n, total):
            return anchors[n * len(anchors) // total] if anchors else None

        def slab_group(r):
            return (r % LANES) // 16 if r < KR else 8 + ((r - KR) % KU) // 16

        def ln1(blk, anchors1, anchors2=()):
            slabs = (xio_s[blk, r:r + 8, :].astype(F32) for r in range(0, D, 8))
            m, rs = _ln_stats(slabs, D, anchors1)
            if not anchors2:
                return (xio_s[blk].astype(F32) - m) * rs
            m8 = jnp.broadcast_to(m, (8, TM))
            ms = [_tie(m8, a) for a in anchors2]
            ms = [spread_over(ms, slab_group(r), 12) for r in range(0, D, 8)]
            return (xio_s[blk].astype(F32) - cat0(*ms)) * rs

        def dot_k(rows, x, anchors):
            y = None
            for n, k in enumerate(range(0, D, LANES)):
                ks = slice(k, min(k + LANES, D))
                v = _dot(_upk(wt_s[rows, ks]), x[ks])
                anchors.extend(v[r:r + 8, :LANES] for r in ((0, 144) if n % 2 else (72, 216)))
                y = v if y is None else y + v
            return y

        def put_qkv(blk, rows, y):
            pk = _pk(y)
            for c in range(NT):
                qkv_s[1 + blk * NT + c, rows, :] = pk[:, c * LANES:(c + 1) * LANES]

        def qkv_mm(blk, xn, chunks, anchors):
            for r in chunks:
                rows = slice(r * QR // 2, (r + 1) * QR // 2)
                put_qkv(blk, rows, dot_k(rows, xn, anchors))

        def split_k(x):
            hs = (x[:, :TH], x[:, TH:])
            blocks = [[h[k * LANES:(k + 1) * LANES] for k in range(3)] for h in hs]
            units = [[h[KR + k * KU:KR + (k + 1) * KU] for k in range(3)] for h in hs]
            return blocks, units

        def prep_att(pat, anchor):
            assert Q3 == 96
            row0 = pat * 8
            src0 = row0 + ((pat * 43) >> 9) * (2 * Q3)
            w = [_upk(wt_s[rows8(src0 + j * Q3), :D]).astype(F32) for j in range(3)]
            w[0] = cat1(_tie(w[0][:, :LANES], anchor), w[0][:, LANES:])
            tiles = _w_sums([[w[j][:, k * LANES:(k + 1) * LANES] for j in range(3)]
                             for k in range(3)])
            for j in range(3):
                a, b, c = (w[j][:, KR + k * KU:KR + (k + 1) * KU] for k in range(3))
                tiles += [cat1(c, b), cat1(a, c)]
            wl_s[rows8(row0), :15 * LANES] = _pk(cat1(*tiles))

        def att_rhs(x, stash=None):
            blocks, units = split_k(x)
            ops = _x_ops(*blocks) + _x_rem(*units)
            if stash is None:
                return [v.astype(BF16) for v in ops]
            loc = lambda i, r0, n: (slice((i // 2) * 64 + r0, (i // 2) * 64 + r0 + n),
                                    slice((i % 2) * LANES, (i % 2 + 1) * LANES))
            for r in range(0, LANES, 16):
                for i, v in enumerate(ops):
                    r_s.at[0][loc(i, r // 2, 8)] = _pk(v[r:r + 16])
            return [_upk(r_s.at[stash][loc(i, 0, 64)]) for i in range(18)]

        def att_mm(sec, rhs, anchors):
            tl = lambda i: _upk(wl_s[sec * Q3:(sec + 1) * Q3, i * LANES:(i + 1) * LANES])
            raw = lambda k, j: _upk(wt_s[(3 * sec + j) * Q3:(3 * sec + j + 1) * Q3,
                                         k * LANES:(k + 1) * LANES])
            t = {}
            for i in _PAIR_ORDER:
                t[i] = _dot(raw(*_W_RAW[i]) if i in _W_RAW else tl(_W_SUM[i]), rhs[i])
                anchors.append(t[i][:8])
            out = []
            for j in range(3):
                base = []
                for s in range(3):
                    v = _dot(raw(3, j) if s == 1 else tl(9 + 2 * j + s // 2), rhs[15 + s])
                    if (s, j) in _DIAG:
                        i = _DIAG[s, j]
                        v = _dot(tl(_W_SUM[i]), rhs[i]) + v
                    base.append(v)
                    anchors.append(base[-1][:8])
                out.append(cat1(*_column(t, base, j)))
            return cat0(*out)

        def qkv_fast(blk, rhs, anchors):
            for sec in range(3):
                put_qkv(blk, slice(sec * RP, (sec + 1) * RP), att_mm(sec, rhs, anchors))

        def shifted(ln, cur, prev, w):
            if w == 0:
                return cur
            sh = DIL * w
            return pltpu.roll(jnp.where(ln < LANES - sh, cur, prev), sh, axis=1)

        def att_group(blk, c, hg, anchor, win):
            tile = blk * NT + c
            base = hg * 8 * DP
            if isinstance(hg, int):
                cur, prev, o_t = qkv_s.at[1 + tile], qkv_s.at[tile], o_s.at[c]
            else:
                n = 2 * RP + 8 * DP
                base = pl.multiple_of(base, 8)
                cur = qkv_s.at[1 + tile, pl.ds(base, n)]
                prev = qkv_s.at[tile, pl.ds(base, n)]
                o_t = o_s.at[c, pl.ds(base, RP + 8 * DP)]
                base = 0
            ln = lane + _zero_like_dep(anchor).astype(jnp.int32)
            logits = [None] * W
            done = []
            for dd in range(DP):
                q = cur[pl.ds(base + dd, 8, stride=DP), :]
                kc = cur[pl.ds(RP + base + dd, 8, stride=DP), :]
                if dd >= win:
                    kc = kc | _zero_like_dep(done[dd - win])
                kp = prev[pl.ds(RP + base + dd, 8, stride=DP), :]
                q0, q1 = _lo(q), _hi(q)
                for w in range(W):
                    ks = shifted(ln, kc, kp, w)
                    t = q0 * _lo(ks) + q1 * _hi(ks)
                    logits[w] = t if logits[w] is None else logits[w] + t
                done.append(ks)
            logits = [l * scale for l in logits]
            if not (isinstance(c, int) and c > 0):
                pos = lane + tile * LANES
                logits = [l if w == 0 else jnp.where(pos >= DIL * w, l, -1e9)
                          for w, l in enumerate(logits)]
            m = _tree_sum(logits, jnp.maximum)
            ln = lane + _zero_like_dep(m).astype(jnp.int32)
            e = [jnp.exp(l - m) for l in logits]
            den = _tree_sum(e)
            if cfg['rcp']:
                r = pl.reciprocal(den, approx=True)
                r = r * (2.0 - den * r)
            else:
                r = 1.0 / den
            p = e if cfg['late'] else [x * r for x in e]
            done = []
            for dd in range(DP):
                vc = cur[pl.ds(2 * RP + base + dd, 8, stride=DP), :]
                if dd >= win:
                    vc = vc | _zero_like_dep(done[dd - win])
                vp = prev[pl.ds(2 * RP + base + dd, 8, stride=DP), :]
                o0 = o1 = None
                for w in range(W):
                    vs = shifted(ln, vc, vp, w)
                    t0, t1 = p[w] * _lo(vs), p[w] * _hi(vs)
                    o0 = t0 if o0 is None else o0 + t0
                    o1 = t1 if o1 is None else o1 + t1
                done.append(vs)
                if cfg['late']:
                    o0, o1 = o0 * r, o1 * r
                o_t[pl.ds(base + dd, 8, stride=DP), :] = o0
                o_t[pl.ds(RP + base + dd, 8, stride=DP), :] = o1

        def attention(blk, anchors, win):
            for c in range(NT):
                for hg in range(NG):
                    att_group(blk, c, hg, anchors[c * NG + hg], win)

        def wo_mm(blk, anchors, fast, anchors_in=(), stash=None):
            o = cat1(*[o_s[c] for c in range(NT)])
            if anchors_in:
                o = cat0(*[_tie(o[r:r + 8], spread_over(anchors_in, slab_group(r), 12))
                           for r in range(0, D, 8)])
            if fast:
                y = att_mm(3, att_rhs(o, stash), anchors)
            else:
                o = o.astype(BF16)
                q = D2 // 2
                y = cat0(*[dot_k(slice(h * q, (h + 1) * q), o, anchors) for h in (6, 7)])
            xm = xio_s[blk].astype(F32) + y
            xmid_s[blk] = xm
            return _ln_stats((xm[r:r + 8] for r in range(0, D, 8)), D)

        def ffn_lhs(blk, stats, anchors):
            m, rs = stats
            m8 = jnp.broadcast_to(m, (8, TM))
            xs = []
            for k in range(3):
                mt = cat0(*[_tie(m8, spread_over(anchors, k, 3))] * (D3 // 8))
                xs.append((xmid_s[blk, k * D3:(k + 1) * D3, :] - mt) * rs)
            ops = _x_ops([x[:, :TH] for x in xs], [x[:, TH:] for x in xs])
            for i, v in enumerate(ops):
                for s, t in enumerate((v[KU:], v[:2 * KU], cat0(v[:KU], v[2 * KU:]))):
                    a_s[3 * i + s] = _pk(t.astype(BF16).T)

        def plain_lhs(blk, stats):
            m, rs = stats
            blocks, units = split_k((xmid_s[blk] - m) * rs)
            for i, v in enumerate(blocks[0] + blocks[1] + _x_rem(*units)):
                a_s[45 + i] = _pk(v.astype(BF16).T)

        def plain_piece(p, anchors):
            h = {}
            for j in range(3):
                hs = []
                for n in range(PW // LANES):
                    cs = slice(n * LANES, (n + 1) * LANES)
                    w = lambda r0, r1: cat1(wg_v[p, j, r0:r1, cs], wu_v[p, j, r0:r1, cs])
                    u = lambda k: w(KR + k * KU, KR + (k + 1) * KU)
                    ps = cfg['psplit']
                    q = TH // 2 // ps
                    hh = []
                    for s in range(ps):
                        tl = lambda *i: _upk(cat1(*[a_s[45 + k, s * q:(s + 1) * q] for k in i]))
                        y0 = _dot(tl(6), cat0(u(2), u(1)))
                        y1 = _dot(tl(0, 1, 2, 7), w(0, KR + 2 * KU))
                        y2 = _dot(tl(3, 4, 5, 8), cat0(w(0, KR + KU), u(2)))
                        if s == 0:
                            anchors.append(y0[:8, :LANES])
                        for y in (y1, y2):
                            anchors.extend(y[r:r + 8, c:c + LANES] for c in (0, LANES)
                                           for r in range(0, 2 * q, TH // 2))
                        hh.append([_gelu_mul2(*[(y + y0)[:, c:c + LANES] for c in (0, LANES)])
                                   for y in (y1, y2)])
                    hs.append([cat0(*[v[i] for v in hh]) for i in range(2)])
                h[j] = [cat1(*[v[i] for v in hs]) for i in range(2)]
            return h_ops(h)

        def prep_d(p, anchors):
            PR = 16
            for n in range(2 * D3 // PR):
                r, cs = (n // 2) * PR, slice((n % 2) * LANES, (n % 2 + 1) * LANES)
                w = [[wdt_v[p, k, j * D3 + r:j * D3 + r + PR, cs].astype(F32)
                      for j in range(3)] for k in range(3)]
                w[0][1] = _tie(w[0][1], spread_over(anchors, n, 2 * D3 // PR))
                for i, v in enumerate(_w_sums(w)):
                    ds_s.at[p, i][r // 2:(r + PR) // 2, cs] = _pk(v)

        GU = ((wg_v, gs_s), (wu_v, us_s))

        def prep_gu(p, anchors, ids=tuple(range(15))):
            PR = 16
            nr = D3 // PR
            for n in range(4 * nr):
                c, (w_v, s_s), r = n % 2, GU[(n // 2) % 2], (n // 4) * PR
                cache = {}

                def w(k, j):
                    if (k, j) not in cache:
                        ld = lambda c: w_v[p, j, k * D3 + r:k * D3 + r + PR,
                                           c * LANES:(c + 1) * LANES].astype(F32)
                        v = ld(c)
                        if k != j:
                            v = _tie(v, spread_over(anchors, n, 4 * nr))
                        cache[k, j] = v - ld(1 - c) if r // KU == 1 + c else v
                    return cache[k, j]

                for i in ids:
                    v = None
                    for k, j, sg in _W_TERMS[i]:
                        v = w(k, j) if v is None else (v + w(k, j) if sg > 0 else v - w(k, j))
                    s_s.at[p, i][r // 2:(r + PR) // 2, c * LANES:(c + 1) * LANES] = _pk(v)

        NS = cfg['msplit']

        def gu_prod(p, i, t, anchors, slabs, slot=0):
            u = KU // 2

            def rhs(s, s_s):
                if s == 1:
                    return s_s[p, i, :2 * u, :LANES]
                if s == 0:
                    return cat0(s_s[p, i, u:2 * u, LANES:], s_s[p, i, 2 * u:, :LANES])
                return cat0(s_s[p, i, :u, LANES:], s_s[p, i, 2 * u:, LANES:])

            q = TH // 2 // NS
            for n, h in enumerate(slabs):
                y = []
                for s in range(3):
                    r = _upk(cat1(rhs(s, gs_s), rhs(s, us_s)))
                    y.append(_dot(_upk(a_s[3 * i + s, h * q:(h + 1) * q]), r))
                    if (3 * n + s) % len(slabs) == 0:
                        anchors.append(y[-1][:8, :LANES])
                y1, y2 = y[1] + y[0], y[2] + y[0]
                for m in range(2):
                    cs = slice(m * LANES, (m + 1) * LANES)
                    v = cat1(y1[:, cs], y2[:, cs])
                    if i < 9 and 't' in cfg['stash']:
                        k = p if isinstance(p, int) else slot
                        t_s[k, m, i, 2 * h * q:2 * (h + 1) * q] = v
                        v = lambda k=k, m=m, h=h: t_s[k, m, i, 2 * h * q:2 * (h + 1) * q]
                    t.setdefault((m, h), {})[i] = v

        def gu_col(t, hv, p, j, anchors, slabs):
            ids = [_DIAG.get((s, j)) for s in range(3)]
            if cfg['fslab']:
                for h in slabs:
                    for i in ids:
                        if i is not None:
                            gu_prod(p, i, t, anchors if h == slabs[0] else [], [h])
            else:
                for i in ids:
                    if i is not None:
                        gu_prod(p, i, t, anchors, slabs)
            for h in slabs:
                g, u = [_column(t[m, h], [None if i is None else t[m, h][i] for i in ids], j)
                        for m in range(2)]
                hv[j, h] = [_gelu_mul2(g[i], u[i]) for i in range(2)]

        def h_ops(h):
            return [v.astype(BF16) for v in _x_ops(*[[h[j][i] for j in range(3)]
                                                     for i in range(2)])]

        def h_join(hv):
            return h_ops({j: [cat0(*[hv[j, h][i] for h in range(NS)]) for i in range(2)]
                          for j in range(3)})

        def gu_piece(p, order, anchors, slot):
            t, hv = {}, {}
            for slabs in ([[h] for h in range(NS)] if cfg['slab'] else [list(range(NS))]):
                for step in order:
                    if step[0] == 'S':
                        for i in _PARTS[int(step[1])]:
                            gu_prod(p, i, t, anchors, slabs, slot)
                    else:
                        gu_col(t, hv, p, int(step[1]), anchors, slabs)
            return h_join(hv)

        D_ORDER = _PAIR_ORDER + (9, 10, 11, 12, 13, 14)

        def down_mm(acc, bs, lo, anchors, which=D_ORDER, fine=False):
            p = [None] * 15 if acc is None else list(acc)
            for i in which:
                y = None
                for n, b in enumerate(bs):
                    if i in _W_RAW:
                        k, j = _W_RAW[i]
                        v = _dot_nt(wdt_v[lo + n, k, j * D3:(j + 1) * D3, :], b[i])
                    elif len(bs) % 2 and i == 14 and n == 0:
                        v = cat0(*[_dot_nt(_upk(ds_s[lo, _W_SUM[i],
                                                     h * Q3 // 2:(h + 1) * Q3 // 2, :]), b[i])
                                   for h in range(2)])
                    else:
                        v = _dot_nt(_upk(ds_s[lo + n, _W_SUM[i]]), b[i])
                    y = v if y is None else y + v
                p[i] = y if p[i] is None else p[i] + y
                anchors.append(p[i][:8])
                if fine:
                    anchors.append(p[i][D3 // 2:D3 // 2 + 8])
            return p

        def finish(blk, acc):
            y = [cat1(*_column(acc, [acc[_DIAG[s, j]] if (s, j) in _DIAG else None
                                     for s in range(3)], j)) for j in range(3)]
            xio_s[blk] = (xmid_s[blk] + 0.5 * cat0(*y)).astype(BF16)

        def load_acc(k):
            return [acc_s[k, i] for i in range(15)]

        def store_acc(k, acc):
            for i in range(15):
                acc_s[k, i] = acc[i]

        def load_b(k=0):
            return [_upk(b_s[i * TH // 2:(i + 1) * TH // 2, :])
                    for i in range(15 * k, 15 * k + 15)]

        def store_b(b, k=0):
            for i in range(15):
                b_s[(15 * k + i) * TH // 2:(15 * k + i + 1) * TH // 2, :] = _pk(b[i])

        def pre_phase():
            x0_cp, x1_cp = x_cp(0, 0), x_cp(1, 3)
            order = [x0_cp, wq_cp(0), wq_cp(1), x1_cp, wq_cp(2)]
            for p in range(NP + 1):
                order += group_cp(p)
            xr_cp = [x_cp(b, SEM_P + NP + 1) for b in range(2, NB)]
            order += xr_cp
            for cp in order:
                cp.start()
            get = lambda an, name: [an[min(i, len(an) - 1)] for i in cfg[name]]
            e_grp = lambda e: ((e >> 1) & 1, ((e >> 2) << 1) | (e & 1))
            if 'a' in cfg['sub']:
                pre_a(x0_cp, x1_cp, get, e_grp)
            if 'b' in cfg['sub']:
                pre_b(get, e_grp)
            if 'c' in cfg['sub']:
                pre_c(get)
            wait('WX', xr_cp)

        def pre_a(x0_cp, x1_cp, get, e_grp):
            qkv_s[0] = jnp.zeros(qkv_s.shape[1:], U32)
            acc_s[...] = jnp.zeros(acc_s.shape, F32)
            wait('WX0', [x0_cp])
            xn0 = ln1(0, ()).astype(BF16)
            done = 0
            for i in range(3):
                wait('WQ%d' % i, [wq_cp(i)] + ([x1_cp] if i == 2 else []))
                wt = _pk(wqkv_v[:, WQ[i]:WQ[i + 1]].T)
                wt_s[WQ[i] // 2:WQ[i + 1] // 2, :D] = wt
                anchors = []
                qkv_mm(0, xn0, range(done, WQ[i + 1] // QR), anchors)
                done = WQ[i + 1] // QR
                if i > 0:
                    for n, a in enumerate(get(anchors, 'a_w%d' % i)):
                        prep_att(12 * (i - 1) + n, a)
            xn1 = ln1(1, get(anchors, 'a_ln'), get(anchors, 'a_lnb')).astype(BF16)
            qkv_mm(1, xn1, (0, 2, 4, 1), anchors)
            for e in range(8):
                att_group(0, *e_grp(e), anchors[cfg['att0'][e]], 9)
            wait('WO', group_cp(0))
            wo = pltpu.bitcast(wo_v[...], U32)
            wt_s[3 * RP:, :D] = _pk(cat0(_lo(wo), _hi(wo)).astype(BF16).T)
            an = []
            stats = wo_mm(0, an, False)
            qkv_mm(1, xn1, [3], an)
            plain_lhs(0, stats)
            b = plain_piece(0, an)
            qkv_mm(1, xn1, [5], an)
            prep_gu(0, get(an, 'z_g'))
            if cfg['fast0']:
                ffn_lhs(0, stats, get(an, 'z_l'))
            for e in range(3):
                att_group(1, *e_grp(e), an[cfg['z_att'][e]], 9)
            store_b(b)

        def pre_b(get, e_grp):
            def piece(p, carry):
                wait('WP', group_cp(p))
                b_prev = load_b()
                an = []
                if cfg['fast0']:
                    acc = down_mm(load_acc(0), [b_prev], p - 1, an, D_ORDER[:6], True)
                    t, hv, done = {}, {}, set()
                    for step in cfg['order1']:
                        k = int(step[1])
                        part = k if step[0] == 'S' else 3
                        slabs = [int(step[2])] if len(step) > 2 else list(range(NS))
                        if part not in done:
                            prep_gu(p, get(an, 'f_g%d' % part), _PARTS[part])
                            done.add(part)
                        if step[0] == 'S':
                            for i in _PARTS[k]:
                                gu_prod(p, i, t, an, slabs)
                        else:
                            gu_col(t, hv, p, k, an, slabs)
                    b = h_join(hv)
                    prep_d(p - 1, get(an, 'p_d'))
                    store_acc(0, down_mm(acc, [b_prev], p - 1, an, D_ORDER[6:]))
                else:
                    b = plain_piece(p, an)
                    prep_d(p - 1, get(an, 'p_d'))
                    store_acc(0, down_mm(load_acc(0), [b_prev], p - 1, an))
                    prep_gu(p, get(an, 'p_g'))
                att_group(1, *e_grp(p + 2), an[cfg['p_att'][0]], 9)
                for i, a in enumerate(get(an, 'p_w')):
                    prep_att(jnp.minimum(24 + (p - 1) * 5 + i, 47), a)
                store_b(b)
                return carry

            lax.fori_loop(1, NP, piece, 0)

        def pre_c(get):
            wait('WD', group_cp(NP))
            an = []
            stats = wo_mm(1, an, True)
            prep_d(NP - 1, get(an, 't_d'))
            acc = down_mm(load_acc(0), [load_b()], NP - 1, [])
            ffn_lhs(1, stats, [])
            finish(0, acc)

        if 'pre' in cfg['phases']:
            pre_phase()

        def body(u, carry):
            bu = u & (NB - 1)
            ba = (u + 1) & (NB - 1)
            acc, stats, an, b = None, None, {}, {}
            get = lambda name: [an[k][i] for k, i in cfg[name]]
            for step in cfg['body']:
                an[step] = []
                if step == 'Q':
                    qkv_fast(ba, att_rhs(ln1(ba, get('ln1'), get('ln1b')), u >> 8 if 'q' in cfg['stash'] else None),
                             an[step])
                elif step == 'W':
                    attention(ba, get('att'), cfg['win'])
                    stats = wo_mm(ba, an[step], True, get('orhs'),
                                  u >> 8 if 'w' in cfg['stash'] else None)
                elif step == 'L':
                    ffn_lhs(ba, stats, get('lhs'))
                elif step[0] == 'S':
                    slabs = [int(step[3])] if len(step) > 3 else list(range(NS))
                    for i in _PARTS[int(step[2])]:
                        gu_prod(int(step[1]), i, b.setdefault(step[:2], {}), an[step], slabs)
                elif step[0] == 'F':
                    j, c = int(step[1]), int(step[2])
                    slabs = [int(step[3])] if len(step) > 3 else list(range(NS))
                    hv = b.setdefault(step[:2], {})
                    gu_col(b['S' + step[1]], hv, j, c, an[step], slabs)
                    if len(hv) == 3 * NS:
                        b[j] = h_join(hv)
                        if 'b' in cfg['stash']:
                            store_b(b[j], j)
                            b[j] = load_b(j)
                else:
                    js = [int(c) for c in step[1:]]
                    acc = down_mm(acc, [b[j] for j in js], js[0], an[step])
            finish(bu, acc)

            @pl.when(u >= NB)
            def _():
                out_copy(bu).start()
            return carry

        if scopes:
            with jax.named_scope('LOOP'):
                lax.fori_loop(1, NU - 1, body, 0)
        elif 'main' in cfg['phases']:
            lax.fori_loop(1, NU - 1, body, 0)

        def last(c, carry):
            los = [2 * c + j for j in range(2)]
            b = [gu_piece(lo, cfg['order'], [], j) for j, lo in enumerate(los)]
            acc = load_acc(1)
            for j in range(2):
                acc = down_mm(acc, [b[j]], los[j], [])
            store_acc(1, acc)
            return carry

        if 'last' in cfg['phases']:
            lax.fori_loop(0, NP // 2, last, 0)
        if len(cfg['phases']) < 3:
            def keep(i, c):
                v = (gs_s[i, i, :8, :LANES] + us_s[i, i, :8, :LANES] + ds_s[i, i, :8, :LANES]
                     + wl_s[rows8(i * 8), :LANES] + a_s[i, :8] + qkv_s[i, :8]
                     + b_s[rows8(i * 8), :LANES] + wt_s[rows8(i * 8), :LANES])
                acc_s[1, 0, :8] = (lax.bitcast_convert_type(v, F32) + o_s[i, :8]
                                   + acc_s[i, i, :8])
                return c
            lax.fori_loop(0, 2, keep, 0)
        finish(NB - 1, load_acc(1))
        out_copy(NB - 1).start()
        wait('WOUT', [out_copy(b) for b in range(NB)])

    scratch = [
        pltpu.VMEM((NB, D, TM), BF16),
        pltpu.VMEM((D, 3 * D), BF16),
        pltpu.VMEM((D, D), BF16),
        pltpu.VMEM((NP, 3, D, PW), BF16),
        pltpu.VMEM((NP, 3, D, PW), BF16),
        pltpu.VMEM((NP, 3, D, PW), BF16),
        pltpu.VMEM((2 * D, 8 * LANES), U32),
        pltpu.VMEM((4 * Q3, 16 * LANES), U32),
        pltpu.VMEM((NP, 15, Q3, PW), U32),
        pltpu.VMEM((NP, 15, Q3, PW), U32),
        pltpu.VMEM((NP, 9, Q3, PW), U32),
        pltpu.VMEM((NB, D, TM), F32),
        pltpu.VMEM((54, TH // 2, LANES), U32),
        pltpu.VMEM((S // LANES + 1, 3 * RP, LANES), U32),
        pltpu.VMEM((NT, D, LANES), F32),
        pltpu.VMEM((2, 15, D3, TH), F32),
        pltpu.VMEM((NP * 15 * TH // 2, PW), U32),
        pltpu.VMEM((1, 9 * 64, 2 * LANES), U32),
        pltpu.VMEM((NP, 2, 9, TH, PW), F32),
        pltpu.SemaphoreType.DMA((SEM_P + NP + 2,)),
        pltpu.SemaphoreType.DMA((1,)),
    ]
    return kernel, scratch


_CFG = dict(
    scopes=False,
    fast0=True,
    psplit=1,
    rcp=False,
    late=True,
    stash='qw',
    slab=True,
    fslab=False,
    win=9,
    sub='abc',
    orhs=(),
    msplit=2,
    phases=('pre', 'main', 'last'),
    order=('S0', 'S1', 'F0', 'S2', 'F1', 'F2'),
    body=('S010', 'S000', 'F000', 'S020', 'F010', 'F020', 'S001', 'S011', 'F001',
        'S110', 'S021', 'F021', 'S100', 'F100', 'S120', 'S101', 'F110', 'F011', 'Q',
        'F120', 'S111', 'F101', 'S121', 'F111', 'F121', 'S200', 'S210', 'F200', 'S220',
        'F210', 'F220', 'S300', 'S201', 'S211', 'F201', 'S320', 'S221', 'F211', 'F221',
        'S310', 'D01', 'F300', 'S301', 'S311', 'F301', 'S321', 'F311', 'F321', 'S400',
        'F310', 'F320', 'S420', 'F410', 'S410', 'S401', 'F420', 'S411', 'F400', 'S421',
        'F411', 'F421', 'S500', 'F401', 'S501', 'S510', 'D23', 'F500', 'S520', 'W',
        'F520', 'S511', 'F510', 'S521', 'F501', 'F511', 'F521', 'D4', 'D5', 'L'),
    ln1=(('S010', 4), ('S010', 5), ('S010', 6), ('S010', 7), ('S010', 8), ('S000', 0),
        ('S000', 1), ('S000', 2), ('S000', 3)),
    ln1b=(('S110', 2), ('S110', 3), ('S110', 5), ('S110', 6), ('S110', 8), ('S021', 0),
        ('S021', 2), ('S021', 3), ('S021', 5), ('S021', 6), ('S021', 8), ('F021', 0)),
    att=(('S300', 8), ('D01', 1), ('D01', 7), ('D01', 8), ('D01', 10), ('F300', 4),
        ('D23', 5), ('D23', 9)),
    lhs=(('D4', 3), ('D5', 1), ('D5', 4)),
    att0=(15, 18, 21, 24, 27, 30, 33, 37),
    order0=('S0', 'S1', 'S2', 'F0', 'F1', 'F2'),
    order1=('S0', 'S1', 'S2', 'F0', 'F1', 'F2'),
    a_w1=(0, 1, 2, 3, 5, 5, 8, 9, 10, 11, 12, 14),
    a_w2=(0, 0, 2, 3, 4, 4, 6, 6, 8, 9, 11, 16),
    a_ln=(0, 3, 7),
    a_lnb=(6, 6, 8),
    z_g=(3, 4, 5, 6, 8, 9, 10, 12, 13, 14, 15, 17, 18, 19, 21, 22, 23, 25, 26, 27, 28,
        30, 31, 32, 34, 35, 36, 38, 39, 40, 41, 43, 44, 45, 47, 48, 49, 51, 52, 53, 54,
        56, 57, 58, 60, 61, 62, 64),
    z_att=(72, 77, 83),
    p_g0=(0, 1, 2, 3, 4, 5),
    p_g1=(6, 7, 8, 9, 10, 10),
    p_g2=(12, 13, 14, 15, 16, 17),
    p_g3=(14, 16, 18, 20, 22, 24, 26, 28, 30, 32, 34, 36),
    t_d=(0, 0, 1, 1, 2, 3, 3, 4, 5, 6, 6, 7, 8, 9, 9, 9, 10, 11, 11, 12, 13, 14, 15,
        16),
    p_d=(32, 33, 35, 35, 35, 37, 37, 38, 39, 41, 42, 43, 44, 45, 45, 46, 47, 48, 49, 51,
        52, 53, 54, 56),
    p_att=(60,),
    p_w=(12, 60, 63, 65, 65),
    p_g=(0, 1, 2, 3, 4, 5, 6, 7, 9, 10, 11, 12, 13, 14, 15, 16, 18, 19, 20, 21, 22, 23,
        24, 25, 27, 28, 29, 30, 31, 32, 33, 34, 36, 37, 38, 39, 40, 41, 42, 43, 45, 46,
        47, 48, 49, 50, 51, 53),
    z_l=(42, 48, 55),
    f_g0=(0, 0, 0, 1, 1, 2, 3, 3, 4, 4, 5, 5),
    f_g1=(4, 5, 5, 7, 8, 9, 9, 10, 11, 12, 13, 15),
    f_g2=(1, 12, 12, 15, 15, 16, 17, 18, 19, 20, 20, 24),
    f_g3=(4, 14, 16, 17, 18, 19, 21, 22, 23, 23, 24, 25, 26, 27, 28, 29, 30, 31, 32, 33,
        34, 35, 36, 37),
)


def _run(A_x, A_wqkv, A_wo, B_w_gate, B_w_up, B_w_down, **kw):
    _, S, D = A_x.shape
    F = B_w_gate.shape[1]
    kernel, scratch = _make_kernel(S, D, F, 256, {**_CFG, **kw})
    hbm = pl.BlockSpec(memory_space=pl.ANY)
    out_t = pl.pallas_call(
        kernel,
        in_specs=[hbm] * 6,
        out_specs=hbm,
        out_shape=jax.ShapeDtypeStruct((D, S), A_x.dtype),
        scratch_shapes=scratch,
        compiler_params=pltpu.CompilerParams(vmem_limit_bytes=110 * 1024 * 1024),
    )(A_x.reshape(S, D).T, A_wqkv, A_wo, B_w_gate, B_w_up, B_w_down.T)
    return out_t.T.reshape(A_x.shape)


@jax.jit
def pallas_interleave_layers__sliding_local_dilated__glu_gated_geglu__prompt_kernel(
    A_x: jax.Array,
    A_wqkv: jax.Array,
    A_wo: jax.Array,
    B_x: jax.Array,
    B_w_gate: jax.Array,
    B_w_up: jax.Array,
    B_w_down: jax.Array,
):
    del B_x
    return _run(A_x, A_wqkv, A_wo, B_w_gate, B_w_up, B_w_down)
```

```python
import functools

import jax
import jax.numpy as jnp
import jax.experimental.pallas as pl
import jax.experimental.pallas.tpu as pltpu
from jax import lax

H = 32
W = 8
DIL = 2
EPS = 1e-5
LANES = 128

F32 = jnp.float32
BF16 = jnp.bfloat16
U32 = jnp.uint32

_NT = (((1,), (1,)), ((), ()))


def _tree_sum(parts, op=jnp.add):
    while len(parts) > 1:
        nxt = [op(parts[i], parts[i + 1]) for i in range(0, len(parts) - 1, 2)]
        if len(parts) % 2:
            nxt.append(parts[-1])
        parts = nxt
    return parts[0]


def _ln_stats(slabs, d, anchors=()):
    n_acc = 4
    s1, s2, pilot = [None] * n_acc, [None] * n_acc, None
    for i, x in enumerate(slabs):
        if pilot is None:
            pilot = x[0:1, :]
            pil = jnp.broadcast_to(pilot, x.shape)
            pils = [_tie(pil, a) for a in anchors] or [pil]
        dx = x - pils[i * len(pils) // (d // 8)]
        j = i % n_acc
        s1[j] = dx if s1[j] is None else s1[j] + dx
        s2[j] = dx * dx if s2[j] is None else s2[j] + dx * dx
    e1 = jnp.sum(_tree_sum(s1), axis=0, keepdims=True) * (1.0 / d)
    e2 = jnp.sum(_tree_sum(s2), axis=0, keepdims=True) * (1.0 / d)
    var = jnp.maximum(e2 - e1 * e1, 0.0)
    return pilot + e1, lax.rsqrt(var + EPS)


def _zero_like_dep(v):
    return (lax.bitcast_convert_type(v, U32) >> 31) >> 1


def _tie(x, anchor):
    if anchor is None:
        return x
    z = lax.bitcast_convert_type(_zero_like_dep(anchor), F32)
    z = jnp.concatenate([z] * -(-x.shape[1] // LANES), axis=1)[:, :x.shape[1]]
    if x.shape[0] == 8:
        return x + z
    return jnp.concatenate([x[:8] + z, x[8:]], axis=0)


def _gelu_mul2(g, u):
    c0 = 0.7978845608028654
    c1 = c0 * 0.044715
    t = jnp.tanh(g * (c0 + c1 * (g * g)))
    return (g * u) * (1.0 + t)


def _lo(x):
    return lax.bitcast_convert_type(x << 16, F32)


def _hi(x):
    return lax.bitcast_convert_type(x & jnp.uint32(0xFFFF0000), F32)


def _pk(x):
    return pltpu.bitcast(x.astype(BF16), U32)


def _upk(x):
    return pltpu.bitcast(x, BF16)


def _dot(a, b):
    return jnp.dot(a, b, preferred_element_type=F32)


def _dot_nt(a, b):
    return lax.dot_general(a, b, _NT, preferred_element_type=F32)


def _x_ops(x1, x2):
    d = [a - b for a, b in zip(x1, x2)]
    return [x1[0] + x2[1], x2[0] + x2[1], x1[0] + x1[1],
            d[1] + x1[2], x1[1] + x1[2], d[1] + d[2],
            d[0] - x2[2], d[0] + d[2], x2[0] + x2[2],
            x1[0], d[0], x2[1], d[1], x1[2], x2[2]]


def _x_rem(x1, x2):
    a, b, c = 0, 1, 2
    cat = lambda u, v: jnp.concatenate([u, v], axis=0)
    return [cat(x1[c], x2[b]), cat(x1[a], x1[b] - x2[b]), cat(x2[a], x2[c] - x1[c])]


def _w_sums(w):
    return [w[0][1] + w[1][0], w[1][2] + w[2][1], w[0][2] + w[2][0],
            w[0][0] + w[0][2] - w[1][0], w[2][0] - w[0][0] - w[0][1],
            w[1][1] + w[1][2] - w[0][1], w[1][0] + w[1][1] - w[2][1],
            w[2][0] + w[2][2] - w[1][2], w[2][1] + w[2][2] - w[0][2]]


_W_TERMS = {0: ((0, 1, 1), (1, 0, 1)), 3: ((1, 2, 1), (2, 1, 1)), 6: ((0, 2, 1), (2, 0, 1)),
            9: ((0, 0, 1), (0, 2, 1), (1, 0, -1)), 10: ((2, 0, 1), (0, 0, -1), (0, 1, -1)),
            11: ((1, 1, 1), (1, 2, 1), (0, 1, -1)), 12: ((1, 0, 1), (1, 1, 1), (2, 1, -1)),
            13: ((2, 0, 1), (2, 2, 1), (1, 2, -1)), 14: ((2, 1, 1), (2, 2, 1), (0, 2, -1)),
            1: ((0, 1, 1),), 2: ((1, 0, 1),), 4: ((1, 2, 1),), 5: ((2, 1, 1),),
            7: ((2, 0, 1),), 8: ((0, 2, 1),)}
_PARTS = ((1, 2, 0), (7, 8, 6), (4, 5, 3), (9, 10, 11, 12, 13, 14))
_W_SUM = {0: 0, 3: 1, 6: 2, 9: 3, 10: 4, 11: 5, 12: 6, 13: 7, 14: 8}
_W_RAW = {1: (0, 1), 2: (1, 0), 4: (1, 2), 5: (2, 1), 7: (2, 0), 8: (0, 2)}
_PAIR_ORDER = (1, 2, 4, 5, 7, 8, 0, 3, 6)
_DIAG = {(0, 0): 9, (2, 0): 10, (0, 1): 11, (1, 1): 12, (1, 2): 13, (2, 2): 14}
_PAIR = {(0, 0): ((6, -1), (8, -1)), (1, 0): ((2, 1), (7, 1)), (2, 0): ((0, 1), (1, -1)),
         (0, 1): ((3, 1), (4, -1)), (1, 1): ((0, 1), (2, -1)), (2, 1): ((1, 1), (5, -1)),
         (0, 2): ((4, 1), (8, 1)), (1, 2): ((6, 1), (7, -1)), (2, 2): ((5, 1), (3, -1))}


def _column(t, base, j):
    s = []
    for k in range(3):
        v = base[k]
        for i, sg in _PAIR[k, j]:
            ti = t[i]() if callable(t[i]) else t[i]
            v = ti if v is None else (v + ti if sg > 0 else v - ti)
        s.append(v)
    return s[1] + s[0], s[2] + s[0]


def _make_kernel(S, D, F, TM, cfg):
    NB = S // TM
    NT = TM // LANES
    DH = D // H
    DP = DH // 2
    RP = D // 2
    NG = H // 8
    scale = float(DH) ** -0.5
    NU = 2 * NB
    TH = TM // 2
    FT = F // 3
    D2 = D // 2
    D3 = D // 3
    Q3 = D3 // 2
    KU = D // 9
    KR = 3 * LANES
    NQ = 6
    QR = 3 * D // NQ
    WQ = (0, 640, 1152, 3 * D)
    PW = 256
    NP = FT // PW
    scopes = cfg['scopes']
    assert NG == 4 and NB & (NB - 1) == 0
    SEM_P = 4

    def kernel(x_hbm, wqkv_hbm, wo_hbm, wg_hbm, wu_hbm, wdt_hbm, out_hbm,
               xio_s, wqkv_v, wo_v, wg_v, wu_v, wdt_v, wt_s, wl_s,
               gs_s, us_s, ds_s, xmid_s, a_s, qkv_s, o_s, acc_s, b_s, r_s, t_s,
               sem_i, sem_o):

        def wait(name, cps):
            if scopes:
                with jax.named_scope(name):
                    for cp in cps:
                        cp.wait()
            else:
                for cp in cps:
                    cp.wait()

        def cols(lo, n):
            if not isinstance(lo, int):
                lo = pl.multiple_of(lo, LANES)
            return pl.ds(lo, n)

        def rows8(lo, n=8):
            if not isinstance(lo, int):
                lo = pl.multiple_of(lo, 8)
            return pl.ds(lo, n)

        def out_copy(b):
            return pltpu.make_async_copy(
                xio_s.at[b], out_hbm.at[:, cols(b * TM, TM)], sem_o.at[0])

        def x_cp(b, sem):
            return pltpu.make_async_copy(x_hbm.at[:, cols(b * TM, TM)], xio_s.at[b],
                                         sem_i.at[sem])

        def wq_cp(i):
            sl = cols(WQ[i], WQ[i + 1] - WQ[i])
            return pltpu.make_async_copy(wqkv_hbm.at[:, sl], wqkv_v.at[:, sl],
                                         sem_i.at[1 + i])

        def piece_cp(src, dst, p, sem):
            return [pltpu.make_async_copy(src.at[:, cols(j * FT + p * PW, PW)],
                                          dst.at[p, j],
                                          sem_i.at[sem]) for j in range(3)]

        def group_cp(p):
            sem = SEM_P + p
            cps = []
            if not (isinstance(p, int) and p == NP):
                cps += piece_cp(wg_hbm, wg_v, p, sem) + piece_cp(wu_hbm, wu_v, p, sem)
            if not (isinstance(p, int) and p == 0):
                cps += piece_cp(wdt_hbm, wdt_v, p - 1, sem)
            return cps

        lane = lax.broadcasted_iota(jnp.int32, (8, LANES), 1)
        cat0 = lambda *v: jnp.concatenate(v, axis=0)
        cat1 = lambda *v: jnp.concatenate(v, axis=1)

        def spread_over(anchors, n, total):
            return anchors[n * len(anchors) // total] if anchors else None

        def slab_group(r):
            return (r % LANES) // 16 if r < KR else 8 + ((r - KR) % KU) // 16

        def ln1(blk, anchors1, anchors2=()):
            slabs = (xio_s[blk, r:r + 8, :].astype(F32) for r in range(0, D, 8))
            m, rs = _ln_stats(slabs, D, anchors1)
            if not anchors2:
                return (xio_s[blk].astype(F32) - m) * rs
            m8 = jnp.broadcast_to(m, (8, TM))
            ms = [_tie(m8, a) for a in anchors2]
            ms = [spread_over(ms, slab_group(r), 12) for r in range(0, D, 8)]
            return (xio_s[blk].astype(F32) - cat0(*ms)) * rs

        def dot_k(rows, x, anchors, even=False):
            y = None
            for n, k in enumerate(range(0, D, LANES)):
                ks = slice(k, min(k + LANES, D))
                if even and k + LANES >= D:
                    mid = (rows.start + rows.stop) // 2
                    v = cat0(_dot(_upk(wt_s[rows.start:mid, ks]), x[ks]),
                             _dot(_upk(wt_s[mid:rows.stop, ks]), x[ks]))
                else:
                    v = _dot(_upk(wt_s[rows, ks]), x[ks])
                anchors.extend(v[r:r + 8, :LANES] for r in ((0, 144) if n % 2 else (72, 216)))
                y = v if y is None else y + v
            return y

        def put_qkv(blk, rows, y):
            pk = _pk(y)
            for c in range(NT):
                qkv_s[1 + blk * NT + c, rows, :] = pk[:, c * LANES:(c + 1) * LANES]

        def qkv_mm(blk, xn, chunks, anchors, even=False):
            for r in chunks:
                rows = slice(r * QR // 2, (r + 1) * QR // 2)
                put_qkv(blk, rows, dot_k(rows, xn, anchors, even))

        def split_k(x):
            hs = (x[:, :TH], x[:, TH:])
            blocks = [[h[k * LANES:(k + 1) * LANES] for k in range(3)] for h in hs]
            units = [[h[KR + k * KU:KR + (k + 1) * KU] for k in range(3)] for h in hs]
            return blocks, units

        def prep_att(pat, anchor):
            assert Q3 == 96
            row0 = pat * 8
            src0 = row0 + ((pat * 43) >> 9) * (2 * Q3)
            w = [_upk(wt_s[rows8(src0 + j * Q3), :D]).astype(F32) for j in range(3)]
            w[0] = cat1(_tie(w[0][:, :LANES], anchor), w[0][:, LANES:])
            tiles = _w_sums([[w[j][:, k * LANES:(k + 1) * LANES] for j in range(3)]
                             for k in range(3)])
            for j in range(3):
                a, b, c = (w[j][:, KR + k * KU:KR + (k + 1) * KU] for k in range(3))
                tiles += [cat1(c, b), cat1(a, c)]
            wl_s[rows8(row0), :15 * LANES] = _pk(cat1(*tiles))

        def att_rhs(x, stash=None):
            blocks, units = split_k(x)
            ops = _x_ops(*blocks) + _x_rem(*units)
            if stash is None:
                return [v.astype(BF16) for v in ops]
            loc = lambda i, r0, n: (slice((i // 2) * 64 + r0, (i // 2) * 64 + r0 + n),
                                    slice((i % 2) * LANES, (i % 2 + 1) * LANES))
            for r in range(0, LANES, 16):
                for i, v in enumerate(ops):
                    r_s.at[0][loc(i, r // 2, 8)] = _pk(v[r:r + 16])
            return [_upk(r_s.at[stash][loc(i, 0, 64)]) for i in range(18)]

        def att_mm(sec, rhs, anchors):
            tl = lambda i: _upk(wl_s[sec * Q3:(sec + 1) * Q3, i * LANES:(i + 1) * LANES])
            raw = lambda k, j: _upk(wt_s[(3 * sec + j) * Q3:(3 * sec + j + 1) * Q3,
                                         k * LANES:(k + 1) * LANES])
            t = {}
            for i in _PAIR_ORDER:
                t[i] = _dot(raw(*_W_RAW[i]) if i in _W_RAW else tl(_W_SUM[i]), rhs[i])
                anchors.append(t[i][:8])
            out = []
            for j in range(3):
                base = []
                for s in range(3):
                    v = _dot(raw(3, j) if s == 1 else tl(9 + 2 * j + s // 2), rhs[15 + s])
                    if (s, j) in _DIAG:
                        i = _DIAG[s, j]
                        v = _dot(tl(_W_SUM[i]), rhs[i]) + v
                    base.append(v)
                    anchors.append(base[-1][:8])
                out.append(cat1(*_column(t, base, j)))
            return cat0(*out)

        def qkv_fast(blk, rhs, anchors):
            for sec in range(3):
                put_qkv(blk, slice(sec * RP, (sec + 1) * RP), att_mm(sec, rhs, anchors))

        def shifted(ln, cur, prev, w):
            if w == 0:
                return cur
            sh = DIL * w
            return pltpu.roll(jnp.where(ln < LANES - sh, cur, prev), sh, axis=1)

        def att_group(blk, c, hg, anchor, win):
            att_values(blk, c, hg, anchor, win)(None)

        def att_values(blk, c, hg, anchor, win):
            tile = blk * NT + c
            base = hg * 8 * DP
            if isinstance(hg, int):
                cur, prev, o_t = qkv_s.at[1 + tile], qkv_s.at[tile], o_s.at[c]
            else:
                n = 2 * RP + 8 * DP
                base = pl.multiple_of(base, 8)
                cur = qkv_s.at[1 + tile, pl.ds(base, n)]
                prev = qkv_s.at[tile, pl.ds(base, n)]
                o_t = o_s.at[c, pl.ds(base, RP + 8 * DP)]
                base = 0
            ln = lane + _zero_like_dep(anchor).astype(jnp.int32)
            logits = [None] * W
            done = []
            for dd in range(DP):
                q = cur[pl.ds(base + dd, 8, stride=DP), :]
                kc = cur[pl.ds(RP + base + dd, 8, stride=DP), :]
                if dd >= win:
                    kc = kc | _zero_like_dep(done[dd - win])
                kp = prev[pl.ds(RP + base + dd, 8, stride=DP), :]
                q0, q1 = _lo(q), _hi(q)
                for w in range(W):
                    ks = shifted(ln, kc, kp, w)
                    t = q0 * _lo(ks) + q1 * _hi(ks)
                    logits[w] = t if logits[w] is None else logits[w] + t
                done.append(ks)
            logits = [l * scale for l in logits]
            if not (isinstance(c, int) and c > 0):
                pos = lane + tile * LANES
                logits = [l if w == 0 else jnp.where(pos >= DIL * w, l, -1e9)
                          for w, l in enumerate(logits)]
            m = _tree_sum(logits, jnp.maximum)
            e = [jnp.exp(l - m) for l in logits]
            den = _tree_sum(e)
            if cfg['rcp']:
                r = pl.reciprocal(den, approx=True)
                r = r * (2.0 - den * r)
            else:
                r = 1.0 / den
            p = e if cfg['late'] else [x * r for x in e]

            def apply(anchor2):
                ln = lane + _zero_like_dep(m if anchor2 is None else anchor2).astype(jnp.int32)
                done = []
                for dd in range(DP):
                    vc = cur[pl.ds(2 * RP + base + dd, 8, stride=DP), :]
                    if dd >= win:
                        vc = vc | _zero_like_dep(done[dd - win])
                    vp = prev[pl.ds(2 * RP + base + dd, 8, stride=DP), :]
                    o0 = o1 = None
                    for w in range(W):
                        vs = shifted(ln, vc, vp, w)
                        t0, t1 = p[w] * _lo(vs), p[w] * _hi(vs)
                        o0 = t0 if o0 is None else o0 + t0
                        o1 = t1 if o1 is None else o1 + t1
                    done.append(vs)
                    if cfg['late']:
                        o0, o1 = o0 * r, o1 * r
                    o_t[pl.ds(base + dd, 8, stride=DP), :] = o0
                    o_t[pl.ds(RP + base + dd, 8, stride=DP), :] = o1

            return apply

        def attention(blk, anchors, win):
            for c in range(NT):
                for hg in range(NG):
                    att_group(blk, c, hg, anchors[c * NG + hg], win)

        def wo_mm(blk, anchors, fast, anchors_in=(), stash=None):
            o = cat1(*[o_s[c] for c in range(NT)])
            if anchors_in:
                o = cat0(*[_tie(o[r:r + 8], spread_over(anchors_in, slab_group(r), 12))
                           for r in range(0, D, 8)])
            if fast:
                y = att_mm(3, att_rhs(o, stash), anchors)
            else:
                o = o.astype(BF16)
                q = D2 // 2
                y = cat0(*[dot_k(slice(h * q, (h + 1) * q), o, anchors) for h in (6, 7)])
            xm = xio_s[blk].astype(F32) + y
            xmid_s[blk] = xm
            return _ln_stats((xm[r:r + 8] for r in range(0, D, 8)), D)

        def ffn_lhs(blk, stats, anchors):
            m, rs = stats
            m8 = jnp.broadcast_to(m, (8, TM))
            xs = []
            for k in range(3):
                mt = cat0(*[_tie(m8, spread_over(anchors, k, 3))] * (D3 // 8))
                xs.append((xmid_s[blk, k * D3:(k + 1) * D3, :] - mt) * rs)
            ops = _x_ops([x[:, :TH] for x in xs], [x[:, TH:] for x in xs])
            for i, v in enumerate(ops):
                for s, t in enumerate((v[KU:], v[:2 * KU], cat0(v[:KU], v[2 * KU:]))):
                    a_s[3 * i + s] = _pk(t.astype(BF16).T)

        def plain_lhs(blk, stats):
            m, rs = stats
            blocks, units = split_k((xmid_s[blk] - m) * rs)
            for i, v in enumerate(blocks[0] + blocks[1] + _x_rem(*units)):
                a_s[45 + i] = _pk(v.astype(BF16).T)

        def plain_piece(p, anchors):
            h = {}
            for j in range(3):
                hs = []
                for n in range(PW // LANES):
                    cs = slice(n * LANES, (n + 1) * LANES)
                    w = lambda r0, r1: cat1(wg_v[p, j, r0:r1, cs], wu_v[p, j, r0:r1, cs])
                    u = lambda k: w(KR + k * KU, KR + (k + 1) * KU)
                    ps = cfg['psplit']
                    q = TH // 2 // ps
                    hh = []
                    for s in range(ps):
                        tl = lambda *i: _upk(cat1(*[a_s[45 + k, s * q:(s + 1) * q] for k in i]))
                        y0 = _dot(tl(6), cat0(u(2), u(1)))
                        y1 = _dot(tl(0, 1, 2, 7), w(0, KR + 2 * KU))
                        y2 = _dot(tl(3, 4, 5, 8), cat0(w(0, KR + KU), u(2)))
                        if s == 0:
                            anchors.append(y0[:8, :LANES])
                        for y in (y1, y2):
                            anchors.extend(y[r:r + 8, c:c + LANES] for c in (0, LANES)
                                           for r in range(0, 2 * q, TH // 2))
                        hh.append([_gelu_mul2(*[(y + y0)[:, c:c + LANES] for c in (0, LANES)])
                                   for y in (y1, y2)])
                    hs.append([cat0(*[v[i] for v in hh]) for i in range(2)])
                h[j] = [cat1(*[v[i] for v in hs]) for i in range(2)]
            return h_ops(h)

        def prep_d(p, anchors):
            PR = 16
            for n in range(2 * D3 // PR):
                r, cs = (n // 2) * PR, slice((n % 2) * LANES, (n % 2 + 1) * LANES)
                w = [[wdt_v[p, k, j * D3 + r:j * D3 + r + PR, cs].astype(F32)
                      for j in range(3)] for k in range(3)]
                w[0][1] = _tie(w[0][1], spread_over(anchors, n, 2 * D3 // PR))
                for i, v in enumerate(_w_sums(w)):
                    ds_s.at[p, i][r // 2:(r + PR) // 2, cs] = _pk(v)

        GU = ((wg_v, gs_s), (wu_v, us_s))

        def prep_gu(p, anchors, ids=tuple(range(15))):
            PR = 16
            nr = D3 // PR
            for n in range(4 * nr):
                c, (w_v, s_s), r = n % 2, GU[(n // 2) % 2], (n // 4) * PR
                cache = {}

                def w(k, j):
                    if (k, j) not in cache:
                        ld = lambda c: w_v[p, j, k * D3 + r:k * D3 + r + PR,
                                           c * LANES:(c + 1) * LANES].astype(F32)
                        v = ld(c)
                        if k != j:
                            v = _tie(v, spread_over(anchors, n, 4 * nr))
                        cache[k, j] = v - ld(1 - c) if r // KU == 1 + c else v
                    return cache[k, j]

                for i in ids:
                    v = None
                    for k, j, sg in _W_TERMS[i]:
                        v = w(k, j) if v is None else (v + w(k, j) if sg > 0 else v - w(k, j))
                    s_s.at[p, i][r // 2:(r + PR) // 2, c * LANES:(c + 1) * LANES] = _pk(v)

        NS = cfg['msplit']

        def gu_prod(p, i, t, anchors, slabs, slot=0):
            u = KU // 2

            def rhs(s, s_s):
                if s == 1:
                    return s_s[p, i, :2 * u, :LANES]
                if s == 0:
                    return cat0(s_s[p, i, u:2 * u, LANES:], s_s[p, i, 2 * u:, :LANES])
                return cat0(s_s[p, i, :u, LANES:], s_s[p, i, 2 * u:, LANES:])

            q = TH // 2 // NS
            for n, h in enumerate(slabs):
                y = []
                for s in range(3):
                    r = _upk(cat1(rhs(s, gs_s), rhs(s, us_s)))
                    y.append(_dot(_upk(a_s[3 * i + s, h * q:(h + 1) * q]), r))
                    if (3 * n + s) % len(slabs) == 0:
                        anchors.append(y[-1][:8, :LANES])
                y1, y2 = y[1] + y[0], y[2] + y[0]
                for m in range(2):
                    cs = slice(m * LANES, (m + 1) * LANES)
                    v = cat1(y1[:, cs], y2[:, cs])
                    if i < 9 and 't' in cfg['stash']:
                        k = p if isinstance(p, int) else slot
                        t_s[k, m, i, 2 * h * q:2 * (h + 1) * q] = v
                        v = lambda k=k, m=m, h=h: t_s[k, m, i, 2 * h * q:2 * (h + 1) * q]
                    t.setdefault((m, h), {})[i] = v

        def gu_col(t, hv, p, j, anchors, slabs):
            ids = [_DIAG.get((s, j)) for s in range(3)]
            if cfg['fslab']:
                for h in slabs:
                    for i in ids:
                        if i is not None:
                            gu_prod(p, i, t, anchors if h == slabs[0] else [], [h])
            else:
                for i in ids:
                    if i is not None:
                        gu_prod(p, i, t, anchors, slabs)
            for h in slabs:
                g, u = [_column(t[m, h], [None if i is None else t[m, h][i] for i in ids], j)
                        for m in range(2)]
                hv[j, h] = [_gelu_mul2(g[i], u[i]) for i in range(2)]

        def h_ops(h):
            return [v.astype(BF16) for v in _x_ops(*[[h[j][i] for j in range(3)]
                                                     for i in range(2)])]

        def h_join(hv):
            return h_ops({j: [cat0(*[hv[j, h][i] for h in range(NS)]) for i in range(2)]
                          for j in range(3)})

        def gu_piece(p, order, anchors, slot):
            t, hv = {}, {}
            for slabs in ([[h] for h in range(NS)] if cfg['slab'] else [list(range(NS))]):
                for step in order:
                    if step[0] == 'S':
                        for i in _PARTS[int(step[1])]:
                            gu_prod(p, i, t, anchors, slabs, slot)
                    else:
                        gu_col(t, hv, p, int(step[1]), anchors, slabs)
            return h_join(hv)

        D_ORDER = _PAIR_ORDER + (9, 10, 11, 12, 13, 14)

        def down_mm(acc, bs, lo, anchors, which=D_ORDER, fine=False):
            p = [None] * 15 if acc is None else list(acc)
            for i in which:
                y = None
                for n, b in enumerate(bs):
                    if i in _W_RAW:
                        k, j = _W_RAW[i]
                        v = _dot_nt(wdt_v[lo + n, k, j * D3:(j + 1) * D3, :], b[i])
                    elif len(bs) % 2 and i == 14 and n == 0:
                        v = cat0(*[_dot_nt(_upk(ds_s[lo, _W_SUM[i],
                                                     h * Q3 // 2:(h + 1) * Q3 // 2, :]), b[i])
                                   for h in range(2)])
                    else:
                        v = _dot_nt(_upk(ds_s[lo + n, _W_SUM[i]]), b[i])
                    y = v if y is None else y + v
                p[i] = y if p[i] is None else p[i] + y
                anchors.append(p[i][:8])
                if fine:
                    anchors.append(p[i][D3 // 2:D3 // 2 + 8])
            return p

        def finish(blk, acc):
            y = [cat1(*_column(acc, [acc[_DIAG[s, j]] if (s, j) in _DIAG else None
                                     for s in range(3)], j)) for j in range(3)]
            xio_s[blk] = (xmid_s[blk] + 0.5 * cat0(*y)).astype(BF16)

        def load_acc(k):
            return [acc_s[k, i] for i in range(15)]

        def store_acc(k, acc):
            for i in range(15):
                acc_s[k, i] = acc[i]

        def load_b(k=0):
            return [_upk(b_s[i * TH // 2:(i + 1) * TH // 2, :])
                    for i in range(15 * k, 15 * k + 15)]

        def store_b(b, k=0):
            for i in range(15):
                b_s[(15 * k + i) * TH // 2:(15 * k + i + 1) * TH // 2, :] = _pk(b[i])

        def pre_phase():
            first = [[x_cp(0, 0)], [wq_cp(0)], [x_cp(1, 2), wq_cp(1)],
                     [wq_cp(2), pltpu.make_async_copy(wo_hbm, wo_v, sem_i.at[3])]]
            order = sum(first, [])
            for p in range(NP + 1):
                order += group_cp(p)
            xr_cp = [x_cp(b, SEM_P + NP + 1) for b in range(2, NB)]
            order += xr_cp
            for cp in order:
                cp.start()
            get = lambda an, name: [an[min(i, len(an) - 1)] for i in cfg[name]]
            e_grp = lambda e: ((e >> 1) & 1, ((e >> 2) << 1) | (e & 1))
            if 'a' in cfg['sub']:
                pre_a(first, get, e_grp)
            if 'b' in cfg['sub']:
                pre_b(get, e_grp)
            if 'c' in cfg['sub']:
                pre_c(get)
            wait('WX', xr_cp)

        def pre_a(first, get, e_grp):
            def transpose_wq(i):
                wt_s[WQ[i] // 2:WQ[i + 1] // 2, :D] = _pk(wqkv_v[:, WQ[i]:WQ[i + 1]].T)

            qkv_s[0] = jnp.zeros(qkv_s.shape[1:], U32)
            acc_s[...] = jnp.zeros(acc_s.shape, F32)
            wait('WX0', first[0])
            xn0 = ln1(0, ()).astype(BF16)

            wait('WQ0', first[1])
            transpose_wq(0)
            qkv_mm(0, xn0, (0, 1), [])

            wait('WQ1', first[2])
            transpose_wq(1)
            an = []
            qkv_mm(0, xn0, (2, 3), an)
            xn1 = ln1(1, get(an, 'a_ln'), get(an, 'a_lnb')).astype(BF16)
            qkv_mm(1, xn1, (0,), an, True)
            for n, a in enumerate(get(an, 'a_w1')):
                prep_att(n, a)
            nk = len(cfg['a_k'])
            apply = [att_values(0, *e_grp(e), a, 9) for e, a in enumerate(get(an, 'a_k'))]

            wait('WQ2', first[3])
            an = []
            qkv_mm(1, xn1, (2,), an)
            transpose_wq(2)
            qkv_mm(0, xn0, (4, 5), an)
            qkv_mm(1, xn1, (4, 1), an)
            apply += [att_values(0, *e_grp(nk + e), a, 9)
                      for e, a in enumerate(get(an, 'a_k2')[:8 - nk])]
            for e, a in enumerate(get(an, 'a_v')):
                apply[e](a)
            wo = pltpu.bitcast(wo_v[...], U32)
            wo = cat0(_lo(wo), _hi(wo))
            wo = cat0(*[_tie(wo[n * LANES:(n + 1) * LANES], a)
                        for n, a in enumerate(get(an, 'a_wo'))])
            wt_s[3 * RP:, :D] = _pk(wo.astype(BF16).T)
            stats = wo_mm(0, an, False)
            qkv_mm(1, xn1, (3,), an)
            for n, a in enumerate(get(an, 'a_w2')):
                prep_att(12 + n, a)
            plain_lhs(0, stats)
            n1 = len(cfg['a_att'])
            for e, a in enumerate(get(an, 'a_att')):
                att_group(1, *e_grp(e), a, 9)

            wait('WO', group_cp(0))
            an = []
            b = plain_piece(0, an)
            qkv_mm(1, xn1, (5,), an, True)
            prep_gu(0, get(an, 'z_g'))
            ffn_lhs(0, stats, get(an, 'z_l'))
            for e, a in enumerate(get(an, 'z_att')[:3 - n1]):
                att_group(1, *e_grp(n1 + e), a, 9)
            store_b(b)

        def pre_b(get, e_grp):
            def piece(p, carry):
                wait('WP', group_cp(p))
                b_prev = load_b()
                an = []
                if cfg['fast0']:
                    acc = down_mm(load_acc(0), [b_prev], p - 1, an, D_ORDER[:6], True)
                    t, hv, done = {}, {}, set()
                    for step in cfg['order1']:
                        k = int(step[1])
                        part = k if step[0] == 'S' else 3
                        slabs = [int(step[2])] if len(step) > 2 else list(range(NS))
                        if part not in done:
                            prep_gu(p, get(an, 'f_g%d' % part), _PARTS[part])
                            done.add(part)
                        if step[0] == 'S':
                            for i in _PARTS[k]:
                                gu_prod(p, i, t, an, slabs)
                        else:
                            gu_col(t, hv, p, k, an, slabs)
                    b = h_join(hv)
                    prep_d(p - 1, get(an, 'p_d'))
                    store_acc(0, down_mm(acc, [b_prev], p - 1, an, D_ORDER[6:]))
                else:
                    b = plain_piece(p, an)
                    prep_d(p - 1, get(an, 'p_d'))
                    store_acc(0, down_mm(load_acc(0), [b_prev], p - 1, an))
                    prep_gu(p, get(an, 'p_g'))
                att_group(1, *e_grp(p + 2), an[cfg['p_att'][0]], 9)
                for i, a in enumerate(get(an, 'p_w')):
                    prep_att(jnp.minimum(24 + (p - 1) * 5 + i, 47), a)
                store_b(b)
                return carry

            lax.fori_loop(1, NP, piece, 0)

        def pre_c(get):
            wait('WD', group_cp(NP))
            an = []
            stats = wo_mm(1, an, True)
            prep_d(NP - 1, get(an, 't_d'))
            acc = down_mm(load_acc(0), [load_b()], NP - 1, [])
            ffn_lhs(1, stats, [])
            finish(0, acc)

        if 'pre' in cfg['phases']:
            pre_phase()

        def body(u, carry):
            bu = u & (NB - 1)
            ba = (u + 1) & (NB - 1)
            acc, stats, an, b = None, None, {}, {}
            get = lambda name: [an[k][i] for k, i in cfg[name]]
            for step in cfg['body']:
                an[step] = []
                if step == 'Q':
                    qkv_fast(ba, att_rhs(ln1(ba, get('ln1'), get('ln1b')), u >> 8 if 'q' in cfg['stash'] else None),
                             an[step])
                elif step == 'W':
                    attention(ba, get('att'), cfg['win'])
                    stats = wo_mm(ba, an[step], True, get('orhs'),
                                  u >> 8 if 'w' in cfg['stash'] else None)
                elif step == 'L':
                    ffn_lhs(ba, stats, get('lhs'))
                elif step[0] == 'S':
                    slabs = [int(step[3])] if len(step) > 3 else list(range(NS))
                    for i in _PARTS[int(step[2])]:
                        gu_prod(int(step[1]), i, b.setdefault(step[:2], {}), an[step], slabs)
                elif step[0] == 'F':
                    j, c = int(step[1]), int(step[2])
                    slabs = [int(step[3])] if len(step) > 3 else list(range(NS))
                    hv = b.setdefault(step[:2], {})
                    gu_col(b['S' + step[1]], hv, j, c, an[step], slabs)
                    if len(hv) == 3 * NS:
                        b[j] = h_join(hv)
                        if 'b' in cfg['stash']:
                            store_b(b[j], j)
                            b[j] = load_b(j)
                else:
                    js = [int(c) for c in step[1:]]
                    acc = down_mm(acc, [b[j] for j in js], js[0], an[step])
            finish(bu, acc)

            @pl.when(u >= NB)
            def _():
                out_copy(bu).start()
            return carry

        if scopes:
            with jax.named_scope('LOOP'):
                lax.fori_loop(1, NU - 1, body, 0)
        elif 'main' in cfg['phases']:
            lax.fori_loop(1, NU - 1, body, 0)

        def last(c, carry):
            los = [2 * c + j for j in range(2)]
            b = [gu_piece(lo, cfg['order'], [], j) for j, lo in enumerate(los)]
            acc = load_acc(1)
            for j in range(2):
                acc = down_mm(acc, [b[j]], los[j], [])
            store_acc(1, acc)
            return carry

        if 'last' in cfg['phases']:
            lax.fori_loop(0, NP // 2, last, 0)
        if len(cfg['phases']) < 3:
            def keep(i, c):
                v = (gs_s[i, i, :8, :LANES] + us_s[i, i, :8, :LANES] + ds_s[i, i, :8, :LANES]
                     + wl_s[rows8(i * 8), :LANES] + a_s[i, :8] + qkv_s[i, :8]
                     + b_s[rows8(i * 8), :LANES] + wt_s[rows8(i * 8), :LANES])
                acc_s[1, 0, :8] = (lax.bitcast_convert_type(v, F32) + o_s[i, :8]
                                   + acc_s[i, i, :8])
                return c
            lax.fori_loop(0, 2, keep, 0)
        finish(NB - 1, load_acc(1))
        out_copy(NB - 1).start()
        wait('WOUT', [out_copy(b) for b in range(NB)])

    scratch = [
        pltpu.VMEM((NB, D, TM), BF16),
        pltpu.VMEM((D, 3 * D), BF16),
        pltpu.VMEM((D, D), BF16),
        pltpu.VMEM((NP, 3, D, PW), BF16),
        pltpu.VMEM((NP, 3, D, PW), BF16),
        pltpu.VMEM((NP, 3, D, PW), BF16),
        pltpu.VMEM((2 * D, 8 * LANES), U32),
        pltpu.VMEM((4 * Q3, 16 * LANES), U32),
        pltpu.VMEM((NP, 15, Q3, PW), U32),
        pltpu.VMEM((NP, 15, Q3, PW), U32),
        pltpu.VMEM((NP, 9, Q3, PW), U32),
        pltpu.VMEM((NB, D, TM), F32),
        pltpu.VMEM((54, TH // 2, LANES), U32),
        pltpu.VMEM((S // LANES + 1, 3 * RP, LANES), U32),
        pltpu.VMEM((NT, D, LANES), F32),
        pltpu.VMEM((2, 15, D3, TH), F32),
        pltpu.VMEM((NP * 15 * TH // 2, PW), U32),
        pltpu.VMEM((1, 9 * 64, 2 * LANES), U32),
        pltpu.VMEM((NP, 2, 9, TH, PW), F32),
        pltpu.SemaphoreType.DMA((SEM_P + NP + 2,)),
        pltpu.SemaphoreType.DMA((1,)),
    ]
    return kernel, scratch


_CFG = dict(
    scopes=False,
    fast0=True,
    psplit=1,
    rcp=False,
    late=True,
    stash='qw',
    slab=True,
    fslab=False,
    win=9,
    sub='abc',
    orhs=(),
    msplit=2,
    phases=('pre', 'main', 'last'),
    order=('S0', 'S1', 'F0', 'S2', 'F1', 'F2'),
    body=('S010', 'S000', 'F000', 'S020', 'F010', 'F020', 'S001', 'S011', 'F001',
        'S110', 'S021', 'F021', 'S100', 'F100', 'S120', 'S101', 'F110', 'F011', 'Q',
        'F120', 'S111', 'F101', 'S121', 'F111', 'F121', 'S200', 'S210', 'F200', 'S220',
        'F210', 'F220', 'S300', 'S201', 'S211', 'F201', 'S320', 'S221', 'F211', 'F221',
        'S310', 'D01', 'F300', 'S301', 'S311', 'F301', 'S321', 'F311', 'F321', 'S400',
        'F310', 'F320', 'S420', 'F410', 'S410', 'S401', 'F420', 'S411', 'F400', 'S421',
        'F411', 'F421', 'S500', 'F401', 'S501', 'S510', 'D23', 'F500', 'S520', 'W',
        'F520', 'S511', 'F510', 'S521', 'F501', 'F511', 'F521', 'D4', 'D5', 'L'),
    ln1=(('S010', 4), ('S010', 5), ('S010', 6), ('S010', 7), ('S010', 8), ('S000', 0),
        ('S000', 1), ('S000', 2), ('S000', 3)),
    ln1b=(('S110', 2), ('S110', 3), ('S110', 5), ('S110', 6), ('S110', 8), ('S021', 0),
        ('S021', 2), ('S021', 3), ('S021', 5), ('S021', 6), ('S021', 8), ('F021', 0)),
    att=(('S300', 8), ('D01', 1), ('D01', 7), ('D01', 8), ('D01', 10), ('F300', 4),
        ('D23', 5), ('D23', 9)),
    lhs=(('D4', 3), ('D5', 1), ('D5', 4)),
    att0=(15, 18, 21, 24, 27, 30, 33, 37),
    order0=('S0', 'S1', 'S2', 'F0', 'F1', 'F2'),
    order1=('S0', 'S1', 'S2', 'F0', 'F1', 'F2'),
    a_w1=(0, 0, 1, 2, 2, 3, 3, 4, 4, 5, 6, 7),
    a_w2=(20, 23, 26, 30, 33, 36, 40, 43, 46, 50, 53, 57),
    a_ln=(0, 3, 6),
    a_lnb=(5, 9, 9),
    z_g=(5, 6, 7, 8, 11, 11, 12, 13, 14, 15, 17, 18, 19, 20, 21, 22, 23, 24, 25, 26, 28,
        29, 30, 31, 32, 35, 36, 37, 38, 40, 41, 42, 43, 45, 46, 47, 48, 49, 50, 51, 52,
        54, 55, 57, 58, 59, 60, 62),
    z_att=(53, 54, 56),
    p_g0=(0, 1, 2, 3, 4, 5),
    p_g1=(6, 7, 8, 9, 10, 10),
    p_g2=(12, 13, 14, 15, 16, 17),
    p_g3=(14, 16, 18, 20, 22, 24, 26, 28, 30, 32, 34, 36),
    t_d=(0, 0, 1, 1, 2, 3, 3, 4, 5, 6, 6, 7, 8, 9, 9, 9, 10, 11, 11, 12, 13, 14, 15,
        16),
    p_d=(32, 33, 35, 35, 35, 37, 37, 38, 39, 41, 42, 43, 44, 45, 45, 46, 47, 48, 49, 51,
        52, 53, 54, 56),
    p_att=(60,),
    p_w=(12, 60, 63, 65, 65),
    p_g=(0, 1, 2, 3, 4, 5, 6, 7, 9, 10, 11, 12, 13, 14, 15, 16, 18, 19, 20, 21, 22, 23,
        24, 25, 27, 28, 29, 30, 31, 32, 33, 34, 36, 37, 38, 39, 40, 41, 42, 43, 45, 46,
        47, 48, 49, 50, 51, 53),
    z_l=(2, 13, 32),
    f_g0=(0, 0, 0, 1, 1, 2, 3, 3, 4, 4, 5, 5),
    f_g1=(4, 5, 5, 7, 8, 9, 9, 10, 11, 12, 13, 15),
    f_g2=(1, 12, 12, 15, 15, 16, 17, 18, 19, 20, 20, 24),
    f_g3=(4, 14, 16, 17, 18, 19, 21, 22, 23, 23, 24, 25, 26, 27, 28, 29, 30, 31, 32, 33,
        34, 35, 36, 37),
    a_k=(15, 19, 20, 24),
    a_k2=(0, 4, 8, 12),
    a_v=(13, 14, 22, 26, 30, 34, 38, 39),
    a_att=(12, 60),
    a_wo=(30, 35, 36, 38, 41),
)


def _run(A_x, A_wqkv, A_wo, B_w_gate, B_w_up, B_w_down, **kw):
    _, S, D = A_x.shape
    F = B_w_gate.shape[1]
    kernel, scratch = _make_kernel(S, D, F, 256, {**_CFG, **kw})
    hbm = pl.BlockSpec(memory_space=pl.ANY)
    out_t = pl.pallas_call(
        kernel,
        in_specs=[hbm] * 6,
        out_specs=hbm,
        out_shape=jax.ShapeDtypeStruct((D, S), A_x.dtype),
        scratch_shapes=scratch,
        compiler_params=pltpu.CompilerParams(vmem_limit_bytes=110 * 1024 * 1024),
    )(A_x.reshape(S, D).T, A_wqkv, A_wo, B_w_gate, B_w_up, B_w_down.T)
    return out_t.T.reshape(A_x.shape)


@jax.jit
def pallas_interleave_layers__sliding_local_dilated__glu_gated_geglu__prompt_kernel(
    A_x: jax.Array,
    A_wqkv: jax.Array,
    A_wo: jax.Array,
    B_x: jax.Array,
    B_w_gate: jax.Array,
    B_w_up: jax.Array,
    B_w_down: jax.Array,
):
    del B_x
    return _run(A_x, A_wqkv, A_wo, B_w_gate, B_w_up, B_w_down)
```

```python
import functools

import jax
import jax.numpy as jnp
import jax.experimental.pallas as pl
import jax.experimental.pallas.tpu as pltpu
from jax import lax

H = 32
W = 8
DIL = 2
EPS = 1e-5
LANES = 128

F32 = jnp.float32
BF16 = jnp.bfloat16
U32 = jnp.uint32

_NT = (((1,), (1,)), ((), ()))


def _tree_sum(parts, op=jnp.add):
    while len(parts) > 1:
        nxt = [op(parts[i], parts[i + 1]) for i in range(0, len(parts) - 1, 2)]
        if len(parts) % 2:
            nxt.append(parts[-1])
        parts = nxt
    return parts[0]


def _ln_stats(slabs, d, anchors=()):
    n_acc = 4
    s1, s2, pilot = [None] * n_acc, [None] * n_acc, None
    for i, x in enumerate(slabs):
        if pilot is None:
            pilot = x[0:1, :]
            pil = jnp.broadcast_to(pilot, x.shape)
            pils = [_tie(pil, a) for a in anchors] or [pil]
        dx = x - pils[i * len(pils) // (d // 8)]
        j = i % n_acc
        s1[j] = dx if s1[j] is None else s1[j] + dx
        s2[j] = dx * dx if s2[j] is None else s2[j] + dx * dx
    e1 = jnp.sum(_tree_sum(s1), axis=0, keepdims=True) * (1.0 / d)
    e2 = jnp.sum(_tree_sum(s2), axis=0, keepdims=True) * (1.0 / d)
    var = jnp.maximum(e2 - e1 * e1, 0.0)
    return pilot + e1, lax.rsqrt(var + EPS)


def _zero_like_dep(v):
    return (lax.bitcast_convert_type(v, U32) >> 31) >> 1


def _tie(x, anchor):
    if anchor is None:
        return x
    z = lax.bitcast_convert_type(_zero_like_dep(anchor), F32)
    z = jnp.concatenate([z] * -(-x.shape[1] // LANES), axis=1)[:, :x.shape[1]]
    if x.shape[0] == 8:
        return x + z
    return jnp.concatenate([x[:8] + z, x[8:]], axis=0)


def _gelu_mul2(g, u):
    c0 = 0.7978845608028654
    c1 = c0 * 0.044715
    t = jnp.tanh(g * (c0 + c1 * (g * g)))
    return (g * u) * (1.0 + t)


def _lo(x):
    return lax.bitcast_convert_type(x << 16, F32)


def _hi(x):
    return lax.bitcast_convert_type(x & jnp.uint32(0xFFFF0000), F32)


def _pk(x):
    return pltpu.bitcast(x.astype(BF16), U32)


def _upk(x):
    return pltpu.bitcast(x, BF16)


def _dot(a, b):
    return jnp.dot(a, b, preferred_element_type=F32)


def _dot_nt(a, b):
    return lax.dot_general(a, b, _NT, preferred_element_type=F32)


def _x_ops(x1, x2):
    d = [a - b for a, b in zip(x1, x2)]
    return [x1[0] + x2[1], x2[0] + x2[1], x1[0] + x1[1],
            d[1] + x1[2], x1[1] + x1[2], d[1] + d[2],
            d[0] - x2[2], d[0] + d[2], x2[0] + x2[2],
            x1[0], d[0], x2[1], d[1], x1[2], x2[2]]


def _x_rem(x1, x2):
    a, b, c = 0, 1, 2
    cat = lambda u, v: jnp.concatenate([u, v], axis=0)
    return [cat(x1[c], x2[b]), cat(x1[a], x1[b] - x2[b]), cat(x2[a], x2[c] - x1[c])]


def _w_sums(w):
    return [w[0][1] + w[1][0], w[1][2] + w[2][1], w[0][2] + w[2][0],
            w[0][0] + w[0][2] - w[1][0], w[2][0] - w[0][0] - w[0][1],
            w[1][1] + w[1][2] - w[0][1], w[1][0] + w[1][1] - w[2][1],
            w[2][0] + w[2][2] - w[1][2], w[2][1] + w[2][2] - w[0][2]]


_W_TERMS = {0: ((0, 1, 1), (1, 0, 1)), 3: ((1, 2, 1), (2, 1, 1)), 6: ((0, 2, 1), (2, 0, 1)),
            9: ((0, 0, 1), (0, 2, 1), (1, 0, -1)), 10: ((2, 0, 1), (0, 0, -1), (0, 1, -1)),
            11: ((1, 1, 1), (1, 2, 1), (0, 1, -1)), 12: ((1, 0, 1), (1, 1, 1), (2, 1, -1)),
            13: ((2, 0, 1), (2, 2, 1), (1, 2, -1)), 14: ((2, 1, 1), (2, 2, 1), (0, 2, -1)),
            1: ((0, 1, 1),), 2: ((1, 0, 1),), 4: ((1, 2, 1),), 5: ((2, 1, 1),),
            7: ((2, 0, 1),), 8: ((0, 2, 1),)}
_PARTS = ((1, 2, 0), (7, 8, 6), (4, 5, 3), (9, 10, 11, 12, 13, 14))
_W_SUM = {0: 0, 3: 1, 6: 2, 9: 3, 10: 4, 11: 5, 12: 6, 13: 7, 14: 8}
_W_RAW = {1: (0, 1), 2: (1, 0), 4: (1, 2), 5: (2, 1), 7: (2, 0), 8: (0, 2)}
_PAIR_ORDER = (1, 2, 4, 5, 7, 8, 0, 3, 6)
_DIAG = {(0, 0): 9, (2, 0): 10, (0, 1): 11, (1, 1): 12, (1, 2): 13, (2, 2): 14}
_PAIR = {(0, 0): ((6, -1), (8, -1)), (1, 0): ((2, 1), (7, 1)), (2, 0): ((0, 1), (1, -1)),
         (0, 1): ((3, 1), (4, -1)), (1, 1): ((0, 1), (2, -1)), (2, 1): ((1, 1), (5, -1)),
         (0, 2): ((4, 1), (8, 1)), (1, 2): ((6, 1), (7, -1)), (2, 2): ((5, 1), (3, -1))}


def _column(t, base, j):
    s = []
    for k in range(3):
        v = base[k]
        for i, sg in _PAIR[k, j]:
            ti = t[i]() if callable(t[i]) else t[i]
            v = ti if v is None else (v + ti if sg > 0 else v - ti)
        s.append(v)
    return s[1] + s[0], s[2] + s[0]


def _make_kernel(S, D, F, TM, cfg):
    NB = S // TM
    NT = TM // LANES
    DH = D // H
    DP = DH // 2
    RP = D // 2
    NG = H // 8
    scale = float(DH) ** -0.5
    NU = 2 * NB
    TH = TM // 2
    FT = F // 3
    D2 = D // 2
    D3 = D // 3
    Q3 = D3 // 2
    KU = D // 9
    KR = 3 * LANES
    NQ = 6
    QR = 3 * D // NQ
    WQ = (0, 640, 1152, 3 * D)
    PW = 256
    NP = FT // PW
    scopes = cfg['scopes']
    assert NG == 4 and NB & (NB - 1) == 0
    SEM_P = 4

    def kernel(x_hbm, wqkv_hbm, wo_hbm, wg_hbm, wu_hbm, wdt_hbm, out_hbm,
               xio_s, wqkv_v, wo_v, wg_v, wu_v, wdt_v, wt_s, wl_s,
               gs_s, us_s, ds_s, xmid_s, a_s, qkv_s, o_s, acc_s, b_s, r_s, t_s,
               sem_i, sem_o):

        def wait(name, cps):
            if scopes:
                with jax.named_scope(name):
                    for cp in cps:
                        cp.wait()
            else:
                for cp in cps:
                    cp.wait()

        def cols(lo, n):
            if not isinstance(lo, int):
                lo = pl.multiple_of(lo, LANES)
            return pl.ds(lo, n)

        def rows8(lo, n=8):
            if not isinstance(lo, int):
                lo = pl.multiple_of(lo, 8)
            return pl.ds(lo, n)

        def out_copy(b):
            return pltpu.make_async_copy(
                xio_s.at[b], out_hbm.at[:, cols(b * TM, TM)], sem_o.at[0])

        def x_cp(b, sem):
            return pltpu.make_async_copy(x_hbm.at[:, cols(b * TM, TM)], xio_s.at[b],
                                         sem_i.at[sem])

        def wq_cp(i):
            sl = cols(WQ[i], WQ[i + 1] - WQ[i])
            return pltpu.make_async_copy(wqkv_hbm.at[:, sl], wqkv_v.at[:, sl],
                                         sem_i.at[1 + i])

        def piece_cp(src, dst, p, sem):
            return [pltpu.make_async_copy(src.at[:, cols(j * FT + p * PW, PW)],
                                          dst.at[p, j],
                                          sem_i.at[sem]) for j in range(3)]

        def group_cp(p):
            sem = SEM_P + p
            cps = []
            if not (isinstance(p, int) and p == NP):
                cps += piece_cp(wg_hbm, wg_v, p, sem) + piece_cp(wu_hbm, wu_v, p, sem)
            if not (isinstance(p, int) and p == 0):
                cps += piece_cp(wdt_hbm, wdt_v, p - 1, sem)
            return cps

        lane = lax.broadcasted_iota(jnp.int32, (8, LANES), 1)
        cat0 = lambda *v: jnp.concatenate(v, axis=0)
        cat1 = lambda *v: jnp.concatenate(v, axis=1)

        def spread_over(anchors, n, total):
            return anchors[n * len(anchors) // total] if anchors else None

        def slab_group(r):
            return (r % LANES) // 16 if r < KR else 8 + ((r - KR) % KU) // 16

        def ln1(blk, anchors1, anchors2=()):
            slabs = (xio_s[blk, r:r + 8, :].astype(F32) for r in range(0, D, 8))
            m, rs = _ln_stats(slabs, D, anchors1)
            if not anchors2:
                return (xio_s[blk].astype(F32) - m) * rs
            m8 = jnp.broadcast_to(m, (8, TM))
            ms = [_tie(m8, a) for a in anchors2]
            ms = [spread_over(ms, slab_group(r), 12) for r in range(0, D, 8)]
            return (xio_s[blk].astype(F32) - cat0(*ms)) * rs

        def dot_k(rows, x, anchors, even=False):
            y = None
            for n, k in enumerate(range(0, D, LANES)):
                ks = slice(k, min(k + LANES, D))
                if even and k + LANES >= D:
                    mid = (rows.start + rows.stop) // 2
                    v = cat0(_dot(_upk(wt_s[rows.start:mid, ks]), x[ks]),
                             _dot(_upk(wt_s[mid:rows.stop, ks]), x[ks]))
                else:
                    v = _dot(_upk(wt_s[rows, ks]), x[ks])
                anchors.extend(v[r:r + 8, :LANES] for r in ((0, 144) if n % 2 else (72, 216)))
                y = v if y is None else y + v
            return y

        def put_qkv(blk, rows, y):
            pk = _pk(y)
            for c in range(NT):
                qkv_s[1 + blk * NT + c, rows, :] = pk[:, c * LANES:(c + 1) * LANES]

        def qkv_mm(blk, xn, chunks, anchors, even=False):
            for r in chunks:
                rows = slice(r * QR // 2, (r + 1) * QR // 2)
                put_qkv(blk, rows, dot_k(rows, xn, anchors, even))

        def split_k(x):
            hs = (x[:, :TH], x[:, TH:])
            blocks = [[h[k * LANES:(k + 1) * LANES] for k in range(3)] for h in hs]
            units = [[h[KR + k * KU:KR + (k + 1) * KU] for k in range(3)] for h in hs]
            return blocks, units

        def prep_att(pat, anchor):
            assert Q3 == 96
            row0 = pat * 8
            src0 = row0 + ((pat * 43) >> 9) * (2 * Q3)
            w = [_upk(wt_s[rows8(src0 + j * Q3), :D]).astype(F32) for j in range(3)]
            w[0] = cat1(_tie(w[0][:, :LANES], anchor), w[0][:, LANES:])
            tiles = _w_sums([[w[j][:, k * LANES:(k + 1) * LANES] for j in range(3)]
                             for k in range(3)])
            for j in range(3):
                a, b, c = (w[j][:, KR + k * KU:KR + (k + 1) * KU] for k in range(3))
                tiles += [cat1(c, b), cat1(a, c)]
            wl_s[rows8(row0), :15 * LANES] = _pk(cat1(*tiles))

        def att_rhs(x, stash=None):
            blocks, units = split_k(x)
            ops = _x_ops(*blocks) + _x_rem(*units)
            if stash is None:
                return [v.astype(BF16) for v in ops]
            loc = lambda i, r0, n: (slice((i // 2) * 64 + r0, (i // 2) * 64 + r0 + n),
                                    slice((i % 2) * LANES, (i % 2 + 1) * LANES))
            for r in range(0, LANES, 16):
                for i, v in enumerate(ops):
                    r_s.at[0][loc(i, r // 2, 8)] = _pk(v[r:r + 16])
            return [_upk(r_s.at[stash][loc(i, 0, 64)]) for i in range(18)]

        def att_mm(sec, rhs, anchors):
            tl = lambda i: _upk(wl_s[sec * Q3:(sec + 1) * Q3, i * LANES:(i + 1) * LANES])
            raw = lambda k, j: _upk(wt_s[(3 * sec + j) * Q3:(3 * sec + j + 1) * Q3,
                                         k * LANES:(k + 1) * LANES])
            t = {}
            for i in _PAIR_ORDER:
                t[i] = _dot(raw(*_W_RAW[i]) if i in _W_RAW else tl(_W_SUM[i]), rhs[i])
                anchors.append(t[i][:8])
            out = []
            for j in range(3):
                base = []
                for s in range(3):
                    v = _dot(raw(3, j) if s == 1 else tl(9 + 2 * j + s // 2), rhs[15 + s])
                    if (s, j) in _DIAG:
                        i = _DIAG[s, j]
                        v = _dot(tl(_W_SUM[i]), rhs[i]) + v
                    base.append(v)
                    anchors.append(base[-1][:8])
                out.append(cat1(*_column(t, base, j)))
            return cat0(*out)

        def qkv_fast(blk, rhs, anchors):
            for sec in range(3):
                put_qkv(blk, slice(sec * RP, (sec + 1) * RP), att_mm(sec, rhs, anchors))

        def shifted(ln, cur, prev, w):
            if w == 0:
                return cur
            sh = DIL * w
            return pltpu.roll(jnp.where(ln < LANES - sh, cur, prev), sh, axis=1)

        def att_group(blk, c, hg, anchor, win):
            att_values(blk, c, hg, anchor, win)(None)

        def att_values(blk, c, hg, anchor, win):
            tile = blk * NT + c
            base = hg * 8 * DP
            if isinstance(hg, int):
                cur, prev, o_t = qkv_s.at[1 + tile], qkv_s.at[tile], o_s.at[c]
            else:
                n = 2 * RP + 8 * DP
                base = pl.multiple_of(base, 8)
                cur = qkv_s.at[1 + tile, pl.ds(base, n)]
                prev = qkv_s.at[tile, pl.ds(base, n)]
                o_t = o_s.at[c, pl.ds(base, RP + 8 * DP)]
                base = 0
            ln = lane + _zero_like_dep(anchor).astype(jnp.int32)
            logits = [None] * W
            done = []
            for dd in range(DP):
                q = cur[pl.ds(base + dd, 8, stride=DP), :]
                kc = cur[pl.ds(RP + base + dd, 8, stride=DP), :]
                if dd >= win:
                    kc = kc | _zero_like_dep(done[dd - win])
                kp = prev[pl.ds(RP + base + dd, 8, stride=DP), :]
                q0, q1 = _lo(q), _hi(q)
                for w in range(W):
                    ks = shifted(ln, kc, kp, w)
                    t = q0 * _lo(ks) + q1 * _hi(ks)
                    logits[w] = t if logits[w] is None else logits[w] + t
                done.append(ks)
            logits = [l * scale for l in logits]
            if not (isinstance(c, int) and c > 0):
                pos = lane + tile * LANES
                logits = [l if w == 0 else jnp.where(pos >= DIL * w, l, -1e9)
                          for w, l in enumerate(logits)]
            m = _tree_sum(logits, jnp.maximum)
            e = [jnp.exp(l - m) for l in logits]
            den = _tree_sum(e)
            if cfg['rcp']:
                r = pl.reciprocal(den, approx=True)
                r = r * (2.0 - den * r)
            else:
                r = 1.0 / den
            p = e if cfg['late'] else [x * r for x in e]

            def apply(anchor2):
                ln = lane + _zero_like_dep(m if anchor2 is None else anchor2).astype(jnp.int32)
                done = []
                for dd in range(DP):
                    vc = cur[pl.ds(2 * RP + base + dd, 8, stride=DP), :]
                    if dd >= win:
                        vc = vc | _zero_like_dep(done[dd - win])
                    vp = prev[pl.ds(2 * RP + base + dd, 8, stride=DP), :]
                    o0 = o1 = None
                    for w in range(W):
                        vs = shifted(ln, vc, vp, w)
                        t0, t1 = p[w] * _lo(vs), p[w] * _hi(vs)
                        o0 = t0 if o0 is None else o0 + t0
                        o1 = t1 if o1 is None else o1 + t1
                    done.append(vs)
                    if cfg['late']:
                        o0, o1 = o0 * r, o1 * r
                    o_t[pl.ds(base + dd, 8, stride=DP), :] = o0
                    o_t[pl.ds(RP + base + dd, 8, stride=DP), :] = o1

            return apply

        def attention(blk, anchors, win):
            for c in range(NT):
                for hg in range(NG):
                    att_group(blk, c, hg, anchors[c * NG + hg], win)

        def wo_mm(blk, anchors, fast, anchors_in=(), stash=None):
            o = cat1(*[o_s[c] for c in range(NT)])
            if anchors_in:
                o = cat0(*[_tie(o[r:r + 8], spread_over(anchors_in, slab_group(r), 12))
                           for r in range(0, D, 8)])
            if fast:
                y = att_mm(3, att_rhs(o, stash), anchors)
            else:
                o = o.astype(BF16)
                q = D2 // 2
                y = cat0(*[dot_k(slice(h * q, (h + 1) * q), o, anchors) for h in (6, 7)])
            xm = xio_s[blk].astype(F32) + y
            xmid_s[blk] = xm
            return _ln_stats((xm[r:r + 8] for r in range(0, D, 8)), D)

        def ffn_lhs(blk, stats, anchors):
            m, rs = stats
            m8 = jnp.broadcast_to(m, (8, TM))
            xs = []
            for k in range(3):
                mt = cat0(*[_tie(m8, spread_over(anchors, k, 3))] * (D3 // 8))
                xs.append((xmid_s[blk, k * D3:(k + 1) * D3, :] - mt) * rs)
            ops = _x_ops([x[:, :TH] for x in xs], [x[:, TH:] for x in xs])
            for i, v in enumerate(ops):
                for s, t in enumerate((v[KU:], v[:2 * KU], cat0(v[:KU], v[2 * KU:]))):
                    a_s[3 * i + s] = _pk(t.astype(BF16).T)

        def plain_lhs(blk, stats):
            m, rs = stats
            blocks, units = split_k((xmid_s[blk] - m) * rs)
            for i, v in enumerate(blocks[0] + blocks[1] + _x_rem(*units)):
                a_s[45 + i] = _pk(v.astype(BF16).T)

        def plain_piece(p, anchors):
            h = {}
            for j in range(3):
                hs = []
                for n in range(PW // LANES):
                    cs = slice(n * LANES, (n + 1) * LANES)
                    w = lambda r0, r1: cat1(wg_v[p, j, r0:r1, cs], wu_v[p, j, r0:r1, cs])
                    u = lambda k: w(KR + k * KU, KR + (k + 1) * KU)
                    ps = cfg['psplit']
                    q = TH // 2 // ps
                    hh = []
                    for s in range(ps):
                        tl = lambda *i: _upk(cat1(*[a_s[45 + k, s * q:(s + 1) * q] for k in i]))
                        y0 = _dot(tl(6), cat0(u(2), u(1)))
                        y1 = _dot(tl(0, 1, 2, 7), w(0, KR + 2 * KU))
                        y2 = _dot(tl(3, 4, 5, 8), cat0(w(0, KR + KU), u(2)))
                        if s == 0:
                            anchors.append(y0[:8, :LANES])
                        for y in (y1, y2):
                            anchors.extend(y[r:r + 8, c:c + LANES] for c in (0, LANES)
                                           for r in range(0, 2 * q, TH // 2))
                        hh.append([_gelu_mul2(*[(y + y0)[:, c:c + LANES] for c in (0, LANES)])
                                   for y in (y1, y2)])
                    hs.append([cat0(*[v[i] for v in hh]) for i in range(2)])
                h[j] = [cat1(*[v[i] for v in hs]) for i in range(2)]
            return h_ops(h)

        def prep_d(p, anchors):
            PR = 16
            for n in range(2 * D3 // PR):
                r, cs = (n // 2) * PR, slice((n % 2) * LANES, (n % 2 + 1) * LANES)
                w = [[wdt_v[p, k, j * D3 + r:j * D3 + r + PR, cs].astype(F32)
                      for j in range(3)] for k in range(3)]
                w[0][1] = _tie(w[0][1], spread_over(anchors, n, 2 * D3 // PR))
                for i, v in enumerate(_w_sums(w)):
                    ds_s.at[p, i][r // 2:(r + PR) // 2, cs] = _pk(v)

        GU = ((wg_v, gs_s), (wu_v, us_s))

        def prep_gu(p, anchors, ids=tuple(range(15))):
            PR = 16
            nr = D3 // PR
            for n in range(4 * nr):
                c, (w_v, s_s), r = n % 2, GU[(n // 2) % 2], (n // 4) * PR
                cache = {}

                def w(k, j):
                    if (k, j) not in cache:
                        ld = lambda c: w_v[p, j, k * D3 + r:k * D3 + r + PR,
                                           c * LANES:(c + 1) * LANES].astype(F32)
                        v = ld(c)
                        if k != j:
                            v = _tie(v, spread_over(anchors, n, 4 * nr))
                        cache[k, j] = v - ld(1 - c) if r // KU == 1 + c else v
                    return cache[k, j]

                for i in ids:
                    v = None
                    for k, j, sg in _W_TERMS[i]:
                        v = w(k, j) if v is None else (v + w(k, j) if sg > 0 else v - w(k, j))
                    s_s.at[p, i][r // 2:(r + PR) // 2, c * LANES:(c + 1) * LANES] = _pk(v)

        NS = cfg['msplit']

        def gu_prod(p, i, t, anchors, slabs, slot=0):
            u = KU // 2

            def rhs(s, s_s):
                if s == 1:
                    return s_s[p, i, :2 * u, :LANES]
                if s == 0:
                    return cat0(s_s[p, i, u:2 * u, LANES:], s_s[p, i, 2 * u:, :LANES])
                return cat0(s_s[p, i, :u, LANES:], s_s[p, i, 2 * u:, LANES:])

            q = TH // 2 // NS
            for n, h in enumerate(slabs):
                y = []
                for s in range(3):
                    r = _upk(cat1(rhs(s, gs_s), rhs(s, us_s)))
                    y.append(_dot(_upk(a_s[3 * i + s, h * q:(h + 1) * q]), r))
                    if (3 * n + s) % len(slabs) == 0:
                        anchors.append(y[-1][:8, :LANES])
                y1, y2 = y[1] + y[0], y[2] + y[0]
                for m in range(2):
                    cs = slice(m * LANES, (m + 1) * LANES)
                    v = cat1(y1[:, cs], y2[:, cs])
                    if i < 9 and 't' in cfg['stash']:
                        k = p if isinstance(p, int) else slot
                        t_s[k, m, i, 2 * h * q:2 * (h + 1) * q] = v
                        v = lambda k=k, m=m, h=h: t_s[k, m, i, 2 * h * q:2 * (h + 1) * q]
                    t.setdefault((m, h), {})[i] = v

        def gu_col(t, hv, p, j, anchors, slabs):
            ids = [_DIAG.get((s, j)) for s in range(3)]
            if cfg['fslab']:
                for h in slabs:
                    for i in ids:
                        if i is not None:
                            gu_prod(p, i, t, anchors if h == slabs[0] else [], [h])
            else:
                for i in ids:
                    if i is not None:
                        gu_prod(p, i, t, anchors, slabs)
            for h in slabs:
                g, u = [_column(t[m, h], [None if i is None else t[m, h][i] for i in ids], j)
                        for m in range(2)]
                hv[j, h] = [_gelu_mul2(g[i], u[i]) for i in range(2)]

        def h_ops(h):
            return [v.astype(BF16) for v in _x_ops(*[[h[j][i] for j in range(3)]
                                                     for i in range(2)])]

        def h_join(hv):
            return h_ops({j: [cat0(*[hv[j, h][i] for h in range(NS)]) for i in range(2)]
                          for j in range(3)})

        def gu_piece(p, order, anchors, slot):
            t, hv = {}, {}
            for slabs in ([[h] for h in range(NS)] if cfg['slab'] else [list(range(NS))]):
                for step in order:
                    if step[0] == 'S':
                        for i in _PARTS[int(step[1])]:
                            gu_prod(p, i, t, anchors, slabs, slot)
                    else:
                        gu_col(t, hv, p, int(step[1]), anchors, slabs)
            return h_join(hv)

        D_ORDER = _PAIR_ORDER + (9, 10, 11, 12, 13, 14)

        def down_mm(acc, bs, lo, anchors, which=D_ORDER, fine=False):
            p = [None] * 15 if acc is None else list(acc)
            for i in which:
                y = None
                for n, b in enumerate(bs):
                    if i in _W_RAW:
                        k, j = _W_RAW[i]
                        v = _dot_nt(wdt_v[lo + n, k, j * D3:(j + 1) * D3, :], b[i])
                    elif len(bs) % 2 and i == 14 and n == 0:
                        v = cat0(*[_dot_nt(_upk(ds_s[lo, _W_SUM[i],
                                                     h * Q3 // 2:(h + 1) * Q3 // 2, :]), b[i])
                                   for h in range(2)])
                    else:
                        v = _dot_nt(_upk(ds_s[lo + n, _W_SUM[i]]), b[i])
                    y = v if y is None else y + v
                p[i] = y if p[i] is None else p[i] + y
                anchors.append(p[i][:8])
                if fine:
                    anchors.append(p[i][D3 // 2:D3 // 2 + 8])
            return p

        def finish(blk, acc):
            y = [cat1(*_column(acc, [acc[_DIAG[s, j]] if (s, j) in _DIAG else None
                                     for s in range(3)], j)) for j in range(3)]
            xio_s[blk] = (xmid_s[blk] + 0.5 * cat0(*y)).astype(BF16)

        def load_acc(k):
            return [acc_s[k, i] for i in range(15)]

        def store_acc(k, acc):
            for i in range(15):
                acc_s[k, i] = acc[i]

        def load_b(k=0):
            return [_upk(b_s[i * TH // 2:(i + 1) * TH // 2, :])
                    for i in range(15 * k, 15 * k + 15)]

        def store_b(b, k=0):
            for i in range(15):
                b_s[(15 * k + i) * TH // 2:(15 * k + i + 1) * TH // 2, :] = _pk(b[i])

        def pre_phase():
            first = [[x_cp(0, 0)], [wq_cp(0)], [x_cp(1, 2), wq_cp(1)],
                     [wq_cp(2), pltpu.make_async_copy(wo_hbm, wo_v, sem_i.at[3])]]
            order = sum(first, [])
            for p in range(NP + 1):
                order += group_cp(p)
            xr_cp = [x_cp(b, SEM_P + NP + 1) for b in range(2, NB)]
            order += xr_cp
            for cp in order:
                cp.start()
            get = lambda an, name: [an[min(i, len(an) - 1)] for i in cfg[name]]
            e_grp = lambda e: ((e >> 1) & 1, ((e >> 2) << 1) | (e & 1))
            if 'a' in cfg['sub']:
                pre_a(first, get, e_grp)
            if 'b' in cfg['sub']:
                pre_b(get, e_grp)
            if 'c' in cfg['sub']:
                pre_c(get)
            wait('WX', xr_cp)

        def pre_a(first, get, e_grp):
            def transpose_wq(i):
                wt_s[WQ[i] // 2:WQ[i + 1] // 2, :D] = _pk(wqkv_v[:, WQ[i]:WQ[i + 1]].T)

            def clear(i, carry):
                for k in range(2):
                    acc_s[k, i] = jnp.zeros((D3, TH), F32)
                r = jnp.minimum(i, 11) * (RP // 4)
                qkv_s[0, rows8(r, RP // 4)] = jnp.zeros((RP // 4, LANES), U32)
                return carry

            lax.fori_loop(0, 15, clear, 0)
            wait('WX0', first[0])
            xn0 = ln1(0, ()).astype(BF16)

            wait('WQ0', first[1])
            transpose_wq(0)
            qkv_mm(0, xn0, (0, 1), [])

            wait('WQ1', first[2])
            transpose_wq(1)
            an = []
            qkv_mm(0, xn0, (2, 3), an)
            xn1 = ln1(1, get(an, 'a_ln'), get(an, 'a_lnb')).astype(BF16)
            qkv_mm(1, xn1, (0,), an, True)
            for n, a in enumerate(get(an, 'a_w1')):
                prep_att(n, a)
            nk = len(cfg['a_k'])
            apply = [att_values(0, *e_grp(e), a, 9) for e, a in enumerate(get(an, 'a_k'))]

            wait('WQ2', first[3])
            an = []
            qkv_mm(1, xn1, (2,), an)
            transpose_wq(2)
            qkv_mm(0, xn0, (4, 5), an)
            qkv_mm(1, xn1, (4, 1), an)
            apply += [att_values(0, *e_grp(nk + e), a, 9)
                      for e, a in enumerate(get(an, 'a_k2')[:8 - nk])]
            for e, a in enumerate(get(an, 'a_v')):
                apply[e](a)
            wo = pltpu.bitcast(wo_v[...], U32)
            wo = cat0(_lo(wo), _hi(wo))
            wo = cat0(*[_tie(wo[n * LANES:(n + 1) * LANES], a)
                        for n, a in enumerate(get(an, 'a_wo'))])
            wt_s[3 * RP:, :D] = _pk(wo.astype(BF16).T)
            stats = wo_mm(0, an, False)
            qkv_mm(1, xn1, (3,), an)
            for n, a in enumerate(get(an, 'a_w2')):
                prep_att(12 + n, a)
            plain_lhs(0, stats)
            n1 = len(cfg['a_att'])
            for e, a in enumerate(get(an, 'a_att')):
                att_group(1, *e_grp(e), a, 9)

            wait('WO', group_cp(0))
            an = []
            b = plain_piece(0, an)
            qkv_mm(1, xn1, (5,), an, True)
            prep_gu(0, get(an, 'z_g'))
            ffn_lhs(0, stats, get(an, 'z_l'))
            for e, a in enumerate(get(an, 'z_att')[:3 - n1]):
                att_group(1, *e_grp(n1 + e), a, 9)
            store_b(b)

        def pre_b(get, e_grp):
            def piece(p, carry):
                wait('WP', group_cp(p))
                b_prev = load_b()
                an = []
                if cfg['fast0']:
                    acc = down_mm(load_acc(0), [b_prev], p - 1, an, D_ORDER[:6], True)
                    t, hv, done = {}, {}, set()
                    for step in cfg['order1']:
                        k = int(step[1])
                        part = k if step[0] == 'S' else 3
                        slabs = [int(step[2])] if len(step) > 2 else list(range(NS))
                        if part not in done:
                            prep_gu(p, get(an, 'f_g%d' % part), _PARTS[part])
                            done.add(part)
                        if step[0] == 'S':
                            for i in _PARTS[k]:
                                gu_prod(p, i, t, an, slabs)
                        else:
                            gu_col(t, hv, p, k, an, slabs)
                    b = h_join(hv)
                    prep_d(p - 1, get(an, 'p_d'))
                    store_acc(0, down_mm(acc, [b_prev], p - 1, an, D_ORDER[6:]))
                else:
                    b = plain_piece(p, an)
                    prep_d(p - 1, get(an, 'p_d'))
                    store_acc(0, down_mm(load_acc(0), [b_prev], p - 1, an))
                    prep_gu(p, get(an, 'p_g'))
                att_group(1, *e_grp(p + 2), an[cfg['p_att'][0]], 9)
                for i, a in enumerate(get(an, 'p_w')):
                    prep_att(jnp.minimum(24 + (p - 1) * 5 + i, 47), a)
                store_b(b)
                return carry

            lax.fori_loop(1, NP, piece, 0)

        def pre_c(get):
            wait('WD', group_cp(NP))
            an = []
            stats = wo_mm(1, an, True)
            prep_d(NP - 1, get(an, 't_d'))
            acc = down_mm(load_acc(0), [load_b()], NP - 1, [])
            ffn_lhs(1, stats, [])
            finish(0, acc)

        if 'pre' in cfg['phases']:
            pre_phase()

        def body(u, carry):
            bu = u & (NB - 1)
            ba = (u + 1) & (NB - 1)
            acc, stats, an, b = None, None, {}, {}
            get = lambda name: [an[k][i] for k, i in cfg[name]]
            for step in cfg['body']:
                an[step] = []
                if step == 'Q':
                    qkv_fast(ba, att_rhs(ln1(ba, get('ln1'), get('ln1b')), u >> 8 if 'q' in cfg['stash'] else None),
                             an[step])
                elif step == 'W':
                    attention(ba, get('att'), cfg['win'])
                    stats = wo_mm(ba, an[step], True, get('orhs'),
                                  u >> 8 if 'w' in cfg['stash'] else None)
                elif step == 'L':
                    ffn_lhs(ba, stats, get('lhs'))
                elif step[0] == 'S':
                    slabs = [int(step[3])] if len(step) > 3 else list(range(NS))
                    for i in _PARTS[int(step[2])]:
                        gu_prod(int(step[1]), i, b.setdefault(step[:2], {}), an[step], slabs)
                elif step[0] == 'F':
                    j, c = int(step[1]), int(step[2])
                    slabs = [int(step[3])] if len(step) > 3 else list(range(NS))
                    hv = b.setdefault(step[:2], {})
                    gu_col(b['S' + step[1]], hv, j, c, an[step], slabs)
                    if len(hv) == 3 * NS:
                        b[j] = h_join(hv)
                        if 'b' in cfg['stash']:
                            store_b(b[j], j)
                            b[j] = load_b(j)
                else:
                    js = [int(c) for c in step[1:]]
                    acc = down_mm(acc, [b[j] for j in js], js[0], an[step])
            finish(bu, acc)

            @pl.when(u >= NB)
            def _():
                out_copy(bu).start()
            return carry

        if scopes:
            with jax.named_scope('LOOP'):
                lax.fori_loop(1, NU - 1, body, 0)
        elif 'main' in cfg['phases']:
            lax.fori_loop(1, NU - 1, body, 0)

        def last(c, carry):
            los = [2 * c + j for j in range(2)]
            b = [gu_piece(lo, cfg['order'], [], j) for j, lo in enumerate(los)]
            acc = load_acc(1)
            for j in range(2):
                acc = down_mm(acc, [b[j]], los[j], [])
            store_acc(1, acc)
            return carry

        if 'last' in cfg['phases']:
            lax.fori_loop(0, NP // 2, last, 0)
        if len(cfg['phases']) < 3:
            def keep(i, c):
                v = (gs_s[i, i, :8, :LANES] + us_s[i, i, :8, :LANES] + ds_s[i, i, :8, :LANES]
                     + wl_s[rows8(i * 8), :LANES] + a_s[i, :8] + qkv_s[i, :8]
                     + b_s[rows8(i * 8), :LANES] + wt_s[rows8(i * 8), :LANES])
                acc_s[1, 0, :8] = (lax.bitcast_convert_type(v, F32) + o_s[i, :8]
                                   + acc_s[i, i, :8])
                return c
            lax.fori_loop(0, 2, keep, 0)
        finish(NB - 1, load_acc(1))
        out_copy(NB - 1).start()
        wait('WOUT', [out_copy(b) for b in range(NB)])

    scratch = [
        pltpu.VMEM((NB, D, TM), BF16),
        pltpu.VMEM((D, 3 * D), BF16),
        pltpu.VMEM((D, D), BF16),
        pltpu.VMEM((NP, 3, D, PW), BF16),
        pltpu.VMEM((NP, 3, D, PW), BF16),
        pltpu.VMEM((NP, 3, D, PW), BF16),
        pltpu.VMEM((2 * D, 8 * LANES), U32),
        pltpu.VMEM((4 * Q3, 16 * LANES), U32),
        pltpu.VMEM((NP, 15, Q3, PW), U32),
        pltpu.VMEM((NP, 15, Q3, PW), U32),
        pltpu.VMEM((NP, 9, Q3, PW), U32),
        pltpu.VMEM((NB, D, TM), F32),
        pltpu.VMEM((54, TH // 2, LANES), U32),
        pltpu.VMEM((S // LANES + 1, 3 * RP, LANES), U32),
        pltpu.VMEM((NT, D, LANES), F32),
        pltpu.VMEM((2, 15, D3, TH), F32),
        pltpu.VMEM((NP * 15 * TH // 2, PW), U32),
        pltpu.VMEM((1, 9 * 64, 2 * LANES), U32),
        pltpu.VMEM((NP, 2, 9, TH, PW), F32),
        pltpu.SemaphoreType.DMA((SEM_P + NP + 2,)),
        pltpu.SemaphoreType.DMA((1,)),
    ]

    def wrapped(*refs):
        @pl.when(pl.program_id(0) == 0)
        def _():
            kernel(*refs)

    return wrapped, scratch


_CFG = dict(
    scopes=False,
    fast0=True,
    psplit=1,
    rcp=False,
    late=True,
    stash='qw',
    slab=True,
    fslab=False,
    win=9,
    sub='abc',
    orhs=(),
    msplit=2,
    phases=('pre', 'main', 'last'),
    order=('S0', 'S1', 'F0', 'S2', 'F1', 'F2'),
    body=('S010', 'S000', 'F000', 'S020', 'F010', 'F020', 'S001', 'S011', 'F001',
        'S110', 'S021', 'F021', 'S100', 'F100', 'S120', 'S101', 'F110', 'F011', 'Q',
        'F120', 'S111', 'F101', 'S121', 'F111', 'F121', 'S200', 'S210', 'F200', 'S220',
        'F210', 'F220', 'S300', 'S201', 'S211', 'F201', 'S320', 'S221', 'F211', 'F221',
        'S310', 'D01', 'F300', 'S301', 'S311', 'F301', 'S321', 'F311', 'F321', 'S400',
        'F310', 'F320', 'S420', 'F410', 'S410', 'S401', 'F420', 'S411', 'F400', 'S421',
        'F411', 'F421', 'S500', 'F401', 'S501', 'S510', 'D23', 'F500', 'S520', 'W',
        'F520', 'S511', 'F510', 'S521', 'F501', 'F511', 'F521', 'D4', 'D5', 'L'),
    ln1=(('S010', 4), ('S010', 5), ('S010', 6), ('S010', 7), ('S010', 8), ('S000', 0),
        ('S000', 1), ('S000', 2), ('S000', 3)),
    ln1b=(('S110', 2), ('S110', 3), ('S110', 5), ('S110', 6), ('S110', 8), ('S021', 0),
        ('S021', 2), ('S021', 3), ('S021', 5), ('S021', 6), ('S021', 8), ('F021', 0)),
    att=(('S300', 8), ('D01', 1), ('D01', 7), ('D01', 8), ('D01', 10), ('F300', 4),
        ('D23', 5), ('D23', 9)),
    lhs=(('D4', 3), ('D5', 1), ('D5', 4)),
    att0=(15, 18, 21, 24, 27, 30, 33, 37),
    order0=('S0', 'S1', 'S2', 'F0', 'F1', 'F2'),
    order1=('S0', 'S1', 'S2', 'F0', 'F1', 'F2'),
    a_w1=(0, 0, 1, 2, 2, 3, 3, 4, 4, 5, 6, 7),
    a_w2=(20, 23, 26, 30, 33, 36, 40, 43, 46, 50, 53, 57),
    a_ln=(0, 3, 6),
    a_lnb=(5, 9, 9),
    z_g=(5, 6, 7, 8, 11, 11, 12, 13, 14, 15, 17, 18, 19, 20, 21, 22, 23, 24, 25, 26, 28,
        29, 30, 31, 32, 35, 36, 37, 38, 40, 41, 42, 43, 45, 46, 47, 48, 49, 50, 51, 52,
        54, 55, 57, 58, 59, 60, 62),
    z_att=(53, 54, 56),
    p_g0=(0, 1, 2, 3, 4, 5),
    p_g1=(6, 7, 8, 9, 10, 10),
    p_g2=(12, 13, 14, 15, 16, 17),
    p_g3=(14, 16, 18, 20, 22, 24, 26, 28, 30, 32, 34, 36),
    t_d=(0, 0, 1, 1, 2, 3, 3, 4, 5, 6, 6, 7, 8, 9, 9, 9, 10, 11, 11, 12, 13, 14, 15,
        16),
    p_d=(32, 33, 35, 35, 35, 37, 37, 38, 39, 41, 42, 43, 44, 45, 45, 46, 47, 48, 49, 51,
        52, 53, 54, 56),
    p_att=(60,),
    p_w=(12, 60, 63, 65, 65),
    p_g=(0, 1, 2, 3, 4, 5, 6, 7, 9, 10, 11, 12, 13, 14, 15, 16, 18, 19, 20, 21, 22, 23,
        24, 25, 27, 28, 29, 30, 31, 32, 33, 34, 36, 37, 38, 39, 40, 41, 42, 43, 45, 46,
        47, 48, 49, 50, 51, 53),
    z_l=(2, 13, 32),
    f_g0=(0, 0, 0, 1, 1, 2, 3, 3, 4, 4, 5, 5),
    f_g1=(4, 5, 5, 7, 8, 9, 9, 10, 11, 12, 13, 15),
    f_g2=(1, 12, 12, 15, 15, 16, 17, 18, 19, 20, 20, 24),
    f_g3=(4, 14, 16, 17, 18, 19, 21, 22, 23, 23, 24, 25, 26, 27, 28, 29, 30, 31, 32, 33,
        34, 35, 36, 37),
    a_k=(15, 19, 20, 24),
    a_k2=(0, 4, 8, 12),
    a_v=(13, 14, 22, 26, 30, 34, 38, 39),
    a_att=(12, 60),
    a_wo=(30, 35, 36, 38, 41),
)


def _run(A_x, A_wqkv, A_wo, B_w_gate, B_w_up, B_w_down, **kw):
    _, S, D = A_x.shape
    F = B_w_gate.shape[1]
    kernel, scratch = _make_kernel(S, D, F, 256, {**_CFG, **kw})
    hbm = pl.BlockSpec(memory_space=pl.ANY)
    out_t = pl.pallas_call(
        kernel,
        grid=(2,),
        in_specs=[hbm] * 6,
        out_specs=hbm,
        out_shape=jax.ShapeDtypeStruct((D, S), A_x.dtype),
        scratch_shapes=scratch,
        compiler_params=pltpu.CompilerParams(
            dimension_semantics=('arbitrary',), vmem_limit_bytes=110 * 1024 * 1024),
    )(A_x.reshape(S, D).T, A_wqkv, A_wo, B_w_gate, B_w_up, B_w_down.T)
    return out_t.T.reshape(A_x.shape)


@jax.jit
def pallas_interleave_layers__sliding_local_dilated__glu_gated_geglu__prompt_kernel(
    A_x: jax.Array,
    A_wqkv: jax.Array,
    A_wo: jax.Array,
    B_x: jax.Array,
    B_w_gate: jax.Array,
    B_w_up: jax.Array,
    B_w_down: jax.Array,
):
    del B_x
    return _run(A_x, A_wqkv, A_wo, B_w_gate, B_w_up, B_w_down)
```

```python
import functools

import jax
import jax.numpy as jnp
import jax.experimental.pallas as pl
import jax.experimental.pallas.tpu as pltpu
from jax import lax

H = 32
W = 8
DIL = 2
EPS = 1e-5
LANES = 128

F32 = jnp.float32
BF16 = jnp.bfloat16
U32 = jnp.uint32

_NT = (((1,), (1,)), ((), ()))


def _tree_sum(parts, op=jnp.add):
    while len(parts) > 1:
        nxt = [op(parts[i], parts[i + 1]) for i in range(0, len(parts) - 1, 2)]
        if len(parts) % 2:
            nxt.append(parts[-1])
        parts = nxt
    return parts[0]


def _ln_stats(slabs, d, anchors=()):
    n_acc = 4
    s1, s2, pilot = [None] * n_acc, [None] * n_acc, None
    for i, x in enumerate(slabs):
        if pilot is None:
            pilot = x[0:1, :]
            pil = jnp.broadcast_to(pilot, x.shape)
            pils = [_tie(pil, a) for a in anchors] or [pil]
        dx = x - pils[i * len(pils) // (d // 8)]
        j = i % n_acc
        s1[j] = dx if s1[j] is None else s1[j] + dx
        s2[j] = dx * dx if s2[j] is None else s2[j] + dx * dx
    e1 = jnp.sum(_tree_sum(s1), axis=0, keepdims=True) * (1.0 / d)
    e2 = jnp.sum(_tree_sum(s2), axis=0, keepdims=True) * (1.0 / d)
    var = jnp.maximum(e2 - e1 * e1, 0.0)
    return pilot + e1, lax.rsqrt(var + EPS)


def _zero_like_dep(v):
    return (lax.bitcast_convert_type(v, U32) >> 31) >> 1


def _tie(x, anchor):
    if anchor is None:
        return x
    z = lax.bitcast_convert_type(_zero_like_dep(anchor), F32)
    z = jnp.concatenate([z] * -(-x.shape[1] // LANES), axis=1)[:, :x.shape[1]]
    if x.shape[0] == 8:
        return x + z
    return jnp.concatenate([x[:8] + z, x[8:]], axis=0)


def _gelu_mul2(g, u):
    c0 = 0.7978845608028654
    c1 = c0 * 0.044715
    t = jnp.tanh(g * (c0 + c1 * (g * g)))
    return (g * u) * (1.0 + t)


def _lo(x):
    return lax.bitcast_convert_type(x << 16, F32)


def _hi(x):
    return lax.bitcast_convert_type(x & jnp.uint32(0xFFFF0000), F32)


def _pk(x):
    return pltpu.bitcast(x.astype(BF16), U32)


def _upk(x):
    return pltpu.bitcast(x, BF16)


def _dot(a, b):
    return jnp.dot(a, b, preferred_element_type=F32)


def _dot_nt(a, b):
    return lax.dot_general(a, b, _NT, preferred_element_type=F32)


def _x_ops(x1, x2):
    d = [a - b for a, b in zip(x1, x2)]
    return [x1[0] + x2[1], x2[0] + x2[1], x1[0] + x1[1],
            d[1] + x1[2], x1[1] + x1[2], d[1] + d[2],
            d[0] - x2[2], d[0] + d[2], x2[0] + x2[2],
            x1[0], d[0], x2[1], d[1], x1[2], x2[2]]


def _x_rem(x1, x2):
    a, b, c = 0, 1, 2
    cat = lambda u, v: jnp.concatenate([u, v], axis=0)
    return [cat(x1[c], x2[b]), cat(x1[a], x1[b] - x2[b]), cat(x2[a], x2[c] - x1[c])]


def _w_sums(w):
    return [w[0][1] + w[1][0], w[1][2] + w[2][1], w[0][2] + w[2][0],
            w[0][0] + w[0][2] - w[1][0], w[2][0] - w[0][0] - w[0][1],
            w[1][1] + w[1][2] - w[0][1], w[1][0] + w[1][1] - w[2][1],
            w[2][0] + w[2][2] - w[1][2], w[2][1] + w[2][2] - w[0][2]]


_W_TERMS = {0: ((0, 1, 1), (1, 0, 1)), 3: ((1, 2, 1), (2, 1, 1)), 6: ((0, 2, 1), (2, 0, 1)),
            9: ((0, 0, 1), (0, 2, 1), (1, 0, -1)), 10: ((2, 0, 1), (0, 0, -1), (0, 1, -1)),
            11: ((1, 1, 1), (1, 2, 1), (0, 1, -1)), 12: ((1, 0, 1), (1, 1, 1), (2, 1, -1)),
            13: ((2, 0, 1), (2, 2, 1), (1, 2, -1)), 14: ((2, 1, 1), (2, 2, 1), (0, 2, -1)),
            1: ((0, 1, 1),), 2: ((1, 0, 1),), 4: ((1, 2, 1),), 5: ((2, 1, 1),),
            7: ((2, 0, 1),), 8: ((0, 2, 1),)}
_PARTS = ((1, 2, 0), (7, 8, 6), (4, 5, 3), (9, 10, 11, 12, 13, 14))
_W_SUM = {0: 0, 3: 1, 6: 2, 9: 3, 10: 4, 11: 5, 12: 6, 13: 7, 14: 8}
_W_RAW = {1: (0, 1), 2: (1, 0), 4: (1, 2), 5: (2, 1), 7: (2, 0), 8: (0, 2)}
_PAIR_ORDER = (1, 2, 4, 5, 7, 8, 0, 3, 6)
_DIAG = {(0, 0): 9, (2, 0): 10, (0, 1): 11, (1, 1): 12, (1, 2): 13, (2, 2): 14}
_PAIR = {(0, 0): ((6, -1), (8, -1)), (1, 0): ((2, 1), (7, 1)), (2, 0): ((0, 1), (1, -1)),
         (0, 1): ((3, 1), (4, -1)), (1, 1): ((0, 1), (2, -1)), (2, 1): ((1, 1), (5, -1)),
         (0, 2): ((4, 1), (8, 1)), (1, 2): ((6, 1), (7, -1)), (2, 2): ((5, 1), (3, -1))}


def _column(t, base, j):
    s = []
    for k in range(3):
        v = base[k]
        for i, sg in _PAIR[k, j]:
            ti = t[i]() if callable(t[i]) else t[i]
            v = ti if v is None else (v + ti if sg > 0 else v - ti)
        s.append(v)
    return s[1] + s[0], s[2] + s[0]


def _make_kernel(S, D, F, TM, cfg):
    NB = S // TM
    NT = TM // LANES
    DH = D // H
    DP = DH // 2
    RP = D // 2
    NG = H // 8
    scale = float(DH) ** -0.5
    NU = 2 * NB
    TH = TM // 2
    FT = F // 3
    D2 = D // 2
    D3 = D // 3
    Q3 = D3 // 2
    KU = D // 9
    KR = 3 * LANES
    NQ = 6
    QR = 3 * D // NQ
    WQ = (0, 640, 1152, 3 * D)
    PW = 256
    NP = FT // PW
    scopes = cfg['scopes']
    assert NG == 4 and NB & (NB - 1) == 0
    SEM_P = 4

    def kernel(x_hbm, wqkv_hbm, wo_hbm, wg_hbm, wu_hbm, wdt_hbm, out_hbm,
               xio_s, wqkv_v, wo_v, wg_v, wu_v, wdt_v, wt_s, wl_s,
               gs_s, us_s, ds_s, xmid_s, a_s, qkv_s, o_s, acc_s, b_s, r_s, t_s,
               sem_i, sem_o):

        def wait(name, cps):
            if scopes:
                with jax.named_scope(name):
                    for cp in cps:
                        cp.wait()
            else:
                for cp in cps:
                    cp.wait()

        def cols(lo, n):
            if not isinstance(lo, int):
                lo = pl.multiple_of(lo, LANES)
            return pl.ds(lo, n)

        def rows8(lo, n=8):
            if not isinstance(lo, int):
                lo = pl.multiple_of(lo, 8)
            return pl.ds(lo, n)

        def out_copy(b):
            return pltpu.make_async_copy(
                xio_s.at[b], out_hbm.at[:, cols(b * TM, TM)], sem_o.at[0])

        def x_cp(b, sem):
            return pltpu.make_async_copy(x_hbm.at[:, cols(b * TM, TM)], xio_s.at[b],
                                         sem_i.at[sem])

        def wq_cp(i):
            sl = cols(WQ[i], WQ[i + 1] - WQ[i])
            return pltpu.make_async_copy(wqkv_hbm.at[:, sl], wqkv_v.at[:, sl],
                                         sem_i.at[1 + i])

        def piece_cp(src, dst, p, sem):
            return [pltpu.make_async_copy(src.at[:, cols(j * FT + p * PW, PW)],
                                          dst.at[p, j],
                                          sem_i.at[sem]) for j in range(3)]

        def group_cp(p):
            sem = SEM_P + p
            cps = []
            if not (isinstance(p, int) and p == NP):
                cps += piece_cp(wg_hbm, wg_v, p, sem) + piece_cp(wu_hbm, wu_v, p, sem)
            if not (isinstance(p, int) and p == 0):
                cps += piece_cp(wdt_hbm, wdt_v, p - 1, sem)
            return cps

        lane = lax.broadcasted_iota(jnp.int32, (8, LANES), 1)
        cat0 = lambda *v: jnp.concatenate(v, axis=0)
        cat1 = lambda *v: jnp.concatenate(v, axis=1)

        def spread_over(anchors, n, total):
            return anchors[n * len(anchors) // total] if anchors else None

        def slab_group(r):
            return (r % LANES) // 16 if r < KR else 8 + ((r - KR) % KU) // 16

        def ln1(blk, anchors1, anchors2=()):
            slabs = (xio_s[blk, r:r + 8, :].astype(F32) for r in range(0, D, 8))
            m, rs = _ln_stats(slabs, D, anchors1)
            if not anchors2:
                return (xio_s[blk].astype(F32) - m) * rs
            m8 = jnp.broadcast_to(m, (8, TM))
            ms = [_tie(m8, a) for a in anchors2]
            ms = [spread_over(ms, slab_group(r), 12) for r in range(0, D, 8)]
            return (xio_s[blk].astype(F32) - cat0(*ms)) * rs

        def dot_k(rows, x, anchors, even=False):
            y = None
            for n, k in enumerate(range(0, D, LANES)):
                ks = slice(k, min(k + LANES, D))
                if even and k + LANES >= D:
                    mid = (rows.start + rows.stop) // 2
                    v = cat0(_dot(_upk(wt_s[rows.start:mid, ks]), x[ks]),
                             _dot(_upk(wt_s[mid:rows.stop, ks]), x[ks]))
                else:
                    v = _dot(_upk(wt_s[rows, ks]), x[ks])
                anchors.extend(v[r:r + 8, :LANES] for r in ((0, 144) if n % 2 else (72, 216)))
                y = v if y is None else y + v
            return y

        def put_qkv(blk, rows, y):
            pk = _pk(y)
            for c in range(NT):
                qkv_s[1 + blk * NT + c, rows, :] = pk[:, c * LANES:(c + 1) * LANES]

        def qkv_mm(blk, xn, chunks, anchors, even=False):
            for r in chunks:
                rows = slice(r * QR // 2, (r + 1) * QR // 2)
                put_qkv(blk, rows, dot_k(rows, xn, anchors, even))

        def split_k(x):
            hs = (x[:, :TH], x[:, TH:])
            blocks = [[h[k * LANES:(k + 1) * LANES] for k in range(3)] for h in hs]
            units = [[h[KR + k * KU:KR + (k + 1) * KU] for k in range(3)] for h in hs]
            return blocks, units

        def prep_att(pat, anchor):
            assert Q3 == 96
            row0 = pat * 8
            src0 = row0 + ((pat * 43) >> 9) * (2 * Q3)
            w = [_upk(wt_s[rows8(src0 + j * Q3), :D]).astype(F32) for j in range(3)]
            w[0] = cat1(_tie(w[0][:, :LANES], anchor), w[0][:, LANES:])
            tiles = _w_sums([[w[j][:, k * LANES:(k + 1) * LANES] for j in range(3)]
                             for k in range(3)])
            for j in range(3):
                a, b, c = (w[j][:, KR + k * KU:KR + (k + 1) * KU] for k in range(3))
                tiles += [cat1(c, b), cat1(a, c)]
            wl_s[rows8(row0), :15 * LANES] = _pk(cat1(*tiles))

        def att_rhs(x, stash=None):
            blocks, units = split_k(x)
            ops = _x_ops(*blocks) + _x_rem(*units)
            if stash is None:
                return [v.astype(BF16) for v in ops]
            loc = lambda i, r0, n: (slice((i // 2) * 64 + r0, (i // 2) * 64 + r0 + n),
                                    slice((i % 2) * LANES, (i % 2 + 1) * LANES))
            for r in range(0, LANES, 16):
                for i, v in enumerate(ops):
                    r_s.at[0][loc(i, r // 2, 8)] = _pk(v[r:r + 16])
            return [_upk(r_s.at[stash][loc(i, 0, 64)]) for i in range(18)]

        def att_mm(sec, rhs, anchors):
            tl = lambda i: _upk(wl_s[sec * Q3:(sec + 1) * Q3, i * LANES:(i + 1) * LANES])
            raw = lambda k, j: _upk(wt_s[(3 * sec + j) * Q3:(3 * sec + j + 1) * Q3,
                                         k * LANES:(k + 1) * LANES])
            t = {}
            for i in _PAIR_ORDER:
                t[i] = _dot(raw(*_W_RAW[i]) if i in _W_RAW else tl(_W_SUM[i]), rhs[i])
                anchors.append(t[i][:8])
            out = []
            for j in range(3):
                base = []
                for s in range(3):
                    v = _dot(raw(3, j) if s == 1 else tl(9 + 2 * j + s // 2), rhs[15 + s])
                    if (s, j) in _DIAG:
                        i = _DIAG[s, j]
                        v = _dot(tl(_W_SUM[i]), rhs[i]) + v
                    base.append(v)
                    anchors.append(base[-1][:8])
                out.append(cat1(*_column(t, base, j)))
            return cat0(*out)

        def qkv_fast(blk, rhs, anchors):
            for sec in range(3):
                put_qkv(blk, slice(sec * RP, (sec + 1) * RP), att_mm(sec, rhs, anchors))

        def shifted(ln, cur, prev, w):
            if w == 0:
                return cur
            sh = DIL * w
            return pltpu.roll(jnp.where(ln < LANES - sh, cur, prev), sh, axis=1)

        def att_group(blk, c, hg, anchor, win):
            att_values(blk, c, hg, anchor, win)(None)

        def att_values(blk, c, hg, anchor, win):
            tile = blk * NT + c
            base = hg * 8 * DP
            if isinstance(hg, int):
                cur, prev, o_t = qkv_s.at[1 + tile], qkv_s.at[tile], o_s.at[c]
            else:
                n = 2 * RP + 8 * DP
                base = pl.multiple_of(base, 8)
                cur = qkv_s.at[1 + tile, pl.ds(base, n)]
                prev = qkv_s.at[tile, pl.ds(base, n)]
                o_t = o_s.at[c, pl.ds(base, RP + 8 * DP)]
                base = 0
            ln = lane + _zero_like_dep(anchor).astype(jnp.int32)
            logits = [None] * W
            done = []
            for dd in range(DP):
                q = cur[pl.ds(base + dd, 8, stride=DP), :]
                kc = cur[pl.ds(RP + base + dd, 8, stride=DP), :]
                if dd >= win:
                    kc = kc | _zero_like_dep(done[dd - win])
                kp = prev[pl.ds(RP + base + dd, 8, stride=DP), :]
                q0, q1 = _lo(q), _hi(q)
                for w in range(W):
                    ks = shifted(ln, kc, kp, w)
                    t = q0 * _lo(ks) + q1 * _hi(ks)
                    logits[w] = t if logits[w] is None else logits[w] + t
                done.append(ks)
            logits = [l * scale for l in logits]
            if not (isinstance(c, int) and c > 0):
                pos = lane + tile * LANES
                logits = [l if w == 0 else jnp.where(pos >= DIL * w, l, -1e9)
                          for w, l in enumerate(logits)]
            m = _tree_sum(logits, jnp.maximum)
            e = [jnp.exp(l - m) for l in logits]
            den = _tree_sum(e)
            if cfg['rcp']:
                r = pl.reciprocal(den, approx=True)
                r = r * (2.0 - den * r)
            else:
                r = 1.0 / den
            p = e if cfg['late'] else [x * r for x in e]

            def apply(anchor2):
                ln = lane + _zero_like_dep(m if anchor2 is None else anchor2).astype(jnp.int32)
                done = []
                for dd in range(DP):
                    vc = cur[pl.ds(2 * RP + base + dd, 8, stride=DP), :]
                    if dd >= win:
                        vc = vc | _zero_like_dep(done[dd - win])
                    vp = prev[pl.ds(2 * RP + base + dd, 8, stride=DP), :]
                    o0 = o1 = None
                    for w in range(W):
                        vs = shifted(ln, vc, vp, w)
                        t0, t1 = p[w] * _lo(vs), p[w] * _hi(vs)
                        o0 = t0 if o0 is None else o0 + t0
                        o1 = t1 if o1 is None else o1 + t1
                    done.append(vs)
                    if cfg['late']:
                        o0, o1 = o0 * r, o1 * r
                    o_t[pl.ds(base + dd, 8, stride=DP), :] = o0
                    o_t[pl.ds(RP + base + dd, 8, stride=DP), :] = o1

            return apply

        def attention(blk, anchors, win):
            for c in range(NT):
                for hg in range(NG):
                    att_group(blk, c, hg, anchors[c * NG + hg], win)

        def wo_mm(blk, anchors, fast, anchors_in=(), stash=None):
            o = cat1(*[o_s[c] for c in range(NT)])
            if anchors_in:
                o = cat0(*[_tie(o[r:r + 8], spread_over(anchors_in, slab_group(r), 12))
                           for r in range(0, D, 8)])
            if fast:
                y = att_mm(3, att_rhs(o, stash), anchors)
            else:
                o = o.astype(BF16)
                q = D2 // 2
                y = cat0(*[dot_k(slice(h * q, (h + 1) * q), o, anchors) for h in (6, 7)])
            xm = xio_s[blk].astype(F32) + y
            xmid_s[blk] = xm
            return _ln_stats((xm[r:r + 8] for r in range(0, D, 8)), D)

        def ffn_lhs(blk, stats, anchors):
            m, rs = stats
            m8 = jnp.broadcast_to(m, (8, TM))
            xs = []
            for k in range(3):
                mt = cat0(*[_tie(m8, spread_over(anchors, k, 3))] * (D3 // 8))
                xs.append((xmid_s[blk, k * D3:(k + 1) * D3, :] - mt) * rs)
            ops = _x_ops([x[:, :TH] for x in xs], [x[:, TH:] for x in xs])
            for i, v in enumerate(ops):
                for s, t in enumerate((v[KU:], v[:2 * KU], cat0(v[:KU], v[2 * KU:]))):
                    a_s[3 * i + s] = _pk(t.astype(BF16).T)

        def plain_lhs(blk, stats):
            m, rs = stats
            blocks, units = split_k((xmid_s[blk] - m) * rs)
            for i, v in enumerate(blocks[0] + blocks[1] + _x_rem(*units)):
                a_s[45 + i] = _pk(v.astype(BF16).T)

        def plain_piece(p, anchors):
            h = {}
            for j in range(3):
                hs = []
                for n in range(PW // LANES):
                    cs = slice(n * LANES, (n + 1) * LANES)
                    w = lambda r0, r1: cat1(wg_v[p, j, r0:r1, cs], wu_v[p, j, r0:r1, cs])
                    u = lambda k: w(KR + k * KU, KR + (k + 1) * KU)
                    ps = cfg['psplit']
                    q = TH // 2 // ps
                    hh = []
                    for s in range(ps):
                        tl = lambda *i: _upk(cat1(*[a_s[45 + k, s * q:(s + 1) * q] for k in i]))
                        y0 = _dot(tl(6), cat0(u(2), u(1)))
                        y1 = _dot(tl(0, 1, 2, 7), w(0, KR + 2 * KU))
                        y2 = _dot(tl(3, 4, 5, 8), cat0(w(0, KR + KU), u(2)))
                        if s == 0:
                            anchors.append(y0[:8, :LANES])
                        for y in (y1, y2):
                            anchors.extend(y[r:r + 8, c:c + LANES] for c in (0, LANES)
                                           for r in range(0, 2 * q, TH // 2))
                        hh.append([_gelu_mul2(*[(y + y0)[:, c:c + LANES] for c in (0, LANES)])
                                   for y in (y1, y2)])
                    hs.append([cat0(*[v[i] for v in hh]) for i in range(2)])
                h[j] = [cat1(*[v[i] for v in hs]) for i in range(2)]
            return h_ops(h)

        def prep_d(p, anchors):
            PR = 16
            for n in range(2 * D3 // PR):
                r, cs = (n // 2) * PR, slice((n % 2) * LANES, (n % 2 + 1) * LANES)
                w = [[wdt_v[p, k, j * D3 + r:j * D3 + r + PR, cs].astype(F32)
                      for j in range(3)] for k in range(3)]
                w[0][1] = _tie(w[0][1], spread_over(anchors, n, 2 * D3 // PR))
                for i, v in enumerate(_w_sums(w)):
                    ds_s.at[p, i][r // 2:(r + PR) // 2, cs] = _pk(v)

        GU = ((wg_v, gs_s), (wu_v, us_s))

        def prep_gu(p, anchors, ids=tuple(range(15))):
            PR = 16
            nr = D3 // PR
            for n in range(4 * nr):
                c, (w_v, s_s), r = n % 2, GU[(n // 2) % 2], (n // 4) * PR
                cache = {}

                def w(k, j):
                    if (k, j) not in cache:
                        ld = lambda c: w_v[p, j, k * D3 + r:k * D3 + r + PR,
                                           c * LANES:(c + 1) * LANES].astype(F32)
                        v = ld(c)
                        if k != j:
                            v = _tie(v, spread_over(anchors, n, 4 * nr))
                        cache[k, j] = v - ld(1 - c) if r // KU == 1 + c else v
                    return cache[k, j]

                for i in ids:
                    v = None
                    for k, j, sg in _W_TERMS[i]:
                        v = w(k, j) if v is None else (v + w(k, j) if sg > 0 else v - w(k, j))
                    s_s.at[p, i][r // 2:(r + PR) // 2, c * LANES:(c + 1) * LANES] = _pk(v)

        NS = cfg['msplit']

        def gu_prod(p, i, t, anchors, slabs, slot=0):
            u = KU // 2

            def rhs(s, s_s):
                if s == 1:
                    return s_s[p, i, :2 * u, :LANES]
                if s == 0:
                    return cat0(s_s[p, i, u:2 * u, LANES:], s_s[p, i, 2 * u:, :LANES])
                return cat0(s_s[p, i, :u, LANES:], s_s[p, i, 2 * u:, LANES:])

            q = TH // 2 // NS
            for n, h in enumerate(slabs):
                y = []
                for s in range(3):
                    r = _upk(cat1(rhs(s, gs_s), rhs(s, us_s)))
                    y.append(_dot(_upk(a_s[3 * i + s, h * q:(h + 1) * q]), r))
                    if (3 * n + s) % len(slabs) == 0:
                        anchors.append(y[-1][:8, :LANES])
                y1, y2 = y[1] + y[0], y[2] + y[0]
                for m in range(2):
                    cs = slice(m * LANES, (m + 1) * LANES)
                    v = cat1(y1[:, cs], y2[:, cs])
                    if i < 9 and 't' in cfg['stash']:
                        k = p if isinstance(p, int) else slot
                        t_s[k, m, i, 2 * h * q:2 * (h + 1) * q] = v
                        v = lambda k=k, m=m, h=h: t_s[k, m, i, 2 * h * q:2 * (h + 1) * q]
                    t.setdefault((m, h), {})[i] = v

        def gu_col(t, hv, p, j, anchors, slabs):
            ids = [_DIAG.get((s, j)) for s in range(3)]
            if cfg['fslab']:
                for h in slabs:
                    for i in ids:
                        if i is not None:
                            gu_prod(p, i, t, anchors if h == slabs[0] else [], [h])
            else:
                for i in ids:
                    if i is not None:
                        gu_prod(p, i, t, anchors, slabs)
            for h in slabs:
                g, u = [_column(t[m, h], [None if i is None else t[m, h][i] for i in ids], j)
                        for m in range(2)]
                hv[j, h] = [_gelu_mul2(g[i], u[i]) for i in range(2)]

        def h_ops(h):
            return [v.astype(BF16) for v in _x_ops(*[[h[j][i] for j in range(3)]
                                                     for i in range(2)])]

        def h_join(hv):
            return h_ops({j: [cat0(*[hv[j, h][i] for h in range(NS)]) for i in range(2)]
                          for j in range(3)})

        def gu_piece(p, order, anchors, slot):
            t, hv = {}, {}
            for slabs in ([[h] for h in range(NS)] if cfg['slab'] else [list(range(NS))]):
                for step in order:
                    if step[0] == 'S':
                        for i in _PARTS[int(step[1])]:
                            gu_prod(p, i, t, anchors, slabs, slot)
                    else:
                        gu_col(t, hv, p, int(step[1]), anchors, slabs)
            return h_join(hv)

        D_ORDER = _PAIR_ORDER + (9, 10, 11, 12, 13, 14)

        def down_mm(acc, bs, lo, anchors, which=D_ORDER, fine=False):
            p = [None] * 15 if acc is None else list(acc)
            for i in which:
                y = None
                for n, b in enumerate(bs):
                    if i in _W_RAW:
                        k, j = _W_RAW[i]
                        v = _dot_nt(wdt_v[lo + n, k, j * D3:(j + 1) * D3, :], b[i])
                    elif len(bs) % 2 and i == 14 and n == 0:
                        v = cat0(*[_dot_nt(_upk(ds_s[lo, _W_SUM[i],
                                                     h * Q3 // 2:(h + 1) * Q3 // 2, :]), b[i])
                                   for h in range(2)])
                    else:
                        v = _dot_nt(_upk(ds_s[lo + n, _W_SUM[i]]), b[i])
                    y = v if y is None else y + v
                p[i] = y if p[i] is None else p[i] + y
                anchors.append(p[i][:8])
                if fine:
                    anchors.append(p[i][D3 // 2:D3 // 2 + 8])
            return p

        def finish(blk, acc):
            y = [cat1(*_column(acc, [acc[_DIAG[s, j]] if (s, j) in _DIAG else None
                                     for s in range(3)], j)) for j in range(3)]
            xio_s[blk] = (xmid_s[blk] + 0.5 * cat0(*y)).astype(BF16)

        def load_acc(k):
            return [acc_s[k, i] for i in range(15)]

        def store_acc(k, acc):
            for i in range(15):
                acc_s[k, i] = acc[i]

        def load_b(k=0):
            return [_upk(b_s[i * TH // 2:(i + 1) * TH // 2, :])
                    for i in range(15 * k, 15 * k + 15)]

        def store_b(b, k=0):
            for i in range(15):
                b_s[(15 * k + i) * TH // 2:(15 * k + i + 1) * TH // 2, :] = _pk(b[i])

        def pre_phase():
            first = [[x_cp(0, 0)], [wq_cp(0)], [x_cp(1, 2), wq_cp(1)],
                     [wq_cp(2), pltpu.make_async_copy(wo_hbm, wo_v, sem_i.at[3])]]
            order = sum(first, [])
            for p in range(NP + 1):
                order += group_cp(p)
            xr_cp = [x_cp(b, SEM_P + NP + 1) for b in range(2, NB)]
            order += xr_cp
            for cp in order:
                cp.start()
            get = lambda an, name: [an[min(i, len(an) - 1)] for i in cfg[name]]
            e_grp = lambda e: ((e >> 1) & 1, ((e >> 2) << 1) | (e & 1))
            if 'a' in cfg['sub']:
                pre_a(first, get, e_grp)
            if 'b' in cfg['sub']:
                pre_b(get, e_grp)
            if 'c' in cfg['sub']:
                pre_c(get)
            wait('WX', xr_cp)

        def pre_a(first, get, e_grp):
            def transpose_wq(i):
                wt_s[WQ[i] // 2:WQ[i + 1] // 2, :D] = _pk(wqkv_v[:, WQ[i]:WQ[i + 1]].T)

            def clear(i, carry):
                for k in range(2):
                    acc_s[k, i] = jnp.zeros((D3, TH), F32)
                r = jnp.minimum(i, 11) * (RP // 4)
                qkv_s[0, rows8(r, RP // 4)] = jnp.zeros((RP // 4, LANES), U32)
                return carry

            lax.fori_loop(0, 15, clear, 0)
            wait('WX0', first[0])
            xn0 = ln1(0, ()).astype(BF16)

            wait('WQ0', first[1])
            transpose_wq(0)
            qkv_mm(0, xn0, (0, 1), [])

            wait('WQ1', first[2])
            transpose_wq(1)
            an = []
            qkv_mm(0, xn0, (2, 3), an)
            xn1 = ln1(1, get(an, 'a_ln'), get(an, 'a_lnb')).astype(BF16)
            qkv_mm(1, xn1, (0,), an, True)
            for n, a in enumerate(get(an, 'a_w1')):
                prep_att(n, a)
            nk = len(cfg['a_k'])
            apply = [att_values(0, *e_grp(e), a, 9) for e, a in enumerate(get(an, 'a_k'))]

            wait('WQ2', first[3])
            an = []
            qkv_mm(1, xn1, (2,), an)
            transpose_wq(2)
            qkv_mm(0, xn0, (4, 5), an)
            qkv_mm(1, xn1, (4, 1), an)
            apply += [att_values(0, *e_grp(nk + e), a, 9)
                      for e, a in enumerate(get(an, 'a_k2')[:8 - nk])]
            for e, a in enumerate(get(an, 'a_v')):
                apply[e](a)
            wo = pltpu.bitcast(wo_v[...], U32)
            wo = cat0(_lo(wo), _hi(wo))
            wo = cat0(*[_tie(wo[n * LANES:(n + 1) * LANES], a)
                        for n, a in enumerate(get(an, 'a_wo'))])
            wt_s[3 * RP:, :D] = _pk(wo.astype(BF16).T)
            stats = wo_mm(0, an, False)
            qkv_mm(1, xn1, (3,), an)
            for n, a in enumerate(get(an, 'a_w2')):
                prep_att(12 + n, a)
            plain_lhs(0, stats)
            n1 = len(cfg['a_att'])
            for e, a in enumerate(get(an, 'a_att')):
                att_group(1, *e_grp(e), a, 9)

            wait('WO', group_cp(0))
            an = []
            b = plain_piece(0, an)
            qkv_mm(1, xn1, (5,), an, True)
            prep_gu(0, get(an, 'z_g'))
            ffn_lhs(0, stats, get(an, 'z_l'))
            for e, a in enumerate(get(an, 'z_att')[:3 - n1]):
                att_group(1, *e_grp(n1 + e), a, 9)
            store_b(b)

        def pre_b(get, e_grp):
            def piece(p, carry):
                wait('WP', group_cp(p))
                b_prev = load_b()
                an = []
                if cfg['fast0']:
                    acc = down_mm(load_acc(0), [b_prev], p - 1, an, D_ORDER[:6], True)
                    t, hv, done = {}, {}, set()
                    for step in cfg['order1']:
                        k = int(step[1])
                        part = k if step[0] == 'S' else 3
                        slabs = [int(step[2])] if len(step) > 2 else list(range(NS))
                        if part not in done:
                            prep_gu(p, get(an, 'f_g%d' % part), _PARTS[part])
                            done.add(part)
                        if step[0] == 'S':
                            for i in _PARTS[k]:
                                gu_prod(p, i, t, an, slabs)
                        else:
                            gu_col(t, hv, p, k, an, slabs)
                    b = h_join(hv)
                    prep_d(p - 1, get(an, 'p_d'))
                    store_acc(0, down_mm(acc, [b_prev], p - 1, an, D_ORDER[6:]))
                else:
                    b = plain_piece(p, an)
                    prep_d(p - 1, get(an, 'p_d'))
                    store_acc(0, down_mm(load_acc(0), [b_prev], p - 1, an))
                    prep_gu(p, get(an, 'p_g'))
                att_group(1, *e_grp(p + 2), an[cfg['p_att'][0]], 9)
                for i, a in enumerate(get(an, 'p_w')):
                    prep_att(jnp.minimum(24 + (p - 1) * 5 + i, 47), a)
                store_b(b)
                return carry

            lax.fori_loop(1, NP, piece, 0)

        def pre_c(get):
            wait('WD', group_cp(NP))
            an = []
            stats = wo_mm(1, an, True)
            prep_d(NP - 1, get(an, 't_d'))
            acc = down_mm(load_acc(0), [load_b()], NP - 1, [])
            ffn_lhs(1, stats, [])
            finish(0, acc)

        if 'pre' in cfg['phases']:
            pre_phase()

        def body(u, carry):
            bu = u & (NB - 1)
            ba = (u + 1) & (NB - 1)
            acc, stats, an, b = None, None, {}, {}
            get = lambda name: [an[k][i] for k, i in cfg[name]]
            for step in cfg['body']:
                an[step] = []
                if step == 'Q':
                    qkv_fast(ba, att_rhs(ln1(ba, get('ln1'), get('ln1b')), u >> 8 if 'q' in cfg['stash'] else None),
                             an[step])
                elif step == 'W':
                    attention(ba, get('att'), cfg['win'])
                    stats = wo_mm(ba, an[step], True, get('orhs'),
                                  u >> 8 if 'w' in cfg['stash'] else None)
                elif step == 'L':
                    ffn_lhs(ba, stats, get('lhs'))
                elif step[0] == 'S':
                    slabs = [int(step[3])] if len(step) > 3 else list(range(NS))
                    for i in _PARTS[int(step[2])]:
                        gu_prod(int(step[1]), i, b.setdefault(step[:2], {}), an[step], slabs)
                elif step[0] == 'F':
                    j, c = int(step[1]), int(step[2])
                    slabs = [int(step[3])] if len(step) > 3 else list(range(NS))
                    hv = b.setdefault(step[:2], {})
                    gu_col(b['S' + step[1]], hv, j, c, an[step], slabs)
                    if len(hv) == 3 * NS:
                        b[j] = h_join(hv)
                        if 'b' in cfg['stash']:
                            store_b(b[j], j)
                            b[j] = load_b(j)
                else:
                    js = [int(c) for c in step[1:]]
                    acc = down_mm(acc, [b[j] for j in js], js[0], an[step])
            finish(bu, acc)

            @pl.when(u >= NB)
            def _():
                out_copy(bu).start()
            return carry

        if scopes:
            with jax.named_scope('LOOP'):
                lax.fori_loop(1, NU - 1, body, 0)
        elif 'main' in cfg['phases']:
            lax.fori_loop(1, NU - 1, body, 0)

        LP = cfg['lp']

        def last(c, carry):
            b = [gu_piece(LP * c + j, cfg['order'], [], j) for j in range(LP)]
            acc = down_mm(load_acc(1), b[:-1], LP * c, [])
            acc = down_mm(acc, b[-1:], LP * c + LP - 1, [])
            store_acc(1, acc)
            if cfg['lfin']:
                finish(NB - 1, acc)
            return carry

        if 'last' in cfg['phases']:
            lax.fori_loop(0, NP // LP, last, 0)
        if len(cfg['phases']) < 3:
            def keep(i, c):
                v = (gs_s[i, i, :8, :LANES] + us_s[i, i, :8, :LANES] + ds_s[i, i, :8, :LANES]
                     + wl_s[rows8(i * 8), :LANES] + a_s[i, :8] + qkv_s[i, :8]
                     + b_s[rows8(i * 8), :LANES] + wt_s[rows8(i * 8), :LANES])
                acc_s[1, 0, :8] = (lax.bitcast_convert_type(v, F32) + o_s[i, :8]
                                   + acc_s[i, i, :8])
                return c
            lax.fori_loop(0, 2, keep, 0)
        if not cfg['lfin']:
            finish(NB - 1, load_acc(1))
        out_copy(NB - 1).start()
        wait('WOUT', [out_copy(b) for b in range(NB)])

    scratch = [
        pltpu.VMEM((NB, D, TM), BF16),
        pltpu.VMEM((D, 3 * D), BF16),
        pltpu.VMEM((D, D), BF16),
        pltpu.VMEM((NP, 3, D, PW), BF16),
        pltpu.VMEM((NP, 3, D, PW), BF16),
        pltpu.VMEM((NP, 3, D, PW), BF16),
        pltpu.VMEM((2 * D, 8 * LANES), U32),
        pltpu.VMEM((4 * Q3, 16 * LANES), U32),
        pltpu.VMEM((NP, 15, Q3, PW), U32),
        pltpu.VMEM((NP, 15, Q3, PW), U32),
        pltpu.VMEM((NP, 9, Q3, PW), U32),
        pltpu.VMEM((NB, D, TM), F32),
        pltpu.VMEM((54, TH // 2, LANES), U32),
        pltpu.VMEM((S // LANES + 1, 3 * RP, LANES), U32),
        pltpu.VMEM((NT, D, LANES), F32),
        pltpu.VMEM((2, 15, D3, TH), F32),
        pltpu.VMEM((NP * 15 * TH // 2, PW), U32),
        pltpu.VMEM((1, 9 * 64, 2 * LANES), U32),
        pltpu.VMEM((NP, 2, 9, TH, PW), F32),
        pltpu.SemaphoreType.DMA((SEM_P + NP + 2,)),
        pltpu.SemaphoreType.DMA((1,)),
    ]

    def wrapped(*refs):
        @pl.when(pl.program_id(0) == 0)
        def _():
            kernel(*refs)

    return wrapped, scratch


_CFG = dict(
    scopes=False, lp=3, lfin=True,
    fast0=True,
    psplit=1,
    rcp=False,
    late=True,
    stash='qw',
    slab=True,
    fslab=False,
    win=9,
    sub='abc',
    orhs=(),
    msplit=2,
    phases=('pre', 'main', 'last'),
    order=('S0', 'S1', 'F0', 'S2', 'F1', 'F2'),
    body=('S010', 'S000', 'F000', 'S020', 'F010', 'F020', 'S001', 'S011', 'F001',
        'S110', 'S021', 'F021', 'S100', 'F100', 'S120', 'S101', 'F110', 'F011', 'Q',
        'F120', 'S111', 'F101', 'S121', 'F111', 'F121', 'S200', 'S210', 'F200', 'S220',
        'F210', 'F220', 'S300', 'S201', 'S211', 'F201', 'S320', 'S221', 'F211', 'F221',
        'S310', 'D01', 'F300', 'S301', 'S311', 'F301', 'S321', 'F311', 'F321', 'S400',
        'F310', 'F320', 'S420', 'F410', 'S410', 'S401', 'F420', 'S411', 'F400', 'S421',
        'F411', 'F421', 'S500', 'F401', 'S501', 'S510', 'D23', 'F500', 'S520', 'W',
        'F520', 'S511', 'F510', 'S521', 'F501', 'F511', 'F521', 'D4', 'D5', 'L'),
    ln1=(('S010', 4), ('S010', 5), ('S010', 6), ('S010', 7), ('S010', 8), ('S000', 0),
        ('S000', 1), ('S000', 2), ('S000', 3)),
    ln1b=(('S110', 2), ('S110', 3), ('S110', 5), ('S110', 6), ('S110', 8), ('S021', 0),
        ('S021', 2), ('S021', 3), ('S021', 5), ('S021', 6), ('S021', 8), ('F021', 0)),
    att=(('S300', 8), ('D01', 1), ('D01', 7), ('D01', 8), ('D01', 10), ('F300', 4),
        ('D23', 5), ('D23', 9)),
    lhs=(('D4', 3), ('D5', 1), ('D5', 4)),
    att0=(15, 18, 21, 24, 27, 30, 33, 37),
    order0=('S0', 'S1', 'S2', 'F0', 'F1', 'F2'),
    order1=('S0', 'S1', 'S2', 'F0', 'F1', 'F2'),
    a_w1=(0, 0, 1, 2, 2, 3, 3, 4, 4, 5, 6, 7),
    a_w2=(20, 23, 26, 30, 33, 36, 40, 43, 46, 50, 53, 57),
    a_ln=(0, 3, 6),
    a_lnb=(5, 9, 9),
    z_g=(5, 6, 7, 8, 11, 11, 12, 13, 14, 15, 17, 18, 19, 20, 21, 22, 23, 24, 25, 26, 28,
        29, 30, 31, 32, 35, 36, 37, 38, 40, 41, 42, 43, 45, 46, 47, 48, 49, 50, 51, 52,
        54, 55, 57, 58, 59, 60, 62),
    z_att=(53, 54, 56),
    p_g0=(0, 1, 2, 3, 4, 5),
    p_g1=(6, 7, 8, 9, 10, 10),
    p_g2=(12, 13, 14, 15, 16, 17),
    p_g3=(14, 16, 18, 20, 22, 24, 26, 28, 30, 32, 34, 36),
    t_d=(0, 0, 1, 1, 2, 3, 3, 4, 5, 6, 6, 7, 8, 9, 9, 9, 10, 11, 11, 12, 13, 14, 15,
        16),
    p_d=(32, 33, 35, 35, 35, 37, 37, 38, 39, 41, 42, 43, 44, 45, 45, 46, 47, 48, 49, 51,
        52, 53, 54, 56),
    p_att=(60,),
    p_w=(12, 60, 63, 65, 65),
    p_g=(0, 1, 2, 3, 4, 5, 6, 7, 9, 10, 11, 12, 13, 14, 15, 16, 18, 19, 20, 21, 22, 23,
        24, 25, 27, 28, 29, 30, 31, 32, 33, 34, 36, 37, 38, 39, 40, 41, 42, 43, 45, 46,
        47, 48, 49, 50, 51, 53),
    z_l=(2, 13, 32),
    f_g0=(0, 0, 0, 1, 1, 2, 3, 3, 4, 4, 5, 5),
    f_g1=(4, 5, 5, 7, 8, 9, 9, 10, 11, 12, 13, 15),
    f_g2=(1, 12, 12, 15, 15, 16, 17, 18, 19, 20, 20, 24),
    f_g3=(4, 14, 16, 17, 18, 19, 21, 22, 23, 23, 24, 25, 26, 27, 28, 29, 30, 31, 32, 33,
        34, 35, 36, 37),
    a_k=(15, 19, 20, 24),
    a_k2=(0, 4, 8, 12),
    a_v=(13, 14, 22, 26, 30, 34, 38, 39),
    a_att=(12, 60),
    a_wo=(30, 35, 36, 38, 41),
)


def _run(A_x, A_wqkv, A_wo, B_w_gate, B_w_up, B_w_down, **kw):
    _, S, D = A_x.shape
    F = B_w_gate.shape[1]
    kernel, scratch = _make_kernel(S, D, F, 256, {**_CFG, **kw})
    hbm = pl.BlockSpec(memory_space=pl.ANY)
    out_t = pl.pallas_call(
        kernel,
        grid=(2,),
        in_specs=[hbm] * 6,
        out_specs=hbm,
        out_shape=jax.ShapeDtypeStruct((D, S), A_x.dtype),
        scratch_shapes=scratch,
        compiler_params=pltpu.CompilerParams(
            dimension_semantics=('arbitrary',), vmem_limit_bytes=110 * 1024 * 1024),
    )(A_x.reshape(S, D).T, A_wqkv, A_wo, B_w_gate, B_w_up, B_w_down.T)
    return out_t.T.reshape(A_x.shape)


@jax.jit
def pallas_interleave_layers__sliding_local_dilated__glu_gated_geglu__prompt_kernel(
    A_x: jax.Array,
    A_wqkv: jax.Array,
    A_wo: jax.Array,
    B_x: jax.Array,
    B_w_gate: jax.Array,
    B_w_up: jax.Array,
    B_w_down: jax.Array,
):
    del B_x
    return _run(A_x, A_wqkv, A_wo, B_w_gate, B_w_up, B_w_down)
```

```python
import functools

import jax
import jax.numpy as jnp
import jax.experimental.pallas as pl
import jax.experimental.pallas.tpu as pltpu
from jax import lax

H = 32
W = 8
DIL = 2
EPS = 1e-5
LANES = 128

F32 = jnp.float32
BF16 = jnp.bfloat16
U32 = jnp.uint32

_NT = (((1,), (1,)), ((), ()))


def _tree_sum(parts, op=jnp.add):
    while len(parts) > 1:
        nxt = [op(parts[i], parts[i + 1]) for i in range(0, len(parts) - 1, 2)]
        if len(parts) % 2:
            nxt.append(parts[-1])
        parts = nxt
    return parts[0]


def _ln_stats(slabs, d, anchors=()):
    n_acc = 4
    s1, s2, pilot = [None] * n_acc, [None] * n_acc, None
    for i, x in enumerate(slabs):
        if pilot is None:
            pilot = x[0:1, :]
            pil = jnp.broadcast_to(pilot, x.shape)
            pils = [_tie(pil, a) for a in anchors] or [pil]
        dx = x - pils[i * len(pils) // (d // 8)]
        j = i % n_acc
        s1[j] = dx if s1[j] is None else s1[j] + dx
        s2[j] = dx * dx if s2[j] is None else s2[j] + dx * dx
    e1 = jnp.sum(_tree_sum(s1), axis=0, keepdims=True) * (1.0 / d)
    e2 = jnp.sum(_tree_sum(s2), axis=0, keepdims=True) * (1.0 / d)
    var = jnp.maximum(e2 - e1 * e1, 0.0)
    return pilot + e1, lax.rsqrt(var + EPS)


def _zero_like_dep(v):
    return (lax.bitcast_convert_type(v, U32) >> 31) >> 1


def _tie(x, anchor):
    if anchor is None:
        return x
    z = lax.bitcast_convert_type(_zero_like_dep(anchor), F32)
    z = jnp.concatenate([z] * -(-x.shape[1] // LANES), axis=1)[:, :x.shape[1]]
    if x.shape[0] == 8:
        return x + z
    return jnp.concatenate([x[:8] + z, x[8:]], axis=0)


def _gelu_mul2(g, u):
    c0 = 0.7978845608028654
    c1 = c0 * 0.044715
    t = jnp.tanh(g * (c0 + c1 * (g * g)))
    return (g * u) * (1.0 + t)


def _lo(x):
    return lax.bitcast_convert_type(x << 16, F32)


def _hi(x):
    return lax.bitcast_convert_type(x & jnp.uint32(0xFFFF0000), F32)


def _pk(x):
    return pltpu.bitcast(x.astype(BF16), U32)


def _upk(x):
    return pltpu.bitcast(x, BF16)


def _dot(a, b):
    return jnp.dot(a, b, preferred_element_type=F32)


def _dot_nt(a, b):
    return lax.dot_general(a, b, _NT, preferred_element_type=F32)


def _x_ops(x1, x2):
    d = [a - b for a, b in zip(x1, x2)]
    return [x1[0] + x2[1], x2[0] + x2[1], x1[0] + x1[1],
            d[1] + x1[2], x1[1] + x1[2], d[1] + d[2],
            d[0] - x2[2], d[0] + d[2], x2[0] + x2[2],
            x1[0], d[0], x2[1], d[1], x1[2], x2[2]]


def _x_rem(x1, x2):
    a, b, c = 0, 1, 2
    cat = lambda u, v: jnp.concatenate([u, v], axis=0)
    return [cat(x1[c], x2[b]), cat(x1[a], x1[b] - x2[b]), cat(x2[a], x2[c] - x1[c])]


def _w_sums(w):
    return [w[0][1] + w[1][0], w[1][2] + w[2][1], w[0][2] + w[2][0],
            w[0][0] + w[0][2] - w[1][0], w[2][0] - w[0][0] - w[0][1],
            w[1][1] + w[1][2] - w[0][1], w[1][0] + w[1][1] - w[2][1],
            w[2][0] + w[2][2] - w[1][2], w[2][1] + w[2][2] - w[0][2]]


_W_TERMS = {0: ((0, 1, 1), (1, 0, 1)), 3: ((1, 2, 1), (2, 1, 1)), 6: ((0, 2, 1), (2, 0, 1)),
            9: ((0, 0, 1), (0, 2, 1), (1, 0, -1)), 10: ((2, 0, 1), (0, 0, -1), (0, 1, -1)),
            11: ((1, 1, 1), (1, 2, 1), (0, 1, -1)), 12: ((1, 0, 1), (1, 1, 1), (2, 1, -1)),
            13: ((2, 0, 1), (2, 2, 1), (1, 2, -1)), 14: ((2, 1, 1), (2, 2, 1), (0, 2, -1)),
            1: ((0, 1, 1),), 2: ((1, 0, 1),), 4: ((1, 2, 1),), 5: ((2, 1, 1),),
            7: ((2, 0, 1),), 8: ((0, 2, 1),)}


def _w_op(i, w):
    v = None
    for k, j, sg in _W_TERMS[i]:
        v = w(k, j) if v is None else (v + w(k, j) if sg > 0 else v - w(k, j))
    return v


_PARTS = ((1, 2, 0), (7, 8, 6), (4, 5, 3), (9, 10, 11, 12, 13, 14))
_W_SUM = {0: 0, 3: 1, 6: 2, 9: 3, 10: 4, 11: 5, 12: 6, 13: 7, 14: 8}
_W_RAW = {1: (0, 1), 2: (1, 0), 4: (1, 2), 5: (2, 1), 7: (2, 0), 8: (0, 2)}
_PAIR_ORDER = (1, 2, 4, 5, 7, 8, 0, 3, 6)
_DIAG = {(0, 0): 9, (2, 0): 10, (0, 1): 11, (1, 1): 12, (1, 2): 13, (2, 2): 14}
_PAIR = {(0, 0): ((6, -1), (8, -1)), (1, 0): ((2, 1), (7, 1)), (2, 0): ((0, 1), (1, -1)),
         (0, 1): ((3, 1), (4, -1)), (1, 1): ((0, 1), (2, -1)), (2, 1): ((1, 1), (5, -1)),
         (0, 2): ((4, 1), (8, 1)), (1, 2): ((6, 1), (7, -1)), (2, 2): ((5, 1), (3, -1))}


def _column(t, base, j):
    s = []
    for k in range(3):
        v = base[k]
        for i, sg in _PAIR[k, j]:
            ti = t[i]() if callable(t[i]) else t[i]
            v = ti if v is None else (v + ti if sg > 0 else v - ti)
        s.append(v)
    return s[1] + s[0], s[2] + s[0]


def _make_kernel(S, D, F, TM, cfg):
    NB = S // TM
    NT = TM // LANES
    DH = D // H
    DP = DH // 2
    RP = D // 2
    NG = H // 8
    scale = float(DH) ** -0.5
    NU = 2 * NB
    TH = TM // 2
    FT = F // 3
    D2 = D // 2
    D3 = D // 3
    Q3 = D3 // 2
    KU = D // 9
    KR = 3 * LANES
    NQ = 6
    QR = 3 * D // NQ
    WQ = (0, 640, 1152, 3 * D)
    PW = 256
    NP = FT // PW
    scopes = cfg['scopes']
    assert NG == 4 and NB & (NB - 1) == 0
    SEM_P = 4

    def kernel(x_hbm, wqkv_hbm, wo_hbm, wg_hbm, wu_hbm, wdt_hbm, out_hbm,
               xio_s, wqkv_v, wo_v, wg_v, wu_v, wdt_v, wt_s, wl_s,
               gs_s, us_s, ds_s, xmid_s, a_s, qkv_s, o_s, acc_s, b_s, r_s, t_s,
               sem_i, sem_o):

        def wait(name, cps):
            if scopes:
                with jax.named_scope(name):
                    for cp in cps:
                        cp.wait()
            else:
                for cp in cps:
                    cp.wait()

        def cols(lo, n):
            if not isinstance(lo, int):
                lo = pl.multiple_of(lo, LANES)
            return pl.ds(lo, n)

        def rows8(lo, n=8):
            if not isinstance(lo, int):
                lo = pl.multiple_of(lo, 8)
            return pl.ds(lo, n)

        def out_copy(b):
            return pltpu.make_async_copy(
                xio_s.at[b], out_hbm.at[:, cols(b * TM, TM)], sem_o.at[0])

        def x_cp(b, sem):
            return pltpu.make_async_copy(x_hbm.at[:, cols(b * TM, TM)], xio_s.at[b],
                                         sem_i.at[sem])

        def wq_cp(i):
            sl = cols(WQ[i], WQ[i + 1] - WQ[i])
            return pltpu.make_async_copy(wqkv_hbm.at[:, sl], wqkv_v.at[:, sl],
                                         sem_i.at[1 + i])

        def piece_cp(src, dst, p, sem):
            return [pltpu.make_async_copy(src.at[:, cols(j * FT + p * PW, PW)],
                                          dst.at[p, j],
                                          sem_i.at[sem]) for j in range(3)]

        def group_cp(p):
            sem = SEM_P + p
            cps = []
            if not (isinstance(p, int) and p == NP):
                cps += piece_cp(wg_hbm, wg_v, p, sem) + piece_cp(wu_hbm, wu_v, p, sem)
            if not (isinstance(p, int) and p == 0):
                cps += piece_cp(wdt_hbm, wdt_v, p - 1, sem)
            return cps

        lane = lax.broadcasted_iota(jnp.int32, (8, LANES), 1)
        cat0 = lambda *v: jnp.concatenate(v, axis=0)
        cat1 = lambda *v: jnp.concatenate(v, axis=1)

        def spread_over(anchors, n, total):
            return anchors[n * len(anchors) // total] if anchors else None

        def slab_group(r):
            return (r % LANES) // 16 if r < KR else 8 + ((r - KR) % KU) // 16

        def ln1(blk, anchors1, anchors2=()):
            slabs = (xio_s[blk, r:r + 8, :].astype(F32) for r in range(0, D, 8))
            m, rs = _ln_stats(slabs, D, anchors1)
            if not anchors2:
                return (xio_s[blk].astype(F32) - m) * rs
            m8 = jnp.broadcast_to(m, (8, TM))
            ms = [_tie(m8, a) for a in anchors2]
            ms = [spread_over(ms, slab_group(r), 12) for r in range(0, D, 8)]
            return (xio_s[blk].astype(F32) - cat0(*ms)) * rs

        def dot_k(rows, x, anchors, even=False):
            y = None
            for n, k in enumerate(range(0, D, LANES)):
                ks = slice(k, min(k + LANES, D))
                if even and k + LANES >= D:
                    mid = (rows.start + rows.stop) // 2
                    v = cat0(_dot(_upk(wt_s[rows.start:mid, ks]), x[ks]),
                             _dot(_upk(wt_s[mid:rows.stop, ks]), x[ks]))
                else:
                    v = _dot(_upk(wt_s[rows, ks]), x[ks])
                anchors.extend(v[r:r + 8, :LANES] for r in ((0, 144) if n % 2 else (72, 216)))
                y = v if y is None else y + v
            return y

        def put_qkv(blk, rows, y):
            pk = _pk(y)
            for c in range(NT):
                qkv_s[1 + blk * NT + c, rows, :] = pk[:, c * LANES:(c + 1) * LANES]

        def qkv_mm(blk, xn, chunks, anchors, even=False):
            for r in chunks:
                rows = slice(r * QR // 2, (r + 1) * QR // 2)
                put_qkv(blk, rows, dot_k(rows, xn, anchors, even))

        def split_k(x):
            hs = (x[:, :TH], x[:, TH:])
            blocks = [[h[k * LANES:(k + 1) * LANES] for k in range(3)] for h in hs]
            units = [[h[KR + k * KU:KR + (k + 1) * KU] for k in range(3)] for h in hs]
            return blocks, units

        def prep_att(pat, anchor):
            assert Q3 == 96
            row0 = pat * 8
            src0 = row0 + ((pat * 43) >> 9) * (2 * Q3)
            w = [_upk(wt_s[rows8(src0 + j * Q3), :D]).astype(F32) for j in range(3)]
            w[0] = cat1(_tie(w[0][:, :LANES], anchor), w[0][:, LANES:])
            tiles = _w_sums([[w[j][:, k * LANES:(k + 1) * LANES] for j in range(3)]
                             for k in range(3)])
            for j in range(3):
                a, b, c = (w[j][:, KR + k * KU:KR + (k + 1) * KU] for k in range(3))
                tiles += [cat1(c, b), cat1(a, c)]
            wl_s[rows8(row0), :15 * LANES] = _pk(cat1(*tiles))

        def att_rhs(x, stash=None):
            blocks, units = split_k(x)
            ops = _x_ops(*blocks) + _x_rem(*units)
            if stash is None:
                return [v.astype(BF16) for v in ops]
            loc = lambda i, r0, n: (slice((i // 2) * 64 + r0, (i // 2) * 64 + r0 + n),
                                    slice((i % 2) * LANES, (i % 2 + 1) * LANES))
            for r in range(0, LANES, 16):
                for i, v in enumerate(ops):
                    r_s.at[0][loc(i, r // 2, 8)] = _pk(v[r:r + 16])
            return [_upk(r_s.at[stash][loc(i, 0, 64)]) for i in range(18)]

        def att_mm(sec, rhs, anchors):
            tl = lambda i: _upk(wl_s[sec * Q3:(sec + 1) * Q3, i * LANES:(i + 1) * LANES])
            raw = lambda k, j: _upk(wt_s[(3 * sec + j) * Q3:(3 * sec + j + 1) * Q3,
                                         k * LANES:(k + 1) * LANES])
            t = {}
            for i in _PAIR_ORDER:
                t[i] = _dot(raw(*_W_RAW[i]) if i in _W_RAW else tl(_W_SUM[i]), rhs[i])
                anchors.append(t[i][:8])
            out = []
            for j in range(3):
                base = []
                for s in range(3):
                    v = _dot(raw(3, j) if s == 1 else tl(9 + 2 * j + s // 2), rhs[15 + s])
                    if (s, j) in _DIAG:
                        i = _DIAG[s, j]
                        v = _dot(tl(_W_SUM[i]), rhs[i]) + v
                    base.append(v)
                    anchors.append(base[-1][:8])
                out.append(cat1(*_column(t, base, j)))
            return cat0(*out)

        def qkv_fast(blk, rhs, anchors):
            for sec in range(3):
                put_qkv(blk, slice(sec * RP, (sec + 1) * RP), att_mm(sec, rhs, anchors))

        def shifted(ln, cur, prev, w):
            if w == 0:
                return cur
            sh = DIL * w
            return pltpu.roll(jnp.where(ln < LANES - sh, cur, prev), sh, axis=1)

        def att_group(blk, c, hg, anchor, win):
            att_values(blk, c, hg, anchor, win)(None)

        def att_values(blk, c, hg, anchor, win):
            tile = blk * NT + c
            base = hg * 8 * DP
            if isinstance(hg, int):
                cur, prev, o_t = qkv_s.at[1 + tile], qkv_s.at[tile], o_s.at[c]
            else:
                n = 2 * RP + 8 * DP
                base = pl.multiple_of(base, 8)
                cur = qkv_s.at[1 + tile, pl.ds(base, n)]
                prev = qkv_s.at[tile, pl.ds(base, n)]
                o_t = o_s.at[c, pl.ds(base, RP + 8 * DP)]
                base = 0
            ln = lane + _zero_like_dep(anchor).astype(jnp.int32)
            logits = [None] * W
            done = []
            for dd in range(DP):
                q = cur[pl.ds(base + dd, 8, stride=DP), :]
                kc = cur[pl.ds(RP + base + dd, 8, stride=DP), :]
                if dd >= win:
                    kc = kc | _zero_like_dep(done[dd - win])
                kp = prev[pl.ds(RP + base + dd, 8, stride=DP), :]
                q0, q1 = _lo(q), _hi(q)
                for w in range(W):
                    ks = shifted(ln, kc, kp, w)
                    t = q0 * _lo(ks) + q1 * _hi(ks)
                    logits[w] = t if logits[w] is None else logits[w] + t
                done.append(ks)
            logits = [l * scale for l in logits]
            if not (isinstance(c, int) and c > 0):
                pos = lane + tile * LANES
                logits = [l if w == 0 else jnp.where(pos >= DIL * w, l, -1e9)
                          for w, l in enumerate(logits)]
            m = _tree_sum(logits, jnp.maximum)
            e = [jnp.exp(l - m) for l in logits]
            den = _tree_sum(e)
            if cfg['rcp']:
                r = pl.reciprocal(den, approx=True)
                r = r * (2.0 - den * r)
            else:
                r = 1.0 / den
            p = e if cfg['late'] else [x * r for x in e]

            def apply(anchor2):
                ln = lane + _zero_like_dep(m if anchor2 is None else anchor2).astype(jnp.int32)
                done = []
                for dd in range(DP):
                    vc = cur[pl.ds(2 * RP + base + dd, 8, stride=DP), :]
                    if dd >= win:
                        vc = vc | _zero_like_dep(done[dd - win])
                    vp = prev[pl.ds(2 * RP + base + dd, 8, stride=DP), :]
                    o0 = o1 = None
                    for w in range(W):
                        vs = shifted(ln, vc, vp, w)
                        t0, t1 = p[w] * _lo(vs), p[w] * _hi(vs)
                        o0 = t0 if o0 is None else o0 + t0
                        o1 = t1 if o1 is None else o1 + t1
                    done.append(vs)
                    if cfg['late']:
                        o0, o1 = o0 * r, o1 * r
                    o_t[pl.ds(base + dd, 8, stride=DP), :] = o0
                    o_t[pl.ds(RP + base + dd, 8, stride=DP), :] = o1

            return apply

        def attention(blk, anchors, win):
            for c in range(NT):
                for hg in range(NG):
                    att_group(blk, c, hg, anchors[c * NG + hg], win)

        def wo_mm(blk, anchors, fast, anchors_in=(), stash=None):
            o = cat1(*[o_s[c] for c in range(NT)])
            if anchors_in:
                o = cat0(*[_tie(o[r:r + 8], spread_over(anchors_in, slab_group(r), 12))
                           for r in range(0, D, 8)])
            if fast:
                y = att_mm(3, att_rhs(o, stash), anchors)
            else:
                o = o.astype(BF16)
                q = D2 // 2
                y = cat0(*[dot_k(slice(h * q, (h + 1) * q), o, anchors) for h in (6, 7)])
            xm = xio_s[blk].astype(F32) + y
            xmid_s[blk] = xm
            return _ln_stats((xm[r:r + 8] for r in range(0, D, 8)), D)

        def ffn_lhs(blk, stats, anchors):
            m, rs = stats
            m8 = jnp.broadcast_to(m, (8, TM))
            xs = []
            for k in range(3):
                mt = cat0(*[_tie(m8, spread_over(anchors, k, 3))] * (D3 // 8))
                xs.append((xmid_s[blk, k * D3:(k + 1) * D3, :] - mt) * rs)
            ops = _x_ops([x[:, :TH] for x in xs], [x[:, TH:] for x in xs])
            for i, v in enumerate(ops):
                for s, t in enumerate((v[KU:], v[:2 * KU], cat0(v[:KU], v[2 * KU:]))):
                    a_s[3 * i + s] = _pk(t.astype(BF16).T)

        def plain_lhs(blk, stats):
            m, rs = stats
            blocks, units = split_k((xmid_s[blk] - m) * rs)
            for i, v in enumerate(blocks[0] + blocks[1] + _x_rem(*units)):
                a_s[45 + i] = _pk(v.astype(BF16).T)

        def plain_piece(p, anchors):
            h = {}
            for j in range(3):
                hs = []
                for n in range(PW // LANES):
                    cs = slice(n * LANES, (n + 1) * LANES)
                    w = lambda r0, r1: cat1(wg_v[p, j, r0:r1, cs], wu_v[p, j, r0:r1, cs])
                    u = lambda k: w(KR + k * KU, KR + (k + 1) * KU)
                    ps = cfg['psplit']
                    q = TH // 2 // ps
                    hh = []
                    for s in range(ps):
                        tl = lambda *i: _upk(cat1(*[a_s[45 + k, s * q:(s + 1) * q] for k in i]))
                        y0 = _dot(tl(6), cat0(u(2), u(1)))
                        y1 = _dot(tl(0, 1, 2, 7), w(0, KR + 2 * KU))
                        y2 = _dot(tl(3, 4, 5, 8), cat0(w(0, KR + KU), u(2)))
                        if s == 0:
                            anchors.append(y0[:8, :LANES])
                        for y in (y1, y2):
                            anchors.extend(y[r:r + 8, c:c + LANES] for c in (0, LANES)
                                           for r in range(0, 2 * q, TH // 2))
                        hh.append([_gelu_mul2(*[(y + y0)[:, c:c + LANES] for c in (0, LANES)])
                                   for y in (y1, y2)])
                    hs.append([cat0(*[v[i] for v in hh]) for i in range(2)])
                h[j] = [cat1(*[v[i] for v in hs]) for i in range(2)]
            return h_ops(h)

        def prep_d(p, anchors):
            PR = 16
            for n in range(2 * D3 // PR):
                r, cs = (n // 2) * PR, slice((n % 2) * LANES, (n % 2 + 1) * LANES)
                w = [[wdt_v[p, k, j * D3 + r:j * D3 + r + PR, cs].astype(F32)
                      for j in range(3)] for k in range(3)]
                w[0][1] = _tie(w[0][1], spread_over(anchors, n, 2 * D3 // PR))
                for i, v in enumerate(_w_sums(w)):
                    ds_s.at[p, i][r // 2:(r + PR) // 2, cs] = _pk(v)

        GU = ((wg_v, gs_s), (wu_v, us_s))

        def prep_gu(p, anchors, ids=tuple(range(15))):
            PR = 16
            nr = D3 // PR
            for n in range(4 * nr):
                c, (w_v, s_s), r = n % 2, GU[(n // 2) % 2], (n // 4) * PR
                cache = {}

                def w(k, j):
                    if (k, j) not in cache:
                        ld = lambda c: w_v[p, j, k * D3 + r:k * D3 + r + PR,
                                           c * LANES:(c + 1) * LANES].astype(F32)
                        v = ld(c)
                        if k != j:
                            v = _tie(v, spread_over(anchors, n, 4 * nr))
                        cache[k, j] = v - ld(1 - c) if r // KU == 1 + c else v
                    return cache[k, j]

                for i in ids:
                    v = None
                    for k, j, sg in _W_TERMS[i]:
                        v = w(k, j) if v is None else (v + w(k, j) if sg > 0 else v - w(k, j))
                    s_s.at[p, i][r // 2:(r + PR) // 2, c * LANES:(c + 1) * LANES] = _pk(v)

        def prep_gu_part(p, part, anchors):
            PR = 16
            nr = D3 // PR
            ids = _PARTS[part]
            for n in range(2 * nr):
                (w_v, s_s), r = GU[n % 2], (n // 2) * PR
                unit = r // KU
                put = lambda i, c, v: s_s.at[p, i].__setitem__(
                    (slice(r // 2, (r + PR) // 2), slice(c * LANES, (c + 1) * LANES)), _pk(v))
                if part < 3:
                    cache = {}

                    def w(k, j):
                        if (k, j) not in cache:
                            v = w_v[p, j, k * D3 + r:k * D3 + r + PR, :].astype(F32)
                            v = _tie(v, spread_over(anchors, n, 2 * nr))
                            l, h = v[:, :LANES], v[:, LANES:]
                            cache[k, j] = (v, cat1(l - h, h), cat1(l, h - l))[unit]
                        return cache[k, j]

                    for i in ids:
                        s_s.at[p, i][r // 2:(r + PR) // 2, :] = _pk(_w_op(i, w))
                    continue
                prev = None
                for m, c in enumerate((1, 0) if unit == 1 else (0, 1)):
                    cache = {}

                    def w(k, j):
                        if (k, j) not in cache:
                            v = w_v[p, j, k * D3 + r:k * D3 + r + PR,
                                    c * LANES:(c + 1) * LANES].astype(F32)
                            if k == j:
                                v = _tie(v, spread_over(anchors, 2 * n + m, 4 * nr))
                            cache[k, j] = v
                        return cache[k, j]

                    sums = [_w_op(i, w) for i in ids]
                    for q, i in enumerate(ids):
                        put(i, c, sums[q] - prev[q] if m and unit else sums[q])
                    prev = sums

        NS = cfg['msplit']

        def gu_prod(p, i, t, anchors, slabs, slot=0):
            u = KU // 2

            def rhs(s, s_s):
                if s == 1:
                    return s_s[p, i, :2 * u, :LANES]
                if s == 0:
                    return cat0(s_s[p, i, u:2 * u, LANES:], s_s[p, i, 2 * u:, :LANES])
                return cat0(s_s[p, i, :u, LANES:], s_s[p, i, 2 * u:, LANES:])

            q = TH // 2 // NS
            for n, h in enumerate(slabs):
                y = []
                for s in range(3):
                    r = _upk(cat1(rhs(s, gs_s), rhs(s, us_s)))
                    y.append(_dot(_upk(a_s[3 * i + s, h * q:(h + 1) * q]), r))
                    if (3 * n + s) % len(slabs) == 0:
                        anchors.append(y[-1][:8, :LANES])
                y1, y2 = y[1] + y[0], y[2] + y[0]
                for m in range(2):
                    cs = slice(m * LANES, (m + 1) * LANES)
                    v = cat1(y1[:, cs], y2[:, cs])
                    if i < 9 and 't' in cfg['stash']:
                        k = p if isinstance(p, int) else slot
                        t_s[k, m, i, 2 * h * q:2 * (h + 1) * q] = v
                        v = lambda k=k, m=m, h=h: t_s[k, m, i, 2 * h * q:2 * (h + 1) * q]
                    t.setdefault((m, h), {})[i] = v

        def gu_col(t, hv, p, j, anchors, slabs):
            ids = [_DIAG.get((s, j)) for s in range(3)]
            if cfg['fslab']:
                for h in slabs:
                    for i in ids:
                        if i is not None:
                            gu_prod(p, i, t, anchors if h == slabs[0] else [], [h])
            else:
                for i in ids:
                    if i is not None:
                        gu_prod(p, i, t, anchors, slabs)
            for h in slabs:
                g, u = [_column(t[m, h], [None if i is None else t[m, h][i] for i in ids], j)
                        for m in range(2)]
                hv[j, h] = [_gelu_mul2(g[i], u[i]) for i in range(2)]

        def h_ops(h):
            return [v.astype(BF16) for v in _x_ops(*[[h[j][i] for j in range(3)]
                                                     for i in range(2)])]

        def h_join(hv):
            return h_ops({j: [cat0(*[hv[j, h][i] for h in range(NS)]) for i in range(2)]
                          for j in range(3)})

        def gu_piece(p, order, anchors, slot):
            t, hv = {}, {}
            for slabs in ([[h] for h in range(NS)] if cfg['slab'] else [list(range(NS))]):
                for step in order:
                    if step[0] == 'S':
                        for i in _PARTS[int(step[1])]:
                            gu_prod(p, i, t, anchors, slabs, slot)
                    else:
                        gu_col(t, hv, p, int(step[1]), anchors, slabs)
            return h_join(hv)

        D_ORDER = _PAIR_ORDER + (9, 10, 11, 12, 13, 14)

        def down_mm(acc, bs, lo, anchors, which=D_ORDER, fine=False):
            p = [None] * 15 if acc is None else list(acc)
            for i in which:
                y = None
                for n, b in enumerate(bs):
                    if i in _W_RAW:
                        k, j = _W_RAW[i]
                        v = _dot_nt(wdt_v[lo + n, k, j * D3:(j + 1) * D3, :], b[i])
                    elif len(bs) % 2 and i == 14 and n == 0:
                        v = cat0(*[_dot_nt(_upk(ds_s[lo, _W_SUM[i],
                                                     h * Q3 // 2:(h + 1) * Q3 // 2, :]), b[i])
                                   for h in range(2)])
                    else:
                        v = _dot_nt(_upk(ds_s[lo + n, _W_SUM[i]]), b[i])
                    y = v if y is None else y + v
                p[i] = y if p[i] is None else p[i] + y
                anchors.append(p[i][:8])
                if fine:
                    anchors.append(p[i][D3 // 2:D3 // 2 + 8])
            return p

        def finish(blk, acc):
            y = [cat1(*_column(acc, [acc[_DIAG[s, j]] if (s, j) in _DIAG else None
                                     for s in range(3)], j)) for j in range(3)]
            xio_s[blk] = (xmid_s[blk] + 0.5 * cat0(*y)).astype(BF16)

        def load_acc(k):
            return [acc_s[k, i] for i in range(15)]

        def store_acc(k, acc):
            for i in range(15):
                acc_s[k, i] = acc[i]

        def load_b(k=0):
            return [_upk(b_s[i * TH // 2:(i + 1) * TH // 2, :])
                    for i in range(15 * k, 15 * k + 15)]

        def store_b(b, k=0):
            for i in range(15):
                b_s[(15 * k + i) * TH // 2:(15 * k + i + 1) * TH // 2, :] = _pk(b[i])

        def pre_phase():
            first = [[x_cp(0, 0)], [wq_cp(0)], [x_cp(1, 2), wq_cp(1)],
                     [wq_cp(2), pltpu.make_async_copy(wo_hbm, wo_v, sem_i.at[3])]]
            order = sum(first, [])
            for p in range(NP + 1):
                order += group_cp(p)
            xr_cp = [x_cp(b, SEM_P + NP + 1) for b in range(2, NB)]
            order += xr_cp
            for cp in order:
                cp.start()
            get = lambda an, name: [an[min(i, len(an) - 1)] for i in cfg[name]]
            e_grp = lambda e: ((e >> 1) & 1, ((e >> 2) << 1) | (e & 1))
            if 'a' in cfg['sub']:
                pre_a(first, get, e_grp)
            if 'b' in cfg['sub']:
                pre_b(get, e_grp)
            if 'c' in cfg['sub']:
                pre_c(get)
            wait('WX', xr_cp)

        def pre_a(first, get, e_grp):
            def transpose_wq(i):
                wt_s[WQ[i] // 2:WQ[i + 1] // 2, :D] = _pk(wqkv_v[:, WQ[i]:WQ[i + 1]].T)

            def clear(i, carry):
                for k in range(2):
                    acc_s[k, i] = jnp.zeros((D3, TH), F32)
                r = jnp.minimum(i, 11) * (RP // 4)
                qkv_s[0, rows8(r, RP // 4)] = jnp.zeros((RP // 4, LANES), U32)
                return carry

            lax.fori_loop(0, 15, clear, 0)
            wait('WX0', first[0])
            xn0 = ln1(0, ()).astype(BF16)

            wait('WQ0', first[1])
            transpose_wq(0)
            qkv_mm(0, xn0, (0, 1), [])

            wait('WQ1', first[2])
            transpose_wq(1)
            an = []
            qkv_mm(0, xn0, (2, 3), an)
            xn1 = ln1(1, get(an, 'a_ln'), get(an, 'a_lnb')).astype(BF16)
            qkv_mm(1, xn1, (0,), an, True)
            for n, a in enumerate(get(an, 'a_w1')):
                prep_att(n, a)
            nk = len(cfg['a_k'])
            apply = [att_values(0, *e_grp(e), a, 9) for e, a in enumerate(get(an, 'a_k'))]

            wait('WQ2', first[3])
            an = []
            qkv_mm(1, xn1, (2,), an)
            transpose_wq(2)
            qkv_mm(0, xn0, (4, 5), an)
            qkv_mm(1, xn1, (4, 1), an)
            apply += [att_values(0, *e_grp(nk + e), a, 9)
                      for e, a in enumerate(get(an, 'a_k2')[:8 - nk])]
            for e, a in enumerate(get(an, 'a_v')):
                apply[e](a)
            wo = pltpu.bitcast(wo_v[...], U32)
            wo = cat0(_lo(wo), _hi(wo))
            wo = cat0(*[_tie(wo[n * LANES:(n + 1) * LANES], a)
                        for n, a in enumerate(get(an, 'a_wo'))])
            wt_s[3 * RP:, :D] = _pk(wo.astype(BF16).T)
            stats = wo_mm(0, an, False)
            qkv_mm(1, xn1, (3,), an)
            for n, a in enumerate(get(an, 'a_w2')):
                prep_att(12 + n, a)
            plain_lhs(0, stats)
            n1 = len(cfg['a_att'])
            for e, a in enumerate(get(an, 'a_att')):
                att_group(1, *e_grp(e), a, 9)

            wait('WO', group_cp(0))
            an = []
            b = plain_piece(0, an)
            qkv_mm(1, xn1, (5,), an, True)
            prep_gu(0, get(an, 'z_g'))
            ffn_lhs(0, stats, get(an, 'z_l'))
            for e, a in enumerate(get(an, 'z_att')[:3 - n1]):
                att_group(1, *e_grp(n1 + e), a, 9)
            store_b(b)

        def pre_b(get, e_grp):
            def piece(p, carry):
                wait('WP', group_cp(p))
                b_prev = load_b()
                an = []
                if cfg['fast0']:
                    acc = down_mm(load_acc(0), [b_prev], p - 1, an, D_ORDER[:6], True)
                    t, hv, done = {}, {}, set()
                    for step in cfg['order1']:
                        k = int(step[1])
                        part = k if step[0] == 'S' else 3
                        slabs = [int(step[2])] if len(step) > 2 else list(range(NS))
                        if part not in done:
                            prep_gu_part(p, part, get(an, 'f_g%d' % part))
                            done.add(part)
                        if step[0] == 'S':
                            for i in _PARTS[k]:
                                gu_prod(p, i, t, an, slabs)
                        else:
                            gu_col(t, hv, p, k, an, slabs)
                    b = h_join(hv)
                    prep_d(p - 1, get(an, 'p_d'))
                    store_acc(0, down_mm(acc, [b_prev], p - 1, an, D_ORDER[6:]))
                else:
                    b = plain_piece(p, an)
                    prep_d(p - 1, get(an, 'p_d'))
                    store_acc(0, down_mm(load_acc(0), [b_prev], p - 1, an))
                    prep_gu(p, get(an, 'p_g'))
                att_group(1, *e_grp(p + 2), an[cfg['p_att'][0]], 9)
                for i, a in enumerate(get(an, 'p_w')):
                    prep_att(jnp.minimum(24 + (p - 1) * 5 + i, 47), a)
                store_b(b)
                return carry

            lax.fori_loop(1, NP, piece, 0)

        def pre_c(get):
            wait('WD', group_cp(NP))
            an = []
            stats = wo_mm(1, an, True)
            prep_d(NP - 1, get(an, 't_d'))
            acc = down_mm(load_acc(0), [load_b()], NP - 1, [])
            ffn_lhs(1, stats, [])
            finish(0, acc)

        if 'pre' in cfg['phases']:
            pre_phase()

        def body(u, carry):
            bu = u & (NB - 1)
            ba = (u + 1) & (NB - 1)
            acc, stats, an, b = None, None, {}, {}
            get = lambda name: [an[k][i] for k, i in cfg[name]]
            for step in cfg['body']:
                an[step] = []
                if step == 'Q':
                    qkv_fast(ba, att_rhs(ln1(ba, get('ln1'), get('ln1b')), u >> 8 if 'q' in cfg['stash'] else None),
                             an[step])
                elif step == 'W':
                    attention(ba, get('att'), cfg['win'])
                    stats = wo_mm(ba, an[step], True, get('orhs'),
                                  u >> 8 if 'w' in cfg['stash'] else None)
                elif step == 'L':
                    ffn_lhs(ba, stats, get('lhs'))
                elif step[0] == 'S':
                    slabs = [int(step[3])] if len(step) > 3 else list(range(NS))
                    for i in _PARTS[int(step[2])]:
                        gu_prod(int(step[1]), i, b.setdefault(step[:2], {}), an[step], slabs)
                elif step[0] == 'F':
                    j, c = int(step[1]), int(step[2])
                    slabs = [int(step[3])] if len(step) > 3 else list(range(NS))
                    hv = b.setdefault(step[:2], {})
                    gu_col(b['S' + step[1]], hv, j, c, an[step], slabs)
                    if len(hv) == 3 * NS:
                        b[j] = h_join(hv)
                        if 'b' in cfg['stash']:
                            store_b(b[j], j)
                            b[j] = load_b(j)
                else:
                    js = [int(c) for c in step[1:]]
                    acc = down_mm(acc, [b[j] for j in js], js[0], an[step])
            finish(bu, acc)

            @pl.when(u >= NB)
            def _():
                out_copy(bu).start()
            return carry

        if scopes:
            with jax.named_scope('LOOP'):
                lax.fori_loop(1, NU - 1, body, 0)
        elif 'main' in cfg['phases']:
            lax.fori_loop(1, NU - 1, body, 0)

        LP = cfg['lp']

        def last(c, carry):
            b = [gu_piece(LP * c + j, cfg['order'], [], j) for j in range(LP)]
            acc = down_mm(load_acc(1), b[:-1], LP * c, [])
            acc = down_mm(acc, b[-1:], LP * c + LP - 1, [])
            store_acc(1, acc)
            if cfg['lfin']:
                finish(NB - 1, acc)
            return carry

        if 'last' in cfg['phases']:
            lax.fori_loop(0, NP // LP, last, 0)
        if len(cfg['phases']) < 3:
            def keep(i, c):
                v = (gs_s[i, i, :8, :LANES] + us_s[i, i, :8, :LANES] + ds_s[i, i, :8, :LANES]
                     + wl_s[rows8(i * 8), :LANES] + a_s[i, :8] + qkv_s[i, :8]
                     + b_s[rows8(i * 8), :LANES] + wt_s[rows8(i * 8), :LANES])
                acc_s[1, 0, :8] = (lax.bitcast_convert_type(v, F32) + o_s[i, :8]
                                   + acc_s[i, i, :8])
                return c
            lax.fori_loop(0, 2, keep, 0)
        if not cfg['lfin']:
            finish(NB - 1, load_acc(1))
        out_copy(NB - 1).start()
        wait('WOUT', [out_copy(b) for b in range(NB)])

    scratch = [
        pltpu.VMEM((NB, D, TM), BF16),
        pltpu.VMEM((D, 3 * D), BF16),
        pltpu.VMEM((D, D), BF16),
        pltpu.VMEM((NP, 3, D, PW), BF16),
        pltpu.VMEM((NP, 3, D, PW), BF16),
        pltpu.VMEM((NP, 3, D, PW), BF16),
        pltpu.VMEM((2 * D, 8 * LANES), U32),
        pltpu.VMEM((4 * Q3, 16 * LANES), U32),
        pltpu.VMEM((NP, 15, Q3, PW), U32),
        pltpu.VMEM((NP, 15, Q3, PW), U32),
        pltpu.VMEM((NP, 9, Q3, PW), U32),
        pltpu.VMEM((NB, D, TM), F32),
        pltpu.VMEM((54, TH // 2, LANES), U32),
        pltpu.VMEM((S // LANES + 1, 3 * RP, LANES), U32),
        pltpu.VMEM((NT, D, LANES), F32),
        pltpu.VMEM((2, 15, D3, TH), F32),
        pltpu.VMEM((NP * 15 * TH // 2, PW), U32),
        pltpu.VMEM((1, 9 * 64, 2 * LANES), U32),
        pltpu.VMEM((NP, 2, 9, TH, PW), F32),
        pltpu.SemaphoreType.DMA((SEM_P + NP + 2,)),
        pltpu.SemaphoreType.DMA((1,)),
    ]

    def wrapped(*refs):
        @pl.when(pl.program_id(0) == 0)
        def _():
            kernel(*refs)

    return wrapped, scratch


_CFG = dict(
    scopes=False,
    lp=3,
    lfin=True,
    fast0=True,
    psplit=1,
    rcp=False,
    late=True,
    stash='qw',
    slab=True,
    fslab=False,
    win=9,
    sub='abc',
    orhs=(),
    msplit=2,
    phases=('pre', 'main', 'last'),
    order=('S0', 'S1', 'F0', 'S2', 'F1', 'F2'),
    body=('S010', 'S000', 'F000', 'S020', 'F010', 'F020', 'S001', 'S011', 'F001',
        'S110', 'S021', 'F021', 'S100', 'F100', 'S120', 'S101', 'F110', 'F011', 'Q',
        'F120', 'S111', 'F101', 'S121', 'F111', 'F121', 'S200', 'S210', 'F200', 'S220',
        'F210', 'F220', 'S300', 'S201', 'S211', 'F201', 'S320', 'S221', 'F211', 'F221',
        'S310', 'D01', 'F300', 'S301', 'S311', 'F301', 'S321', 'F311', 'F321', 'S400',
        'F310', 'F320', 'S420', 'F410', 'S410', 'S401', 'F420', 'S411', 'F400', 'S421',
        'F411', 'F421', 'S500', 'F401', 'S501', 'S510', 'D23', 'F500', 'S520', 'W',
        'F520', 'S511', 'F510', 'S521', 'F501', 'F511', 'F521', 'D4', 'D5', 'L'),
    ln1=(('S010', 4), ('S010', 5), ('S010', 6), ('S010', 7), ('S010', 8), ('S000', 0),
        ('S000', 1), ('S000', 2), ('S000', 3)),
    ln1b=(('S110', 2), ('S110', 3), ('S110', 5), ('S110', 6), ('S110', 8), ('S021', 0),
        ('S021', 2), ('S021', 3), ('S021', 5), ('S021', 6), ('S021', 8), ('F021', 0)),
    att=(('S300', 8), ('D01', 1), ('D01', 7), ('D01', 8), ('D01', 10), ('F300', 4),
        ('D23', 5), ('D23', 9)),
    lhs=(('D4', 3), ('D5', 1), ('D5', 4)),
    att0=(15, 18, 21, 24, 27, 30, 33, 37),
    order0=('S0', 'S1', 'S2', 'F0', 'F1', 'F2'),
    order1=('S0', 'S1', 'S2', 'F0', 'F1', 'F2'),
    a_w1=(0, 0, 1, 2, 2, 3, 3, 4, 4, 5, 6, 7),
    a_w2=(20, 23, 26, 30, 33, 36, 40, 43, 46, 50, 53, 57),
    a_ln=(0, 3, 6),
    a_lnb=(5, 9, 9),
    z_g=(5, 6, 7, 8, 11, 11, 12, 13, 14, 15, 17, 18, 19, 20, 21, 22, 23, 24, 25, 26, 28,
        29, 30, 31, 32, 35, 36, 37, 38, 40, 41, 42, 43, 45, 46, 47, 48, 49, 50, 51, 52,
        54, 55, 57, 58, 59, 60, 62),
    z_att=(53, 54, 56),
    p_g0=(0, 1, 2, 3, 4, 5),
    p_g1=(6, 7, 8, 9, 10, 10),
    p_g2=(12, 13, 14, 15, 16, 17),
    p_g3=(14, 16, 18, 20, 22, 24, 26, 28, 30, 32, 34, 36),
    t_d=(0, 0, 1, 1, 2, 3, 3, 4, 5, 6, 6, 7, 8, 9, 9, 9, 10, 11, 11, 12, 13, 14, 15,
        16),
    p_d=(26, 26, 27, 27, 29, 29, 29, 30, 31, 31, 32, 33, 33, 34, 35, 35, 36, 36, 37, 37,
        38, 39, 39, 41),
    p_att=(59,),
    p_w=(12, 60, 62, 65, 65),
    p_g=(0, 1, 2, 3, 4, 5, 6, 7, 9, 10, 11, 12, 13, 14, 15, 16, 18, 19, 20, 21, 22, 23,
        24, 25, 27, 28, 29, 30, 31, 32, 33, 34, 36, 37, 38, 39, 40, 41, 42, 43, 45, 46,
        47, 48, 49, 50, 51, 53),
    z_l=(2, 13, 32),
    f_g0=(0, 0, 0, 1, 1, 2, 2, 3, 4, 4, 4, 5),
    f_g1=(4, 6, 7, 7, 8, 10, 10, 11, 11, 12, 13, 14),
    f_g2=(5, 10, 11, 11, 13, 15, 16, 17, 19, 20, 21, 22),
    f_g3=(6, 7, 14, 16, 17, 18, 19, 19, 21, 22, 23, 23, 24, 25, 27, 28, 29, 30, 31, 33,
        34, 36, 36, 37),
    a_k=(15, 19, 20, 24),
    a_k2=(0, 4, 8, 12),
    a_v=(13, 14, 22, 26, 30, 34, 38, 39),
    a_att=(12, 60),
    a_wo=(30, 35, 36, 38, 41),
)


def _run(A_x, A_wqkv, A_wo, B_w_gate, B_w_up, B_w_down, **kw):
    _, S, D = A_x.shape
    F = B_w_gate.shape[1]
    kernel, scratch = _make_kernel(S, D, F, 256, {**_CFG, **kw})
    hbm = pl.BlockSpec(memory_space=pl.ANY)
    out_t = pl.pallas_call(
        kernel,
        grid=(2,),
        in_specs=[hbm] * 6,
        out_specs=hbm,
        out_shape=jax.ShapeDtypeStruct((D, S), A_x.dtype),
        scratch_shapes=scratch,
        compiler_params=pltpu.CompilerParams(
            dimension_semantics=('arbitrary',), vmem_limit_bytes=110 * 1024 * 1024),
    )(A_x.reshape(S, D).T, A_wqkv, A_wo, B_w_gate, B_w_up, B_w_down.T)
    return out_t.T.reshape(A_x.shape)


@jax.jit
def pallas_interleave_layers__sliding_local_dilated__glu_gated_geglu__prompt_kernel(
    A_x: jax.Array,
    A_wqkv: jax.Array,
    A_wo: jax.Array,
    B_x: jax.Array,
    B_w_gate: jax.Array,
    B_w_up: jax.Array,
    B_w_down: jax.Array,
):
    del B_x
    return _run(A_x, A_wqkv, A_wo, B_w_gate, B_w_up, B_w_down)
```

```python
import jax
import jax.numpy as jnp
import jax.experimental.pallas as pl
import jax.experimental.pallas.tpu as pltpu
from jax import lax

H = 32
W = 8
DIL = 2
EPS = 1e-5
LANES = 128

F32 = jnp.float32
BF16 = jnp.bfloat16
U32 = jnp.uint32

_NT = (((1,), (1,)), ((), ()))


def _tree_sum(parts, op=jnp.add):
    while len(parts) > 1:
        nxt = [op(parts[i], parts[i + 1]) for i in range(0, len(parts) - 1, 2)]
        if len(parts) % 2:
            nxt.append(parts[-1])
        parts = nxt
    return parts[0]


def _ln_stats(slabs, d, anchors=()):
    n_acc = 4
    s1, s2, pilot = [None] * n_acc, [None] * n_acc, None
    for i, x in enumerate(slabs):
        if pilot is None:
            pilot = x[0:1, :]
            pil = jnp.broadcast_to(pilot, x.shape)
            pils = [_tie(pil, a) for a in anchors] or [pil]
        dx = x - pils[i * len(pils) // (d // 8)]
        j = i % n_acc
        s1[j] = dx if s1[j] is None else s1[j] + dx
        s2[j] = dx * dx if s2[j] is None else s2[j] + dx * dx
    e1 = jnp.sum(_tree_sum(s1), axis=0, keepdims=True) * (1.0 / d)
    e2 = jnp.sum(_tree_sum(s2), axis=0, keepdims=True) * (1.0 / d)
    var = jnp.maximum(e2 - e1 * e1, 0.0)
    return pilot + e1, lax.rsqrt(var + EPS)


def _zero_like_dep(v):
    return (lax.bitcast_convert_type(v, U32) >> 31) >> 1


def _tie(x, anchor):
    if anchor is None:
        return x
    z = lax.bitcast_convert_type(_zero_like_dep(anchor), F32)
    z = jnp.concatenate([z] * -(-x.shape[1] // LANES), axis=1)[:, :x.shape[1]]
    if x.shape[0] == 8:
        return x + z
    return jnp.concatenate([x[:8] + z, x[8:]], axis=0)


def _gelu_mul2(g, u):
    c0 = 0.7978845608028654
    c1 = c0 * 0.044715
    t = jnp.tanh(g * (c0 + c1 * (g * g)))
    return (g * u) * (1.0 + t)


def _lo(x):
    return lax.bitcast_convert_type(x << 16, F32)


def _hi(x):
    return lax.bitcast_convert_type(x & jnp.uint32(0xFFFF0000), F32)


def _pk(x):
    return pltpu.bitcast(x.astype(BF16), U32)


def _upk(x):
    return pltpu.bitcast(x, BF16)


def _dot(a, b):
    return jnp.dot(a, b, preferred_element_type=F32)


def _dot_nt(a, b):
    return lax.dot_general(a, b, _NT, preferred_element_type=F32)


def _x_ops(x1, x2):
    d = [a - b for a, b in zip(x1, x2)]
    return [x1[0] + x2[1], x2[0] + x2[1], x1[0] + x1[1],
            d[1] + x1[2], x1[1] + x1[2], d[1] + d[2],
            d[0] - x2[2], d[0] + d[2], x2[0] + x2[2],
            x1[0], d[0], x2[1], d[1], x1[2], x2[2]]


def _x_rem(x1, x2):
    a, b, c = 0, 1, 2
    cat = lambda u, v: jnp.concatenate([u, v], axis=0)
    return [cat(x1[c], x2[b]), cat(x1[a], x1[b] - x2[b]), cat(x2[a], x2[c] - x1[c])]


_W_TERMS = {0: ((0, 1, 1), (1, 0, 1)), 3: ((1, 2, 1), (2, 1, 1)), 6: ((0, 2, 1), (2, 0, 1)),
            9: ((0, 0, 1), (0, 2, 1), (1, 0, -1)), 10: ((2, 0, 1), (0, 0, -1), (0, 1, -1)),
            11: ((1, 1, 1), (1, 2, 1), (0, 1, -1)), 12: ((1, 0, 1), (1, 1, 1), (2, 1, -1)),
            13: ((2, 0, 1), (2, 2, 1), (1, 2, -1)), 14: ((2, 1, 1), (2, 2, 1), (0, 2, -1)),
            1: ((0, 1, 1),), 2: ((1, 0, 1),), 4: ((1, 2, 1),), 5: ((2, 1, 1),),
            7: ((2, 0, 1),), 8: ((0, 2, 1),)}


def _w_op(i, w):
    v = None
    for k, j, sg in _W_TERMS[i]:
        v = w(k, j) if v is None else (v + w(k, j) if sg > 0 else v - w(k, j))
    return v


def _w_sums(w):
    return [_w_op(i, lambda k, j: w[k][j]) for i in _W_SUM]


_PARTS = ((1, 2, 0), (7, 8, 6), (4, 5, 3), (9, 10, 11, 12, 13, 14))
_W_SUM = {0: 0, 3: 1, 6: 2, 9: 3, 10: 4, 11: 5, 12: 6, 13: 7, 14: 8}
_W_RAW = {1: (0, 1), 2: (1, 0), 4: (1, 2), 5: (2, 1), 7: (2, 0), 8: (0, 2)}
_PAIR_ORDER = (1, 2, 4, 5, 7, 8, 0, 3, 6)
_DIAG = {(0, 0): 9, (2, 0): 10, (0, 1): 11, (1, 1): 12, (1, 2): 13, (2, 2): 14}
_PAIR = {(0, 0): ((6, -1), (8, -1)), (1, 0): ((2, 1), (7, 1)), (2, 0): ((0, 1), (1, -1)),
         (0, 1): ((3, 1), (4, -1)), (1, 1): ((0, 1), (2, -1)), (2, 1): ((1, 1), (5, -1)),
         (0, 2): ((4, 1), (8, 1)), (1, 2): ((6, 1), (7, -1)), (2, 2): ((5, 1), (3, -1))}


def _column(t, base, j):
    s = []
    for k in range(3):
        v = base[k]
        for i, sg in _PAIR[k, j]:
            v = t[i] if v is None else (v + t[i] if sg > 0 else v - t[i])
        s.append(v)
    return s[1] + s[0], s[2] + s[0]


def _make_kernel(S, D, F, TM, cfg):
    NB = S // TM
    NT = TM // LANES
    DH = D // H
    DP = DH // 2
    RP = D // 2
    NG = H // 8
    scale = float(DH) ** -0.5
    NU = 2 * NB
    TH = TM // 2
    FT = F // 3
    D2 = D // 2
    D3 = D // 3
    Q3 = D3 // 2
    KU = D // 9
    KR = 3 * LANES
    NQ = 6
    QR = 3 * D // NQ
    WQ = (0, 640, 1152, 3 * D)
    PW = 256
    NP = FT // PW
    scopes = cfg['scopes']
    assert NG == 4 and NB & (NB - 1) == 0
    SEM_P = 4

    def kernel(x_hbm, wqkv_hbm, wo_hbm, wg_hbm, wu_hbm, wdt_hbm, out_hbm,
               xio_s, wqkv_v, wo_v, wg_v, wu_v, wdt_v, wt_s, wl_s,
               gs_s, us_s, ds_s, xmid_s, a_s, qkv_s, o_s, acc_s, b_s, r_s,
               sem_i, sem_o):

        def wait(name, cps):
            if scopes:
                with jax.named_scope(name):
                    for cp in cps:
                        cp.wait()
            else:
                for cp in cps:
                    cp.wait()

        def cols(lo, n):
            if not isinstance(lo, int):
                lo = pl.multiple_of(lo, LANES)
            return pl.ds(lo, n)

        def rows8(lo, n=8):
            if not isinstance(lo, int):
                lo = pl.multiple_of(lo, 8)
            return pl.ds(lo, n)

        def out_copy(b):
            return pltpu.make_async_copy(
                xio_s.at[b], out_hbm.at[:, cols(b * TM, TM)], sem_o.at[0])

        def x_cp(b, sem):
            return pltpu.make_async_copy(x_hbm.at[:, cols(b * TM, TM)], xio_s.at[b],
                                         sem_i.at[sem])

        def wq_cp(i):
            sl = cols(WQ[i], WQ[i + 1] - WQ[i])
            return pltpu.make_async_copy(wqkv_hbm.at[:, sl], wqkv_v.at[:, sl],
                                         sem_i.at[1 + i])

        def piece_cp(src, dst, p, sem):
            return [pltpu.make_async_copy(src.at[:, cols(j * FT + p * PW, PW)],
                                          dst.at[p, j],
                                          sem_i.at[sem]) for j in range(3)]

        def group_cp(p):
            sem = SEM_P + p
            cps = []
            if not (isinstance(p, int) and p == NP):
                cps += piece_cp(wg_hbm, wg_v, p, sem) + piece_cp(wu_hbm, wu_v, p, sem)
            if not (isinstance(p, int) and p == 0):
                cps += piece_cp(wdt_hbm, wdt_v, p - 1, sem)
            return cps

        lane = lax.broadcasted_iota(jnp.int32, (8, LANES), 1)
        cat0 = lambda *v: jnp.concatenate(v, axis=0)
        cat1 = lambda *v: jnp.concatenate(v, axis=1)

        def spread_over(anchors, n, total):
            return anchors[n * len(anchors) // total] if anchors else None

        def slab_group(r):
            return (r % LANES) // 16 if r < KR else 8 + ((r - KR) % KU) // 16

        def ln1(blk, anchors1, anchors2=()):
            slabs = (xio_s[blk, r:r + 8, :].astype(F32) for r in range(0, D, 8))
            m, rs = _ln_stats(slabs, D, anchors1)
            if not anchors2:
                return (xio_s[blk].astype(F32) - m) * rs
            m8 = jnp.broadcast_to(m, (8, TM))
            ms = [_tie(m8, a) for a in anchors2]
            ms = [spread_over(ms, slab_group(r), 12) for r in range(0, D, 8)]
            return (xio_s[blk].astype(F32) - cat0(*ms)) * rs

        def dot_k(rows, x, anchors, even=False):
            y = None
            for n, k in enumerate(range(0, D, LANES)):
                ks = slice(k, min(k + LANES, D))
                if even and k + LANES >= D:
                    mid = (rows.start + rows.stop) // 2
                    v = cat0(_dot(_upk(wt_s[rows.start:mid, ks]), x[ks]),
                             _dot(_upk(wt_s[mid:rows.stop, ks]), x[ks]))
                else:
                    v = _dot(_upk(wt_s[rows, ks]), x[ks])
                anchors.extend(v[r:r + 8, :LANES] for r in ((0, 144) if n % 2 else (72, 216)))
                y = v if y is None else y + v
            return y

        def put_qkv(blk, rows, y):
            pk = _pk(y)
            for c in range(NT):
                qkv_s[1 + blk * NT + c, rows, :] = pk[:, c * LANES:(c + 1) * LANES]

        def qkv_mm(blk, xn, chunks, anchors, even=False):
            for r in chunks:
                rows = slice(r * QR // 2, (r + 1) * QR // 2)
                put_qkv(blk, rows, dot_k(rows, xn, anchors, even))

        def split_k(x):
            hs = (x[:, :TH], x[:, TH:])
            blocks = [[h[k * LANES:(k + 1) * LANES] for k in range(3)] for h in hs]
            units = [[h[KR + k * KU:KR + (k + 1) * KU] for k in range(3)] for h in hs]
            return blocks, units

        def prep_att(pat, anchor):
            assert Q3 == 96
            row0 = pat * 8
            src0 = row0 + ((pat * 43) >> 9) * (2 * Q3)
            w = [_upk(wt_s[rows8(src0 + j * Q3), :D]).astype(F32) for j in range(3)]
            w[0] = cat1(_tie(w[0][:, :LANES], anchor), w[0][:, LANES:])
            tiles = _w_sums([[w[j][:, k * LANES:(k + 1) * LANES] for j in range(3)]
                             for k in range(3)])
            for j in range(3):
                a, b, c = (w[j][:, KR + k * KU:KR + (k + 1) * KU] for k in range(3))
                tiles += [cat1(c, b), cat1(a, c)]
            wl_s[rows8(row0), :15 * LANES] = _pk(cat1(*tiles))

        def att_rhs(x, stash=None):
            blocks, units = split_k(x)
            ops = _x_ops(*blocks) + _x_rem(*units)
            if stash is None:
                return [v.astype(BF16) for v in ops]
            loc = lambda i, r0, n: (slice((i // 2) * 64 + r0, (i // 2) * 64 + r0 + n),
                                    slice((i % 2) * LANES, (i % 2 + 1) * LANES))
            for r in range(0, LANES, 16):
                for i, v in enumerate(ops):
                    r_s.at[0][loc(i, r // 2, 8)] = _pk(v[r:r + 16])
            return [_upk(r_s.at[stash][loc(i, 0, 64)]) for i in range(18)]

        def att_mm(sec, rhs, anchors):
            tl = lambda i: _upk(wl_s[sec * Q3:(sec + 1) * Q3, i * LANES:(i + 1) * LANES])
            raw = lambda k, j: _upk(wt_s[(3 * sec + j) * Q3:(3 * sec + j + 1) * Q3,
                                         k * LANES:(k + 1) * LANES])
            t = {}
            for i in _PAIR_ORDER:
                t[i] = _dot(raw(*_W_RAW[i]) if i in _W_RAW else tl(_W_SUM[i]), rhs[i])
                anchors.append(t[i][:8])
            out = []
            for j in range(3):
                base = []
                for s in range(3):
                    v = _dot(raw(3, j) if s == 1 else tl(9 + 2 * j + s // 2), rhs[15 + s])
                    if (s, j) in _DIAG:
                        i = _DIAG[s, j]
                        v = _dot(tl(_W_SUM[i]), rhs[i]) + v
                    base.append(v)
                    anchors.append(base[-1][:8])
                out.append(cat1(*_column(t, base, j)))
            return cat0(*out)

        def qkv_fast(blk, rhs, anchors):
            for sec in range(3):
                put_qkv(blk, slice(sec * RP, (sec + 1) * RP), att_mm(sec, rhs, anchors))

        def shifted(ln, cur, prev, w):
            if w == 0:
                return cur
            sh = DIL * w
            return pltpu.roll(jnp.where(ln < LANES - sh, cur, prev), sh, axis=1)

        def att_group(blk, c, hg, anchor):
            att_values(blk, c, hg, anchor)(None)

        def att_values(blk, c, hg, anchor):
            tile = blk * NT + c
            base = hg * 8 * DP
            if isinstance(hg, int):
                cur, prev, o_t = qkv_s.at[1 + tile], qkv_s.at[tile], o_s.at[c]
            else:
                n = 2 * RP + 8 * DP
                base = pl.multiple_of(base, 8)
                cur = qkv_s.at[1 + tile, pl.ds(base, n)]
                prev = qkv_s.at[tile, pl.ds(base, n)]
                o_t = o_s.at[c, pl.ds(base, RP + 8 * DP)]
                base = 0
            ln = lane + _zero_like_dep(anchor).astype(jnp.int32)
            logits = [None] * W
            for dd in range(DP):
                q = cur[pl.ds(base + dd, 8, stride=DP), :]
                kc = cur[pl.ds(RP + base + dd, 8, stride=DP), :]
                kp = prev[pl.ds(RP + base + dd, 8, stride=DP), :]
                q0, q1 = _lo(q), _hi(q)
                for w in range(W):
                    ks = shifted(ln, kc, kp, w)
                    t = q0 * _lo(ks) + q1 * _hi(ks)
                    logits[w] = t if logits[w] is None else logits[w] + t
            logits = [l * scale for l in logits]
            if not (isinstance(c, int) and c > 0):
                pos = lane + tile * LANES
                logits = [l if w == 0 else jnp.where(pos >= DIL * w, l, -1e9)
                          for w, l in enumerate(logits)]
            m = _tree_sum(logits, jnp.maximum)
            p = [jnp.exp(l - m) for l in logits]
            r = 1.0 / _tree_sum(p)

            def apply(anchor2):
                ln = lane + _zero_like_dep(m if anchor2 is None else anchor2).astype(jnp.int32)
                for dd in range(DP):
                    vc = cur[pl.ds(2 * RP + base + dd, 8, stride=DP), :]
                    vp = prev[pl.ds(2 * RP + base + dd, 8, stride=DP), :]
                    o0 = o1 = None
                    for w in range(W):
                        vs = shifted(ln, vc, vp, w)
                        t0, t1 = p[w] * _lo(vs), p[w] * _hi(vs)
                        o0 = t0 if o0 is None else o0 + t0
                        o1 = t1 if o1 is None else o1 + t1
                    o0, o1 = o0 * r, o1 * r
                    o_t[pl.ds(base + dd, 8, stride=DP), :] = o0
                    o_t[pl.ds(RP + base + dd, 8, stride=DP), :] = o1

            return apply

        def attention(blk, anchors):
            for c in range(NT):
                for hg in range(NG):
                    att_group(blk, c, hg, anchors[c * NG + hg])

        def wo_mm(blk, anchors, fast, stash=None):
            o = cat1(*[o_s[c] for c in range(NT)])
            if fast:
                y = att_mm(3, att_rhs(o, stash), anchors)
            else:
                o = o.astype(BF16)
                q = D2 // 2
                y = cat0(*[dot_k(slice(h * q, (h + 1) * q), o, anchors) for h in (6, 7)])
            xm = xio_s[blk].astype(F32) + y
            xmid_s[blk] = xm
            return _ln_stats((xm[r:r + 8] for r in range(0, D, 8)), D)

        def ffn_lhs(blk, stats, anchors):
            m, rs = stats
            m8 = jnp.broadcast_to(m, (8, TM))
            xs = []
            for k in range(3):
                mt = cat0(*[_tie(m8, spread_over(anchors, k, 3))] * (D3 // 8))
                xs.append((xmid_s[blk, k * D3:(k + 1) * D3, :] - mt) * rs)
            ops = _x_ops([x[:, :TH] for x in xs], [x[:, TH:] for x in xs])
            for i, v in enumerate(ops):
                for s, t in enumerate((v[KU:], v[:2 * KU], cat0(v[:KU], v[2 * KU:]))):
                    a_s[3 * i + s] = _pk(t.astype(BF16).T)

        def plain_lhs(blk, stats):
            m, rs = stats
            blocks, units = split_k((xmid_s[blk] - m) * rs)
            for i, v in enumerate(blocks[0] + blocks[1] + _x_rem(*units)):
                a_s[45 + i] = _pk(v.astype(BF16).T)

        def plain_piece(p, anchors):
            h = {}
            for j in range(3):
                hs = []
                for n in range(PW // LANES):
                    cs = slice(n * LANES, (n + 1) * LANES)
                    w = lambda r0, r1: cat1(wg_v[p, j, r0:r1, cs], wu_v[p, j, r0:r1, cs])
                    u = lambda k: w(KR + k * KU, KR + (k + 1) * KU)
                    tl = lambda *i: _upk(cat1(*[a_s[45 + k] for k in i]))
                    y0 = _dot(tl(6), cat0(u(2), u(1)))
                    y1 = _dot(tl(0, 1, 2, 7), w(0, KR + 2 * KU))
                    y2 = _dot(tl(3, 4, 5, 8), cat0(w(0, KR + KU), u(2)))
                    anchors.append(y0[:8, :LANES])
                    for y in (y1, y2):
                        anchors.extend(y[r:r + 8, c:c + LANES] for c in (0, LANES)
                                       for r in (0, TH // 2))
                    hs.append([_gelu_mul2(*[(y + y0)[:, c:c + LANES] for c in (0, LANES)])
                               for y in (y1, y2)])
                h[j] = [cat1(*[v[i] for v in hs]) for i in range(2)]
            return h_ops(h)

        def prep_d(p, anchors):
            PR = 16
            for n in range(2 * D3 // PR):
                r, cs = (n // 2) * PR, slice((n % 2) * LANES, (n % 2 + 1) * LANES)
                w = [[wdt_v[p, k, j * D3 + r:j * D3 + r + PR, cs].astype(F32)
                      for j in range(3)] for k in range(3)]
                w[0][1] = _tie(w[0][1], spread_over(anchors, n, 2 * D3 // PR))
                for i, v in enumerate(_w_sums(w)):
                    ds_s.at[p, i][r // 2:(r + PR) // 2, cs] = _pk(v)

        GU = ((wg_v, gs_s), (wu_v, us_s))

        def prep_gu(p, anchors):
            PR = 16
            nr = D3 // PR
            for n in range(4 * nr):
                c, (w_v, s_s), r = n % 2, GU[(n // 2) % 2], (n // 4) * PR
                cache = {}

                def w(k, j):
                    if (k, j) not in cache:
                        ld = lambda c: w_v[p, j, k * D3 + r:k * D3 + r + PR,
                                           c * LANES:(c + 1) * LANES].astype(F32)
                        v = ld(c)
                        if k != j:
                            v = _tie(v, spread_over(anchors, n, 4 * nr))
                        cache[k, j] = v - ld(1 - c) if r // KU == 1 + c else v
                    return cache[k, j]

                for i in range(15):
                    s_s.at[p, i][r // 2:(r + PR) // 2,
                                 c * LANES:(c + 1) * LANES] = _pk(_w_op(i, w))

        def prep_gu_part(p, part, anchors):
            PR = 16
            nr = D3 // PR
            ids = _PARTS[part]
            for n in range(2 * nr):
                (w_v, s_s), r = GU[n % 2], (n // 2) * PR
                unit = r // KU
                if part < 3:
                    cache = {}

                    def w(k, j):
                        if (k, j) not in cache:
                            v = w_v[p, j, k * D3 + r:k * D3 + r + PR, :].astype(F32)
                            v = _tie(v, spread_over(anchors, n, 2 * nr))
                            l, h = v[:, :LANES], v[:, LANES:]
                            cache[k, j] = (v, cat1(l - h, h), cat1(l, h - l))[unit]
                        return cache[k, j]

                    for i in ids:
                        s_s.at[p, i][r // 2:(r + PR) // 2, :] = _pk(_w_op(i, w))
                    continue
                prev = None
                for m, c in enumerate((1, 0) if unit == 1 else (0, 1)):
                    cache = {}

                    def w(k, j):
                        if (k, j) not in cache:
                            v = w_v[p, j, k * D3 + r:k * D3 + r + PR,
                                    c * LANES:(c + 1) * LANES].astype(F32)
                            if k == j:
                                v = _tie(v, spread_over(anchors, 2 * n + m, 4 * nr))
                            cache[k, j] = v
                        return cache[k, j]

                    sums = [_w_op(i, w) for i in ids]
                    for q, i in enumerate(ids):
                        v = sums[q] - prev[q] if m and unit else sums[q]
                        s_s.at[p, i][r // 2:(r + PR) // 2, c * LANES:(c + 1) * LANES] = _pk(v)
                    prev = sums

        NS = 2

        def gu_prod(p, i, t, anchors, slabs):
            u = KU // 2

            def rhs(s, s_s):
                if s == 1:
                    return s_s[p, i, :2 * u, :LANES]
                if s == 0:
                    return cat0(s_s[p, i, u:2 * u, LANES:], s_s[p, i, 2 * u:, :LANES])
                return cat0(s_s[p, i, :u, LANES:], s_s[p, i, 2 * u:, LANES:])

            q = TH // 2 // NS
            for n, h in enumerate(slabs):
                y = []
                for s in range(3):
                    r = _upk(cat1(rhs(s, gs_s), rhs(s, us_s)))
                    y.append(_dot(_upk(a_s[3 * i + s, h * q:(h + 1) * q]), r))
                    if (3 * n + s) % len(slabs) == 0:
                        anchors.append(y[-1][:8, :LANES])
                y1, y2 = y[1] + y[0], y[2] + y[0]
                for m in range(2):
                    cs = slice(m * LANES, (m + 1) * LANES)
                    t.setdefault((m, h), {})[i] = cat1(y1[:, cs], y2[:, cs])

        def gu_col(t, hv, p, j, anchors, slabs):
            ids = [_DIAG.get((s, j)) for s in range(3)]
            for i in ids:
                if i is not None:
                    gu_prod(p, i, t, anchors, slabs)
            for h in slabs:
                g, u = [_column(t[m, h], [None if i is None else t[m, h][i] for i in ids], j)
                        for m in range(2)]
                hv[j, h] = [_gelu_mul2(g[i], u[i]) for i in range(2)]

        def h_ops(h):
            return [v.astype(BF16) for v in _x_ops(*[[h[j][i] for j in range(3)]
                                                     for i in range(2)])]

        def h_join(hv):
            return h_ops({j: [cat0(*[hv[j, h][i] for h in range(NS)]) for i in range(2)]
                          for j in range(3)})

        def gu_piece(p):
            t, hv = {}, {}
            for h in range(NS):
                for step in ('S0', 'S1', 'F0', 'S2', 'F1', 'F2'):
                    if step[0] == 'S':
                        for i in _PARTS[int(step[1])]:
                            gu_prod(p, i, t, [], [h])
                    else:
                        gu_col(t, hv, p, int(step[1]), [], [h])
            return h_join(hv)

        D_ORDER = _PAIR_ORDER + (9, 10, 11, 12, 13, 14)

        def down_mm(acc, bs, lo, anchors, which=D_ORDER, fine=False):
            p = [None] * 15 if acc is None else list(acc)
            for i in which:
                y = None
                for n, b in enumerate(bs):
                    if i in _W_RAW:
                        k, j = _W_RAW[i]
                        v = _dot_nt(wdt_v[lo + n, k, j * D3:(j + 1) * D3, :], b[i])
                    elif len(bs) % 2 and i == 14 and n == 0:
                        v = cat0(*[_dot_nt(_upk(ds_s[lo, _W_SUM[i],
                                                     h * Q3 // 2:(h + 1) * Q3 // 2, :]), b[i])
                                   for h in range(2)])
                    else:
                        v = _dot_nt(_upk(ds_s[lo + n, _W_SUM[i]]), b[i])
                    y = v if y is None else y + v
                p[i] = y if p[i] is None else p[i] + y
                anchors.append(p[i][:8])
                if fine:
                    anchors.append(p[i][D3 // 2:D3 // 2 + 8])
            return p

        def finish(blk, acc):
            y = [cat1(*_column(acc, [acc[_DIAG[s, j]] if (s, j) in _DIAG else None
                                     for s in range(3)], j)) for j in range(3)]
            xio_s[blk] = (xmid_s[blk] + 0.5 * cat0(*y)).astype(BF16)

        def load_acc(k):
            return [acc_s[k, i] for i in range(15)]

        def store_acc(k, acc):
            for i in range(15):
                acc_s[k, i] = acc[i]

        def load_b():
            return [_upk(b_s[i * TH // 2:(i + 1) * TH // 2, :]) for i in range(15)]

        def store_b(b):
            for i in range(15):
                b_s[i * TH // 2:(i + 1) * TH // 2, :] = _pk(b[i])

        def pre_phase():
            first = [[x_cp(0, 0)], [wq_cp(0)], [x_cp(1, 2), wq_cp(1)],
                     [wq_cp(2), pltpu.make_async_copy(wo_hbm, wo_v, sem_i.at[3])]]
            order = sum(first, [])
            for p in range(NP + 1):
                order += group_cp(p)
            xr_cp = [x_cp(b, SEM_P + NP + 1) for b in range(2, NB)]
            order += xr_cp
            for cp in order:
                cp.start()
            get = lambda an, name: [an[min(i, len(an) - 1)] for i in cfg[name]]
            e_grp = lambda e: ((e >> 1) & 1, ((e >> 2) << 1) | (e & 1))
            if 'a' in cfg['sub']:
                pre_a(first, get, e_grp)
            if 'b' in cfg['sub']:
                pre_b(get, e_grp)
            if 'c' in cfg['sub']:
                pre_c(get)
            wait('WX', xr_cp)

        def pre_a(first, get, e_grp):
            def transpose_wq(i):
                wt_s[WQ[i] // 2:WQ[i + 1] // 2, :D] = _pk(wqkv_v[:, WQ[i]:WQ[i + 1]].T)

            def clear(i, carry):
                for k in range(2):
                    acc_s[k, i] = jnp.zeros((D3, TH), F32)
                r = jnp.minimum(i, 11) * (RP // 4)
                qkv_s[0, rows8(r, RP // 4)] = jnp.zeros((RP // 4, LANES), U32)
                return carry

            lax.fori_loop(0, 15, clear, 0)
            wait('WX0', first[0])
            xn0 = ln1(0, ()).astype(BF16)

            wait('WQ0', first[1])
            transpose_wq(0)
            qkv_mm(0, xn0, (0, 1), [])

            wait('WQ1', first[2])
            transpose_wq(1)
            an = []
            qkv_mm(0, xn0, (2, 3), an)
            xn1 = ln1(1, get(an, 'a_ln'), get(an, 'a_lnb')).astype(BF16)
            qkv_mm(1, xn1, (0,), an, True)
            for n, a in enumerate(get(an, 'a_w1')):
                prep_att(n, a)
            nk = len(cfg['a_k'])
            apply = [att_values(0, *e_grp(e), a) for e, a in enumerate(get(an, 'a_k'))]

            wait('WQ2', first[3])
            an = []
            qkv_mm(1, xn1, (2,), an)
            transpose_wq(2)
            qkv_mm(0, xn0, (4, 5), an)
            qkv_mm(1, xn1, (4, 1), an)
            apply += [att_values(0, *e_grp(nk + e), a)
                      for e, a in enumerate(get(an, 'a_k2')[:8 - nk])]
            for e, a in enumerate(get(an, 'a_v')):
                apply[e](a)
            wo = pltpu.bitcast(wo_v[...], U32)
            wo = cat0(_lo(wo), _hi(wo))
            wo = cat0(*[_tie(wo[n * LANES:(n + 1) * LANES], a)
                        for n, a in enumerate(get(an, 'a_wo'))])
            wt_s[3 * RP:, :D] = _pk(wo.astype(BF16).T)
            stats = wo_mm(0, an, False)
            qkv_mm(1, xn1, (3,), an)
            for n, a in enumerate(get(an, 'a_w2')):
                prep_att(12 + n, a)
            plain_lhs(0, stats)
            n1 = len(cfg['a_att'])
            for e, a in enumerate(get(an, 'a_att')):
                att_group(1, *e_grp(e), a)

            wait('WO', group_cp(0))
            an = []
            b = plain_piece(0, an)
            qkv_mm(1, xn1, (5,), an, True)
            prep_gu(0, get(an, 'z_g'))
            ffn_lhs(0, stats, get(an, 'z_l'))
            for e, a in enumerate(get(an, 'z_att')[:3 - n1]):
                att_group(1, *e_grp(n1 + e), a)
            store_b(b)

        def pre_b(get, e_grp):
            def piece(p, carry):
                wait('WP', group_cp(p))
                b_prev = load_b()
                an = []
                acc = down_mm(load_acc(0), [b_prev], p - 1, an, D_ORDER[:6], True)
                t, hv, slabs = {}, {}, list(range(NS))
                for part in range(4):
                    prep_gu_part(p, part, get(an, 'f_g%d' % part))
                    for k in range(3):
                        if part < 3:
                            gu_prod(p, _PARTS[part][k], t, an, slabs)
                        else:
                            gu_col(t, hv, p, k, an, slabs)
                b = h_join(hv)
                prep_d(p - 1, get(an, 'p_d'))
                store_acc(0, down_mm(acc, [b_prev], p - 1, an, D_ORDER[6:]))
                att_group(1, *e_grp(p + 2), an[cfg['p_att'][0]])
                for i, a in enumerate(get(an, 'p_w')):
                    prep_att(jnp.minimum(24 + (p - 1) * 5 + i, 47), a)
                store_b(b)
                return carry

            lax.fori_loop(1, NP, piece, 0)

        def pre_c(get):
            wait('WD', group_cp(NP))
            an = []
            stats = wo_mm(1, an, True)
            prep_d(NP - 1, get(an, 't_d'))
            acc = down_mm(load_acc(0), [load_b()], NP - 1, [])
            ffn_lhs(1, stats, [])
            finish(0, acc)

        if 'pre' in cfg['phases']:
            pre_phase()

        def body(u, carry):
            bu = u & (NB - 1)
            ba = (u + 1) & (NB - 1)
            acc, stats, an, b = None, None, {}, {}
            get = lambda name: [an[k][i] for k, i in cfg[name]]
            for step in cfg['body']:
                an[step] = []
                if step == 'Q':
                    xn = ln1(ba, get('ln1'), get('ln1b'))
                    qkv_fast(ba, att_rhs(xn, u >> 8), an[step])
                elif step == 'W':
                    attention(ba, get('att'))
                    stats = wo_mm(ba, an[step], True, u >> 8)
                elif step == 'L':
                    ffn_lhs(ba, stats, get('lhs'))
                elif step[0] == 'S':
                    slabs = [int(step[3])]
                    for i in _PARTS[int(step[2])]:
                        gu_prod(int(step[1]), i, b.setdefault(step[:2], {}), an[step], slabs)
                elif step[0] == 'F':
                    j, c = int(step[1]), int(step[2])
                    slabs = [int(step[3])]
                    hv = b.setdefault(step[:2], {})
                    gu_col(b['S' + step[1]], hv, j, c, an[step], slabs)
                    if len(hv) == 3 * NS:
                        b[j] = h_join(hv)
                else:
                    js = [int(c) for c in step[1:]]
                    acc = down_mm(acc, [b[j] for j in js], js[0], an[step])
            finish(bu, acc)

            @pl.when(u >= NB)
            def _():
                out_copy(bu).start()
            return carry

        if scopes:
            with jax.named_scope('LOOP'):
                lax.fori_loop(1, NU - 1, body, 0)
        elif 'main' in cfg['phases']:
            lax.fori_loop(1, NU - 1, body, 0)

        LP = 3

        def last(c, carry):
            b = [gu_piece(LP * c + j) for j in range(LP)]
            acc = down_mm(load_acc(1), b[:-1], LP * c, [])
            acc = down_mm(acc, b[-1:], LP * c + LP - 1, [])
            store_acc(1, acc)
            finish(NB - 1, acc)
            return carry

        if 'last' in cfg['phases']:
            lax.fori_loop(0, NP // LP, last, 0)
        if len(cfg['phases']) < 3:
            def keep(i, c):
                v = (gs_s[i, i, :8, :LANES] + us_s[i, i, :8, :LANES] + ds_s[i, i, :8, :LANES]
                     + wl_s[rows8(i * 8), :LANES] + a_s[i, :8] + qkv_s[i, :8]
                     + b_s[rows8(i * 8), :LANES] + wt_s[rows8(i * 8), :LANES])
                acc_s[1, 0, :8] = (lax.bitcast_convert_type(v, F32) + o_s[i, :8]
                                   + acc_s[i, i, :8])
                return c
            lax.fori_loop(0, 2, keep, 0)
            finish(NB - 1, load_acc(1))
        out_copy(NB - 1).start()
        wait('WOUT', [out_copy(b) for b in range(NB)])

    scratch = [
        pltpu.VMEM((NB, D, TM), BF16),
        pltpu.VMEM((D, 3 * D), BF16),
        pltpu.VMEM((D, D), BF16),
        pltpu.VMEM((NP, 3, D, PW), BF16),
        pltpu.VMEM((NP, 3, D, PW), BF16),
        pltpu.VMEM((NP, 3, D, PW), BF16),
        pltpu.VMEM((2 * D, 8 * LANES), U32),
        pltpu.VMEM((4 * Q3, 16 * LANES), U32),
        pltpu.VMEM((NP, 15, Q3, PW), U32),
        pltpu.VMEM((NP, 15, Q3, PW), U32),
        pltpu.VMEM((NP, 9, Q3, PW), U32),
        pltpu.VMEM((NB, D, TM), F32),
        pltpu.VMEM((54, TH // 2, LANES), U32),
        pltpu.VMEM((S // LANES + 1, 3 * RP, LANES), U32),
        pltpu.VMEM((NT, D, LANES), F32),
        pltpu.VMEM((2, 15, D3, TH), F32),
        pltpu.VMEM((15 * TH // 2, PW), U32),
        pltpu.VMEM((1, 9 * 64, 2 * LANES), U32),
        pltpu.SemaphoreType.DMA((SEM_P + NP + 2,)),
        pltpu.SemaphoreType.DMA((1,)),
    ]

    def wrapped(*refs):
        @pl.when(pl.program_id(0) == 0)
        def _():
            kernel(*refs)

    return wrapped, scratch


_CFG = dict(
    scopes=False,
    sub='abc',
    phases=('pre', 'main', 'last'),
    body=('S010', 'S000', 'F000', 'S020', 'F010', 'F020', 'S001', 'S011', 'F001',
        'S110', 'S021', 'F021', 'S100', 'F100', 'S120', 'S101', 'F110', 'F011', 'Q',
        'F120', 'S111', 'F101', 'S121', 'F111', 'F121', 'S200', 'S210', 'F200', 'S220',
        'F210', 'F220', 'S300', 'S201', 'S211', 'F201', 'S320', 'S221', 'F211', 'F221',
        'S310', 'D01', 'F300', 'S301', 'S311', 'F301', 'S321', 'F311', 'F321', 'S400',
        'F310', 'F320', 'S420', 'F410', 'S410', 'S401', 'F420', 'S411', 'F400', 'S421',
        'F411', 'F421', 'S500', 'F401', 'S501', 'S510', 'D23', 'F500', 'S520', 'W',
        'F520', 'S511', 'F510', 'S521', 'F501', 'F511', 'F521', 'D4', 'D5', 'L'),
    ln1=(('S010', 4), ('S010', 5), ('S010', 6), ('S010', 7), ('S010', 8), ('S000', 0),
        ('S000', 1), ('S000', 2), ('S000', 3)),
    ln1b=(('S110', 2), ('S110', 3), ('S110', 5), ('S110', 6), ('S110', 8), ('S021', 0),
        ('S021', 2), ('S021', 3), ('S021', 5), ('S021', 6), ('S021', 8), ('F021', 0)),
    att=(('S300', 8), ('D01', 1), ('D01', 7), ('D01', 8), ('D01', 10), ('F300', 4),
        ('D23', 5), ('D23', 9)),
    lhs=(('D4', 3), ('D5', 1), ('D5', 4)),
    a_w1=(0, 0, 1, 2, 2, 3, 3, 4, 4, 5, 6, 7),
    a_w2=(20, 23, 26, 30, 33, 36, 40, 43, 46, 50, 53, 57),
    a_ln=(0, 3, 6),
    a_lnb=(5, 9, 9),
    z_g=(5, 6, 7, 8, 11, 11, 12, 13, 14, 15, 17, 18, 19, 20, 21, 22, 23, 24, 25, 26, 28,
        29, 30, 31, 32, 35, 36, 37, 38, 40, 41, 42, 43, 45, 46, 47, 48, 49, 50, 51, 52,
        54, 55, 57, 58, 59, 60, 62),
    z_att=(53, 54, 56),
    t_d=(0, 0, 1, 1, 2, 3, 3, 4, 5, 6, 6, 7, 8, 9, 9, 9, 10, 11, 11, 12, 13, 14, 15,
        16),
    p_d=(26, 26, 27, 27, 29, 29, 29, 30, 31, 31, 32, 33, 33, 34, 35, 35, 36, 36, 37, 37,
        38, 39, 39, 41),
    p_att=(59,),
    p_w=(12, 60, 62, 65, 65),
    z_l=(2, 13, 32),
    f_g0=(0, 0, 0, 1, 1, 2, 2, 3, 4, 4, 4, 5),
    f_g1=(4, 6, 7, 7, 8, 10, 10, 11, 11, 12, 13, 14),
    f_g2=(5, 10, 11, 11, 13, 15, 16, 17, 19, 20, 21, 22),
    f_g3=(6, 7, 14, 16, 17, 18, 19, 19, 21, 22, 23, 23, 24, 25, 27, 28, 29, 30, 31, 33,
        34, 36, 36, 37),
    a_k=(15, 19, 20, 24),
    a_k2=(0, 4, 8, 12),
    a_v=(13, 14, 22, 26, 30, 34, 38, 39),
    a_att=(12, 60),
    a_wo=(30, 35, 36, 38, 41),
)


def _run(A_x, A_wqkv, A_wo, B_w_gate, B_w_up, B_w_down, **kw):
    _, S, D = A_x.shape
    F = B_w_gate.shape[1]
    kernel, scratch = _make_kernel(S, D, F, 256, {**_CFG, **kw})
    hbm = pl.BlockSpec(memory_space=pl.ANY)
    out_t = pl.pallas_call(
        kernel,
        grid=(2,),
        in_specs=[hbm] * 6,
        out_specs=hbm,
        out_shape=jax.ShapeDtypeStruct((D, S), A_x.dtype),
        scratch_shapes=scratch,
        compiler_params=pltpu.CompilerParams(
            dimension_semantics=('arbitrary',), vmem_limit_bytes=110 * 1024 * 1024),
    )(A_x.reshape(S, D).T, A_wqkv, A_wo, B_w_gate, B_w_up, B_w_down.T)
    return out_t.T.reshape(A_x.shape)


@jax.jit
def pallas_interleave_layers__sliding_local_dilated__glu_gated_geglu__prompt_kernel(
    A_x: jax.Array,
    A_wqkv: jax.Array,
    A_wo: jax.Array,
    B_x: jax.Array,
    B_w_gate: jax.Array,
    B_w_up: jax.Array,
    B_w_down: jax.Array,
):
    del B_x
    return _run(A_x, A_wqkv, A_wo, B_w_gate, B_w_up, B_w_down)
```

```python
import jax
import jax.numpy as jnp
import jax.experimental.pallas as pl
import jax.experimental.pallas.tpu as pltpu
from jax import lax

H = 32
W = 8
DIL = 2
EPS = 1e-5
LANES = 128

F32 = jnp.float32
BF16 = jnp.bfloat16
U32 = jnp.uint32

_NT = (((1,), (1,)), ((), ()))


def _tree_sum(parts, op=jnp.add):
    while len(parts) > 1:
        nxt = [op(parts[i], parts[i + 1]) for i in range(0, len(parts) - 1, 2)]
        if len(parts) % 2:
            nxt.append(parts[-1])
        parts = nxt
    return parts[0]


def _ln_stats(slabs, d, anchors=()):
    n_acc = 4
    s1, s2, pilot = [None] * n_acc, [None] * n_acc, None
    for i, x in enumerate(slabs):
        if pilot is None:
            pilot = x[0:1, :]
            pil = jnp.broadcast_to(pilot, x.shape)
            pils = [_tie(pil, a) for a in anchors] or [pil]
        dx = x - pils[i * len(pils) // (d // 8)]
        j = i % n_acc
        s1[j] = dx if s1[j] is None else s1[j] + dx
        s2[j] = dx * dx if s2[j] is None else s2[j] + dx * dx
    e1 = jnp.sum(_tree_sum(s1), axis=0, keepdims=True) * (1.0 / d)
    e2 = jnp.sum(_tree_sum(s2), axis=0, keepdims=True) * (1.0 / d)
    var = jnp.maximum(e2 - e1 * e1, 0.0)
    return pilot + e1, lax.rsqrt(var + EPS)


def _zero_like_dep(v):
    return (lax.bitcast_convert_type(v, U32) >> 31) >> 1


def _tie(x, anchor):
    if anchor is None:
        return x
    z = lax.bitcast_convert_type(_zero_like_dep(anchor), F32)
    z = jnp.concatenate([z] * -(-x.shape[1] // LANES), axis=1)[:, :x.shape[1]]
    if x.shape[0] == 8:
        return x + z
    return jnp.concatenate([x[:8] + z, x[8:]], axis=0)


def _gelu_mul2(g, u):
    c0 = 0.7978845608028654
    c1 = c0 * 0.044715
    t = jnp.tanh(g * (c0 + c1 * (g * g)))
    return (g * u) * (1.0 + t)


def _lo(x):
    return lax.bitcast_convert_type(x << 16, F32)


def _hi(x):
    return lax.bitcast_convert_type(x & jnp.uint32(0xFFFF0000), F32)


def _pk(x):
    return pltpu.bitcast(x.astype(BF16), U32)


def _upk(x):
    return pltpu.bitcast(x, BF16)


def _dot(a, b):
    return jnp.dot(a, b, preferred_element_type=F32)


def _dot_nt(a, b):
    return lax.dot_general(a, b, _NT, preferred_element_type=F32)


def _x_ops(x1, x2):
    d = [a - b for a, b in zip(x1, x2)]
    return [x1[0] + x2[1], x2[0] + x2[1], x1[0] + x1[1],
            d[1] + x1[2], x1[1] + x1[2], d[1] + d[2],
            d[0] - x2[2], d[0] + d[2], x2[0] + x2[2],
            x1[0], d[0], x2[1], d[1], x1[2], x2[2]]


def _x_rem(x1, x2):
    a, b, c = 0, 1, 2
    cat = lambda u, v: jnp.concatenate([u, v], axis=0)
    return [cat(x1[c], x2[b]), cat(x1[a], x1[b] - x2[b]), cat(x2[a], x2[c] - x1[c])]


_W_TERMS = {0: ((0, 1, 1), (1, 0, 1)), 3: ((1, 2, 1), (2, 1, 1)), 6: ((0, 2, 1), (2, 0, 1)),
            9: ((0, 0, 1), (0, 2, 1), (1, 0, -1)), 10: ((2, 0, 1), (0, 0, -1), (0, 1, -1)),
            11: ((1, 1, 1), (1, 2, 1), (0, 1, -1)), 12: ((1, 0, 1), (1, 1, 1), (2, 1, -1)),
            13: ((2, 0, 1), (2, 2, 1), (1, 2, -1)), 14: ((2, 1, 1), (2, 2, 1), (0, 2, -1)),
            1: ((0, 1, 1),), 2: ((1, 0, 1),), 4: ((1, 2, 1),), 5: ((2, 1, 1),),
            7: ((2, 0, 1),), 8: ((0, 2, 1),)}


def _w_op(i, w):
    v = None
    for k, j, sg in _W_TERMS[i]:
        v = w(k, j) if v is None else (v + w(k, j) if sg > 0 else v - w(k, j))
    return v


def _w_sums(w):
    return [_w_op(i, lambda k, j: w[k][j]) for i in _W_SUM]


_PARTS = ((1, 2, 0), (7, 8, 6), (4, 5, 3), (9, 10, 11, 12, 13, 14))
_W_SUM = {0: 0, 3: 1, 6: 2, 9: 3, 10: 4, 11: 5, 12: 6, 13: 7, 14: 8}
_W_RAW = {1: (0, 1), 2: (1, 0), 4: (1, 2), 5: (2, 1), 7: (2, 0), 8: (0, 2)}
_PAIR_ORDER = (1, 2, 4, 5, 7, 8, 0, 3, 6)
_DIAG = {(0, 0): 9, (2, 0): 10, (0, 1): 11, (1, 1): 12, (1, 2): 13, (2, 2): 14}
_PAIR = {(0, 0): ((6, -1), (8, -1)), (1, 0): ((2, 1), (7, 1)), (2, 0): ((0, 1), (1, -1)),
         (0, 1): ((3, 1), (4, -1)), (1, 1): ((0, 1), (2, -1)), (2, 1): ((1, 1), (5, -1)),
         (0, 2): ((4, 1), (8, 1)), (1, 2): ((6, 1), (7, -1)), (2, 2): ((5, 1), (3, -1))}


def _column(t, base, j):
    s = []
    for k in range(3):
        v = base[k]
        for i, sg in _PAIR[k, j]:
            v = t[i] if v is None else (v + t[i] if sg > 0 else v - t[i])
        s.append(v)
    return s[1] + s[0], s[2] + s[0]


def _make_kernel(S, D, F, TM, cfg):
    NB = S // TM
    NT = TM // LANES
    DH = D // H
    DP = DH // 2
    RP = D // 2
    NG = H // 8
    scale = float(DH) ** -0.5
    NU = 2 * NB
    TH = TM // 2
    FT = F // 3
    D2 = D // 2
    D3 = D // 3
    Q3 = D3 // 2
    KU = D // 9
    KR = 3 * LANES
    NQ = 6
    QR = 3 * D // NQ
    WQ = (0, 640, 1152, 3 * D)
    PW = 256
    NP = FT // PW
    scopes = cfg['scopes']
    assert NG == 4 and NB & (NB - 1) == 0
    SEM_P = 4

    def kernel(x_hbm, wqkv_hbm, wo_hbm, wg_hbm, wu_hbm, wdt_hbm, out_hbm,
               xio_s, wqkv_v, wo_v, wg_v, wu_v, wdt_v, wt_s, wl_s,
               gs_s, us_s, ds_s, xmid_s, a_s, qkv_s, o_s, acc_s, b_s, r_s,
               sem_i, sem_o):

        def wait(name, cps):
            if scopes:
                with jax.named_scope(name):
                    for cp in cps:
                        cp.wait()
            else:
                for cp in cps:
                    cp.wait()

        def cols(lo, n):
            if not isinstance(lo, int):
                lo = pl.multiple_of(lo, LANES)
            return pl.ds(lo, n)

        def rows8(lo, n=8):
            if not isinstance(lo, int):
                lo = pl.multiple_of(lo, 8)
            return pl.ds(lo, n)

        def out_copy(b):
            return pltpu.make_async_copy(
                xio_s.at[b], out_hbm.at[:, cols(b * TM, TM)], sem_o.at[0])

        def x_cp(b, sem):
            return pltpu.make_async_copy(x_hbm.at[:, cols(b * TM, TM)], xio_s.at[b],
                                         sem_i.at[sem])

        def wq_cp(i):
            sl = cols(WQ[i], WQ[i + 1] - WQ[i])
            return pltpu.make_async_copy(wqkv_hbm.at[:, sl], wqkv_v.at[:, sl],
                                         sem_i.at[1 + i])

        def piece_cp(src, dst, p, sem):
            return [pltpu.make_async_copy(src.at[:, cols(j * FT + p * PW, PW)],
                                          dst.at[p, j],
                                          sem_i.at[sem]) for j in range(3)]

        def group_cp(p):
            sem = SEM_P + p
            cps = []
            if not (isinstance(p, int) and p == NP):
                cps += piece_cp(wg_hbm, wg_v, p, sem) + piece_cp(wu_hbm, wu_v, p, sem)
            if not (isinstance(p, int) and p == 0):
                cps += piece_cp(wdt_hbm, wdt_v, p - 1, sem)
            return cps

        lane = lax.broadcasted_iota(jnp.int32, (8, LANES), 1)
        cat0 = lambda *v: jnp.concatenate(v, axis=0)
        cat1 = lambda *v: jnp.concatenate(v, axis=1)

        def spread_over(anchors, n, total):
            return anchors[n * len(anchors) // total] if anchors else None

        def slab_group(r):
            return (r % LANES) // 16 if r < KR else 8 + ((r - KR) % KU) // 16

        def ln1(blk, anchors1, anchors2=()):
            slabs = (xio_s[blk, r:r + 8, :].astype(F32) for r in range(0, D, 8))
            m, rs = _ln_stats(slabs, D, anchors1)
            if not anchors2:
                return (xio_s[blk].astype(F32) - m) * rs
            m8 = jnp.broadcast_to(m, (8, TM))
            ms = [_tie(m8, a) for a in anchors2]
            ms = [spread_over(ms, slab_group(r), 12) for r in range(0, D, 8)]
            return (xio_s[blk].astype(F32) - cat0(*ms)) * rs

        def dot_k(rows, x, anchors, even=False):
            y = None
            for n, k in enumerate(range(0, D, LANES)):
                ks = slice(k, min(k + LANES, D))
                if even and k + LANES >= D:
                    mid = (rows.start + rows.stop) // 2
                    v = cat0(_dot(_upk(wt_s[rows.start:mid, ks]), x[ks]),
                             _dot(_upk(wt_s[mid:rows.stop, ks]), x[ks]))
                else:
                    v = _dot(_upk(wt_s[rows, ks]), x[ks])
                anchors.extend(v[r:r + 8, :LANES] for r in ((0, 144) if n % 2 else (72, 216)))
                y = v if y is None else y + v
            return y

        def put_qkv(blk, rows, y):
            pk = _pk(y)
            for c in range(NT):
                qkv_s[1 + blk * NT + c, rows, :] = pk[:, c * LANES:(c + 1) * LANES]

        def qkv_mm(blk, xn, chunks, anchors, even=False):
            for r in chunks:
                rows = slice(r * QR // 2, (r + 1) * QR // 2)
                put_qkv(blk, rows, dot_k(rows, xn, anchors, even))

        def split_k(x):
            hs = (x[:, :TH], x[:, TH:])
            blocks = [[h[k * LANES:(k + 1) * LANES] for k in range(3)] for h in hs]
            units = [[h[KR + k * KU:KR + (k + 1) * KU] for k in range(3)] for h in hs]
            return blocks, units

        def prep_att(pat, anchor):
            assert Q3 == 96
            row0 = pat * 8
            src0 = row0 + ((pat * 43) >> 9) * (2 * Q3)
            w = [_upk(wt_s[rows8(src0 + j * Q3), :D]).astype(F32) for j in range(3)]
            w[0] = cat1(_tie(w[0][:, :LANES], anchor), w[0][:, LANES:])
            tiles = _w_sums([[w[j][:, k * LANES:(k + 1) * LANES] for j in range(3)]
                             for k in range(3)])
            for j in range(3):
                a, b, c = (w[j][:, KR + k * KU:KR + (k + 1) * KU] for k in range(3))
                tiles += [cat1(c, b), cat1(a, c)]
            wl_s[rows8(row0), :15 * LANES] = _pk(cat1(*tiles))

        def att_rhs(x, stash=None):
            blocks, units = split_k(x)
            ops = _x_ops(*blocks) + _x_rem(*units)
            if stash is None:
                return [v.astype(BF16) for v in ops]
            loc = lambda i, r0, n: (slice((i // 2) * 64 + r0, (i // 2) * 64 + r0 + n),
                                    slice((i % 2) * LANES, (i % 2 + 1) * LANES))
            for r in range(0, LANES, 16):
                for i, v in enumerate(ops):
                    r_s.at[0][loc(i, r // 2, 8)] = _pk(v[r:r + 16])
            return [_upk(r_s.at[stash][loc(i, 0, 64)]) for i in range(18)]

        def att_mm(sec, rhs, anchors):
            tl = lambda i: _upk(wl_s[sec * Q3:(sec + 1) * Q3, i * LANES:(i + 1) * LANES])
            raw = lambda k, j: _upk(wt_s[(3 * sec + j) * Q3:(3 * sec + j + 1) * Q3,
                                         k * LANES:(k + 1) * LANES])
            t = {}
            for i in _PAIR_ORDER:
                t[i] = _dot(raw(*_W_RAW[i]) if i in _W_RAW else tl(_W_SUM[i]), rhs[i])
                anchors.append(t[i][:8])
            out = []
            for j in range(3):
                base = []
                for s in range(3):
                    v = _dot(raw(3, j) if s == 1 else tl(9 + 2 * j + s // 2), rhs[15 + s])
                    if (s, j) in _DIAG:
                        i = _DIAG[s, j]
                        v = _dot(tl(_W_SUM[i]), rhs[i]) + v
                    base.append(v)
                    anchors.append(base[-1][:8])
                out.append(cat1(*_column(t, base, j)))
            return cat0(*out)

        def qkv_fast(blk, rhs, anchors):
            for sec in range(3):
                put_qkv(blk, slice(sec * RP, (sec + 1) * RP), att_mm(sec, rhs, anchors))

        def shifted(ln, cur, prev, w):
            if w == 0:
                return cur
            sh = DIL * w
            return pltpu.roll(jnp.where(ln < LANES - sh, cur, prev), sh, axis=1)

        def att_group(blk, c, hg, anchor):
            att_values(blk, c, hg, anchor)(None)

        def att_values(blk, c, hg, anchor):
            tile = blk * NT + c
            base = hg * 8 * DP
            if isinstance(hg, int):
                cur, prev, o_t = qkv_s.at[1 + tile], qkv_s.at[tile], o_s.at[c]
            else:
                n = 2 * RP + 8 * DP
                base = pl.multiple_of(base, 8)
                cur = qkv_s.at[1 + tile, pl.ds(base, n)]
                prev = qkv_s.at[tile, pl.ds(base, n)]
                o_t = o_s.at[c, pl.ds(base, RP + 8 * DP)]
                base = 0
            ln = lane + _zero_like_dep(anchor).astype(jnp.int32)
            logits = [None] * W
            for dd in range(DP):
                q = cur[pl.ds(base + dd, 8, stride=DP), :]
                kc = cur[pl.ds(RP + base + dd, 8, stride=DP), :]
                kp = prev[pl.ds(RP + base + dd, 8, stride=DP), :]
                q0, q1 = _lo(q), _hi(q)
                for w in range(W):
                    ks = shifted(ln, kc, kp, w)
                    t = q0 * _lo(ks) + q1 * _hi(ks)
                    logits[w] = t if logits[w] is None else logits[w] + t
            logits = [l * scale for l in logits]
            if not (isinstance(c, int) and c > 0):
                pos = lane + tile * LANES
                logits = [l if w == 0 else jnp.where(pos >= DIL * w, l, -1e9)
                          for w, l in enumerate(logits)]
            m = _tree_sum(logits, jnp.maximum)
            p = [jnp.exp(l - m) for l in logits]
            r = 1.0 / _tree_sum(p)

            def apply(anchor2):
                ln = lane + _zero_like_dep(m if anchor2 is None else anchor2).astype(jnp.int32)
                for dd in range(DP):
                    vc = cur[pl.ds(2 * RP + base + dd, 8, stride=DP), :]
                    vp = prev[pl.ds(2 * RP + base + dd, 8, stride=DP), :]
                    o0 = o1 = None
                    for w in range(W):
                        vs = shifted(ln, vc, vp, w)
                        t0, t1 = p[w] * _lo(vs), p[w] * _hi(vs)
                        o0 = t0 if o0 is None else o0 + t0
                        o1 = t1 if o1 is None else o1 + t1
                    o0, o1 = o0 * r, o1 * r
                    o_t[pl.ds(base + dd, 8, stride=DP), :] = o0
                    o_t[pl.ds(RP + base + dd, 8, stride=DP), :] = o1

            return apply

        def attention(blk, anchors):
            for c in range(NT):
                for hg in range(NG):
                    att_group(blk, c, hg, anchors[c * NG + hg])

        def wo_mm(blk, anchors, fast, stash=None):
            o = cat1(*[o_s[c] for c in range(NT)])
            if fast:
                y = att_mm(3, att_rhs(o, stash), anchors)
            else:
                o = o.astype(BF16)
                q = D2 // 2
                y = cat0(*[dot_k(slice(h * q, (h + 1) * q), o, anchors) for h in (6, 7)])
            xm = xio_s[blk].astype(F32) + y
            xmid_s[blk] = xm
            return _ln_stats((xm[r:r + 8] for r in range(0, D, 8)), D)

        def ffn_lhs(blk, stats, anchors):
            m, rs = stats
            m8 = jnp.broadcast_to(m, (8, TM))
            xs = []
            for k in range(3):
                mt = cat0(*[_tie(m8, spread_over(anchors, k, 3))] * (D3 // 8))
                xs.append((xmid_s[blk, k * D3:(k + 1) * D3, :] - mt) * rs)
            ops = _x_ops([x[:, :TH] for x in xs], [x[:, TH:] for x in xs])
            for i, v in enumerate(ops):
                for s, t in enumerate((v[KU:], v[:2 * KU], cat0(v[:KU], v[2 * KU:]))):
                    a_s[3 * i + s] = _pk(t.astype(BF16).T)

        def plain_lhs(blk, stats):
            m, rs = stats
            blocks, units = split_k((xmid_s[blk] - m) * rs)
            for i, v in enumerate(blocks[0] + blocks[1] + _x_rem(*units)):
                a_s[45 + i] = _pk(v.astype(BF16).T)

        def plain_piece(p, anchors):
            h = {}
            for j in range(3):
                hs = []
                for n in range(PW // LANES):
                    cs = slice(n * LANES, (n + 1) * LANES)
                    w = lambda r0, r1: cat1(wg_v[p, j, r0:r1, cs], wu_v[p, j, r0:r1, cs])
                    u = lambda k: w(KR + k * KU, KR + (k + 1) * KU)
                    tl = lambda *i: _upk(cat1(*[a_s[45 + k] for k in i]))
                    y0 = _dot(tl(6), cat0(u(2), u(1)))
                    y1 = _dot(tl(0, 1, 2, 7), w(0, KR + 2 * KU))
                    y2 = _dot(tl(3, 4, 5, 8), cat0(w(0, KR + KU), u(2)))
                    anchors.append(y0[:8, :LANES])
                    for y in (y1, y2):
                        anchors.extend(y[r:r + 8, c:c + LANES] for c in (0, LANES)
                                       for r in (0, TH // 2))
                    hs.append([_gelu_mul2(*[(y + y0)[:, c:c + LANES] for c in (0, LANES)])
                               for y in (y1, y2)])
                h[j] = [cat1(*[v[i] for v in hs]) for i in range(2)]
            return h_ops(h)

        def prep_d(p, anchors):
            PR = 16
            for n in range(2 * D3 // PR):
                r, cs = (n // 2) * PR, slice((n % 2) * LANES, (n % 2 + 1) * LANES)
                w = [[wdt_v[p, k, j * D3 + r:j * D3 + r + PR, cs].astype(F32)
                      for j in range(3)] for k in range(3)]
                w[0][1] = _tie(w[0][1], spread_over(anchors, n, 2 * D3 // PR))
                for i, v in enumerate(_w_sums(w)):
                    ds_s.at[p, i][r // 2:(r + PR) // 2, cs] = _pk(v)

        GU = ((wg_v, gs_s), (wu_v, us_s))

        def prep_gu(p, anchors):
            PR = 16
            nr = D3 // PR
            for n in range(4 * nr):
                c, (w_v, s_s), r = n % 2, GU[(n // 2) % 2], (n // 4) * PR
                cache = {}

                def w(k, j):
                    if (k, j) not in cache:
                        ld = lambda c: w_v[p, j, k * D3 + r:k * D3 + r + PR,
                                           c * LANES:(c + 1) * LANES].astype(F32)
                        v = ld(c)
                        if k != j:
                            v = _tie(v, spread_over(anchors, n, 4 * nr))
                        cache[k, j] = v - ld(1 - c) if r // KU == 1 + c else v
                    return cache[k, j]

                for i in range(15):
                    s_s.at[p, i][r // 2:(r + PR) // 2,
                                 c * LANES:(c + 1) * LANES] = _pk(_w_op(i, w))

        def prep_gu_part(p, part, anchors):
            PR = 16
            nr = D3 // PR
            ids = _PARTS[part]
            for n in range(2 * nr):
                (w_v, s_s), r = GU[n % 2], (n // 2) * PR
                unit = r // KU
                if part < 3:
                    cache = {}

                    def w(k, j):
                        if (k, j) not in cache:
                            v = w_v[p, j, k * D3 + r:k * D3 + r + PR, :].astype(F32)
                            v = _tie(v, spread_over(anchors, n, 2 * nr))
                            l, h = v[:, :LANES], v[:, LANES:]
                            cache[k, j] = (v, cat1(l - h, h), cat1(l, h - l))[unit]
                        return cache[k, j]

                    for i in ids:
                        s_s.at[p, i][r // 2:(r + PR) // 2, :] = _pk(_w_op(i, w))
                    continue
                prev = None
                for m, c in enumerate((1, 0) if unit == 1 else (0, 1)):
                    cache = {}

                    def w(k, j):
                        if (k, j) not in cache:
                            v = w_v[p, j, k * D3 + r:k * D3 + r + PR,
                                    c * LANES:(c + 1) * LANES].astype(F32)
                            if k == j:
                                v = _tie(v, spread_over(anchors, 2 * n + m, 4 * nr))
                            cache[k, j] = v
                        return cache[k, j]

                    sums = [_w_op(i, w) for i in ids]
                    for q, i in enumerate(ids):
                        v = sums[q] - prev[q] if m and unit else sums[q]
                        s_s.at[p, i][r // 2:(r + PR) // 2, c * LANES:(c + 1) * LANES] = _pk(v)
                    prev = sums

        NS = 2

        def gu_prod(p, i, t, anchors, slabs):
            u = KU // 2

            def rhs(s, s_s):
                if s == 1:
                    return s_s[p, i, :2 * u, :LANES]
                if s == 0:
                    return cat0(s_s[p, i, u:2 * u, LANES:], s_s[p, i, 2 * u:, :LANES])
                return cat0(s_s[p, i, :u, LANES:], s_s[p, i, 2 * u:, LANES:])

            q = TH // 2 // NS
            for n, h in enumerate(slabs):
                y = []
                for s in range(3):
                    r = _upk(cat1(rhs(s, gs_s), rhs(s, us_s)))
                    y.append(_dot(_upk(a_s[3 * i + s, h * q:(h + 1) * q]), r))
                    if (3 * n + s) % len(slabs) == 0:
                        anchors.append(y[-1][:8, :LANES])
                y1, y2 = y[1] + y[0], y[2] + y[0]
                for m in range(2):
                    cs = slice(m * LANES, (m + 1) * LANES)
                    t.setdefault((m, h), {})[i] = cat1(y1[:, cs], y2[:, cs])

        def gu_col(t, hv, p, j, anchors, slabs):
            ids = [_DIAG.get((s, j)) for s in range(3)]
            for i in ids:
                if i is not None:
                    gu_prod(p, i, t, anchors, slabs)
            for h in slabs:
                g, u = [_column(t[m, h], [None if i is None else t[m, h][i] for i in ids], j)
                        for m in range(2)]
                hv[j, h] = [_gelu_mul2(g[i], u[i]) for i in range(2)]

        def h_ops(h):
            return [v.astype(BF16) for v in _x_ops(*[[h[j][i] for j in range(3)]
                                                     for i in range(2)])]

        def h_join(hv):
            return h_ops({j: [cat0(*[hv[j, h][i] for h in range(NS)]) for i in range(2)]
                          for j in range(3)})

        def gu_piece(p):
            t, hv = {}, {}
            for h in range(NS):
                for step in ('S0', 'S1', 'F0', 'S2', 'F1', 'F2'):
                    if step[0] == 'S':
                        for i in _PARTS[int(step[1])]:
                            gu_prod(p, i, t, [], [h])
                    else:
                        gu_col(t, hv, p, int(step[1]), [], [h])
            return h_join(hv)

        D_ORDER = _PAIR_ORDER + (9, 10, 11, 12, 13, 14)

        def down_mm(acc, bs, lo, anchors, which=D_ORDER, fine=False):
            p = [None] * 15 if acc is None else list(acc)
            for i in which:
                y = None
                for n, b in enumerate(bs):
                    if i in _W_RAW:
                        k, j = _W_RAW[i]
                        v = _dot_nt(wdt_v[lo + n, k, j * D3:(j + 1) * D3, :], b[i])
                    elif len(bs) % 2 and i == 14 and n == 0:
                        v = cat0(*[_dot_nt(_upk(ds_s[lo, _W_SUM[i],
                                                     h * Q3 // 2:(h + 1) * Q3 // 2, :]), b[i])
                                   for h in range(2)])
                    else:
                        v = _dot_nt(_upk(ds_s[lo + n, _W_SUM[i]]), b[i])
                    y = v if y is None else y + v
                p[i] = y if p[i] is None else p[i] + y
                anchors.append(p[i][:8])
                if fine:
                    anchors.append(p[i][D3 // 2:D3 // 2 + 8])
            return p

        def finish(blk, acc):
            y = [cat1(*_column(acc, [acc[_DIAG[s, j]] if (s, j) in _DIAG else None
                                     for s in range(3)], j)) for j in range(3)]
            xio_s[blk] = (xmid_s[blk] + 0.5 * cat0(*y)).astype(BF16)

        def load_acc(k):
            return [acc_s[k, i] for i in range(15)]

        def store_acc(k, acc):
            for i in range(15):
                acc_s[k, i] = acc[i]

        def load_b():
            return [_upk(b_s[i * TH // 2:(i + 1) * TH // 2, :]) for i in range(15)]

        def store_b(b):
            for i in range(15):
                b_s[i * TH // 2:(i + 1) * TH // 2, :] = _pk(b[i])

        def pre_phase():
            first = [[x_cp(0, 0)], [wq_cp(0)], [x_cp(1, 2), wq_cp(1)],
                     [wq_cp(2), pltpu.make_async_copy(wo_hbm, wo_v, sem_i.at[3])]]
            order = sum(first, [])
            for p in range(NP + 1):
                order += group_cp(p)
            xr_cp = [x_cp(b, SEM_P + NP + 1) for b in range(2, NB)]
            order += xr_cp
            for cp in order:
                cp.start()
            get = lambda an, name: [an[min(i, len(an) - 1)] for i in cfg[name]]
            e_grp = lambda e: ((e >> 1) & 1, ((e >> 2) << 1) | (e & 1))
            if 'a' in cfg['sub']:
                pre_a(first, get, e_grp)
            if 'b' in cfg['sub']:
                pre_b(get, e_grp)
            if 'c' in cfg['sub']:
                pre_c(get)
            wait('WX', xr_cp)

        def pre_a(first, get, e_grp):
            def transpose_wq(i):
                wt_s[WQ[i] // 2:WQ[i + 1] // 2, :D] = _pk(wqkv_v[:, WQ[i]:WQ[i + 1]].T)

            def clear(i, carry):
                for k in range(2):
                    acc_s[k, i] = jnp.zeros((D3, TH), F32)
                r = jnp.minimum(i, 11) * (RP // 4)
                qkv_s[0, rows8(r, RP // 4)] = jnp.zeros((RP // 4, LANES), U32)
                return carry

            lax.fori_loop(0, 15, clear, 0)
            wait('WX0', first[0])
            xn0 = ln1(0, ()).astype(BF16)

            wait('WQ0', first[1])
            transpose_wq(0)
            qkv_mm(0, xn0, (0, 1), [])

            wait('WQ1', first[2])
            transpose_wq(1)
            an = []
            qkv_mm(0, xn0, (2, 3), an)
            xn1 = ln1(1, get(an, 'a_ln'), get(an, 'a_lnb')).astype(BF16)
            qkv_mm(1, xn1, (0,), an, True)
            for n, a in enumerate(get(an, 'a_w1')):
                prep_att(n, a)
            nk = len(cfg['a_k'])
            apply = [att_values(0, *e_grp(e), a) for e, a in enumerate(get(an, 'a_k'))]

            wait('WQ2', first[3])
            an = []
            qkv_mm(1, xn1, (2,), an)
            transpose_wq(2)
            qkv_mm(0, xn0, (4, 5), an)
            qkv_mm(1, xn1, (4, 1), an)
            apply += [att_values(0, *e_grp(nk + e), a)
                      for e, a in enumerate(get(an, 'a_k2')[:8 - nk])]
            for e, a in enumerate(get(an, 'a_v')):
                apply[e](a)
            wo = pltpu.bitcast(wo_v[...], U32)
            wo = cat0(_lo(wo), _hi(wo))
            wo = cat0(*[_tie(wo[n * LANES:(n + 1) * LANES], a)
                        for n, a in enumerate(get(an, 'a_wo'))])
            wt_s[3 * RP:, :D] = _pk(wo.astype(BF16).T)
            stats = wo_mm(0, an, False)
            qkv_mm(1, xn1, (3,), an)
            for n, a in enumerate(get(an, 'a_w2')):
                prep_att(12 + n, a)
            plain_lhs(0, stats)
            n1 = len(cfg['a_att'])
            for e, a in enumerate(get(an, 'a_att')):
                att_group(1, *e_grp(e), a)

            wait('WO', group_cp(0))
            an = []
            b = plain_piece(0, an)
            qkv_mm(1, xn1, (5,), an, True)
            prep_gu(0, get(an, 'z_g'))
            ffn_lhs(0, stats, get(an, 'z_l'))
            for e, a in enumerate(get(an, 'z_att')[:3 - n1]):
                att_group(1, *e_grp(n1 + e), a)
            store_b(b)

        def pre_b(get, e_grp):
            def piece(p, carry):
                wait('WP', group_cp(p))
                b_prev = load_b()
                an = []
                acc = down_mm(load_acc(0), [b_prev], p - 1, an, D_ORDER[:6], True)
                t, hv, slabs = {}, {}, list(range(NS))
                for part in range(4):
                    prep_gu_part(p, part, get(an, 'f_g%d' % part))
                    for k in range(3):
                        if part < 3:
                            gu_prod(p, _PARTS[part][k], t, an, slabs)
                        else:
                            gu_col(t, hv, p, k, an, slabs)
                b = h_join(hv)
                prep_d(p - 1, get(an, 'p_d'))
                store_acc(0, down_mm(acc, [b_prev], p - 1, an, D_ORDER[6:]))
                att_group(1, *e_grp(p + 2), an[cfg['p_att'][0]])
                for i, a in enumerate(get(an, 'p_w')):
                    prep_att(jnp.minimum(24 + (p - 1) * 5 + i, 47), a)
                store_b(b)
                return carry

            lax.fori_loop(1, NP, piece, 0)

        def pre_c(get):
            wait('WD', group_cp(NP))
            an = []
            stats = wo_mm(1, an, True)
            prep_d(NP - 1, get(an, 't_d'))
            acc = down_mm(load_acc(0), [load_b()], NP - 1, [])
            ffn_lhs(1, stats, [])
            finish(0, acc)

        if 'pre' in cfg['phases']:
            pre_phase()

        def body(u, carry):
            bu = u & (NB - 1)
            ba = (u + 1) & (NB - 1)
            acc, stats, an, b = None, None, {}, {}
            get = lambda name: [an[k][i] for k, i in cfg[name]]
            for step in cfg['body']:
                an[step] = []
                if step == 'Q':
                    xn = ln1(ba, get('ln1'), get('ln1b'))
                    qkv_fast(ba, att_rhs(xn, u >> 8), an[step])
                elif step == 'W':
                    attention(ba, get('att'))
                    stats = wo_mm(ba, an[step], True, u >> 8)
                elif step == 'L':
                    ffn_lhs(ba, stats, get('lhs'))
                elif step[0] == 'S':
                    slabs = [int(step[3])]
                    for i in _PARTS[int(step[2])]:
                        gu_prod(int(step[1]), i, b.setdefault(step[:2], {}), an[step], slabs)
                elif step[0] == 'F':
                    j, c = int(step[1]), int(step[2])
                    slabs = [int(step[3])]
                    hv = b.setdefault(step[:2], {})
                    gu_col(b['S' + step[1]], hv, j, c, an[step], slabs)
                    if len(hv) == 3 * NS:
                        b[j] = h_join(hv)
                else:
                    js = [int(c) for c in step[1:]]
                    acc = down_mm(acc, [b[j] for j in js], js[0], an[step])
            finish(bu, acc)

            @pl.when(u >= NB)
            def _():
                out_copy(bu).start()
            return carry

        if scopes:
            with jax.named_scope('LOOP'):
                lax.fori_loop(1, NU - 1, body, 0)
        elif 'main' in cfg['phases']:
            lax.fori_loop(1, NU - 1, body, 0)

        LP = 3

        def last(c, carry):
            b = [gu_piece(LP * c + j) for j in range(LP)]
            acc = down_mm(load_acc(1), b[:-1], LP * c, [])
            acc = down_mm(acc, b[-1:], LP * c + LP - 1, [])
            store_acc(1, acc)
            finish(NB - 1, acc)
            return carry

        if 'last' in cfg['phases']:
            lax.fori_loop(0, NP // LP, last, 0)
        if len(cfg['phases']) < 3:
            def keep(i, c):
                v = (gs_s[i, i, :8, :LANES] + us_s[i, i, :8, :LANES] + ds_s[i, i, :8, :LANES]
                     + wl_s[rows8(i * 8), :LANES] + a_s[i, :8] + qkv_s[i, :8]
                     + b_s[rows8(i * 8), :LANES] + wt_s[rows8(i * 8), :LANES])
                acc_s[1, 0, :8] = (lax.bitcast_convert_type(v, F32) + o_s[i, :8]
                                   + acc_s[i, i, :8])
                return c
            lax.fori_loop(0, 2, keep, 0)
            finish(NB - 1, load_acc(1))
        out_copy(NB - 1).start()
        wait('WOUT', [out_copy(b) for b in range(NB)])

    scratch = [
        pltpu.VMEM((NB, D, TM), BF16),
        pltpu.VMEM((D, 3 * D), BF16),
        pltpu.VMEM((D, D), BF16),
        pltpu.VMEM((NP, 3, D, PW), BF16),
        pltpu.VMEM((NP, 3, D, PW), BF16),
        pltpu.VMEM((NP, 3, D, PW), BF16),
        pltpu.VMEM((2 * D, 8 * LANES), U32),
        pltpu.VMEM((4 * Q3, 16 * LANES), U32),
        pltpu.VMEM((NP, 15, Q3, PW), U32),
        pltpu.VMEM((NP, 15, Q3, PW), U32),
        pltpu.VMEM((NP, 9, Q3, PW), U32),
        pltpu.VMEM((NB, D, TM), F32),
        pltpu.VMEM((54, TH // 2, LANES), U32),
        pltpu.VMEM((S // LANES + 1, 3 * RP, LANES), U32),
        pltpu.VMEM((NT, D, LANES), F32),
        pltpu.VMEM((2, 15, D3, TH), F32),
        pltpu.VMEM((15 * TH // 2, PW), U32),
        pltpu.VMEM((1, 9 * 64, 2 * LANES), U32),
        pltpu.SemaphoreType.DMA((SEM_P + NP + 2,)),
        pltpu.SemaphoreType.DMA((1,)),
    ]

    def wrapped(*refs):
        @pl.when(pl.program_id(0) == 0)
        def _():
            kernel(*refs)

    return wrapped, scratch


_CFG = dict(
    scopes=False,
    sub='abc',
    phases=('pre', 'main', 'last'),
    body=('S010', 'S000', 'F000', 'S020', 'F010', 'F020', 'S011', 'S001', 'S110',
        'S021', 'F021', 'S100', 'F100', 'S120', 'F001', 'S101', 'F110', 'F011', 'F120',
        'Q', 'S111', 'F101', 'S121', 'F111', 'F121', 'S300', 'S200', 'S210', 'S220',
        'F200', 'F210', 'F220', 'S201', 'S221', 'S211', 'F201', 'S320', 'F211', 'F221',
        'S310', 'D01', 'F300', 'S301', 'S311', 'F301', 'S321', 'F311', 'F321', 'S400',
        'F310', 'S420', 'F320', 'S410', 'S401', 'F410', 'F420', 'S411', 'F400', 'S421',
        'F411', 'F421', 'S500', 'D23', 'F401', 'S501', 'S510', 'S520', 'F500', 'W',
        'F520', 'S511', 'F510', 'S521', 'F501', 'F511', 'F521', 'D4', 'D5', 'L'),
    ln1=(('S010', 2), ('S010', 3), ('S010', 5), ('S010', 6), ('S010', 8), ('S000', 0),
        ('S000', 2), ('S000', 3), ('S000', 5)),
    ln1b=(('S110', 2), ('S110', 3), ('S110', 5), ('S110', 6), ('S110', 8), ('S021', 0),
        ('S021', 2), ('S021', 3), ('S021', 5), ('S021', 6), ('S021', 8), ('F021', 0)),
    att=(('S300', 6), ('D01', 2), ('D01', 6), ('D01', 7), ('D01', 10), ('F300', 4),
        ('D23', 5), ('D23', 9)),
    lhs=(('S521', 0), ('D5', 0), ('D5', 4)),
    a_w1=(0, 0, 1, 2, 2, 3, 3, 4, 4, 5, 6, 7),
    a_w2=(20, 23, 26, 30, 33, 36, 40, 43, 46, 50, 53, 57),
    a_ln=(0, 3, 6),
    a_lnb=(5, 9, 9),
    z_g=(5, 6, 7, 8, 11, 11, 12, 13, 14, 15, 17, 18, 19, 20, 21, 22, 23, 24, 25, 26, 28,
        29, 30, 31, 32, 35, 36, 37, 38, 40, 41, 42, 43, 45, 46, 47, 48, 49, 50, 51, 52,
        54, 55, 57, 58, 59, 60, 62),
    z_att=(53, 54, 56),
    t_d=(0, 0, 1, 1, 2, 3, 3, 4, 5, 6, 6, 7, 8, 9, 9, 9, 10, 11, 11, 12, 13, 14, 15,
        16),
    p_d=(26, 26, 27, 27, 29, 29, 29, 30, 31, 31, 32, 33, 33, 34, 35, 35, 36, 36, 37, 37,
        38, 39, 39, 41),
    p_att=(59,),
    p_w=(12, 60, 62, 65, 65),
    z_l=(2, 13, 32),
    f_g0=(0, 0, 0, 1, 1, 2, 2, 3, 4, 4, 4, 5),
    f_g1=(4, 6, 7, 7, 8, 10, 10, 11, 11, 12, 13, 14),
    f_g2=(5, 10, 11, 11, 13, 15, 16, 17, 19, 20, 21, 22),
    f_g3=(6, 7, 14, 16, 17, 18, 19, 19, 21, 22, 23, 23, 24, 25, 27, 28, 29, 30, 31, 33,
        34, 36, 36, 37),
    a_k=(15, 19, 20, 24),
    a_k2=(0, 4, 8, 12),
    a_v=(13, 14, 22, 26, 30, 34, 38, 39),
    a_att=(12, 60),
    a_wo=(30, 35, 36, 38, 41),
)


def _run(A_x, A_wqkv, A_wo, B_w_gate, B_w_up, B_w_down, **kw):
    _, S, D = A_x.shape
    F = B_w_gate.shape[1]
    kernel, scratch = _make_kernel(S, D, F, 256, {**_CFG, **kw})
    hbm = pl.BlockSpec(memory_space=pl.ANY)
    out_t = pl.pallas_call(
        kernel,
        grid=(2,),
        in_specs=[hbm] * 6,
        out_specs=hbm,
        out_shape=jax.ShapeDtypeStruct((D, S), A_x.dtype),
        scratch_shapes=scratch,
        compiler_params=pltpu.CompilerParams(
            dimension_semantics=('arbitrary',), vmem_limit_bytes=110 * 1024 * 1024),
    )(A_x.reshape(S, D).T, A_wqkv, A_wo, B_w_gate, B_w_up, B_w_down.T)
    return out_t.T.reshape(A_x.shape)


@jax.jit
def pallas_interleave_layers__sliding_local_dilated__glu_gated_geglu__prompt_kernel(
    A_x: jax.Array,
    A_wqkv: jax.Array,
    A_wo: jax.Array,
    B_x: jax.Array,
    B_w_gate: jax.Array,
    B_w_up: jax.Array,
    B_w_down: jax.Array,
):
    del B_x
    return _run(A_x, A_wqkv, A_wo, B_w_gate, B_w_up, B_w_down)
```

```python
import jax
import jax.numpy as jnp
import jax.experimental.pallas as pl
import jax.experimental.pallas.tpu as pltpu
from jax import lax

H = 32
W = 8
DIL = 2
EPS = 1e-5
LANES = 128

F32 = jnp.float32
BF16 = jnp.bfloat16
U32 = jnp.uint32

_NT = (((1,), (1,)), ((), ()))


def _tree_sum(parts, op=jnp.add):
    while len(parts) > 1:
        nxt = [op(parts[i], parts[i + 1]) for i in range(0, len(parts) - 1, 2)]
        if len(parts) % 2:
            nxt.append(parts[-1])
        parts = nxt
    return parts[0]


def _ln_stats(slabs, d, anchors=()):
    n_acc = 4
    s1, s2, pilot = [None] * n_acc, [None] * n_acc, None
    for i, x in enumerate(slabs):
        if pilot is None:
            pilot = x[0:1, :]
            pil = jnp.broadcast_to(pilot, x.shape)
            pils = [_tie(pil, a) for a in anchors] or [pil]
        dx = x - pils[i * len(pils) // (d // 8)]
        j = i % n_acc
        s1[j] = dx if s1[j] is None else s1[j] + dx
        s2[j] = dx * dx if s2[j] is None else s2[j] + dx * dx
    e1 = jnp.sum(_tree_sum(s1), axis=0, keepdims=True) * (1.0 / d)
    e2 = jnp.sum(_tree_sum(s2), axis=0, keepdims=True) * (1.0 / d)
    var = jnp.maximum(e2 - e1 * e1, 0.0)
    return pilot + e1, lax.rsqrt(var + EPS)


def _zero_like_dep(v):
    return (lax.bitcast_convert_type(v, U32) >> 31) >> 1


def _tie(x, anchor):
    if anchor is None:
        return x
    z = lax.bitcast_convert_type(_zero_like_dep(anchor), F32)
    z = jnp.concatenate([z] * -(-x.shape[1] // LANES), axis=1)[:, :x.shape[1]]
    if x.shape[0] == 8:
        return x + z
    return jnp.concatenate([x[:8] + z, x[8:]], axis=0)


def _gelu_mul2(g, u):
    c0 = 0.7978845608028654
    c1 = c0 * 0.044715
    t = jnp.tanh(g * (c0 + c1 * (g * g)))
    return (g * u) * (1.0 + t)


def _lo(x):
    return lax.bitcast_convert_type(x << 16, F32)


def _hi(x):
    return lax.bitcast_convert_type(x & jnp.uint32(0xFFFF0000), F32)


def _pk(x):
    return pltpu.bitcast(x.astype(BF16), U32)


def _upk(x):
    return pltpu.bitcast(x, BF16)


def _dot(a, b):
    return jnp.dot(a, b, preferred_element_type=F32)


def _dot_nt(a, b):
    return lax.dot_general(a, b, _NT, preferred_element_type=F32)


def _x_ops(x1, x2):
    d = [a - b for a, b in zip(x1, x2)]
    return [x1[0] + x2[1], x2[0] + x2[1], x1[0] + x1[1],
            d[1] + x1[2], x1[1] + x1[2], d[1] + d[2],
            d[0] - x2[2], d[0] + d[2], x2[0] + x2[2],
            x1[0], d[0], x2[1], d[1], x1[2], x2[2]]


def _x_rem(x1, x2):
    a, b, c = 0, 1, 2
    cat = lambda u, v: jnp.concatenate([u, v], axis=0)
    return [cat(x1[c], x2[b]), cat(x1[a], x1[b] - x2[b]), cat(x2[a], x2[c] - x1[c])]


_W_TERMS = {0: ((0, 1, 1), (1, 0, 1)), 3: ((1, 2, 1), (2, 1, 1)), 6: ((0, 2, 1), (2, 0, 1)),
            9: ((0, 0, 1), (0, 2, 1), (1, 0, -1)), 10: ((2, 0, 1), (0, 0, -1), (0, 1, -1)),
            11: ((1, 1, 1), (1, 2, 1), (0, 1, -1)), 12: ((1, 0, 1), (1, 1, 1), (2, 1, -1)),
            13: ((2, 0, 1), (2, 2, 1), (1, 2, -1)), 14: ((2, 1, 1), (2, 2, 1), (0, 2, -1)),
            1: ((0, 1, 1),), 2: ((1, 0, 1),), 4: ((1, 2, 1),), 5: ((2, 1, 1),),
            7: ((2, 0, 1),), 8: ((0, 2, 1),)}


def _w_op(i, w):
    v = None
    for k, j, sg in _W_TERMS[i]:
        v = w(k, j) if v is None else (v + w(k, j) if sg > 0 else v - w(k, j))
    return v


def _w_sums(w):
    return [_w_op(i, lambda k, j: w[k][j]) for i in _W_SUM]


_PARTS = ((1, 2, 0), (7, 8, 6), (4, 5, 3), (9, 10, 11, 12, 13, 14))
_W_SUM = {0: 0, 3: 1, 6: 2, 9: 3, 10: 4, 11: 5, 12: 6, 13: 7, 14: 8}
_W_RAW = {1: (0, 1), 2: (1, 0), 4: (1, 2), 5: (2, 1), 7: (2, 0), 8: (0, 2)}
_PAIR_ORDER = (1, 2, 4, 5, 7, 8, 0, 3, 6)
_DIAG = {(0, 0): 9, (2, 0): 10, (0, 1): 11, (1, 1): 12, (1, 2): 13, (2, 2): 14}
_PAIR = {(0, 0): ((6, -1), (8, -1)), (1, 0): ((2, 1), (7, 1)), (2, 0): ((0, 1), (1, -1)),
         (0, 1): ((3, 1), (4, -1)), (1, 1): ((0, 1), (2, -1)), (2, 1): ((1, 1), (5, -1)),
         (0, 2): ((4, 1), (8, 1)), (1, 2): ((6, 1), (7, -1)), (2, 2): ((5, 1), (3, -1))}


def _column(t, base, j, skew=False):
    s = []
    for k in range(3):
        v = base[k]
        for i, sg in _PAIR[k, j]:
            v = t[i] if v is None else (v + t[i] if sg > 0 else v - t[i])
        s.append(v)
    if skew:
        return s[1] + s[0], s[2] + 0.5 * (s[0] - s[1])
    return s[1] + s[0], s[2] + s[0]


def _make_kernel(S, D, F, TM, cfg):
    NB = S // TM
    NT = TM // LANES
    DH = D // H
    DP = DH // 2
    RP = D // 2
    NG = H // 8
    scale = float(DH) ** -0.5
    NU = 2 * NB
    TH = TM // 2
    FT = F // 3
    D2 = D // 2
    D3 = D // 3
    Q3 = D3 // 2
    KU = D // 9
    KR = 3 * LANES
    NQ = 6
    QR = 3 * D // NQ
    WQ = (0, 640, 1152, 3 * D)
    PW = 256
    NP = FT // PW
    scopes = cfg['scopes']
    assert NG == 4 and NB & (NB - 1) == 0
    SEM_P = 4

    def kernel(x_hbm, wqkv_hbm, wo_hbm, wg_hbm, wu_hbm, wdt_hbm, out_hbm,
               xio_s, wqkv_v, wo_v, wg_v, wu_v, wdt_v, wt_s, wl_s,
               gs_s, us_s, ds_s, xmid_s, a_s, qkv_s, o_s, acc_s, b_s, r_s,
               sem_i, sem_o):

        def wait(name, cps):
            if scopes:
                with jax.named_scope(name):
                    for cp in cps:
                        cp.wait()
            else:
                for cp in cps:
                    cp.wait()

        def cols(lo, n):
            if not isinstance(lo, int):
                lo = pl.multiple_of(lo, LANES)
            return pl.ds(lo, n)

        def rows8(lo, n=8):
            if not isinstance(lo, int):
                lo = pl.multiple_of(lo, 8)
            return pl.ds(lo, n)

        def out_copy(b):
            return pltpu.make_async_copy(
                xio_s.at[b], out_hbm.at[:, cols(b * TM, TM)], sem_o.at[0])

        def x_cp(b, sem):
            return pltpu.make_async_copy(x_hbm.at[:, cols(b * TM, TM)], xio_s.at[b],
                                         sem_i.at[sem])

        def wq_cp(i):
            sl = cols(WQ[i], WQ[i + 1] - WQ[i])
            return pltpu.make_async_copy(wqkv_hbm.at[:, sl], wqkv_v.at[:, sl],
                                         sem_i.at[1 + i])

        def piece_cp(src, dst, p, sem):
            return [pltpu.make_async_copy(src.at[:, cols(j * FT + p * PW, PW)],
                                          dst.at[p, j],
                                          sem_i.at[sem]) for j in range(3)]

        def group_cp(p):
            sem = SEM_P + p
            cps = []
            if not (isinstance(p, int) and p == NP):
                cps += piece_cp(wg_hbm, wg_v, p, sem) + piece_cp(wu_hbm, wu_v, p, sem)
            if not (isinstance(p, int) and p == 0):
                cps += piece_cp(wdt_hbm, wdt_v, p - 1, sem)
            return cps

        lane = lax.broadcasted_iota(jnp.int32, (8, LANES), 1)
        cat0 = lambda *v: jnp.concatenate(v, axis=0)
        cat1 = lambda *v: jnp.concatenate(v, axis=1)

        def spread_over(anchors, n, total):
            return anchors[n * len(anchors) // total] if anchors else None

        def slab_group(r):
            return (r % LANES) // 16 if r < KR else 8 + ((r - KR) % KU) // 16

        def ln1(blk, anchors1, anchors2=()):
            slabs = (xio_s[blk, r:r + 8, :].astype(F32) for r in range(0, D, 8))
            m, rs = _ln_stats(slabs, D, anchors1)
            if not anchors2:
                return (xio_s[blk].astype(F32) - m) * rs
            m8 = jnp.broadcast_to(m, (8, TM))
            ms = [_tie(m8, a) for a in anchors2]
            ms = [spread_over(ms, slab_group(r), 12) for r in range(0, D, 8)]
            return (xio_s[blk].astype(F32) - cat0(*ms)) * rs

        def dot_k(rows, x, anchors, even=False):
            y = None
            for n, k in enumerate(range(0, D, LANES)):
                ks = slice(k, min(k + LANES, D))
                if even and k + LANES >= D:
                    mid = (rows.start + rows.stop) // 2
                    v = cat0(_dot(_upk(wt_s[rows.start:mid, ks]), x[ks]),
                             _dot(_upk(wt_s[mid:rows.stop, ks]), x[ks]))
                else:
                    v = _dot(_upk(wt_s[rows, ks]), x[ks])
                anchors.extend(v[r:r + 8, :LANES] for r in ((0, 144) if n % 2 else (72, 216)))
                y = v if y is None else y + v
            return y

        def put_qkv(blk, rows, y):
            pk = _pk(y)
            for c in range(NT):
                qkv_s[1 + blk * NT + c, rows, :] = pk[:, c * LANES:(c + 1) * LANES]

        def qkv_mm(blk, xn, chunks, anchors, even=False):
            for r in chunks:
                rows = slice(r * QR // 2, (r + 1) * QR // 2)
                put_qkv(blk, rows, dot_k(rows, xn, anchors, even))

        def split_k(x):
            hs = (x[:, :TH], x[:, TH:])
            blocks = [[h[k * LANES:(k + 1) * LANES] for k in range(3)] for h in hs]
            units = [[h[KR + k * KU:KR + (k + 1) * KU] for k in range(3)] for h in hs]
            return blocks, units

        def prep_att(pat, anchor):
            assert Q3 == 96
            row0 = pat * 8
            src0 = row0 + ((pat * 43) >> 9) * (2 * Q3)
            w = [_upk(wt_s[rows8(src0 + j * Q3), :D]).astype(F32) for j in range(3)]
            w[0] = cat1(_tie(w[0][:, :LANES], anchor), w[0][:, LANES:])
            tiles = _w_sums([[w[j][:, k * LANES:(k + 1) * LANES] for j in range(3)]
                             for k in range(3)])
            for j in range(3):
                a, b, c = (w[j][:, KR + k * KU:KR + (k + 1) * KU] for k in range(3))
                tiles += [cat1(c, b), cat1(a, c)]
            wl_s[rows8(row0), :15 * LANES] = _pk(cat1(*tiles))

        def att_rhs(x, stash=None):
            blocks, units = split_k(cat1(x[:, :TH], x[:, TH:] + 0.5 * x[:, :TH]))
            ops = _x_ops(*blocks) + _x_rem(*units)
            if stash is None:
                return [v.astype(BF16) for v in ops]
            loc = lambda i, r0, n: (slice((i // 2) * 64 + r0, (i // 2) * 64 + r0 + n),
                                    slice((i % 2) * LANES, (i % 2 + 1) * LANES))
            for r in range(0, LANES, 16):
                for i, v in enumerate(ops):
                    r_s.at[0][loc(i, r // 2, 8)] = _pk(v[r:r + 16])
            return [_upk(r_s.at[stash][loc(i, 0, 64)]) for i in range(18)]

        def att_mm(sec, rhs, anchors):
            tl = lambda i: _upk(wl_s[sec * Q3:(sec + 1) * Q3, i * LANES:(i + 1) * LANES])
            raw = lambda k, j: _upk(wt_s[(3 * sec + j) * Q3:(3 * sec + j + 1) * Q3,
                                         k * LANES:(k + 1) * LANES])
            t = {}
            for i in _PAIR_ORDER:
                t[i] = _dot(raw(*_W_RAW[i]) if i in _W_RAW else tl(_W_SUM[i]), rhs[i])
                anchors.append(t[i][:8])
            out = []
            for j in range(3):
                base = []
                for s in range(3):
                    v = _dot(raw(3, j) if s == 1 else tl(9 + 2 * j + s // 2), rhs[15 + s])
                    if (s, j) in _DIAG:
                        i = _DIAG[s, j]
                        v = _dot(tl(_W_SUM[i]), rhs[i]) + v
                    base.append(v)
                    anchors.append(base[-1][:8])
                out.append(cat1(*_column(t, base, j, True)))
            return cat0(*out)

        def qkv_fast(blk, rhs, anchors):
            for sec in range(3):
                put_qkv(blk, slice(sec * RP, (sec + 1) * RP), att_mm(sec, rhs, anchors))

        def shifted(ln, cur, prev, w):
            if w == 0:
                return cur
            sh = DIL * w
            return pltpu.roll(jnp.where(ln < LANES - sh, cur, prev), sh, axis=1)

        def att_group(blk, c, hg, anchor):
            att_values(blk, c, hg, anchor)(None)

        def att_values(blk, c, hg, anchor):
            tile = blk * NT + c
            base = hg * 8 * DP
            if isinstance(hg, int):
                cur, prev, o_t = qkv_s.at[1 + tile], qkv_s.at[tile], o_s.at[c]
            else:
                n = 2 * RP + 8 * DP
                base = pl.multiple_of(base, 8)
                cur = qkv_s.at[1 + tile, pl.ds(base, n)]
                prev = qkv_s.at[tile, pl.ds(base, n)]
                o_t = o_s.at[c, pl.ds(base, RP + 8 * DP)]
                base = 0
            ln = lane + _zero_like_dep(anchor).astype(jnp.int32)
            logits = [None] * W
            for dd in range(DP):
                q = cur[pl.ds(base + dd, 8, stride=DP), :]
                kc = cur[pl.ds(RP + base + dd, 8, stride=DP), :]
                kp = prev[pl.ds(RP + base + dd, 8, stride=DP), :]
                q0, q1 = _lo(q), _hi(q)
                for w in range(W):
                    ks = shifted(ln, kc, kp, w)
                    t = q0 * _lo(ks) + q1 * _hi(ks)
                    logits[w] = t if logits[w] is None else logits[w] + t
            logits = [l * scale for l in logits]
            if not (isinstance(c, int) and c > 0):
                pos = lane + tile * LANES
                logits = [l if w == 0 else jnp.where(pos >= DIL * w, l, -1e9)
                          for w, l in enumerate(logits)]
            m = _tree_sum(logits, jnp.maximum)
            p = [jnp.exp(l - m) for l in logits]
            r = 1.0 / _tree_sum(p)

            def apply(anchor2):
                ln = lane + _zero_like_dep(m if anchor2 is None else anchor2).astype(jnp.int32)
                for dd in range(DP):
                    vc = cur[pl.ds(2 * RP + base + dd, 8, stride=DP), :]
                    vp = prev[pl.ds(2 * RP + base + dd, 8, stride=DP), :]
                    o0 = o1 = None
                    for w in range(W):
                        vs = shifted(ln, vc, vp, w)
                        t0, t1 = p[w] * _lo(vs), p[w] * _hi(vs)
                        o0 = t0 if o0 is None else o0 + t0
                        o1 = t1 if o1 is None else o1 + t1
                    o0, o1 = o0 * r, o1 * r
                    o_t[pl.ds(base + dd, 8, stride=DP), :] = o0
                    o_t[pl.ds(RP + base + dd, 8, stride=DP), :] = o1

            return apply

        def attention(blk, anchors):
            for c in range(NT):
                for hg in range(NG):
                    att_group(blk, c, hg, anchors[c * NG + hg])

        def wo_mm(blk, anchors, fast, stash=None):
            o = cat1(*[o_s[c] for c in range(NT)])
            if fast:
                y = att_mm(3, att_rhs(o, stash), anchors)
            else:
                o = o.astype(BF16)
                q = D2 // 2
                y = cat0(*[dot_k(slice(h * q, (h + 1) * q), o, anchors) for h in (6, 7)])
            xm = xio_s[blk].astype(F32) + y
            xmid_s[blk] = xm
            return _ln_stats((xm[r:r + 8] for r in range(0, D, 8)), D)

        def ffn_lhs(blk, stats, anchors):
            m, rs = stats
            m8 = jnp.broadcast_to(m, (8, TM))
            xs = []
            for k in range(3):
                mt = cat0(*[_tie(m8, spread_over(anchors, k, 3))] * (D3 // 8))
                xs.append((xmid_s[blk, k * D3:(k + 1) * D3, :] - mt) * rs)
            ops = _x_ops([x[:, :TH] for x in xs], [x[:, TH:] for x in xs])
            for i, v in enumerate(ops):
                for s, t in enumerate((v[KU:], v[:2 * KU], cat0(v[:KU], v[2 * KU:]))):
                    a_s[3 * i + s] = _pk(t.astype(BF16).T)

        def plain_lhs(blk, stats):
            m, rs = stats
            blocks, units = split_k((xmid_s[blk] - m) * rs)
            for i, v in enumerate(blocks[0] + blocks[1] + _x_rem(*units)):
                a_s[45 + i] = _pk(v.astype(BF16).T)

        def plain_piece(p, anchors):
            h = {}
            for j in range(3):
                hs = []
                for n in range(PW // LANES):
                    cs = slice(n * LANES, (n + 1) * LANES)
                    w = lambda r0, r1: cat1(wg_v[p, j, r0:r1, cs], wu_v[p, j, r0:r1, cs])
                    u = lambda k: w(KR + k * KU, KR + (k + 1) * KU)
                    tl = lambda *i: _upk(cat1(*[a_s[45 + k] for k in i]))
                    y0 = _dot(tl(6), cat0(u(2), u(1)))
                    y1 = _dot(tl(0, 1, 2, 7), w(0, KR + 2 * KU))
                    y2 = _dot(tl(3, 4, 5, 8), cat0(w(0, KR + KU), u(2)))
                    anchors.append(y0[:8, :LANES])
                    for y in (y1, y2):
                        anchors.extend(y[r:r + 8, c:c + LANES] for c in (0, LANES)
                                       for r in (0, TH // 2))
                    hs.append([_gelu_mul2(*[(y + y0)[:, c:c + LANES] for c in (0, LANES)])
                               for y in (y1, y2)])
                h[j] = [cat1(*[v[i] for v in hs]) for i in range(2)]
            return h_ops(h)

        def prep_d(p, anchors):
            PR = 16
            for n in range(2 * D3 // PR):
                r, cs = (n // 2) * PR, slice((n % 2) * LANES, (n % 2 + 1) * LANES)
                w = [[wdt_v[p, k, j * D3 + r:j * D3 + r + PR, cs].astype(F32)
                      for j in range(3)] for k in range(3)]
                w[0][1] = _tie(w[0][1], spread_over(anchors, n, 2 * D3 // PR))
                for i, v in enumerate(_w_sums(w)):
                    ds_s.at[p, i][r // 2:(r + PR) // 2, cs] = _pk(v)

        GU = ((wg_v, gs_s), (wu_v, us_s))

        def prep_gu(p, anchors):
            PR = 16
            nr = D3 // PR
            for n in range(4 * nr):
                c, (w_v, s_s), r = n % 2, GU[(n // 2) % 2], (n // 4) * PR
                cache = {}

                def w(k, j):
                    if (k, j) not in cache:
                        ld = lambda c: w_v[p, j, k * D3 + r:k * D3 + r + PR,
                                           c * LANES:(c + 1) * LANES].astype(F32)
                        v = ld(c)
                        if k != j:
                            v = _tie(v, spread_over(anchors, n, 4 * nr))
                        cache[k, j] = v - ld(1 - c) if r // KU == 1 + c else v
                    return cache[k, j]

                for i in range(15):
                    s_s.at[p, i][r // 2:(r + PR) // 2,
                                 c * LANES:(c + 1) * LANES] = _pk(_w_op(i, w))

        def prep_gu_part(p, part, anchors):
            PR = 16
            nr = D3 // PR
            ids = _PARTS[part]
            for n in range(2 * nr):
                (w_v, s_s), r = GU[n % 2], (n // 2) * PR
                unit = r // KU
                if part < 3:
                    cache = {}

                    def w(k, j):
                        if (k, j) not in cache:
                            v = w_v[p, j, k * D3 + r:k * D3 + r + PR, :].astype(F32)
                            v = _tie(v, spread_over(anchors, n, 2 * nr))
                            l, h = v[:, :LANES], v[:, LANES:]
                            cache[k, j] = (v, cat1(l - h, h), cat1(l, h - l))[unit]
                        return cache[k, j]

                    for i in ids:
                        s_s.at[p, i][r // 2:(r + PR) // 2, :] = _pk(_w_op(i, w))
                    continue
                prev = None
                for m, c in enumerate((1, 0) if unit == 1 else (0, 1)):
                    cache = {}

                    def w(k, j):
                        if (k, j) not in cache:
                            v = w_v[p, j, k * D3 + r:k * D3 + r + PR,
                                    c * LANES:(c + 1) * LANES].astype(F32)
                            if k == j:
                                v = _tie(v, spread_over(anchors, 2 * n + m, 4 * nr))
                            cache[k, j] = v
                        return cache[k, j]

                    sums = [_w_op(i, w) for i in ids]
                    for q, i in enumerate(ids):
                        v = sums[q] - prev[q] if m and unit else sums[q]
                        s_s.at[p, i][r // 2:(r + PR) // 2, c * LANES:(c + 1) * LANES] = _pk(v)
                    prev = sums

        NS = 2

        def gu_prod(p, i, t, anchors, slabs):
            u = KU // 2

            def rhs(s, s_s):
                if s == 1:
                    return s_s[p, i, :2 * u, :LANES]
                if s == 0:
                    return cat0(s_s[p, i, u:2 * u, LANES:], s_s[p, i, 2 * u:, :LANES])
                return cat0(s_s[p, i, :u, LANES:], s_s[p, i, 2 * u:, LANES:])

            q = TH // 2 // NS
            for n, h in enumerate(slabs):
                y = []
                for s in range(3):
                    r = _upk(cat1(rhs(s, gs_s), rhs(s, us_s)))
                    y.append(_dot(_upk(a_s[3 * i + s, h * q:(h + 1) * q]), r))
                    if (3 * n + s) % len(slabs) == 0:
                        anchors.append(y[-1][:8, :LANES])
                y1, y2 = y[1] + y[0], y[2] + y[0]
                for m in range(2):
                    cs = slice(m * LANES, (m + 1) * LANES)
                    t.setdefault((m, h), {})[i] = cat1(y1[:, cs], y2[:, cs])

        def gu_col(t, hv, p, j, anchors, slabs):
            ids = [_DIAG.get((s, j)) for s in range(3)]
            for i in ids:
                if i is not None:
                    gu_prod(p, i, t, anchors, slabs)
            for h in slabs:
                g, u = [_column(t[m, h], [None if i is None else t[m, h][i] for i in ids], j)
                        for m in range(2)]
                hv[j, h] = [_gelu_mul2(g[i], u[i]) for i in range(2)]

        def h_ops(h):
            return [v.astype(BF16) for v in _x_ops(*[[h[j][i] for j in range(3)]
                                                     for i in range(2)])]

        def h_join(hv):
            return h_ops({j: [cat0(*[hv[j, h][i] for h in range(NS)]) for i in range(2)]
                          for j in range(3)})

        def gu_piece(p):
            t, hv = {}, {}
            for h in range(NS):
                for step in ('S0', 'S1', 'F0', 'S2', 'F1', 'F2'):
                    if step[0] == 'S':
                        for i in _PARTS[int(step[1])]:
                            gu_prod(p, i, t, [], [h])
                    else:
                        gu_col(t, hv, p, int(step[1]), [], [h])
            return h_join(hv)

        D_ORDER = _PAIR_ORDER + (9, 10, 11, 12, 13, 14)

        def down_mm(acc, bs, lo, anchors, which=D_ORDER, fine=False):
            p = [None] * 15 if acc is None else list(acc)
            for i in which:
                y = None
                for n, b in enumerate(bs):
                    if i in _W_RAW:
                        k, j = _W_RAW[i]
                        v = _dot_nt(wdt_v[lo + n, k, j * D3:(j + 1) * D3, :], b[i])
                    elif len(bs) % 2 and i == 14 and n == 0:
                        v = cat0(*[_dot_nt(_upk(ds_s[lo, _W_SUM[i],
                                                     h * Q3 // 2:(h + 1) * Q3 // 2, :]), b[i])
                                   for h in range(2)])
                    else:
                        v = _dot_nt(_upk(ds_s[lo + n, _W_SUM[i]]), b[i])
                    y = v if y is None else y + v
                p[i] = y if p[i] is None else p[i] + y
                anchors.append(p[i][:8])
                if fine:
                    anchors.append(p[i][D3 // 2:D3 // 2 + 8])
            return p

        def finish(blk, acc):
            y = [cat1(*_column(acc, [acc[_DIAG[s, j]] if (s, j) in _DIAG else None
                                     for s in range(3)], j)) for j in range(3)]
            xio_s[blk] = (xmid_s[blk] + 0.5 * cat0(*y)).astype(BF16)

        def load_acc(k):
            return [acc_s[k, i] for i in range(15)]

        def store_acc(k, acc):
            for i in range(15):
                acc_s[k, i] = acc[i]

        def load_b():
            return [_upk(b_s[i * TH // 2:(i + 1) * TH // 2, :]) for i in range(15)]

        def store_b(b):
            for i in range(15):
                b_s[i * TH // 2:(i + 1) * TH // 2, :] = _pk(b[i])

        def pre_phase():
            first = [[x_cp(0, 0)], [wq_cp(0)], [x_cp(1, 2), wq_cp(1)],
                     [wq_cp(2), pltpu.make_async_copy(wo_hbm, wo_v, sem_i.at[3])]]
            order = sum(first, [])
            for p in range(NP + 1):
                order += group_cp(p)
            xr_cp = [x_cp(b, SEM_P + NP + 1) for b in range(2, NB)]
            order += xr_cp
            for cp in order:
                cp.start()
            get = lambda an, name: [an[min(i, len(an) - 1)] for i in cfg[name]]
            e_grp = lambda e: ((e >> 1) & 1, ((e >> 2) << 1) | (e & 1))
            if 'a' in cfg['sub']:
                pre_a(first, get, e_grp)
            if 'b' in cfg['sub']:
                pre_b(get, e_grp)
            if 'c' in cfg['sub']:
                pre_c(get)
            wait('WX', xr_cp)

        def pre_a(first, get, e_grp):
            def transpose_wq(i):
                wt_s[WQ[i] // 2:WQ[i + 1] // 2, :D] = _pk(wqkv_v[:, WQ[i]:WQ[i + 1]].T)

            def clear(i, carry):
                for k in range(2):
                    acc_s[k, i] = jnp.zeros((D3, TH), F32)
                r = jnp.minimum(i, 11) * (RP // 4)
                qkv_s[0, rows8(r, RP // 4)] = jnp.zeros((RP // 4, LANES), U32)
                return carry

            lax.fori_loop(0, 15, clear, 0)
            wait('WX0', first[0])
            xn0 = ln1(0, ()).astype(BF16)

            wait('WQ0', first[1])
            transpose_wq(0)
            qkv_mm(0, xn0, (0, 1), [])

            wait('WQ1', first[2])
            transpose_wq(1)
            an = []
            qkv_mm(0, xn0, (2, 3), an)
            xn1 = ln1(1, get(an, 'a_ln'), get(an, 'a_lnb')).astype(BF16)
            qkv_mm(1, xn1, (0,), an, True)
            for n, a in enumerate(get(an, 'a_w1')):
                prep_att(n, a)
            nk = len(cfg['a_k'])
            apply = [att_values(0, *e_grp(e), a) for e, a in enumerate(get(an, 'a_k'))]

            wait('WQ2', first[3])
            an = []
            qkv_mm(1, xn1, (2,), an)
            transpose_wq(2)
            qkv_mm(0, xn0, (4, 5), an)
            qkv_mm(1, xn1, (4, 1), an)
            apply += [att_values(0, *e_grp(nk + e), a)
                      for e, a in enumerate(get(an, 'a_k2')[:8 - nk])]
            for e, a in enumerate(get(an, 'a_v')):
                apply[e](a)
            wo = pltpu.bitcast(wo_v[...], U32)
            wo = cat0(_lo(wo), _hi(wo))
            wo = cat0(*[_tie(wo[n * LANES:(n + 1) * LANES], a)
                        for n, a in enumerate(get(an, 'a_wo'))])
            wt_s[3 * RP:, :D] = _pk(wo.astype(BF16).T)
            stats = wo_mm(0, an, False)
            qkv_mm(1, xn1, (3,), an)
            for n, a in enumerate(get(an, 'a_w2')):
                prep_att(12 + n, a)
            plain_lhs(0, stats)
            n1 = len(cfg['a_att'])
            for e, a in enumerate(get(an, 'a_att')):
                att_group(1, *e_grp(e), a)

            wait('WO', group_cp(0))
            an = []
            b = plain_piece(0, an)
            qkv_mm(1, xn1, (5,), an, True)
            prep_gu(0, get(an, 'z_g'))
            ffn_lhs(0, stats, get(an, 'z_l'))
            for e, a in enumerate(get(an, 'z_att')[:3 - n1]):
                att_group(1, *e_grp(n1 + e), a)
            store_b(b)

        def pre_b(get, e_grp):
            def piece(p, carry):
                wait('WP', group_cp(p))
                b_prev = load_b()
                an = []
                acc = down_mm(load_acc(0), [b_prev], p - 1, an, D_ORDER[:6], True)
                t, hv, slabs = {}, {}, list(range(NS))
                for part in range(4):
                    prep_gu_part(p, part, get(an, 'f_g%d' % part))
                    for k in range(3):
                        if part < 3:
                            gu_prod(p, _PARTS[part][k], t, an, slabs)
                        else:
                            gu_col(t, hv, p, k, an, slabs)
                b = h_join(hv)
                prep_d(p - 1, get(an, 'p_d'))
                store_acc(0, down_mm(acc, [b_prev], p - 1, an, D_ORDER[6:]))
                att_group(1, *e_grp(p + 2), an[cfg['p_att'][0]])
                for i, a in enumerate(get(an, 'p_w')):
                    prep_att(jnp.minimum(24 + (p - 1) * 5 + i, 47), a)
                store_b(b)
                return carry

            lax.fori_loop(1, NP, piece, 0)

        def pre_c(get):
            wait('WD', group_cp(NP))
            an = []
            stats = wo_mm(1, an, True)
            prep_d(NP - 1, get(an, 't_d'))
            acc = down_mm(load_acc(0), [load_b()], NP - 1, [])
            ffn_lhs(1, stats, [])
            finish(0, acc)

        if 'pre' in cfg['phases']:
            pre_phase()

        def body(u, carry):
            bu = u & (NB - 1)
            ba = (u + 1) & (NB - 1)
            acc, stats, an, b = None, None, {}, {}
            get = lambda name: [an[k][i] for k, i in cfg[name]]
            for step in cfg['body']:
                an[step] = []
                if step == 'Q':
                    xn = ln1(ba, get('ln1'), get('ln1b'))
                    qkv_fast(ba, att_rhs(xn, u >> 8), an[step])
                elif step == 'W':
                    attention(ba, get('att'))
                    stats = wo_mm(ba, an[step], True, u >> 8)
                elif step == 'L':
                    ffn_lhs(ba, stats, get('lhs'))
                elif step[0] == 'S':
                    slabs = [int(step[3])]
                    for i in _PARTS[int(step[2])]:
                        gu_prod(int(step[1]), i, b.setdefault(step[:2], {}), an[step], slabs)
                elif step[0] == 'F':
                    j, c = int(step[1]), int(step[2])
                    slabs = [int(step[3])]
                    hv = b.setdefault(step[:2], {})
                    gu_col(b['S' + step[1]], hv, j, c, an[step], slabs)
                    if len(hv) == 3 * NS:
                        b[j] = h_join(hv)
                else:
                    js = [int(c) for c in step[1:]]
                    acc = down_mm(acc, [b[j] for j in js], js[0], an[step])
            finish(bu, acc)

            @pl.when(u >= NB)
            def _():
                out_copy(bu).start()
            return carry

        if scopes:
            with jax.named_scope('LOOP'):
                lax.fori_loop(1, NU - 1, body, 0)
        elif 'main' in cfg['phases']:
            lax.fori_loop(1, NU - 1, body, 0)

        LP = 3

        def last(c, carry):
            b = [gu_piece(LP * c + j) for j in range(LP)]
            acc = down_mm(load_acc(1), b[:-1], LP * c, [])
            acc = down_mm(acc, b[-1:], LP * c + LP - 1, [])
            store_acc(1, acc)
            finish(NB - 1, acc)
            return carry

        if 'last' in cfg['phases']:
            lax.fori_loop(0, NP // LP, last, 0)
        if len(cfg['phases']) < 3:
            def keep(i, c):
                v = (gs_s[i, i, :8, :LANES] + us_s[i, i, :8, :LANES] + ds_s[i, i, :8, :LANES]
                     + wl_s[rows8(i * 8), :LANES] + a_s[i, :8] + qkv_s[i, :8]
                     + b_s[rows8(i * 8), :LANES] + wt_s[rows8(i * 8), :LANES])
                acc_s[1, 0, :8] = (lax.bitcast_convert_type(v, F32) + o_s[i, :8]
                                   + acc_s[i, i, :8])
                return c
            lax.fori_loop(0, 2, keep, 0)
            finish(NB - 1, load_acc(1))
        out_copy(NB - 1).start()
        wait('WOUT', [out_copy(b) for b in range(NB)])

    scratch = [
        pltpu.VMEM((NB, D, TM), BF16),
        pltpu.VMEM((D, 3 * D), BF16),
        pltpu.VMEM((D, D), BF16),
        pltpu.VMEM((NP, 3, D, PW), BF16),
        pltpu.VMEM((NP, 3, D, PW), BF16),
        pltpu.VMEM((NP, 3, D, PW), BF16),
        pltpu.VMEM((2 * D, 8 * LANES), U32),
        pltpu.VMEM((4 * Q3, 16 * LANES), U32),
        pltpu.VMEM((NP, 15, Q3, PW), U32),
        pltpu.VMEM((NP, 15, Q3, PW), U32),
        pltpu.VMEM((NP, 9, Q3, PW), U32),
        pltpu.VMEM((NB, D, TM), F32),
        pltpu.VMEM((54, TH // 2, LANES), U32),
        pltpu.VMEM((S // LANES + 1, 3 * RP, LANES), U32),
        pltpu.VMEM((NT, D, LANES), F32),
        pltpu.VMEM((2, 15, D3, TH), F32),
        pltpu.VMEM((15 * TH // 2, PW), U32),
        pltpu.VMEM((1, 9 * 64, 2 * LANES), U32),
        pltpu.SemaphoreType.DMA((SEM_P + NP + 2,)),
        pltpu.SemaphoreType.DMA((1,)),
    ]

    def wrapped(*refs):
        @pl.when(pl.program_id(0) == 0)
        def _():
            kernel(*refs)

    return wrapped, scratch


_CFG = dict(
    scopes=False,
    sub='abc',
    phases=('pre', 'main', 'last'),
    body=('S010', 'S000', 'F000', 'S020', 'F010', 'F020', 'S011', 'S001', 'S110',
        'S021', 'F021', 'S100', 'F100', 'S120', 'F001', 'S101', 'F110', 'F011', 'F120',
        'Q', 'S111', 'F101', 'S121', 'F111', 'F121', 'S300', 'S200', 'S210', 'S220',
        'F200', 'F210', 'F220', 'S201', 'S221', 'S211', 'F201', 'S320', 'F211', 'F221',
        'S310', 'D01', 'F300', 'S301', 'S311', 'F301', 'S321', 'F311', 'F321', 'S400',
        'F310', 'S420', 'F320', 'S410', 'S401', 'F410', 'F420', 'S411', 'F400', 'S421',
        'F411', 'F421', 'S500', 'D23', 'F401', 'S501', 'S510', 'S520', 'F500', 'W',
        'F520', 'S511', 'F510', 'S521', 'F501', 'F511', 'F521', 'D4', 'D5', 'L'),
    ln1=(('S010', 2), ('S010', 3), ('S010', 5), ('S010', 6), ('S010', 8), ('S000', 0),
        ('S000', 2), ('S000', 3), ('S000', 5)),
    ln1b=(('S110', 2), ('S110', 3), ('S110', 5), ('S110', 6), ('S110', 8), ('S021', 0),
        ('S021', 2), ('S021', 3), ('S021', 5), ('S021', 6), ('S021', 8), ('F021', 0)),
    att=(('S300', 6), ('D01', 2), ('D01', 6), ('D01', 7), ('D01', 10), ('F300', 4),
        ('D23', 5), ('D23', 9)),
    lhs=(('S521', 0), ('D5', 0), ('D5', 4)),
    a_w1=(0, 0, 1, 2, 2, 3, 3, 4, 4, 5, 6, 7),
    a_w2=(20, 23, 26, 30, 33, 36, 40, 43, 46, 50, 53, 57),
    a_ln=(0, 3, 6),
    a_lnb=(5, 9, 9),
    z_g=(5, 6, 7, 8, 11, 11, 12, 13, 14, 15, 17, 18, 19, 20, 21, 22, 23, 24, 25, 26, 28,
        29, 30, 31, 32, 35, 36, 37, 38, 40, 41, 42, 43, 45, 46, 47, 48, 49, 50, 51, 52,
        54, 55, 57, 58, 59, 60, 62),
    z_att=(53, 54, 56),
    t_d=(0, 0, 1, 1, 2, 3, 3, 4, 5, 6, 6, 7, 8, 9, 9, 9, 10, 11, 11, 12, 13, 14, 15,
        16),
    p_d=(26, 26, 27, 27, 29, 29, 29, 30, 31, 31, 32, 33, 33, 34, 35, 35, 36, 36, 37, 37,
        38, 39, 39, 41),
    p_att=(59,),
    p_w=(12, 60, 62, 65, 65),
    z_l=(2, 13, 32),
    f_g0=(0, 0, 0, 1, 1, 2, 2, 3, 4, 4, 4, 5),
    f_g1=(4, 6, 7, 7, 8, 10, 10, 11, 11, 12, 13, 14),
    f_g2=(5, 10, 11, 11, 13, 15, 16, 17, 19, 20, 21, 22),
    f_g3=(6, 7, 14, 16, 17, 18, 19, 19, 21, 22, 23, 23, 24, 25, 27, 28, 29, 30, 31, 33,
        34, 36, 36, 37),
    a_k=(15, 19, 20, 24),
    a_k2=(0, 4, 8, 12),
    a_v=(13, 14, 22, 26, 30, 34, 38, 39),
    a_att=(12, 60),
    a_wo=(30, 35, 36, 38, 41),
)


def _run(A_x, A_wqkv, A_wo, B_w_gate, B_w_up, B_w_down, **kw):
    _, S, D = A_x.shape
    F = B_w_gate.shape[1]
    kernel, scratch = _make_kernel(S, D, F, 256, {**_CFG, **kw})
    hbm = pl.BlockSpec(memory_space=pl.ANY)
    out_t = pl.pallas_call(
        kernel,
        grid=(2,),
        in_specs=[hbm] * 6,
        out_specs=hbm,
        out_shape=jax.ShapeDtypeStruct((D, S), A_x.dtype),
        scratch_shapes=scratch,
        compiler_params=pltpu.CompilerParams(
            dimension_semantics=('arbitrary',), vmem_limit_bytes=110 * 1024 * 1024),
    )(A_x.reshape(S, D).T, A_wqkv, A_wo, B_w_gate, B_w_up, B_w_down.T)
    return out_t.T.reshape(A_x.shape)


@jax.jit
def pallas_interleave_layers__sliding_local_dilated__glu_gated_geglu__prompt_kernel(
    A_x: jax.Array,
    A_wqkv: jax.Array,
    A_wo: jax.Array,
    B_x: jax.Array,
    B_w_gate: jax.Array,
    B_w_up: jax.Array,
    B_w_down: jax.Array,
):
    del B_x
    return _run(A_x, A_wqkv, A_wo, B_w_gate, B_w_up, B_w_down)
```

```python
import jax
import jax.numpy as jnp
import jax.experimental.pallas as pl
import jax.experimental.pallas.tpu as pltpu
from jax import lax

H = 32
W = 8
DIL = 2
EPS = 1e-5
LANES = 128

F32 = jnp.float32
BF16 = jnp.bfloat16
U32 = jnp.uint32

_NT = (((1,), (1,)), ((), ()))


def _tree_sum(parts, op=jnp.add):
    while len(parts) > 1:
        nxt = [op(parts[i], parts[i + 1]) for i in range(0, len(parts) - 1, 2)]
        if len(parts) % 2:
            nxt.append(parts[-1])
        parts = nxt
    return parts[0]


def _ln_stats(slabs, d, anchors=()):
    n_acc = 4
    s1, s2, pilot = [None] * n_acc, [None] * n_acc, None
    for i, x in enumerate(slabs):
        if pilot is None:
            pilot = x[0:1, :]
            pil = jnp.broadcast_to(pilot, x.shape)
            pils = [_tie(pil, a) for a in anchors] or [pil]
        dx = x - pils[i * len(pils) // (d // 8)]
        j = i % n_acc
        s1[j] = dx if s1[j] is None else s1[j] + dx
        s2[j] = dx * dx if s2[j] is None else s2[j] + dx * dx
    e1 = jnp.sum(_tree_sum(s1), axis=0, keepdims=True) * (1.0 / d)
    e2 = jnp.sum(_tree_sum(s2), axis=0, keepdims=True) * (1.0 / d)
    var = jnp.maximum(e2 - e1 * e1, 0.0)
    return pilot + e1, lax.rsqrt(var + EPS)


def _zero_like_dep(v):
    return (lax.bitcast_convert_type(v, U32) >> 31) >> 1


def _tie(x, anchor):
    if anchor is None:
        return x
    z = lax.bitcast_convert_type(_zero_like_dep(anchor), F32)
    z = jnp.concatenate([z] * -(-x.shape[1] // LANES), axis=1)[:, :x.shape[1]]
    if x.shape[0] == 8:
        return x + z
    return jnp.concatenate([x[:8] + z, x[8:]], axis=0)


def _gelu_mul2(g, u):
    c0 = 0.7978845608028654
    c1 = c0 * 0.044715
    t = jnp.tanh(g * (c0 + c1 * (g * g)))
    return (g * u) * (1.0 + t)


def _lo(x):
    return lax.bitcast_convert_type(x << 16, F32)


def _hi(x):
    return lax.bitcast_convert_type(x & jnp.uint32(0xFFFF0000), F32)


def _pk(x):
    return pltpu.bitcast(x.astype(BF16), U32)


def _upk(x):
    return pltpu.bitcast(x, BF16)


def _dot(a, b):
    return jnp.dot(a, b, preferred_element_type=F32)


def _dot_nt(a, b):
    return lax.dot_general(a, b, _NT, preferred_element_type=F32)


def _x_ops(x1, x2):
    d = [a - b for a, b in zip(x1, x2)]
    return [x1[0] + x2[1], x2[0] + x2[1], x1[0] + x1[1],
            d[1] + x1[2], x1[1] + x1[2], d[1] + d[2],
            d[0] - x2[2], d[0] + d[2], x2[0] + x2[2],
            x1[0], d[0], x2[1], d[1], x1[2], x2[2]]


def _x_rem(x1, x2):
    a, b, c = 0, 1, 2
    cat = lambda u, v: jnp.concatenate([u, v], axis=0)
    return [cat(x1[c], x2[b]), cat(x1[a], x1[b] - x2[b]), cat(x2[a], x2[c] - x1[c])]


_W_TERMS = {0: ((0, 1, 1), (1, 0, 1)), 3: ((1, 2, 1), (2, 1, 1)), 6: ((0, 2, 1), (2, 0, 1)),
            9: ((0, 0, 1), (0, 2, 1), (1, 0, -1)), 10: ((2, 0, 1), (0, 0, -1), (0, 1, -1)),
            11: ((1, 1, 1), (1, 2, 1), (0, 1, -1)), 12: ((1, 0, 1), (1, 1, 1), (2, 1, -1)),
            13: ((2, 0, 1), (2, 2, 1), (1, 2, -1)), 14: ((2, 1, 1), (2, 2, 1), (0, 2, -1)),
            1: ((0, 1, 1),), 2: ((1, 0, 1),), 4: ((1, 2, 1),), 5: ((2, 1, 1),),
            7: ((2, 0, 1),), 8: ((0, 2, 1),)}


def _w_sums(w):
    return [_signed(_W_TERMS[i], lambda k, j: w[k][j]) for i in _W_SUM]


_W_SUM = {0: 0, 3: 1, 6: 2, 9: 3, 10: 4, 11: 5, 12: 6, 13: 7, 14: 8}
_W_RAW = {1: (0, 1), 2: (1, 0), 4: (1, 2), 5: (2, 1), 7: (2, 0), 8: (0, 2)}
_PAIR_ORDER = (1, 2, 4, 5, 7, 8, 0, 3, 6)
_DIAG = {(0, 0): 9, (2, 0): 10, (0, 1): 11, (1, 1): 12, (1, 2): 13, (2, 2): 14}
_PAIR = {(0, 0): ((6, -1), (8, -1)), (1, 0): ((2, 1), (7, 1)), (2, 0): ((0, 1), (1, -1)),
         (0, 1): ((3, 1), (4, -1)), (1, 1): ((0, 1), (2, -1)), (2, 1): ((1, 1), (5, -1)),
         (0, 2): ((4, 1), (8, 1)), (1, 2): ((6, 1), (7, -1)), (2, 2): ((5, 1), (3, -1))}


def _column(t, base, j, skew=False):
    s = []
    for k in range(3):
        v = base[k]
        for i, sg in _PAIR[k, j]:
            v = t[i] if v is None else (v + t[i] if sg > 0 else v - t[i])
        s.append(v)
    if skew:
        return s[1] + s[0], s[2] + 0.5 * (s[0] - s[1])
    return s[1] + s[0], s[2] + s[0]


_SA = (((0, 0, 1), (1, 1, 1)), ((1, 0, 1), (1, 1, 1)), ((0, 0, 1),), ((1, 1, 1),),
       ((0, 0, 1), (0, 1, 1)), ((1, 0, 1), (0, 0, -1)), ((0, 1, 1), (1, 1, -1)))
_SB = (((0, 0, 1), (1, 1, 1)), ((0, 0, 1),), ((0, 1, 1), (1, 1, -1)), ((1, 0, 1), (0, 0, -1)),
       ((1, 1, 1),), ((0, 0, 1), (0, 1, 1)), ((1, 0, 1), (1, 1, 1)))
_SCOL = {2: 1, 3: 0, 5: 1, 6: 0}


def _signed(terms, f):
    v = None
    for a, b, sg in terms:
        v = f(a, b) if v is None else (v + f(a, b) if sg > 0 else v - f(a, b))
    return v


def _s_out(m):
    return [[m[0] + m[3] - m[4] + m[6], m[2] + m[4]],
            [m[1] + m[3], m[0] - m[1] + m[2] + m[5]]]


def _make_kernel(S, D, F, TM, cfg):
    NB = S // TM
    NT = TM // LANES
    DH = D // H
    DP = DH // 2
    RP = D // 2
    NG = H // 8
    scale = float(DH) ** -0.5
    NU = 2 * NB
    TH = TM // 2
    TQ = TM // 4
    D2 = D // 2
    D3 = D // 3
    Q3 = D3 // 2
    KU = D // 9
    KR = 3 * LANES
    NQ = 6
    QR = 3 * D // NQ
    WQ = (0, 640, 1152, 3 * D)
    PW = 4 * LANES
    NP = F // PW
    AOFF, fill = {}, [0, 0]
    for key in [(m1, m2) for m1 in range(7) for m2 in range(7)] + list(range(9)):
        c = int(fill[1] < fill[0])
        AOFF[key] = (fill[c], slice(c * LANES, (c + 1) * LANES))
        fill[c] += (64 if isinstance(key, int) else
                    48 if key[0] in _SCOL and key[1] in _SCOL else 32)
    scopes = cfg['scopes']
    assert NG == 4 and NB & (NB - 1) == 0
    SEM_P = 4

    def kernel(x_hbm, wqkv_hbm, wo_hbm, wg_hbm, wu_hbm, wdt_hbm, out_hbm,
               xio_s, wqkv_v, wo_v, wg_v, wu_v, wdt_v, wt_s, wl_s,
               gu_s, ds_s, xmid_s, a_s, qkv_s, o_s, acc_s, b_s, h3_s, r_s,
               sem_i, sem_o):

        def wait(name, cps):
            if scopes:
                with jax.named_scope(name):
                    for cp in cps:
                        cp.wait()
            else:
                for cp in cps:
                    cp.wait()

        def cols(lo, n):
            if not isinstance(lo, int):
                lo = pl.multiple_of(lo, LANES)
            return pl.ds(lo, n)

        def rows8(lo, n=8):
            if not isinstance(lo, int):
                lo = pl.multiple_of(lo, 8)
            return pl.ds(lo, n)

        def out_copy(b):
            return pltpu.make_async_copy(
                xio_s.at[b], out_hbm.at[:, cols(b * TM, TM)], sem_o.at[0])

        def x_cp(b, sem):
            return pltpu.make_async_copy(x_hbm.at[:, cols(b * TM, TM)], xio_s.at[b],
                                         sem_i.at[sem])

        def wq_cp(i):
            sl = cols(WQ[i], WQ[i + 1] - WQ[i])
            return pltpu.make_async_copy(wqkv_hbm.at[:, sl], wqkv_v.at[:, sl],
                                         sem_i.at[1 + i])

        def piece_cp(src, dst, p, sem):
            return [pltpu.make_async_copy(src.at[:, cols(p * PW, PW)], dst.at[p],
                                          sem_i.at[sem])]

        def group_cp(p):
            sem = SEM_P + p
            cps = []
            if not (isinstance(p, int) and p == NP):
                cps += piece_cp(wg_hbm, wg_v, p, sem) + piece_cp(wu_hbm, wu_v, p, sem)
            if not (isinstance(p, int) and p == 0):
                cps += piece_cp(wdt_hbm, wdt_v, p - 1, sem)
            return cps

        lane = lax.broadcasted_iota(jnp.int32, (8, LANES), 1)
        cat0 = lambda *v: jnp.concatenate(v, axis=0)
        cat1 = lambda *v: jnp.concatenate(v, axis=1)

        def spread_over(anchors, n, total):
            return anchors[n * len(anchors) // total] if anchors else None

        def slab_group(r):
            return (r % LANES) // 16 if r < KR else 8 + ((r - KR) % KU) // 16

        def ln1(blk, anchors1, anchors2=()):
            slabs = (xio_s[blk, r:r + 8, :].astype(F32) for r in range(0, D, 8))
            m, rs = _ln_stats(slabs, D, anchors1)
            if not anchors2:
                return (xio_s[blk].astype(F32) - m) * rs
            m8 = jnp.broadcast_to(m, (8, TM))
            ms = [_tie(m8, a) for a in anchors2]
            ms = [spread_over(ms, slab_group(r), 12) for r in range(0, D, 8)]
            return (xio_s[blk].astype(F32) - cat0(*ms)) * rs

        def dot_k(rows, x, anchors, even=False):
            y = None
            for n, k in enumerate(range(0, D, LANES)):
                ks = slice(k, min(k + LANES, D))
                if even and k + LANES >= D:
                    mid = (rows.start + rows.stop) // 2
                    v = cat0(_dot(_upk(wt_s[rows.start:mid, ks]), x[ks]),
                             _dot(_upk(wt_s[mid:rows.stop, ks]), x[ks]))
                else:
                    v = _dot(_upk(wt_s[rows, ks]), x[ks])
                anchors.extend(v[r:r + 8, :LANES] for r in ((0, 144) if n % 2 else (72, 216)))
                y = v if y is None else y + v
            return y

        def put_qkv(blk, rows, y):
            pk = _pk(y)
            for c in range(NT):
                qkv_s[1 + blk * NT + c, rows, :] = pk[:, c * LANES:(c + 1) * LANES]

        def qkv_mm(blk, xn, chunks, anchors, even=False):
            for r in chunks:
                rows = slice(r * QR // 2, (r + 1) * QR // 2)
                put_qkv(blk, rows, dot_k(rows, xn, anchors, even))

        def split_k(x):
            hs = (x[:, :TH], x[:, TH:])
            blocks = [[h[k * LANES:(k + 1) * LANES] for k in range(3)] for h in hs]
            units = [[h[KR + k * KU:KR + (k + 1) * KU] for k in range(3)] for h in hs]
            return blocks, units

        def prep_att(pat, anchor):
            assert Q3 == 96
            row0 = pat * 8
            src0 = row0 + ((pat * 43) >> 9) * (2 * Q3)
            w = [_upk(wt_s[rows8(src0 + j * Q3), :D]).astype(F32) for j in range(3)]
            w[0] = cat1(_tie(w[0][:, :LANES], anchor), w[0][:, LANES:])
            tiles = _w_sums([[w[j][:, k * LANES:(k + 1) * LANES] for j in range(3)]
                             for k in range(3)])
            for j in range(3):
                a, b, c = (w[j][:, KR + k * KU:KR + (k + 1) * KU] for k in range(3))
                tiles += [cat1(c, b), cat1(a, c)]
            wl_s[rows8(row0), :15 * LANES] = _pk(cat1(*tiles))

        def att_rhs(x, stash=None):
            blocks, units = split_k(cat1(x[:, :TH], x[:, TH:] + 0.5 * x[:, :TH]))
            ops = _x_ops(*blocks) + _x_rem(*units)
            if stash is None:
                return [v.astype(BF16) for v in ops]
            loc = lambda i, r0, n: (slice((i // 2) * 64 + r0, (i // 2) * 64 + r0 + n),
                                    slice((i % 2) * LANES, (i % 2 + 1) * LANES))
            for r in range(0, LANES, 16):
                for i, v in enumerate(ops):
                    r_s.at[0][loc(i, r // 2, 8)] = _pk(v[r:r + 16])
            return [_upk(r_s.at[stash][loc(i, 0, 64)]) for i in range(18)]

        def att_mm(sec, rhs, anchors):
            tl = lambda i: _upk(wl_s[sec * Q3:(sec + 1) * Q3, i * LANES:(i + 1) * LANES])
            raw = lambda k, j: _upk(wt_s[(3 * sec + j) * Q3:(3 * sec + j + 1) * Q3,
                                         k * LANES:(k + 1) * LANES])
            t = {}
            for i in _PAIR_ORDER:
                t[i] = _dot(raw(*_W_RAW[i]) if i in _W_RAW else tl(_W_SUM[i]), rhs[i])
                anchors.append(t[i][:8])
            out = []
            for j in range(3):
                base = []
                for s in range(3):
                    v = _dot(raw(3, j) if s == 1 else tl(9 + 2 * j + s // 2), rhs[15 + s])
                    if (s, j) in _DIAG:
                        i = _DIAG[s, j]
                        v = _dot(tl(_W_SUM[i]), rhs[i]) + v
                    base.append(v)
                    anchors.append(base[-1][:8])
                out.append(cat1(*_column(t, base, j, True)))
            return cat0(*out)

        def qkv_fast(blk, rhs, anchors):
            for sec in range(3):
                put_qkv(blk, slice(sec * RP, (sec + 1) * RP), att_mm(sec, rhs, anchors))

        def shifted(ln, cur, prev, w):
            if w == 0:
                return cur
            sh = DIL * w
            return pltpu.roll(jnp.where(ln < LANES - sh, cur, prev), sh, axis=1)

        def att_group(blk, c, hg, anchor):
            att_values(blk, c, hg, anchor)(None)

        def att_values(blk, c, hg, anchor):
            tile = blk * NT + c
            base = hg * 8 * DP
            if isinstance(hg, int):
                cur, prev, o_t = qkv_s.at[1 + tile], qkv_s.at[tile], o_s.at[c]
            else:
                n = 2 * RP + 8 * DP
                base = pl.multiple_of(base, 8)
                cur = qkv_s.at[1 + tile, pl.ds(base, n)]
                prev = qkv_s.at[tile, pl.ds(base, n)]
                o_t = o_s.at[c, pl.ds(base, RP + 8 * DP)]
                base = 0
            ln = lane + _zero_like_dep(anchor).astype(jnp.int32)
            logits = [None] * W
            for dd in range(DP):
                q = cur[pl.ds(base + dd, 8, stride=DP), :]
                kc = cur[pl.ds(RP + base + dd, 8, stride=DP), :]
                kp = prev[pl.ds(RP + base + dd, 8, stride=DP), :]
                q0, q1 = _lo(q), _hi(q)
                for w in range(W):
                    ks = shifted(ln, kc, kp, w)
                    t = q0 * _lo(ks) + q1 * _hi(ks)
                    logits[w] = t if logits[w] is None else logits[w] + t
            logits = [l * scale for l in logits]
            if not (isinstance(c, int) and c > 0):
                pos = lane + tile * LANES
                logits = [l if w == 0 else jnp.where(pos >= DIL * w, l, -1e9)
                          for w, l in enumerate(logits)]
            m = _tree_sum(logits, jnp.maximum)
            p = [jnp.exp(l - m) for l in logits]
            r = 1.0 / _tree_sum(p)

            def apply(anchor2):
                ln = lane + _zero_like_dep(m if anchor2 is None else anchor2).astype(jnp.int32)
                for dd in range(DP):
                    vc = cur[pl.ds(2 * RP + base + dd, 8, stride=DP), :]
                    vp = prev[pl.ds(2 * RP + base + dd, 8, stride=DP), :]
                    o0 = o1 = None
                    for w in range(W):
                        vs = shifted(ln, vc, vp, w)
                        t0, t1 = p[w] * _lo(vs), p[w] * _hi(vs)
                        o0 = t0 if o0 is None else o0 + t0
                        o1 = t1 if o1 is None else o1 + t1
                    o0, o1 = o0 * r, o1 * r
                    o_t[pl.ds(base + dd, 8, stride=DP), :] = o0
                    o_t[pl.ds(RP + base + dd, 8, stride=DP), :] = o1

            return apply

        def attention(blk, anchors):
            for c in range(NT):
                for hg in range(NG):
                    att_group(blk, c, hg, anchors[c * NG + hg])

        def wo_mm(blk, anchors, fast, stash=None):
            o = cat1(*[o_s[c] for c in range(NT)])
            if fast:
                y = att_mm(3, att_rhs(o, stash), anchors)
            else:
                o = o.astype(BF16)
                q = D2 // 2
                y = cat0(*[dot_k(slice(h * q, (h + 1) * q), o, anchors) for h in (6, 7)])
            xm = xio_s[blk].astype(F32) + y
            xmid_s[blk] = xm
            return _ln_stats((xm[r:r + 8] for r in range(0, D, 8)), D)

        def ffn_lhs(blk, stats, anchors):
            m, rs = stats
            m8 = jnp.broadcast_to(m, (8, TM))
            xt = []
            for k in range(5):
                mt = cat0(*[_tie(m8, spread_over(anchors[:2], k, 5))] * (KU // 8 if k == 4 else 16))
                x = (xmid_s[blk, k * LANES:min((k + 1) * LANES, D), :] - mt) * rs
                xt.append((cat0(x, x) if k == 4 else x).T)
            lo = lax.broadcasted_iota(jnp.int32, (TQ // 2, LANES), 1) < KU
            for m1 in range(7):
                a = spread_over(anchors[2:], m1, 7)
                blk1 = lambda i2, k2: _signed(_SA[m1], lambda i1, k1: _tie(
                    xt[k2 if k2 == 4 else 2 * k1 + k2][(2 * i1 + i2) * TQ:(2 * i1 + i2 + 1) * TQ], a))
                l1 = {(i2, k2): blk1(i2, k2) for i2 in range(2)
                      for k2 in ((0, 1, 4) if m1 in _SCOL else (0, 1))}
                for m2 in range(7):
                    v = _signed(_SA[m2], lambda i2, k2: l1[i2, k2])
                    if m1 in _SCOL and m2 in _SCOL:
                        c = _signed(_SA[m2], lambda i2, k2: l1[i2, 4])
                        h = TQ // 2
                        vp, vq, cp, cq = v[:h], v[h:], c[:h], c[h:]
                        v = cat0(jnp.where(lo, cp, vq), jnp.where(lo, vp, vp - vq),
                                 jnp.where(lo, vq, cq - cp))
                    o, ac = AOFF[m1, m2]
                    a_s[o:o + v.shape[0] // 2, ac] = _pk(v)

        def plain_lhs(blk, stats):
            m, rs = stats
            blocks, units = split_k((xmid_s[blk] - m) * rs)
            for i, v in enumerate(blocks[0] + blocks[1] + _x_rem(*units)):
                a_s[AOFF[i][0]:AOFF[i][0] + 64, AOFF[i][1]] = _pk(v.astype(BF16).T)

        def plain_piece(p, anchors):
            h = []
            for n in range(4):
                cs = slice(n * LANES, (n + 1) * LANES)
                w = lambda r0, r1: cat1(wg_v[p, r0:r1, cs], wu_v[p, r0:r1, cs])
                u = lambda k: w(KR + k * KU, KR + (k + 1) * KU)
                tl = lambda *i: _upk(cat1(*[a_s[AOFF[k][0]:AOFF[k][0] + 64, AOFF[k][1]]
                                            for k in i]))
                y0 = _dot(tl(6), cat0(u(2), u(1)))
                y1 = _dot(tl(0, 1, 2, 7), w(0, KR + 2 * KU))
                y2 = _dot(tl(3, 4, 5, 8), cat0(w(0, KR + KU), u(2)))
                anchors.append(y0[:8, :LANES])
                for y in (y1, y2):
                    anchors.extend(y[r:r + 8, c:c + LANES] for c in (0, LANES)
                                   for r in (0, TH // 2))
                h.append([_gelu_mul2(*[(y + y0)[:, c:c + LANES] for c in (0, LANES)])
                          for y in (y1, y2)])
            return h

        def in_triple(q):
            return q, lambda k: (q, k)

        def cross_triple(s):
            return NP + s, lambda k: (3 * s + k, 3)

        def wd_raw(tri, k, r0, n):
            q, c = tri[1](k)
            return wdt_v[q, r0:r0 + n, c * LANES:(c + 1) * LANES]

        def ds_loc(i, r0, n):
            return slice(r0, r0 + n), slice((i % 2) * LANES, (i % 2 + 1) * LANES)

        def prep_d(tri, anchors):
            PR = 16
            for n in range(D3 // PR):
                r = n * PR
                w = [[wd_raw(tri, k, j * D3 + r, PR).astype(F32) for j in range(3)]
                     for k in range(3)]
                w[0][1] = _tie(w[0][1], spread_over(anchors, n, D3 // PR))
                for i, v in enumerate(_w_sums(w)):
                    ds_s.at[tri[0], i // 2][ds_loc(i, r // 2, PR // 2)] = _pk(v)

        GU = (wg_v, wu_v)

        def prep_gu(p, m, m1, anchors):
            PR = 16
            cs = slice(m * LANES, (m + 1) * LANES)
            for n in range(LANES // PR):
                r = n * PR
                a = spread_over(anchors, n, LANES // PR)
                b1 = [_signed(_SB[m1], lambda k1, j1: _tie(
                    GU[m][p, (2 * k1 + k2) * LANES + r:(2 * k1 + k2) * LANES + r + PR,
                          2 * j1 * LANES:2 * (j1 + 1) * LANES].astype(F32),
                    a if (k1, j1) == _SB[m1][0][:2] else None)) for k2 in range(2)]
                for m2 in range(7):
                    v = _signed(_SB[m2], lambda k2, j2: b1[k2][:, j2 * LANES:(j2 + 1) * LANES])
                    gu_s.at[p, 7 * m1 + m2][r // 2:(r + PR) // 2, cs] = _pk(v)

        def prep_tail(p, m, anchor):
            v = _tie(GU[m][p, 4 * LANES:, :].astype(F32), anchor)
            for j in range(4):
                gu_s.at[p, 49 + j // 2][(j % 2) * 32:(j % 2 + 1) * 32,
                                        m * LANES:(m + 1) * LANES] = _pk(
                                            v[:, j * LANES:(j + 1) * LANES])

        def gu_outer(p, m, m1, anchors):
            cs = slice(m * LANES, (m + 1) * LANES)
            y = {}
            for m2 in cfg['inner']:
                i, (o, ac) = 7 * m1 + m2, AOFF[m1, m2]
                if m1 in _SCOL and m2 in _SCOL:
                    j = 2 * _SCOL[m1] + _SCOL[m2]
                    tail = lambda: gu_s[p, 49 + j // 2, (j % 2) * 32:(j % 2 + 1) * 32, cs]
                    rhs = (cat0(tail(), gu_s[p, i, 32:, cs]), gu_s[p, i, :, cs],
                           cat0(gu_s[p, i, :32, cs], tail()))
                    r = [_dot(_upk(a_s[o + 16 * s:o + 16 * (s + 1), ac]), _upk(rhs[s]))
                         for s in range(3)]
                    y[m2] = cat0(r[1] + r[0], r[2] + r[0])
                else:
                    y[m2] = _dot(_upk(a_s[o:o + TQ // 2, ac]), _upk(gu_s[p, i, :, cs]))
            anchors.append(y[cfg['inner'][0]][:8])
            anchors.append(y[cfg['inner'][4]][:8])
            return _s_out(y)

        def gu_finish(t):
            gu = [{(i2, j2): _s_out([t[m][m1][i2][j2] for m1 in range(7)])
                   for i2 in range(2) for j2 in range(2)} for m in range(2)]
            return [[cat0(*[_gelu_mul2(*[gu[m][i2, j % 2][i1][j // 2] for m in range(2)])
                            for i2 in range(2)]) for i1 in range(2)] for j in range(4)]

        def gu_piece(p, anchors):
            t = ({}, {})
            for m, m1 in cfg['gorder']:
                t[m][m1] = gu_outer(p, m, m1, anchors)
            return gu_finish(t)

        def h_ops(h):
            return [v.astype(BF16) for v in _x_ops(*[[h[k][i] for k in range(3)]
                                                     for i in range(2)])]

        D_ORDER = _PAIR_ORDER + (9, 10, 11, 12, 13, 14)

        def down_mm(acc, work, anchors, which=D_ORDER, fine=False):
            p = [None] * 15 if acc is None else list(acc)
            jobs = [(i, n) for i in which for n in range(len(work))]
            split = {0: (), 1: (4,), 2: (2, 2), 3: (2, 2, 4)}[len(jobs) % 4]
            split = dict(zip(jobs[len(jobs) - len(split):], split))
            for i in which:
                y = None
                for n, (tri, b) in enumerate(work):
                    ns = split.get((i, n), 1)
                    nr = D3 // ns
                    if i in _W_RAW:
                        k, j = _W_RAW[i]
                        lhs = lambda h: wd_raw(tri, k, j * D3 + h * nr, nr)
                    else:
                        s = _W_SUM[i]
                        lhs = lambda h: _upk(ds_s.at[tri[0], s // 2][ds_loc(s, h * nr // 2, nr // 2)])
                    v = cat0(*[_dot_nt(lhs(h), b[i]) for h in range(ns)])
                    y = v if y is None else y + v
                p[i] = y if p[i] is None else p[i] + y
                anchors.append(p[i][:8])
                if fine:
                    anchors.append(p[i][D3 // 2:D3 // 2 + 8])
            return p

        def finish(blk, acc):
            y = [cat1(*_column(acc, [acc[_DIAG[s, j]] if (s, j) in _DIAG else None
                                     for s in range(3)], j)) for j in range(3)]
            xio_s[blk] = (xmid_s[blk] + 0.5 * cat0(*y)).astype(BF16)

        def load_acc(k):
            return [acc_s[k, i] for i in range(15)]

        def store_acc(k, acc):
            for i in range(15):
                acc_s[k, i] = acc[i]

        def b_loc(i):
            return (slice((i // 2) * 64, (i // 2 + 1) * 64),
                    slice((i % 2) * LANES, (i % 2 + 1) * LANES))

        def load_b():
            return [_upk(b_s[b_loc(i)]) for i in range(15)]

        def store_h(p, h):
            for i, v in enumerate(h_ops(h[:3])):
                b_s[b_loc(i)] = _pk(v)
            h3_s[p] = cat0(*h[3])

        def pre_phase():
            first = [[x_cp(0, 0)], [wq_cp(0)], [x_cp(1, 2), wq_cp(1)],
                     [wq_cp(2), pltpu.make_async_copy(wo_hbm, wo_v, sem_i.at[3])]]
            order = sum(first, [])
            for p in range(NP + 1):
                order += group_cp(p)
            xr_cp = [x_cp(b, SEM_P + NP + 1) for b in range(2, NB)]
            order += xr_cp
            for cp in order:
                cp.start()
            get = lambda an, name: [an[min(i, len(an) - 1)] for i in cfg[name]]
            e_grp = lambda e: ((e >> 1) & 1, ((e >> 2) << 1) | (e & 1))
            if 'a' in cfg['sub']:
                pre_a(first, get, e_grp)
            if 'b' in cfg['sub']:
                pre_b(get, e_grp)
            if 'c' in cfg['sub']:
                pre_c(get)
            wait('WX', xr_cp)

        def pre_a(first, get, e_grp):
            def transpose_wq(i):
                wt_s[WQ[i] // 2:WQ[i + 1] // 2, :D] = _pk(wqkv_v[:, WQ[i]:WQ[i + 1]].T)

            def clear(i, carry):
                for k in range(2):
                    acc_s[k, i] = jnp.zeros((D3, TH), F32)
                r = jnp.minimum(i, 11) * (RP // 4)
                qkv_s[0, rows8(r, RP // 4)] = jnp.zeros((RP // 4, LANES), U32)
                return carry

            lax.fori_loop(0, 15, clear, 0)
            wait('WX0', first[0])
            xn0 = ln1(0, ()).astype(BF16)

            wait('WQ0', first[1])
            transpose_wq(0)
            qkv_mm(0, xn0, (0, 1), [])

            wait('WQ1', first[2])
            transpose_wq(1)
            an = []
            qkv_mm(0, xn0, (2, 3), an)
            xn1 = ln1(1, get(an, 'a_ln'), get(an, 'a_lnb')).astype(BF16)
            qkv_mm(1, xn1, (0,), an, True)
            for n, a in enumerate(get(an, 'a_w1')):
                prep_att(n, a)
            nk = len(cfg['a_k'])
            apply = [att_values(0, *e_grp(e), a) for e, a in enumerate(get(an, 'a_k'))]

            wait('WQ2', first[3])
            an = []
            qkv_mm(1, xn1, (2,), an)
            transpose_wq(2)
            qkv_mm(0, xn0, (4, 5), an)
            qkv_mm(1, xn1, (4, 1), an)
            apply += [att_values(0, *e_grp(nk + e), a)
                      for e, a in enumerate(get(an, 'a_k2')[:8 - nk])]
            for e, a in enumerate(get(an, 'a_v')):
                apply[e](a)
            wo = pltpu.bitcast(wo_v[...], U32)
            wo = cat0(_lo(wo), _hi(wo))
            wo = cat0(*[_tie(wo[n * LANES:(n + 1) * LANES], a)
                        for n, a in enumerate(get(an, 'a_wo'))])
            wt_s[3 * RP:, :D] = _pk(wo.astype(BF16).T)
            stats = wo_mm(0, an, False)
            qkv_mm(1, xn1, (3,), an)
            for n, a in enumerate(get(an, 'a_w2')):
                prep_att(12 + n, a)
            plain_lhs(0, stats)

            wait('WO', group_cp(0))
            an = []
            h = plain_piece(0, an)
            qkv_mm(1, xn1, (5,), an, True)
            zg = get(an, 'z_g')
            for n, (m, m1) in enumerate(cfg['gorder']):
                prep_gu(0, m, m1, zg[2 * n:2 * n + 2])
            for m in range(2):
                prep_tail(0, m, zg[m])
            ffn_lhs(0, stats, get(an, 'z_l'))
            store_h(0, h)

        def pre_b(get, e_grp):
            def piece(p, carry):
                wait('WP', group_cp(p))
                work = [(in_triple(p - 1), load_b())]
                an = []
                acc = down_mm(load_acc(0), work, an, D_ORDER[:6], True)
                t = ({}, {})
                for m in range(2):
                    prep_tail(p, m, get(an, 'f_t')[m])
                for n, (m, m1) in enumerate(cfg['gorder0']):
                    prep_gu(p, m, m1, get(an, 'f_g')[2 * n:2 * n + 2])
                    t[m][m1] = gu_outer(p, m, m1, an)
                h = gu_finish(t)
                prep_d(work[0][0], get(an, 'p_d'))
                store_acc(0, down_mm(acc, work, an, D_ORDER[6:]))
                att_group(1, *e_grp(p - 1), an[cfg['p_att'][0]])
                for i, a in enumerate(get(an, 'p_w')):
                    prep_att(21 + 3 * p + i, a)
                store_h(p, h)
                return carry

            lax.fori_loop(1, NP, piece, 0)

        def pre_c(get):
            wait('WD', group_cp(NP))
            work = [(in_triple(NP - 1), load_b())]
            for s in range(3):
                h3 = [h3_s[3 * s + k] for k in range(3)]
                work.append((cross_triple(s), h_ops([[v[:TH], v[TH:]] for v in h3])))
            an = []
            stats = wo_mm(1, an, True)
            acc = down_mm(load_acc(0), work, an, D_ORDER[:6], True)
            td = get(an, 't_d')
            for n, (tri, _) in enumerate(work):
                prep_d(tri, td[n * len(td) // 4:(n + 1) * len(td) // 4])
            acc = down_mm(acc, work, an, D_ORDER[6:])
            ffn_lhs(1, stats, get(an, 't_l'))
            finish(0, acc)

        if 'pre' in cfg['phases']:
            pre_phase()

        def body(u, carry):
            bu = u & (NB - 1)
            ba = (u + 1) & (NB - 1)
            acc, stats, an, b, hh = None, None, {}, {}, {}
            get = lambda name: [an[k][i] for k, i in cfg[name]]
            for step in cfg['body']:
                an[step] = []
                if step == 'Q':
                    xn = ln1(ba, get('ln1'), get('ln1b'))
                    qkv_fast(ba, att_rhs(xn, u >> 8), an[step])
                elif step == 'W':
                    attention(ba, get('att'))
                    stats = wo_mm(ba, an[step], True, u >> 8)
                elif step == 'L':
                    ffn_lhs(ba, stats, get('lhs'))
                elif step[0] == 'G':
                    q, go = int(step[1]), cfg['gorder']
                    t = b.setdefault(step[:2], ({}, {}))
                    for m, m1 in (go[:7] if step[2] == '0' else go[7:]):
                        t[m][m1] = gu_outer(q, m, m1, an[step])
                    if len(t[0]) + len(t[1]) == 14:
                        hh[q] = gu_finish(t)
                else:
                    work = []
                    for c in step[1:]:
                        if c.isdigit():
                            work.append((in_triple(int(c)), h_ops(hh[int(c)][:3])))
                        else:
                            s = ord(c) - ord('a')
                            work.append((cross_triple(s),
                                         h_ops([hh[3 * s + k][3] for k in range(3)])))
                    acc = down_mm(acc, work, an[step])
            finish(bu, acc)

            @pl.when(u >= NB)
            def _():
                out_copy(bu).start()
            return carry

        if scopes:
            with jax.named_scope('LOOP'):
                lax.fori_loop(1, NU - 1, body, 0)
        elif 'main' in cfg['phases']:
            lax.fori_loop(1, NU - 1, body, 0)

        def last(s, carry):
            h = [gu_piece(3 * s + k, []) for k in range(3)]
            work = [(in_triple(3 * s + k), h_ops(h[k][:3])) for k in range(3)]
            work.append((cross_triple(s), h_ops([h[k][3] for k in range(3)])))
            acc = down_mm(down_mm(load_acc(1), work[:2], []), work[2:], [])
            store_acc(1, acc)
            finish(NB - 1, acc)
            return carry

        if 'last' in cfg['phases']:
            lax.fori_loop(0, NP // 3, last, 0)
        if len(cfg['phases']) < 3:
            def keep(i, c):
                v = (gu_s[i, i, :8, :LANES] + ds_s[i, i, :8, :LANES]
                     + wl_s[rows8(i * 8), :LANES] + a_s[rows8(i * 8), :LANES] + qkv_s[i, :8]
                     + b_s[rows8(i * 8), :LANES] + wt_s[rows8(i * 8), :LANES])
                acc_s[1, 0, :8] = (lax.bitcast_convert_type(v, F32) + o_s[i, :8]
                                   + acc_s[i, i, :8] + h3_s[i, :8])
                return c
            lax.fori_loop(0, 2, keep, 0)
            finish(NB - 1, load_acc(1))
        out_copy(NB - 1).start()
        wait('WOUT', [out_copy(b) for b in range(NB)])

    scratch = [
        pltpu.VMEM((NB, D, TM), BF16),
        pltpu.VMEM((D, 3 * D), BF16),
        pltpu.VMEM((D, D), BF16),
        pltpu.VMEM((NP, D, PW), BF16),
        pltpu.VMEM((NP, D, PW), BF16),
        pltpu.VMEM((NP, D, PW), BF16),
        pltpu.VMEM((2 * D, 8 * LANES), U32),
        pltpu.VMEM((4 * Q3, 16 * LANES), U32),
        pltpu.VMEM((NP, 51, 64, 2 * LANES), U32),
        pltpu.VMEM((NP + 3, 5, Q3, 2 * LANES), U32),
        pltpu.VMEM((NB, D, TM), F32),
        pltpu.VMEM((max(fill), 2 * LANES), U32),
        pltpu.VMEM((S // LANES + 1, 3 * RP, LANES), U32),
        pltpu.VMEM((NT, D, LANES), F32),
        pltpu.VMEM((2, 15, D3, TH), F32),
        pltpu.VMEM((8 * 64, 2 * LANES), U32),
        pltpu.VMEM((NP, TM, LANES), F32),
        pltpu.VMEM((1, 9 * 64, 2 * LANES), U32),
        pltpu.SemaphoreType.DMA((SEM_P + NP + 2,)),
        pltpu.SemaphoreType.DMA((1,)),
    ]

    def wrapped(*refs):
        @pl.when(pl.program_id(0) == 0)
        def _():
            kernel(*refs)

    return wrapped, scratch


_CFG = dict(
    scopes=False,
    sub='abc',
    phases=('pre', 'main', 'last'),
    body=('G00', 'G01', 'G10', 'G11', 'Q', 'G20', 'G21', 'G30', 'G31', 'G40', 'G50',
        'D012a', 'G41', 'G51', 'G60', 'D345b', 'G61', 'G70', 'G71', 'G80', 'W', 'G81',
        'D67', 'D8c', 'L'),
    ln1=(('G00', 0), ('G00', 1), ('G00', 2), ('G00', 3), ('G00', 4), ('G00', 5), ('G00',
        6), ('G00', 7), ('G00', 8)),
    ln1b=(('G10', 1), ('G10', 2), ('G10', 3), ('G10', 4), ('G10', 5), ('G10', 6),
        ('G10', 7), ('G10', 8), ('G10', 9), ('G10', 10), ('G10', 11), ('G10', 12)),
    att=(('D012a', 0), ('D012a', 4), ('D012a', 5), ('D012a', 6), ('D012a', 10),
        ('D345b', 5), ('D345b', 7), ('D345b', 11)),
    lhs=(('D67', 0), ('D67', 0), ('D67', 4), ('D67', 6), ('D67', 8), ('D67', 10),
        ('D67', 12), ('D67', 13), ('D8c', 6)),
    a_w1=(0, 0, 1, 2, 2, 3, 3, 4, 4, 5, 6, 7),
    a_w2=(20, 23, 26, 30, 33, 36, 40, 43, 46, 50, 53, 57),
    a_ln=(0, 3, 6),
    a_lnb=(5, 9, 9),
    z_g=(0, 1, 3, 4, 6, 7, 9, 10, 12, 14, 15, 17, 18, 20, 21, 23, 24, 26, 28, 29, 31,
        32, 34, 35, 37, 38, 40, 42),
    t_d=(0, 0, 1, 1, 2, 2, 3, 4, 4, 5, 5, 6, 7, 7, 8, 8, 9, 10, 10, 11, 11, 12, 13, 13,
        14, 14, 15, 16, 16, 17, 17, 18, 19, 19, 20, 20, 21, 22, 22, 23, 23, 24, 25, 25,
        26, 26, 27, 28),
    p_d=(20, 21, 23, 24, 26, 28, 29, 31, 33, 34, 36, 38),
    p_att=(41,),
    p_w=(14, 42, 45),
    z_l=(4, 8, 12, 16, 20, 24, 28, 32, 36),
    a_k=(15, 19, 20, 24),
    a_k2=(0, 4, 8, 12),
    a_v=(13, 14, 22, 26, 30, 34, 38, 39),
    a_wo=(30, 35, 36, 38, 41),
    inner=(3, 4, 0, 6, 1, 2, 5),
    gorder=((0, 3), (0, 4), (0, 0), (1, 3), (0, 6), (1, 4), (0, 1), (1, 0), (0, 2), (1,
        6), (0, 5), (1, 1), (1, 2), (1, 5)),
    gorder0=((0, 4), (0, 1), (0, 3), (0, 0), (0, 6), (0, 2), (0, 5), (1, 4), (1, 1), (1,
        3), (1, 0), (1, 6), (1, 2), (1, 5)),
    f_t=(0, 6),
    f_g=(0, 1, 2, 3, 10, 11, 12, 13, 14, 15, 16, 17, 18, 19, 20, 21, 22, 23, 24, 25, 26,
        27, 28, 29, 30, 31, 32, 33),
    t_l=(20, 21, 23, 25, 27, 28, 30, 32, 34),
)


def _run(A_x, A_wqkv, A_wo, B_w_gate, B_w_up, B_w_down, **kw):
    _, S, D = A_x.shape
    F = B_w_gate.shape[1]
    kernel, scratch = _make_kernel(S, D, F, 256, {**_CFG, **kw})
    hbm = pl.BlockSpec(memory_space=pl.ANY)
    out_t = pl.pallas_call(
        kernel,
        grid=(2,),
        in_specs=[hbm] * 6,
        out_specs=hbm,
        out_shape=jax.ShapeDtypeStruct((D, S), A_x.dtype),
        scratch_shapes=scratch,
        compiler_params=pltpu.CompilerParams(
            dimension_semantics=('arbitrary',), vmem_limit_bytes=110 * 1024 * 1024),
    )(A_x.reshape(S, D).T, A_wqkv, A_wo, B_w_gate, B_w_up, B_w_down.T)
    return out_t.T.reshape(A_x.shape)


@jax.jit
def pallas_interleave_layers__sliding_local_dilated__glu_gated_geglu__prompt_kernel(
    A_x: jax.Array,
    A_wqkv: jax.Array,
    A_wo: jax.Array,
    B_x: jax.Array,
    B_w_gate: jax.Array,
    B_w_up: jax.Array,
    B_w_down: jax.Array,
):
    del B_x
    return _run(A_x, A_wqkv, A_wo, B_w_gate, B_w_up, B_w_down)
```

```python
import jax
import jax.numpy as jnp
import jax.experimental.pallas as pl
import jax.experimental.pallas.tpu as pltpu
from jax import lax

H = 32
W = 8
DIL = 2
EPS = 1e-5
LANES = 128

F32 = jnp.float32
BF16 = jnp.bfloat16
U32 = jnp.uint32

_NT = (((1,), (1,)), ((), ()))


def _tree_sum(parts, op=jnp.add):
    while len(parts) > 1:
        nxt = [op(parts[i], parts[i + 1]) for i in range(0, len(parts) - 1, 2)]
        if len(parts) % 2:
            nxt.append(parts[-1])
        parts = nxt
    return parts[0]


def _ln_stats(slabs, d, anchors=()):
    n_acc = 4
    s1, s2, pilot = [None] * n_acc, [None] * n_acc, None
    for i, x in enumerate(slabs):
        if pilot is None:
            pilot = x[0:1, :]
            pil = jnp.broadcast_to(pilot, x.shape)
            pils = [_tie(pil, a) for a in anchors] or [pil]
        dx = x - pils[i * len(pils) // (d // 8)]
        j = i % n_acc
        s1[j] = dx if s1[j] is None else s1[j] + dx
        s2[j] = dx * dx if s2[j] is None else s2[j] + dx * dx
    e1 = jnp.sum(_tree_sum(s1), axis=0, keepdims=True) * (1.0 / d)
    e2 = jnp.sum(_tree_sum(s2), axis=0, keepdims=True) * (1.0 / d)
    var = jnp.maximum(e2 - e1 * e1, 0.0)
    return pilot + e1, lax.rsqrt(var + EPS)


def _zero_like_dep(v):
    return (lax.bitcast_convert_type(v, U32) >> 31) >> 1


def _tie(x, anchor):
    if anchor is None:
        return x
    z = lax.bitcast_convert_type(_zero_like_dep(anchor), F32)
    z = jnp.concatenate([z] * -(-x.shape[1] // LANES), axis=1)[:, :x.shape[1]]
    if x.shape[0] == 8:
        return x + z
    return jnp.concatenate([x[:8] + z, x[8:]], axis=0)


def _gelu_mul2(g, u):
    c0 = 0.7978845608028654
    c1 = c0 * 0.044715
    t = jnp.tanh(g * (c0 + c1 * (g * g)))
    return (g * u) * (1.0 + t)


def _lo(x):
    return lax.bitcast_convert_type(x << 16, F32)


def _hi(x):
    return lax.bitcast_convert_type(x & jnp.uint32(0xFFFF0000), F32)


def _pk(x):
    return pltpu.bitcast(x.astype(BF16), U32)


def _upk(x):
    return pltpu.bitcast(x, BF16)


def _dot(a, b):
    return jnp.dot(a, b, preferred_element_type=F32)


def _dot_nt(a, b):
    return lax.dot_general(a, b, _NT, preferred_element_type=F32)


def _x_ops(x1, x2):
    d = [a - b for a, b in zip(x1, x2)]
    return [x1[0] + x2[1], x2[0] + x2[1], x1[0] + x1[1],
            d[1] + x1[2], x1[1] + x1[2], d[1] + d[2],
            d[0] - x2[2], d[0] + d[2], x2[0] + x2[2],
            x1[0], d[0], x2[1], d[1], x1[2], x2[2]]


def _x_rem(x1, x2):
    a, b, c = 0, 1, 2
    cat = lambda u, v: jnp.concatenate([u, v], axis=0)
    return [cat(x1[c], x2[b]), cat(x1[a], x1[b] - x2[b]), cat(x2[a], x2[c] - x1[c])]


_W_TERMS = {0: ((0, 1, 1), (1, 0, 1)), 3: ((1, 2, 1), (2, 1, 1)), 6: ((0, 2, 1), (2, 0, 1)),
            9: ((0, 0, 1), (0, 2, 1), (1, 0, -1)), 10: ((2, 0, 1), (0, 0, -1), (0, 1, -1)),
            11: ((1, 1, 1), (1, 2, 1), (0, 1, -1)), 12: ((1, 0, 1), (1, 1, 1), (2, 1, -1)),
            13: ((2, 0, 1), (2, 2, 1), (1, 2, -1)), 14: ((2, 1, 1), (2, 2, 1), (0, 2, -1)),
            1: ((0, 1, 1),), 2: ((1, 0, 1),), 4: ((1, 2, 1),), 5: ((2, 1, 1),),
            7: ((2, 0, 1),), 8: ((0, 2, 1),)}


def _w_sums(w):
    return [_signed(_W_TERMS[i], lambda k, j: w[k][j]) for i in _W_SUM]


_W_SUM = {0: 0, 3: 1, 6: 2, 9: 3, 10: 4, 11: 5, 12: 6, 13: 7, 14: 8}
_W_RAW = {1: (0, 1), 2: (1, 0), 4: (1, 2), 5: (2, 1), 7: (2, 0), 8: (0, 2)}
_PAIR_ORDER = (1, 2, 4, 5, 7, 8, 0, 3, 6)
_DIAG = {(0, 0): 9, (2, 0): 10, (0, 1): 11, (1, 1): 12, (1, 2): 13, (2, 2): 14}
_PAIR = {(0, 0): ((6, -1), (8, -1)), (1, 0): ((2, 1), (7, 1)), (2, 0): ((0, 1), (1, -1)),
         (0, 1): ((3, 1), (4, -1)), (1, 1): ((0, 1), (2, -1)), (2, 1): ((1, 1), (5, -1)),
         (0, 2): ((4, 1), (8, 1)), (1, 2): ((6, 1), (7, -1)), (2, 2): ((5, 1), (3, -1))}


def _column(t, base, j, skew=False):
    s = []
    for k in range(3):
        v = base[k]
        for i, sg in _PAIR[k, j]:
            v = t[i] if v is None else (v + t[i] if sg > 0 else v - t[i])
        s.append(v)
    if skew:
        return s[1] + s[0], s[2] + 0.5 * (s[0] - s[1])
    return s[1] + s[0], s[2] + s[0]


_SA = (((0, 0, 1), (1, 1, 1)), ((1, 0, 1), (1, 1, 1)), ((0, 0, 1),), ((1, 1, 1),),
       ((0, 0, 1), (0, 1, 1)), ((1, 0, 1), (0, 0, -1)), ((0, 1, 1), (1, 1, -1)))
_SB = (((0, 0, 1), (1, 1, 1)), ((0, 0, 1),), ((0, 1, 1), (1, 1, -1)), ((1, 0, 1), (0, 0, -1)),
       ((1, 1, 1),), ((0, 0, 1), (0, 1, 1)), ((1, 0, 1), (1, 1, 1)))
_SCOL = {2: 1, 3: 0, 5: 1, 6: 0}
_SGRP = ((1, 4, 0), (3, 6), (2, 5))


def _signed(terms, f):
    v = None
    for a, b, sg in terms:
        v = f(a, b) if v is None else (v + f(a, b) if sg > 0 else v - f(a, b))
    return v


def _s_out(m):
    return [[m[0] + m[3] - m[4] + m[6], m[2] + m[4]],
            [m[1] + m[3], m[0] - m[1] + m[2] + m[5]]]


def _make_kernel(S, D, F, TM, cfg):
    NB = S // TM
    NT = TM // LANES
    DH = D // H
    DP = DH // 2
    RP = D // 2
    NG = H // 8
    scale = float(DH) ** -0.5
    NU = 2 * NB
    TH = TM // 2
    TQ = TM // 4
    D2 = D // 2
    D3 = D // 3
    Q3 = D3 // 2
    KU = D // 9
    KR = 3 * LANES
    NQ = 6
    QR = 3 * D // NQ
    WQ = (0, 640, 1152, 3 * D)
    PW = 4 * LANES
    NP = F // PW
    AOFF, fill = {}, [0, 0]
    for key in [(m1, m2) for m1 in range(7) for m2 in range(7)] + list(range(9)):
        c = int(fill[1] < fill[0])
        AOFF[key] = (fill[c], slice(c * LANES, (c + 1) * LANES))
        fill[c] += (64 if isinstance(key, int) else
                    48 if key[0] in _SCOL and key[1] in _SCOL else 32)
    scopes = cfg['scopes']
    assert NG == 4 and NB & (NB - 1) == 0
    SEM_P = 4

    def kernel(x_hbm, wqkv_hbm, wo_hbm, wg_hbm, wu_hbm, wdt_hbm, out_hbm,
               xio_s, wqkv_v, wo_v, wg_v, wu_v, wdt_v, wt_s, wl_s,
               gu_s, ds_s, xmid_s, a_s, qkv_s, o_s, acc_s, b_s, h3_s, r_s,
               sem_i, sem_o):

        def wait(name, cps):
            if scopes:
                with jax.named_scope(name):
                    for cp in cps:
                        cp.wait()
            else:
                for cp in cps:
                    cp.wait()

        def cols(lo, n):
            if not isinstance(lo, int):
                lo = pl.multiple_of(lo, LANES)
            return pl.ds(lo, n)

        def rows8(lo, n=8):
            if not isinstance(lo, int):
                lo = pl.multiple_of(lo, 8)
            return pl.ds(lo, n)

        def out_copy(b):
            return pltpu.make_async_copy(
                xio_s.at[b], out_hbm.at[:, cols(b * TM, TM)], sem_o.at[0])

        def x_cp(b, sem):
            return pltpu.make_async_copy(x_hbm.at[:, cols(b * TM, TM)], xio_s.at[b],
                                         sem_i.at[sem])

        def wq_cp(i):
            sl = cols(WQ[i], WQ[i + 1] - WQ[i])
            return pltpu.make_async_copy(wqkv_hbm.at[:, sl], wqkv_v.at[:, sl],
                                         sem_i.at[1 + i])

        def piece_cp(src, dst, p, sem):
            return [pltpu.make_async_copy(src.at[:, cols(p * PW, PW)], dst.at[p],
                                          sem_i.at[sem])]

        def group_cp(p):
            sem = SEM_P + p
            cps = []
            if not (isinstance(p, int) and p == NP):
                cps += piece_cp(wg_hbm, wg_v, p, sem) + piece_cp(wu_hbm, wu_v, p, sem)
            if not (isinstance(p, int) and p == 0):
                cps += piece_cp(wdt_hbm, wdt_v, p - 1, sem)
            return cps

        lane = lax.broadcasted_iota(jnp.int32, (8, LANES), 1)
        cat0 = lambda *v: jnp.concatenate(v, axis=0)
        cat1 = lambda *v: jnp.concatenate(v, axis=1)

        def spread_over(anchors, n, total):
            return anchors[n * len(anchors) // total] if anchors else None

        def slab_group(r):
            return (r % LANES) // 16 if r < KR else 8 + ((r - KR) % KU) // 16

        def ln1(blk, anchors1, anchors2=()):
            slabs = (xio_s[blk, r:r + 8, :].astype(F32) for r in range(0, D, 8))
            m, rs = _ln_stats(slabs, D, anchors1)
            if not anchors2:
                return (xio_s[blk].astype(F32) - m) * rs
            m8 = jnp.broadcast_to(m, (8, TM))
            ms = [_tie(m8, a) for a in anchors2]
            ms = [spread_over(ms, slab_group(r), 12) for r in range(0, D, 8)]
            return (xio_s[blk].astype(F32) - cat0(*ms)) * rs

        def dot_k(rows, x, anchors, even=False):
            y = None
            for n, k in enumerate(range(0, D, LANES)):
                ks = slice(k, min(k + LANES, D))
                if even and k + LANES >= D:
                    mid = (rows.start + rows.stop) // 2
                    v = cat0(_dot(_upk(wt_s[rows.start:mid, ks]), x[ks]),
                             _dot(_upk(wt_s[mid:rows.stop, ks]), x[ks]))
                else:
                    v = _dot(_upk(wt_s[rows, ks]), x[ks])
                anchors.extend(v[r:r + 8, :LANES] for r in ((0, 144) if n % 2 else (72, 216)))
                y = v if y is None else y + v
            return y

        def put_qkv(blk, rows, y):
            pk = _pk(y)
            for c in range(NT):
                qkv_s[1 + blk * NT + c, rows, :] = pk[:, c * LANES:(c + 1) * LANES]

        def qkv_mm(blk, xn, chunks, anchors, even=False):
            for r in chunks:
                rows = slice(r * QR // 2, (r + 1) * QR // 2)
                put_qkv(blk, rows, dot_k(rows, xn, anchors, even))

        def split_k(x):
            hs = (x[:, :TH], x[:, TH:])
            blocks = [[h[k * LANES:(k + 1) * LANES] for k in range(3)] for h in hs]
            units = [[h[KR + k * KU:KR + (k + 1) * KU] for k in range(3)] for h in hs]
            return blocks, units

        def prep_att(pat, anchor):
            assert Q3 == 96
            row0 = pat * 8
            src0 = row0 + ((pat * 43) >> 9) * (2 * Q3)
            w = [_upk(wt_s[rows8(src0 + j * Q3), :D]).astype(F32) for j in range(3)]
            w[0] = cat1(_tie(w[0][:, :LANES], anchor), w[0][:, LANES:])
            tiles = _w_sums([[w[j][:, k * LANES:(k + 1) * LANES] for j in range(3)]
                             for k in range(3)])
            for j in range(3):
                a, b, c = (w[j][:, KR + k * KU:KR + (k + 1) * KU] for k in range(3))
                tiles += [cat1(c, b), cat1(a, c)]
            wl_s[rows8(row0), :15 * LANES] = _pk(cat1(*tiles))

        def att_rhs(x, stash=None):
            blocks, units = split_k(cat1(x[:, :TH], x[:, TH:] + 0.5 * x[:, :TH]))
            ops = _x_ops(*blocks) + _x_rem(*units)
            if stash is None:
                return [v.astype(BF16) for v in ops]
            loc = lambda i, r0, n: (slice((i // 2) * 64 + r0, (i // 2) * 64 + r0 + n),
                                    slice((i % 2) * LANES, (i % 2 + 1) * LANES))
            for r in range(0, LANES, 16):
                for i, v in enumerate(ops):
                    r_s.at[0][loc(i, r // 2, 8)] = _pk(v[r:r + 16])
            return [_upk(r_s.at[stash][loc(i, 0, 64)]) for i in range(18)]

        def att_mm(sec, rhs, anchors):
            tl = lambda i: _upk(wl_s[sec * Q3:(sec + 1) * Q3, i * LANES:(i + 1) * LANES])
            raw = lambda k, j: _upk(wt_s[(3 * sec + j) * Q3:(3 * sec + j + 1) * Q3,
                                         k * LANES:(k + 1) * LANES])
            t = {}
            for i in _PAIR_ORDER:
                t[i] = _dot(raw(*_W_RAW[i]) if i in _W_RAW else tl(_W_SUM[i]), rhs[i])
                anchors.append(t[i][:8])
            out = []
            for j in range(3):
                base = []
                for s in range(3):
                    v = _dot(raw(3, j) if s == 1 else tl(9 + 2 * j + s // 2), rhs[15 + s])
                    if (s, j) in _DIAG:
                        i = _DIAG[s, j]
                        v = _dot(tl(_W_SUM[i]), rhs[i]) + v
                    base.append(v)
                    anchors.append(base[-1][:8])
                out.append(cat1(*_column(t, base, j, True)))
            return cat0(*out)

        def qkv_fast(blk, rhs, anchors):
            for sec in range(3):
                put_qkv(blk, slice(sec * RP, (sec + 1) * RP), att_mm(sec, rhs, anchors))

        def shifted(ln, cur, prev, w):
            if w == 0:
                return cur
            sh = DIL * w
            return pltpu.roll(jnp.where(ln < LANES - sh, cur, prev), sh, axis=1)

        def att_group(blk, c, hg, anchor):
            att_values(blk, c, hg, anchor)(None)

        def att_values(blk, c, hg, anchor):
            tile = blk * NT + c
            base = hg * 8 * DP
            if isinstance(hg, int):
                cur, prev, o_t = qkv_s.at[1 + tile], qkv_s.at[tile], o_s.at[c]
            else:
                n = 2 * RP + 8 * DP
                base = pl.multiple_of(base, 8)
                cur = qkv_s.at[1 + tile, pl.ds(base, n)]
                prev = qkv_s.at[tile, pl.ds(base, n)]
                o_t = o_s.at[c, pl.ds(base, RP + 8 * DP)]
                base = 0
            ln = lane + _zero_like_dep(anchor).astype(jnp.int32)
            logits = [None] * W
            for dd in range(DP):
                q = cur[pl.ds(base + dd, 8, stride=DP), :]
                kc = cur[pl.ds(RP + base + dd, 8, stride=DP), :]
                kp = prev[pl.ds(RP + base + dd, 8, stride=DP), :]
                q0, q1 = _lo(q), _hi(q)
                for w in range(W):
                    ks = shifted(ln, kc, kp, w)
                    t = q0 * _lo(ks) + q1 * _hi(ks)
                    logits[w] = t if logits[w] is None else logits[w] + t
            logits = [l * scale for l in logits]
            if not (isinstance(c, int) and c > 0):
                pos = lane + tile * LANES
                logits = [l if w == 0 else jnp.where(pos >= DIL * w, l, -1e9)
                          for w, l in enumerate(logits)]
            m = _tree_sum(logits, jnp.maximum)
            p = [jnp.exp(l - m) for l in logits]
            r = 1.0 / _tree_sum(p)

            def apply(anchor2):
                ln = lane + _zero_like_dep(m if anchor2 is None else anchor2).astype(jnp.int32)
                for dd in range(DP):
                    vc = cur[pl.ds(2 * RP + base + dd, 8, stride=DP), :]
                    vp = prev[pl.ds(2 * RP + base + dd, 8, stride=DP), :]
                    o0 = o1 = None
                    for w in range(W):
                        vs = shifted(ln, vc, vp, w)
                        t0, t1 = p[w] * _lo(vs), p[w] * _hi(vs)
                        o0 = t0 if o0 is None else o0 + t0
                        o1 = t1 if o1 is None else o1 + t1
                    o0, o1 = o0 * r, o1 * r
                    o_t[pl.ds(base + dd, 8, stride=DP), :] = o0
                    o_t[pl.ds(RP + base + dd, 8, stride=DP), :] = o1

            return apply

        def attention(blk, anchors):
            for c in range(NT):
                for hg in range(NG):
                    att_group(blk, c, hg, anchors[c * NG + hg])

        def wo_mm(blk, anchors, fast, stash=None):
            o = cat1(*[o_s[c] for c in range(NT)])
            if fast:
                y = att_mm(3, att_rhs(o, stash), anchors)
            else:
                o = o.astype(BF16)
                q = D2 // 2
                y = cat0(*[dot_k(slice(h * q, (h + 1) * q), o, anchors) for h in (6, 7)])
            xm = xio_s[blk].astype(F32) + y
            xmid_s[blk] = xm
            return _ln_stats((xm[r:r + 8] for r in range(0, D, 8)), D)

        def ffn_lhs(blk, stats, anchors):
            m, rs = stats
            m8 = jnp.broadcast_to(m, (8, TM))
            xt = []
            for k in range(5):
                mt = cat0(*[_tie(m8, spread_over(anchors[:2], k, 5))] * (KU // 8 if k == 4 else 16))
                x = (xmid_s[blk, k * LANES:min((k + 1) * LANES, D), :] - mt) * rs
                xt.append((cat0(x, x) if k == 4 else x).T)
            lo = lax.broadcasted_iota(jnp.int32, (TQ // 2, LANES), 1) < KU
            for m1 in range(7):
                a = spread_over(anchors[2:], m1, 7)
                blk1 = lambda i2, k2: _signed(_SA[m1], lambda i1, k1: _tie(
                    xt[k2 if k2 == 4 else 2 * k1 + k2][(2 * i1 + i2) * TQ:(2 * i1 + i2 + 1) * TQ], a))
                l1 = {(i2, k2): blk1(i2, k2) for i2 in range(2)
                      for k2 in ((0, 1, 4) if m1 in _SCOL else (0, 1))}
                for m2 in range(7):
                    v = _signed(_SA[m2], lambda i2, k2: l1[i2, k2])
                    if m1 in _SCOL and m2 in _SCOL:
                        c = _signed(_SA[m2], lambda i2, k2: l1[i2, 4])
                        h = TQ // 2
                        vp, vq, cp, cq = v[:h], v[h:], c[:h], c[h:]
                        v = cat0(jnp.where(lo, cp, vq), jnp.where(lo, vp, vp - vq),
                                 jnp.where(lo, vq, cq - cp))
                    o, ac = AOFF[m1, m2]
                    a_s[o:o + v.shape[0] // 2, ac] = _pk(v)

        def plain_lhs(blk, stats):
            m, rs = stats
            blocks, units = split_k((xmid_s[blk] - m) * rs)
            for i, v in enumerate(blocks[0] + blocks[1] + _x_rem(*units)):
                a_s[AOFF[i][0]:AOFF[i][0] + 64, AOFF[i][1]] = _pk(v.astype(BF16).T)

        def plain_piece(p, anchors):
            h = []
            for n in range(4):
                cs = slice(n * LANES, (n + 1) * LANES)
                w = lambda r0, r1: cat1(wg_v[p, r0:r1, cs], wu_v[p, r0:r1, cs])
                u = lambda k: w(KR + k * KU, KR + (k + 1) * KU)
                tl = lambda *i: _upk(cat1(*[a_s[AOFF[k][0]:AOFF[k][0] + 64, AOFF[k][1]]
                                            for k in i]))
                y0 = _dot(tl(6), cat0(u(2), u(1)))
                y1 = _dot(tl(0, 1, 2, 7), w(0, KR + 2 * KU))
                y2 = _dot(tl(3, 4, 5, 8), cat0(w(0, KR + KU), u(2)))
                anchors.append(y0[:8, :LANES])
                for y in (y1, y2):
                    anchors.extend(y[r:r + 8, c:c + LANES] for c in (0, LANES)
                                   for r in (0, TH // 2))
                h.append([_gelu_mul2(*[(y + y0)[:, c:c + LANES] for c in (0, LANES)])
                          for y in (y1, y2)])
            return h

        def in_triple(q):
            return q, lambda k: (q, k)

        def cross_triple(s):
            return NP + s, lambda k: (3 * s + k, 3)

        def wd_raw(tri, k, r0, n):
            q, c = tri[1](k)
            return wdt_v[q, r0:r0 + n, c * LANES:(c + 1) * LANES]

        def ds_loc(i, r0, n):
            return slice(r0, r0 + n), slice((i % 2) * LANES, (i % 2 + 1) * LANES)

        def prep_d(tri, anchors):
            PR = 16
            for n in range(D3 // PR):
                r = n * PR
                w = [[wd_raw(tri, k, j * D3 + r, PR).astype(F32) for j in range(3)]
                     for k in range(3)]
                w[0][1] = _tie(w[0][1], spread_over(anchors, n, D3 // PR))
                for i, v in enumerate(_w_sums(w)):
                    ds_s.at[tri[0], i // 2][ds_loc(i, r // 2, PR // 2)] = _pk(v)

        GU = (wg_v, wu_v)

        def prep_gu(p, m, m1s, anchors):
            PR = 16
            cs = slice(m * LANES, (m + 1) * LANES)
            for n in range(LANES // PR):
                r = n * PR
                cache = {}

                def w(k, j1):
                    if (k, j1) not in cache:
                        v = GU[m][p, k * LANES + r:k * LANES + r + PR,
                                  2 * j1 * LANES:2 * (j1 + 1) * LANES].astype(F32)
                        if (k // 2, j1) in [_SB[m1][0][:2] for m1 in m1s[:2]]:
                            v = _tie(v, spread_over(anchors, n, LANES // PR))
                        cache[k, j1] = v
                    return cache[k, j1]

                for m1 in m1s:
                    b1 = [_signed(_SB[m1], lambda k1, j1: w(2 * k1 + k2, j1)) for k2 in range(2)]
                    for m2 in range(7):
                        v = _signed(_SB[m2],
                                    lambda k2, j2: b1[k2][:, j2 * LANES:(j2 + 1) * LANES])
                        gu_s.at[p, 7 * m1 + m2][r // 2:(r + PR) // 2, cs] = _pk(v)

        def prep_tail(p, m, anchor):
            v = _tie(GU[m][p, 4 * LANES:, :].astype(F32), anchor)
            for j in range(4):
                gu_s.at[p, 49 + j // 2][(j % 2) * 32:(j % 2 + 1) * 32,
                                        m * LANES:(m + 1) * LANES] = _pk(
                                            v[:, j * LANES:(j + 1) * LANES])

        def gu_outer(p, m, m1, anchors, at=(0, 4)):
            cs = slice(m * LANES, (m + 1) * LANES)
            y = {}
            for m2 in cfg['inner']:
                i, (o, ac) = 7 * m1 + m2, AOFF[m1, m2]
                if m1 in _SCOL and m2 in _SCOL:
                    j = 2 * _SCOL[m1] + _SCOL[m2]
                    tail = lambda: gu_s[p, 49 + j // 2, (j % 2) * 32:(j % 2 + 1) * 32, cs]
                    rhs = (cat0(tail(), gu_s[p, i, 32:, cs]), gu_s[p, i, :, cs],
                           cat0(gu_s[p, i, :32, cs], tail()))
                    r = [_dot(_upk(a_s[o + 16 * s:o + 16 * (s + 1), ac]), _upk(rhs[s]))
                         for s in range(3)]
                    y[m2] = cat0(r[1] + r[0], r[2] + r[0])
                else:
                    y[m2] = _dot(_upk(a_s[o:o + TQ // 2, ac]), _upk(gu_s[p, i, :, cs]))
            anchors.extend(y[cfg['inner'][k % 7]][(k // 7) * 32:(k // 7) * 32 + 8] for k in at)
            return _s_out(y)

        def gu_finish(t):
            gu = [{(i2, j2): _s_out([t[m][m1][i2][j2] for m1 in range(7)])
                   for i2 in range(2) for j2 in range(2)} for m in range(2)]
            return [[cat0(*[_gelu_mul2(*[gu[m][i2, j % 2][i1][j // 2] for m in range(2)])
                            for i2 in range(2)]) for i1 in range(2)] for j in range(4)]

        def gu_piece(p, anchors):
            t = ({}, {})
            for m, m1 in cfg['gorder']:
                t[m][m1] = gu_outer(p, m, m1, anchors)
            return gu_finish(t)

        def h_ops(h):
            return [v.astype(BF16) for v in _x_ops(*[[h[k][i] for k in range(3)]
                                                     for i in range(2)])]

        D_ORDER = _PAIR_ORDER + (9, 10, 11, 12, 13, 14)

        def down_mm(acc, work, anchors, which=D_ORDER, fine=False):
            p = [None] * 15 if acc is None else list(acc)
            jobs = [(i, n) for i in which for n in range(len(work))]
            split = {0: (), 1: (4,), 2: (2, 2), 3: (2, 2, 4)}[len(jobs) % 4]
            split = dict(zip(jobs[len(jobs) - len(split):], split))
            for i in which:
                y = None
                for n, (tri, b) in enumerate(work):
                    ns = split.get((i, n), 1)
                    nr = D3 // ns
                    if i in _W_RAW:
                        k, j = _W_RAW[i]
                        lhs = lambda h: wd_raw(tri, k, j * D3 + h * nr, nr)
                    else:
                        s = _W_SUM[i]
                        lhs = lambda h: _upk(ds_s.at[tri[0], s // 2][ds_loc(s, h * nr // 2, nr // 2)])
                    v = cat0(*[_dot_nt(lhs(h), b[i]) for h in range(ns)])
                    y = v if y is None else y + v
                p[i] = y if p[i] is None else p[i] + y
                anchors.append(p[i][:8])
                if fine:
                    anchors.append(p[i][D3 // 2:D3 // 2 + 8])
            return p

        def finish(blk, acc):
            y = [cat1(*_column(acc, [acc[_DIAG[s, j]] if (s, j) in _DIAG else None
                                     for s in range(3)], j)) for j in range(3)]
            xio_s[blk] = (xmid_s[blk] + 0.5 * cat0(*y)).astype(BF16)

        def load_acc(k):
            return [acc_s[k, i] for i in range(15)]

        def store_acc(k, acc):
            for i in range(15):
                acc_s[k, i] = acc[i]

        def b_loc(i):
            return (slice((i // 2) * 64, (i // 2 + 1) * 64),
                    slice((i % 2) * LANES, (i % 2 + 1) * LANES))

        def load_b():
            return [_upk(b_s[b_loc(i)]) for i in range(15)]

        def store_h(p, h):
            for i, v in enumerate(h_ops(h[:3])):
                b_s[b_loc(i)] = _pk(v)
            h3_s[p] = cat0(*h[3])

        def pre_phase():
            first = [[x_cp(0, 0)], [wq_cp(0)], [x_cp(1, 2), wq_cp(1)],
                     [wq_cp(2), pltpu.make_async_copy(wo_hbm, wo_v, sem_i.at[3])]]
            order = sum(first, [])
            for p in range(NP + 1):
                order += group_cp(p)
            xr_cp = [x_cp(b, SEM_P + NP + 1) for b in range(2, NB)]
            order += xr_cp
            for cp in order:
                cp.start()
            get = lambda an, name: [an[min(i, len(an) - 1)] for i in cfg[name]]
            e_grp = lambda e: ((e >> 1) & 1, ((e >> 2) << 1) | (e & 1))
            if 'a' in cfg['sub']:
                pre_a(first, get, e_grp)
            if 'b' in cfg['sub']:
                pre_b(get, e_grp)
            if 'c' in cfg['sub']:
                pre_c(get)
            wait('WX', xr_cp)

        def pre_a(first, get, e_grp):
            def transpose_wq(i):
                wt_s[WQ[i] // 2:WQ[i + 1] // 2, :D] = _pk(wqkv_v[:, WQ[i]:WQ[i + 1]].T)

            def clear(i, carry):
                for k in range(2):
                    acc_s[k, i] = jnp.zeros((D3, TH), F32)
                r = jnp.minimum(i, 11) * (RP // 4)
                qkv_s[0, rows8(r, RP // 4)] = jnp.zeros((RP // 4, LANES), U32)
                return carry

            lax.fori_loop(0, 15, clear, 0)
            wait('WX0', first[0])
            xn0 = ln1(0, ()).astype(BF16)

            wait('WQ0', first[1])
            transpose_wq(0)
            qkv_mm(0, xn0, (0, 1), [])

            wait('WQ1', first[2])
            transpose_wq(1)
            an = []
            qkv_mm(0, xn0, (2, 3), an)
            xn1 = ln1(1, get(an, 'a_ln'), get(an, 'a_lnb')).astype(BF16)
            qkv_mm(1, xn1, (0,), an, True)
            for n, a in enumerate(get(an, 'a_w1')):
                prep_att(n, a)
            nk = len(cfg['a_k'])
            apply = [att_values(0, *e_grp(e), a) for e, a in enumerate(get(an, 'a_k'))]

            wait('WQ2', first[3])
            an = []
            qkv_mm(1, xn1, (2,), an)
            transpose_wq(2)
            qkv_mm(0, xn0, (4, 5), an)
            qkv_mm(1, xn1, (4, 1), an)
            apply += [att_values(0, *e_grp(nk + e), a)
                      for e, a in enumerate(get(an, 'a_k2')[:8 - nk])]
            for e, a in enumerate(get(an, 'a_v')):
                apply[e](a)
            wo = pltpu.bitcast(wo_v[...], U32)
            wo = cat0(_lo(wo), _hi(wo))
            wo = cat0(*[_tie(wo[n * LANES:(n + 1) * LANES], a)
                        for n, a in enumerate(get(an, 'a_wo'))])
            wt_s[3 * RP:, :D] = _pk(wo.astype(BF16).T)
            stats = wo_mm(0, an, False)
            qkv_mm(1, xn1, (3,), an)
            for n, a in enumerate(get(an, 'a_w2')):
                prep_att(12 + n, a)
            plain_lhs(0, stats)

            wait('WO', group_cp(0))
            an = []
            h = plain_piece(0, an)
            qkv_mm(1, xn1, (5,), an, True)
            zg = get(an, 'z_g')
            for n in range(6):
                prep_gu(0, n % 2, _SGRP[n // 2], zg[8 * n:8 * n + 8])
            for m in range(2):
                prep_tail(0, m, zg[m])
            if not cfg['plain0']:
                ffn_lhs(0, stats, get(an, 'z_l'))
            store_h(0, h)

        def pre_b(get, e_grp):
            def piece(p, carry):
                wait('WP', group_cp(p))
                work = [(in_triple(p - 1), load_b())]
                an = []
                if cfg['plain0']:
                    h = plain_piece(p, an)
                    prep_d(work[0][0], get(an, 'p_d'))
                    store_acc(0, down_mm(load_acc(0), work, an))
                    for m in range(2):
                        prep_tail(p, m, get(an, 'f_t')[m])
                    grp = _SGRP if cfg['plain0'] == 2 else [(m1,) for m1 in range(7)]
                    fg = get(an, 'f_g')
                    for n in range(2 * len(grp)):
                        k = len(fg) // (2 * len(grp))
                        prep_gu(p, n % 2, grp[n // 2], fg[k * n:k * n + k])
                else:
                    acc = down_mm(load_acc(0), work, an, D_ORDER[:6], True)
                    t = ({}, {})
                    for m in range(2):
                        prep_tail(p, m, get(an, 'f_t')[m])
                    for n, (m, m1) in enumerate(cfg['gorder0']):
                        prep_gu(p, m, (m1,), get(an, 'f_g')[4 * n:4 * n + 4])
                        t[m][m1] = gu_outer(p, m, m1, an, (0, 7, 4, 11))
                    h = gu_finish(t)
                    prep_d(work[0][0], get(an, 'p_d'))
                    store_acc(0, down_mm(acc, work, an, D_ORDER[6:]))
                att_group(1, *e_grp(p - 1), an[cfg['p_att'][0]])
                for i, a in enumerate(get(an, 'p_w')):
                    prep_att(48 - (NP - p) * len(cfg['p_w']) + i, a)
                store_h(p, h)
                return carry

            lax.fori_loop(1, NP, piece, 0)

        def pre_c(get):
            wait('WD', group_cp(NP))
            work = [(in_triple(NP - 1), load_b())]
            for s in range(3):
                h3 = [h3_s[3 * s + k] for k in range(3)]
                work.append((cross_triple(s), h_ops([[v[:TH], v[TH:]] for v in h3])))
            an = []
            stats = wo_mm(1, an, True)
            acc = down_mm(load_acc(0), work, an, D_ORDER[:6], True)
            td = get(an, 't_d')
            for n, (tri, _) in enumerate(work):
                prep_d(tri, td[n * len(td) // 4:(n + 1) * len(td) // 4])
            acc = down_mm(acc, work, an, D_ORDER[6:])
            ffn_lhs(1, stats, get(an, 't_l'))
            finish(0, acc)

        if 'pre' in cfg['phases']:
            pre_phase()

        def body(u, carry):
            bu = u & (NB - 1)
            ba = (u + 1) & (NB - 1)
            acc, stats, an, b, hh = None, None, {}, {}, {}
            get = lambda name: [an[k][i] for k, i in cfg[name]]
            for step in cfg['body']:
                an[step] = []
                if step == 'Q':
                    xn = ln1(ba, get('ln1'), get('ln1b'))
                    qkv_fast(ba, att_rhs(xn, u >> 8), an[step])
                elif step == 'W':
                    attention(ba, get('att'))
                    stats = wo_mm(ba, an[step], True, u >> 8)
                elif step == 'L':
                    ffn_lhs(ba, stats, get('lhs'))
                elif step[0] == 'G':
                    q, go = int(step[1]), cfg['gorder']
                    t = b.setdefault(step[:2], ({}, {}))
                    for m, m1 in (go[:7] if step[2] == '0' else go[7:]):
                        t[m][m1] = gu_outer(q, m, m1, an[step])
                    if len(t[0]) + len(t[1]) == 14:
                        hh[q] = gu_finish(t)
                else:
                    work = []
                    for c in step[1:]:
                        if c.isdigit():
                            work.append((in_triple(int(c)), h_ops(hh[int(c)][:3])))
                        else:
                            s = ord(c) - ord('a')
                            work.append((cross_triple(s),
                                         h_ops([hh[3 * s + k][3] for k in range(3)])))
                    acc = down_mm(acc, work, an[step])
            finish(bu, acc)

            @pl.when(u >= NB)
            def _():
                out_copy(bu).start()
            return carry

        if scopes:
            with jax.named_scope('LOOP'):
                lax.fori_loop(1, NU - 1, body, 0)
        elif 'main' in cfg['phases']:
            lax.fori_loop(1, NU - 1, body, 0)

        def last(s, carry):
            h = [gu_piece(3 * s + k, []) for k in range(3)]
            work = [(in_triple(3 * s + k), h_ops(h[k][:3])) for k in range(3)]
            work.append((cross_triple(s), h_ops([h[k][3] for k in range(3)])))
            acc = down_mm(down_mm(load_acc(1), work[:2], []), work[2:], [])
            store_acc(1, acc)
            finish(NB - 1, acc)
            return carry

        if 'last' in cfg['phases']:
            lax.fori_loop(0, NP // 3, last, 0)
        if len(cfg['phases']) < 3:
            def keep(i, c):
                v = (gu_s[i, i, :8, :LANES] + ds_s[i, i, :8, :LANES]
                     + wl_s[rows8(i * 8), :LANES] + a_s[rows8(i * 8), :LANES] + qkv_s[i, :8]
                     + b_s[rows8(i * 8), :LANES] + wt_s[rows8(i * 8), :LANES])
                acc_s[1, 0, :8] = (lax.bitcast_convert_type(v, F32) + o_s[i, :8]
                                   + acc_s[i, i, :8] + h3_s[i, :8])
                return c
            lax.fori_loop(0, 2, keep, 0)
            finish(NB - 1, load_acc(1))
        out_copy(NB - 1).start()
        wait('WOUT', [out_copy(b) for b in range(NB)])

    scratch = [
        pltpu.VMEM((NB, D, TM), BF16),
        pltpu.VMEM((D, 3 * D), BF16),
        pltpu.VMEM((D, D), BF16),
        pltpu.VMEM((NP, D, PW), BF16),
        pltpu.VMEM((NP, D, PW), BF16),
        pltpu.VMEM((NP, D, PW), BF16),
        pltpu.VMEM((2 * D, 8 * LANES), U32),
        pltpu.VMEM((4 * Q3, 16 * LANES), U32),
        pltpu.VMEM((NP, 51, 64, 2 * LANES), U32),
        pltpu.VMEM((NP + 3, 5, Q3, 2 * LANES), U32),
        pltpu.VMEM((NB, D, TM), F32),
        pltpu.VMEM((max(fill), 2 * LANES), U32),
        pltpu.VMEM((S // LANES + 1, 3 * RP, LANES), U32),
        pltpu.VMEM((NT, D, LANES), F32),
        pltpu.VMEM((2, 15, D3, TH), F32),
        pltpu.VMEM((8 * 64, 2 * LANES), U32),
        pltpu.VMEM((NP, TM, LANES), F32),
        pltpu.VMEM((1, 9 * 64, 2 * LANES), U32),
        pltpu.SemaphoreType.DMA((SEM_P + NP + 2,)),
        pltpu.SemaphoreType.DMA((1,)),
    ]

    def wrapped(*refs):
        @pl.when(pl.program_id(0) == 0)
        def _():
            kernel(*refs)

    return wrapped, scratch


_CFG = dict(
    scopes=False,
    plain0=2,
    sub='abc',
    phases=('pre', 'main', 'last'),
    body=('G00', 'G01', 'G10', 'G11', 'Q', 'G20', 'G21', 'G30', 'G31', 'G40', 'G50',
        'D012a', 'G41', 'G51', 'G60', 'D345b', 'G61', 'G70', 'G71', 'G80', 'W', 'G81',
        'D67', 'D8c', 'L'),
    ln1=(('G00', 0), ('G00', 1), ('G00', 2), ('G00', 3), ('G00', 4), ('G00', 5), ('G00',
        6), ('G00', 7), ('G00', 8)),
    ln1b=(('G10', 1), ('G10', 2), ('G10', 3), ('G10', 4), ('G10', 5), ('G10', 6),
        ('G10', 7), ('G10', 8), ('G10', 9), ('G10', 10), ('G10', 11), ('G10', 12)),
    att=(('D012a', 0), ('D012a', 4), ('D012a', 5), ('D012a', 6), ('D012a', 10),
        ('D345b', 5), ('D345b', 7), ('D345b', 11)),
    lhs=(('D67', 0), ('D67', 0), ('D67', 4), ('D67', 6), ('D67', 8), ('D67', 10),
        ('D67', 12), ('D67', 13), ('D8c', 6)),
    a_w1=(0, 0, 1, 2, 2, 3, 3, 4, 4, 5, 7, 11),
    a_w2=(0, 1, 3, 4, 6, 8, 9, 12, 13, 14, 16, 18, 44, 45, 46, 48, 49, 50, 52, 53, 55,
        56, 57, 59, 60, 62, 63, 64, 66, 67, 69, 70, 71, 73, 74, 76),
    a_ln=(0, 3, 6),
    a_lnb=(5, 9, 10),
    z_g=(0, 0, 1, 2, 3, 4, 5, 6, 7, 8, 9, 10, 11, 12, 13, 14, 15, 17, 18, 18, 19, 20,
        21, 22, 23, 24, 24, 25, 26, 28, 28, 29, 30, 31, 32, 33, 34, 35, 36, 37, 38, 39,
        40, 41, 42, 43, 44, 45),
    t_d=(0, 0, 0, 1, 2, 3, 4, 4, 4, 4, 5, 6, 8, 8, 9, 10, 10, 10, 11, 11, 11, 13, 14,
        14, 15, 16, 16, 16, 17, 17, 18, 19, 20, 20, 21, 21, 22, 22, 23, 23, 24, 24, 25,
        25, 26, 26, 27, 28),
    p_d=(12, 15, 17, 19, 21, 23, 25, 25, 28, 29, 33, 35),
    p_att=(33,),
    p_w=(),
    z_l=(4, 8, 12, 16, 20, 24, 28, 32, 36),
    a_k=(15, 19, 20, 24),
    a_k2=(4, 7, 10, 14),
    a_v=(11, 13, 22, 26, 30, 34, 37, 38),
    a_wo=(36, 36, 37, 38, 38),
    inner=(3, 4, 0, 6, 1, 2, 5),
    gorder=((0, 3), (0, 4), (0, 0), (1, 3), (0, 6), (1, 4), (0, 1), (1, 0), (0, 2), (1,
        6), (0, 5), (1, 1), (1, 2), (1, 5)),
    gorder0=((0, 1), (1, 1), (0, 4), (1, 4), (0, 0), (1, 0), (0, 3), (1, 3), (0, 6), (1,
        6), (0, 2), (1, 2), (0, 5), (1, 5)),
    f_t=(7, 38),
    f_g=(0, 0, 1, 1, 1, 2, 3, 3, 4, 5, 5, 6, 7, 7, 8, 9, 10, 10, 11, 11, 12, 12, 12, 13,
        14, 14, 15, 16, 17, 18, 18, 19, 20, 20, 21, 21, 21, 22, 23, 23, 24, 25, 25, 26,
        27, 27, 28, 29, 30, 31, 31, 32, 32, 33, 34, 39),
    t_l=(17, 25, 28, 30, 31, 33, 34, 35, 37),
    f_g0=(0, 1, 2, 3, 4, 5, 6, 7),
    f_g1=(8, 9, 11, 13, 14, 16, 18, 20),
    f_g2=(21, 22, 24, 26, 27, 29, 31, 33),
    f_g3=(33, 34, 35, 36, 38, 39, 40, 42),
    f_g4=(42, 43, 44, 45, 46, 47, 48, 50),
    f_g5=(50, 51, 52, 53, 54, 55, 56, 58),
)


def _run(A_x, A_wqkv, A_wo, B_w_gate, B_w_up, B_w_down, **kw):
    _, S, D = A_x.shape
    F = B_w_gate.shape[1]
    kernel, scratch = _make_kernel(S, D, F, 256, {**_CFG, **kw})
    hbm = pl.BlockSpec(memory_space=pl.ANY)
    out_t = pl.pallas_call(
        kernel,
        grid=(2,),
        in_specs=[hbm] * 6,
        out_specs=hbm,
        out_shape=jax.ShapeDtypeStruct((D, S), A_x.dtype),
        scratch_shapes=scratch,
        compiler_params=pltpu.CompilerParams(
            dimension_semantics=('arbitrary',), vmem_limit_bytes=110 * 1024 * 1024),
    )(A_x.reshape(S, D).T, A_wqkv, A_wo, B_w_gate, B_w_up, B_w_down.T)
    return out_t.T.reshape(A_x.shape)


@jax.jit
def pallas_interleave_layers__sliding_local_dilated__glu_gated_geglu__prompt_kernel(
    A_x: jax.Array,
    A_wqkv: jax.Array,
    A_wo: jax.Array,
    B_x: jax.Array,
    B_w_gate: jax.Array,
    B_w_up: jax.Array,
    B_w_down: jax.Array,
):
    del B_x
    return _run(A_x, A_wqkv, A_wo, B_w_gate, B_w_up, B_w_down)
```

```python
import jax
import jax.numpy as jnp
import jax.experimental.pallas as pl
import jax.experimental.pallas.tpu as pltpu
from jax import lax

H = 32
W = 8
DIL = 2
EPS = 1e-5
LANES = 128

F32 = jnp.float32
BF16 = jnp.bfloat16
U32 = jnp.uint32

_NT = (((1,), (1,)), ((), ()))


def _tree_sum(parts, op=jnp.add):
    while len(parts) > 1:
        nxt = [op(parts[i], parts[i + 1]) for i in range(0, len(parts) - 1, 2)]
        if len(parts) % 2:
            nxt.append(parts[-1])
        parts = nxt
    return parts[0]


def _ln_stats(slabs, d, anchors=()):
    n_acc = 4
    s1, s2, pilot = [None] * n_acc, [None] * n_acc, None
    for i, x in enumerate(slabs):
        if pilot is None:
            pilot = x[0:1, :]
            pil = jnp.broadcast_to(pilot, x.shape)
            pils = [_tie(pil, a) for a in anchors] or [pil]
        dx = x - pils[i * len(pils) // (d // 8)]
        j = i % n_acc
        s1[j] = dx if s1[j] is None else s1[j] + dx
        s2[j] = dx * dx if s2[j] is None else s2[j] + dx * dx
    e1 = jnp.sum(_tree_sum(s1), axis=0, keepdims=True) * (1.0 / d)
    e2 = jnp.sum(_tree_sum(s2), axis=0, keepdims=True) * (1.0 / d)
    var = jnp.maximum(e2 - e1 * e1, 0.0)
    return pilot + e1, lax.rsqrt(var + EPS)


def _zero_like_dep(v):
    return (lax.bitcast_convert_type(v, U32) >> 31) >> 1


def _tie(x, anchor):
    if anchor is None:
        return x
    z = lax.bitcast_convert_type(_zero_like_dep(anchor), F32)
    z = jnp.concatenate([z] * -(-x.shape[1] // LANES), axis=1)[:, :x.shape[1]]
    if x.shape[0] == 8:
        return x + z
    return jnp.concatenate([x[:8] + z, x[8:]], axis=0)


def _gelu_mul2(g, u):
    c0 = 0.7978845608028654
    c1 = c0 * 0.044715
    t = jnp.tanh(g * (c0 + c1 * (g * g)))
    return (g * u) * (1.0 + t)


def _lo(x):
    return lax.bitcast_convert_type(x << 16, F32)


def _hi(x):
    return lax.bitcast_convert_type(x & jnp.uint32(0xFFFF0000), F32)


def _pk(x):
    return pltpu.bitcast(x.astype(BF16), U32)


def _upk(x):
    return pltpu.bitcast(x, BF16)


def _dot(a, b):
    return jnp.dot(a, b, preferred_element_type=F32)


def _dot_nt(a, b):
    return lax.dot_general(a, b, _NT, preferred_element_type=F32)


def _x_ops(x1, x2):
    d = [a - b for a, b in zip(x1, x2)]
    return [x1[0] + x2[1], x2[0] + x2[1], x1[0] + x1[1],
            d[1] + x1[2], x1[1] + x1[2], d[1] + d[2],
            d[0] - x2[2], d[0] + d[2], x2[0] + x2[2],
            x1[0], d[0], x2[1], d[1], x1[2], x2[2]]


def _x_rem(x1, x2):
    a, b, c = 0, 1, 2
    cat = lambda u, v: jnp.concatenate([u, v], axis=0)
    return [cat(x1[c], x2[b]), cat(x1[a], x1[b] - x2[b]), cat(x2[a], x2[c] - x1[c])]


_W_TERMS = {0: ((0, 1, 1), (1, 0, 1)), 3: ((1, 2, 1), (2, 1, 1)), 6: ((0, 2, 1), (2, 0, 1)),
            9: ((0, 0, 1), (0, 2, 1), (1, 0, -1)), 10: ((2, 0, 1), (0, 0, -1), (0, 1, -1)),
            11: ((1, 1, 1), (1, 2, 1), (0, 1, -1)), 12: ((1, 0, 1), (1, 1, 1), (2, 1, -1)),
            13: ((2, 0, 1), (2, 2, 1), (1, 2, -1)), 14: ((2, 1, 1), (2, 2, 1), (0, 2, -1)),
            1: ((0, 1, 1),), 2: ((1, 0, 1),), 4: ((1, 2, 1),), 5: ((2, 1, 1),),
            7: ((2, 0, 1),), 8: ((0, 2, 1),)}


def _w_sums(w):
    return [_signed(_W_TERMS[i], lambda k, j: w[k][j]) for i in _W_SUM]


_W_SUM = {0: 0, 3: 1, 6: 2, 9: 3, 10: 4, 11: 5, 12: 6, 13: 7, 14: 8}
_W_RAW = {1: (0, 1), 2: (1, 0), 4: (1, 2), 5: (2, 1), 7: (2, 0), 8: (0, 2)}
_PAIR_ORDER = (1, 2, 4, 5, 7, 8, 0, 3, 6)
_DIAG = {(0, 0): 9, (2, 0): 10, (0, 1): 11, (1, 1): 12, (1, 2): 13, (2, 2): 14}
_PAIR = {(0, 0): ((6, -1), (8, -1)), (1, 0): ((2, 1), (7, 1)), (2, 0): ((0, 1), (1, -1)),
         (0, 1): ((3, 1), (4, -1)), (1, 1): ((0, 1), (2, -1)), (2, 1): ((1, 1), (5, -1)),
         (0, 2): ((4, 1), (8, 1)), (1, 2): ((6, 1), (7, -1)), (2, 2): ((5, 1), (3, -1))}


def _column(t, base, j, skew=False):
    s = []
    for k in range(3):
        v = base[k]
        for i, sg in _PAIR[k, j]:
            v = t[i] if v is None else (v + t[i] if sg > 0 else v - t[i])
        s.append(v)
    if skew:
        return s[1] + s[0], s[2] + 0.5 * (s[0] - s[1])
    return s[1] + s[0], s[2] + s[0]


_SA = (((0, 0, 1), (1, 1, 1)), ((1, 0, 1), (1, 1, 1)), ((0, 0, 1),), ((1, 1, 1),),
       ((0, 0, 1), (0, 1, 1)), ((1, 0, 1), (0, 0, -1)), ((0, 1, 1), (1, 1, -1)))
_SB = (((0, 0, 1), (1, 1, 1)), ((0, 0, 1),), ((0, 1, 1), (1, 1, -1)), ((1, 0, 1), (0, 0, -1)),
       ((1, 1, 1),), ((0, 0, 1), (0, 1, 1)), ((1, 0, 1), (1, 1, 1)))
_SCOL = {2: 1, 3: 0, 5: 1, 6: 0}
_SGRP = ((1, 4, 0), (3, 6), (2, 5))


def _signed(terms, f):
    v = None
    for a, b, sg in terms:
        v = f(a, b) if v is None else (v + f(a, b) if sg > 0 else v - f(a, b))
    return v


def _s_out(m):
    return [[m[0] + m[3] - m[4] + m[6], m[2] + m[4]],
            [m[1] + m[3], m[0] - m[1] + m[2] + m[5]]]


def _make_kernel(S, D, F, TM, cfg):
    NB = S // TM
    NT = TM // LANES
    DH = D // H
    DP = DH // 2
    RP = D // 2
    NG = H // 8
    scale = float(DH) ** -0.5
    NU = 2 * NB
    TH = TM // 2
    TQ = TM // 4
    D2 = D // 2
    D3 = D // 3
    Q3 = D3 // 2
    KU = D // 9
    KR = 3 * LANES
    NQ = 6
    QR = 3 * D // NQ
    WQ = (0, 640, 1152, 3 * D)
    PW = 4 * LANES
    NP = F // PW
    AOFF, fill = {}, [0, 0]
    for key in [(m1, m2) for m1 in range(7) for m2 in range(7)] + list(range(9)):
        c = int(fill[1] < fill[0])
        AOFF[key] = (fill[c], slice(c * LANES, (c + 1) * LANES))
        fill[c] += (64 if isinstance(key, int) else
                    48 if key[0] in _SCOL and key[1] in _SCOL else 32)
    scopes = cfg['scopes']
    assert NG == 4 and NB & (NB - 1) == 0
    SEM_P = 4

    def kernel(x_hbm, wqkv_hbm, wo_hbm, wg_hbm, wu_hbm, wdt_hbm, out_hbm,
               xio_s, wqkv_v, wo_v, wg_v, wu_v, wdt_v, wt_s, wl_s,
               gu_s, ds_s, xmid_s, a_s, qkv_s, o_s, acc_s, b_s, h3_s, r_s,
               sem_i, sem_o):

        def wait(name, cps):
            if scopes:
                with jax.named_scope(name):
                    for cp in cps:
                        cp.wait()
            else:
                for cp in cps:
                    cp.wait()

        def cols(lo, n):
            if not isinstance(lo, int):
                lo = pl.multiple_of(lo, LANES)
            return pl.ds(lo, n)

        def rows8(lo, n=8):
            if not isinstance(lo, int):
                lo = pl.multiple_of(lo, 8)
            return pl.ds(lo, n)

        def out_copy(b):
            return pltpu.make_async_copy(
                xio_s.at[b], out_hbm.at[:, cols(b * TM, TM)], sem_o.at[0])

        def x_cp(b, sem):
            return pltpu.make_async_copy(x_hbm.at[:, cols(b * TM, TM)], xio_s.at[b],
                                         sem_i.at[sem])

        def wq_cp(i):
            sl = cols(WQ[i], WQ[i + 1] - WQ[i])
            return pltpu.make_async_copy(wqkv_hbm.at[:, sl], wqkv_v.at[:, sl],
                                         sem_i.at[1 + i])

        def piece_cp(src, dst, p, sem):
            return [pltpu.make_async_copy(src.at[:, cols(p * PW, PW)], dst.at[p],
                                          sem_i.at[sem])]

        def group_cp(p):
            sem = SEM_P + p
            cps = []
            if not (isinstance(p, int) and p == NP):
                cps += piece_cp(wg_hbm, wg_v, p, sem) + piece_cp(wu_hbm, wu_v, p, sem)
            if not (isinstance(p, int) and p == 0):
                cps += piece_cp(wdt_hbm, wdt_v, p - 1, sem)
            return cps

        lane = lax.broadcasted_iota(jnp.int32, (8, LANES), 1)
        cat0 = lambda *v: jnp.concatenate(v, axis=0)
        cat1 = lambda *v: jnp.concatenate(v, axis=1)

        def spread_over(anchors, n, total):
            return anchors[n * len(anchors) // total] if anchors else None

        def slab_group(r):
            return (r % LANES) // 16 if r < KR else 8 + ((r - KR) % KU) // 16

        def ln1(blk, anchors1, anchors2=()):
            slabs = (xio_s[blk, r:r + 8, :].astype(F32) for r in range(0, D, 8))
            m, rs = _ln_stats(slabs, D, anchors1)
            if not anchors2:
                return (xio_s[blk].astype(F32) - m) * rs
            m8 = jnp.broadcast_to(m, (8, TM))
            ms = [_tie(m8, a) for a in anchors2]
            ms = [spread_over(ms, slab_group(r), 12) for r in range(0, D, 8)]
            return (xio_s[blk].astype(F32) - cat0(*ms)) * rs

        def dot_k(rows, x, anchors, even=False):
            y = None
            for n, k in enumerate(range(0, D, LANES)):
                ks = slice(k, min(k + LANES, D))
                if even and k + LANES >= D:
                    mid = (rows.start + rows.stop) // 2
                    v = cat0(_dot(_upk(wt_s[rows.start:mid, ks]), x[ks]),
                             _dot(_upk(wt_s[mid:rows.stop, ks]), x[ks]))
                else:
                    v = _dot(_upk(wt_s[rows, ks]), x[ks])
                anchors.extend(v[r:r + 8, :LANES] for r in ((0, 144) if n % 2 else (72, 216)))
                y = v if y is None else y + v
            return y

        def put_qkv(blk, rows, y):
            pk = _pk(y)
            for c in range(NT):
                qkv_s[1 + blk * NT + c, rows, :] = pk[:, c * LANES:(c + 1) * LANES]

        def qkv_mm(blk, xn, chunks, anchors, even=False):
            for r in chunks:
                rows = slice(r * QR // 2, (r + 1) * QR // 2)
                put_qkv(blk, rows, dot_k(rows, xn, anchors, even))

        def split_k(x):
            hs = (x[:, :TH], x[:, TH:])
            blocks = [[h[k * LANES:(k + 1) * LANES] for k in range(3)] for h in hs]
            units = [[h[KR + k * KU:KR + (k + 1) * KU] for k in range(3)] for h in hs]
            return blocks, units

        def prep_att(pat, anchor):
            assert Q3 == 96
            row0 = pat * 8
            src0 = row0 + ((pat * 43) >> 9) * (2 * Q3)
            w = [_upk(wt_s[rows8(src0 + j * Q3), :D]).astype(F32) for j in range(3)]
            w[0] = cat1(_tie(w[0][:, :LANES], anchor), w[0][:, LANES:])
            tiles = _w_sums([[w[j][:, k * LANES:(k + 1) * LANES] for j in range(3)]
                             for k in range(3)])
            for j in range(3):
                a, b, c = (w[j][:, KR + k * KU:KR + (k + 1) * KU] for k in range(3))
                tiles += [cat1(c, b), cat1(a, c)]
            wl_s[rows8(row0), :15 * LANES] = _pk(cat1(*tiles))

        def att_rhs(x, stash=None, anchors=()):
            half = 0.5
            if anchors:
                hs = [_tie(jnp.full((8, TH), 0.5, F32), a) for a in anchors]
                half = cat0(*[spread_over(hs, slab_group(r), 12) for r in range(0, D, 8)])
            blocks, units = split_k(cat1(x[:, :TH], x[:, TH:] + half * x[:, :TH]))
            ops = _x_ops(*blocks) + _x_rem(*units)
            if stash is None:
                return [v.astype(BF16) for v in ops]
            loc = lambda i, r0, n: (slice((i // 2) * 64 + r0, (i // 2) * 64 + r0 + n),
                                    slice((i % 2) * LANES, (i % 2 + 1) * LANES))
            for r in range(0, LANES, 16):
                for i, v in enumerate(ops):
                    r_s.at[0][loc(i, r // 2, 8)] = _pk(v[r:r + 16])
            return [_upk(r_s.at[stash][loc(i, 0, 64)]) for i in range(18)]

        def att_mm(sec, rhs, anchors):
            tl = lambda i: _upk(wl_s[sec * Q3:(sec + 1) * Q3, i * LANES:(i + 1) * LANES])
            raw = lambda k, j: _upk(wt_s[(3 * sec + j) * Q3:(3 * sec + j + 1) * Q3,
                                         k * LANES:(k + 1) * LANES])
            t = {}
            for i in _PAIR_ORDER:
                t[i] = _dot(raw(*_W_RAW[i]) if i in _W_RAW else tl(_W_SUM[i]), rhs[i])
                anchors.append(t[i][:8])
            out = []
            for j in range(3):
                base = []
                for s in range(3):
                    v = _dot(raw(3, j) if s == 1 else tl(9 + 2 * j + s // 2), rhs[15 + s])
                    if (s, j) in _DIAG:
                        i = _DIAG[s, j]
                        v = _dot(tl(_W_SUM[i]), rhs[i]) + v
                    base.append(v)
                    anchors.append(base[-1][:8])
                out.append(cat1(*_column(t, base, j, True)))
            return cat0(*out)

        def qkv_fast(blk, rhs, anchors):
            for sec in range(3):
                put_qkv(blk, slice(sec * RP, (sec + 1) * RP), att_mm(sec, rhs, anchors))

        def shifted(ln, cur, prev, w):
            if w == 0:
                return cur
            sh = DIL * w
            return pltpu.roll(jnp.where(ln < LANES - sh, cur, prev), sh, axis=1)

        def att_group(blk, c, hg, anchor):
            att_values(blk, c, hg, anchor)(None)

        def att_values(blk, c, hg, anchor):
            tile = blk * NT + c
            base = hg * 8 * DP
            if isinstance(hg, int):
                cur, prev, o_t = qkv_s.at[1 + tile], qkv_s.at[tile], o_s.at[c]
            else:
                n = 2 * RP + 8 * DP
                base = pl.multiple_of(base, 8)
                cur = qkv_s.at[1 + tile, pl.ds(base, n)]
                prev = qkv_s.at[tile, pl.ds(base, n)]
                o_t = o_s.at[c, pl.ds(base, RP + 8 * DP)]
                base = 0
            ln = lane + _zero_like_dep(anchor).astype(jnp.int32)
            logits = [None] * W
            for dd in range(DP):
                q = cur[pl.ds(base + dd, 8, stride=DP), :]
                kc = cur[pl.ds(RP + base + dd, 8, stride=DP), :]
                kp = prev[pl.ds(RP + base + dd, 8, stride=DP), :]
                q0, q1 = _lo(q), _hi(q)
                for w in range(W):
                    ks = shifted(ln, kc, kp, w)
                    t = q0 * _lo(ks) + q1 * _hi(ks)
                    logits[w] = t if logits[w] is None else logits[w] + t
            logits = [l * scale for l in logits]
            if not (isinstance(c, int) and c > 0):
                pos = lane + tile * LANES
                logits = [l if w == 0 else jnp.where(pos >= DIL * w, l, -1e9)
                          for w, l in enumerate(logits)]
            m = _tree_sum(logits, jnp.maximum)
            p = [jnp.exp(l - m) for l in logits]
            r = 1.0 / _tree_sum(p)

            def apply(anchor2):
                ln = lane + _zero_like_dep(m if anchor2 is None else anchor2).astype(jnp.int32)
                for dd in range(DP):
                    vc = cur[pl.ds(2 * RP + base + dd, 8, stride=DP), :]
                    vp = prev[pl.ds(2 * RP + base + dd, 8, stride=DP), :]
                    o0 = o1 = None
                    for w in range(W):
                        vs = shifted(ln, vc, vp, w)
                        t0, t1 = p[w] * _lo(vs), p[w] * _hi(vs)
                        o0 = t0 if o0 is None else o0 + t0
                        o1 = t1 if o1 is None else o1 + t1
                    o0, o1 = o0 * r, o1 * r
                    o_t[pl.ds(base + dd, 8, stride=DP), :] = o0
                    o_t[pl.ds(RP + base + dd, 8, stride=DP), :] = o1

            return apply

        def attention(blk, anchors):
            for c in range(NT):
                for hg in range(NG):
                    att_group(blk, c, hg, anchors[c * NG + hg])

        def wo_mm(blk, anchors, fast, stash=None, anchors_in=()):
            o = cat1(*[o_s[c] for c in range(NT)])
            if fast:
                y = att_mm(3, att_rhs(o, stash, anchors_in), anchors)
            else:
                o = o.astype(BF16)
                q = D2 // 2
                y = cat0(*[dot_k(slice(h * q, (h + 1) * q), o, anchors) for h in (6, 7)])
            xm = xio_s[blk].astype(F32) + y
            xmid_s[blk] = xm
            return _ln_stats((xm[r:r + 8] for r in range(0, D, 8)), D)

        def ffn_lhs(blk, stats, anchors):
            m, rs = stats
            m8 = jnp.broadcast_to(m, (8, TM))
            xt = []
            for k in range(5):
                mt = cat0(*[_tie(m8, spread_over(anchors[:2], k, 5))] * (KU // 8 if k == 4 else 16))
                x = (xmid_s[blk, k * LANES:min((k + 1) * LANES, D), :] - mt) * rs
                xt.append((cat0(x, x) if k == 4 else x).T)
            lo = lax.broadcasted_iota(jnp.int32, (TQ // 2, LANES), 1) < KU
            for m1 in range(7):
                a = spread_over(anchors[2:], m1, 7)
                blk1 = lambda i2, k2: _signed(_SA[m1], lambda i1, k1: _tie(
                    xt[k2 if k2 == 4 else 2 * k1 + k2][(2 * i1 + i2) * TQ:(2 * i1 + i2 + 1) * TQ], a))
                l1 = {(i2, k2): blk1(i2, k2) for i2 in range(2)
                      for k2 in ((0, 1, 4) if m1 in _SCOL else (0, 1))}
                for m2 in range(7):
                    v = _signed(_SA[m2], lambda i2, k2: l1[i2, k2])
                    if m1 in _SCOL and m2 in _SCOL:
                        c = _signed(_SA[m2], lambda i2, k2: l1[i2, 4])
                        h = TQ // 2
                        vp, vq, cp, cq = v[:h], v[h:], c[:h], c[h:]
                        v = cat0(jnp.where(lo, cp, vq), jnp.where(lo, vp, vp - vq),
                                 jnp.where(lo, vq, cq - cp))
                    o, ac = AOFF[m1, m2]
                    a_s[o:o + v.shape[0] // 2, ac] = _pk(v)

        def plain_lhs(blk, stats):
            m, rs = stats
            blocks, units = split_k((xmid_s[blk] - m) * rs)
            for i, v in enumerate(blocks[0] + blocks[1] + _x_rem(*units)):
                a_s[AOFF[i][0]:AOFF[i][0] + 64, AOFF[i][1]] = _pk(v.astype(BF16).T)

        def plain_piece(p, anchors):
            h = []
            for n in range(4):
                cs = slice(n * LANES, (n + 1) * LANES)
                w = lambda r0, r1: cat1(wg_v[p, r0:r1, cs], wu_v[p, r0:r1, cs])
                u = lambda k: w(KR + k * KU, KR + (k + 1) * KU)
                tl = lambda *i: _upk(cat1(*[a_s[AOFF[k][0]:AOFF[k][0] + 64, AOFF[k][1]]
                                            for k in i]))
                y0 = _dot(tl(6), cat0(u(2), u(1)))
                y1 = _dot(tl(0, 1, 2, 7), w(0, KR + 2 * KU))
                y2 = _dot(tl(3, 4, 5, 8), cat0(w(0, KR + KU), u(2)))
                anchors.append(y0[:8, :LANES])
                for y in (y1, y2):
                    anchors.extend(y[r:r + 8, c:c + LANES] for c in (0, LANES)
                                   for r in (0, TH // 2))
                h.append([_gelu_mul2(*[(y + y0)[:, c:c + LANES] for c in (0, LANES)])
                          for y in (y1, y2)])
            return h

        def in_triple(q):
            return q, lambda k: (q, k)

        def cross_triple(s):
            return NP + s, lambda k: (3 * s + k, 3)

        def wd_raw(tri, k, r0, n):
            q, c = tri[1](k)
            return wdt_v[q, r0:r0 + n, c * LANES:(c + 1) * LANES]

        def ds_loc(i, r0, n):
            return slice(r0, r0 + n), slice((i % 2) * LANES, (i % 2 + 1) * LANES)

        def prep_d(tri, anchors):
            PR = 16
            for n in range(D3 // PR):
                r = n * PR
                w = [[wd_raw(tri, k, j * D3 + r, PR).astype(F32) for j in range(3)]
                     for k in range(3)]
                w[0][1] = _tie(w[0][1], spread_over(anchors, n, D3 // PR))
                for i, v in enumerate(_w_sums(w)):
                    ds_s.at[tri[0], i // 2][ds_loc(i, r // 2, PR // 2)] = _pk(v)

        GU = (wg_v, wu_v)

        def prep_gu(p, m, m1s, anchors):
            PR = 16
            cs = slice(m * LANES, (m + 1) * LANES)
            for n in range(LANES // PR):
                r = n * PR
                cache = {}

                def w(k, j1):
                    if (k, j1) not in cache:
                        v = GU[m][p, k * LANES + r:k * LANES + r + PR,
                                  2 * j1 * LANES:2 * (j1 + 1) * LANES].astype(F32)
                        if (k // 2, j1) in [_SB[m1][0][:2] for m1 in m1s[:2]]:
                            v = _tie(v, spread_over(anchors, n, LANES // PR))
                        cache[k, j1] = v
                    return cache[k, j1]

                for m1 in m1s:
                    b1 = [_signed(_SB[m1], lambda k1, j1: w(2 * k1 + k2, j1)) for k2 in range(2)]
                    for m2 in range(7):
                        v = _signed(_SB[m2],
                                    lambda k2, j2: b1[k2][:, j2 * LANES:(j2 + 1) * LANES])
                        gu_s.at[p, 7 * m1 + m2][r // 2:(r + PR) // 2, cs] = _pk(v)

        def prep_tail(p, m, anchor):
            v = _tie(GU[m][p, 4 * LANES:, :].astype(F32), anchor)
            for j in range(4):
                gu_s.at[p, 49 + j // 2][(j % 2) * 32:(j % 2 + 1) * 32,
                                        m * LANES:(m + 1) * LANES] = _pk(
                                            v[:, j * LANES:(j + 1) * LANES])

        def gu_outer(p, m, m1, anchors, at=(0, 4)):
            cs = slice(m * LANES, (m + 1) * LANES)
            y = {}
            for m2 in cfg['inner']:
                i, (o, ac) = 7 * m1 + m2, AOFF[m1, m2]
                if m1 in _SCOL and m2 in _SCOL:
                    j = 2 * _SCOL[m1] + _SCOL[m2]
                    tail = lambda: gu_s[p, 49 + j // 2, (j % 2) * 32:(j % 2 + 1) * 32, cs]
                    rhs = (cat0(tail(), gu_s[p, i, 32:, cs]), gu_s[p, i, :, cs],
                           cat0(gu_s[p, i, :32, cs], tail()))
                    r = [_dot(_upk(a_s[o + 16 * s:o + 16 * (s + 1), ac]), _upk(rhs[s]))
                         for s in range(3)]
                    y[m2] = cat0(r[1] + r[0], r[2] + r[0])
                else:
                    y[m2] = _dot(_upk(a_s[o:o + TQ // 2, ac]), _upk(gu_s[p, i, :, cs]))
            anchors.extend(y[cfg['inner'][k % 7]][(k // 7) * 32:(k // 7) * 32 + 8] for k in at)
            return _s_out(y)

        def gu_finish(t):
            gu = [{(i2, j2): _s_out([t[m][m1][i2][j2] for m1 in range(7)])
                   for i2 in range(2) for j2 in range(2)} for m in range(2)]
            return [[cat0(*[_gelu_mul2(*[gu[m][i2, j % 2][i1][j // 2] for m in range(2)])
                            for i2 in range(2)]) for i1 in range(2)] for j in range(4)]

        def gu_piece(p, anchors):
            t = ({}, {})
            for m, m1 in cfg['gorder']:
                t[m][m1] = gu_outer(p, m, m1, anchors)
            return gu_finish(t)

        def h_ops(h):
            return [v.astype(BF16) for v in _x_ops(*[[h[k][i] for k in range(3)]
                                                     for i in range(2)])]

        D_ORDER = _PAIR_ORDER + (9, 10, 11, 12, 13, 14)

        def down_mm(acc, work, anchors, which=D_ORDER, fine=False):
            p = [None] * 15 if acc is None else list(acc)
            jobs = [(i, n) for i in which for n in range(len(work))]
            split = {0: (), 1: (4,), 2: (2, 2), 3: (2, 2, 4)}[len(jobs) % 4]
            split = dict(zip(jobs[len(jobs) - len(split):], split))
            for i in which:
                y = None
                for n, (tri, b) in enumerate(work):
                    ns = split.get((i, n), 1)
                    nr = D3 // ns
                    if i in _W_RAW:
                        k, j = _W_RAW[i]
                        lhs = lambda h: wd_raw(tri, k, j * D3 + h * nr, nr)
                    else:
                        s = _W_SUM[i]
                        lhs = lambda h: _upk(ds_s.at[tri[0], s // 2][ds_loc(s, h * nr // 2, nr // 2)])
                    v = cat0(*[_dot_nt(lhs(h), b[i]) for h in range(ns)])
                    y = v if y is None else y + v
                p[i] = y if p[i] is None else p[i] + y
                anchors.append(p[i][:8])
                if fine:
                    anchors.append(p[i][D3 // 2:D3 // 2 + 8])
            return p

        def finish(blk, acc):
            y = [cat1(*_column(acc, [acc[_DIAG[s, j]] if (s, j) in _DIAG else None
                                     for s in range(3)], j)) for j in range(3)]
            xio_s[blk] = (xmid_s[blk] + 0.5 * cat0(*y)).astype(BF16)

        def load_acc(k):
            return [acc_s[k, i] for i in range(15)]

        def store_acc(k, acc):
            for i in range(15):
                acc_s[k, i] = acc[i]

        def b_loc(i):
            return (slice((i // 2) * 64, (i // 2 + 1) * 64),
                    slice((i % 2) * LANES, (i % 2 + 1) * LANES))

        def load_b():
            return [_upk(b_s[b_loc(i)]) for i in range(15)]

        def store_h(p, h):
            for i, v in enumerate(h_ops(h[:3])):
                b_s[b_loc(i)] = _pk(v)
            h3_s[p] = cat0(*h[3])

        def pre_phase():
            first = [[x_cp(0, 0)], [wq_cp(0)], [x_cp(1, 2), wq_cp(1)],
                     [wq_cp(2), pltpu.make_async_copy(wo_hbm, wo_v, sem_i.at[3])]]
            order = sum(first, [])
            for p in range(NP + 1):
                order += group_cp(p)
            xr_cp = [x_cp(b, SEM_P + NP + 1) for b in range(2, NB)]
            order += xr_cp
            for cp in order:
                cp.start()
            get = lambda an, name: [an[min(i, len(an) - 1)] for i in cfg[name]]
            e_grp = lambda e: ((e >> 1) & 1, ((e >> 2) << 1) | (e & 1))
            if 'a' in cfg['sub']:
                pre_a(first, get, e_grp)
            if 'b' in cfg['sub']:
                pre_b(get, e_grp)
            if 'c' in cfg['sub']:
                pre_c(get)
            wait('WX', xr_cp)

        def pre_a(first, get, e_grp):
            def transpose_wq(i):
                wt_s[WQ[i] // 2:WQ[i + 1] // 2, :D] = _pk(wqkv_v[:, WQ[i]:WQ[i + 1]].T)

            def clear(i, carry):
                for k in range(2):
                    acc_s[k, i] = jnp.zeros((D3, TH), F32)
                r = jnp.minimum(i, 11) * (RP // 4)
                qkv_s[0, rows8(r, RP // 4)] = jnp.zeros((RP // 4, LANES), U32)
                return carry

            lax.fori_loop(0, 15, clear, 0)
            wait('WX0', first[0])
            xn0 = ln1(0, ()).astype(BF16)

            wait('WQ0', first[1])
            transpose_wq(0)
            qkv_mm(0, xn0, (0, 1), [])

            wait('WQ1', first[2])
            transpose_wq(1)
            an = []
            qkv_mm(0, xn0, (2, 3), an)
            xn1 = ln1(1, get(an, 'a_ln'), get(an, 'a_lnb')).astype(BF16)
            qkv_mm(1, xn1, (0,), an, True)
            for n, a in enumerate(get(an, 'a_w1')):
                prep_att(n, a)
            nk = len(cfg['a_k'])
            apply = [att_values(0, *e_grp(e), a) for e, a in enumerate(get(an, 'a_k'))]

            wait('WQ2', first[3])
            an = []
            qkv_mm(1, xn1, (2,), an)
            transpose_wq(2)
            qkv_mm(0, xn0, (4, 5), an)
            qkv_mm(1, xn1, (4, 1), an)
            apply += [att_values(0, *e_grp(nk + e), a)
                      for e, a in enumerate(get(an, 'a_k2')[:8 - nk])]
            for e, a in enumerate(get(an, 'a_v')):
                apply[e](a)
            wo = pltpu.bitcast(wo_v[...], U32)
            wo = cat0(_lo(wo), _hi(wo))
            wo = cat0(*[_tie(wo[n * LANES:(n + 1) * LANES], a)
                        for n, a in enumerate(get(an, 'a_wo'))])
            wt_s[3 * RP:, :D] = _pk(wo.astype(BF16).T)
            stats = wo_mm(0, an, False)
            qkv_mm(1, xn1, (3,), an)
            for n, a in enumerate(get(an, 'a_w2')):
                prep_att(12 + n, a)
            plain_lhs(0, stats)

            wait('WO', group_cp(0))
            an = []
            h = plain_piece(0, an)
            qkv_mm(1, xn1, (5,), an, True)
            zg = get(an, 'z_g')
            for n in range(6):
                prep_gu(0, n % 2, _SGRP[n // 2], zg[8 * n:8 * n + 8])
            for m in range(2):
                prep_tail(0, m, zg[m])
            if not cfg['plain0']:
                ffn_lhs(0, stats, get(an, 'z_l'))
            store_h(0, h)

        def pre_b(get, e_grp):
            def piece(p, carry):
                wait('WP', group_cp(p))
                work = [(in_triple(p - 1), load_b())]
                an = []
                if cfg['plain0']:
                    h = plain_piece(p, an)
                    prep_d(work[0][0], get(an, 'p_d'))
                    store_acc(0, down_mm(load_acc(0), work, an))
                    for m in range(2):
                        prep_tail(p, m, get(an, 'f_t')[m])
                    grp = _SGRP if cfg['plain0'] == 2 else [(m1,) for m1 in range(7)]
                    fg = get(an, 'f_g')
                    for n in range(2 * len(grp)):
                        k = len(fg) // (2 * len(grp))
                        prep_gu(p, n % 2, grp[n // 2], fg[k * n:k * n + k])
                else:
                    acc = down_mm(load_acc(0), work, an, D_ORDER[:6], True)
                    t = ({}, {})
                    for m in range(2):
                        prep_tail(p, m, get(an, 'f_t')[m])
                    for n, (m, m1) in enumerate(cfg['gorder0']):
                        prep_gu(p, m, (m1,), get(an, 'f_g')[4 * n:4 * n + 4])
                        t[m][m1] = gu_outer(p, m, m1, an, (0, 7, 4, 11))
                    h = gu_finish(t)
                    prep_d(work[0][0], get(an, 'p_d'))
                    store_acc(0, down_mm(acc, work, an, D_ORDER[6:]))
                att_group(1, *e_grp(p - 1), an[cfg['p_att'][0]])
                for i, a in enumerate(get(an, 'p_w')):
                    prep_att(48 - (NP - p) * len(cfg['p_w']) + i, a)
                store_h(p, h)
                return carry

            lax.fori_loop(1, NP, piece, 0)

        def pre_c(get):
            wait('WD', group_cp(NP))
            work = [(in_triple(NP - 1), load_b())]
            for s in range(3):
                h3 = [h3_s[3 * s + k] for k in range(3)]
                work.append((cross_triple(s), h_ops([[v[:TH], v[TH:]] for v in h3])))
            an = []
            stats = wo_mm(1, an, True)
            acc = down_mm(load_acc(0), work, an, D_ORDER[:6], True)
            td = get(an, 't_d')
            for n, (tri, _) in enumerate(work):
                prep_d(tri, td[n * len(td) // 4:(n + 1) * len(td) // 4])
            acc = down_mm(acc, work, an, D_ORDER[6:])
            ffn_lhs(1, stats, get(an, 't_l'))
            finish(0, acc)

        if 'pre' in cfg['phases']:
            pre_phase()

        def body(u, carry):
            bu = u & (NB - 1)
            ba = (u + 1) & (NB - 1)
            acc, stats, an, b, hh = None, None, {}, {}, {}
            get = lambda name: [an[k][i] for k, i in cfg[name]]
            for step in cfg['body']:
                an[step] = []
                if step == 'Q':
                    xn = ln1(ba, get('ln1'), get('ln1b'))
                    qkv_fast(ba, att_rhs(xn, u >> 8), an[step])
                elif step == 'W':
                    attention(ba, get('att'))
                    stats = wo_mm(ba, an[step], True, u >> 8, get('orhs'))
                elif step == 'L':
                    ffn_lhs(ba, stats, get('lhs'))
                elif step[0] == 'G':
                    q, go = int(step[1]), cfg['gorder']
                    t = b.setdefault(step[:2], ({}, {}))
                    for m, m1 in (go[:7] if step[2] == '0' else go[7:]):
                        t[m][m1] = gu_outer(q, m, m1, an[step])
                    if len(t[0]) + len(t[1]) == 14:
                        hh[q] = gu_finish(t)
                else:
                    work = []
                    for c in step[1:]:
                        if c.isdigit():
                            work.append((in_triple(int(c)), h_ops(hh[int(c)][:3])))
                        else:
                            s = ord(c) - ord('a')
                            work.append((cross_triple(s),
                                         h_ops([hh[3 * s + k][3] for k in range(3)])))
                    acc = down_mm(acc, work, an[step])
            finish(bu, acc)

            @pl.when(u >= NB)
            def _():
                out_copy(bu).start()
            return carry

        if scopes:
            with jax.named_scope('LOOP'):
                lax.fori_loop(1, NU - 1, body, 0)
        elif 'main' in cfg['phases']:
            lax.fori_loop(1, NU - 1, body, 0)

        def last(s, carry):
            h = [gu_piece(3 * s + k, []) for k in range(3)]
            work = [(in_triple(3 * s + k), h_ops(h[k][:3])) for k in range(3)]
            work.append((cross_triple(s), h_ops([h[k][3] for k in range(3)])))
            acc = down_mm(down_mm(load_acc(1), work[:2], []), work[2:], [])
            store_acc(1, acc)
            finish(NB - 1, acc)
            return carry

        if 'last' in cfg['phases']:
            lax.fori_loop(0, NP // 3, last, 0)
        if len(cfg['phases']) < 3:
            def keep(i, c):
                v = (gu_s[i, i, :8, :LANES] + ds_s[i, i, :8, :LANES]
                     + wl_s[rows8(i * 8), :LANES] + a_s[rows8(i * 8), :LANES] + qkv_s[i, :8]
                     + b_s[rows8(i * 8), :LANES] + wt_s[rows8(i * 8), :LANES])
                acc_s[1, 0, :8] = (lax.bitcast_convert_type(v, F32) + o_s[i, :8]
                                   + acc_s[i, i, :8] + h3_s[i, :8])
                return c
            lax.fori_loop(0, 2, keep, 0)
            finish(NB - 1, load_acc(1))
        out_copy(NB - 1).start()
        wait('WOUT', [out_copy(b) for b in range(NB)])

    scratch = [
        pltpu.VMEM((NB, D, TM), BF16),
        pltpu.VMEM((D, 3 * D), BF16),
        pltpu.VMEM((D, D), BF16),
        pltpu.VMEM((NP, D, PW), BF16),
        pltpu.VMEM((NP, D, PW), BF16),
        pltpu.VMEM((NP, D, PW), BF16),
        pltpu.VMEM((2 * D, 8 * LANES), U32),
        pltpu.VMEM((4 * Q3, 16 * LANES), U32),
        pltpu.VMEM((NP, 51, 64, 2 * LANES), U32),
        pltpu.VMEM((NP + 3, 5, Q3, 2 * LANES), U32),
        pltpu.VMEM((NB, D, TM), F32),
        pltpu.VMEM((max(fill), 2 * LANES), U32),
        pltpu.VMEM((S // LANES + 1, 3 * RP, LANES), U32),
        pltpu.VMEM((NT, D, LANES), F32),
        pltpu.VMEM((2, 15, D3, TH), F32),
        pltpu.VMEM((8 * 64, 2 * LANES), U32),
        pltpu.VMEM((NP, TM, LANES), F32),
        pltpu.VMEM((1, 9 * 64, 2 * LANES), U32),
        pltpu.SemaphoreType.DMA((SEM_P + NP + 2,)),
        pltpu.SemaphoreType.DMA((1,)),
    ]

    def wrapped(*refs):
        @pl.when(pl.program_id(0) == 0)
        def _():
            kernel(*refs)

    return wrapped, scratch


_CFG = dict(
    scopes=False,
    orhs=(('G80', 0), ('G80', 1), ('G80', 2), ('G80', 3), ('G80', 4), ('G80', 5),
        ('G80', 6), ('G80', 7), ('G80', 8), ('G80', 9), ('G80', 10), ('G80', 11)),
    plain0=2,
    sub='abc',
    phases=('pre', 'main', 'last'),
    body=('G20', 'G00', 'G01', 'G10', 'G11', 'Q', 'G30', 'G21', 'G40', 'G31', 'G50',
        'D012a', 'G41', 'G51', 'D345b', 'G70', 'G71', 'G60', 'G80', 'W', 'G61', 'G81',
        'D8c', 'D67', 'L'),
    ln1=(('G00', 0), ('G00', 1), ('G00', 2), ('G00', 3), ('G00', 4), ('G00', 5), ('G00',
        6), ('G00', 7), ('G00', 8)),
    ln1b=(('G10', 1), ('G10', 2), ('G10', 3), ('G10', 4), ('G10', 5), ('G10', 6),
        ('G10', 7), ('G10', 8), ('G10', 9), ('G10', 10), ('G10', 11), ('G10', 12)),
    att=(('D012a', 2), ('D012a', 4), ('D012a', 5), ('D012a', 6), ('D012a', 9), ('D345b',
        6), ('D345b', 7), ('D345b', 8)),
    lhs=(('D8c', 2), ('D8c', 3), ('D8c', 6), ('D67', 5), ('D67', 7), ('D67', 8), ('D67',
        10), ('D67', 11), ('D67', 14)),
    a_w1=(0, 0, 1, 2, 2, 3, 3, 4, 4, 5, 7, 11),
    a_w2=(0, 1, 3, 4, 6, 8, 9, 12, 13, 14, 16, 18, 44, 45, 46, 48, 49, 50, 52, 53, 55,
        56, 57, 59, 60, 62, 63, 64, 66, 67, 69, 70, 71, 73, 74, 76),
    a_ln=(0, 3, 6),
    a_lnb=(5, 9, 10),
    z_g=(0, 0, 1, 2, 3, 4, 5, 6, 7, 8, 9, 10, 11, 12, 13, 14, 15, 17, 18, 18, 19, 20,
        21, 22, 23, 24, 24, 25, 26, 28, 28, 29, 30, 31, 32, 33, 34, 35, 36, 37, 38, 39,
        40, 41, 42, 43, 44, 45),
    t_d=(0, 0, 0, 1, 2, 3, 4, 4, 4, 4, 5, 6, 8, 8, 9, 10, 10, 10, 11, 11, 11, 13, 14,
        14, 15, 16, 16, 16, 17, 17, 18, 19, 20, 20, 21, 21, 22, 22, 23, 23, 24, 24, 25,
        25, 26, 26, 27, 28),
    p_d=(12, 15, 17, 19, 21, 23, 25, 25, 28, 29, 33, 35),
    p_att=(33,),
    p_w=(),
    z_l=(4, 8, 12, 16, 20, 24, 28, 32, 36),
    a_k=(15, 19, 20, 24),
    a_k2=(4, 7, 10, 14),
    a_v=(11, 13, 22, 26, 30, 34, 37, 38),
    a_wo=(36, 36, 37, 38, 38),
    inner=(0, 3, 4, 6, 2, 1, 5),
    gorder=((0, 0), (0, 4), (1, 4), (1, 0), (0, 3), (1, 3), (1, 6), (0, 6), (0, 1), (1,
        1), (0, 2), (1, 2), (0, 5), (1, 5)),
    gorder0=((0, 1), (1, 1), (0, 4), (1, 4), (0, 0), (1, 0), (0, 3), (1, 3), (0, 6), (1,
        6), (0, 2), (1, 2), (0, 5), (1, 5)),
    f_t=(7, 38),
    f_g=(0, 0, 1, 1, 1, 2, 3, 3, 4, 5, 5, 6, 7, 7, 8, 9, 10, 10, 11, 11, 12, 12, 12, 13,
        14, 14, 15, 16, 17, 18, 18, 19, 20, 20, 21, 21, 21, 22, 23, 23, 24, 25, 25, 26,
        27, 27, 28, 29, 30, 31, 31, 32, 32, 33, 34, 39),
    t_l=(17, 25, 28, 30, 31, 33, 34, 35, 37),
    f_g0=(0, 1, 2, 3, 4, 5, 6, 7),
    f_g1=(8, 9, 11, 13, 14, 16, 18, 20),
    f_g2=(21, 22, 24, 26, 27, 29, 31, 33),
    f_g3=(33, 34, 35, 36, 38, 39, 40, 42),
    f_g4=(42, 43, 44, 45, 46, 47, 48, 50),
    f_g5=(50, 51, 52, 53, 54, 55, 56, 58),
)


def _run(A_x, A_wqkv, A_wo, B_w_gate, B_w_up, B_w_down, **kw):
    _, S, D = A_x.shape
    F = B_w_gate.shape[1]
    kernel, scratch = _make_kernel(S, D, F, 256, {**_CFG, **kw})
    hbm = pl.BlockSpec(memory_space=pl.ANY)
    out_t = pl.pallas_call(
        kernel,
        grid=(2,),
        in_specs=[hbm] * 6,
        out_specs=hbm,
        out_shape=jax.ShapeDtypeStruct((D, S), A_x.dtype),
        scratch_shapes=scratch,
        compiler_params=pltpu.CompilerParams(
            dimension_semantics=('arbitrary',), vmem_limit_bytes=110 * 1024 * 1024),
    )(A_x.reshape(S, D).T, A_wqkv, A_wo, B_w_gate, B_w_up, B_w_down.T)
    return out_t.T.reshape(A_x.shape)


@jax.jit
def pallas_interleave_layers__sliding_local_dilated__glu_gated_geglu__prompt_kernel(
    A_x: jax.Array,
    A_wqkv: jax.Array,
    A_wo: jax.Array,
    B_x: jax.Array,
    B_w_gate: jax.Array,
    B_w_up: jax.Array,
    B_w_down: jax.Array,
):
    del B_x
    return _run(A_x, A_wqkv, A_wo, B_w_gate, B_w_up, B_w_down)
```

```python
import jax
import jax.numpy as jnp
import jax.experimental.pallas as pl
import jax.experimental.pallas.tpu as pltpu
from jax import lax

H = 32
W = 8
DIL = 2
EPS = 1e-5
LANES = 128

F32 = jnp.float32
BF16 = jnp.bfloat16
U32 = jnp.uint32

_NT = (((1,), (1,)), ((), ()))


def _tree_sum(parts, op=jnp.add):
    while len(parts) > 1:
        nxt = [op(parts[i], parts[i + 1]) for i in range(0, len(parts) - 1, 2)]
        if len(parts) % 2:
            nxt.append(parts[-1])
        parts = nxt
    return parts[0]


def _ln_stats(slabs, d, anchors=()):
    n_acc = 4
    s1, s2, pilot = [None] * n_acc, [None] * n_acc, None
    for i, x in enumerate(slabs):
        if pilot is None:
            pilot = x[0:1, :]
            pil = jnp.broadcast_to(pilot, x.shape)
            pils = [_tie(pil, a) for a in anchors] or [pil]
        dx = x - pils[i * len(pils) // (d // 8)]
        j = i % n_acc
        s1[j] = dx if s1[j] is None else s1[j] + dx
        s2[j] = dx * dx if s2[j] is None else s2[j] + dx * dx
    e1 = jnp.sum(_tree_sum(s1), axis=0, keepdims=True) * (1.0 / d)
    e2 = jnp.sum(_tree_sum(s2), axis=0, keepdims=True) * (1.0 / d)
    var = jnp.maximum(e2 - e1 * e1, 0.0)
    return pilot + e1, lax.rsqrt(var + EPS)


def _zero_like_dep(v):
    return (lax.bitcast_convert_type(v, U32) >> 31) >> 1


def _tie(x, anchor):
    if anchor is None:
        return x
    z = lax.bitcast_convert_type(_zero_like_dep(anchor), F32)
    z = jnp.concatenate([z] * -(-x.shape[1] // LANES), axis=1)[:, :x.shape[1]]
    if x.shape[0] == 8:
        return x + z
    return jnp.concatenate([x[:8] + z, x[8:]], axis=0)


def _gelu_mul2(g, u):
    c0 = 0.7978845608028654
    c1 = c0 * 0.044715
    t = jnp.tanh(g * (c0 + c1 * (g * g)))
    return (g * u) * (1.0 + t)


def _lo(x):
    return lax.bitcast_convert_type(x << 16, F32)


def _hi(x):
    return lax.bitcast_convert_type(x & jnp.uint32(0xFFFF0000), F32)


def _pk(x):
    return pltpu.bitcast(x.astype(BF16), U32)


def _upk(x):
    return pltpu.bitcast(x, BF16)


def _dot(a, b):
    return jnp.dot(a, b, preferred_element_type=F32)


def _dot_nt(a, b):
    return lax.dot_general(a, b, _NT, preferred_element_type=F32)


def _x_ops(x1, x2):
    d = [a - b for a, b in zip(x1, x2)]
    return [x1[0] + x2[1], x2[0] + x2[1], x1[0] + x1[1],
            d[1] + x1[2], x1[1] + x1[2], d[1] + d[2],
            d[0] - x2[2], d[0] + d[2], x2[0] + x2[2],
            x1[0], d[0], x2[1], d[1], x1[2], x2[2]]


def _x_rem(x1, x2):
    a, b, c = 0, 1, 2
    cat = lambda u, v: jnp.concatenate([u, v], axis=0)
    return [cat(x1[c], x2[b]), cat(x1[a], x1[b] - x2[b]), cat(x2[a], x2[c] - x1[c])]


_W_TERMS = {0: ((0, 1, 1), (1, 0, 1)), 3: ((1, 2, 1), (2, 1, 1)), 6: ((0, 2, 1), (2, 0, 1)),
            9: ((0, 0, 1), (0, 2, 1), (1, 0, -1)), 10: ((2, 0, 1), (0, 0, -1), (0, 1, -1)),
            11: ((1, 1, 1), (1, 2, 1), (0, 1, -1)), 12: ((1, 0, 1), (1, 1, 1), (2, 1, -1)),
            13: ((2, 0, 1), (2, 2, 1), (1, 2, -1)), 14: ((2, 1, 1), (2, 2, 1), (0, 2, -1)),
            1: ((0, 1, 1),), 2: ((1, 0, 1),), 4: ((1, 2, 1),), 5: ((2, 1, 1),),
            7: ((2, 0, 1),), 8: ((0, 2, 1),)}


def _w_sums(w):
    return [_signed(_W_TERMS[i], lambda k, j: w[k][j]) for i in _W_SUM]


_W_SUM = {0: 0, 3: 1, 6: 2, 9: 3, 10: 4, 11: 5, 12: 6, 13: 7, 14: 8}
_W_RAW = {1: (0, 1), 2: (1, 0), 4: (1, 2), 5: (2, 1), 7: (2, 0), 8: (0, 2)}
_PAIR_ORDER = (1, 2, 4, 5, 7, 8, 0, 3, 6)
_DIAG = {(0, 0): 9, (2, 0): 10, (0, 1): 11, (1, 1): 12, (1, 2): 13, (2, 2): 14}
_PAIR = {(0, 0): ((6, -1), (8, -1)), (1, 0): ((2, 1), (7, 1)), (2, 0): ((0, 1), (1, -1)),
         (0, 1): ((3, 1), (4, -1)), (1, 1): ((0, 1), (2, -1)), (2, 1): ((1, 1), (5, -1)),
         (0, 2): ((4, 1), (8, 1)), (1, 2): ((6, 1), (7, -1)), (2, 2): ((5, 1), (3, -1))}


def _column(t, base, j, skew=False):
    s = []
    for k in range(3):
        v = base[k]
        for i, sg in _PAIR[k, j]:
            v = t[i] if v is None else (v + t[i] if sg > 0 else v - t[i])
        s.append(v)
    if skew:
        return s[1] + s[0], s[2] + 0.5 * (s[0] - s[1])
    return s[1] + s[0], s[2] + s[0]


_SA = (((0, 0, 1), (1, 1, 1)), ((1, 0, 1), (1, 1, 1)), ((0, 0, 1),), ((1, 1, 1),),
       ((0, 0, 1), (0, 1, 1)), ((1, 0, 1), (0, 0, -1)), ((0, 1, 1), (1, 1, -1)))
_SB = (((0, 0, 1), (1, 1, 1)), ((0, 0, 1),), ((0, 1, 1), (1, 1, -1)), ((1, 0, 1), (0, 0, -1)),
       ((1, 1, 1),), ((0, 0, 1), (0, 1, 1)), ((1, 0, 1), (1, 1, 1)))
_SCOL = {2: 1, 3: 0, 5: 1, 6: 0}
_SGRP = ((1, 4, 0), (3, 6), (2, 5))


def _signed(terms, f):
    v = None
    for a, b, sg in terms:
        v = f(a, b) if v is None else (v + f(a, b) if sg > 0 else v - f(a, b))
    return v


def _s_out(m):
    return [[m[0] + m[3] - m[4] + m[6], m[2] + m[4]],
            [m[1] + m[3], m[0] - m[1] + m[2] + m[5]]]


def _make_kernel(S, D, F, TM, cfg):
    NB = S // TM
    NT = TM // LANES
    DH = D // H
    DP = DH // 2
    RP = D // 2
    NG = H // 8
    scale = float(DH) ** -0.5
    NU = 2 * NB
    TH = TM // 2
    TQ = TM // 4
    D2 = D // 2
    D3 = D // 3
    Q3 = D3 // 2
    KU = D // 9
    KR = 3 * LANES
    NQ = 6
    QR = 3 * D // NQ
    WQ = (0, 640, 1152, 3 * D)
    PW = 4 * LANES
    NP = F // PW
    AOFF, fill = {}, [0, 0]
    for key in [(m1, m2) for m1 in range(7) for m2 in range(7)]:
        c = int(fill[1] < fill[0])
        AOFF[key] = (fill[c], slice(c * LANES, (c + 1) * LANES))
        fill[c] += 48 if key[0] in _SCOL and key[1] in _SCOL else 32
    scopes = cfg['scopes']
    assert NG == 4 and NB & (NB - 1) == 0
    SEM_P = 4

    def kernel(x_hbm, wqkv_hbm, wo_hbm, wg_hbm, wu_hbm, wdt_hbm, out_hbm,
               xio_s, wqkv_v, wo_v, wg_v, wu_v, wdt_v, wt_s, wl_s,
               gu_s, ds_s, xmid_s, a_s, qkv_s, o_s, acc_s, h3_s, r_s,
               sem_i, sem_o):

        def wait(name, cps):
            if scopes:
                with jax.named_scope(name):
                    for cp in cps:
                        cp.wait()
            else:
                for cp in cps:
                    cp.wait()

        def cols(lo, n):
            if not isinstance(lo, int):
                lo = pl.multiple_of(lo, LANES)
            return pl.ds(lo, n)

        def rows8(lo, n=8):
            if not isinstance(lo, int):
                lo = pl.multiple_of(lo, 8)
            return pl.ds(lo, n)

        def out_copy(b):
            return pltpu.make_async_copy(
                xio_s.at[b], out_hbm.at[:, cols(b * TM, TM)], sem_o.at[0])

        def x_cp(b, sem):
            return pltpu.make_async_copy(x_hbm.at[:, cols(b * TM, TM)], xio_s.at[b],
                                         sem_i.at[sem])

        def wq_cp(i):
            sl = cols(WQ[i], WQ[i + 1] - WQ[i])
            return pltpu.make_async_copy(wqkv_hbm.at[:, sl], wqkv_v.at[:, sl],
                                         sem_i.at[1 + i])

        def piece_cp(src, dst, p, sem):
            return [pltpu.make_async_copy(src.at[:, cols(p * PW, PW)], dst.at[p],
                                          sem_i.at[sem])]

        def group_cp(p):
            sem = SEM_P + p
            cps = []
            if not (isinstance(p, int) and p == NP):
                cps += piece_cp(wg_hbm, wg_v, p, sem) + piece_cp(wu_hbm, wu_v, p, sem)
            if not (isinstance(p, int) and p == 0):
                cps += piece_cp(wdt_hbm, wdt_v, p - 1, sem)
            return cps

        lane = lax.broadcasted_iota(jnp.int32, (8, LANES), 1)
        cat0 = lambda *v: jnp.concatenate(v, axis=0)
        cat1 = lambda *v: jnp.concatenate(v, axis=1)

        def spread_over(anchors, n, total):
            return anchors[n * len(anchors) // total] if anchors else None

        def slab_group(r):
            return (r % LANES) // 16 if r < KR else 8 + ((r - KR) % KU) // 16

        def ln1(blk, anchors1, anchors2=()):
            slabs = (xio_s[blk, r:r + 8, :].astype(F32) for r in range(0, D, 8))
            m, rs = _ln_stats(slabs, D, anchors1)
            if not anchors2:
                return (xio_s[blk].astype(F32) - m) * rs
            m8 = jnp.broadcast_to(m, (8, TM))
            ms = [_tie(m8, a) for a in anchors2]
            ms = [spread_over(ms, slab_group(r), 12) for r in range(0, D, 8)]
            return (xio_s[blk].astype(F32) - cat0(*ms)) * rs

        def dot_k(rows, x, anchors, even=False):
            y = None
            for n, k in enumerate(range(0, D, LANES)):
                ks = slice(k, min(k + LANES, D))
                if even and k + LANES >= D:
                    mid = (rows.start + rows.stop) // 2
                    v = cat0(_dot(_upk(wt_s[rows.start:mid, ks]), x[ks]),
                             _dot(_upk(wt_s[mid:rows.stop, ks]), x[ks]))
                else:
                    v = _dot(_upk(wt_s[rows, ks]), x[ks])
                anchors.extend(v[r:r + 8, :LANES] for r in ((0, 144) if n % 2 else (72, 216)))
                y = v if y is None else y + v
            return y

        def put_qkv(blk, rows, y):
            pk = _pk(y)
            for c in range(NT):
                qkv_s[1 + blk * NT + c, rows, :] = pk[:, c * LANES:(c + 1) * LANES]

        def qkv_mm(blk, xn, chunks, anchors, even=False):
            for r in chunks:
                rows = slice(r * QR // 2, (r + 1) * QR // 2)
                put_qkv(blk, rows, dot_k(rows, xn, anchors, even))

        def split_k(x):
            hs = (x[:, :TH], x[:, TH:])
            blocks = [[h[k * LANES:(k + 1) * LANES] for k in range(3)] for h in hs]
            units = [[h[KR + k * KU:KR + (k + 1) * KU] for k in range(3)] for h in hs]
            return blocks, units

        def prep_att(pat, anchor):
            assert Q3 == 96
            row0 = pat * 8
            src0 = row0 + ((pat * 43) >> 9) * (2 * Q3)
            w = [_upk(wt_s[rows8(src0 + j * Q3), :D]).astype(F32) for j in range(3)]
            w[0] = cat1(_tie(w[0][:, :LANES], anchor), w[0][:, LANES:])
            tiles = _w_sums([[w[j][:, k * LANES:(k + 1) * LANES] for j in range(3)]
                             for k in range(3)])
            for j in range(3):
                a, b, c = (w[j][:, KR + k * KU:KR + (k + 1) * KU] for k in range(3))
                tiles += [cat1(c, b), cat1(a, c)]
            wl_s[rows8(row0), :15 * LANES] = _pk(cat1(*tiles))

        def att_rhs(x, stash=None, anchors=()):
            half = 0.5
            if anchors:
                hs = [_tie(jnp.full((8, TH), 0.5, F32), a) for a in anchors]
                half = cat0(*[spread_over(hs, slab_group(r), 12) for r in range(0, D, 8)])
            blocks, units = split_k(cat1(x[:, :TH], x[:, TH:] + half * x[:, :TH]))
            ops = _x_ops(*blocks) + _x_rem(*units)
            if stash is None:
                return [v.astype(BF16) for v in ops]
            loc = lambda i, r0, n: (slice((i // 2) * 64 + r0, (i // 2) * 64 + r0 + n),
                                    slice((i % 2) * LANES, (i % 2 + 1) * LANES))
            for r in range(0, LANES, 16):
                for i, v in enumerate(ops):
                    r_s.at[0][loc(i, r // 2, 8)] = _pk(v[r:r + 16])
            return [_upk(r_s.at[stash][loc(i, 0, 64)]) for i in range(18)]

        def att_mm(sec, rhs, anchors):
            tl = lambda i: _upk(wl_s[sec * Q3:(sec + 1) * Q3, i * LANES:(i + 1) * LANES])
            raw = lambda k, j: _upk(wt_s[(3 * sec + j) * Q3:(3 * sec + j + 1) * Q3,
                                         k * LANES:(k + 1) * LANES])
            t = {}
            for i in _PAIR_ORDER:
                t[i] = _dot(raw(*_W_RAW[i]) if i in _W_RAW else tl(_W_SUM[i]), rhs[i])
                anchors.append(t[i][:8])
            out = []
            for j in range(3):
                base = []
                for s in range(3):
                    v = _dot(raw(3, j) if s == 1 else tl(9 + 2 * j + s // 2), rhs[15 + s])
                    if (s, j) in _DIAG:
                        i = _DIAG[s, j]
                        v = _dot(tl(_W_SUM[i]), rhs[i]) + v
                    base.append(v)
                    anchors.append(base[-1][:8])
                out.append(cat1(*_column(t, base, j, True)))
            return cat0(*out)

        def qkv_fast(blk, rhs, anchors):
            for sec in range(3):
                put_qkv(blk, slice(sec * RP, (sec + 1) * RP), att_mm(sec, rhs, anchors))

        def shifted(ln, cur, prev, w):
            if w == 0:
                return cur
            sh = DIL * w
            return pltpu.roll(jnp.where(ln < LANES - sh, cur, prev), sh, axis=1)

        def att_group(blk, c, hg, anchor):
            att_values(blk, c, hg, anchor)(None)

        def att_values(blk, c, hg, anchor):
            tile = blk * NT + c
            base = hg * 8 * DP
            if isinstance(hg, int):
                cur, prev, o_t = qkv_s.at[1 + tile], qkv_s.at[tile], o_s.at[c]
            else:
                n = 2 * RP + 8 * DP
                base = pl.multiple_of(base, 8)
                cur = qkv_s.at[1 + tile, pl.ds(base, n)]
                prev = qkv_s.at[tile, pl.ds(base, n)]
                o_t = o_s.at[c, pl.ds(base, RP + 8 * DP)]
                base = 0
            ln = lane + _zero_like_dep(anchor).astype(jnp.int32)
            logits = [None] * W
            for dd in range(DP):
                q = cur[pl.ds(base + dd, 8, stride=DP), :]
                kc = cur[pl.ds(RP + base + dd, 8, stride=DP), :]
                kp = prev[pl.ds(RP + base + dd, 8, stride=DP), :]
                q0, q1 = _lo(q), _hi(q)
                for w in range(W):
                    ks = shifted(ln, kc, kp, w)
                    t = q0 * _lo(ks) + q1 * _hi(ks)
                    logits[w] = t if logits[w] is None else logits[w] + t
            logits = [l * scale for l in logits]
            if not (isinstance(c, int) and c > 0):
                pos = lane + tile * LANES
                logits = [l if w == 0 else jnp.where(pos >= DIL * w, l, -1e9)
                          for w, l in enumerate(logits)]
            m = _tree_sum(logits, jnp.maximum)
            p = [jnp.exp(l - m) for l in logits]
            r = 1.0 / _tree_sum(p)

            def apply(anchor2):
                ln = lane + _zero_like_dep(_tie(m, anchor2)).astype(jnp.int32)
                for dd in range(DP):
                    vc = cur[pl.ds(2 * RP + base + dd, 8, stride=DP), :]
                    vp = prev[pl.ds(2 * RP + base + dd, 8, stride=DP), :]
                    o0 = o1 = None
                    for w in range(W):
                        vs = shifted(ln, vc, vp, w)
                        t0, t1 = p[w] * _lo(vs), p[w] * _hi(vs)
                        o0 = t0 if o0 is None else o0 + t0
                        o1 = t1 if o1 is None else o1 + t1
                    o0, o1 = o0 * r, o1 * r
                    o_t[pl.ds(base + dd, 8, stride=DP), :] = o0
                    o_t[pl.ds(RP + base + dd, 8, stride=DP), :] = o1

            return apply

        def attention(blk, anchors):
            for c in range(NT):
                for hg in range(NG):
                    att_group(blk, c, hg, anchors[c * NG + hg])

        def wo_mm(blk, anchors, fast, stash=None, anchors_in=()):
            o = cat1(*[o_s[c] for c in range(NT)])
            if fast:
                y = att_mm(3, att_rhs(o, stash, anchors_in), anchors)
            else:
                o = o.astype(BF16)
                q = D2 // 2
                y = cat0(*[dot_k(slice(h * q, (h + 1) * q), o, anchors) for h in (6, 7)])
            xm = xio_s[blk].astype(F32) + y
            xmid_s[blk] = xm
            return _ln_stats((xm[r:r + 8] for r in range(0, D, 8)), D)

        def ffn_lhs(blk, stats, anchors):
            m, rs = stats
            m8 = jnp.broadcast_to(m, (8, TM))
            xt = []
            for k in range(5):
                mt = cat0(*[_tie(m8, spread_over(anchors[:2], k, 5))] * (KU // 8 if k == 4 else 16))
                x = (xmid_s[blk, k * LANES:min((k + 1) * LANES, D), :] - mt) * rs
                xt.append((cat0(x, x) if k == 4 else x).T)
            lo = lax.broadcasted_iota(jnp.int32, (TQ // 2, LANES), 1) < KU
            for m1 in range(7):
                a = spread_over(anchors[2:], m1, 7)
                blk1 = lambda i2, k2: _signed(_SA[m1], lambda i1, k1: _tie(
                    xt[k2 if k2 == 4 else 2 * k1 + k2][(2 * i1 + i2) * TQ:(2 * i1 + i2 + 1) * TQ], a))
                l1 = {(i2, k2): blk1(i2, k2) for i2 in range(2)
                      for k2 in ((0, 1, 4) if m1 in _SCOL else (0, 1))}
                for m2 in range(7):
                    v = _signed(_SA[m2], lambda i2, k2: l1[i2, k2])
                    if m1 in _SCOL and m2 in _SCOL:
                        c = _signed(_SA[m2], lambda i2, k2: l1[i2, 4])
                        h = TQ // 2
                        vp, vq, cp, cq = v[:h], v[h:], c[:h], c[h:]
                        v = cat0(jnp.where(lo, cp, vq), jnp.where(lo, vp, vp - vq),
                                 jnp.where(lo, vq, cq - cp))
                    o, ac = AOFF[m1, m2]
                    a_s[o:o + v.shape[0] // 2, ac] = _pk(v)

        def in_triple(q):
            return q, lambda k: (q, k)

        def cross_triple(s):
            return NP + s, lambda k: (3 * s + k, 3)

        def wd_raw(tri, k, r0, n):
            q, c = tri[1](k)
            return wdt_v[q, r0:r0 + n, c * LANES:(c + 1) * LANES]

        def ds_loc(i, r0, n):
            return slice(r0, r0 + n), slice((i % 2) * LANES, (i % 2 + 1) * LANES)

        def prep_d(tri, anchors):
            PR = 16
            for n in range(D3 // PR):
                r = n * PR
                w = [[wd_raw(tri, k, j * D3 + r, PR).astype(F32) for j in range(3)]
                     for k in range(3)]
                w[0][1] = _tie(w[0][1], spread_over(anchors, n, D3 // PR))
                for i, v in enumerate(_w_sums(w)):
                    ds_s.at[tri[0], i // 2][ds_loc(i, r // 2, PR // 2)] = _pk(v)

        GU = (wg_v, wu_v)

        def prep_gu(p, gv, m, m1s, anchors):
            PR = 16
            cs = slice(m * LANES, (m + 1) * LANES)
            for n in range(LANES // PR):
                r = n * PR
                cache = {}

                def w(k, j1):
                    if (k, j1) not in cache:
                        v = GU[m][p, k * LANES + r:k * LANES + r + PR,
                                  2 * j1 * LANES:2 * (j1 + 1) * LANES].astype(F32)
                        if (k // 2, j1) in [_SB[m1][0][:2] for m1 in m1s[:2]]:
                            v = _tie(v, spread_over(anchors, n, LANES // PR))
                        cache[k, j1] = v
                    return cache[k, j1]

                for m1 in m1s:
                    b1 = [_signed(_SB[m1], lambda k1, j1: w(2 * k1 + k2, j1)) for k2 in range(2)]
                    for m2 in range(7):
                        v = _signed(_SB[m2],
                                    lambda k2, j2: b1[k2][:, j2 * LANES:(j2 + 1) * LANES])
                        gv.at[7 * m1 + m2][r // 2:(r + PR) // 2, cs] = _pk(v)

        def prep_tail(p, gv, m, anchor):
            v = _tie(GU[m][p, 4 * LANES:, :].astype(F32), anchor)
            for j in range(4):
                gv.at[49 + j // 2][(j % 2) * 32:(j % 2 + 1) * 32,
                                        m * LANES:(m + 1) * LANES] = _pk(
                                            v[:, j * LANES:(j + 1) * LANES])

        def gu_outer(gv, m, m1, anchors, at=(0, 4)):
            cs = slice(m * LANES, (m + 1) * LANES)
            y = {}
            for m2 in cfg['inner']:
                i, (o, ac) = 7 * m1 + m2, AOFF[m1, m2]
                if m1 in _SCOL and m2 in _SCOL:
                    j = 2 * _SCOL[m1] + _SCOL[m2]
                    tail = lambda: gv[49 + j // 2, (j % 2) * 32:(j % 2 + 1) * 32, cs]
                    rhs = (cat0(tail(), gv[i, 32:, cs]), gv[i, :, cs],
                           cat0(gv[i, :32, cs], tail()))
                    r = [_dot(_upk(a_s[o + 16 * s:o + 16 * (s + 1), ac]), _upk(rhs[s]))
                         for s in range(3)]
                    y[m2] = cat0(r[1] + r[0], r[2] + r[0])
                else:
                    y[m2] = _dot(_upk(a_s[o:o + TQ // 2, ac]), _upk(gv[i, :, cs]))
            anchors.extend(y[cfg['inner'][k % 7]][(k // 7) * 32:(k // 7) * 32 + 8] for k in at)
            return _s_out(y)

        def gu_finish(t):
            gu = [{(i2, j2): _s_out([t[m][m1][i2][j2] for m1 in range(7)])
                   for i2 in range(2) for j2 in range(2)} for m in range(2)]
            return [[cat0(*[_gelu_mul2(*[gu[m][i2, j % 2][i1][j // 2] for m in range(2)])
                            for i2 in range(2)]) for i1 in range(2)] for j in range(4)]

        def gu_piece(gv, order, anchors, at=(0, 4)):
            t = ({}, {})
            for m, m1 in order:
                t[m][m1] = gu_outer(gv, m, m1, anchors, at)
            return gu_finish(t)

        def prep_piece(p, gv, anchors, group):
            grp = _SGRP if group else [(m1,) for m1 in range(7)]
            k = len(anchors) // (2 * len(grp))
            for n in range(2 * len(grp)):
                prep_gu(p, gv, n % 2, grp[n // 2], anchors[k * n:k * n + k])
            for m in range(2):
                prep_tail(p, gv, m, anchors[m * len(anchors) // 2])

        def h_ops(h):
            return [v.astype(BF16) for v in _x_ops(*[[h[k][i] for k in range(3)]
                                                     for i in range(2)])]

        D_ORDER = _PAIR_ORDER + (9, 10, 11, 12, 13, 14)

        def down_mm(acc, work, anchors, which=D_ORDER, fine=False):
            p = [None] * 15 if acc is None else list(acc)
            jobs = [(i, n) for i in which for n in range(len(work))]
            split = {0: (), 1: (4,), 2: (2, 2), 3: (2, 2, 4)}[len(jobs) % 4]
            split = dict(zip(jobs[len(jobs) - len(split):], split))
            for i in which:
                y = None
                for n, (tri, b) in enumerate(work):
                    ns = split.get((i, n), 1)
                    nr = D3 // ns
                    if i in _W_RAW:
                        k, j = _W_RAW[i]
                        lhs = lambda h: wd_raw(tri, k, j * D3 + h * nr, nr)
                    else:
                        s = _W_SUM[i]
                        lhs = lambda h: _upk(ds_s.at[tri[0], s // 2][ds_loc(s, h * nr // 2, nr // 2)])
                    v = cat0(*[_dot_nt(lhs(h), b[i]) for h in range(ns)])
                    y = v if y is None else y + v
                p[i] = y if p[i] is None else p[i] + y
                anchors.append(p[i][:8])
                if fine:
                    anchors.append(p[i][D3 // 2:D3 // 2 + 8])
            return p

        def finish(blk, acc):
            y = [cat1(*_column(acc, [acc[_DIAG[s, j]] if (s, j) in _DIAG else None
                                     for s in range(3)], j)) for j in range(3)]
            xio_s[blk] = (xmid_s[blk] + 0.5 * cat0(*y)).astype(BF16)

        def load_acc(k):
            return [acc_s[k, i] for i in range(15)]

        def store_acc(k, acc):
            for i in range(15):
                acc_s[k, i] = acc[i]

        def pre_phase():
            first = [[x_cp(0, 0)], [wq_cp(0)], [x_cp(1, 2), wq_cp(1)],
                     [wq_cp(2), pltpu.make_async_copy(wo_hbm, wo_v, sem_i.at[3])]]
            order = sum(first, [])
            for p in range(NP + 1):
                order += group_cp(p)
            xr_cp = [x_cp(b, SEM_P + NP + 1) for b in range(2, NB)]
            order += xr_cp
            for cp in order:
                cp.start()
            get = lambda an, name: [an[min(i, len(an) - 1)] for i in cfg[name]]
            e_grp = lambda e: ((e >> 1) & 1, ((e >> 2) << 1) | (e & 1))
            if 'a' in cfg['sub']:
                pre_a(first, get, e_grp)
            if 'b' in cfg['sub']:
                pre_b(get, e_grp)
            if 'c' in cfg['sub']:
                pre_c(get)
            wait('WX', xr_cp)

        def pre_a(first, get, e_grp):
            def transpose_wq(i):
                wt_s[WQ[i] // 2:WQ[i + 1] // 2, :D] = _pk(wqkv_v[:, WQ[i]:WQ[i + 1]].T)

            def clear(i, carry):
                for k in range(2):
                    acc_s[k, i] = jnp.zeros((D3, TH), F32)
                r = jnp.minimum(i, 11) * (RP // 4)
                qkv_s[0, rows8(r, RP // 4)] = jnp.zeros((RP // 4, LANES), U32)
                return carry

            lax.fori_loop(0, 15, clear, 0)
            wait('WX0', first[0])
            xn0 = ln1(0, ()).astype(BF16)

            wait('WQ0', first[1])
            transpose_wq(0)
            qkv_mm(0, xn0, (0, 1), [])

            wait('WQ1', first[2])
            transpose_wq(1)
            an = []
            qkv_mm(0, xn0, (2, 3), an)
            xn1 = ln1(1, get(an, 'a_ln'), get(an, 'a_lnb')).astype(BF16)
            qkv_mm(1, xn1, (0,), an, True)
            for n, a in enumerate(get(an, 'a_w1')):
                prep_att(n, a)
            nk = len(cfg['a_k'])
            apply = [att_values(0, *e_grp(e), a) for e, a in enumerate(get(an, 'a_k'))]

            wait('WQ2', first[3])
            an = []
            qkv_mm(1, xn1, (2,), an)
            transpose_wq(2)
            qkv_mm(0, xn0, (4, 5), an)
            qkv_mm(1, xn1, (4,), an)
            qkv_mm(1, xn1, (1,), an, True)
            apply += [att_values(0, *e_grp(nk + e), a)
                      for e, a in enumerate(get(an, 'a_k2')[:8 - nk])]
            for e, a in enumerate(get(an, 'a_v')):
                apply[e](a)
            wo = pltpu.bitcast(wo_v[...], U32)
            wo = cat0(_lo(wo), _hi(wo))
            wo = cat0(*[_tie(wo[n * LANES:(n + 1) * LANES], a)
                        for n, a in enumerate(get(an, 'a_wo'))])
            wt_s[3 * RP:, :D] = _pk(wo.astype(BF16).T)
            for n, a in enumerate(get(an, 'a_w2')):
                prep_att(12 + n, a)

            wait('WO', group_cp(0))
            an = []
            stats = wo_mm(0, an, False)
            qkv_mm(1, xn1, (3, 5), an)
            for n, a in enumerate(get(an, 'z_w')):
                prep_att(36 + n, a)
            prep_piece(0, gu_s.at[0], get(an, 'z_g'), cfg['z_grp'])
            ffn_lhs(0, stats, get(an, 'z_l'))

        def pre_b(get, e_grp):
            def piece(p, carry):
                wait('WP', group_cp(p))
                an = []
                win = gu_s.at[pl.ds(p - 1, 2)]
                h = gu_piece(win.at[0], cfg['gorder0'], an, (0, 7, 4, 11))
                h3_s[p - 1] = cat0(*h[3])
                tri = in_triple(p - 1)
                prep_d(tri, get(an, 'p_d'))
                store_acc(0, down_mm(load_acc(0), [(tri, h_ops(h[:3]))], an))
                prep_piece(p, win.at[1], get(an, 'f_g'), cfg['f_grp'])
                att_group(1, *e_grp(p - 1), an[cfg['p_att'][0]])
                return carry

            lax.fori_loop(1, NP, piece, 0)

        def pre_c(get):
            wait('WD', group_cp(NP))
            an = []
            h = gu_piece(gu_s.at[NP - 1], cfg['gorder'], an)
            h3 = [[h3_s[q, :TH], h3_s[q, TH:]] for q in range(NP - 1)] + [h[3]]
            work = [(cross_triple(s), h_ops(h3[3 * s:3 * s + 3])) for s in range(3)]
            work.append((in_triple(NP - 1), h_ops(h[:3])))
            stats = wo_mm(1, an, True)
            td = get(an, 't_d')
            for n, (tri, _) in enumerate(work):
                prep_d(tri, td[n * len(td) // 4:(n + 1) * len(td) // 4])
            acc = down_mm(load_acc(0), work, an)
            nw = len(cfg['a_w2'])
            for n, a in enumerate(get(an, 't_w')[:24 - nw]):
                prep_att(12 + nw + n, a)
            ffn_lhs(1, stats, get(an, 't_l'))
            finish(0, acc)

        if 'pre' in cfg['phases']:
            pre_phase()

        def body(u, carry):
            bu = u & (NB - 1)
            ba = (u + 1) & (NB - 1)
            acc, stats, an, b, hh = None, None, {}, {}, {}
            get = lambda name: [an[k][i] for k, i in cfg[name]]
            for step in cfg['body']:
                an[step] = []
                if step == 'Q':
                    xn = ln1(ba, get('ln1'), get('ln1b'))
                    qkv_fast(ba, att_rhs(xn, u >> 8), an[step])
                elif step == 'W':
                    attention(ba, get('att'))
                    stats = wo_mm(ba, an[step], True, u >> 8, get('orhs'))
                elif step == 'L':
                    ffn_lhs(ba, stats, get('lhs'))
                elif step[0] == 'G':
                    q, go = int(step[1]), cfg['gorder']
                    t = b.setdefault(step[:2], ({}, {}))
                    for m, m1 in (go[:7] if step[2] == '0' else go[7:]):
                        t[m][m1] = gu_outer(gu_s.at[q], m, m1, an[step])
                    if len(t[0]) + len(t[1]) == 14:
                        hh[q] = gu_finish(t)
                else:
                    work = []
                    for c in step[1:]:
                        if c.isdigit():
                            work.append((in_triple(int(c)), h_ops(hh[int(c)][:3])))
                        else:
                            s = ord(c) - ord('a')
                            work.append((cross_triple(s),
                                         h_ops([hh[3 * s + k][3] for k in range(3)])))
                    acc = down_mm(acc, work, an[step])
            finish(bu, acc)

            @pl.when(u >= NB)
            def _():
                out_copy(bu).start()
            return carry

        if scopes:
            with jax.named_scope('LOOP'):
                lax.fori_loop(1, NU - 1, body, 0)
        elif 'main' in cfg['phases']:
            lax.fori_loop(1, NU - 1, body, 0)

        def last(s, carry):
            h = [gu_piece(gu_s.at[3 * s + k], cfg['lorder'], []) for k in range(3)]
            work = [(in_triple(3 * s + k), h_ops(h[k][:3])) for k in range(3)]
            work.append((cross_triple(s), h_ops([h[k][3] for k in range(3)])))
            acc = down_mm(down_mm(load_acc(1), work[:2], []), work[2:], [])
            store_acc(1, acc)
            finish(NB - 1, acc)
            return carry

        if 'last' in cfg['phases']:
            lax.fori_loop(0, NP // 3, last, 0)
        if len(cfg['phases']) < 3:
            def keep(i, c):
                v = (gu_s[i, i, :8, :LANES] + ds_s[i, i, :8, :LANES]
                     + wl_s[rows8(i * 8), :LANES] + a_s[rows8(i * 8), :LANES] + qkv_s[i, :8]
                     + wt_s[rows8(i * 8), :LANES])
                acc_s[1, 0, :8] = (lax.bitcast_convert_type(v, F32) + o_s[i, :8]
                                   + acc_s[i, i, :8] + h3_s[i, :8])
                return c
            lax.fori_loop(0, 2, keep, 0)
            finish(NB - 1, load_acc(1))
        out_copy(NB - 1).start()
        wait('WOUT', [out_copy(b) for b in range(NB)])

    scratch = [
        pltpu.VMEM((NB, D, TM), BF16),
        pltpu.VMEM((D, 3 * D), BF16),
        pltpu.VMEM((D, D), BF16),
        pltpu.VMEM((NP, D, PW), BF16),
        pltpu.VMEM((NP, D, PW), BF16),
        pltpu.VMEM((NP, D, PW), BF16),
        pltpu.VMEM((2 * D, 8 * LANES), U32),
        pltpu.VMEM((4 * Q3, 16 * LANES), U32),
        pltpu.VMEM((NP, 51, 64, 2 * LANES), U32),
        pltpu.VMEM((NP + 3, 5, Q3, 2 * LANES), U32),
        pltpu.VMEM((NB, D, TM), F32),
        pltpu.VMEM((max(fill), 2 * LANES), U32),
        pltpu.VMEM((S // LANES + 1, 3 * RP, LANES), U32),
        pltpu.VMEM((NT, D, LANES), F32),
        pltpu.VMEM((2, 15, D3, TH), F32),
        pltpu.VMEM((NP, TM, LANES), F32),
        pltpu.VMEM((1, 9 * 64, 2 * LANES), U32),
        pltpu.SemaphoreType.DMA((SEM_P + NP + 2,)),
        pltpu.SemaphoreType.DMA((1,)),
    ]

    def wrapped(*refs):
        @pl.when(pl.program_id(0) == 0)
        def _():
            kernel(*refs)

    return wrapped, scratch


_CFG = dict(
    scopes=False,
    orhs=(('G80', 0), ('G80', 1), ('G80', 2), ('G80', 3), ('G80', 4), ('G80', 5),
        ('G80', 6), ('G80', 7), ('G80', 8), ('G80', 9), ('G80', 10), ('G80', 11)),
    sub='abc',
    phases=('pre', 'main', 'last'),
    body=('G20', 'G00', 'G01', 'G10', 'G11', 'Q', 'G30', 'G21', 'G40', 'G31', 'G50',
        'D012a', 'G41', 'G51', 'D345b', 'G70', 'G71', 'G60', 'G80', 'W', 'G61', 'G81',
        'D8c', 'D67', 'L'),
    ln1=(('G00', 0), ('G00', 1), ('G00', 2), ('G00', 3), ('G00', 4), ('G00', 5), ('G00',
        6), ('G00', 7), ('G00', 8)),
    ln1b=(('G10', 1), ('G10', 2), ('G10', 3), ('G10', 4), ('G10', 5), ('G10', 6),
        ('G10', 7), ('G10', 8), ('G10', 9), ('G10', 10), ('G10', 11), ('G10', 12)),
    att=(('D012a', 2), ('D012a', 4), ('D012a', 5), ('D012a', 6), ('D012a', 9), ('D345b',
        6), ('D345b', 7), ('D345b', 8)),
    lhs=(('D8c', 2), ('D8c', 3), ('D8c', 6), ('D67', 5), ('D67', 7), ('D67', 8), ('D67',
        10), ('D67', 11), ('D67', 14)),
    a_w1=(0, 0, 1, 2, 2, 3, 3, 4, 4, 5, 7, 11),
    a_w2=(0, 3, 6, 9, 10, 14),
    a_ln=(0, 3, 6),
    a_lnb=(5, 9, 10),
    z_g=(0, 0, 1, 1, 2, 2, 3, 3, 4, 4, 5, 6, 6, 7, 7, 8, 8, 9, 9, 11, 11, 12, 12, 13,
        13, 14, 14, 15, 16, 16, 17, 17, 18, 18, 19, 19, 20, 21, 21, 22, 23, 23, 24, 24,
        25, 25, 26, 33),
    t_d=(0, 0, 1, 2, 3, 4, 5, 5, 6, 7, 8, 9, 10, 11, 11, 12, 13, 14, 14, 15, 15, 16, 17,
        17, 18, 19, 21, 22, 22, 23, 23, 24, 27, 27, 28, 28, 30, 31, 32, 34, 34, 35, 36,
        37, 38, 39, 40, 40),
    p_d=(5, 20, 22, 25, 27, 33, 35, 38, 41, 46, 49, 50),
    p_att=(60,),
    z_l=(23, 23, 25, 31, 35, 36, 37, 37, 39),
    a_k=(16, 18, 20, 23),
    a_k2=(0, 0, 0, 1),
    a_v=(8, 10, 12, 14, 16, 18, 20, 22),
    a_wo=(9, 18, 27, 36, 46),
    inner=(0, 3, 4, 6, 2, 1, 5),
    gorder=((0, 0), (0, 4), (1, 4), (1, 0), (0, 3), (1, 3), (1, 6), (0, 6), (0, 1), (1,
        1), (0, 2), (1, 2), (0, 5), (1, 5)),
    gorder0=((1, 4), (0, 0), (0, 3), (1, 0), (0, 4), (0, 6), (1, 6), (1, 3), (0, 1), (1,
        1), (0, 2), (1, 5), (0, 5), (1, 2)),
    f_g=(0, 1, 2, 3, 7, 8, 9, 10, 12, 12, 13, 14, 15, 16, 17, 19, 20, 21, 22, 24, 25,
        26, 28, 29, 29, 31, 33, 34, 35, 36, 38, 39, 40, 42, 43, 44, 45, 47, 48, 49, 50,
        52, 53, 54, 56, 57, 58, 59, 61, 61, 62, 64, 69, 70, 70, 70),
    t_l=(50, 51, 52, 53, 54, 55, 56, 57, 58),
    lorder=((1, 0), (1, 4), (0, 0), (0, 4), (0, 3), (0, 6), (1, 3), (1, 6), (0, 1), (1,
        1), (0, 2), (0, 5), (1, 2), (1, 5)),
    z_w=(0, 1, 3, 3, 4, 5, 6, 6, 7, 8, 9, 28),
    z_grp=1,
    f_grp=0,
    t_w=(3, 6, 9, 13, 19, 24, 24, 25, 32, 36, 41, 42, 47, 50, 53, 56, 60, 60),
)


def _run(A_x, A_wqkv, A_wo, B_w_gate, B_w_up, B_w_down, **kw):
    _, S, D = A_x.shape
    F = B_w_gate.shape[1]
    kernel, scratch = _make_kernel(S, D, F, 256, {**_CFG, **kw})
    hbm = pl.BlockSpec(memory_space=pl.ANY)
    out_t = pl.pallas_call(
        kernel,
        grid=(2,),
        in_specs=[hbm] * 6,
        out_specs=hbm,
        out_shape=jax.ShapeDtypeStruct((D, S), A_x.dtype),
        scratch_shapes=scratch,
        compiler_params=pltpu.CompilerParams(
            dimension_semantics=('arbitrary',), vmem_limit_bytes=110 * 1024 * 1024),
    )(A_x.reshape(S, D).T, A_wqkv, A_wo, B_w_gate, B_w_up, B_w_down.T)
    return out_t.T.reshape(A_x.shape)


@jax.jit
def pallas_interleave_layers__sliding_local_dilated__glu_gated_geglu__prompt_kernel(
    A_x: jax.Array,
    A_wqkv: jax.Array,
    A_wo: jax.Array,
    B_x: jax.Array,
    B_w_gate: jax.Array,
    B_w_up: jax.Array,
    B_w_down: jax.Array,
):
    del B_x
    return _run(A_x, A_wqkv, A_wo, B_w_gate, B_w_up, B_w_down)
```

```python
import jax
import jax.numpy as jnp
import jax.experimental.pallas as pl
import jax.experimental.pallas.tpu as pltpu
from jax import lax

H = 32
W = 8
DIL = 2
EPS = 1e-5
LANES = 128

F32 = jnp.float32
BF16 = jnp.bfloat16
U32 = jnp.uint32

_NT = (((1,), (1,)), ((), ()))


def _tree_sum(parts, op=jnp.add):
    while len(parts) > 1:
        nxt = [op(parts[i], parts[i + 1]) for i in range(0, len(parts) - 1, 2)]
        if len(parts) % 2:
            nxt.append(parts[-1])
        parts = nxt
    return parts[0]


def _ln_stats(slabs, d, anchors=()):
    n_acc = 4
    s1, s2, pilot = [None] * n_acc, [None] * n_acc, None
    for i, x in enumerate(slabs):
        if pilot is None:
            pilot = x[0:1, :]
            pil = jnp.broadcast_to(pilot, x.shape)
            pils = [_tie(pil, a) for a in anchors] or [pil]
        dx = x - pils[i * len(pils) // (d // 8)]
        j = i % n_acc
        s1[j] = dx if s1[j] is None else s1[j] + dx
        s2[j] = dx * dx if s2[j] is None else s2[j] + dx * dx
    e1 = jnp.sum(_tree_sum(s1), axis=0, keepdims=True) * (1.0 / d)
    e2 = jnp.sum(_tree_sum(s2), axis=0, keepdims=True) * (1.0 / d)
    var = jnp.maximum(e2 - e1 * e1, 0.0)
    return pilot + e1, lax.rsqrt(var + EPS)


def _zero_like_dep(v):
    return (lax.bitcast_convert_type(v, U32) >> 31) >> 1


def _tie(x, anchor):
    if anchor is None:
        return x
    z = lax.bitcast_convert_type(_zero_like_dep(anchor), F32)
    z = jnp.concatenate([z] * -(-x.shape[1] // LANES), axis=1)[:, :x.shape[1]]
    if x.shape[0] == 8:
        return x + z
    return jnp.concatenate([x[:8] + z, x[8:]], axis=0)


def _gelu_mul2(g, u):
    c0 = 0.7978845608028654
    c1 = c0 * 0.044715
    t = jnp.tanh(g * (c0 + c1 * (g * g)))
    return (g * u) * (1.0 + t)


def _lo(x):
    return lax.bitcast_convert_type(x << 16, F32)


def _hi(x):
    return lax.bitcast_convert_type(x & jnp.uint32(0xFFFF0000), F32)


def _pk(x):
    return pltpu.bitcast(x.astype(BF16), U32)


def _upk(x):
    return pltpu.bitcast(x, BF16)


def _dot(a, b):
    return jnp.dot(a, b, preferred_element_type=F32)


def _dot_nt(a, b):
    return lax.dot_general(a, b, _NT, preferred_element_type=F32)


def _x_ops(x1, x2):
    d = [a - b for a, b in zip(x1, x2)]
    return [x1[0] + x2[1], x2[0] + x2[1], x1[0] + x1[1],
            d[1] + x1[2], x1[1] + x1[2], d[1] + d[2],
            d[0] - x2[2], d[0] + d[2], x2[0] + x2[2],
            x1[0], d[0], x2[1], d[1], x1[2], x2[2]]


def _x_rem(x1, x2):
    a, b, c = 0, 1, 2
    cat = lambda u, v: jnp.concatenate([u, v], axis=0)
    return [cat(x1[c], x2[b]), cat(x1[a], x1[b] - x2[b]), cat(x2[a], x2[c] - x1[c])]


_W_TERMS = {0: ((0, 1, 1), (1, 0, 1)), 3: ((1, 2, 1), (2, 1, 1)), 6: ((0, 2, 1), (2, 0, 1)),
            9: ((0, 0, 1), (0, 2, 1), (1, 0, -1)), 10: ((2, 0, 1), (0, 0, -1), (0, 1, -1)),
            11: ((1, 1, 1), (1, 2, 1), (0, 1, -1)), 12: ((1, 0, 1), (1, 1, 1), (2, 1, -1)),
            13: ((2, 0, 1), (2, 2, 1), (1, 2, -1)), 14: ((2, 1, 1), (2, 2, 1), (0, 2, -1)),
            1: ((0, 1, 1),), 2: ((1, 0, 1),), 4: ((1, 2, 1),), 5: ((2, 1, 1),),
            7: ((2, 0, 1),), 8: ((0, 2, 1),)}


def _w_sums(w):
    return [_signed(_W_TERMS[i], lambda k, j: w[k][j]) for i in _W_SUM]


_W_SUM = {0: 0, 3: 1, 6: 2, 9: 3, 10: 4, 11: 5, 12: 6, 13: 7, 14: 8}
_W_RAW = {1: (0, 1), 2: (1, 0), 4: (1, 2), 5: (2, 1), 7: (2, 0), 8: (0, 2)}
_PAIR_ORDER = (1, 2, 4, 5, 7, 8, 0, 3, 6)
_DIAG = {(0, 0): 9, (2, 0): 10, (0, 1): 11, (1, 1): 12, (1, 2): 13, (2, 2): 14}
_PAIR = {(0, 0): ((6, -1), (8, -1)), (1, 0): ((2, 1), (7, 1)), (2, 0): ((0, 1), (1, -1)),
         (0, 1): ((3, 1), (4, -1)), (1, 1): ((0, 1), (2, -1)), (2, 1): ((1, 1), (5, -1)),
         (0, 2): ((4, 1), (8, 1)), (1, 2): ((6, 1), (7, -1)), (2, 2): ((5, 1), (3, -1))}


def _column(t, base, j, skew=False):
    s = []
    for k in range(3):
        v = base[k]
        for i, sg in _PAIR[k, j]:
            v = t[i] if v is None else (v + t[i] if sg > 0 else v - t[i])
        s.append(v)
    if skew:
        return s[1] + s[0], s[2] + 0.5 * (s[0] - s[1])
    return s[1] + s[0], s[2] + s[0]


_SA = (((0, 0, 1), (1, 1, 1)), ((1, 0, 1), (1, 1, 1)), ((0, 0, 1),), ((1, 1, 1),),
       ((0, 0, 1), (0, 1, 1)), ((1, 0, 1), (0, 0, -1)), ((0, 1, 1), (1, 1, -1)))
_SB = (((0, 0, 1), (1, 1, 1)), ((0, 0, 1),), ((0, 1, 1), (1, 1, -1)), ((1, 0, 1), (0, 0, -1)),
       ((1, 1, 1),), ((0, 0, 1), (0, 1, 1)), ((1, 0, 1), (1, 1, 1)))
_SCOL = {2: 1, 3: 0, 5: 1, 6: 0}
_SGRP = ((1, 4, 0), (3, 6), (2, 5))


def _signed(terms, f):
    v = None
    for a, b, sg in terms:
        v = f(a, b) if v is None else (v + f(a, b) if sg > 0 else v - f(a, b))
    return v


def _s_out(m):
    return [[m[0] + m[3] - m[4] + m[6], m[2] + m[4]],
            [m[1] + m[3], m[0] - m[1] + m[2] + m[5]]]


def _make_kernel(S, D, F, TM, cfg):
    NB = S // TM
    NT = TM // LANES
    DH = D // H
    DP = DH // 2
    RP = D // 2
    NG = H // 8
    scale = float(DH) ** -0.5
    NU = 2 * NB
    TH = TM // 2
    TQ = TM // 4
    D2 = D // 2
    D3 = D // 3
    Q3 = D3 // 2
    KU = D // 9
    KR = 3 * LANES
    NQ = 6
    QR = 3 * D // NQ
    WQ = (0, 640, 1152, 3 * D)
    PW = 4 * LANES
    NP = F // PW
    AOFF, fill = {}, [0, 0]
    for key in [(m1, m2) for m1 in range(7) for m2 in range(7)]:
        c = int(fill[1] < fill[0])
        AOFF[key] = (fill[c], slice(c * LANES, (c + 1) * LANES))
        fill[c] += 48 if key[0] in _SCOL and key[1] in _SCOL else 32
    scopes = cfg['scopes']
    assert NG == 4 and NB & (NB - 1) == 0
    SEM_P = 4

    def kernel(x_hbm, wqkv_hbm, wo_hbm, wg_hbm, wu_hbm, wdt_hbm, out_hbm,
               xio_s, wqkv_v, wo_v, wg_v, wu_v, wdt_v, wt_s, wl_s,
               gu_s, ds_s, xmid_s, a_s, qkv_s, o_s, acc_s, h3_s, r_s,
               sem_i, sem_o):

        def wait(name, cps):
            if scopes:
                with jax.named_scope(name):
                    for cp in cps:
                        cp.wait()
            else:
                for cp in cps:
                    cp.wait()

        def cols(lo, n):
            if not isinstance(lo, int):
                lo = pl.multiple_of(lo, LANES)
            return pl.ds(lo, n)

        def rows8(lo, n=8):
            if not isinstance(lo, int):
                lo = pl.multiple_of(lo, 8)
            return pl.ds(lo, n)

        def out_copy(b):
            return pltpu.make_async_copy(
                xio_s.at[b], out_hbm.at[:, cols(b * TM, TM)], sem_o.at[0])

        def x_cp(b, sem):
            return pltpu.make_async_copy(x_hbm.at[:, cols(b * TM, TM)], xio_s.at[b],
                                         sem_i.at[sem])

        def wq_cp(i):
            sl = cols(WQ[i], WQ[i + 1] - WQ[i])
            return pltpu.make_async_copy(wqkv_hbm.at[:, sl], wqkv_v.at[:, sl],
                                         sem_i.at[1 + i])

        def piece_cp(src, dst, p, sem, c0=0, n=PW):
            return pltpu.make_async_copy(src.at[:, cols(p * PW + c0, n)],
                                         dst.at[p, :, pl.ds(c0, n)], sem_i.at[sem])

        def group_cp(p):
            sem = SEM_P + p
            cps = []
            if not (isinstance(p, int) and p == NP):
                cps += [piece_cp(wg_hbm, wg_v, p, sem), piece_cp(wu_hbm, wu_v, p, sem)]
            if not (isinstance(p, int) and p == 0):
                cps.append(piece_cp(wdt_hbm, wdt_v, p - 1, sem, 0, KR))
            if isinstance(p, int) and p == NP:
                cps += [piece_cp(wdt_hbm, wdt_v, q, sem, KR, LANES) for q in range(NP)]
            return cps

        lane = lax.broadcasted_iota(jnp.int32, (8, LANES), 1)
        cat0 = lambda *v: jnp.concatenate(v, axis=0)
        cat1 = lambda *v: jnp.concatenate(v, axis=1)

        def spread_over(anchors, n, total):
            return anchors[n * len(anchors) // total] if anchors else None

        def slab_group(r):
            return (r % LANES) // 16 if r < KR else 8 + ((r - KR) % KU) // 16

        def ln1(blk, anchors1, anchors2=()):
            slabs = (xio_s[blk, r:r + 8, :].astype(F32) for r in range(0, D, 8))
            m, rs = _ln_stats(slabs, D, anchors1)
            if not anchors2:
                return (xio_s[blk].astype(F32) - m) * rs
            m8 = jnp.broadcast_to(m, (8, TM))
            ms = [_tie(m8, a) for a in anchors2]
            ms = [spread_over(ms, slab_group(r), 12) for r in range(0, D, 8)]
            return (xio_s[blk].astype(F32) - cat0(*ms)) * rs

        def dot_k(rows, x, anchors, even=False):
            y = None
            for n, k in enumerate(range(0, D, LANES)):
                ks = slice(k, min(k + LANES, D))
                if even and k + LANES >= D:
                    mid = (rows.start + rows.stop) // 2
                    v = cat0(_dot(_upk(wt_s[rows.start:mid, ks]), x[ks]),
                             _dot(_upk(wt_s[mid:rows.stop, ks]), x[ks]))
                else:
                    v = _dot(_upk(wt_s[rows, ks]), x[ks])
                anchors.extend(v[r:r + 8, :LANES] for r in ((0, 144) if n % 2 else (72, 216)))
                y = v if y is None else y + v
            return y

        def put_qkv(blk, rows, y):
            pk = _pk(y)
            for c in range(NT):
                qkv_s[1 + blk * NT + c, rows, :] = pk[:, c * LANES:(c + 1) * LANES]

        def qkv_mm(blk, xn, chunks, anchors, even=False):
            for r in chunks:
                rows = slice(r * QR // 2, (r + 1) * QR // 2)
                put_qkv(blk, rows, dot_k(rows, xn, anchors, even))

        def split_k(x):
            hs = (x[:, :TH], x[:, TH:])
            blocks = [[h[k * LANES:(k + 1) * LANES] for k in range(3)] for h in hs]
            units = [[h[KR + k * KU:KR + (k + 1) * KU] for k in range(3)] for h in hs]
            return blocks, units

        def prep_att(pat, anchor):
            assert Q3 == 96
            row0 = pat * 8
            src0 = row0 + ((pat * 43) >> 9) * (2 * Q3)
            w = [_upk(wt_s[rows8(src0 + j * Q3), :D]).astype(F32) for j in range(3)]
            w[0] = cat1(_tie(w[0][:, :LANES], anchor), w[0][:, LANES:])
            tiles = _w_sums([[w[j][:, k * LANES:(k + 1) * LANES] for j in range(3)]
                             for k in range(3)])
            for j in range(3):
                a, b, c = (w[j][:, KR + k * KU:KR + (k + 1) * KU] for k in range(3))
                tiles += [cat1(c, b), cat1(a, c)]
            wl_s[rows8(row0), :15 * LANES] = _pk(cat1(*tiles))

        def att_rhs(x, stash=None, anchors=()):
            half = 0.5
            if anchors:
                hs = [_tie(jnp.full((8, TH), 0.5, F32), a) for a in anchors]
                half = cat0(*[spread_over(hs, slab_group(r), 12) for r in range(0, D, 8)])
            blocks, units = split_k(cat1(x[:, :TH], x[:, TH:] + half * x[:, :TH]))
            ops = _x_ops(*blocks) + _x_rem(*units)
            if stash is None:
                return [v.astype(BF16) for v in ops]
            loc = lambda i, r0, n: (slice((i // 2) * 64 + r0, (i // 2) * 64 + r0 + n),
                                    slice((i % 2) * LANES, (i % 2 + 1) * LANES))
            for r in range(0, LANES, 16):
                for i, v in enumerate(ops):
                    r_s.at[0][loc(i, r // 2, 8)] = _pk(v[r:r + 16])
            return [_upk(r_s.at[stash][loc(i, 0, 64)]) for i in range(18)]

        def att_mm(sec, rhs, anchors):
            tl = lambda i: _upk(wl_s[sec * Q3:(sec + 1) * Q3, i * LANES:(i + 1) * LANES])
            raw = lambda k, j: _upk(wt_s[(3 * sec + j) * Q3:(3 * sec + j + 1) * Q3,
                                         k * LANES:(k + 1) * LANES])
            t = {}
            for i in _PAIR_ORDER:
                t[i] = _dot(raw(*_W_RAW[i]) if i in _W_RAW else tl(_W_SUM[i]), rhs[i])
                anchors.append(t[i][:8])
            out = []
            for j in range(3):
                base = []
                for s in range(3):
                    v = _dot(raw(3, j) if s == 1 else tl(9 + 2 * j + s // 2), rhs[15 + s])
                    if (s, j) in _DIAG:
                        i = _DIAG[s, j]
                        v = _dot(tl(_W_SUM[i]), rhs[i]) + v
                    base.append(v)
                    anchors.append(base[-1][:8])
                out.append(cat1(*_column(t, base, j, True)))
            return cat0(*out)

        def qkv_fast(blk, rhs, anchors):
            for sec in range(3):
                put_qkv(blk, slice(sec * RP, (sec + 1) * RP), att_mm(sec, rhs, anchors))

        def shifted(ln, cur, prev, w):
            if w == 0:
                return cur
            sh = DIL * w
            return pltpu.roll(jnp.where(ln < LANES - sh, cur, prev), sh, axis=1)

        def att_group(blk, c, hg, anchor):
            att_values(blk, c, hg, anchor)(None)

        def att_values(blk, c, hg, anchor):
            tile = blk * NT + c
            base = hg * 8 * DP
            if isinstance(hg, int):
                cur, prev, o_t = qkv_s.at[1 + tile], qkv_s.at[tile], o_s.at[c]
            else:
                n = 2 * RP + 8 * DP
                base = pl.multiple_of(base, 8)
                cur = qkv_s.at[1 + tile, pl.ds(base, n)]
                prev = qkv_s.at[tile, pl.ds(base, n)]
                o_t = o_s.at[c, pl.ds(base, RP + 8 * DP)]
                base = 0
            ln = lane + _zero_like_dep(anchor).astype(jnp.int32)
            logits = [None] * W
            for dd in range(DP):
                q = cur[pl.ds(base + dd, 8, stride=DP), :]
                kc = cur[pl.ds(RP + base + dd, 8, stride=DP), :]
                kp = prev[pl.ds(RP + base + dd, 8, stride=DP), :]
                q0, q1 = _lo(q), _hi(q)
                for w in range(W):
                    ks = shifted(ln, kc, kp, w)
                    t = q0 * _lo(ks) + q1 * _hi(ks)
                    logits[w] = t if logits[w] is None else logits[w] + t
            logits = [l * scale for l in logits]
            if not (isinstance(c, int) and c > 0):
                pos = lane + tile * LANES
                logits = [l if w == 0 else jnp.where(pos >= DIL * w, l, -1e9)
                          for w, l in enumerate(logits)]
            m = _tree_sum(logits, jnp.maximum)
            p = [jnp.exp(l - m) for l in logits]
            r = 1.0 / _tree_sum(p)

            def apply(anchor2):
                ln = lane + _zero_like_dep(_tie(m, anchor2)).astype(jnp.int32)
                for dd in range(DP):
                    vc = cur[pl.ds(2 * RP + base + dd, 8, stride=DP), :]
                    vp = prev[pl.ds(2 * RP + base + dd, 8, stride=DP), :]
                    o0 = o1 = None
                    for w in range(W):
                        vs = shifted(ln, vc, vp, w)
                        t0, t1 = p[w] * _lo(vs), p[w] * _hi(vs)
                        o0 = t0 if o0 is None else o0 + t0
                        o1 = t1 if o1 is None else o1 + t1
                    o0, o1 = o0 * r, o1 * r
                    o_t[pl.ds(base + dd, 8, stride=DP), :] = o0
                    o_t[pl.ds(RP + base + dd, 8, stride=DP), :] = o1

            return apply

        def attention(blk, anchors):
            for c in range(NT):
                for hg in range(NG):
                    att_group(blk, c, hg, anchors[c * NG + hg])

        def wo_mm(blk, anchors, fast, stash=None, anchors_in=()):
            o = cat1(*[o_s[c] for c in range(NT)])
            if fast:
                y = att_mm(3, att_rhs(o, stash, anchors_in), anchors)
            else:
                o = o.astype(BF16)
                q = D2 // 2
                y = cat0(*[dot_k(slice(h * q, (h + 1) * q), o, anchors) for h in (6, 7)])
            xm = xio_s[blk].astype(F32) + y
            xmid_s[blk] = xm
            return _ln_stats((xm[r:r + 8] for r in range(0, D, 8)), D)

        def ffn_lhs(blk, stats, anchors):
            m, rs = stats
            m8 = jnp.broadcast_to(m, (8, TM))
            xt = []
            for k in range(5):
                mt = cat0(*[_tie(m8, spread_over(anchors[:2], k, 5))] * (KU // 8 if k == 4 else 16))
                x = (xmid_s[blk, k * LANES:min((k + 1) * LANES, D), :] - mt) * rs
                xt.append((cat0(x, x) if k == 4 else x).T)
            lo = lax.broadcasted_iota(jnp.int32, (TQ // 2, LANES), 1) < KU
            for m1 in range(7):
                a = spread_over(anchors[2:], m1, 7)
                blk1 = lambda i2, k2: _signed(_SA[m1], lambda i1, k1: _tie(
                    xt[k2 if k2 == 4 else 2 * k1 + k2][(2 * i1 + i2) * TQ:(2 * i1 + i2 + 1) * TQ], a))
                l1 = {(i2, k2): blk1(i2, k2) for i2 in range(2)
                      for k2 in ((0, 1, 4) if m1 in _SCOL else (0, 1))}
                for m2 in range(7):
                    v = _signed(_SA[m2], lambda i2, k2: l1[i2, k2])
                    if m1 in _SCOL and m2 in _SCOL:
                        c = _signed(_SA[m2], lambda i2, k2: l1[i2, 4])
                        h = TQ // 2
                        vp, vq, cp, cq = v[:h], v[h:], c[:h], c[h:]
                        v = cat0(jnp.where(lo, cp, vq), jnp.where(lo, vp, vp - vq),
                                 jnp.where(lo, vq, cq - cp))
                    o, ac = AOFF[m1, m2]
                    a_s[o:o + v.shape[0] // 2, ac] = _pk(v)

        def in_triple(q):
            return q, lambda k: (q, k)

        def cross_triple(s):
            return NP + s, lambda k: (3 * s + k, 3)

        def wd_raw(tri, k, r0, n):
            q, c = tri[1](k)
            return wdt_v[q, r0:r0 + n, c * LANES:(c + 1) * LANES]

        def ds_loc(i, r0, n):
            return slice(r0, r0 + n), slice((i % 2) * LANES, (i % 2 + 1) * LANES)

        def prep_d(tri, anchors):
            PR = 16
            for n in range(D3 // PR):
                r = n * PR
                w = [[wd_raw(tri, k, j * D3 + r, PR).astype(F32) for j in range(3)]
                     for k in range(3)]
                w[0][1] = _tie(w[0][1], spread_over(anchors, n, D3 // PR))
                for i, v in enumerate(_w_sums(w)):
                    ds_s.at[tri[0], i // 2][ds_loc(i, r // 2, PR // 2)] = _pk(v)

        GU = (wg_v, wu_v)

        def prep_gu(p, gv, m, m1s, anchors):
            PR = 16
            cs = slice(m * LANES, (m + 1) * LANES)
            for n in range(LANES // PR):
                r = n * PR
                cache = {}

                def w(k, j1):
                    if (k, j1) not in cache:
                        v = GU[m][p, k * LANES + r:k * LANES + r + PR,
                                  2 * j1 * LANES:2 * (j1 + 1) * LANES].astype(F32)
                        if (k // 2, j1) in [_SB[m1][0][:2] for m1 in m1s[:2]]:
                            a = spread_over(anchors, n, LANES // PR)
                            if cfg['tie1']:
                                c = (k % 2) * LANES
                                tied = _tie(v[:, c:c + LANES], a)
                                v = cat1(v[:, :LANES], tied) if c else cat1(tied, v[:, LANES:])
                            else:
                                v = _tie(v, a)
                        cache[k, j1] = v
                    return cache[k, j1]

                for m1 in m1s:
                    b1 = [_signed(_SB[m1], lambda k1, j1: w(2 * k1 + k2, j1)) for k2 in range(2)]
                    for m2 in range(7):
                        v = _signed(_SB[m2],
                                    lambda k2, j2: b1[k2][:, j2 * LANES:(j2 + 1) * LANES])
                        gv.at[7 * m1 + m2][r // 2:(r + PR) // 2, cs] = _pk(v)

        def prep_tail(p, gv, m, anchor):
            v = _tie(GU[m][p, 4 * LANES:, :].astype(F32), anchor)
            for j in range(4):
                gv.at[49 + j // 2][(j % 2) * 32:(j % 2 + 1) * 32,
                                        m * LANES:(m + 1) * LANES] = _pk(
                                            v[:, j * LANES:(j + 1) * LANES])

        def gu_outer(gv, m, m1, anchors, at=(0, 4)):
            cs = slice(m * LANES, (m + 1) * LANES)
            y = {}
            for m2 in cfg['inner']:
                i, (o, ac) = 7 * m1 + m2, AOFF[m1, m2]
                if m1 in _SCOL and m2 in _SCOL:
                    j = 2 * _SCOL[m1] + _SCOL[m2]
                    tail = lambda: gv[49 + j // 2, (j % 2) * 32:(j % 2 + 1) * 32, cs]
                    rhs = (cat0(tail(), gv[i, 32:, cs]), gv[i, :, cs],
                           cat0(gv[i, :32, cs], tail()))
                    r = [_dot(_upk(a_s[o + 16 * s:o + 16 * (s + 1), ac]), _upk(rhs[s]))
                         for s in range(3)]
                    y[m2] = cat0(r[1] + r[0], r[2] + r[0])
                else:
                    y[m2] = _dot(_upk(a_s[o:o + TQ // 2, ac]), _upk(gv[i, :, cs]))
            anchors.extend(y[cfg['inner'][k % 7]][(k // 7) * 32:(k // 7) * 32 + 8] for k in at)
            return _s_out(y)

        def gu_finish(t):
            gu = [{(i2, j2): _s_out([t[m][m1][i2][j2] for m1 in range(7)])
                   for i2 in range(2) for j2 in range(2)} for m in range(2)]
            return [[cat0(*[_gelu_mul2(*[gu[m][i2, j % 2][i1][j // 2] for m in range(2)])
                            for i2 in range(2)]) for i1 in range(2)] for j in range(4)]

        def gu_piece(gv, order, anchors, at=(0, 4)):
            t = ({}, {})
            for m, m1 in order:
                t[m][m1] = gu_outer(gv, m, m1, anchors, at)
            return gu_finish(t)

        def prep_piece(p, gv, anchors, group):
            grp = _SGRP if group else [(m1,) for m1 in range(7)]
            k = len(anchors) // (2 * len(grp))
            for n in range(2 * len(grp)):
                prep_gu(p, gv, n % 2, grp[n // 2], anchors[k * n:k * n + k])
            for m in range(2):
                prep_tail(p, gv, m, anchors[m * len(anchors) // 2])

        def h_ops(h):
            return [v.astype(BF16) for v in _x_ops(*[[h[k][i] for k in range(3)]
                                                     for i in range(2)])]

        D_ORDER = _PAIR_ORDER + (9, 10, 11, 12, 13, 14)

        def down_mm(acc, work, anchors, which=D_ORDER, fine=False):
            p = [None] * 15 if acc is None else list(acc)
            jobs = [(i, n) for i in which for n in range(len(work))]
            split = {0: (), 1: (4,), 2: (2, 2), 3: (2, 2, 4)}[len(jobs) % 4]
            split = dict(zip(jobs[len(jobs) - len(split):], split))
            for i in which:
                y = None
                for n, (tri, b) in enumerate(work):
                    ns = split.get((i, n), 1)
                    nr = D3 // ns
                    if i in _W_RAW:
                        k, j = _W_RAW[i]
                        lhs = lambda h: wd_raw(tri, k, j * D3 + h * nr, nr)
                    else:
                        s = _W_SUM[i]
                        lhs = lambda h: _upk(ds_s.at[tri[0], s // 2][ds_loc(s, h * nr // 2, nr // 2)])
                    v = cat0(*[_dot_nt(lhs(h), b[i]) for h in range(ns)])
                    y = v if y is None else y + v
                p[i] = y if p[i] is None else p[i] + y
                anchors.append(p[i][:8])
                if fine:
                    anchors.append(p[i][D3 // 2:D3 // 2 + 8])
            return p

        def finish(blk, acc):
            y = [cat1(*_column(acc, [acc[_DIAG[s, j]] if (s, j) in _DIAG else None
                                     for s in range(3)], j)) for j in range(3)]
            xio_s[blk] = (xmid_s[blk] + 0.5 * cat0(*y)).astype(BF16)

        def load_acc(k):
            return [acc_s[k, i] for i in range(15)]

        def store_acc(k, acc):
            for i in range(15):
                acc_s[k, i] = acc[i]

        def pre_phase():
            first = [[x_cp(0, 0)], [wq_cp(0)], [x_cp(1, 2), wq_cp(1)],
                     [wq_cp(2), pltpu.make_async_copy(wo_hbm, wo_v, sem_i.at[3])]]
            order = sum(first, [])
            for p in range(NP + 1):
                order += group_cp(p)
            xr_cp = [x_cp(b, SEM_P + NP + 1) for b in range(2, NB)]
            order += xr_cp
            for cp in order:
                cp.start()
            get = lambda an, name: [an[min(i, len(an) - 1)] for i in cfg[name]]
            e_grp = lambda e: ((e >> 1) & 1, ((e >> 2) << 1) | (e & 1))
            if 'a' in cfg['sub']:
                pre_a(first, get, e_grp)
            if 'b' in cfg['sub']:
                pre_b(get, e_grp)
            if 'c' in cfg['sub']:
                pre_c(get)
            wait('WX', xr_cp)

        def pre_a(first, get, e_grp):
            def transpose_wq(i):
                wt_s[WQ[i] // 2:WQ[i + 1] // 2, :D] = _pk(wqkv_v[:, WQ[i]:WQ[i + 1]].T)

            def clear(i, carry):
                for k in range(2):
                    acc_s[k, i] = jnp.zeros((D3, TH), F32)
                r = jnp.minimum(i, 11) * (RP // 4)
                qkv_s[0, rows8(r, RP // 4)] = jnp.zeros((RP // 4, LANES), U32)
                return carry

            lax.fori_loop(0, 15, clear, 0)
            wait('WX0', first[0])
            xn0 = ln1(0, ()).astype(BF16)

            wait('WQ0', first[1])
            transpose_wq(0)
            qkv_mm(0, xn0, (0, 1), [])

            wait('WQ1', first[2])
            transpose_wq(1)
            an = []
            qkv_mm(0, xn0, (2, 3), an)
            xn1 = ln1(1, get(an, 'a_ln'), get(an, 'a_lnb')).astype(BF16)
            qkv_mm(1, xn1, (0,), an, True)
            for n, a in enumerate(get(an, 'a_w1')):
                prep_att(n, a)
            nk = len(cfg['a_k'])
            apply = [att_values(0, *e_grp(e), a) for e, a in enumerate(get(an, 'a_k'))]

            wait('WQ2', first[3])
            an = []
            qkv_mm(1, xn1, (2,), an)
            transpose_wq(2)
            qkv_mm(0, xn0, (4, 5), an)
            qkv_mm(1, xn1, (4,), an)
            qkv_mm(1, xn1, (1,), an, True)
            apply += [att_values(0, *e_grp(nk + e), a)
                      for e, a in enumerate(get(an, 'a_k2')[:8 - nk])]
            for e, a in enumerate(get(an, 'a_v')):
                apply[e](a)
            wo = pltpu.bitcast(wo_v[...], U32)
            wo = cat0(_lo(wo), _hi(wo))
            wo = cat0(*[_tie(wo[n * LANES:(n + 1) * LANES], a)
                        for n, a in enumerate(get(an, 'a_wo'))])
            wt_s[3 * RP:, :D] = _pk(wo.astype(BF16).T)
            for n, a in enumerate(get(an, 'a_w2')):
                prep_att(12 + n, a)

            wait('WO', group_cp(0))
            an = []
            stats = wo_mm(0, an, False)
            qkv_mm(1, xn1, (3, 5), an)
            for n, a in enumerate(get(an, 'z_w')):
                prep_att(36 + n, a)
            prep_piece(0, gu_s.at[0], get(an, 'z_g'), cfg['z_grp'])
            ffn_lhs(0, stats, get(an, 'z_l'))

        def pre_b(get, e_grp):
            def piece(p, carry):
                wait('WP', group_cp(p))
                an = []
                win = gu_s.at[pl.ds(p - 1, 2)]
                h = gu_piece(win.at[0], cfg['gorder0'], an, (0, 7, 4, 11))
                h3_s[p - 1] = cat0(*h[3])
                tri = in_triple(p - 1)
                prep_d(tri, get(an, 'p_d'))
                store_acc(0, down_mm(load_acc(0), [(tri, h_ops(h[:3]))], an))
                prep_piece(p, win.at[1], get(an, 'f_g'), cfg['f_grp'])
                att_group(1, *e_grp(p - 1), an[cfg['p_att'][0]])
                return carry

            lax.fori_loop(1, NP, piece, 0)

        def pre_c(get):
            wait('WD', group_cp(NP))
            an = []
            h = gu_piece(gu_s.at[NP - 1], cfg['gorder'], an)
            h3 = [[h3_s[q, :TH], h3_s[q, TH:]] for q in range(NP - 1)] + [h[3]]
            work = [(cross_triple(s), h_ops(h3[3 * s:3 * s + 3])) for s in range(3)]
            work.append((in_triple(NP - 1), h_ops(h[:3])))
            stats = wo_mm(1, an, True)
            td = get(an, 't_d')
            for n, (tri, _) in enumerate(work):
                prep_d(tri, td[n * len(td) // 4:(n + 1) * len(td) // 4])
            acc = down_mm(load_acc(0), work, an)
            nw = len(cfg['a_w2'])
            for n, a in enumerate(get(an, 't_w')[:24 - nw]):
                prep_att(12 + nw + n, a)
            ffn_lhs(1, stats, get(an, 't_l'))
            finish(0, acc)

        if 'pre' in cfg['phases']:
            pre_phase()

        def body(u, carry):
            bu = u & (NB - 1)
            ba = (u + 1) & (NB - 1)
            acc, stats, an, b, hh = None, None, {}, {}, {}
            get = lambda name: [an[k][i] for k, i in cfg[name]]
            for step in cfg['body']:
                an[step] = []
                if step == 'Q':
                    xn = ln1(ba, get('ln1'), get('ln1b'))
                    qkv_fast(ba, att_rhs(xn, u >> 8), an[step])
                elif step == 'W':
                    attention(ba, get('att'))
                    stats = wo_mm(ba, an[step], True, u >> 8, get('orhs'))
                elif step == 'L':
                    ffn_lhs(ba, stats, get('lhs'))
                elif step[0] == 'G':
                    q, go = int(step[1]), cfg['gorder']
                    t = b.setdefault(step[:2], ({}, {}))
                    for m, m1 in (go[:7] if step[2] == '0' else go[7:]):
                        t[m][m1] = gu_outer(gu_s.at[q], m, m1, an[step])
                    if len(t[0]) + len(t[1]) == 14:
                        hh[q] = gu_finish(t)
                else:
                    work = []
                    for c in step[1:]:
                        if c.isdigit():
                            work.append((in_triple(int(c)), h_ops(hh[int(c)][:3])))
                        else:
                            s = ord(c) - ord('a')
                            work.append((cross_triple(s),
                                         h_ops([hh[3 * s + k][3] for k in range(3)])))
                    acc = down_mm(acc, work, an[step])
            finish(bu, acc)

            @pl.when(u >= NB)
            def _():
                out_copy(bu).start()
            return carry

        if scopes:
            with jax.named_scope('LOOP'):
                lax.fori_loop(1, NU - 1, body, 0)
        elif 'main' in cfg['phases']:
            lax.fori_loop(1, NU - 1, body, 0)

        def last(s, carry):
            h = [gu_piece(gu_s.at[3 * s + k], cfg['lorder'], []) for k in range(3)]
            work = [(in_triple(3 * s + k), h_ops(h[k][:3])) for k in range(3)]
            work.append((cross_triple(s), h_ops([h[k][3] for k in range(3)])))
            acc = down_mm(down_mm(load_acc(1), work[:2], []), work[2:], [])
            store_acc(1, acc)
            finish(NB - 1, acc)
            return carry

        if 'last' in cfg['phases']:
            lax.fori_loop(0, NP // 3, last, 0)
        if len(cfg['phases']) < 3:
            def keep(i, c):
                v = (gu_s[i, i, :8, :LANES] + ds_s[i, i, :8, :LANES]
                     + wl_s[rows8(i * 8), :LANES] + a_s[rows8(i * 8), :LANES] + qkv_s[i, :8]
                     + wt_s[rows8(i * 8), :LANES])
                acc_s[1, 0, :8] = (lax.bitcast_convert_type(v, F32) + o_s[i, :8]
                                   + acc_s[i, i, :8] + h3_s[i, :8])
                return c
            lax.fori_loop(0, 2, keep, 0)
            finish(NB - 1, load_acc(1))
        out_copy(NB - 1).start()
        wait('WOUT', [out_copy(b) for b in range(NB)])

    scratch = [
        pltpu.VMEM((NB, D, TM), BF16),
        pltpu.VMEM((D, 3 * D), BF16),
        pltpu.VMEM((D, D), BF16),
        pltpu.VMEM((NP, D, PW), BF16),
        pltpu.VMEM((NP, D, PW), BF16),
        pltpu.VMEM((NP, D, PW), BF16),
        pltpu.VMEM((2 * D, 8 * LANES), U32),
        pltpu.VMEM((4 * Q3, 16 * LANES), U32),
        pltpu.VMEM((NP, 51, 64, 2 * LANES), U32),
        pltpu.VMEM((NP + 3, 5, Q3, 2 * LANES), U32),
        pltpu.VMEM((NB, D, TM), F32),
        pltpu.VMEM((max(fill), 2 * LANES), U32),
        pltpu.VMEM((S // LANES + 1, 3 * RP, LANES), U32),
        pltpu.VMEM((NT, D, LANES), F32),
        pltpu.VMEM((2, 15, D3, TH), F32),
        pltpu.VMEM((NP, TM, LANES), F32),
        pltpu.VMEM((1, 9 * 64, 2 * LANES), U32),
        pltpu.SemaphoreType.DMA((SEM_P + NP + 2,)),
        pltpu.SemaphoreType.DMA((1,)),
    ]

    def wrapped(*refs):
        @pl.when(pl.program_id(0) == 0)
        def _():
            kernel(*refs)

    return wrapped, scratch


_CFG = dict(
    scopes=False,
    tie1=True,
    orhs=(('G80', 0), ('G80', 1), ('G80', 2), ('G80', 3), ('G80', 4), ('G80', 5),
        ('G80', 6), ('G80', 7), ('G80', 8), ('G80', 9), ('G80', 10), ('G80', 11)),
    sub='abc',
    phases=('pre', 'main', 'last'),
    body=('G20', 'G00', 'G01', 'G10', 'G11', 'Q', 'G30', 'G21', 'G40', 'G31', 'G50',
        'D012a', 'G41', 'G51', 'D345b', 'G70', 'G71', 'G60', 'G80', 'W', 'G61', 'G81',
        'D8c', 'D67', 'L'),
    ln1=(('G00', 0), ('G00', 1), ('G00', 2), ('G00', 3), ('G00', 4), ('G00', 5), ('G00',
        6), ('G00', 7), ('G00', 8)),
    ln1b=(('G10', 1), ('G10', 2), ('G10', 3), ('G10', 4), ('G10', 5), ('G10', 6),
        ('G10', 7), ('G10', 8), ('G10', 9), ('G10', 10), ('G10', 11), ('G10', 12)),
    att=(('D012a', 2), ('D012a', 4), ('D012a', 5), ('D012a', 6), ('D012a', 9), ('D345b',
        6), ('D345b', 7), ('D345b', 8)),
    lhs=(('D8c', 2), ('D8c', 3), ('D8c', 6), ('D67', 5), ('D67', 7), ('D67', 8), ('D67',
        10), ('D67', 11), ('D67', 14)),
    a_w1=(0, 0, 1, 2, 2, 3, 3, 4, 5, 6, 7, 11),
    a_w2=(0, 3, 6, 9, 10, 14),
    a_ln=(0, 3, 6),
    a_lnb=(5, 9, 10),
    z_g=(0, 0, 1, 1, 2, 2, 3, 3, 4, 4, 5, 6, 6, 7, 7, 8, 8, 9, 9, 11, 11, 12, 12, 13,
        13, 14, 14, 15, 15, 16, 17, 17, 18, 18, 19, 19, 20, 21, 21, 22, 23, 23, 23, 24,
        24, 25, 26, 33),
    t_d=(0, 0, 1, 2, 3, 4, 5, 5, 6, 7, 8, 9, 10, 11, 11, 12, 13, 14, 14, 15, 15, 16, 17,
        17, 18, 19, 21, 22, 22, 23, 23, 24, 27, 27, 28, 28, 30, 31, 32, 34, 34, 35, 36,
        37, 38, 39, 40, 40),
    p_d=(3, 12, 14, 17, 24, 25, 28, 33, 35, 38, 42, 46),
    p_att=(58,),
    z_l=(23, 23, 25, 31, 35, 36, 37, 37, 39),
    a_k=(16, 18, 20, 23),
    a_k2=(0, 1, 2, 3),
    a_v=(8, 10, 12, 14, 16, 18, 20, 22),
    a_wo=(9, 18, 27, 36, 46),
    inner=(0, 3, 4, 6, 2, 1, 5),
    gorder=((0, 0), (0, 4), (1, 4), (1, 0), (0, 3), (1, 3), (1, 6), (0, 6), (0, 1), (1,
        1), (0, 2), (1, 2), (0, 5), (1, 5)),
    gorder0=((0, 0), (1, 4), (0, 4), (1, 0), (0, 3), (0, 6), (1, 6), (1, 3), (1, 1), (0,
        1), (0, 2), (0, 5), (1, 5), (1, 2)),
    f_g=(0, 0, 1, 2, 5, 5, 6, 7, 8, 9, 9, 10, 12, 13, 14, 16, 17, 17, 19, 20, 21, 23,
        24, 24, 26, 28, 29, 31, 32, 35, 36, 37, 37, 40, 40, 42, 43, 44, 45, 47, 48, 48,
        53, 56, 58, 59, 60, 61, 62, 62, 64, 64, 69, 70, 70, 70),
    t_l=(50, 51, 52, 53, 54, 55, 56, 57, 58),
    lorder=((1, 0), (1, 4), (0, 0), (0, 4), (0, 3), (0, 6), (1, 3), (1, 6), (0, 1), (1,
        1), (0, 2), (0, 5), (1, 2), (1, 5)),
    z_w=(0, 1, 3, 3, 4, 5, 6, 7, 8, 9, 9, 35),
    z_grp=1,
    f_grp=0,
    t_w=(3, 6, 9, 13, 19, 24, 24, 25, 32, 36, 41, 42, 47, 50, 53, 56, 60, 60),
)


def _run(A_x, A_wqkv, A_wo, B_w_gate, B_w_up, B_w_down, **kw):
    _, S, D = A_x.shape
    F = B_w_gate.shape[1]
    kernel, scratch = _make_kernel(S, D, F, 256, {**_CFG, **kw})
    hbm = pl.BlockSpec(memory_space=pl.ANY)
    out_t = pl.pallas_call(
        kernel,
        grid=(2,),
        in_specs=[hbm] * 6,
        out_specs=hbm,
        out_shape=jax.ShapeDtypeStruct((D, S), A_x.dtype),
        scratch_shapes=scratch,
        compiler_params=pltpu.CompilerParams(
            dimension_semantics=('arbitrary',), vmem_limit_bytes=110 * 1024 * 1024),
    )(A_x.reshape(S, D).T, A_wqkv, A_wo, B_w_gate, B_w_up, B_w_down.T)
    return out_t.T.reshape(A_x.shape)


@jax.jit
def pallas_interleave_layers__sliding_local_dilated__glu_gated_geglu__prompt_kernel(
    A_x: jax.Array,
    A_wqkv: jax.Array,
    A_wo: jax.Array,
    B_x: jax.Array,
    B_w_gate: jax.Array,
    B_w_up: jax.Array,
    B_w_down: jax.Array,
):
    del B_x
    return _run(A_x, A_wqkv, A_wo, B_w_gate, B_w_up, B_w_down)
```

```python
import jax
import jax.numpy as jnp
import jax.experimental.pallas as pl
import jax.experimental.pallas.tpu as pltpu
from jax import lax

H = 32
W = 8
DIL = 2
EPS = 1e-5
LANES = 128

F32 = jnp.float32
BF16 = jnp.bfloat16
U32 = jnp.uint32

_NT = (((1,), (1,)), ((), ()))


def _tree_sum(parts, op=jnp.add):
    while len(parts) > 1:
        nxt = [op(parts[i], parts[i + 1]) for i in range(0, len(parts) - 1, 2)]
        if len(parts) % 2:
            nxt.append(parts[-1])
        parts = nxt
    return parts[0]


def _ln_stats(slabs, d, anchors=()):
    n_acc = 4
    s1, s2, pilot = [None] * n_acc, [None] * n_acc, None
    for i, x in enumerate(slabs):
        if pilot is None:
            pilot = x[0:1, :]
            pil = jnp.broadcast_to(pilot, x.shape)
            pils = [_tie(pil, a) for a in anchors] or [pil]
        dx = x - pils[i * len(pils) // (d // 8)]
        j = i % n_acc
        s1[j] = dx if s1[j] is None else s1[j] + dx
        s2[j] = dx * dx if s2[j] is None else s2[j] + dx * dx
    e1 = jnp.sum(_tree_sum(s1), axis=0, keepdims=True) * (1.0 / d)
    e2 = jnp.sum(_tree_sum(s2), axis=0, keepdims=True) * (1.0 / d)
    var = jnp.maximum(e2 - e1 * e1, 0.0)
    return pilot + e1, lax.rsqrt(var + EPS)


def _zero_like_dep(v):
    return (lax.bitcast_convert_type(v, U32) >> 31) >> 1


def _tie(x, anchor):
    if anchor is None:
        return x
    z = lax.bitcast_convert_type(_zero_like_dep(anchor), F32)
    z = jnp.concatenate([z] * -(-x.shape[1] // LANES), axis=1)[:, :x.shape[1]]
    if x.shape[0] == 8:
        return x + z
    return jnp.concatenate([x[:8] + z, x[8:]], axis=0)


def _gelu_mul2(g, u):
    c0 = 0.7978845608028654
    c1 = c0 * 0.044715
    t = jnp.tanh(g * (c0 + c1 * (g * g)))
    return (g * u) * (1.0 + t)


def _lo(x):
    return lax.bitcast_convert_type(x << 16, F32)


def _hi(x):
    return lax.bitcast_convert_type(x & jnp.uint32(0xFFFF0000), F32)


def _pk(x):
    return pltpu.bitcast(x.astype(BF16), U32)


def _upk(x):
    return pltpu.bitcast(x, BF16)


def _dot(a, b):
    return jnp.dot(a, b, preferred_element_type=F32)


def _dot_nt(a, b):
    return lax.dot_general(a, b, _NT, preferred_element_type=F32)


def _x_ops(x1, x2):
    d = [a - b for a, b in zip(x1, x2)]
    return [x1[0] + x2[1], x2[0] + x2[1], x1[0] + x1[1],
            d[1] + x1[2], x1[1] + x1[2], d[1] + d[2],
            d[0] - x2[2], d[0] + d[2], x2[0] + x2[2],
            x1[0], d[0], x2[1], d[1], x1[2], x2[2]]


def _x_rem(x1, x2):
    a, b, c = 0, 1, 2
    cat = lambda u, v: jnp.concatenate([u, v], axis=0)
    return [cat(x1[c], x2[b]), cat(x1[a], x1[b] - x2[b]), cat(x2[a], x2[c] - x1[c])]


_W_TERMS = {0: ((0, 1, 1), (1, 0, 1)), 3: ((1, 2, 1), (2, 1, 1)), 6: ((0, 2, 1), (2, 0, 1)),
            9: ((0, 0, 1), (0, 2, 1), (1, 0, -1)), 10: ((2, 0, 1), (0, 0, -1), (0, 1, -1)),
            11: ((1, 1, 1), (1, 2, 1), (0, 1, -1)), 12: ((1, 0, 1), (1, 1, 1), (2, 1, -1)),
            13: ((2, 0, 1), (2, 2, 1), (1, 2, -1)), 14: ((2, 1, 1), (2, 2, 1), (0, 2, -1)),
            1: ((0, 1, 1),), 2: ((1, 0, 1),), 4: ((1, 2, 1),), 5: ((2, 1, 1),),
            7: ((2, 0, 1),), 8: ((0, 2, 1),)}


def _w_sums(w):
    return [_signed(_W_TERMS[i], lambda k, j: w[k][j]) for i in _W_SUM]


_W_SUM = {0: 0, 3: 1, 6: 2, 9: 3, 10: 4, 11: 5, 12: 6, 13: 7, 14: 8}
_W_RAW = {1: (0, 1), 2: (1, 0), 4: (1, 2), 5: (2, 1), 7: (2, 0), 8: (0, 2)}
_PAIR_ORDER = (1, 2, 4, 5, 7, 8, 0, 3, 6)
_DIAG = {(0, 0): 9, (2, 0): 10, (0, 1): 11, (1, 1): 12, (1, 2): 13, (2, 2): 14}
_PAIR = {(0, 0): ((6, -1), (8, -1)), (1, 0): ((2, 1), (7, 1)), (2, 0): ((0, 1), (1, -1)),
         (0, 1): ((3, 1), (4, -1)), (1, 1): ((0, 1), (2, -1)), (2, 1): ((1, 1), (5, -1)),
         (0, 2): ((4, 1), (8, 1)), (1, 2): ((6, 1), (7, -1)), (2, 2): ((5, 1), (3, -1))}


def _column(t, base, j, skew=False):
    s = []
    for k in range(3):
        v = base[k]
        for i, sg in _PAIR[k, j]:
            v = t[i] if v is None else (v + t[i] if sg > 0 else v - t[i])
        s.append(v)
    if skew:
        return s[1] + s[0], s[2] + 0.5 * (s[0] - s[1])
    return s[1] + s[0], s[2] + s[0]


_SA = (((0, 0, 1), (1, 1, 1)), ((1, 0, 1), (1, 1, 1)), ((0, 0, 1),), ((1, 1, 1),),
       ((0, 0, 1), (0, 1, 1)), ((1, 0, 1), (0, 0, -1)), ((0, 1, 1), (1, 1, -1)))
_SB = (((0, 0, 1), (1, 1, 1)), ((0, 0, 1),), ((0, 1, 1), (1, 1, -1)), ((1, 0, 1), (0, 0, -1)),
       ((1, 1, 1),), ((0, 0, 1), (0, 1, 1)), ((1, 0, 1), (1, 1, 1)))
_SCOL = {2: 1, 3: 0, 5: 1, 6: 0}
_SGRP = ((1, 4, 0), (3, 6), (2, 5))


def _signed(terms, f):
    v = None
    for a, b, sg in terms:
        v = f(a, b) if v is None else (v + f(a, b) if sg > 0 else v - f(a, b))
    return v


def _s_out(m):
    return [[m[0] + m[3] - m[4] + m[6], m[2] + m[4]],
            [m[1] + m[3], m[0] - m[1] + m[2] + m[5]]]


def _make_kernel(S, D, F, TM, cfg):
    NB = S // TM
    NT = TM // LANES
    DH = D // H
    DP = DH // 2
    RP = D // 2
    NG = H // 8
    scale = float(DH) ** -0.5
    NU = 2 * NB
    TH = TM // 2
    TQ = TM // 4
    D2 = D // 2
    D3 = D // 3
    Q3 = D3 // 2
    KU = D // 9
    KR = 3 * LANES
    NQ = 6
    QR = 3 * D // NQ
    WQ = (0, 640, 1152, 3 * D)
    PW = 4 * LANES
    NP = F // PW
    AOFF, fill = {}, [0, 0]
    for key in [(m1, m2) for m1 in range(7) for m2 in range(7)]:
        c = int(fill[1] < fill[0])
        AOFF[key] = (fill[c], slice(c * LANES, (c + 1) * LANES))
        fill[c] += 48 if key[0] in _SCOL and key[1] in _SCOL else 32
    scopes = cfg['scopes']
    assert NG == 4 and NB & (NB - 1) == 0
    SEM_P = 4

    def kernel(x_hbm, wqkv_hbm, wo_hbm, wg_hbm, wu_hbm, wdt_hbm, out_hbm,
               xio_s, wqkv_v, wo_v, wg_v, wu_v, wdt_v, wt_s, wl_s,
               gu_s, ds_s, xmid_s, a_s, qkv_s, o_s, acc_s, h3_s, r_s,
               sem_i, sem_o):

        def wait(name, cps):
            if scopes:
                with jax.named_scope(name):
                    for cp in cps:
                        cp.wait()
            else:
                for cp in cps:
                    cp.wait()

        def cols(lo, n):
            if not isinstance(lo, int):
                lo = pl.multiple_of(lo, LANES)
            return pl.ds(lo, n)

        def rows8(lo, n=8):
            if not isinstance(lo, int):
                lo = pl.multiple_of(lo, 8)
            return pl.ds(lo, n)

        def out_copy(b):
            return pltpu.make_async_copy(
                xio_s.at[b], out_hbm.at[:, cols(b * TM, TM)], sem_o.at[0])

        def x_cp(b, sem):
            return pltpu.make_async_copy(x_hbm.at[:, cols(b * TM, TM)], xio_s.at[b],
                                         sem_i.at[sem])

        def wq_cp(i):
            sl = cols(WQ[i], WQ[i + 1] - WQ[i])
            return pltpu.make_async_copy(wqkv_hbm.at[:, sl], wqkv_v.at[:, sl],
                                         sem_i.at[1 + i])

        def piece_cp(src, dst, p, sem, c0=0, n=PW):
            return pltpu.make_async_copy(src.at[:, cols(p * PW + c0, n)],
                                         dst.at[p, :, pl.ds(c0, n)], sem_i.at[sem])

        def group_cp(p):
            sem = SEM_P + p
            cps = []
            if not (isinstance(p, int) and p == NP):
                cps += [piece_cp(wg_hbm, wg_v, p, sem), piece_cp(wu_hbm, wu_v, p, sem)]
            if not (isinstance(p, int) and p == 0):
                cps.append(piece_cp(wdt_hbm, wdt_v, p - 1, sem, 0, KR))
            if isinstance(p, int) and p == NP:
                cps += [piece_cp(wdt_hbm, wdt_v, q, sem, KR, LANES) for q in range(NP)]
            return cps

        lane = lax.broadcasted_iota(jnp.int32, (8, LANES), 1)
        cat0 = lambda *v: jnp.concatenate(v, axis=0)
        cat1 = lambda *v: jnp.concatenate(v, axis=1)

        def spread_over(anchors, n, total):
            return anchors[n * len(anchors) // total] if anchors else None

        def slab_group(r):
            return (r % LANES) // 16 if r < KR else 8 + ((r - KR) % KU) // 16

        def ln1(blk, anchors1, anchors2=()):
            slabs = (xio_s[blk, r:r + 8, :].astype(F32) for r in range(0, D, 8))
            m, rs = _ln_stats(slabs, D, anchors1)
            if not anchors2:
                return (xio_s[blk].astype(F32) - m) * rs
            m8 = jnp.broadcast_to(m, (8, TM))
            ms = [_tie(m8, a) for a in anchors2]
            ms = [spread_over(ms, slab_group(r), 12) for r in range(0, D, 8)]
            return (xio_s[blk].astype(F32) - cat0(*ms)) * rs

        def dot_k(rows, x, anchors, even=False):
            y = None
            for n, k in enumerate(range(0, D, LANES)):
                ks = slice(k, min(k + LANES, D))
                if even and k + LANES >= D:
                    mid = (rows.start + rows.stop) // 2
                    v = cat0(_dot(_upk(wt_s[rows.start:mid, ks]), x[ks]),
                             _dot(_upk(wt_s[mid:rows.stop, ks]), x[ks]))
                else:
                    v = _dot(_upk(wt_s[rows, ks]), x[ks])
                anchors.extend(v[r:r + 8, :LANES] for r in ((0, 144) if n % 2 else (72, 216)))
                y = v if y is None else y + v
            return y

        def put_qkv(blk, rows, y):
            pk = _pk(y)
            for c in range(NT):
                qkv_s[1 + blk * NT + c, rows, :] = pk[:, c * LANES:(c + 1) * LANES]

        def qkv_mm(blk, xn, chunks, anchors, even=False):
            for r in chunks:
                rows = slice(r * QR // 2, (r + 1) * QR // 2)
                put_qkv(blk, rows, dot_k(rows, xn, anchors, even))

        def split_k(x):
            hs = (x[:, :TH], x[:, TH:])
            blocks = [[h[k * LANES:(k + 1) * LANES] for k in range(3)] for h in hs]
            units = [[h[KR + k * KU:KR + (k + 1) * KU] for k in range(3)] for h in hs]
            return blocks, units

        def prep_att(pat, anchor):
            assert Q3 == 96
            row0 = pat * 8
            src0 = row0 + ((pat * 43) >> 9) * (2 * Q3)
            w = [_upk(wt_s[rows8(src0 + j * Q3), :D]).astype(F32) for j in range(3)]
            w[0] = cat1(_tie(w[0][:, :LANES], anchor), w[0][:, LANES:])
            tiles = _w_sums([[w[j][:, k * LANES:(k + 1) * LANES] for j in range(3)]
                             for k in range(3)])
            for j in range(3):
                a, b, c = (w[j][:, KR + k * KU:KR + (k + 1) * KU] for k in range(3))
                tiles += [cat1(c, b), cat1(a, c)]
            wl_s[rows8(row0), :15 * LANES] = _pk(cat1(*tiles))

        def att_rhs(x, stash=None, anchors=()):
            half = 0.5
            if anchors:
                hs = [_tie(jnp.full((8, TH), 0.5, F32), a) for a in anchors]
                half = cat0(*[spread_over(hs, slab_group(r), 12) for r in range(0, D, 8)])
            blocks, units = split_k(cat1(x[:, :TH], x[:, TH:] + half * x[:, :TH]))
            ops = _x_ops(*blocks) + _x_rem(*units)
            if stash is None:
                return [v.astype(BF16) for v in ops]
            loc = lambda i, r0, n: (slice((i // 2) * 64 + r0, (i // 2) * 64 + r0 + n),
                                    slice((i % 2) * LANES, (i % 2 + 1) * LANES))
            for r in range(0, LANES, 16):
                for i, v in enumerate(ops):
                    r_s.at[0][loc(i, r // 2, 8)] = _pk(v[r:r + 16])
            return [_upk(r_s.at[stash][loc(i, 0, 64)]) for i in range(18)]

        def att_mm(sec, rhs, anchors):
            tl = lambda i: _upk(wl_s[sec * Q3:(sec + 1) * Q3, i * LANES:(i + 1) * LANES])
            raw = lambda k, j: _upk(wt_s[(3 * sec + j) * Q3:(3 * sec + j + 1) * Q3,
                                         k * LANES:(k + 1) * LANES])
            t = {}
            for i in _PAIR_ORDER:
                t[i] = _dot(raw(*_W_RAW[i]) if i in _W_RAW else tl(_W_SUM[i]), rhs[i])
                anchors.append(t[i][:8])
            out = []
            for j in range(3):
                base = []
                for s in range(3):
                    v = _dot(raw(3, j) if s == 1 else tl(9 + 2 * j + s // 2), rhs[15 + s])
                    if (s, j) in _DIAG:
                        i = _DIAG[s, j]
                        v = _dot(tl(_W_SUM[i]), rhs[i]) + v
                    base.append(v)
                    anchors.append(base[-1][:8])
                out.append(cat1(*_column(t, base, j, True)))
            return cat0(*out)

        def qkv_fast(blk, rhs, anchors):
            for sec in range(3):
                put_qkv(blk, slice(sec * RP, (sec + 1) * RP), att_mm(sec, rhs, anchors))

        def shifted(ln, cur, prev, w):
            if w == 0:
                return cur
            sh = DIL * w
            return pltpu.roll(jnp.where(ln < LANES - sh, cur, prev), sh, axis=1)

        def att_group(blk, c, hg, anchor):
            att_values(blk, c, hg, anchor)(None)

        def att_values(blk, c, hg, anchor):
            tile = blk * NT + c
            base = hg * 8 * DP
            if isinstance(hg, int):
                cur, prev, o_t = qkv_s.at[1 + tile], qkv_s.at[tile], o_s.at[c]
            else:
                n = 2 * RP + 8 * DP
                base = pl.multiple_of(base, 8)
                cur = qkv_s.at[1 + tile, pl.ds(base, n)]
                prev = qkv_s.at[tile, pl.ds(base, n)]
                o_t = o_s.at[c, pl.ds(base, RP + 8 * DP)]
                base = 0
            ln = lane + _zero_like_dep(anchor).astype(jnp.int32)
            logits = [None] * W
            for dd in range(DP):
                q = cur[pl.ds(base + dd, 8, stride=DP), :]
                kc = cur[pl.ds(RP + base + dd, 8, stride=DP), :]
                kp = prev[pl.ds(RP + base + dd, 8, stride=DP), :]
                q0, q1 = _lo(q), _hi(q)
                for w in range(W):
                    ks = shifted(ln, kc, kp, w)
                    t = q0 * _lo(ks) + q1 * _hi(ks)
                    logits[w] = t if logits[w] is None else logits[w] + t
            logits = [l * scale for l in logits]
            if not (isinstance(c, int) and c > 0):
                pos = lane + tile * LANES
                logits = [l if w == 0 else jnp.where(pos >= DIL * w, l, -1e9)
                          for w, l in enumerate(logits)]
            m = _tree_sum(logits, jnp.maximum)
            p = [jnp.exp(l - m) for l in logits]
            r = 1.0 / _tree_sum(p)

            def apply(anchor2):
                ln = lane + _zero_like_dep(_tie(m, anchor2)).astype(jnp.int32)
                for dd in range(DP):
                    vc = cur[pl.ds(2 * RP + base + dd, 8, stride=DP), :]
                    vp = prev[pl.ds(2 * RP + base + dd, 8, stride=DP), :]
                    o0 = o1 = None
                    for w in range(W):
                        vs = shifted(ln, vc, vp, w)
                        t0, t1 = p[w] * _lo(vs), p[w] * _hi(vs)
                        o0 = t0 if o0 is None else o0 + t0
                        o1 = t1 if o1 is None else o1 + t1
                    o0, o1 = o0 * r, o1 * r
                    o_t[pl.ds(base + dd, 8, stride=DP), :] = o0
                    o_t[pl.ds(RP + base + dd, 8, stride=DP), :] = o1

            return apply

        def attention(blk, anchors):
            for c in range(NT):
                for hg in range(NG):
                    att_group(blk, c, hg, anchors[c * NG + hg])

        def wo_mm(blk, anchors, fast, stash=None, anchors_in=()):
            o = cat1(*[o_s[c] for c in range(NT)])
            if fast:
                y = att_mm(3, att_rhs(o, stash, anchors_in), anchors)
            else:
                o = o.astype(BF16)
                q = D2 // 2
                y = cat0(*[dot_k(slice(h * q, (h + 1) * q), o, anchors) for h in (6, 7)])
            xm = xio_s[blk].astype(F32) + y
            xmid_s[blk] = xm
            return _ln_stats((xm[r:r + 8] for r in range(0, D, 8)), D)

        def ffn_lhs(blk, stats, anchors):
            m, rs = stats
            m8 = jnp.broadcast_to(m, (8, TM))
            xt = []
            for k in range(5):
                mt = cat0(*[_tie(m8, spread_over(anchors[:2], k, 5))] * (KU // 8 if k == 4 else 16))
                x = (xmid_s[blk, k * LANES:min((k + 1) * LANES, D), :] - mt) * rs
                xt.append((cat0(x, x) if k == 4 else x).T)
            lo = lax.broadcasted_iota(jnp.int32, (TQ // 2, LANES), 1) < KU
            for m1 in range(7):
                a = spread_over(anchors[2:], m1, 7)
                blk1 = lambda i2, k2: _signed(_SA[m1], lambda i1, k1: _tie(
                    xt[k2 if k2 == 4 else 2 * k1 + k2][(2 * i1 + i2) * TQ:(2 * i1 + i2 + 1) * TQ], a))
                l1 = {(i2, k2): blk1(i2, k2) for i2 in range(2)
                      for k2 in ((0, 1, 4) if m1 in _SCOL else (0, 1))}
                for m2 in range(7):
                    v = _signed(_SA[m2], lambda i2, k2: l1[i2, k2])
                    if m1 in _SCOL and m2 in _SCOL:
                        c = _signed(_SA[m2], lambda i2, k2: l1[i2, 4])
                        h = TQ // 2
                        vp, vq, cp, cq = v[:h], v[h:], c[:h], c[h:]
                        v = cat0(jnp.where(lo, cp, vq), jnp.where(lo, vp, vp - vq),
                                 jnp.where(lo, vq, cq - cp))
                    o, ac = AOFF[m1, m2]
                    a_s[o:o + v.shape[0] // 2, ac] = _pk(v)

        def in_triple(q):
            return q, lambda k: (q, k)

        def cross_triple(s):
            return NP + s, lambda k: (3 * s + k, 3)

        def wd_raw(tri, k, r0, n):
            q, c = tri[1](k)
            return wdt_v[q, r0:r0 + n, c * LANES:(c + 1) * LANES]

        def ds_loc(i, r0, n):
            return slice(r0, r0 + n), slice((i % 2) * LANES, (i % 2 + 1) * LANES)

        def prep_d(tri, anchors):
            PR = 16
            for n in range(D3 // PR):
                r = n * PR
                w = [[wd_raw(tri, k, j * D3 + r, PR).astype(F32) for j in range(3)]
                     for k in range(3)]
                w[0][1] = _tie(w[0][1], spread_over(anchors, n, D3 // PR))
                for i, v in enumerate(_w_sums(w)):
                    ds_s.at[tri[0], i // 2][ds_loc(i, r // 2, PR // 2)] = _pk(v)

        GU = (wg_v, wu_v)

        def prep_gu(p, gv, m, m1s, anchors):
            PR = 16
            cs = slice(m * LANES, (m + 1) * LANES)
            for n in range(LANES // PR):
                r = n * PR
                cache = {}

                def w(k, j1):
                    if (k, j1) not in cache:
                        v = GU[m][p, k * LANES + r:k * LANES + r + PR,
                                  2 * j1 * LANES:2 * (j1 + 1) * LANES].astype(F32)
                        if (k // 2, j1) in [_SB[m1][0][:2] for m1 in m1s[:2]]:
                            a = spread_over(anchors, n, LANES // PR)
                            if cfg['tie1']:
                                c = (k % 2) * LANES
                                tied = _tie(v[:, c:c + LANES], a)
                                v = cat1(v[:, :LANES], tied) if c else cat1(tied, v[:, LANES:])
                            else:
                                v = _tie(v, a)
                        cache[k, j1] = v
                    return cache[k, j1]

                for m1 in m1s:
                    b1 = [_signed(_SB[m1], lambda k1, j1: w(2 * k1 + k2, j1)) for k2 in range(2)]
                    for m2 in range(7):
                        v = _signed(_SB[m2],
                                    lambda k2, j2: b1[k2][:, j2 * LANES:(j2 + 1) * LANES])
                        gv.at[7 * m1 + m2][r // 2:(r + PR) // 2, cs] = _pk(v)

        def prep_tail(p, gv, m, anchor):
            v = _tie(GU[m][p, 4 * LANES:, :].astype(F32), anchor)
            for j in range(4):
                gv.at[49 + j // 2][(j % 2) * 32:(j % 2 + 1) * 32,
                                        m * LANES:(m + 1) * LANES] = _pk(
                                            v[:, j * LANES:(j + 1) * LANES])

        def gu_outer(gv, m, m1, anchors, at=(0, 4)):
            cs = slice(m * LANES, (m + 1) * LANES)
            y = {}
            for m2 in cfg['inner']:
                i, (o, ac) = 7 * m1 + m2, AOFF[m1, m2]
                if m1 in _SCOL and m2 in _SCOL:
                    j = 2 * _SCOL[m1] + _SCOL[m2]
                    tail = lambda: gv[49 + j // 2, (j % 2) * 32:(j % 2 + 1) * 32, cs]
                    rhs = (cat0(tail(), gv[i, 32:, cs]), gv[i, :, cs],
                           cat0(gv[i, :32, cs], tail()))
                    r = [_dot(_upk(a_s[o + 16 * s:o + 16 * (s + 1), ac]), _upk(rhs[s]))
                         for s in range(3)]
                    y[m2] = cat0(r[1] + r[0], r[2] + r[0])
                else:
                    y[m2] = _dot(_upk(a_s[o:o + TQ // 2, ac]), _upk(gv[i, :, cs]))
            anchors.extend(y[cfg['inner'][k % 7]][(k // 7) * 32:(k // 7) * 32 + 8] for k in at)
            return _s_out(y)

        def gu_finish(t):
            gu = [{(i2, j2): _s_out([t[m][m1][i2][j2] for m1 in range(7)])
                   for i2 in range(2) for j2 in range(2)} for m in range(2)]
            return [[cat0(*[_gelu_mul2(*[gu[m][i2, j % 2][i1][j // 2] for m in range(2)])
                            for i2 in range(2)]) for i1 in range(2)] for j in range(4)]

        def gu_piece(gv, order, anchors, at=(0, 4)):
            t = ({}, {})
            for m, m1 in order:
                t[m][m1] = gu_outer(gv, m, m1, anchors, at)
            return gu_finish(t)

        def prep_piece(p, gv, anchors, group):
            grp = _SGRP if group else [(m1,) for m1 in range(7)]
            k = len(anchors) // (2 * len(grp))
            for n in range(2 * len(grp)):
                prep_gu(p, gv, n % 2, grp[n // 2], anchors[k * n:k * n + k])
            for m in range(2):
                prep_tail(p, gv, m, anchors[m * len(anchors) // 2])

        def h_ops(h):
            return [v.astype(BF16) for v in _x_ops(*[[h[k][i] for k in range(3)]
                                                     for i in range(2)])]

        D_ORDER = _PAIR_ORDER + (9, 10, 11, 12, 13, 14)

        def down_mm(acc, work, anchors, which=D_ORDER, fine=False):
            p = [None] * 15 if acc is None else list(acc)
            jobs = [(i, n) for i in which for n in range(len(work))]
            split = {0: (), 1: (4,), 2: (2, 2), 3: (2, 2, 4)}[len(jobs) % 4]
            split = dict(zip(jobs[len(jobs) - len(split):], split))
            for i in which:
                y = None
                for n, (tri, b) in enumerate(work):
                    ns = split.get((i, n), 1)
                    nr = D3 // ns
                    if i in _W_RAW:
                        k, j = _W_RAW[i]
                        lhs = lambda h: wd_raw(tri, k, j * D3 + h * nr, nr)
                    else:
                        s = _W_SUM[i]
                        lhs = lambda h: _upk(ds_s.at[tri[0], s // 2][ds_loc(s, h * nr // 2, nr // 2)])
                    v = cat0(*[_dot_nt(lhs(h), b[i]) for h in range(ns)])
                    y = v if y is None else y + v
                p[i] = y if p[i] is None else p[i] + y
                anchors.append(p[i][:8])
                if fine:
                    anchors.append(p[i][D3 // 2:D3 // 2 + 8])
            return p

        def finish(blk, acc):
            y = [cat1(*_column(acc, [acc[_DIAG[s, j]] if (s, j) in _DIAG else None
                                     for s in range(3)], j)) for j in range(3)]
            xio_s[blk] = (xmid_s[blk] + 0.5 * cat0(*y)).astype(BF16)

        def load_acc(k):
            return [acc_s[k, i] for i in range(15)]

        def store_acc(k, acc):
            for i in range(15):
                acc_s[k, i] = acc[i]

        def pre_phase():
            first = [[x_cp(0, 0)], [wq_cp(0)], [x_cp(1, 2), wq_cp(1)],
                     [wq_cp(2), pltpu.make_async_copy(wo_hbm, wo_v, sem_i.at[3])]]
            order = sum(first, [])
            for p in range(NP + 1):
                order += group_cp(p)
            xr_cp = [x_cp(b, SEM_P + NP + 1) for b in range(2, NB)]
            order += xr_cp
            for cp in order:
                cp.start()
            get = lambda an, name: [an[min(i, len(an) - 1)] for i in cfg[name]]
            e_grp = lambda e: ((e >> 1) & 1, ((e >> 2) << 1) | (e & 1))
            if 'a' in cfg['sub']:
                pre_a(first, get, e_grp)
            if 'b' in cfg['sub']:
                pre_b(get, e_grp)
            if 'c' in cfg['sub']:
                pre_c(get)
            wait('WX', xr_cp)

        def pre_a(first, get, e_grp):
            def transpose_wq(i):
                wt_s[WQ[i] // 2:WQ[i + 1] // 2, :D] = _pk(wqkv_v[:, WQ[i]:WQ[i + 1]].T)

            def clear(i, carry):
                for k in range(2):
                    acc_s[k, i] = jnp.zeros((D3, TH), F32)
                r = jnp.minimum(i, 11) * (RP // 4)
                qkv_s[0, rows8(r, RP // 4)] = jnp.zeros((RP // 4, LANES), U32)
                return carry

            lax.fori_loop(0, 15, clear, 0)
            wait('WX0', first[0])
            xn0 = ln1(0, ()).astype(BF16)

            wait('WQ0', first[1])
            transpose_wq(0)
            qkv_mm(0, xn0, (0, 1), [])

            wait('WQ1', first[2])
            transpose_wq(1)
            an = []
            qkv_mm(0, xn0, (2, 3), an)
            xn1 = ln1(1, get(an, 'a_ln'), get(an, 'a_lnb')).astype(BF16)
            qkv_mm(1, xn1, (0,), an, True)
            for n, a in enumerate(get(an, 'a_w1')):
                prep_att(n, a)
            nk = len(cfg['a_k'])
            apply = [att_values(0, *e_grp(e), a) for e, a in enumerate(get(an, 'a_k'))]

            wait('WQ2', first[3])
            an = []
            qkv_mm(1, xn1, (2,), an)
            transpose_wq(2)
            qkv_mm(0, xn0, (4, 5), an)
            qkv_mm(1, xn1, (4,), an)
            qkv_mm(1, xn1, (1,), an, True)
            apply += [att_values(0, *e_grp(nk + e), a)
                      for e, a in enumerate(get(an, 'a_k2')[:8 - nk])]
            for e, a in enumerate(get(an, 'a_v')):
                apply[e](a)
            wo = pltpu.bitcast(wo_v[...], U32)
            wo = cat0(_lo(wo), _hi(wo))
            wo = cat0(*[_tie(wo[n * LANES:(n + 1) * LANES], a)
                        for n, a in enumerate(get(an, 'a_wo'))])
            wt_s[3 * RP:, :D] = _pk(wo.astype(BF16).T)
            for n, a in enumerate(get(an, 'a_w2')):
                prep_att(len(cfg['a_w1']) + n, a)

            wait('WO', group_cp(0))
            an = []
            stats = wo_mm(0, an, False)
            qkv_mm(1, xn1, (3, 5), an)
            for n, a in enumerate(get(an, 'z_w')):
                prep_att(36 + n, a)
            prep_piece(0, gu_s.at[0], get(an, 'z_g'), cfg['z_grp'])
            ffn_lhs(0, stats, get(an, 'z_l'))

        def pre_b(get, e_grp):
            def piece(p, carry):
                wait('WP', group_cp(p))
                an = []
                win = gu_s.at[pl.ds(p - 1, 2)]
                h = gu_piece(win.at[0], cfg['gorder0'], an, (0, 7, 4, 11))
                h3_s[p - 1] = cat0(*h[3])
                tri = in_triple(p - 1)
                prep_d(tri, get(an, 'p_d'))
                store_acc(0, down_mm(load_acc(0), [(tri, h_ops(h[:3]))], an))
                prep_piece(p, win.at[1], get(an, 'f_g'), cfg['f_grp'])
                att_group(1, *e_grp(p - 1), an[cfg['p_att'][0]])
                return carry

            lax.fori_loop(1, NP, piece, 0)

        def pre_c(get):
            wait('WD', group_cp(NP))
            an = []
            h = gu_piece(gu_s.at[NP - 1], cfg['gorder'], an)
            h3 = [[h3_s[q, :TH], h3_s[q, TH:]] for q in range(NP - 1)] + [h[3]]
            work = [(cross_triple(s), h_ops(h3[3 * s:3 * s + 3])) for s in range(3)]
            work.append((in_triple(NP - 1), h_ops(h[:3])))
            stats = wo_mm(1, an, True)
            td = get(an, 't_d')
            for n, (tri, _) in enumerate(work):
                prep_d(tri, td[n * len(td) // 4:(n + 1) * len(td) // 4])
            acc = down_mm(load_acc(0), work, an)
            nw = len(cfg['a_w1']) + len(cfg['a_w2'])
            for n, a in enumerate(get(an, 't_w')[:36 - nw]):
                prep_att(nw + n, a)
            ffn_lhs(1, stats, get(an, 't_l'))
            finish(0, acc)

        if 'pre' in cfg['phases']:
            pre_phase()

        def body(u, carry):
            bu = u & (NB - 1)
            ba = (u + 1) & (NB - 1)
            acc, stats, an, b, hh = None, None, {}, {}, {}
            get = lambda name: [an[k][i] for k, i in cfg[name]]
            for step in cfg['body']:
                an[step] = []
                if step == 'Q':
                    xn = ln1(ba, get('ln1'), get('ln1b'))
                    qkv_fast(ba, att_rhs(xn, u >> 8), an[step])
                elif step == 'W':
                    attention(ba, get('att'))
                    stats = wo_mm(ba, an[step], True, u >> 8, get('orhs'))
                elif step == 'L':
                    ffn_lhs(ba, stats, get('lhs'))
                elif step[0] == 'G':
                    q, go = int(step[1]), cfg['gorder']
                    t = b.setdefault(step[:2], ({}, {}))
                    for m, m1 in (go[:7] if step[2] == '0' else go[7:]):
                        t[m][m1] = gu_outer(gu_s.at[q], m, m1, an[step])
                    if len(t[0]) + len(t[1]) == 14:
                        hh[q] = gu_finish(t)
                else:
                    work = []
                    for c in step[1:]:
                        if c.isdigit():
                            work.append((in_triple(int(c)), h_ops(hh[int(c)][:3])))
                        else:
                            s = ord(c) - ord('a')
                            work.append((cross_triple(s),
                                         h_ops([hh[3 * s + k][3] for k in range(3)])))
                    acc = down_mm(acc, work, an[step])
            finish(bu, acc)

            @pl.when(u >= NB)
            def _():
                out_copy(bu).start()
            return carry

        if scopes:
            with jax.named_scope('LOOP'):
                lax.fori_loop(1, NU - 1, body, 0)
        elif 'main' in cfg['phases']:
            lax.fori_loop(1, NU - 1, body, 0)

        def last(s, carry):
            h = [gu_piece(gu_s.at[3 * s + k], cfg['lorder'], []) for k in range(3)]
            work = [(in_triple(3 * s + k), h_ops(h[k][:3])) for k in range(3)]
            work.append((cross_triple(s), h_ops([h[k][3] for k in range(3)])))
            acc = down_mm(down_mm(load_acc(1), work[:2], []), work[2:], [])
            store_acc(1, acc)
            finish(NB - 1, acc)
            return carry

        if 'last' in cfg['phases']:
            lax.fori_loop(0, NP // 3, last, 0)
        if len(cfg['phases']) < 3:
            def keep(i, c):
                v = (gu_s[i, i, :8, :LANES] + ds_s[i, i, :8, :LANES]
                     + wl_s[rows8(i * 8), :LANES] + a_s[rows8(i * 8), :LANES] + qkv_s[i, :8]
                     + wt_s[rows8(i * 8), :LANES])
                acc_s[1, 0, :8] = (lax.bitcast_convert_type(v, F32) + o_s[i, :8]
                                   + acc_s[i, i, :8] + h3_s[i, :8])
                return c
            lax.fori_loop(0, 2, keep, 0)
            finish(NB - 1, load_acc(1))
        out_copy(NB - 1).start()
        wait('WOUT', [out_copy(b) for b in range(NB)])

    scratch = [
        pltpu.VMEM((NB, D, TM), BF16),
        pltpu.VMEM((D, 3 * D), BF16),
        pltpu.VMEM((D, D), BF16),
        pltpu.VMEM((NP, D, PW), BF16),
        pltpu.VMEM((NP, D, PW), BF16),
        pltpu.VMEM((NP, D, PW), BF16),
        pltpu.VMEM((2 * D, 8 * LANES), U32),
        pltpu.VMEM((4 * Q3, 16 * LANES), U32),
        pltpu.VMEM((NP, 51, 64, 2 * LANES), U32),
        pltpu.VMEM((NP + 3, 5, Q3, 2 * LANES), U32),
        pltpu.VMEM((NB, D, TM), F32),
        pltpu.VMEM((max(fill), 2 * LANES), U32),
        pltpu.VMEM((S // LANES + 1, 3 * RP, LANES), U32),
        pltpu.VMEM((NT, D, LANES), F32),
        pltpu.VMEM((2, 15, D3, TH), F32),
        pltpu.VMEM((NP, TM, LANES), F32),
        pltpu.VMEM((1, 9 * 64, 2 * LANES), U32),
        pltpu.SemaphoreType.DMA((SEM_P + NP + 2,)),
        pltpu.SemaphoreType.DMA((1,)),
    ]

    def wrapped(*refs):
        @pl.when(pl.program_id(0) == 0)
        def _():
            kernel(*refs)

    return wrapped, scratch


_CFG = dict(
    scopes=False,
    tie1=True,
    orhs=(('G80', 0), ('G80', 1), ('G80', 2), ('G80', 3), ('G80', 4), ('G80', 5),
        ('G80', 6), ('G80', 7), ('G80', 8), ('G80', 9), ('G80', 10), ('G80', 11)),
    sub='abc',
    phases=('pre', 'main', 'last'),
    body=('G20', 'G00', 'G01', 'G10', 'G11', 'Q', 'G30', 'G21', 'G40', 'G31', 'G50',
        'D012a', 'G41', 'G51', 'D345b', 'G70', 'G71', 'G60', 'G80', 'W', 'G61', 'G81',
        'D8c', 'D67', 'L'),
    ln1=(('G00', 0), ('G00', 1), ('G00', 2), ('G00', 3), ('G00', 4), ('G00', 5), ('G00',
        6), ('G00', 7), ('G00', 8)),
    ln1b=(('G10', 1), ('G10', 2), ('G10', 3), ('G10', 4), ('G10', 5), ('G10', 6),
        ('G10', 7), ('G10', 8), ('G10', 9), ('G10', 10), ('G10', 11), ('G10', 12)),
    att=(('D012a', 2), ('D012a', 4), ('D012a', 5), ('D012a', 6), ('D012a', 9), ('D345b',
        6), ('D345b', 7), ('D345b', 8)),
    lhs=(('D8c', 2), ('D8c', 3), ('D8c', 6), ('D67', 5), ('D67', 7), ('D67', 8), ('D67',
        10), ('D67', 11), ('D67', 14)),
    a_w1=(0, 0, 1, 2, 2, 3, 3, 4, 5, 6, 7, 11, 13, 18, 19, 20, 21, 22, 23, 24, 26, 27,
        28, 29),
    a_w2=(25, 30, 33, 36, 44, 45),
    a_ln=(3, 6, 7),
    a_lnb=(3, 9, 15),
    z_g=(0, 0, 1, 1, 2, 2, 3, 3, 4, 4, 5, 5, 6, 6, 7, 7, 8, 8, 9, 11, 12, 12, 13, 14,
        14, 14, 15, 15, 16, 16, 17, 17, 18, 18, 19, 19, 20, 21, 21, 22, 23, 23, 23, 24,
        25, 26, 27, 33),
    t_d=(0, 0, 0, 2, 2, 4, 5, 5, 7, 7, 8, 8, 9, 10, 11, 11, 12, 12, 13, 14, 14, 15, 16,
        16, 17, 17, 18, 18, 21, 22, 24, 24, 25, 28, 28, 30, 32, 32, 35, 35, 36, 37, 37,
        37, 39, 40, 40, 42),
    p_d=(3, 12, 14, 17, 24, 25, 28, 33, 35, 38, 42, 46),
    p_att=(58,),
    z_l=(23, 23, 28, 31, 35, 36, 37, 37, 39),
    a_k=(13, 17, 20, 26),
    a_k2=(0, 1, 3, 9),
    a_v=(13, 13, 14, 15, 16, 17, 18, 19),
    a_wo=(9, 18, 25, 36, 46),
    inner=(0, 3, 4, 6, 2, 1, 5),
    gorder=((0, 0), (0, 4), (1, 4), (1, 0), (0, 3), (1, 3), (1, 6), (0, 6), (0, 1), (1,
        1), (0, 2), (1, 2), (0, 5), (1, 5)),
    gorder0=((0, 0), (1, 4), (0, 4), (1, 0), (0, 3), (0, 6), (1, 6), (1, 3), (1, 1), (0,
        1), (0, 2), (0, 5), (1, 5), (1, 2)),
    f_g=(0, 0, 1, 2, 5, 5, 6, 7, 8, 9, 9, 10, 12, 13, 14, 16, 17, 17, 19, 20, 21, 23,
        24, 24, 26, 28, 29, 31, 32, 35, 36, 37, 37, 40, 40, 42, 43, 44, 45, 47, 48, 48,
        53, 56, 58, 59, 60, 61, 62, 62, 64, 64, 69, 70, 70, 70),
    t_l=(49, 50, 51, 53, 54, 55, 57, 57, 60),
    lorder=((1, 0), (1, 4), (0, 0), (0, 4), (0, 3), (0, 6), (1, 3), (1, 6), (0, 1), (1,
        1), (0, 2), (0, 5), (1, 2), (1, 5)),
    z_w=(1, 1, 3, 3, 5, 5, 6, 6, 8, 9, 17, 35),
    z_grp=1,
    f_grp=0,
    t_w=(47, 49, 49, 50, 52, 54),
)


def _run(A_x, A_wqkv, A_wo, B_w_gate, B_w_up, B_w_down, **kw):
    _, S, D = A_x.shape
    F = B_w_gate.shape[1]
    kernel, scratch = _make_kernel(S, D, F, 256, {**_CFG, **kw})
    hbm = pl.BlockSpec(memory_space=pl.ANY)
    out_t = pl.pallas_call(
        kernel,
        grid=(2,),
        in_specs=[hbm] * 6,
        out_specs=hbm,
        out_shape=jax.ShapeDtypeStruct((D, S), A_x.dtype),
        scratch_shapes=scratch,
        compiler_params=pltpu.CompilerParams(
            dimension_semantics=('arbitrary',), vmem_limit_bytes=110 * 1024 * 1024),
    )(A_x.reshape(S, D).T, A_wqkv, A_wo, B_w_gate, B_w_up, B_w_down.T)
    return out_t.T.reshape(A_x.shape)


@jax.jit
def pallas_interleave_layers__sliding_local_dilated__glu_gated_geglu__prompt_kernel(
    A_x: jax.Array,
    A_wqkv: jax.Array,
    A_wo: jax.Array,
    B_x: jax.Array,
    B_w_gate: jax.Array,
    B_w_up: jax.Array,
    B_w_down: jax.Array,
):
    del B_x
    return _run(A_x, A_wqkv, A_wo, B_w_gate, B_w_up, B_w_down)
```

```python
import jax
import jax.numpy as jnp
import jax.experimental.pallas as pl
import jax.experimental.pallas.tpu as pltpu
from jax import lax

H = 32
W = 8
DIL = 2
EPS = 1e-5
LANES = 128

F32 = jnp.float32
BF16 = jnp.bfloat16
U32 = jnp.uint32

_NT = (((1,), (1,)), ((), ()))


def _tree_sum(parts, op=jnp.add):
    while len(parts) > 1:
        nxt = [op(parts[i], parts[i + 1]) for i in range(0, len(parts) - 1, 2)]
        if len(parts) % 2:
            nxt.append(parts[-1])
        parts = nxt
    return parts[0]


def _ln_stats(slabs, d, anchors=()):
    n_acc = 4
    s1, s2, pilot = [None] * n_acc, [None] * n_acc, None
    for i, x in enumerate(slabs):
        if pilot is None:
            pilot = x[0:1, :]
            pil = jnp.broadcast_to(pilot, x.shape)
            pils = [_tie(pil, a) for a in anchors] or [pil]
        dx = x - pils[i * len(pils) // (d // 8)]
        j = i % n_acc
        s1[j] = dx if s1[j] is None else s1[j] + dx
        s2[j] = dx * dx if s2[j] is None else s2[j] + dx * dx
    e1 = jnp.sum(_tree_sum(s1), axis=0, keepdims=True) * (1.0 / d)
    e2 = jnp.sum(_tree_sum(s2), axis=0, keepdims=True) * (1.0 / d)
    var = jnp.maximum(e2 - e1 * e1, 0.0)
    return pilot + e1, lax.rsqrt(var + EPS)


def _zero_like_dep(v):
    return (lax.bitcast_convert_type(v, U32) >> 31) >> 1


def _tie(x, anchor):
    if anchor is None:
        return x
    z = lax.bitcast_convert_type(_zero_like_dep(anchor), F32)
    z = jnp.concatenate([z] * -(-x.shape[1] // LANES), axis=1)[:, :x.shape[1]]
    if x.shape[0] == 8:
        return x + z
    return jnp.concatenate([x[:8] + z, x[8:]], axis=0)


def _gelu_mul2(g, u):
    c0 = 0.7978845608028654
    c1 = c0 * 0.044715
    t = jnp.tanh(g * (c0 + c1 * (g * g)))
    return (g * u) * (1.0 + t)


def _lo(x):
    return lax.bitcast_convert_type(x << 16, F32)


def _hi(x):
    return lax.bitcast_convert_type(x & jnp.uint32(0xFFFF0000), F32)


def _pk(x):
    return pltpu.bitcast(x.astype(BF16), U32)


def _upk(x):
    return pltpu.bitcast(x, BF16)


def _dot(a, b):
    return jnp.dot(a, b, preferred_element_type=F32)


def _dot_nt(a, b):
    return lax.dot_general(a, b, _NT, preferred_element_type=F32)


def _x_ops(x1, x2):
    d = [a - b for a, b in zip(x1, x2)]
    return [x1[0] + x2[1], x2[0] + x2[1], x1[0] + x1[1],
            d[1] + x1[2], x1[1] + x1[2], d[1] + d[2],
            d[0] - x2[2], d[0] + d[2], x2[0] + x2[2],
            x1[0], d[0], x2[1], d[1], x1[2], x2[2]]


def _x_rem(x1, x2):
    a, b, c = 0, 1, 2
    cat = lambda u, v: jnp.concatenate([u, v], axis=0)
    return [cat(x1[c], x2[b]), cat(x1[a], x1[b] - x2[b]), cat(x2[a], x2[c] - x1[c])]


_W_TERMS = {0: ((0, 1, 1), (1, 0, 1)), 3: ((1, 2, 1), (2, 1, 1)), 6: ((0, 2, 1), (2, 0, 1)),
            9: ((0, 0, 1), (0, 2, 1), (1, 0, -1)), 10: ((2, 0, 1), (0, 0, -1), (0, 1, -1)),
            11: ((1, 1, 1), (1, 2, 1), (0, 1, -1)), 12: ((1, 0, 1), (1, 1, 1), (2, 1, -1)),
            13: ((2, 0, 1), (2, 2, 1), (1, 2, -1)), 14: ((2, 1, 1), (2, 2, 1), (0, 2, -1)),
            1: ((0, 1, 1),), 2: ((1, 0, 1),), 4: ((1, 2, 1),), 5: ((2, 1, 1),),
            7: ((2, 0, 1),), 8: ((0, 2, 1),)}


def _w_sums(w):
    return [_signed(_W_TERMS[i], lambda k, j: w[k][j]) for i in _W_SUM]


_W_SUM = {0: 0, 3: 1, 6: 2, 9: 3, 10: 4, 11: 5, 12: 6, 13: 7, 14: 8}
_W_RAW = {1: (0, 1), 2: (1, 0), 4: (1, 2), 5: (2, 1), 7: (2, 0), 8: (0, 2)}
_PAIR_ORDER = (1, 2, 4, 5, 7, 8, 0, 3, 6)
_DIAG = {(0, 0): 9, (2, 0): 10, (0, 1): 11, (1, 1): 12, (1, 2): 13, (2, 2): 14}
_PAIR = {(0, 0): ((6, -1), (8, -1)), (1, 0): ((2, 1), (7, 1)), (2, 0): ((0, 1), (1, -1)),
         (0, 1): ((3, 1), (4, -1)), (1, 1): ((0, 1), (2, -1)), (2, 1): ((1, 1), (5, -1)),
         (0, 2): ((4, 1), (8, 1)), (1, 2): ((6, 1), (7, -1)), (2, 2): ((5, 1), (3, -1))}


def _column(t, base, j, skew=False):
    s = []
    for k in range(3):
        v = base[k]
        for i, sg in _PAIR[k, j]:
            v = t[i] if v is None else (v + t[i] if sg > 0 else v - t[i])
        s.append(v)
    if skew:
        return s[1] + s[0], s[2] + 0.5 * (s[0] - s[1])
    return s[1] + s[0], s[2] + s[0]


_SA = (((0, 0, 1), (1, 1, 1)), ((1, 0, 1), (1, 1, 1)), ((0, 0, 1),), ((1, 1, 1),),
       ((0, 0, 1), (0, 1, 1)), ((1, 0, 1), (0, 0, -1)), ((0, 1, 1), (1, 1, -1)))
_SB = (((0, 0, 1), (1, 1, 1)), ((0, 0, 1),), ((0, 1, 1), (1, 1, -1)), ((1, 0, 1), (0, 0, -1)),
       ((1, 1, 1),), ((0, 0, 1), (0, 1, 1)), ((1, 0, 1), (1, 1, 1)))
_SCOL = {2: 1, 3: 0, 5: 1, 6: 0}
_SGRP = ((1, 4, 0), (3, 6), (2, 5))


def _signed(terms, f):
    v = None
    for a, b, sg in terms:
        v = f(a, b) if v is None else (v + f(a, b) if sg > 0 else v - f(a, b))
    return v


def _s_out(m):
    return [[m[0] + m[3] - m[4] + m[6], m[2] + m[4]],
            [m[1] + m[3], m[0] - m[1] + m[2] + m[5]]]


def _make_kernel(S, D, F, TM, cfg):
    NB = S // TM
    NT = TM // LANES
    DH = D // H
    DP = DH // 2
    RP = D // 2
    NG = H // 8
    scale = float(DH) ** -0.5
    NU = 2 * NB
    TH = TM // 2
    TQ = TM // 4
    D2 = D // 2
    D3 = D // 3
    Q3 = D3 // 2
    KU = D // 9
    KR = 3 * LANES
    NQ = 6
    QR = 3 * D // NQ
    WQ = (0, 640, 1152, 3 * D)
    PW = 4 * LANES
    NP = F // PW
    AOFF, fill = {}, [0, 0]
    for key in [(m1, m2) for m1 in range(7) for m2 in range(7)]:
        c = int(fill[1] < fill[0])
        AOFF[key] = (fill[c], slice(c * LANES, (c + 1) * LANES))
        fill[c] += 48 if key[0] in _SCOL and key[1] in _SCOL else 32
    scopes = cfg['scopes']
    assert NG == 4 and NB & (NB - 1) == 0
    SEM_P = 4

    def kernel(x_hbm, wqkv_hbm, wo_hbm, wg_hbm, wu_hbm, wdt_hbm, out_hbm,
               xio_s, wqkv_v, wo_v, wg_v, wu_v, wdt_v, wt_s, wl_s,
               gu_s, ds_s, xmid_s, a_s, qkv_s, o_s, acc_s, h3_s, r_s,
               sem_i, sem_o):

        def wait(name, cps):
            if scopes:
                with jax.named_scope(name):
                    for cp in cps:
                        cp.wait()
            else:
                for cp in cps:
                    cp.wait()

        def cols(lo, n):
            if not isinstance(lo, int):
                lo = pl.multiple_of(lo, LANES)
            return pl.ds(lo, n)

        def rows8(lo, n=8):
            if not isinstance(lo, int):
                lo = pl.multiple_of(lo, 8)
            return pl.ds(lo, n)

        def out_copy(b):
            return pltpu.make_async_copy(
                xio_s.at[b], out_hbm.at[:, cols(b * TM, TM)], sem_o.at[0])

        def x_cp(b, sem):
            return pltpu.make_async_copy(x_hbm.at[:, cols(b * TM, TM)], xio_s.at[b],
                                         sem_i.at[sem])

        def wq_cp(i):
            sl = cols(WQ[i], WQ[i + 1] - WQ[i])
            return pltpu.make_async_copy(wqkv_hbm.at[:, sl], wqkv_v.at[:, sl],
                                         sem_i.at[1 + i])

        def piece_cp(src, dst, p, sem, c0=0, n=PW):
            return pltpu.make_async_copy(src.at[:, cols(p * PW + c0, n)],
                                         dst.at[p, :, pl.ds(c0, n)], sem_i.at[sem])

        def group_cp(p):
            sem = SEM_P + p
            cps = []
            if not (isinstance(p, int) and p == NP):
                cps += [piece_cp(wg_hbm, wg_v, p, sem), piece_cp(wu_hbm, wu_v, p, sem)]
            if not (isinstance(p, int) and p == 0):
                cps.append(piece_cp(wdt_hbm, wdt_v, p - 1, sem, 0, KR))
            if isinstance(p, int) and p == NP:
                cps += [piece_cp(wdt_hbm, wdt_v, q, sem, KR, LANES) for q in range(NP)]
            return cps

        lane = lax.broadcasted_iota(jnp.int32, (8, LANES), 1)
        cat0 = lambda *v: jnp.concatenate(v, axis=0)
        cat1 = lambda *v: jnp.concatenate(v, axis=1)

        def spread_over(anchors, n, total):
            return anchors[n * len(anchors) // total] if anchors else None

        def slab_group(r):
            return (r % LANES) // 16 if r < KR else 8 + ((r - KR) % KU) // 16

        def ln1(blk, anchors1, anchors2=()):
            slabs = (xio_s[blk, r:r + 8, :].astype(F32) for r in range(0, D, 8))
            m, rs = _ln_stats(slabs, D, anchors1)
            if not anchors2:
                return (xio_s[blk].astype(F32) - m) * rs
            m8 = jnp.broadcast_to(m, (8, TM))
            ms = [_tie(m8, a) for a in anchors2]
            ms = [spread_over(ms, slab_group(r), 12) for r in range(0, D, 8)]
            return (xio_s[blk].astype(F32) - cat0(*ms)) * rs

        def dot_k(rows, x, anchors, even=False):
            y = None
            for n, k in enumerate(range(0, D, LANES)):
                ks = slice(k, min(k + LANES, D))
                if even and k + LANES >= D:
                    mid = (rows.start + rows.stop) // 2
                    v = cat0(_dot(_upk(wt_s[rows.start:mid, ks]), x[ks]),
                             _dot(_upk(wt_s[mid:rows.stop, ks]), x[ks]))
                else:
                    v = _dot(_upk(wt_s[rows, ks]), x[ks])
                anchors.extend(v[r:r + 8, :LANES] for r in ((0, 144) if n % 2 else (72, 216)))
                y = v if y is None else y + v
            return y

        def put_qkv(blk, rows, y):
            pk = _pk(y)
            for c in range(NT):
                qkv_s[1 + blk * NT + c, rows, :] = pk[:, c * LANES:(c + 1) * LANES]

        def qkv_mm(blk, xn, chunks, anchors, even=False):
            for r in chunks:
                rows = slice(r * QR // 2, (r + 1) * QR // 2)
                put_qkv(blk, rows, dot_k(rows, xn, anchors, even))

        def split_k(x):
            hs = (x[:, :TH], x[:, TH:])
            blocks = [[h[k * LANES:(k + 1) * LANES] for k in range(3)] for h in hs]
            units = [[h[KR + k * KU:KR + (k + 1) * KU] for k in range(3)] for h in hs]
            return blocks, units

        def prep_att(pat, anchor):
            assert Q3 == 96
            row0 = pat * 8
            src0 = row0 + ((pat * 43) >> 9) * (2 * Q3)
            w = [_upk(wt_s[rows8(src0 + j * Q3), :D]).astype(F32) for j in range(3)]
            w[0] = cat1(_tie(w[0][:, :LANES], anchor), w[0][:, LANES:])
            tiles = _w_sums([[w[j][:, k * LANES:(k + 1) * LANES] for j in range(3)]
                             for k in range(3)])
            for j in range(3):
                a, b, c = (w[j][:, KR + k * KU:KR + (k + 1) * KU] for k in range(3))
                tiles += [cat1(c, b), cat1(a, c)]
            wl_s[rows8(row0), :15 * LANES] = _pk(cat1(*tiles))

        def att_rhs(x, stash=None, anchors=()):
            half = 0.5
            if anchors:
                hs = [_tie(jnp.full((8, TH), 0.5, F32), a) for a in anchors]
                half = cat0(*[spread_over(hs, slab_group(r), 12) for r in range(0, D, 8)])
            blocks, units = split_k(cat1(x[:, :TH], x[:, TH:] + half * x[:, :TH]))
            ops = _x_ops(*blocks) + _x_rem(*units)
            if stash is None:
                return [v.astype(BF16) for v in ops]
            loc = lambda i, r0, n: (slice((i // 2) * 64 + r0, (i // 2) * 64 + r0 + n),
                                    slice((i % 2) * LANES, (i % 2 + 1) * LANES))
            for r in range(0, LANES, 16):
                for i, v in enumerate(ops):
                    r_s.at[0][loc(i, r // 2, 8)] = _pk(v[r:r + 16])
            return [_upk(r_s.at[stash][loc(i, 0, 64)]) for i in range(18)]

        def att_mm(sec, rhs, anchors):
            tl = lambda i: _upk(wl_s[sec * Q3:(sec + 1) * Q3, i * LANES:(i + 1) * LANES])
            raw = lambda k, j: _upk(wt_s[(3 * sec + j) * Q3:(3 * sec + j + 1) * Q3,
                                         k * LANES:(k + 1) * LANES])
            t = {}
            for i in _PAIR_ORDER:
                t[i] = _dot(raw(*_W_RAW[i]) if i in _W_RAW else tl(_W_SUM[i]), rhs[i])
                anchors.append(t[i][:8])
            out = []
            for j in range(3):
                base = []
                for s in range(3):
                    v = _dot(raw(3, j) if s == 1 else tl(9 + 2 * j + s // 2), rhs[15 + s])
                    if (s, j) in _DIAG:
                        i = _DIAG[s, j]
                        v = _dot(tl(_W_SUM[i]), rhs[i]) + v
                    base.append(v)
                    anchors.append(base[-1][:8])
                out.append(cat1(*_column(t, base, j, True)))
            return cat0(*out)

        def qkv_fast(blk, rhs, anchors):
            for sec in range(3):
                put_qkv(blk, slice(sec * RP, (sec + 1) * RP), att_mm(sec, rhs, anchors))

        def shifted(ln, cur, prev, w):
            if w == 0:
                return cur
            sh = DIL * w
            return pltpu.roll(jnp.where(ln < LANES - sh, cur, prev), sh, axis=1)

        def att_group(blk, c, hg, anchor):
            att_values(blk, c, hg, anchor)(None)

        def att_values(blk, c, hg, anchor):
            tile = blk * NT + c
            base = hg * 8 * DP
            if isinstance(hg, int):
                cur, prev, o_t = qkv_s.at[1 + tile], qkv_s.at[tile], o_s.at[c]
            else:
                n = 2 * RP + 8 * DP
                base = pl.multiple_of(base, 8)
                cur = qkv_s.at[1 + tile, pl.ds(base, n)]
                prev = qkv_s.at[tile, pl.ds(base, n)]
                o_t = o_s.at[c, pl.ds(base, RP + 8 * DP)]
                base = 0
            ln = lane + _zero_like_dep(anchor).astype(jnp.int32)
            logits = [None] * W
            for dd in range(DP):
                q = cur[pl.ds(base + dd, 8, stride=DP), :]
                kc = cur[pl.ds(RP + base + dd, 8, stride=DP), :]
                kp = prev[pl.ds(RP + base + dd, 8, stride=DP), :]
                q0, q1 = _lo(q), _hi(q)
                for w in range(W):
                    ks = shifted(ln, kc, kp, w)
                    t = q0 * _lo(ks) + q1 * _hi(ks)
                    logits[w] = t if logits[w] is None else logits[w] + t
            logits = [l * scale for l in logits]
            if not (isinstance(c, int) and c > 0):
                pos = lane + tile * LANES
                logits = [l if w == 0 else jnp.where(pos >= DIL * w, l, -1e9)
                          for w, l in enumerate(logits)]
            m = _tree_sum(logits, jnp.maximum)
            p = [jnp.exp(l - m) for l in logits]
            r = 1.0 / _tree_sum(p)

            def apply(anchor2):
                ln = lane + _zero_like_dep(_tie(m, anchor2)).astype(jnp.int32)
                for dd in range(DP):
                    vc = cur[pl.ds(2 * RP + base + dd, 8, stride=DP), :]
                    vp = prev[pl.ds(2 * RP + base + dd, 8, stride=DP), :]
                    o0 = o1 = None
                    for w in range(W):
                        vs = shifted(ln, vc, vp, w)
                        t0, t1 = p[w] * _lo(vs), p[w] * _hi(vs)
                        o0 = t0 if o0 is None else o0 + t0
                        o1 = t1 if o1 is None else o1 + t1
                    o0, o1 = o0 * r, o1 * r
                    o_t[pl.ds(base + dd, 8, stride=DP), :] = o0
                    o_t[pl.ds(RP + base + dd, 8, stride=DP), :] = o1

            return apply

        def attention(blk, anchors):
            for c in range(NT):
                for hg in range(NG):
                    att_group(blk, c, hg, anchors[c * NG + hg])

        def wo_mm(blk, anchors, fast, stash=None, anchors_in=()):
            o = cat1(*[o_s[c] for c in range(NT)])
            if fast:
                y = att_mm(3, att_rhs(o, stash, anchors_in), anchors)
            else:
                o = o.astype(BF16)
                q = D2 // 2
                y = cat0(*[dot_k(slice(h * q, (h + 1) * q), o, anchors) for h in (6, 7)])
            xm = xio_s[blk].astype(F32) + y
            xmid_s[blk] = xm
            return _ln_stats((xm[r:r + 8] for r in range(0, D, 8)), D)

        def ffn_lhs(blk, stats, anchors):
            m, rs = stats
            m8 = jnp.broadcast_to(m, (8, TM))
            xt = []
            for k in range(5):
                mt = cat0(*[_tie(m8, spread_over(anchors[:2], k, 5))] * (KU // 8 if k == 4 else 16))
                x = (xmid_s[blk, k * LANES:min((k + 1) * LANES, D), :] - mt) * rs
                xt.append((cat0(x, x) if k == 4 else x).T)
            lo = lax.broadcasted_iota(jnp.int32, (TQ // 2, LANES), 1) < KU
            for m1 in range(7):
                a = spread_over(anchors[2:], m1, 7)
                blk1 = lambda i2, k2: _signed(_SA[m1], lambda i1, k1: _tie(
                    xt[k2 if k2 == 4 else 2 * k1 + k2][(2 * i1 + i2) * TQ:(2 * i1 + i2 + 1) * TQ], a))
                l1 = {(i2, k2): blk1(i2, k2) for i2 in range(2)
                      for k2 in ((0, 1, 4) if m1 in _SCOL else (0, 1))}
                for m2 in range(7):
                    v = _signed(_SA[m2], lambda i2, k2: l1[i2, k2])
                    if m1 in _SCOL and m2 in _SCOL:
                        c = _signed(_SA[m2], lambda i2, k2: l1[i2, 4])
                        h = TQ // 2
                        vp, vq, cp, cq = v[:h], v[h:], c[:h], c[h:]
                        v = cat0(jnp.where(lo, cp, vq), jnp.where(lo, vp, vp - vq),
                                 jnp.where(lo, vq, cq - cp))
                    o, ac = AOFF[m1, m2]
                    a_s[o:o + v.shape[0] // 2, ac] = _pk(v)

        def in_triple(q):
            return q, lambda k: (q, k)

        def cross_triple(s):
            return NP + s, lambda k: (3 * s + k, 3)

        def wd_raw(tri, k, r0, n):
            q, c = tri[1](k)
            return wdt_v[q, r0:r0 + n, c * LANES:(c + 1) * LANES]

        def ds_loc(i, r0, n):
            return slice(r0, r0 + n), slice((i % 2) * LANES, (i % 2 + 1) * LANES)

        def prep_d(tri, anchors):
            PR = 16
            for n in range(D3 // PR):
                r = n * PR
                w = [[wd_raw(tri, k, j * D3 + r, PR).astype(F32) for j in range(3)]
                     for k in range(3)]
                w[0][1] = _tie(w[0][1], spread_over(anchors, n, D3 // PR))
                for i, v in enumerate(_w_sums(w)):
                    ds_s.at[tri[0], i // 2][ds_loc(i, r // 2, PR // 2)] = _pk(v)

        GU = (wg_v, wu_v)

        def prep_gu(p, gv, m, m1s, anchors):
            PR = 16
            cs = slice(m * LANES, (m + 1) * LANES)
            for n in range(LANES // PR):
                r = n * PR
                cache = {}

                def w(k, j1):
                    if (k, j1) not in cache:
                        v = GU[m][p, k * LANES + r:k * LANES + r + PR,
                                  2 * j1 * LANES:2 * (j1 + 1) * LANES].astype(F32)
                        if (k // 2, j1) in [_SB[m1][0][:2] for m1 in m1s[:2]]:
                            a = spread_over(anchors, n, LANES // PR)
                            if cfg['tie1']:
                                c = (k % 2) * LANES
                                tied = _tie(v[:, c:c + LANES], a)
                                v = cat1(v[:, :LANES], tied) if c else cat1(tied, v[:, LANES:])
                            else:
                                v = _tie(v, a)
                        cache[k, j1] = v
                    return cache[k, j1]

                for m1 in m1s:
                    b1 = [_signed(_SB[m1], lambda k1, j1: w(2 * k1 + k2, j1)) for k2 in range(2)]
                    for m2 in range(7):
                        v = _signed(_SB[m2],
                                    lambda k2, j2: b1[k2][:, j2 * LANES:(j2 + 1) * LANES])
                        gv.at[7 * m1 + m2][r // 2:(r + PR) // 2, cs] = _pk(v)

        def prep_tail(p, gv, m, anchor):
            v = _tie(GU[m][p, 4 * LANES:, :].astype(F32), anchor)
            for j in range(4):
                gv.at[49 + j // 2][(j % 2) * 32:(j % 2 + 1) * 32,
                                        m * LANES:(m + 1) * LANES] = _pk(
                                            v[:, j * LANES:(j + 1) * LANES])

        def gu_outer(gv, m, m1, anchors, at=(0, 4)):
            cs = slice(m * LANES, (m + 1) * LANES)
            y = {}
            for m2 in cfg['inner']:
                i, (o, ac) = 7 * m1 + m2, AOFF[m1, m2]
                if m1 in _SCOL and m2 in _SCOL:
                    j = 2 * _SCOL[m1] + _SCOL[m2]
                    tail = lambda: gv[49 + j // 2, (j % 2) * 32:(j % 2 + 1) * 32, cs]
                    rhs = (cat0(tail(), gv[i, 32:, cs]), gv[i, :, cs],
                           cat0(gv[i, :32, cs], tail()))
                    r = [_dot(_upk(a_s[o + 16 * s:o + 16 * (s + 1), ac]), _upk(rhs[s]))
                         for s in range(3)]
                    y[m2] = cat0(r[1] + r[0], r[2] + r[0])
                else:
                    y[m2] = _dot(_upk(a_s[o:o + TQ // 2, ac]), _upk(gv[i, :, cs]))
            anchors.extend(y[cfg['inner'][k % 7]][(k // 7) * 32:(k // 7) * 32 + 8] for k in at)
            return _s_out(y)

        def gu_finish(t):
            gu = [{(i2, j2): _s_out([t[m][m1][i2][j2] for m1 in range(7)])
                   for i2 in range(2) for j2 in range(2)} for m in range(2)]
            return [[cat0(*[_gelu_mul2(*[gu[m][i2, j % 2][i1][j // 2] for m in range(2)])
                            for i2 in range(2)]) for i1 in range(2)] for j in range(4)]

        def gu_piece(gv, order, anchors, at=(0, 4)):
            t = ({}, {})
            for m, m1 in order:
                t[m][m1] = gu_outer(gv, m, m1, anchors, at)
            return gu_finish(t)

        def prep_piece(p, gv, anchors, group):
            grp = _SGRP if group else [(m1,) for m1 in range(7)]
            k = len(anchors) // (2 * len(grp))
            for n in range(2 * len(grp)):
                prep_gu(p, gv, n % 2, grp[n // 2], anchors[k * n:k * n + k])
            for m in range(2):
                prep_tail(p, gv, m, anchors[m * len(anchors) // 2])

        def h_ops(h):
            return [v.astype(BF16) for v in _x_ops(*[[h[k][i] for k in range(3)]
                                                     for i in range(2)])]

        D_ORDER = _PAIR_ORDER + (9, 10, 11, 12, 13, 14)

        def down_mm(acc, work, anchors, which=D_ORDER, fine=False):
            p = [None] * 15 if acc is None else list(acc)
            jobs = [(i, n) for i in which for n in range(len(work))]
            split = {0: (), 1: (4,), 2: (2, 2), 3: (2, 2, 4)}[len(jobs) % 4]
            split = dict(zip(jobs[len(jobs) - len(split):], split))
            for i in which:
                y = None
                for n, (tri, b) in enumerate(work):
                    ns = split.get((i, n), 1)
                    nr = D3 // ns
                    if i in _W_RAW:
                        k, j = _W_RAW[i]
                        lhs = lambda h: wd_raw(tri, k, j * D3 + h * nr, nr)
                    else:
                        s = _W_SUM[i]
                        lhs = lambda h: _upk(ds_s.at[tri[0], s // 2][ds_loc(s, h * nr // 2, nr // 2)])
                    v = cat0(*[_dot_nt(lhs(h), b[i]) for h in range(ns)])
                    y = v if y is None else y + v
                p[i] = y if p[i] is None else p[i] + y
                anchors.append(p[i][:8])
                if fine:
                    anchors.append(p[i][D3 // 2:D3 // 2 + 8])
            return p

        def finish(blk, acc):
            y = [cat1(*_column(acc, [acc[_DIAG[s, j]] if (s, j) in _DIAG else None
                                     for s in range(3)], j)) for j in range(3)]
            xio_s[blk] = (xmid_s[blk] + 0.5 * cat0(*y)).astype(BF16)

        def load_acc(k):
            return [acc_s[k, i] for i in range(15)]

        def store_acc(k, acc):
            for i in range(15):
                acc_s[k, i] = acc[i]

        def pre_phase():
            first = [[x_cp(0, 0)], [wq_cp(0)], [x_cp(1, 2), wq_cp(1)],
                     [wq_cp(2), pltpu.make_async_copy(wo_hbm, wo_v, sem_i.at[3])]]
            order = sum(first, [])
            for p in range(NP + 1):
                order += group_cp(p)
            xr_cp = [x_cp(b, SEM_P + NP + 1) for b in range(2, NB)]
            order += xr_cp
            for cp in order:
                cp.start()
            get = lambda an, name: [an[min(i, len(an) - 1)] for i in cfg[name]]
            e_grp = lambda e: ((e >> 1) & 1, ((e >> 2) << 1) | (e & 1))
            if 'a' in cfg['sub']:
                pre_a(first, get, e_grp)
            if 'b' in cfg['sub']:
                pre_b(get, e_grp)
            if 'c' in cfg['sub']:
                pre_c(get)
            wait('WX', xr_cp)

        def pre_a(first, get, e_grp):
            def transpose_wq(i):
                wt_s[WQ[i] // 2:WQ[i + 1] // 2, :D] = _pk(wqkv_v[:, WQ[i]:WQ[i + 1]].T)

            def clear(i, carry):
                for k in range(2):
                    acc_s[k, i] = jnp.zeros((D3, TH), F32)
                r = jnp.minimum(i, 11) * (RP // 4)
                qkv_s[0, rows8(r, RP // 4)] = jnp.zeros((RP // 4, LANES), U32)
                return carry

            lax.fori_loop(0, 15, clear, 0)
            wait('WX0', first[0])
            xn0 = ln1(0, ()).astype(BF16)

            wait('WQ0', first[1])
            transpose_wq(0)
            qkv_mm(0, xn0, (0, 1), [])

            wait('WQ1', first[2])
            transpose_wq(1)
            an = []
            qkv_mm(0, xn0, (2, 3), an)
            xn1 = ln1(1, get(an, 'a_ln'), get(an, 'a_lnb')).astype(BF16)
            qkv_mm(1, xn1, (0,), an, True)
            for n, a in enumerate(get(an, 'a_w1')):
                prep_att(n, a)
            nk = len(cfg['a_k'])
            apply = [att_values(0, *e_grp(e), a) for e, a in enumerate(get(an, 'a_k'))]

            wait('WQ2', first[3])
            an = []
            qkv_mm(1, xn1, (2,), an)
            transpose_wq(2)
            qkv_mm(0, xn0, (4, 5), an)
            qkv_mm(1, xn1, (4,), an)
            qkv_mm(1, xn1, (1,), an, True)
            apply += [att_values(0, *e_grp(nk + e), a)
                      for e, a in enumerate(get(an, 'a_k2')[:8 - nk])]
            for e, a in enumerate(get(an, 'a_v')):
                apply[e](a)
            wo = pltpu.bitcast(wo_v[...], U32)
            wo = cat0(_lo(wo), _hi(wo))
            wo = cat0(*[_tie(wo[n * LANES:(n + 1) * LANES], a)
                        for n, a in enumerate(get(an, 'a_wo'))])
            wt_s[3 * RP:, :D] = _pk(wo.astype(BF16).T)
            for n, a in enumerate(get(an, 'a_w2')):
                prep_att(len(cfg['a_w1']) + n, a)

            wait('WO', group_cp(0))
            an = []
            stats = wo_mm(0, an, False)
            qkv_mm(1, xn1, (3, 5), an)
            for n, a in enumerate(get(an, 'z_w')):
                prep_att(36 + n, a)
            prep_piece(0, gu_s.at[0], get(an, 'z_g'), cfg['z_grp'])
            ffn_lhs(0, stats, get(an, 'z_l'))

        def pre_b(get, e_grp):
            def piece(p, carry):
                wait('WP', group_cp(p))
                an = []
                win = gu_s.at[pl.ds(p - 1, 2)]
                h = gu_piece(win.at[0], cfg['gorder0'], an, (0, 7, 4, 11))
                h3_s[p - 1] = cat0(*h[3])
                tri = in_triple(p - 1)
                prep_d(tri, get(an, 'p_d'))
                store_acc(0, down_mm(load_acc(0), [(tri, h_ops(h[:3]))], an))
                prep_piece(p, win.at[1], get(an, 'f_g'), cfg['f_grp'])
                att_group(1, *e_grp(p - 1), an[cfg['p_att'][0]])
                return carry

            lax.fori_loop(1, NP, piece, 0)

        def pre_c(get):
            wait('WD', group_cp(NP))
            an = []
            h = gu_piece(gu_s.at[NP - 1], cfg['torder'], an)
            h3 = [[h3_s[q, :TH], h3_s[q, TH:]] for q in range(NP - 1)] + [h[3]]
            work = [(cross_triple(s), h_ops(h3[3 * s:3 * s + 3])) for s in range(3)]
            work.append((in_triple(NP - 1), h_ops(h[:3])))
            stats = wo_mm(1, an, True)
            td = get(an, 't_d')
            for n, (tri, _) in enumerate(work):
                prep_d(tri, td[n * len(td) // 4:(n + 1) * len(td) // 4])
            acc = down_mm(load_acc(0), work, an)
            nw = len(cfg['a_w1']) + len(cfg['a_w2'])
            for n, a in enumerate(get(an, 't_w')[:36 - nw]):
                prep_att(nw + n, a)
            ffn_lhs(1, stats, get(an, 't_l'))
            finish(0, acc)

        if 'pre' in cfg['phases']:
            pre_phase()

        def body(u, carry):
            bu = u & (NB - 1)
            ba = (u + 1) & (NB - 1)
            acc, stats, an, b, hh = None, None, {}, {}, {}
            get = lambda name: [an[k][i] for k, i in cfg[name]]
            for step in cfg['body']:
                an[step] = []
                if step == 'Q':
                    xn = ln1(ba, get('ln1'), get('ln1b'))
                    qkv_fast(ba, att_rhs(xn, u >> 8), an[step])
                elif step == 'W':
                    attention(ba, get('att'))
                    stats = wo_mm(ba, an[step], True, u >> 8, get('orhs'))
                elif step == 'L':
                    ffn_lhs(ba, stats, get('lhs'))
                elif step[0] == 'G':
                    q, go = int(step[1]), cfg['gorder']
                    t = b.setdefault(step[:2], ({}, {}))
                    for m, m1 in (go[:7] if step[2] == '0' else go[7:]):
                        t[m][m1] = gu_outer(gu_s.at[q], m, m1, an[step])
                    if len(t[0]) + len(t[1]) == 14:
                        hh[q] = gu_finish(t)
                else:
                    work = []
                    for c in step[1:]:
                        if c.isdigit():
                            work.append((in_triple(int(c)), h_ops(hh[int(c)][:3])))
                        else:
                            s = ord(c) - ord('a')
                            work.append((cross_triple(s),
                                         h_ops([hh[3 * s + k][3] for k in range(3)])))
                    acc = down_mm(acc, work, an[step])
            finish(bu, acc)

            @pl.when(u >= NB)
            def _():
                out_copy(bu).start()
            return carry

        if scopes:
            with jax.named_scope('LOOP'):
                lax.fori_loop(1, NU - 1, body, 0)
        elif 'main' in cfg['phases']:
            lax.fori_loop(1, NU - 1, body, 0)

        def last(s, carry):
            h = [gu_piece(gu_s.at[3 * s + k], cfg['lorder'], []) for k in range(3)]
            work = [(in_triple(3 * s + k), h_ops(h[k][:3])) for k in range(3)]
            work.append((cross_triple(s), h_ops([h[k][3] for k in range(3)])))
            acc = down_mm(down_mm(load_acc(1), work[:2], []), work[2:], [])
            store_acc(1, acc)
            finish(NB - 1, acc)
            return carry

        if 'last' in cfg['phases']:
            lax.fori_loop(0, NP // 3, last, 0)
        if len(cfg['phases']) < 3:
            def keep(i, c):
                v = (gu_s[i, i, :8, :LANES] + ds_s[i, i, :8, :LANES]
                     + wl_s[rows8(i * 8), :LANES] + a_s[rows8(i * 8), :LANES] + qkv_s[i, :8]
                     + wt_s[rows8(i * 8), :LANES])
                acc_s[1, 0, :8] = (lax.bitcast_convert_type(v, F32) + o_s[i, :8]
                                   + acc_s[i, i, :8] + h3_s[i, :8])
                return c
            lax.fori_loop(0, 2, keep, 0)
            finish(NB - 1, load_acc(1))
        out_copy(NB - 1).start()
        wait('WOUT', [out_copy(b) for b in range(NB)])

    scratch = [
        pltpu.VMEM((NB, D, TM), BF16),
        pltpu.VMEM((D, 3 * D), BF16),
        pltpu.VMEM((D, D), BF16),
        pltpu.VMEM((NP, D, PW), BF16),
        pltpu.VMEM((NP, D, PW), BF16),
        pltpu.VMEM((NP, D, PW), BF16),
        pltpu.VMEM((2 * D, 8 * LANES), U32),
        pltpu.VMEM((4 * Q3, 16 * LANES), U32),
        pltpu.VMEM((NP, 51, 64, 2 * LANES), U32),
        pltpu.VMEM((NP + 3, 5, Q3, 2 * LANES), U32),
        pltpu.VMEM((NB, D, TM), F32),
        pltpu.VMEM((max(fill), 2 * LANES), U32),
        pltpu.VMEM((S // LANES + 1, 3 * RP, LANES), U32),
        pltpu.VMEM((NT, D, LANES), F32),
        pltpu.VMEM((2, 15, D3, TH), F32),
        pltpu.VMEM((NP, TM, LANES), F32),
        pltpu.VMEM((1, 9 * 64, 2 * LANES), U32),
        pltpu.SemaphoreType.DMA((SEM_P + NP + 2,)),
        pltpu.SemaphoreType.DMA((1,)),
    ]

    def wrapped(*refs):
        @pl.when(pl.program_id(0) == 0)
        def _():
            kernel(*refs)

    return wrapped, scratch


_CFG = dict(
    scopes=False,
    tie1=True,
    orhs=(('G80', 0), ('G80', 1), ('G80', 2), ('G80', 3), ('G80', 4), ('G80', 5),
        ('G80', 6), ('G80', 7), ('G80', 8), ('G80', 9), ('G80', 10), ('G80', 11)),
    sub='abc',
    phases=('pre', 'main', 'last'),
    body=('G20', 'G00', 'G01', 'G10', 'G11', 'Q', 'G30', 'G21', 'G40', 'G31', 'G50',
        'D012a', 'G41', 'G51', 'D345b', 'G70', 'G60', 'G71', 'G80', 'W', 'G61', 'G81',
        'D8c', 'D67', 'L'),
    ln1=(('G00', 0), ('G00', 1), ('G00', 2), ('G00', 3), ('G00', 4), ('G00', 5), ('G00',
        6), ('G00', 7), ('G00', 8)),
    ln1b=(('G10', 1), ('G10', 2), ('G10', 3), ('G10', 4), ('G10', 5), ('G10', 6),
        ('G10', 7), ('G10', 8), ('G10', 9), ('G10', 10), ('G10', 11), ('G10', 12)),
    att=(('D012a', 2), ('D012a', 4), ('D012a', 5), ('D012a', 8), ('D012a', 9), ('D345b',
        5), ('D345b', 6), ('D345b', 8)),
    lhs=(('D8c', 2), ('D8c', 3), ('D8c', 9), ('D8c', 11), ('D67', 5), ('D67', 8),
        ('D67', 10), ('D67', 11), ('D67', 14)),
    a_w1=(0, 0, 1, 2, 2, 3, 3, 4, 5, 6, 7, 11, 13, 18, 19, 20, 21, 22, 23, 24, 26, 27,
        28, 29),
    a_w2=(25, 30, 33, 36, 44, 45),
    a_ln=(3, 6, 7),
    a_lnb=(3, 9, 15),
    z_g=(0, 0, 1, 1, 2, 2, 3, 3, 4, 4, 5, 5, 6, 6, 7, 7, 8, 8, 9, 11, 12, 12, 13, 14,
        14, 14, 15, 15, 16, 16, 17, 17, 18, 18, 19, 19, 20, 21, 21, 22, 23, 23, 23, 24,
        25, 26, 27, 33),
    t_d=(0, 0, 0, 2, 2, 4, 5, 5, 7, 7, 8, 8, 9, 10, 11, 11, 12, 12, 13, 14, 14, 15, 16,
        16, 17, 17, 18, 18, 21, 22, 24, 24, 25, 28, 28, 30, 32, 32, 35, 35, 36, 37, 37,
        37, 39, 40, 40, 42),
    p_d=(3, 12, 14, 17, 24, 25, 28, 33, 35, 38, 42, 46),
    p_att=(58,),
    z_l=(23, 23, 28, 31, 35, 36, 37, 37, 39),
    a_k=(13, 17, 20, 26),
    a_k2=(0, 1, 3, 9),
    a_v=(13, 13, 14, 15, 16, 17, 18, 19),
    a_wo=(9, 18, 25, 36, 46),
    inner=(0, 3, 4, 6, 2, 1, 5),
    gorder=((0, 4), (0, 0), (1, 4), (1, 0), (1, 6), (0, 3), (1, 3), (0, 6), (0, 1), (1,
        1), (0, 2), (1, 2), (0, 5), (1, 5)),
    gorder0=((0, 0), (1, 4), (0, 4), (1, 0), (0, 3), (0, 6), (1, 6), (1, 3), (1, 1), (0,
        1), (0, 2), (0, 5), (1, 5), (1, 2)),
    f_g=(0, 0, 1, 2, 5, 5, 6, 7, 8, 9, 9, 10, 12, 13, 14, 16, 17, 17, 19, 20, 21, 23,
        24, 24, 26, 28, 29, 31, 32, 35, 36, 37, 37, 40, 40, 42, 43, 44, 45, 47, 48, 48,
        53, 56, 58, 59, 60, 61, 62, 62, 64, 64, 69, 70, 70, 70),
    t_l=(49, 50, 51, 53, 54, 55, 57, 57, 60),
    lorder=((1, 0), (1, 4), (0, 0), (0, 4), (0, 3), (0, 6), (1, 3), (1, 6), (0, 1), (1,
        1), (0, 2), (0, 5), (1, 2), (1, 5)),
    z_w=(1, 1, 3, 3, 5, 5, 6, 6, 8, 9, 17, 35),
    z_grp=1,
    f_grp=0,
    t_w=(47, 49, 49, 50, 52, 54),
    torder=((0, 0), (0, 4), (1, 4), (1, 0), (0, 3), (1, 3), (1, 6), (0, 6), (0, 1), (1,
        1), (0, 2), (1, 2), (0, 5), (1, 5)),
)


def _run(A_x, A_wqkv, A_wo, B_w_gate, B_w_up, B_w_down, **kw):
    _, S, D = A_x.shape
    F = B_w_gate.shape[1]
    kernel, scratch = _make_kernel(S, D, F, 256, {**_CFG, **kw})
    hbm = pl.BlockSpec(memory_space=pl.ANY)
    out_t = pl.pallas_call(
        kernel,
        grid=(2,),
        in_specs=[hbm] * 6,
        out_specs=hbm,
        out_shape=jax.ShapeDtypeStruct((D, S), A_x.dtype),
        scratch_shapes=scratch,
        compiler_params=pltpu.CompilerParams(
            dimension_semantics=('arbitrary',), vmem_limit_bytes=110 * 1024 * 1024),
    )(A_x.reshape(S, D).T, A_wqkv, A_wo, B_w_gate, B_w_up, B_w_down.T)
    return out_t.T.reshape(A_x.shape)


@jax.jit
def pallas_interleave_layers__sliding_local_dilated__glu_gated_geglu__prompt_kernel(
    A_x: jax.Array,
    A_wqkv: jax.Array,
    A_wo: jax.Array,
    B_x: jax.Array,
    B_w_gate: jax.Array,
    B_w_up: jax.Array,
    B_w_down: jax.Array,
):
    del B_x
    return _run(A_x, A_wqkv, A_wo, B_w_gate, B_w_up, B_w_down)
```

```python
import jax
import jax.numpy as jnp
import jax.experimental.pallas as pl
import jax.experimental.pallas.tpu as pltpu
from jax import lax

H = 32
W = 8
DIL = 2
EPS = 1e-5
LANES = 128

F32 = jnp.float32
BF16 = jnp.bfloat16
U32 = jnp.uint32

_NT = (((1,), (1,)), ((), ()))


def _tree_sum(parts, op=jnp.add):
    while len(parts) > 1:
        nxt = [op(parts[i], parts[i + 1]) for i in range(0, len(parts) - 1, 2)]
        if len(parts) % 2:
            nxt.append(parts[-1])
        parts = nxt
    return parts[0]


def _ln_stats(slabs, d, anchors=()):
    n_acc = 4
    s1, s2, pilot = [None] * n_acc, [None] * n_acc, None
    for i, x in enumerate(slabs):
        if pilot is None:
            pilot = x[0:1, :]
            pil = jnp.broadcast_to(pilot, x.shape)
            pils = [_tie(pil, a) for a in anchors] or [pil]
        dx = x - pils[i * len(pils) // (d // 8)]
        j = i % n_acc
        s1[j] = dx if s1[j] is None else s1[j] + dx
        s2[j] = dx * dx if s2[j] is None else s2[j] + dx * dx
    e1 = jnp.sum(_tree_sum(s1), axis=0, keepdims=True) * (1.0 / d)
    e2 = jnp.sum(_tree_sum(s2), axis=0, keepdims=True) * (1.0 / d)
    var = jnp.maximum(e2 - e1 * e1, 0.0)
    return pilot + e1, lax.rsqrt(var + EPS)


def _zero_like_dep(v):
    return (lax.bitcast_convert_type(v, U32) >> 31) >> 1


def _tie(x, anchor):
    if anchor is None:
        return x
    z = lax.bitcast_convert_type(_zero_like_dep(anchor), F32)
    z = jnp.concatenate([z] * -(-x.shape[1] // LANES), axis=1)[:, :x.shape[1]]
    if x.shape[0] == 8:
        return x + z
    return jnp.concatenate([x[:8] + z, x[8:]], axis=0)


def _gelu_mul2(g, u):
    c0 = 0.7978845608028654
    c1 = c0 * 0.044715
    t = jnp.tanh(g * (c0 + c1 * (g * g)))
    return (g * u) * (1.0 + t)


def _lo(x):
    return lax.bitcast_convert_type(x << 16, F32)


def _hi(x):
    return lax.bitcast_convert_type(x & jnp.uint32(0xFFFF0000), F32)


def _pk(x):
    return pltpu.bitcast(x.astype(BF16), U32)


def _upk(x):
    return pltpu.bitcast(x, BF16)


def _dot(a, b):
    return jnp.dot(a, b, preferred_element_type=F32)


def _dot_nt(a, b):
    return lax.dot_general(a, b, _NT, preferred_element_type=F32)


def _x_ops(x1, x2):
    d = [a - b for a, b in zip(x1, x2)]
    return [x1[0] + x2[1], x2[0] + x2[1], x1[0] + x1[1],
            d[1] + x1[2], x1[1] + x1[2], d[1] + d[2],
            d[0] - x2[2], d[0] + d[2], x2[0] + x2[2],
            x1[0], d[0], x2[1], d[1], x1[2], x2[2]]


def _x_rem(x1, x2):
    a, b, c = 0, 1, 2
    cat = lambda u, v: jnp.concatenate([u, v], axis=0)
    return [cat(x1[c], x2[b]), cat(x1[a], x1[b] - x2[b]), cat(x2[a], x2[c] - x1[c])]


_W_TERMS = {0: ((0, 1, 1), (1, 0, 1)), 3: ((1, 2, 1), (2, 1, 1)), 6: ((0, 2, 1), (2, 0, 1)),
            9: ((0, 0, 1), (0, 2, 1), (1, 0, -1)), 10: ((2, 0, 1), (0, 0, -1), (0, 1, -1)),
            11: ((1, 1, 1), (1, 2, 1), (0, 1, -1)), 12: ((1, 0, 1), (1, 1, 1), (2, 1, -1)),
            13: ((2, 0, 1), (2, 2, 1), (1, 2, -1)), 14: ((2, 1, 1), (2, 2, 1), (0, 2, -1)),
            1: ((0, 1, 1),), 2: ((1, 0, 1),), 4: ((1, 2, 1),), 5: ((2, 1, 1),),
            7: ((2, 0, 1),), 8: ((0, 2, 1),)}


def _w_sums(w):
    return [_signed(_W_TERMS[i], lambda k, j: w[k][j]) for i in _W_SUM]


_W_SUM = {0: 0, 3: 1, 6: 2, 9: 3, 10: 4, 11: 5, 12: 6, 13: 7, 14: 8}
_W_RAW = {1: (0, 1), 2: (1, 0), 4: (1, 2), 5: (2, 1), 7: (2, 0), 8: (0, 2)}
_PAIR_ORDER = (1, 2, 4, 5, 7, 8, 0, 3, 6)
_DIAG = {(0, 0): 9, (2, 0): 10, (0, 1): 11, (1, 1): 12, (1, 2): 13, (2, 2): 14}
_PAIR = {(0, 0): ((6, -1), (8, -1)), (1, 0): ((2, 1), (7, 1)), (2, 0): ((0, 1), (1, -1)),
         (0, 1): ((3, 1), (4, -1)), (1, 1): ((0, 1), (2, -1)), (2, 1): ((1, 1), (5, -1)),
         (0, 2): ((4, 1), (8, 1)), (1, 2): ((6, 1), (7, -1)), (2, 2): ((5, 1), (3, -1))}


def _column(t, base, j, skew=False):
    s = []
    for k in range(3):
        v = base[k]
        for i, sg in _PAIR[k, j]:
            v = t[i] if v is None else (v + t[i] if sg > 0 else v - t[i])
        s.append(v)
    if skew:
        return s[1] + s[0], s[2] + 0.5 * (s[0] - s[1])
    return s[1] + s[0], s[2] + s[0]


_SA = (((0, 0, 1), (1, 1, 1)), ((1, 0, 1), (1, 1, 1)), ((0, 0, 1),), ((1, 1, 1),),
       ((0, 0, 1), (0, 1, 1)), ((1, 0, 1), (0, 0, -1)), ((0, 1, 1), (1, 1, -1)))
_SB = (((0, 0, 1), (1, 1, 1)), ((0, 0, 1),), ((0, 1, 1), (1, 1, -1)), ((1, 0, 1), (0, 0, -1)),
       ((1, 1, 1),), ((0, 0, 1), (0, 1, 1)), ((1, 0, 1), (1, 1, 1)))
_SCOL = {2: 1, 3: 0, 5: 1, 6: 0}
_SGRP = ((1, 4, 0), (3, 6), (2, 5))


def _signed(terms, f):
    v = None
    for a, b, sg in terms:
        v = f(a, b) if v is None else (v + f(a, b) if sg > 0 else v - f(a, b))
    return v


def _s_out(m):
    return [[m[0] + m[3] - m[4] + m[6], m[2] + m[4]],
            [m[1] + m[3], m[0] - m[1] + m[2] + m[5]]]


def _make_kernel(S, D, F, TM, cfg):
    NB = S // TM
    NT = TM // LANES
    DH = D // H
    DP = DH // 2
    RP = D // 2
    NG = H // 8
    scale = float(DH) ** -0.5
    NU = 2 * NB
    TH = TM // 2
    TQ = TM // 4
    D2 = D // 2
    D3 = D // 3
    Q3 = D3 // 2
    KU = D // 9
    KR = 3 * LANES
    NQ = 6
    QR = 3 * D // NQ
    WQ = (0, 640, 1152, 3 * D)
    PW = 4 * LANES
    NP = F // PW
    AOFF, fill = {}, [0, 0]
    for key in [(m1, m2) for m1 in range(7) for m2 in range(7)]:
        c = int(fill[1] < fill[0])
        AOFF[key] = (fill[c], slice(c * LANES, (c + 1) * LANES))
        fill[c] += 48 if key[0] in _SCOL and key[1] in _SCOL else 32
    scopes = cfg['scopes']
    assert NG == 4 and NB & (NB - 1) == 0
    SEM_P = 4

    def kernel(x_hbm, wqkv_hbm, wo_hbm, wg_hbm, wu_hbm, wdt_hbm, out_hbm,
               xio_s, wqkv_v, wo_v, wg_v, wu_v, wdt_v, wt_s, wl_s,
               gu_s, ds_s, xmid_s, a_s, qkv_s, o_s, acc_s, h3_s, r_s,
               sem_i, sem_o):

        def wait(name, cps):
            if scopes:
                with jax.named_scope(name):
                    for cp in cps:
                        cp.wait()
            else:
                for cp in cps:
                    cp.wait()

        def cols(lo, n):
            if not isinstance(lo, int):
                lo = pl.multiple_of(lo, LANES)
            return pl.ds(lo, n)

        def rows8(lo, n=8):
            if not isinstance(lo, int):
                lo = pl.multiple_of(lo, 8)
            return pl.ds(lo, n)

        def out_copy(b):
            return pltpu.make_async_copy(
                xio_s.at[b], out_hbm.at[:, cols(b * TM, TM)], sem_o.at[0])

        def x_cp(b, sem):
            return pltpu.make_async_copy(x_hbm.at[:, cols(b * TM, TM)], xio_s.at[b],
                                         sem_i.at[sem])

        def wq_cp(i):
            sl = cols(WQ[i], WQ[i + 1] - WQ[i])
            return pltpu.make_async_copy(wqkv_hbm.at[:, sl], wqkv_v.at[:, sl],
                                         sem_i.at[1 + i])

        def piece_cp(src, dst, p, sem, c0=0, n=PW):
            return pltpu.make_async_copy(src.at[:, cols(p * PW + c0, n)],
                                         dst.at[p, :, pl.ds(c0, n)], sem_i.at[sem])

        def group_cp(p):
            sem = SEM_P + p
            cps = []
            if not (isinstance(p, int) and p == NP):
                cps += [piece_cp(wg_hbm, wg_v, p, sem), piece_cp(wu_hbm, wu_v, p, sem)]
            if not (isinstance(p, int) and p == 0):
                cps.append(piece_cp(wdt_hbm, wdt_v, p - 1, sem, 0, KR))
            if isinstance(p, int) and p == NP:
                cps += [piece_cp(wdt_hbm, wdt_v, q, sem, KR, LANES) for q in range(NP)]
            return cps

        lane = lax.broadcasted_iota(jnp.int32, (8, LANES), 1)
        cat0 = lambda *v: jnp.concatenate(v, axis=0)
        cat1 = lambda *v: jnp.concatenate(v, axis=1)

        def spread_over(anchors, n, total):
            return anchors[n * len(anchors) // total] if anchors else None

        def slab_group(r):
            return (r % LANES) // 16 if r < KR else 8 + ((r - KR) % KU) // 16

        def ln1(blk, anchors1, anchors2=()):
            slabs = (xio_s[blk, r:r + 8, :].astype(F32) for r in range(0, D, 8))
            m, rs = _ln_stats(slabs, D, anchors1)
            if not anchors2:
                return (xio_s[blk].astype(F32) - m) * rs
            m8 = jnp.broadcast_to(m, (8, TM))
            ms = [_tie(m8, a) for a in anchors2]
            ms = [spread_over(ms, slab_group(r), 12) for r in range(0, D, 8)]
            return (xio_s[blk].astype(F32) - cat0(*ms)) * rs

        def dot_k(rows, x, anchors, even=False):
            y = None
            for n, k in enumerate(range(0, D, LANES)):
                ks = slice(k, min(k + LANES, D))
                if even and k + LANES >= D:
                    mid = (rows.start + rows.stop) // 2
                    v = cat0(_dot(_upk(wt_s[rows.start:mid, ks]), x[ks]),
                             _dot(_upk(wt_s[mid:rows.stop, ks]), x[ks]))
                else:
                    v = _dot(_upk(wt_s[rows, ks]), x[ks])
                anchors.extend(v[r:r + 8, :LANES] for r in ((0, 144) if n % 2 else (72, 216)))
                y = v if y is None else y + v
            return y

        def put_qkv(blk, rows, y):
            pk = _pk(y)
            for c in range(NT):
                qkv_s[1 + blk * NT + c, rows, :] = pk[:, c * LANES:(c + 1) * LANES]

        def qkv_mm(blk, xn, chunks, anchors, even=False):
            for r in chunks:
                rows = slice(r * QR // 2, (r + 1) * QR // 2)
                put_qkv(blk, rows, dot_k(rows, xn, anchors, even))

        def split_k(x):
            hs = (x[:, :TH], x[:, TH:])
            blocks = [[h[k * LANES:(k + 1) * LANES] for k in range(3)] for h in hs]
            units = [[h[KR + k * KU:KR + (k + 1) * KU] for k in range(3)] for h in hs]
            return blocks, units

        def prep_att(pat, anchor):
            assert Q3 == 96
            row0 = pat * 8
            src0 = row0 + ((pat * 43) >> 9) * (2 * Q3)
            w = [_upk(wt_s[rows8(src0 + j * Q3), :D]).astype(F32) for j in range(3)]
            w[0] = cat1(_tie(w[0][:, :LANES], anchor), w[0][:, LANES:])
            tiles = _w_sums([[w[j][:, k * LANES:(k + 1) * LANES] for j in range(3)]
                             for k in range(3)])
            for j in range(3):
                a, b, c = (w[j][:, KR + k * KU:KR + (k + 1) * KU] for k in range(3))
                tiles += [cat1(c, b), cat1(a, c)]
            wl_s[rows8(row0), :15 * LANES] = _pk(cat1(*tiles))

        def att_rhs(x, stash=None, anchors=()):
            half = 0.5
            if anchors:
                hs = [_tie(jnp.full((8, TH), 0.5, F32), a) for a in anchors]
                half = cat0(*[spread_over(hs, slab_group(r), 12) for r in range(0, D, 8)])
            blocks, units = split_k(cat1(x[:, :TH], x[:, TH:] + half * x[:, :TH]))
            ops = _x_ops(*blocks) + _x_rem(*units)
            if stash is None:
                return [v.astype(BF16) for v in ops]
            loc = lambda i, r0, n: (slice((i // 2) * 64 + r0, (i // 2) * 64 + r0 + n),
                                    slice((i % 2) * LANES, (i % 2 + 1) * LANES))
            for r in range(0, LANES, 16):
                for i, v in enumerate(ops):
                    r_s.at[0][loc(i, r // 2, 8)] = _pk(v[r:r + 16])
            return [_upk(r_s.at[stash][loc(i, 0, 64)]) for i in range(18)]

        def att_mm(sec, rhs, anchors):
            tl = lambda i: _upk(wl_s[sec * Q3:(sec + 1) * Q3, i * LANES:(i + 1) * LANES])
            raw = lambda k, j: _upk(wt_s[(3 * sec + j) * Q3:(3 * sec + j + 1) * Q3,
                                         k * LANES:(k + 1) * LANES])
            t = {}
            for i in _PAIR_ORDER:
                t[i] = _dot(raw(*_W_RAW[i]) if i in _W_RAW else tl(_W_SUM[i]), rhs[i])
                anchors.append(t[i][:8])
            out = []
            for j in range(3):
                base = []
                for s in range(3):
                    v = _dot(raw(3, j) if s == 1 else tl(9 + 2 * j + s // 2), rhs[15 + s])
                    if (s, j) in _DIAG:
                        i = _DIAG[s, j]
                        v = _dot(tl(_W_SUM[i]), rhs[i]) + v
                    base.append(v)
                    anchors.append(base[-1][:8])
                out.append(cat1(*_column(t, base, j, True)))
            return cat0(*out)

        def qkv_fast(blk, rhs, anchors):
            for sec in range(3):
                put_qkv(blk, slice(sec * RP, (sec + 1) * RP), att_mm(sec, rhs, anchors))

        def shifted(ln, cur, prev, w):
            if w == 0:
                return cur
            sh = DIL * w
            return pltpu.roll(jnp.where(ln < LANES - sh, cur, prev), sh, axis=1)

        def att_group(blk, c, hg, anchor):
            att_values(blk, c, hg, anchor)(None)

        def att_values(blk, c, hg, anchor):
            tile = blk * NT + c
            base = hg * 8 * DP
            if isinstance(hg, int):
                cur, prev, o_t = qkv_s.at[1 + tile], qkv_s.at[tile], o_s.at[c]
            else:
                n = 2 * RP + 8 * DP
                base = pl.multiple_of(base, 8)
                cur = qkv_s.at[1 + tile, pl.ds(base, n)]
                prev = qkv_s.at[tile, pl.ds(base, n)]
                o_t = o_s.at[c, pl.ds(base, RP + 8 * DP)]
                base = 0
            ln = lane + _zero_like_dep(anchor).astype(jnp.int32)
            logits = [None] * W
            for dd in range(DP):
                q = cur[pl.ds(base + dd, 8, stride=DP), :]
                kc = cur[pl.ds(RP + base + dd, 8, stride=DP), :]
                kp = prev[pl.ds(RP + base + dd, 8, stride=DP), :]
                q0, q1 = _lo(q), _hi(q)
                for w in range(W):
                    ks = shifted(ln, kc, kp, w)
                    t = q0 * _lo(ks) + q1 * _hi(ks)
                    logits[w] = t if logits[w] is None else logits[w] + t
            logits = [l * scale for l in logits]
            if not (isinstance(c, int) and c > 0):
                pos = lane + tile * LANES
                logits = [l if w == 0 else jnp.where(pos >= DIL * w, l, -1e9)
                          for w, l in enumerate(logits)]
            m = _tree_sum(logits, jnp.maximum)
            p = [jnp.exp(l - m) for l in logits]
            r = 1.0 / _tree_sum(p)

            def apply(anchor2):
                ln = lane + _zero_like_dep(_tie(m, anchor2)).astype(jnp.int32)
                for dd in range(DP):
                    vc = cur[pl.ds(2 * RP + base + dd, 8, stride=DP), :]
                    vp = prev[pl.ds(2 * RP + base + dd, 8, stride=DP), :]
                    o0 = o1 = None
                    for w in range(W):
                        vs = shifted(ln, vc, vp, w)
                        t0, t1 = p[w] * _lo(vs), p[w] * _hi(vs)
                        o0 = t0 if o0 is None else o0 + t0
                        o1 = t1 if o1 is None else o1 + t1
                    o0, o1 = o0 * r, o1 * r
                    o_t[pl.ds(base + dd, 8, stride=DP), :] = o0
                    o_t[pl.ds(RP + base + dd, 8, stride=DP), :] = o1

            return apply

        def attention(blk, anchors):
            for c in range(NT):
                for hg in range(NG):
                    att_group(blk, c, hg, anchors[c * NG + hg])

        def wo_mm(blk, anchors, fast, stash=None, anchors_in=()):
            o = cat1(*[o_s[c] for c in range(NT)])
            if fast:
                y = att_mm(3, att_rhs(o, stash, anchors_in), anchors)
            else:
                o = o.astype(BF16)
                q = D2 // 2
                y = cat0(*[dot_k(slice(h * q, (h + 1) * q), o, anchors) for h in (6, 7)])
            xm = xio_s[blk].astype(F32) + y
            xmid_s[blk] = xm
            return _ln_stats((xm[r:r + 8] for r in range(0, D, 8)), D)

        def ffn_lhs(blk, stats, anchors):
            m, rs = stats
            m8 = jnp.broadcast_to(m, (8, TM))
            xt = []
            for k in range(5):
                mt = cat0(*[_tie(m8, spread_over(anchors[:2], k, 5))] * (KU // 8 if k == 4 else 16))
                x = (xmid_s[blk, k * LANES:min((k + 1) * LANES, D), :] - mt) * rs
                xt.append((cat0(x, x) if k == 4 else x).T)
            lo = lax.broadcasted_iota(jnp.int32, (TQ // 2, LANES), 1) < KU
            for m1 in range(7):
                a = spread_over(anchors[2:], m1, 7)
                blk1 = lambda i2, k2: _signed(_SA[m1], lambda i1, k1: _tie(
                    xt[k2 if k2 == 4 else 2 * k1 + k2][(2 * i1 + i2) * TQ:(2 * i1 + i2 + 1) * TQ], a))
                l1 = {(i2, k2): blk1(i2, k2) for i2 in range(2)
                      for k2 in ((0, 1, 4) if m1 in _SCOL else (0, 1))}
                for m2 in range(7):
                    v = _signed(_SA[m2], lambda i2, k2: l1[i2, k2])
                    if m1 in _SCOL and m2 in _SCOL:
                        c = _signed(_SA[m2], lambda i2, k2: l1[i2, 4])
                        h = TQ // 2
                        vp, vq, cp, cq = v[:h], v[h:], c[:h], c[h:]
                        v = cat0(jnp.where(lo, cp, vq), jnp.where(lo, vp, vp - vq),
                                 jnp.where(lo, vq, cq - cp))
                    o, ac = AOFF[m1, m2]
                    a_s[o:o + v.shape[0] // 2, ac] = _pk(v)

        def in_triple(q):
            return q, lambda k: (q, k)

        def cross_triple(s):
            return NP + s, lambda k: (3 * s + k, 3)

        def wd_raw(tri, k, r0, n):
            q, c = tri[1](k)
            return wdt_v[q, r0:r0 + n, c * LANES:(c + 1) * LANES]

        def ds_loc(i, r0, n):
            return slice(r0, r0 + n), slice((i % 2) * LANES, (i % 2 + 1) * LANES)

        def prep_d(tri, anchors):
            PR = 16
            for n in range(D3 // PR):
                r = n * PR
                w = [[wd_raw(tri, k, j * D3 + r, PR).astype(F32) for j in range(3)]
                     for k in range(3)]
                w[0][1] = _tie(w[0][1], spread_over(anchors, n, D3 // PR))
                for i, v in enumerate(_w_sums(w)):
                    ds_s.at[tri[0], i // 2][ds_loc(i, r // 2, PR // 2)] = _pk(v)

        GU = (wg_v, wu_v)

        def prep_gu(p, gv, m, m1s, anchors):
            PR = 16
            cs = slice(m * LANES, (m + 1) * LANES)
            for n in range(LANES // PR):
                r = n * PR
                cache = {}

                def w(k, j1):
                    if (k, j1) not in cache:
                        v = GU[m][p, k * LANES + r:k * LANES + r + PR,
                                  2 * j1 * LANES:2 * (j1 + 1) * LANES].astype(F32)
                        if (k // 2, j1) in [_SB[m1][0][:2] for m1 in m1s[:2]]:
                            a = spread_over(anchors, n, LANES // PR)
                            if cfg['tie1']:
                                c = (k % 2) * LANES
                                tied = _tie(v[:, c:c + LANES], a)
                                v = cat1(v[:, :LANES], tied) if c else cat1(tied, v[:, LANES:])
                            else:
                                v = _tie(v, a)
                        cache[k, j1] = v
                    return cache[k, j1]

                for m1 in m1s:
                    b1 = [_signed(_SB[m1], lambda k1, j1: w(2 * k1 + k2, j1)) for k2 in range(2)]
                    for m2 in range(7):
                        v = _signed(_SB[m2],
                                    lambda k2, j2: b1[k2][:, j2 * LANES:(j2 + 1) * LANES])
                        gv.at[7 * m1 + m2][r // 2:(r + PR) // 2, cs] = _pk(v)

        def prep_tail(p, gv, m, anchor):
            v = _tie(GU[m][p, 4 * LANES:, :].astype(F32), anchor)
            for j in range(4):
                gv.at[49 + j // 2][(j % 2) * 32:(j % 2 + 1) * 32,
                                        m * LANES:(m + 1) * LANES] = _pk(
                                            v[:, j * LANES:(j + 1) * LANES])

        def gu_outer(gv, m, m1, anchors, at=(0, 4)):
            cs = slice(m * LANES, (m + 1) * LANES)
            y = {}
            for m2 in cfg['inner']:
                i, (o, ac) = 7 * m1 + m2, AOFF[m1, m2]
                if m1 in _SCOL and m2 in _SCOL:
                    j = 2 * _SCOL[m1] + _SCOL[m2]
                    tail = lambda: gv[49 + j // 2, (j % 2) * 32:(j % 2 + 1) * 32, cs]
                    rhs = (cat0(tail(), gv[i, 32:, cs]), gv[i, :, cs],
                           cat0(gv[i, :32, cs], tail()))
                    r = [_dot(_upk(a_s[o + 16 * s:o + 16 * (s + 1), ac]), _upk(rhs[s]))
                         for s in range(3)]
                    y[m2] = cat0(r[1] + r[0], r[2] + r[0])
                else:
                    y[m2] = _dot(_upk(a_s[o:o + TQ // 2, ac]), _upk(gv[i, :, cs]))
            anchors.extend(y[cfg['inner'][k % 7]][(k // 7) * 32:(k // 7) * 32 + 8] for k in at)
            return _s_out(y)

        def gu_finish(t):
            gu = [{(i2, j2): _s_out([t[m][m1][i2][j2] for m1 in range(7)])
                   for i2 in range(2) for j2 in range(2)} for m in range(2)]
            return [[cat0(*[_gelu_mul2(*[gu[m][i2, j % 2][i1][j // 2] for m in range(2)])
                            for i2 in range(2)]) for i1 in range(2)] for j in range(4)]

        def gu_piece(gv, order, anchors, at=(0, 4)):
            t = ({}, {})
            for m, m1 in order:
                t[m][m1] = gu_outer(gv, m, m1, anchors, at)
            return gu_finish(t)

        def prep_piece(p, gv, anchors, group):
            grp = _SGRP if group else [(m1,) for m1 in range(7)]
            k = len(anchors) // (2 * len(grp))
            for n in range(2 * len(grp)):
                prep_gu(p, gv, n % 2, grp[n // 2], anchors[k * n:k * n + k])
            for m in range(2):
                prep_tail(p, gv, m, anchors[m * len(anchors) // 2])

        def h_ops(h):
            return [v.astype(BF16) for v in _x_ops(*[[h[k][i] for k in range(3)]
                                                     for i in range(2)])]

        D_ORDER = _PAIR_ORDER + (9, 10, 11, 12, 13, 14)

        def down_mm(acc, work, anchors, which=D_ORDER, fine=False):
            p = [None] * 15 if acc is None else list(acc)
            jobs = [(i, n) for i in which for n in range(len(work))]
            split = {0: (), 1: (4,), 2: (2, 2), 3: (2, 2, 4)}[len(jobs) % 4]
            split = dict(zip(jobs[len(jobs) - len(split):], split))
            for i in which:
                y = None
                for n, (tri, b) in enumerate(work):
                    ns = split.get((i, n), 1)
                    nr = D3 // ns
                    if i in _W_RAW:
                        k, j = _W_RAW[i]
                        lhs = lambda h: wd_raw(tri, k, j * D3 + h * nr, nr)
                    else:
                        s = _W_SUM[i]
                        lhs = lambda h: _upk(ds_s.at[tri[0], s // 2][ds_loc(s, h * nr // 2, nr // 2)])
                    v = cat0(*[_dot_nt(lhs(h), b[i]) for h in range(ns)])
                    y = v if y is None else y + v
                p[i] = y if p[i] is None else p[i] + y
                anchors.append(p[i][:8])
                if fine:
                    anchors.append(p[i][D3 // 2:D3 // 2 + 8])
            return p

        def finish(blk, acc, after=None):
            y = [cat1(*_column(acc, [acc[_DIAG[s, j]] if (s, j) in _DIAG else None
                                     for s in range(3)], j)) for j in range(3)]
            if after is None:
                xio_s[blk] = (xmid_s[blk] + 0.5 * cat0(*y)).astype(BF16)
                return
            for j in range(3):
                rows = slice(j * D3, (j + 1) * D3)
                xio_s[blk, rows] = (xmid_s[blk, rows] + 0.5 * y[j]).astype(BF16)
                after(j)

        def load_acc(k):
            return [acc_s[k, i] for i in range(15)]

        def store_acc(k, acc):
            for i in range(15):
                acc_s[k, i] = acc[i]

        def pre_phase():
            first = [[x_cp(0, 0)], [wq_cp(0)], [x_cp(1, 2), wq_cp(1)],
                     [wq_cp(2), pltpu.make_async_copy(wo_hbm, wo_v, sem_i.at[3])]]
            order = sum(first, [])
            for p in range(NP + 1):
                order += group_cp(p)
            xr_cp = [x_cp(b, SEM_P + NP + 1) for b in range(2, NB)]
            order += xr_cp
            for cp in order:
                cp.start()
            get = lambda an, name: [an[min(i, len(an) - 1)] for i in cfg[name]]
            e_grp = lambda e: ((e >> 1) & 1, ((e >> 2) << 1) | (e & 1))
            if 'a' in cfg['sub']:
                pre_a(first, get, e_grp)
            if 'b' in cfg['sub']:
                pre_b(get, e_grp)
            if 'c' in cfg['sub']:
                pre_c(get)
            wait('WX', xr_cp)

        def pre_a(first, get, e_grp):
            def transpose_wq(i):
                wt_s[WQ[i] // 2:WQ[i + 1] // 2, :D] = _pk(wqkv_v[:, WQ[i]:WQ[i + 1]].T)

            def clear(i, carry):
                for k in range(2):
                    acc_s[k, i] = jnp.zeros((D3, TH), F32)
                r = jnp.minimum(i, 11) * (RP // 4)
                qkv_s[0, rows8(r, RP // 4)] = jnp.zeros((RP // 4, LANES), U32)
                return carry

            lax.fori_loop(0, 15, clear, 0)
            wait('WX0', first[0])
            xn0 = ln1(0, ()).astype(BF16)

            wait('WQ0', first[1])
            transpose_wq(0)
            qkv_mm(0, xn0, (0, 1), [])

            wait('WQ1', first[2])
            transpose_wq(1)
            an = []
            qkv_mm(0, xn0, (2, 3), an)
            xn1 = ln1(1, get(an, 'a_ln'), get(an, 'a_lnb')).astype(BF16)
            qkv_mm(1, xn1, (0,), an, True)
            for n, a in enumerate(get(an, 'a_w1')):
                prep_att(n, a)
            nk = len(cfg['a_k'])
            apply = [att_values(0, *e_grp(e), a) for e, a in enumerate(get(an, 'a_k'))]

            wait('WQ2', first[3])
            an = []
            qkv_mm(1, xn1, (2,), an)
            transpose_wq(2)
            qkv_mm(0, xn0, (4, 5), an)
            qkv_mm(1, xn1, (4,), an)
            qkv_mm(1, xn1, (1,), an, True)
            apply += [att_values(0, *e_grp(nk + e), a)
                      for e, a in enumerate(get(an, 'a_k2')[:8 - nk])]
            for e, a in enumerate(get(an, 'a_v')):
                apply[e](a)
            wo = pltpu.bitcast(wo_v[...], U32)
            wo = cat0(_lo(wo), _hi(wo))
            wo = cat0(*[_tie(wo[n * LANES:(n + 1) * LANES], a)
                        for n, a in enumerate(get(an, 'a_wo'))])
            wt_s[3 * RP:, :D] = _pk(wo.astype(BF16).T)
            for n, a in enumerate(get(an, 'a_w2')):
                prep_att(len(cfg['a_w1']) + n, a)

            wait('WO', group_cp(0))
            an = []
            stats = wo_mm(0, an, False)
            qkv_mm(1, xn1, (3, 5), an)
            for n, a in enumerate(get(an, 'z_w')):
                prep_att(36 + n, a)
            prep_piece(0, gu_s.at[0], get(an, 'z_g'), cfg['z_grp'])
            ffn_lhs(0, stats, get(an, 'z_l'))

        def pre_b(get, e_grp):
            def piece(p, carry):
                wait('WP', group_cp(p))
                an = []
                win = gu_s.at[pl.ds(p - 1, 2)]
                h = gu_piece(win.at[0], cfg['gorder0'], an, (0, 7, 4, 11))
                h3_s[p - 1] = cat0(*h[3])
                tri = in_triple(p - 1)
                prep_d(tri, get(an, 'p_d'))
                store_acc(0, down_mm(load_acc(0), [(tri, h_ops(h[:3]))], an))
                prep_piece(p, win.at[1], get(an, 'f_g'), cfg['f_grp'])
                att_group(1, *e_grp(p - 1), an[cfg['p_att'][0]])
                return carry

            lax.fori_loop(1, NP, piece, 0)

        def pre_c(get):
            wait('WD', group_cp(NP))
            an = []
            h = gu_piece(gu_s.at[NP - 1], cfg['torder'], an)
            h3 = [[h3_s[q, :TH], h3_s[q, TH:]] for q in range(NP - 1)] + [h[3]]
            work = [(cross_triple(s), h_ops(h3[3 * s:3 * s + 3])) for s in range(3)]
            work.append((in_triple(NP - 1), h_ops(h[:3])))
            stats = wo_mm(1, an, True)
            td = get(an, 't_d')
            for n, (tri, _) in enumerate(work):
                prep_d(tri, td[n * len(td) // 4:(n + 1) * len(td) // 4])
            acc = down_mm(load_acc(0), work, an)
            nw = len(cfg['a_w1']) + len(cfg['a_w2'])
            for n, a in enumerate(get(an, 't_w')[:36 - nw]):
                prep_att(nw + n, a)
            ffn_lhs(1, stats, get(an, 't_l'))
            finish(0, acc)

        if 'pre' in cfg['phases']:
            pre_phase()

        def body(u, carry):
            bu = u & (NB - 1)
            ba = (u + 1) & (NB - 1)
            acc, stats, an, b, hh = None, None, {}, {}, {}
            get = lambda name: [an[k][i] for k, i in cfg[name]]
            for step in cfg['body']:
                an[step] = []
                if step == 'Q':
                    xn = ln1(ba, get('ln1'), get('ln1b'))
                    qkv_fast(ba, att_rhs(xn, u >> 8), an[step])
                elif step == 'W':
                    attention(ba, get('att'))
                    stats = wo_mm(ba, an[step], True, u >> 8, get('orhs'))
                elif step == 'L':
                    ffn_lhs(ba, stats, get('lhs'))
                elif step[0] == 'G':
                    q, go = int(step[1]), cfg['gorder']
                    t = b.setdefault(step[:2], ({}, {}))
                    for m, m1 in (go[:7] if step[2] == '0' else go[7:]):
                        t[m][m1] = gu_outer(gu_s.at[q], m, m1, an[step])
                    if len(t[0]) + len(t[1]) == 14:
                        hh[q] = gu_finish(t)
                else:
                    work = []
                    for c in step[1:]:
                        if c.isdigit():
                            work.append((in_triple(int(c)), h_ops(hh[int(c)][:3])))
                        else:
                            s = ord(c) - ord('a')
                            work.append((cross_triple(s),
                                         h_ops([hh[3 * s + k][3] for k in range(3)])))
                    acc = down_mm(acc, work, an[step])
            finish(bu, acc)

            @pl.when(u >= NB)
            def _():
                out_copy(bu).start()
            return carry

        if scopes:
            with jax.named_scope('LOOP'):
                lax.fori_loop(1, NU - 1, body, 0)
        elif 'main' in cfg['phases']:
            lax.fori_loop(1, NU - 1, body, 0)

        fin_cp = [pltpu.make_async_copy(
            xio_s.at[NB - 1, pl.ds(j * D3, D3)],
            out_hbm.at[pl.ds(j * D3, D3), cols((NB - 1) * TM, TM)], sem_o.at[0])
            for j in range(3)]

        def last(s, carry):
            h = [gu_piece(gu_s.at[3 * s + k], cfg['lorder'], []) for k in range(3)]
            work = [(in_triple(3 * s + k), h_ops(h[k][:3])) for k in range(3)]
            work.append((cross_triple(s), h_ops([h[k][3] for k in range(3)])))
            acc = down_mm(down_mm(load_acc(1), work[:2], []), work[2:], [], cfg['ldord'])
            store_acc(1, acc)
            finish(NB - 1, acc, lambda j: pl.when(s == NP // 3 - 1)(fin_cp[j].start))
            return carry

        if 'last' in cfg['phases']:
            lax.fori_loop(0, NP // 3, last, 0)
        if len(cfg['phases']) < 3:
            def keep(i, c):
                v = (gu_s[i, i, :8, :LANES] + ds_s[i, i, :8, :LANES]
                     + wl_s[rows8(i * 8), :LANES] + a_s[rows8(i * 8), :LANES] + qkv_s[i, :8]
                     + wt_s[rows8(i * 8), :LANES])
                acc_s[1, 0, :8] = (lax.bitcast_convert_type(v, F32) + o_s[i, :8]
                                   + acc_s[i, i, :8] + h3_s[i, :8])
                return c
            lax.fori_loop(0, 2, keep, 0)
            finish(NB - 1, load_acc(1))
        wait('WOUT', [out_copy(b) for b in range(NB - 1)] + fin_cp)

    scratch = [
        pltpu.VMEM((NB, D, TM), BF16),
        pltpu.VMEM((D, 3 * D), BF16),
        pltpu.VMEM((D, D), BF16),
        pltpu.VMEM((NP, D, PW), BF16),
        pltpu.VMEM((NP, D, PW), BF16),
        pltpu.VMEM((NP, D, PW), BF16),
        pltpu.VMEM((2 * D, 8 * LANES), U32),
        pltpu.VMEM((4 * Q3, 16 * LANES), U32),
        pltpu.VMEM((NP, 51, 64, 2 * LANES), U32),
        pltpu.VMEM((NP + 3, 5, Q3, 2 * LANES), U32),
        pltpu.VMEM((NB, D, TM), F32),
        pltpu.VMEM((max(fill), 2 * LANES), U32),
        pltpu.VMEM((S // LANES + 1, 3 * RP, LANES), U32),
        pltpu.VMEM((NT, D, LANES), F32),
        pltpu.VMEM((2, 15, D3, TH), F32),
        pltpu.VMEM((NP, TM, LANES), F32),
        pltpu.VMEM((1, 9 * 64, 2 * LANES), U32),
        pltpu.SemaphoreType.DMA((SEM_P + NP + 2,)),
        pltpu.SemaphoreType.DMA((1,)),
    ]

    def wrapped(*refs):
        @pl.when(pl.program_id(0) == 0)
        def _():
            kernel(*refs)

    return wrapped, scratch


_CFG = dict(
    scopes=False, ldord=(1, 2, 0, 7, 8, 6, 9, 10, 4, 5, 3, 11, 12, 13, 14),
    tie1=True,
    orhs=(('G80', 0), ('G80', 1), ('G80', 2), ('G80', 3), ('G80', 4), ('G80', 5),
        ('G80', 6), ('G80', 7), ('G80', 8), ('G80', 9), ('G80', 10), ('G80', 11)),
    sub='abc',
    phases=('pre', 'main', 'last'),
    body=('G20', 'G00', 'G01', 'G10', 'G11', 'Q', 'G30', 'G21', 'G40', 'G31', 'G50',
        'D012a', 'G41', 'G51', 'D345b', 'G70', 'G60', 'G71', 'G80', 'W', 'G61', 'G81',
        'D8c', 'D67', 'L'),
    ln1=(('G00', 0), ('G00', 1), ('G00', 2), ('G00', 3), ('G00', 4), ('G00', 5), ('G00',
        6), ('G00', 7), ('G00', 8)),
    ln1b=(('G10', 1), ('G10', 2), ('G10', 3), ('G10', 4), ('G10', 5), ('G10', 6),
        ('G10', 7), ('G10', 8), ('G10', 9), ('G10', 10), ('G10', 11), ('G10', 12)),
    att=(('D012a', 2), ('D012a', 4), ('D012a', 5), ('D012a', 8), ('D012a', 9), ('D345b',
        5), ('D345b', 6), ('D345b', 8)),
    lhs=(('D8c', 2), ('D8c', 3), ('D8c', 9), ('D8c', 11), ('D67', 5), ('D67', 8),
        ('D67', 10), ('D67', 11), ('D67', 14)),
    a_w1=(0, 0, 1, 2, 2, 3, 3, 4, 5, 6, 7, 11, 13, 18, 19, 20, 21, 22, 23, 24, 26, 27,
        28, 29),
    a_w2=(25, 30, 33, 36, 44, 45),
    a_ln=(3, 6, 7),
    a_lnb=(3, 9, 15),
    z_g=(0, 0, 1, 1, 2, 2, 3, 3, 4, 4, 5, 5, 6, 6, 7, 7, 8, 8, 9, 11, 12, 12, 13, 14,
        14, 14, 15, 15, 16, 16, 17, 17, 18, 18, 19, 19, 20, 21, 21, 22, 23, 23, 23, 24,
        25, 26, 27, 33),
    t_d=(0, 0, 0, 2, 2, 4, 5, 5, 7, 7, 8, 8, 9, 10, 11, 11, 12, 12, 13, 14, 14, 15, 16,
        16, 17, 17, 18, 18, 21, 22, 24, 24, 25, 28, 28, 30, 32, 32, 35, 35, 36, 37, 37,
        37, 39, 40, 40, 42),
    p_d=(3, 12, 14, 17, 24, 25, 28, 33, 35, 38, 42, 46),
    p_att=(58,),
    z_l=(23, 23, 28, 31, 35, 36, 37, 37, 39),
    a_k=(13, 17, 20, 26),
    a_k2=(0, 1, 3, 9),
    a_v=(13, 13, 14, 15, 16, 17, 18, 19),
    a_wo=(9, 18, 25, 36, 46),
    inner=(0, 3, 4, 6, 2, 1, 5),
    gorder=((0, 4), (0, 0), (1, 4), (1, 0), (1, 6), (0, 3), (1, 3), (0, 6), (0, 1), (1,
        1), (0, 2), (1, 2), (0, 5), (1, 5)),
    gorder0=((0, 0), (1, 4), (0, 4), (1, 0), (0, 3), (0, 6), (1, 6), (1, 3), (1, 1), (0,
        1), (0, 2), (0, 5), (1, 5), (1, 2)),
    f_g=(0, 0, 1, 2, 5, 5, 6, 7, 8, 9, 9, 10, 12, 13, 14, 16, 17, 17, 19, 20, 21, 23,
        24, 24, 26, 28, 29, 31, 32, 35, 36, 37, 37, 40, 40, 42, 43, 44, 45, 47, 48, 48,
        53, 56, 58, 59, 60, 61, 62, 62, 64, 64, 69, 70, 70, 70),
    t_l=(49, 50, 51, 53, 54, 55, 57, 57, 60),
    lorder=((1, 0), (1, 4), (0, 0), (0, 4), (0, 3), (0, 6), (1, 3), (1, 6), (0, 1), (1,
        1), (0, 2), (0, 5), (1, 2), (1, 5)),
    z_w=(1, 1, 3, 3, 5, 5, 6, 6, 8, 9, 17, 35),
    z_grp=1,
    f_grp=0,
    t_w=(47, 49, 49, 50, 52, 54),
    torder=((0, 0), (0, 4), (1, 4), (1, 0), (0, 3), (1, 3), (1, 6), (0, 6), (0, 1), (1,
        1), (0, 2), (1, 2), (0, 5), (1, 5)),
)


def _run(A_x, A_wqkv, A_wo, B_w_gate, B_w_up, B_w_down, **kw):
    _, S, D = A_x.shape
    F = B_w_gate.shape[1]
    kernel, scratch = _make_kernel(S, D, F, 256, {**_CFG, **kw})
    hbm = pl.BlockSpec(memory_space=pl.ANY)
    out_t = pl.pallas_call(
        kernel,
        grid=(2,),
        in_specs=[hbm] * 6,
        out_specs=hbm,
        out_shape=jax.ShapeDtypeStruct((D, S), A_x.dtype),
        scratch_shapes=scratch,
        compiler_params=pltpu.CompilerParams(
            dimension_semantics=('arbitrary',), vmem_limit_bytes=110 * 1024 * 1024),
    )(A_x.reshape(S, D).T, A_wqkv, A_wo, B_w_gate, B_w_up, B_w_down.T)
    return out_t.T.reshape(A_x.shape)


@jax.jit
def pallas_interleave_layers__sliding_local_dilated__glu_gated_geglu__prompt_kernel(
    A_x: jax.Array,
    A_wqkv: jax.Array,
    A_wo: jax.Array,
    B_x: jax.Array,
    B_w_gate: jax.Array,
    B_w_up: jax.Array,
    B_w_down: jax.Array,
):
    del B_x
    return _run(A_x, A_wqkv, A_wo, B_w_gate, B_w_up, B_w_down)
```

```python
import jax
import jax.numpy as jnp
import jax.experimental.pallas as pl
import jax.experimental.pallas.tpu as pltpu
from jax import lax

H = 32
W = 8
DIL = 2
EPS = 1e-5
LANES = 128

F32 = jnp.float32
BF16 = jnp.bfloat16
U32 = jnp.uint32

_NT = (((1,), (1,)), ((), ()))


def _tree_sum(parts, op=jnp.add):
    while len(parts) > 1:
        nxt = [op(parts[i], parts[i + 1]) for i in range(0, len(parts) - 1, 2)]
        if len(parts) % 2:
            nxt.append(parts[-1])
        parts = nxt
    return parts[0]


def _ln_stats(slabs, d, anchors=()):
    n_acc = 4
    s1, s2, pilot = [None] * n_acc, [None] * n_acc, None
    for i, x in enumerate(slabs):
        if pilot is None:
            pilot = x[0:1, :]
            pil = jnp.broadcast_to(pilot, x.shape)
            pils = [_tie(pil, a) for a in anchors] or [pil]
        dx = x - pils[i * len(pils) // (d // 8)]
        j = i % n_acc
        s1[j] = dx if s1[j] is None else s1[j] + dx
        s2[j] = dx * dx if s2[j] is None else s2[j] + dx * dx
    e1 = jnp.sum(_tree_sum(s1), axis=0, keepdims=True) * (1.0 / d)
    e2 = jnp.sum(_tree_sum(s2), axis=0, keepdims=True) * (1.0 / d)
    var = jnp.maximum(e2 - e1 * e1, 0.0)
    return pilot + e1, lax.rsqrt(var + EPS)


def _zero_like_dep(v):
    return (lax.bitcast_convert_type(v, U32) >> 31) >> 1


def _tie(x, anchor):
    if anchor is None:
        return x
    z = lax.bitcast_convert_type(_zero_like_dep(anchor), F32)
    z = jnp.concatenate([z] * -(-x.shape[1] // LANES), axis=1)[:, :x.shape[1]]
    if x.shape[0] == 8:
        return x + z
    return jnp.concatenate([x[:8] + z, x[8:]], axis=0)


def _gelu_mul2(g, u):
    c0 = 0.7978845608028654
    c1 = c0 * 0.044715
    t = jnp.tanh(g * (c0 + c1 * (g * g)))
    return (g * u) * (1.0 + t)


def _lo(x):
    return lax.bitcast_convert_type(x << 16, F32)


def _hi(x):
    return lax.bitcast_convert_type(x & jnp.uint32(0xFFFF0000), F32)


def _pk(x):
    return pltpu.bitcast(x.astype(BF16), U32)


def _upk(x):
    return pltpu.bitcast(x, BF16)


def _dot(a, b):
    return jnp.dot(a, b, preferred_element_type=F32)


def _dot_nt(a, b):
    return lax.dot_general(a, b, _NT, preferred_element_type=F32)


def _x_ops(x1, x2):
    d = [a - b for a, b in zip(x1, x2)]
    return [x1[0] + x2[1], x2[0] + x2[1], x1[0] + x1[1],
            d[1] + x1[2], x1[1] + x1[2], d[1] + d[2],
            d[0] - x2[2], d[0] + d[2], x2[0] + x2[2],
            x1[0], d[0], x2[1], d[1], x1[2], x2[2]]


def _x_rem(x1, x2):
    a, b, c = 0, 1, 2
    cat = lambda u, v: jnp.concatenate([u, v], axis=0)
    return [cat(x1[c], x2[b]), cat(x1[a], x1[b] - x2[b]), cat(x2[a], x2[c] - x1[c])]


_W_TERMS = {0: ((0, 1, 1), (1, 0, 1)), 3: ((1, 2, 1), (2, 1, 1)), 6: ((0, 2, 1), (2, 0, 1)),
            9: ((0, 0, 1), (0, 2, 1), (1, 0, -1)), 10: ((2, 0, 1), (0, 0, -1), (0, 1, -1)),
            11: ((1, 1, 1), (1, 2, 1), (0, 1, -1)), 12: ((1, 0, 1), (1, 1, 1), (2, 1, -1)),
            13: ((2, 0, 1), (2, 2, 1), (1, 2, -1)), 14: ((2, 1, 1), (2, 2, 1), (0, 2, -1)),
            1: ((0, 1, 1),), 2: ((1, 0, 1),), 4: ((1, 2, 1),), 5: ((2, 1, 1),),
            7: ((2, 0, 1),), 8: ((0, 2, 1),)}


def _w_sums(w):
    return [_signed(_W_TERMS[i], lambda k, j: w[k][j]) for i in _W_SUM]


_W_SUM = {0: 0, 3: 1, 6: 2, 9: 3, 10: 4, 11: 5, 12: 6, 13: 7, 14: 8}
_W_RAW = {1: (0, 1), 2: (1, 0), 4: (1, 2), 5: (2, 1), 7: (2, 0), 8: (0, 2)}
_PAIR_ORDER = (1, 2, 4, 5, 7, 8, 0, 3, 6)
_DIAG = {(0, 0): 9, (2, 0): 10, (0, 1): 11, (1, 1): 12, (1, 2): 13, (2, 2): 14}
_PAIR = {(0, 0): ((6, -1), (8, -1)), (1, 0): ((2, 1), (7, 1)), (2, 0): ((0, 1), (1, -1)),
         (0, 1): ((3, 1), (4, -1)), (1, 1): ((0, 1), (2, -1)), (2, 1): ((1, 1), (5, -1)),
         (0, 2): ((4, 1), (8, 1)), (1, 2): ((6, 1), (7, -1)), (2, 2): ((5, 1), (3, -1))}


def _column(t, base, j, skew=False):
    s = []
    for k in range(3):
        v = base[k]
        for i, sg in _PAIR[k, j]:
            v = t[i] if v is None else (v + t[i] if sg > 0 else v - t[i])
        s.append(v)
    if skew:
        return s[1] + s[0], s[2] + 0.5 * (s[0] - s[1])
    return s[1] + s[0], s[2] + s[0]


_SA = (((0, 0, 1), (1, 1, 1)), ((1, 0, 1), (1, 1, 1)), ((0, 0, 1),), ((1, 1, 1),),
       ((0, 0, 1), (0, 1, 1)), ((1, 0, 1), (0, 0, -1)), ((0, 1, 1), (1, 1, -1)))
_SB = (((0, 0, 1), (1, 1, 1)), ((0, 0, 1),), ((0, 1, 1), (1, 1, -1)), ((1, 0, 1), (0, 0, -1)),
       ((1, 1, 1),), ((0, 0, 1), (0, 1, 1)), ((1, 0, 1), (1, 1, 1)))
_SCOL = {2: 1, 3: 0, 5: 1, 6: 0}
_SGRP = ((1, 4, 0), (3, 6), (2, 5))


def _signed(terms, f):
    v = None
    for a, b, sg in terms:
        v = f(a, b) if v is None else (v + f(a, b) if sg > 0 else v - f(a, b))
    return v


def _s_out(m):
    return [[m[0] + m[3] - m[4] + m[6], m[2] + m[4]],
            [m[1] + m[3], m[0] - m[1] + m[2] + m[5]]]


def _make_kernel(S, D, F, TM, cfg):
    NB = S // TM
    NT = TM // LANES
    DH = D // H
    DP = DH // 2
    RP = D // 2
    NG = H // 8
    scale = float(DH) ** -0.5
    NU = 2 * NB
    TH = TM // 2
    TQ = TM // 4
    D2 = D // 2
    D3 = D // 3
    Q3 = D3 // 2
    KU = D // 9
    KR = 3 * LANES
    NQ = 6
    QR = 3 * D // NQ
    WQ = (0, 640, 1152, 3 * D)
    PW = 4 * LANES
    NP = F // PW
    AOFF, fill = {}, [0, 0]
    for key in [(m1, m2) for m1 in range(7) for m2 in range(7)]:
        c = int(fill[1] < fill[0])
        AOFF[key] = (fill[c], slice(c * LANES, (c + 1) * LANES))
        fill[c] += 48 if key[0] in _SCOL and key[1] in _SCOL else 32
    scopes = cfg['scopes']
    assert NG == 4 and NB & (NB - 1) == 0
    SEM_P = 4

    def kernel(x_hbm, wqkv_hbm, wo_hbm, wg_hbm, wu_hbm, wdt_hbm, out_hbm,
               xio_s, wqkv_v, wo_v, wg_v, wu_v, wdt_v, wt_s, wl_s,
               gu_s, ds_s, xmid_s, a_s, qkv_s, o_s, acc_s, h3_s, r_s,
               sem_i, sem_o):

        def wait(name, cps):
            if scopes:
                with jax.named_scope(name):
                    for cp in cps:
                        cp.wait()
            else:
                for cp in cps:
                    cp.wait()

        def cols(lo, n):
            if not isinstance(lo, int):
                lo = pl.multiple_of(lo, LANES)
            return pl.ds(lo, n)

        def rows8(lo, n=8):
            if not isinstance(lo, int):
                lo = pl.multiple_of(lo, 8)
            return pl.ds(lo, n)

        def out_copy(b):
            return pltpu.make_async_copy(
                xio_s.at[b], out_hbm.at[:, cols(b * TM, TM)], sem_o.at[0])

        def x_cp(b, sem):
            return pltpu.make_async_copy(x_hbm.at[:, cols(b * TM, TM)], xio_s.at[b],
                                         sem_i.at[sem])

        def wq_cp(i):
            sl = cols(WQ[i], WQ[i + 1] - WQ[i])
            return pltpu.make_async_copy(wqkv_hbm.at[:, sl], wqkv_v.at[:, sl],
                                         sem_i.at[1 + i])

        def piece_cp(src, dst, p, sem, c0=0, n=PW):
            return pltpu.make_async_copy(src.at[:, cols(p * PW + c0, n)],
                                         dst.at[p, :, pl.ds(c0, n)], sem_i.at[sem])

        def group_cp(p):
            sem = SEM_P + p
            cps = []
            if not (isinstance(p, int) and p == NP):
                cps += [piece_cp(wg_hbm, wg_v, p, sem), piece_cp(wu_hbm, wu_v, p, sem)]
            if not (isinstance(p, int) and p == 0):
                cps.append(piece_cp(wdt_hbm, wdt_v, p - 1, sem, 0, KR))
            if isinstance(p, int) and p == NP:
                cps += [piece_cp(wdt_hbm, wdt_v, q, sem, KR, LANES) for q in range(NP)]
            return cps

        lane = lax.broadcasted_iota(jnp.int32, (8, LANES), 1)
        cat0 = lambda *v: jnp.concatenate(v, axis=0)
        cat1 = lambda *v: jnp.concatenate(v, axis=1)

        def spread_over(anchors, n, total):
            return anchors[n * len(anchors) // total] if anchors else None

        def slab_group(r):
            return (r % LANES) // 16 if r < KR else 8 + ((r - KR) % KU) // 16

        def ln1(blk, anchors1, anchors2=()):
            slabs = (xio_s[blk, r:r + 8, :].astype(F32) for r in range(0, D, 8))
            m, rs = _ln_stats(slabs, D, anchors1)
            if not anchors2:
                return (xio_s[blk].astype(F32) - m) * rs
            m8 = jnp.broadcast_to(m, (8, TM))
            ms = [_tie(m8, a) for a in anchors2]
            ms = [spread_over(ms, slab_group(r), 12) for r in range(0, D, 8)]
            return (xio_s[blk].astype(F32) - cat0(*ms)) * rs

        def dot_k(rows, x, anchors, even=False):
            y = None
            for n, k in enumerate(range(0, D, LANES)):
                ks = slice(k, min(k + LANES, D))
                if even and k + LANES >= D:
                    mid = (rows.start + rows.stop) // 2
                    v = cat0(_dot(_upk(wt_s[rows.start:mid, ks]), x[ks]),
                             _dot(_upk(wt_s[mid:rows.stop, ks]), x[ks]))
                else:
                    v = _dot(_upk(wt_s[rows, ks]), x[ks])
                anchors.extend(v[r:r + 8, :LANES] for r in ((0, 144) if n % 2 else (72, 216)))
                y = v if y is None else y + v
            return y

        def put_qkv(blk, rows, y):
            pk = _pk(y)
            for c in range(NT):
                qkv_s[1 + blk * NT + c, rows, :] = pk[:, c * LANES:(c + 1) * LANES]

        def qkv_mm(blk, xn, chunks, anchors, even=False):
            for r in chunks:
                rows = slice(r * QR // 2, (r + 1) * QR // 2)
                put_qkv(blk, rows, dot_k(rows, xn, anchors, even))

        def split_k(x):
            hs = (x[:, :TH], x[:, TH:])
            blocks = [[h[k * LANES:(k + 1) * LANES] for k in range(3)] for h in hs]
            units = [[h[KR + k * KU:KR + (k + 1) * KU] for k in range(3)] for h in hs]
            return blocks, units

        def prep_att(pat, anchor):
            assert Q3 == 96
            row0 = pat * 8
            src0 = row0 + ((pat * 43) >> 9) * (2 * Q3)
            w = [_upk(wt_s[rows8(src0 + j * Q3), :D]).astype(F32) for j in range(3)]
            w[0] = cat1(_tie(w[0][:, :LANES], anchor), w[0][:, LANES:])
            tiles = _w_sums([[w[j][:, k * LANES:(k + 1) * LANES] for j in range(3)]
                             for k in range(3)])
            for j in range(3):
                a, b, c = (w[j][:, KR + k * KU:KR + (k + 1) * KU] for k in range(3))
                tiles += [cat1(c, b), cat1(a, c)]
            wl_s[rows8(row0), :15 * LANES] = _pk(cat1(*tiles))

        def att_rhs(x, stash=None, anchors=()):
            half = 0.5
            if anchors:
                hs = [_tie(jnp.full((8, TH), 0.5, F32), a) for a in anchors]
                half = cat0(*[spread_over(hs, slab_group(r), 12) for r in range(0, D, 8)])
            blocks, units = split_k(cat1(x[:, :TH], x[:, TH:] + half * x[:, :TH]))
            ops = _x_ops(*blocks) + _x_rem(*units)
            if stash is None:
                return [v.astype(BF16) for v in ops]
            loc = lambda i, r0, n: (slice((i // 2) * 64 + r0, (i // 2) * 64 + r0 + n),
                                    slice((i % 2) * LANES, (i % 2 + 1) * LANES))
            for r in range(0, LANES, 16):
                for i, v in enumerate(ops):
                    r_s.at[0][loc(i, r // 2, 8)] = _pk(v[r:r + 16])
            return [_upk(r_s.at[stash][loc(i, 0, 64)]) for i in range(18)]

        def att_mm(sec, rhs, anchors):
            tl = lambda i: _upk(wl_s[sec * Q3:(sec + 1) * Q3, i * LANES:(i + 1) * LANES])
            raw = lambda k, j: _upk(wt_s[(3 * sec + j) * Q3:(3 * sec + j + 1) * Q3,
                                         k * LANES:(k + 1) * LANES])
            t = {}
            for i in _PAIR_ORDER:
                t[i] = _dot(raw(*_W_RAW[i]) if i in _W_RAW else tl(_W_SUM[i]), rhs[i])
                anchors.append(t[i][:8])
            out = []
            for j in range(3):
                base = []
                for s in range(3):
                    v = _dot(raw(3, j) if s == 1 else tl(9 + 2 * j + s // 2), rhs[15 + s])
                    if (s, j) in _DIAG:
                        i = _DIAG[s, j]
                        v = _dot(tl(_W_SUM[i]), rhs[i]) + v
                    base.append(v)
                    anchors.append(base[-1][:8])
                out.append(cat1(*_column(t, base, j, True)))
            return cat0(*out)

        def qkv_fast(blk, rhs, anchors):
            for sec in range(3):
                put_qkv(blk, slice(sec * RP, (sec + 1) * RP), att_mm(sec, rhs, anchors))

        def shifted(ln, cur, prev, w):
            if w == 0:
                return cur
            sh = DIL * w
            return pltpu.roll(jnp.where(ln < LANES - sh, cur, prev), sh, axis=1)

        def att_group(blk, c, hg, anchor):
            att_values(blk, c, hg, anchor)(None)

        def att_values(blk, c, hg, anchor):
            tile = blk * NT + c
            base = hg * 8 * DP
            if isinstance(hg, int):
                cur, prev, o_t = qkv_s.at[1 + tile], qkv_s.at[tile], o_s.at[c]
            else:
                n = 2 * RP + 8 * DP
                base = pl.multiple_of(base, 8)
                cur = qkv_s.at[1 + tile, pl.ds(base, n)]
                prev = qkv_s.at[tile, pl.ds(base, n)]
                o_t = o_s.at[c, pl.ds(base, RP + 8 * DP)]
                base = 0
            ln = lane + _zero_like_dep(anchor).astype(jnp.int32)
            logits = [None] * W
            for dd in range(DP):
                q = cur[pl.ds(base + dd, 8, stride=DP), :]
                kc = cur[pl.ds(RP + base + dd, 8, stride=DP), :]
                kp = prev[pl.ds(RP + base + dd, 8, stride=DP), :]
                q0, q1 = _lo(q), _hi(q)
                for w in range(W):
                    ks = shifted(ln, kc, kp, w)
                    t = q0 * _lo(ks) + q1 * _hi(ks)
                    logits[w] = t if logits[w] is None else logits[w] + t
            logits = [l * scale for l in logits]
            if not (isinstance(c, int) and c > 0):
                pos = lane + tile * LANES
                logits = [l if w == 0 else jnp.where(pos >= DIL * w, l, -1e9)
                          for w, l in enumerate(logits)]
            m = _tree_sum(logits, jnp.maximum)
            p = [jnp.exp(l - m) for l in logits]
            r = 1.0 / _tree_sum(p)

            def apply(anchor2):
                ln = lane + _zero_like_dep(_tie(m, anchor2)).astype(jnp.int32)
                for dd in range(DP):
                    vc = cur[pl.ds(2 * RP + base + dd, 8, stride=DP), :]
                    vp = prev[pl.ds(2 * RP + base + dd, 8, stride=DP), :]
                    o0 = o1 = None
                    for w in range(W):
                        vs = shifted(ln, vc, vp, w)
                        t0, t1 = p[w] * _lo(vs), p[w] * _hi(vs)
                        o0 = t0 if o0 is None else o0 + t0
                        o1 = t1 if o1 is None else o1 + t1
                    o0, o1 = o0 * r, o1 * r
                    o_t[pl.ds(base + dd, 8, stride=DP), :] = o0
                    o_t[pl.ds(RP + base + dd, 8, stride=DP), :] = o1

            return apply

        def attention(blk, anchors):
            for c in range(NT):
                for hg in range(NG):
                    att_group(blk, c, hg, anchors[c * NG + hg])

        def wo_mm(blk, anchors, fast, stash=None, anchors_in=()):
            o = cat1(*[o_s[c] for c in range(NT)])
            if fast:
                y = att_mm(3, att_rhs(o, stash, anchors_in), anchors)
            else:
                o = o.astype(BF16)
                q = D2 // 2
                y = cat0(*[dot_k(slice(h * q, (h + 1) * q), o, anchors) for h in (6, 7)])
            xm = xio_s[blk].astype(F32) + y
            xmid_s[blk] = xm
            return _ln_stats((xm[r:r + 8] for r in range(0, D, 8)), D)

        def ffn_lhs(blk, stats, anchors):
            m, rs = stats
            m8 = jnp.broadcast_to(m, (8, TM))
            xt = []
            for k in range(5):
                mt = cat0(*[_tie(m8, spread_over(anchors[:2], k, 5))] * (KU // 8 if k == 4 else 16))
                x = (xmid_s[blk, k * LANES:min((k + 1) * LANES, D), :] - mt) * rs
                xt.append((cat0(x, x) if k == 4 else x).T)
            lo = lax.broadcasted_iota(jnp.int32, (TQ // 2, LANES), 1) < KU
            for m1 in range(7):
                a = spread_over(anchors[2:], m1, 7)
                blk1 = lambda i2, k2: _signed(_SA[m1], lambda i1, k1: _tie(
                    xt[k2 if k2 == 4 else 2 * k1 + k2][(2 * i1 + i2) * TQ:(2 * i1 + i2 + 1) * TQ], a))
                l1 = {(i2, k2): blk1(i2, k2) for i2 in range(2)
                      for k2 in ((0, 1, 4) if m1 in _SCOL else (0, 1))}
                for m2 in range(7):
                    v = _signed(_SA[m2], lambda i2, k2: l1[i2, k2])
                    if m1 in _SCOL and m2 in _SCOL:
                        c = _signed(_SA[m2], lambda i2, k2: l1[i2, 4])
                        h = TQ // 2
                        vp, vq, cp, cq = v[:h], v[h:], c[:h], c[h:]
                        v = cat0(jnp.where(lo, cp, vq), jnp.where(lo, vp, vp - vq),
                                 jnp.where(lo, vq, cq - cp))
                    o, ac = AOFF[m1, m2]
                    a_s[o:o + v.shape[0] // 2, ac] = _pk(v)

        def in_triple(q):
            return q, lambda k: (q, k)

        def cross_triple(s):
            return NP + s, lambda k: (3 * s + k, 3)

        def wd_raw(tri, k, r0, n):
            q, c = tri[1](k)
            return wdt_v[q, r0:r0 + n, c * LANES:(c + 1) * LANES]

        def ds_loc(i, r0, n):
            return slice(r0, r0 + n), slice((i % 2) * LANES, (i % 2 + 1) * LANES)

        def prep_d(tri, anchors):
            PR = 16
            for n in range(D3 // PR):
                r = n * PR
                w = [[wd_raw(tri, k, j * D3 + r, PR).astype(F32) for j in range(3)]
                     for k in range(3)]
                w[0][1] = _tie(w[0][1], spread_over(anchors, n, D3 // PR))
                for i, v in enumerate(_w_sums(w)):
                    ds_s.at[tri[0], i // 2][ds_loc(i, r // 2, PR // 2)] = _pk(v)

        GU = (wg_v, wu_v)

        def prep_gu(p, gv, m, m1s, anchors):
            PR = 16
            cs = slice(m * LANES, (m + 1) * LANES)
            for n in range(LANES // PR):
                r = n * PR
                cache = {}

                def w(k, j1):
                    if (k, j1) not in cache:
                        v = GU[m][p, k * LANES + r:k * LANES + r + PR,
                                  2 * j1 * LANES:2 * (j1 + 1) * LANES].astype(F32)
                        if (k // 2, j1) in [_SB[m1][0][:2] for m1 in m1s[:2]]:
                            a = spread_over(anchors, n, LANES // PR)
                            c = (k % 2) * LANES
                            tied = _tie(v[:, c:c + LANES], a)
                            v = cat1(v[:, :LANES], tied) if c else cat1(tied, v[:, LANES:])
                        cache[k, j1] = v
                    return cache[k, j1]

                for m1 in m1s:
                    b1 = [_signed(_SB[m1], lambda k1, j1: w(2 * k1 + k2, j1)) for k2 in range(2)]
                    for m2 in range(7):
                        v = _signed(_SB[m2],
                                    lambda k2, j2: b1[k2][:, j2 * LANES:(j2 + 1) * LANES])
                        gv.at[7 * m1 + m2][r // 2:(r + PR) // 2, cs] = _pk(v)

        def prep_tail(p, gv, m, anchor):
            v = _tie(GU[m][p, 4 * LANES:, :].astype(F32), anchor)
            for j in range(4):
                gv.at[49 + j // 2][(j % 2) * 32:(j % 2 + 1) * 32,
                                        m * LANES:(m + 1) * LANES] = _pk(
                                            v[:, j * LANES:(j + 1) * LANES])

        def gu_outer(gv, m, m1, anchors, at=(0, 4)):
            cs = slice(m * LANES, (m + 1) * LANES)
            y = {}
            for m2 in cfg['inner']:
                i, (o, ac) = 7 * m1 + m2, AOFF[m1, m2]
                if m1 in _SCOL and m2 in _SCOL:
                    j = 2 * _SCOL[m1] + _SCOL[m2]
                    tail = lambda: gv[49 + j // 2, (j % 2) * 32:(j % 2 + 1) * 32, cs]
                    rhs = (cat0(tail(), gv[i, 32:, cs]), gv[i, :, cs],
                           cat0(gv[i, :32, cs], tail()))
                    r = [_dot(_upk(a_s[o + 16 * s:o + 16 * (s + 1), ac]), _upk(rhs[s]))
                         for s in range(3)]
                    y[m2] = cat0(r[1] + r[0], r[2] + r[0])
                else:
                    y[m2] = _dot(_upk(a_s[o:o + TQ // 2, ac]), _upk(gv[i, :, cs]))
            anchors.extend(y[cfg['inner'][k % 7]][(k // 7) * 32:(k // 7) * 32 + 8] for k in at)
            return _s_out(y)

        def gu_finish(t):
            gu = [{(i2, j2): _s_out([t[m][m1][i2][j2] for m1 in range(7)])
                   for i2 in range(2) for j2 in range(2)} for m in range(2)]
            return [[cat0(*[_gelu_mul2(*[gu[m][i2, j % 2][i1][j // 2] for m in range(2)])
                            for i2 in range(2)]) for i1 in range(2)] for j in range(4)]

        def gu_piece(gv, order, anchors, at=(0, 4)):
            t = ({}, {})
            for m, m1 in order:
                t[m][m1] = gu_outer(gv, m, m1, anchors, at)
            return gu_finish(t)

        def prep_piece(p, gv, anchors, group):
            grp = _SGRP if group else [(m1,) for m1 in range(7)]
            k = len(anchors) // (2 * len(grp))
            for n in range(2 * len(grp)):
                prep_gu(p, gv, n % 2, grp[n // 2], anchors[k * n:k * n + k])
            for m in range(2):
                prep_tail(p, gv, m, anchors[m * len(anchors) // 2])

        def h_ops(h):
            return [v.astype(BF16) for v in _x_ops(*[[h[k][i] for k in range(3)]
                                                     for i in range(2)])]

        D_ORDER = _PAIR_ORDER + (9, 10, 11, 12, 13, 14)

        def down_mm(acc, work, anchors, which=D_ORDER):
            p = [None] * 15 if acc is None else list(acc)
            jobs = [(i, n) for i in which for n in range(len(work))]
            split = {0: (), 1: (4,), 2: (2, 2), 3: (2, 2, 4)}[len(jobs) % 4]
            split = dict(zip(jobs[len(jobs) - len(split):], split))
            for i in which:
                y = None
                for n, (tri, b) in enumerate(work):
                    ns = split.get((i, n), 1)
                    nr = D3 // ns
                    if i in _W_RAW:
                        k, j = _W_RAW[i]
                        lhs = lambda h: wd_raw(tri, k, j * D3 + h * nr, nr)
                    else:
                        s = _W_SUM[i]
                        lhs = lambda h: _upk(ds_s.at[tri[0], s // 2][ds_loc(s, h * nr // 2, nr // 2)])
                    v = cat0(*[_dot_nt(lhs(h), b[i]) for h in range(ns)])
                    y = v if y is None else y + v
                p[i] = y if p[i] is None else p[i] + y
                anchors.append(p[i][:8])
            return p

        def finish(blk, acc, after=None):
            y = [cat1(*_column(acc, [acc[_DIAG[s, j]] if (s, j) in _DIAG else None
                                     for s in range(3)], j)) for j in range(3)]
            if after is None:
                xio_s[blk] = (xmid_s[blk] + 0.5 * cat0(*y)).astype(BF16)
                return
            for j in range(3):
                rows = slice(j * D3, (j + 1) * D3)
                xio_s[blk, rows] = (xmid_s[blk, rows] + 0.5 * y[j]).astype(BF16)
                after(j)

        def load_acc(k):
            return [acc_s[k, i] for i in range(15)]

        def store_acc(k, acc):
            for i in range(15):
                acc_s[k, i] = acc[i]

        def pre_phase():
            first = [[x_cp(0, 0)], [wq_cp(0)], [x_cp(1, 2), wq_cp(1)],
                     [wq_cp(2), pltpu.make_async_copy(wo_hbm, wo_v, sem_i.at[3])]]
            order = sum(first, [])
            for p in range(NP + 1):
                order += group_cp(p)
            xr_cp = [x_cp(b, SEM_P + NP + 1) for b in range(2, NB)]
            order += xr_cp
            for cp in order:
                cp.start()
            get = lambda an, name: [an[min(i, len(an) - 1)] for i in cfg[name]]
            e_grp = lambda e: ((e >> 1) & 1, ((e >> 2) << 1) | (e & 1))
            if 'a' in cfg['sub']:
                pre_a(first, get, e_grp)
            if 'b' in cfg['sub']:
                pre_b(get, e_grp)
            if 'c' in cfg['sub']:
                pre_c(get)
            wait('WX', xr_cp)

        def pre_a(first, get, e_grp):
            def transpose_wq(i):
                wt_s[WQ[i] // 2:WQ[i + 1] // 2, :D] = _pk(wqkv_v[:, WQ[i]:WQ[i + 1]].T)

            def clear(i, carry):
                for k in range(2):
                    acc_s[k, i] = jnp.zeros((D3, TH), F32)
                r = jnp.minimum(i, 11) * (RP // 4)
                qkv_s[0, rows8(r, RP // 4)] = jnp.zeros((RP // 4, LANES), U32)
                return carry

            lax.fori_loop(0, 15, clear, 0)
            wait('WX0', first[0])
            xn0 = ln1(0, ()).astype(BF16)

            wait('WQ0', first[1])
            transpose_wq(0)
            qkv_mm(0, xn0, (0, 1), [])

            wait('WQ1', first[2])
            transpose_wq(1)
            an = []
            qkv_mm(0, xn0, (2, 3), an)
            xn1 = ln1(1, get(an, 'a_ln'), get(an, 'a_lnb')).astype(BF16)
            qkv_mm(1, xn1, (0,), an, True)
            for n, a in enumerate(get(an, 'a_w1')):
                prep_att(n, a)
            nk = len(cfg['a_k'])
            apply = [att_values(0, *e_grp(e), a) for e, a in enumerate(get(an, 'a_k'))]

            wait('WQ2', first[3])
            an = []
            qkv_mm(1, xn1, (2,), an)
            transpose_wq(2)
            qkv_mm(0, xn0, (4, 5), an)
            qkv_mm(1, xn1, (4,), an)
            qkv_mm(1, xn1, (1,), an, True)
            apply += [att_values(0, *e_grp(nk + e), a)
                      for e, a in enumerate(get(an, 'a_k2')[:8 - nk])]
            for e, a in enumerate(get(an, 'a_v')):
                apply[e](a)
            wo = pltpu.bitcast(wo_v[...], U32)
            wo = cat0(_lo(wo), _hi(wo))
            wo = cat0(*[_tie(wo[n * LANES:(n + 1) * LANES], a)
                        for n, a in enumerate(get(an, 'a_wo'))])
            wt_s[3 * RP:, :D] = _pk(wo.astype(BF16).T)
            for n, a in enumerate(get(an, 'a_w2')):
                prep_att(len(cfg['a_w1']) + n, a)

            wait('WO', group_cp(0))
            an = []
            stats = wo_mm(0, an, False)
            qkv_mm(1, xn1, (3, 5), an)
            for n, a in enumerate(get(an, 'z_w')):
                prep_att(36 + n, a)
            prep_piece(0, gu_s.at[0], get(an, 'z_g'), cfg['z_grp'])
            ffn_lhs(0, stats, get(an, 'z_l'))

        def pre_b(get, e_grp):
            def piece(p, carry):
                wait('WP', group_cp(p))
                an = []
                win = gu_s.at[pl.ds(p - 1, 2)]
                h = gu_piece(win.at[0], cfg['gorder0'], an, (0, 7, 4, 11))
                h3_s[p - 1] = cat0(*h[3])
                tri = in_triple(p - 1)
                prep_d(tri, get(an, 'p_d'))
                store_acc(0, down_mm(load_acc(0), [(tri, h_ops(h[:3]))], an))
                prep_piece(p, win.at[1], get(an, 'f_g'), cfg['f_grp'])
                att_group(1, *e_grp(p - 1), an[cfg['p_att'][0]])
                return carry

            lax.fori_loop(1, NP, piece, 0)

        def pre_c(get):
            wait('WD', group_cp(NP))
            an = []
            h = gu_piece(gu_s.at[NP - 1], cfg['torder'], an)
            h3 = [[h3_s[q, :TH], h3_s[q, TH:]] for q in range(NP - 1)] + [h[3]]
            work = [(cross_triple(s), h_ops(h3[3 * s:3 * s + 3])) for s in range(3)]
            work.append((in_triple(NP - 1), h_ops(h[:3])))
            stats = wo_mm(1, an, True)
            td = get(an, 't_d')
            for n, (tri, _) in enumerate(work):
                prep_d(tri, td[n * len(td) // 4:(n + 1) * len(td) // 4])
            acc = down_mm(load_acc(0), work, an)
            nw = len(cfg['a_w1']) + len(cfg['a_w2'])
            for n, a in enumerate(get(an, 't_w')[:36 - nw]):
                prep_att(nw + n, a)
            ffn_lhs(1, stats, get(an, 't_l'))
            finish(0, acc)

        if 'pre' in cfg['phases']:
            pre_phase()

        def body(u, carry):
            bu = u & (NB - 1)
            ba = (u + 1) & (NB - 1)
            acc, stats, an, b, hh = None, None, {}, {}, {}
            get = lambda name: [an[k][i] for k, i in cfg[name]]
            for step in cfg['body']:
                an[step] = []
                if step == 'Q':
                    xn = ln1(ba, get('ln1'), get('ln1b'))
                    qkv_fast(ba, att_rhs(xn, u >> 8), an[step])
                elif step == 'W':
                    attention(ba, get('att'))
                    stats = wo_mm(ba, an[step], True, u >> 8, get('orhs'))
                elif step == 'L':
                    ffn_lhs(ba, stats, get('lhs'))
                elif step[0] == 'G':
                    q, go = int(step[1]), cfg['gorder']
                    t = b.setdefault(step[:2], ({}, {}))
                    for m, m1 in (go[:7] if step[2] == '0' else go[7:]):
                        t[m][m1] = gu_outer(gu_s.at[q], m, m1, an[step])
                    if len(t[0]) + len(t[1]) == 14:
                        hh[q] = gu_finish(t)
                else:
                    work = []
                    for c in step[1:]:
                        if c.isdigit():
                            work.append((in_triple(int(c)), h_ops(hh[int(c)][:3])))
                        else:
                            s = ord(c) - ord('a')
                            work.append((cross_triple(s),
                                         h_ops([hh[3 * s + k][3] for k in range(3)])))
                    acc = down_mm(acc, work, an[step])
            finish(bu, acc)

            @pl.when(u >= NB)
            def _():
                out_copy(bu).start()
            return carry

        if scopes:
            with jax.named_scope('LOOP'):
                lax.fori_loop(1, NU - 1, body, 0)
        elif 'main' in cfg['phases']:
            lax.fori_loop(1, NU - 1, body, 0)

        fin_cp = [pltpu.make_async_copy(
            xio_s.at[NB - 1, pl.ds(j * D3, D3)],
            out_hbm.at[pl.ds(j * D3, D3), cols((NB - 1) * TM, TM)], sem_o.at[0])
            for j in range(3)]

        def last(s, carry):
            h = [gu_piece(gu_s.at[3 * s + k], cfg['lorder'], []) for k in range(3)]
            work = [(in_triple(3 * s + k), h_ops(h[k][:3])) for k in range(3)]
            work.append((cross_triple(s), h_ops([h[k][3] for k in range(3)])))
            acc = down_mm(down_mm(load_acc(1), work[:2], []), work[2:], [], cfg['ldord'])
            store_acc(1, acc)
            finish(NB - 1, acc, lambda j: pl.when(s == NP // 3 - 1)(fin_cp[j].start))
            return carry

        if 'last' in cfg['phases']:
            lax.fori_loop(0, NP // 3, last, 0)
        if len(cfg['phases']) < 3:
            def keep(i, c):
                v = (gu_s[i, i, :8, :LANES] + ds_s[i, i, :8, :LANES]
                     + wl_s[rows8(i * 8), :LANES] + a_s[rows8(i * 8), :LANES] + qkv_s[i, :8]
                     + wt_s[rows8(i * 8), :LANES])
                acc_s[1, 0, :8] = (lax.bitcast_convert_type(v, F32) + o_s[i, :8]
                                   + acc_s[i, i, :8] + h3_s[i, :8])
                return c
            lax.fori_loop(0, 2, keep, 0)
            finish(NB - 1, load_acc(1))
        wait('WOUT', [out_copy(b) for b in range(NB - 1)] + fin_cp)

    scratch = [
        pltpu.VMEM((NB, D, TM), BF16),
        pltpu.VMEM((D, 3 * D), BF16),
        pltpu.VMEM((D, D), BF16),
        pltpu.VMEM((NP, D, PW), BF16),
        pltpu.VMEM((NP, D, PW), BF16),
        pltpu.VMEM((NP, D, PW), BF16),
        pltpu.VMEM((2 * D, 8 * LANES), U32),
        pltpu.VMEM((4 * Q3, 16 * LANES), U32),
        pltpu.VMEM((NP, 51, 64, 2 * LANES), U32),
        pltpu.VMEM((NP + 3, 5, Q3, 2 * LANES), U32),
        pltpu.VMEM((NB, D, TM), F32),
        pltpu.VMEM((max(fill), 2 * LANES), U32),
        pltpu.VMEM((S // LANES + 1, 3 * RP, LANES), U32),
        pltpu.VMEM((NT, D, LANES), F32),
        pltpu.VMEM((2, 15, D3, TH), F32),
        pltpu.VMEM((NP, TM, LANES), F32),
        pltpu.VMEM((1, 9 * 64, 2 * LANES), U32),
        pltpu.SemaphoreType.DMA((SEM_P + NP + 2,)),
        pltpu.SemaphoreType.DMA((1,)),
    ]

    def wrapped(*refs):
        @pl.when(pl.program_id(0) == 0)
        def _():
            kernel(*refs)

    return wrapped, scratch


_CFG = dict(
    scopes=False, ldord=(1, 2, 0, 7, 8, 6, 9, 10, 4, 5, 3, 11, 12, 13, 14),
    orhs=(('G80', 0), ('G80', 1), ('G80', 2), ('G80', 3), ('G80', 4), ('G80', 5),
        ('G80', 6), ('G80', 7), ('G80', 8), ('G80', 9), ('G80', 10), ('G80', 11)),
    sub='abc',
    phases=('pre', 'main', 'last'),
    body=('G20', 'G00', 'G01', 'G10', 'G11', 'Q', 'G30', 'G21', 'G40', 'G31', 'G50',
        'D012a', 'G41', 'G51', 'D345b', 'G70', 'G60', 'G71', 'G80', 'W', 'G61', 'G81',
        'D8c', 'D67', 'L'),
    ln1=(('G00', 0), ('G00', 1), ('G00', 2), ('G00', 3), ('G00', 4), ('G00', 5), ('G00',
        6), ('G00', 7), ('G00', 8)),
    ln1b=(('G10', 1), ('G10', 2), ('G10', 3), ('G10', 4), ('G10', 5), ('G10', 6),
        ('G10', 7), ('G10', 8), ('G10', 9), ('G10', 10), ('G10', 11), ('G10', 12)),
    att=(('D012a', 2), ('D012a', 4), ('D012a', 5), ('D012a', 8), ('D012a', 9), ('D345b',
        5), ('D345b', 6), ('D345b', 8)),
    lhs=(('D8c', 2), ('D8c', 3), ('D8c', 9), ('D8c', 11), ('D67', 5), ('D67', 8),
        ('D67', 10), ('D67', 11), ('D67', 14)),
    a_w1=(0, 0, 1, 2, 2, 3, 3, 4, 5, 6, 7, 11, 13, 18, 19, 20, 21, 22, 23, 24, 26, 27,
        28, 29),
    a_w2=(25, 30, 33, 36, 44, 45),
    a_ln=(3, 6, 7),
    a_lnb=(3, 9, 15),
    z_g=(0, 0, 1, 1, 2, 2, 3, 3, 4, 4, 5, 5, 6, 6, 7, 7, 8, 8, 9, 11, 12, 12, 13, 14,
        14, 14, 15, 15, 16, 16, 17, 17, 18, 18, 19, 19, 20, 21, 21, 22, 23, 23, 23, 24,
        25, 26, 27, 33),
    t_d=(0, 0, 0, 2, 2, 4, 5, 5, 7, 7, 8, 8, 9, 10, 11, 11, 12, 12, 13, 14, 14, 15, 16,
        16, 17, 17, 18, 18, 21, 22, 24, 24, 25, 28, 28, 30, 32, 32, 35, 35, 36, 37, 37,
        37, 39, 40, 40, 42),
    p_d=(3, 12, 14, 17, 24, 25, 28, 33, 35, 38, 42, 46),
    p_att=(58,),
    z_l=(23, 23, 28, 31, 35, 36, 37, 37, 39),
    a_k=(13, 17, 20, 26),
    a_k2=(0, 1, 3, 9),
    a_v=(13, 13, 14, 15, 16, 17, 18, 19),
    a_wo=(9, 18, 25, 36, 46),
    inner=(0, 3, 4, 6, 2, 1, 5),
    gorder=((0, 4), (0, 0), (1, 4), (1, 0), (1, 6), (0, 3), (1, 3), (0, 6), (0, 1), (1,
        1), (0, 2), (1, 2), (0, 5), (1, 5)),
    gorder0=((0, 0), (1, 4), (0, 4), (1, 0), (0, 3), (0, 6), (1, 6), (1, 3), (1, 1), (0,
        1), (0, 2), (0, 5), (1, 5), (1, 2)),
    f_g=(0, 0, 1, 2, 5, 5, 6, 7, 8, 9, 9, 10, 12, 13, 14, 16, 17, 17, 19, 20, 21, 23,
        24, 24, 26, 28, 29, 31, 32, 35, 36, 37, 37, 40, 40, 42, 43, 44, 45, 47, 48, 48,
        53, 56, 58, 59, 60, 61, 62, 62, 64, 64, 69, 70, 70, 70),
    t_l=(49, 50, 51, 53, 54, 55, 57, 57, 60),
    lorder=((1, 0), (1, 4), (0, 0), (0, 4), (0, 3), (0, 6), (1, 3), (1, 6), (0, 1), (1,
        1), (0, 2), (0, 5), (1, 2), (1, 5)),
    z_w=(1, 1, 3, 3, 5, 5, 6, 6, 8, 9, 17, 35),
    z_grp=1,
    f_grp=0,
    t_w=(47, 49, 49, 50, 52, 54),
    torder=((0, 0), (0, 4), (1, 4), (1, 0), (0, 3), (1, 3), (1, 6), (0, 6), (0, 1), (1,
        1), (0, 2), (1, 2), (0, 5), (1, 5)),
)


def _run(A_x, A_wqkv, A_wo, B_w_gate, B_w_up, B_w_down, **kw):
    _, S, D = A_x.shape
    F = B_w_gate.shape[1]
    kernel, scratch = _make_kernel(S, D, F, 256, {**_CFG, **kw})
    hbm = pl.BlockSpec(memory_space=pl.ANY)
    out_t = pl.pallas_call(
        kernel,
        grid=(2,),
        in_specs=[hbm] * 6,
        out_specs=hbm,
        out_shape=jax.ShapeDtypeStruct((D, S), A_x.dtype),
        scratch_shapes=scratch,
        compiler_params=pltpu.CompilerParams(
            dimension_semantics=('arbitrary',), vmem_limit_bytes=110 * 1024 * 1024),
    )(A_x.reshape(S, D).T, A_wqkv, A_wo, B_w_gate, B_w_up, B_w_down.T)
    return out_t.T.reshape(A_x.shape)


@jax.jit
def pallas_interleave_layers__sliding_local_dilated__glu_gated_geglu__prompt_kernel(
    A_x: jax.Array,
    A_wqkv: jax.Array,
    A_wo: jax.Array,
    B_x: jax.Array,
    B_w_gate: jax.Array,
    B_w_up: jax.Array,
    B_w_down: jax.Array,
):
    del B_x
    return _run(A_x, A_wqkv, A_wo, B_w_gate, B_w_up, B_w_down)
```

```python
import jax
import jax.numpy as jnp
import jax.experimental.pallas as pl
import jax.experimental.pallas.tpu as pltpu
from jax import lax

H = 32
W = 8
DIL = 2
EPS = 1e-5
LANES = 128

F32 = jnp.float32
BF16 = jnp.bfloat16
U32 = jnp.uint32

_NT = (((1,), (1,)), ((), ()))


def _tree_sum(parts, op=jnp.add):
    while len(parts) > 1:
        nxt = [op(parts[i], parts[i + 1]) for i in range(0, len(parts) - 1, 2)]
        if len(parts) % 2:
            nxt.append(parts[-1])
        parts = nxt
    return parts[0]


def _ln_stats(slabs, d, anchors=()):
    n_acc = 4
    s1, s2, pilot = [None] * n_acc, [None] * n_acc, None
    for i, x in enumerate(slabs):
        if pilot is None:
            pilot = x[0:1, :]
            pil = jnp.broadcast_to(pilot, x.shape)
            pils = [_tie(pil, a) for a in anchors] or [pil]
        dx = x - pils[i * len(pils) // (d // 8)]
        j = i % n_acc
        s1[j] = dx if s1[j] is None else s1[j] + dx
        s2[j] = dx * dx if s2[j] is None else s2[j] + dx * dx
    e1 = jnp.sum(_tree_sum(s1), axis=0, keepdims=True) * (1.0 / d)
    e2 = jnp.sum(_tree_sum(s2), axis=0, keepdims=True) * (1.0 / d)
    var = jnp.maximum(e2 - e1 * e1, 0.0)
    return pilot + e1, lax.rsqrt(var + EPS)


def _zero_like_dep(v):
    return (lax.bitcast_convert_type(v, U32) >> 31) >> 1


def _tie(x, anchor):
    if anchor is None:
        return x
    z = lax.bitcast_convert_type(_zero_like_dep(anchor), F32)
    z = jnp.concatenate([z] * -(-x.shape[1] // LANES), axis=1)[:, :x.shape[1]]
    if x.shape[0] == 8:
        return x + z
    return jnp.concatenate([x[:8] + z, x[8:]], axis=0)


def _gelu_mul2(g, u):
    c0 = 0.7978845608028654
    c1 = c0 * 0.044715
    t = jnp.tanh(g * (c0 + c1 * (g * g)))
    return (g * u) * (1.0 + t)


def _lo(x):
    return lax.bitcast_convert_type(x << 16, F32)


def _hi(x):
    return lax.bitcast_convert_type(x & jnp.uint32(0xFFFF0000), F32)


def _pk(x):
    return pltpu.bitcast(x.astype(BF16), U32)


def _upk(x):
    return pltpu.bitcast(x, BF16)


def _dot(a, b):
    return jnp.dot(a, b, preferred_element_type=F32)


def _dot_nt(a, b):
    return lax.dot_general(a, b, _NT, preferred_element_type=F32)


def _x_ops(x1, x2):
    d = [a - b for a, b in zip(x1, x2)]
    return [x1[0] + x2[1], x2[0] + x2[1], x1[0] + x1[1],
            d[1] + x1[2], x1[1] + x1[2], d[1] + d[2],
            d[0] - x2[2], d[0] + d[2], x2[0] + x2[2],
            x1[0], d[0], x2[1], d[1], x1[2], x2[2]]


def _x_rem(x1, x2):
    a, b, c = 0, 1, 2
    cat = lambda u, v: jnp.concatenate([u, v], axis=0)
    return [cat(x1[c], x2[b]), cat(x1[a], x1[b] - x2[b]), cat(x2[a], x2[c] - x1[c])]


_W_TERMS = {0: ((0, 1, 1), (1, 0, 1)), 3: ((1, 2, 1), (2, 1, 1)), 6: ((0, 2, 1), (2, 0, 1)),
            9: ((0, 0, 1), (0, 2, 1), (1, 0, -1)), 10: ((2, 0, 1), (0, 0, -1), (0, 1, -1)),
            11: ((1, 1, 1), (1, 2, 1), (0, 1, -1)), 12: ((1, 0, 1), (1, 1, 1), (2, 1, -1)),
            13: ((2, 0, 1), (2, 2, 1), (1, 2, -1)), 14: ((2, 1, 1), (2, 2, 1), (0, 2, -1)),
            1: ((0, 1, 1),), 2: ((1, 0, 1),), 4: ((1, 2, 1),), 5: ((2, 1, 1),),
            7: ((2, 0, 1),), 8: ((0, 2, 1),)}


def _w_sums(w):
    return [_signed(_W_TERMS[i], lambda k, j: w[k][j]) for i in _W_SUM]


_W_SUM = {0: 0, 3: 1, 6: 2, 9: 3, 10: 4, 11: 5, 12: 6, 13: 7, 14: 8}
_W_RAW = {1: (0, 1), 2: (1, 0), 4: (1, 2), 5: (2, 1), 7: (2, 0), 8: (0, 2)}
_PAIR_ORDER = (1, 2, 4, 5, 7, 8, 0, 3, 6)
_DIAG = {(0, 0): 9, (2, 0): 10, (0, 1): 11, (1, 1): 12, (1, 2): 13, (2, 2): 14}
_PAIR = {(0, 0): ((6, -1), (8, -1)), (1, 0): ((2, 1), (7, 1)), (2, 0): ((0, 1), (1, -1)),
         (0, 1): ((3, 1), (4, -1)), (1, 1): ((0, 1), (2, -1)), (2, 1): ((1, 1), (5, -1)),
         (0, 2): ((4, 1), (8, 1)), (1, 2): ((6, 1), (7, -1)), (2, 2): ((5, 1), (3, -1))}


def _column(t, base, j, skew=False):
    s = []
    for k in range(3):
        v = base[k]
        for i, sg in _PAIR[k, j]:
            v = t[i] if v is None else (v + t[i] if sg > 0 else v - t[i])
        s.append(v)
    if skew:
        return s[1] + s[0], s[2] + 0.5 * (s[0] - s[1])
    return s[1] + s[0], s[2] + s[0]


_SA = (((0, 0, 1), (1, 1, 1)), ((1, 0, 1), (1, 1, 1)), ((0, 0, 1),), ((1, 1, 1),),
       ((0, 0, 1), (0, 1, 1)), ((1, 0, 1), (0, 0, -1)), ((0, 1, 1), (1, 1, -1)))
_SB = (((0, 0, 1), (1, 1, 1)), ((0, 0, 1),), ((0, 1, 1), (1, 1, -1)), ((1, 0, 1), (0, 0, -1)),
       ((1, 1, 1),), ((0, 0, 1), (0, 1, 1)), ((1, 0, 1), (1, 1, 1)))
_SCOL = {2: 1, 3: 0, 5: 1, 6: 0}
_SGRP = ((1, 4, 0), (3, 6), (2, 5))


def _signed(terms, f):
    v = None
    for a, b, sg in terms:
        v = f(a, b) if v is None else (v + f(a, b) if sg > 0 else v - f(a, b))
    return v


def _s_out(m):
    return [[m[0] + m[3] - m[4] + m[6], m[2] + m[4]],
            [m[1] + m[3], m[0] - m[1] + m[2] + m[5]]]


def _make_kernel(S, D, F, TM, cfg):
    NB = S // TM
    NT = TM // LANES
    DH = D // H
    DP = DH // 2
    RP = D // 2
    NG = H // 8
    scale = float(DH) ** -0.5
    NU = 2 * NB
    TH = TM // 2
    TQ = TM // 4
    D2 = D // 2
    D3 = D // 3
    Q3 = D3 // 2
    KU = D // 9
    KR = 3 * LANES
    NQ = 6
    QR = 3 * D // NQ
    WQ = (0, 640, 1152, 3 * D)
    PW = 4 * LANES
    NP = F // PW
    AOFF, fill = {}, [0, 0]
    for key in [(m1, m2) for m1 in range(7) for m2 in range(7)]:
        c = int(fill[1] < fill[0])
        AOFF[key] = (fill[c], slice(c * LANES, (c + 1) * LANES))
        fill[c] += 48 if key[0] in _SCOL and key[1] in _SCOL else 32
    scopes = cfg['scopes']
    assert NG == 4 and NB & (NB - 1) == 0
    SEM_P = 4

    def kernel(x_hbm, wqkv_hbm, wo_hbm, wg_hbm, wu_hbm, wdt_hbm, out_hbm,
               xio_s, wqkv_v, wo_v, wg_v, wu_v, wdt_v, wt_s, wl_s,
               gu_s, ds_s, xmid_s, a_s, qkv_s, o_s, acc_s, h3_s, r_s,
               sem_i, sem_o):

        def wait(name, cps):
            if scopes:
                with jax.named_scope(name):
                    for cp in cps:
                        cp.wait()
            else:
                for cp in cps:
                    cp.wait()

        def cols(lo, n):
            if not isinstance(lo, int):
                lo = pl.multiple_of(lo, LANES)
            return pl.ds(lo, n)

        def rows8(lo, n=8):
            if not isinstance(lo, int):
                lo = pl.multiple_of(lo, 8)
            return pl.ds(lo, n)

        def out_copy(b):
            return pltpu.make_async_copy(
                xio_s.at[b], out_hbm.at[:, cols(b * TM, TM)], sem_o.at[0])

        def x_cp(b, sem):
            return pltpu.make_async_copy(x_hbm.at[:, cols(b * TM, TM)], xio_s.at[b],
                                         sem_i.at[sem])

        def wq_cp(i):
            sl = cols(WQ[i], WQ[i + 1] - WQ[i])
            return pltpu.make_async_copy(wqkv_hbm.at[:, sl], wqkv_v.at[:, sl],
                                         sem_i.at[1 + i])

        def piece_cp(src, dst, p, sem, c0=0, n=PW):
            return pltpu.make_async_copy(src.at[:, cols(p * PW + c0, n)],
                                         dst.at[p, :, pl.ds(c0, n)], sem_i.at[sem])

        def group_cp(p):
            sem = SEM_P + p
            cps = []
            if not (isinstance(p, int) and p == NP):
                cps += [piece_cp(wg_hbm, wg_v, p, sem), piece_cp(wu_hbm, wu_v, p, sem)]
            if not (isinstance(p, int) and p == 0):
                cps.append(piece_cp(wdt_hbm, wdt_v, p - 1, sem, 0, KR))
            if isinstance(p, int) and p == NP:
                cps += [piece_cp(wdt_hbm, wdt_v, q, sem, KR, LANES) for q in range(NP)]
            return cps

        lane = lax.broadcasted_iota(jnp.int32, (8, LANES), 1)
        cat0 = lambda *v: jnp.concatenate(v, axis=0)
        cat1 = lambda *v: jnp.concatenate(v, axis=1)

        def spread_over(anchors, n, total):
            return anchors[n * len(anchors) // total] if anchors else None

        def slab_group(r):
            return (r % LANES) // 16 if r < KR else 8 + ((r - KR) % KU) // 16

        def ln1(blk, anchors1, anchors2=()):
            slabs = (xio_s[blk, r:r + 8, :].astype(F32) for r in range(0, D, 8))
            m, rs = _ln_stats(slabs, D, anchors1)
            if not anchors2:
                return (xio_s[blk].astype(F32) - m) * rs
            m8 = jnp.broadcast_to(m, (8, TM))
            ms = [_tie(m8, a) for a in anchors2]
            ms = [spread_over(ms, slab_group(r), 12) for r in range(0, D, 8)]
            return (xio_s[blk].astype(F32) - cat0(*ms)) * rs

        def dot_k(rows, x, anchors, even=False):
            y = None
            for n, k in enumerate(range(0, D, LANES)):
                ks = slice(k, min(k + LANES, D))
                if even and k + LANES >= D:
                    mid = (rows.start + rows.stop) // 2
                    v = cat0(_dot(_upk(wt_s[rows.start:mid, ks]), x[ks]),
                             _dot(_upk(wt_s[mid:rows.stop, ks]), x[ks]))
                else:
                    v = _dot(_upk(wt_s[rows, ks]), x[ks])
                anchors.extend(v[r:r + 8, :LANES] for r in ((0, 144) if n % 2 else (72, 216)))
                y = v if y is None else y + v
            return y

        def put_qkv(blk, rows, y):
            pk = _pk(y)
            for c in range(NT):
                qkv_s[1 + blk * NT + c, rows, :] = pk[:, c * LANES:(c + 1) * LANES]

        def qkv_mm(blk, xn, chunks, anchors, even=False):
            for r in chunks:
                rows = slice(r * QR // 2, (r + 1) * QR // 2)
                put_qkv(blk, rows, dot_k(rows, xn, anchors, even))

        def split_k(x):
            hs = (x[:, :TH], x[:, TH:])
            blocks = [[h[k * LANES:(k + 1) * LANES] for k in range(3)] for h in hs]
            units = [[h[KR + k * KU:KR + (k + 1) * KU] for k in range(3)] for h in hs]
            return blocks, units

        def prep_att(pat, anchor):
            assert Q3 == 96
            row0 = pat * 8
            src0 = row0 + ((pat * 43) >> 9) * (2 * Q3)
            w = [_upk(wt_s[rows8(src0 + j * Q3), :D]).astype(F32) for j in range(3)]
            w[0] = cat1(_tie(w[0][:, :LANES], anchor), w[0][:, LANES:])
            tiles = _w_sums([[w[j][:, k * LANES:(k + 1) * LANES] for j in range(3)]
                             for k in range(3)])
            for j in range(3):
                a, b, c = (w[j][:, KR + k * KU:KR + (k + 1) * KU] for k in range(3))
                tiles += [cat1(c, b), cat1(a, c)]
            wl_s[rows8(row0), :15 * LANES] = _pk(cat1(*tiles))

        def att_rhs(x, stash=None, anchors=()):
            half = 0.5
            if anchors:
                hs = [_tie(jnp.full((8, TH), 0.5, F32), a) for a in anchors]
                half = cat0(*[spread_over(hs, slab_group(r), 12) for r in range(0, D, 8)])
            blocks, units = split_k(cat1(x[:, :TH], x[:, TH:] + half * x[:, :TH]))
            ops = _x_ops(*blocks) + _x_rem(*units)
            if stash is None:
                return [v.astype(BF16) for v in ops]
            loc = lambda i, r0, n: (slice((i // 2) * 64 + r0, (i // 2) * 64 + r0 + n),
                                    slice((i % 2) * LANES, (i % 2 + 1) * LANES))
            for r in range(0, LANES, 16):
                for i, v in enumerate(ops):
                    r_s.at[0][loc(i, r // 2, 8)] = _pk(v[r:r + 16])
            return [_upk(r_s.at[stash][loc(i, 0, 64)]) for i in range(18)]

        def att_mm(sec, rhs, anchors):
            tl = lambda i: _upk(wl_s[sec * Q3:(sec + 1) * Q3, i * LANES:(i + 1) * LANES])
            raw = lambda k, j: _upk(wt_s[(3 * sec + j) * Q3:(3 * sec + j + 1) * Q3,
                                         k * LANES:(k + 1) * LANES])
            t = {}
            for i in _PAIR_ORDER:
                t[i] = _dot(raw(*_W_RAW[i]) if i in _W_RAW else tl(_W_SUM[i]), rhs[i])
                anchors.append(t[i][:8])
            out = []
            for j in range(3):
                base = []
                for s in range(3):
                    v = _dot(raw(3, j) if s == 1 else tl(9 + 2 * j + s // 2), rhs[15 + s])
                    if (s, j) in _DIAG:
                        i = _DIAG[s, j]
                        v = _dot(tl(_W_SUM[i]), rhs[i]) + v
                    base.append(v)
                    anchors.append(base[-1][:8])
                out.append(cat1(*_column(t, base, j, True)))
            return cat0(*out)

        def qkv_fast(blk, rhs, anchors):
            for sec in range(3):
                put_qkv(blk, slice(sec * RP, (sec + 1) * RP), att_mm(sec, rhs, anchors))

        def shifted(ln, cur, prev, w):
            if w == 0:
                return cur
            sh = DIL * w
            return pltpu.roll(jnp.where(ln < LANES - sh, cur, prev), sh, axis=1)

        def att_group(blk, c, hg, anchor):
            att_values(blk, c, hg, anchor)(None)

        def att_values(blk, c, hg, anchor):
            tile = blk * NT + c
            base = hg * 8 * DP
            if isinstance(hg, int):
                cur, prev, o_t = qkv_s.at[1 + tile], qkv_s.at[tile], o_s.at[c]
            else:
                n = 2 * RP + 8 * DP
                base = pl.multiple_of(base, 8)
                cur = qkv_s.at[1 + tile, pl.ds(base, n)]
                prev = qkv_s.at[tile, pl.ds(base, n)]
                o_t = o_s.at[c, pl.ds(base, RP + 8 * DP)]
                base = 0
            ln = lane + _zero_like_dep(anchor).astype(jnp.int32)
            logits = [None] * W
            for dd in range(DP):
                q = cur[pl.ds(base + dd, 8, stride=DP), :]
                kc = cur[pl.ds(RP + base + dd, 8, stride=DP), :]
                kp = prev[pl.ds(RP + base + dd, 8, stride=DP), :]
                q0, q1 = _lo(q), _hi(q)
                for w in range(W):
                    ks = shifted(ln, kc, kp, w)
                    t = q0 * _lo(ks) + q1 * _hi(ks)
                    logits[w] = t if logits[w] is None else logits[w] + t
            logits = [l * scale for l in logits]
            if not (isinstance(c, int) and c > 0):
                pos = lane + tile * LANES
                logits = [l if w == 0 else jnp.where(pos >= DIL * w, l, -1e9)
                          for w, l in enumerate(logits)]
            m = _tree_sum(logits, jnp.maximum)
            p = [jnp.exp(l - m) for l in logits]
            r = 1.0 / _tree_sum(p)

            def apply(anchor2):
                ln = lane + _zero_like_dep(_tie(m, anchor2)).astype(jnp.int32)
                for dd in range(DP):
                    vc = cur[pl.ds(2 * RP + base + dd, 8, stride=DP), :]
                    vp = prev[pl.ds(2 * RP + base + dd, 8, stride=DP), :]
                    o0 = o1 = None
                    for w in range(W):
                        vs = shifted(ln, vc, vp, w)
                        t0, t1 = p[w] * _lo(vs), p[w] * _hi(vs)
                        o0 = t0 if o0 is None else o0 + t0
                        o1 = t1 if o1 is None else o1 + t1
                    o0, o1 = o0 * r, o1 * r
                    o_t[pl.ds(base + dd, 8, stride=DP), :] = o0
                    o_t[pl.ds(RP + base + dd, 8, stride=DP), :] = o1

            return apply

        def attention(blk, anchors):
            for c in range(NT):
                for hg in range(NG):
                    att_group(blk, c, hg, anchors[c * NG + hg])

        def wo_mm(blk, anchors, fast, stash=None, anchors_in=()):
            o = cat1(*[o_s[c] for c in range(NT)])
            if fast:
                y = att_mm(3, att_rhs(o, stash, anchors_in), anchors)
            else:
                o = o.astype(BF16)
                q = D2 // 2
                y = cat0(*[dot_k(slice(h * q, (h + 1) * q), o, anchors) for h in (6, 7)])
            xm = xio_s[blk].astype(F32) + y
            xmid_s[blk] = xm
            return _ln_stats((xm[r:r + 8] for r in range(0, D, 8)), D)

        def ffn_lhs(blk, stats, anchors):
            m, rs = stats
            m8 = jnp.broadcast_to(m, (8, TM))
            xt = []
            for k in range(5):
                mt = cat0(*[_tie(m8, spread_over(anchors[:2], k, 5))] * (KU // 8 if k == 4 else 16))
                x = (xmid_s[blk, k * LANES:min((k + 1) * LANES, D), :] - mt) * rs
                xt.append((cat0(x, x) if k == 4 else x).T)
            lo = lax.broadcasted_iota(jnp.int32, (TQ // 2, LANES), 1) < KU
            for m1 in range(7):
                a = spread_over(anchors[2:], m1, 7)
                blk1 = lambda i2, k2: _signed(_SA[m1], lambda i1, k1: _tie(
                    xt[k2 if k2 == 4 else 2 * k1 + k2][(2 * i1 + i2) * TQ:(2 * i1 + i2 + 1) * TQ], a))
                l1 = {(i2, k2): blk1(i2, k2) for i2 in range(2)
                      for k2 in ((0, 1, 4) if m1 in _SCOL else (0, 1))}
                for m2 in range(7):
                    v = _signed(_SA[m2], lambda i2, k2: l1[i2, k2])
                    if m1 in _SCOL and m2 in _SCOL:
                        c = _signed(_SA[m2], lambda i2, k2: l1[i2, 4])
                        h = TQ // 2
                        vp, vq, cp, cq = v[:h], v[h:], c[:h], c[h:]
                        v = cat0(jnp.where(lo, cp, vq), jnp.where(lo, vp, vp - vq),
                                 jnp.where(lo, vq, cq - cp))
                    o, ac = AOFF[m1, m2]
                    a_s[o:o + v.shape[0] // 2, ac] = _pk(v)

        def in_triple(q):
            return q, lambda k: (q, k)

        def cross_triple(s):
            return NP + s, lambda k: (3 * s + k, 3)

        def wd_raw(tri, k, r0, n):
            q, c = tri[1](k)
            return wdt_v[q, r0:r0 + n, c * LANES:(c + 1) * LANES]

        def ds_loc(i, r0, n):
            return slice(r0, r0 + n), slice((i % 2) * LANES, (i % 2 + 1) * LANES)

        def prep_d(tri, anchors):
            PR = 16
            for n in range(D3 // PR):
                r = n * PR
                w = [[wd_raw(tri, k, j * D3 + r, PR).astype(F32) for j in range(3)]
                     for k in range(3)]
                w[0][1] = _tie(w[0][1], spread_over(anchors, n, D3 // PR))
                for i, v in enumerate(_w_sums(w)):
                    ds_s.at[tri[0], i // 2][ds_loc(i, r // 2, PR // 2)] = _pk(v)

        GU = (wg_v, wu_v)

        def prep_gu(p, gv, m, m1s, anchors):
            PR = 16
            cs = slice(m * LANES, (m + 1) * LANES)
            for n in range(LANES // PR):
                r = n * PR
                cache = {}

                def w(k, j1):
                    if (k, j1) not in cache:
                        v = GU[m][p, k * LANES + r:k * LANES + r + PR,
                                  2 * j1 * LANES:2 * (j1 + 1) * LANES].astype(F32)
                        if (k // 2, j1) in [_SB[m1][0][:2] for m1 in m1s[:2]]:
                            a = spread_over(anchors, n, LANES // PR)
                            c = (k % 2) * LANES
                            tied = _tie(v[:, c:c + LANES], a)
                            v = cat1(v[:, :LANES], tied) if c else cat1(tied, v[:, LANES:])
                        cache[k, j1] = v
                    return cache[k, j1]

                for m1 in m1s:
                    b1 = [_signed(_SB[m1], lambda k1, j1: w(2 * k1 + k2, j1)) for k2 in range(2)]
                    for m2 in range(7):
                        v = _signed(_SB[m2],
                                    lambda k2, j2: b1[k2][:, j2 * LANES:(j2 + 1) * LANES])
                        gv.at[7 * m1 + m2][r // 2:(r + PR) // 2, cs] = _pk(v)

        def prep_tail(p, gv, m, anchor):
            v = _tie(GU[m][p, 4 * LANES:, :].astype(F32), anchor)
            for j in range(4):
                gv.at[49 + j // 2][(j % 2) * 32:(j % 2 + 1) * 32,
                                        m * LANES:(m + 1) * LANES] = _pk(
                                            v[:, j * LANES:(j + 1) * LANES])

        def gu_outer(gv, m, m1, anchors, at=(0, 4)):
            cs = slice(m * LANES, (m + 1) * LANES)
            y = {}
            for m2 in cfg['inner']:
                i, (o, ac) = 7 * m1 + m2, AOFF[m1, m2]
                if m1 in _SCOL and m2 in _SCOL:
                    j = 2 * _SCOL[m1] + _SCOL[m2]
                    tail = lambda: gv[49 + j // 2, (j % 2) * 32:(j % 2 + 1) * 32, cs]
                    rhs = (cat0(tail(), gv[i, 32:, cs]), gv[i, :, cs],
                           cat0(gv[i, :32, cs], tail()))
                    r = [_dot(_upk(a_s[o + 16 * s:o + 16 * (s + 1), ac]), _upk(rhs[s]))
                         for s in range(3)]
                    y[m2] = cat0(r[1] + r[0], r[2] + r[0])
                else:
                    y[m2] = _dot(_upk(a_s[o:o + TQ // 2, ac]), _upk(gv[i, :, cs]))
            anchors.extend(y[cfg['inner'][k % 7]][(k // 7) * 32:(k // 7) * 32 + 8] for k in at)
            return _s_out(y)

        def gu_finish(t):
            gu = [{(i2, j2): _s_out([t[m][m1][i2][j2] for m1 in range(7)])
                   for i2 in range(2) for j2 in range(2)} for m in range(2)]
            return [[cat0(*[_gelu_mul2(*[gu[m][i2, j % 2][i1][j // 2] for m in range(2)])
                            for i2 in range(2)]) for i1 in range(2)] for j in range(4)]

        def gu_piece(gv, order, anchors, at=(0, 4)):
            t = ({}, {})
            for m, m1 in order:
                t[m][m1] = gu_outer(gv, m, m1, anchors, at)
            return gu_finish(t)

        def prep_piece(p, gv, anchors, group):
            if group in (0, 1):
                grp = _SGRP if group else [(m1,) for m1 in range(7)]
                k = len(anchors) // (2 * len(grp))
                for n in range(2 * len(grp)):
                    prep_gu(p, gv, n % 2, grp[n // 2], anchors[k * n:k * n + k])
            else:
                k, n = len(anchors) // 14, 0
                for g in group:
                    for m in range(2):
                        prep_gu(p, gv, m, g, anchors[n:n + k * len(g)])
                        n += k * len(g)
            for m in range(2):
                prep_tail(p, gv, m, anchors[m * len(anchors) // 2])

        def h_ops(h):
            return [v.astype(BF16) for v in _x_ops(*[[h[k][i] for k in range(3)]
                                                     for i in range(2)])]

        D_ORDER = _PAIR_ORDER + (9, 10, 11, 12, 13, 14)

        def down_mm(acc, work, anchors, which=D_ORDER):
            p = [None] * 15 if acc is None else list(acc)
            jobs = [(i, n) for i in which for n in range(len(work))]
            split = {0: (), 1: (4,), 2: (2, 2), 3: (2, 2, 4)}[len(jobs) % 4]
            split = dict(zip(jobs[len(jobs) - len(split):], split))
            for i in which:
                y = None
                for n, (tri, b) in enumerate(work):
                    ns = split.get((i, n), 1)
                    nr = D3 // ns
                    if i in _W_RAW:
                        k, j = _W_RAW[i]
                        lhs = lambda h: wd_raw(tri, k, j * D3 + h * nr, nr)
                    else:
                        s = _W_SUM[i]
                        lhs = lambda h: _upk(ds_s.at[tri[0], s // 2][ds_loc(s, h * nr // 2, nr // 2)])
                    v = cat0(*[_dot_nt(lhs(h), b[i]) for h in range(ns)])
                    y = v if y is None else y + v
                p[i] = y if p[i] is None else p[i] + y
                anchors.append(p[i][:8])
            return p

        def finish(blk, acc, after=None):
            y = [cat1(*_column(acc, [acc[_DIAG[s, j]] if (s, j) in _DIAG else None
                                     for s in range(3)], j)) for j in range(3)]
            if after is None:
                xio_s[blk] = (xmid_s[blk] + 0.5 * cat0(*y)).astype(BF16)
                return
            for j in range(3):
                rows = slice(j * D3, (j + 1) * D3)
                xio_s[blk, rows] = (xmid_s[blk, rows] + 0.5 * y[j]).astype(BF16)
                after(j)

        def load_acc(k):
            return [acc_s[k, i] for i in range(15)]

        def store_acc(k, acc):
            for i in range(15):
                acc_s[k, i] = acc[i]

        def pre_phase():
            first = [[x_cp(0, 0)], [wq_cp(0)], [x_cp(1, 2), wq_cp(1)],
                     [wq_cp(2), pltpu.make_async_copy(wo_hbm, wo_v, sem_i.at[3])]]
            order = sum(first, [])
            for p in range(NP + 1):
                order += group_cp(p)
            xr_cp = [x_cp(b, SEM_P + NP + 1) for b in range(2, NB)]
            order += xr_cp
            for cp in order:
                cp.start()
            get = lambda an, name: [an[min(i, len(an) - 1)] for i in cfg[name]]
            e_grp = lambda e: ((e >> 1) & 1, ((e >> 2) << 1) | (e & 1))
            if 'a' in cfg['sub']:
                pre_a(first, get, e_grp)
            if 'b' in cfg['sub']:
                pre_b(get, e_grp)
            if 'c' in cfg['sub']:
                pre_c(get)
            wait('WX', xr_cp)

        def pre_a(first, get, e_grp):
            def transpose_wq(i):
                wt_s[WQ[i] // 2:WQ[i + 1] // 2, :D] = _pk(wqkv_v[:, WQ[i]:WQ[i + 1]].T)

            def clear(i, carry):
                for k in range(2):
                    acc_s[k, i] = jnp.zeros((D3, TH), F32)
                r = jnp.minimum(i, 11) * (RP // 4)
                qkv_s[0, rows8(r, RP // 4)] = jnp.zeros((RP // 4, LANES), U32)
                return carry

            lax.fori_loop(0, 15, clear, 0)
            wait('WX0', first[0])
            xn0 = ln1(0, ()).astype(BF16)

            wait('WQ0', first[1])
            transpose_wq(0)
            qkv_mm(0, xn0, (0, 1), [])

            wait('WQ1', first[2])
            transpose_wq(1)
            an = []
            qkv_mm(0, xn0, (2, 3), an)
            xn1 = ln1(1, get(an, 'a_ln'), get(an, 'a_lnb')).astype(BF16)
            qkv_mm(1, xn1, (0,), an, True)
            for n, a in enumerate(get(an, 'a_w1')):
                prep_att(n, a)
            nk = len(cfg['a_k'])
            apply = [att_values(0, *e_grp(e), a) for e, a in enumerate(get(an, 'a_k'))]

            wait('WQ2', first[3])
            an = []
            qkv_mm(1, xn1, (2,), an)
            transpose_wq(2)
            qkv_mm(0, xn0, (4, 5), an)
            qkv_mm(1, xn1, (4,), an)
            qkv_mm(1, xn1, (1,), an, True)
            apply += [att_values(0, *e_grp(nk + e), a)
                      for e, a in enumerate(get(an, 'a_k2')[:8 - nk])]
            for e, a in enumerate(get(an, 'a_v')):
                apply[e](a)
            wo = pltpu.bitcast(wo_v[...], U32)
            wo = cat0(_lo(wo), _hi(wo))
            wo = cat0(*[_tie(wo[n * LANES:(n + 1) * LANES], a)
                        for n, a in enumerate(get(an, 'a_wo'))])
            wt_s[3 * RP:, :D] = _pk(wo.astype(BF16).T)
            for n, a in enumerate(get(an, 'a_w2')):
                prep_att(len(cfg['a_w1']) + n, a)

            wait('WO', group_cp(0))
            an = []
            stats = wo_mm(0, an, False)
            qkv_mm(1, xn1, (3, 5), an)
            for n, a in enumerate(get(an, 'z_w')):
                prep_att(36 + n, a)
            prep_piece(0, gu_s.at[0], get(an, 'z_g'), cfg['z_grp'])
            ffn_lhs(0, stats, get(an, 'z_l'))

        def pre_b(get, e_grp):
            def piece(p, carry):
                wait('WP', group_cp(p))
                o, ac = AOFF[cfg['gorder0'][0][1], cfg['inner'][0]]
                an = [a_s[o + 8 * k:o + 8 * k + 8, ac] for k in range(4)]
                win = gu_s.at[pl.ds(p - 1, 2)]
                h = gu_piece(win.at[0], cfg['gorder0'], an, (0, 7, 4, 11))
                h3_s[p - 1] = cat0(*h[3])
                tri = in_triple(p - 1)
                prep_d(tri, get(an, 'p_d'))
                store_acc(0, down_mm(load_acc(0), [(tri, h_ops(h[:3]))], an))
                prep_piece(p, win.at[1], get(an, 'f_g'), cfg['f_grp'])
                att_group(1, *e_grp(p - 1), an[cfg['p_att'][0]])
                return carry

            lax.fori_loop(1, NP, piece, 0)

        def pre_c(get):
            wait('WD', group_cp(NP))
            an = []
            h = gu_piece(gu_s.at[NP - 1], cfg['torder'], an)
            h3 = [[h3_s[q, :TH], h3_s[q, TH:]] for q in range(NP - 1)] + [h[3]]
            work = [(cross_triple(s), h_ops(h3[3 * s:3 * s + 3])) for s in range(3)]
            work.append((in_triple(NP - 1), h_ops(h[:3])))
            stats = wo_mm(1, an, True)
            td = get(an, 't_d')
            for n, (tri, _) in enumerate(work):
                prep_d(tri, td[n * len(td) // 4:(n + 1) * len(td) // 4])
            acc = down_mm(load_acc(0), work, an)
            nw = len(cfg['a_w1']) + len(cfg['a_w2'])
            for n, a in enumerate(get(an, 't_w')[:36 - nw]):
                prep_att(nw + n, a)
            ffn_lhs(1, stats, get(an, 't_l'))
            finish(0, acc)

        if 'pre' in cfg['phases']:
            pre_phase()

        def body(u, carry):
            bu = u & (NB - 1)
            ba = (u + 1) & (NB - 1)
            acc, stats, an, b, hh = None, None, {}, {}, {}
            get = lambda name: [an[k][i] for k, i in cfg[name]]
            for step in cfg['body']:
                an[step] = []
                if step == 'Q':
                    xn = ln1(ba, get('ln1'), get('ln1b'))
                    qkv_fast(ba, att_rhs(xn, u >> 8), an[step])
                elif step == 'W':
                    attention(ba, get('att'))
                    stats = wo_mm(ba, an[step], True, u >> 8, get('orhs'))
                elif step == 'L':
                    ffn_lhs(ba, stats, get('lhs'))
                elif step[0] == 'G':
                    q, go = int(step[1]), cfg['gorder']
                    t = b.setdefault(step[:2], ({}, {}))
                    for m, m1 in (go[:7] if step[2] == '0' else go[7:]):
                        t[m][m1] = gu_outer(gu_s.at[q], m, m1, an[step])
                    if len(t[0]) + len(t[1]) == 14:
                        hh[q] = gu_finish(t)
                else:
                    work = []
                    for c in step[1:]:
                        if c.isdigit():
                            work.append((in_triple(int(c)), h_ops(hh[int(c)][:3])))
                        else:
                            s = ord(c) - ord('a')
                            work.append((cross_triple(s),
                                         h_ops([hh[3 * s + k][3] for k in range(3)])))
                    acc = down_mm(acc, work, an[step])
            finish(bu, acc)

            @pl.when(u >= NB)
            def _():
                out_copy(bu).start()
            return carry

        if scopes:
            with jax.named_scope('LOOP'):
                lax.fori_loop(1, NU - 1, body, 0)
        elif 'main' in cfg['phases']:
            lax.fori_loop(1, NU - 1, body, 0)

        fin_cp = [pltpu.make_async_copy(
            xio_s.at[NB - 1, pl.ds(j * D3, D3)],
            out_hbm.at[pl.ds(j * D3, D3), cols((NB - 1) * TM, TM)], sem_o.at[0])
            for j in range(3)]

        def last(s, carry):
            h = [gu_piece(gu_s.at[3 * s + k], cfg['lorder'], []) for k in range(3)]
            work = [(in_triple(3 * s + k), h_ops(h[k][:3])) for k in range(3)]
            work.append((cross_triple(s), h_ops([h[k][3] for k in range(3)])))
            acc = down_mm(down_mm(load_acc(1), work[:2], []), work[2:], [], cfg['ldord'])
            store_acc(1, acc)
            finish(NB - 1, acc, lambda j: pl.when(s == NP // 3 - 1)(fin_cp[j].start))
            return carry

        if 'last' in cfg['phases']:
            lax.fori_loop(0, NP // 3, last, 0)
        if len(cfg['phases']) < 3:
            def keep(i, c):
                v = (gu_s[i, i, :8, :LANES] + ds_s[i, i, :8, :LANES]
                     + wl_s[rows8(i * 8), :LANES] + a_s[rows8(i * 8), :LANES] + qkv_s[i, :8]
                     + wt_s[rows8(i * 8), :LANES])
                acc_s[1, 0, :8] = (lax.bitcast_convert_type(v, F32) + o_s[i, :8]
                                   + acc_s[i, i, :8] + h3_s[i, :8])
                return c
            lax.fori_loop(0, 2, keep, 0)
            finish(NB - 1, load_acc(1))
        wait('WOUT', [out_copy(b) for b in range(NB - 1)] + fin_cp)

    scratch = [
        pltpu.VMEM((NB, D, TM), BF16),
        pltpu.VMEM((D, 3 * D), BF16),
        pltpu.VMEM((D, D), BF16),
        pltpu.VMEM((NP, D, PW), BF16),
        pltpu.VMEM((NP, D, PW), BF16),
        pltpu.VMEM((NP, D, PW), BF16),
        pltpu.VMEM((2 * D, 8 * LANES), U32),
        pltpu.VMEM((4 * Q3, 16 * LANES), U32),
        pltpu.VMEM((NP, 51, 64, 2 * LANES), U32),
        pltpu.VMEM((NP + 3, 5, Q3, 2 * LANES), U32),
        pltpu.VMEM((NB, D, TM), F32),
        pltpu.VMEM((max(fill), 2 * LANES), U32),
        pltpu.VMEM((S // LANES + 1, 3 * RP, LANES), U32),
        pltpu.VMEM((NT, D, LANES), F32),
        pltpu.VMEM((2, 15, D3, TH), F32),
        pltpu.VMEM((NP, TM, LANES), F32),
        pltpu.VMEM((1, 9 * 64, 2 * LANES), U32),
        pltpu.SemaphoreType.DMA((SEM_P + NP + 2,)),
        pltpu.SemaphoreType.DMA((1,)),
    ]

    def wrapped(*refs):
        @pl.when(pl.program_id(0) == 0)
        def _():
            kernel(*refs)

    return wrapped, scratch


_CFG = dict(
    scopes=False,
    ldord=(1, 2, 0, 7, 8, 6, 9, 10, 4, 5, 3, 11, 12, 13, 14),
    orhs=(('G80', 0), ('G80', 1), ('G80', 2), ('G80', 3), ('G80', 4), ('G80', 5),
        ('G80', 6), ('G80', 7), ('G80', 8), ('G80', 9), ('G80', 10), ('G80', 11)),
    sub='abc',
    phases=('pre', 'main', 'last'),
    body=('G20', 'G00', 'G01', 'G10', 'G11', 'Q', 'G30', 'G21', 'G40', 'G31', 'G50',
        'D012a', 'G41', 'G51', 'D345b', 'G70', 'G60', 'G71', 'G80', 'W', 'G61', 'G81',
        'D8c', 'D67', 'L'),
    ln1=(('G00', 0), ('G00', 1), ('G00', 2), ('G00', 3), ('G00', 4), ('G00', 5), ('G00',
        6), ('G00', 7), ('G00', 8)),
    ln1b=(('G10', 1), ('G10', 2), ('G10', 3), ('G10', 4), ('G10', 5), ('G10', 6),
        ('G10', 7), ('G10', 8), ('G10', 9), ('G10', 10), ('G10', 11), ('G10', 12)),
    att=(('D012a', 2), ('D012a', 4), ('D012a', 5), ('D012a', 8), ('D012a', 9), ('D345b',
        5), ('D345b', 6), ('D345b', 8)),
    lhs=(('D8c', 2), ('D8c', 3), ('D8c', 9), ('D8c', 11), ('D67', 5), ('D67', 8),
        ('D67', 10), ('D67', 11), ('D67', 14)),
    a_w1=(0, 0, 1, 2, 2, 3, 3, 4, 5, 6, 7, 11, 13, 18, 19, 20, 21, 22, 23, 24, 26, 27,
        28, 29),
    a_w2=(25, 30, 33, 36, 44, 45),
    a_ln=(3, 6, 7),
    a_lnb=(3, 9, 15),
    z_g=(0, 0, 1, 1, 2, 2, 3, 3, 4, 4, 5, 5, 6, 6, 7, 7, 8, 8, 9, 11, 12, 12, 13, 14,
        14, 14, 15, 15, 16, 16, 17, 17, 18, 18, 19, 19, 20, 21, 21, 22, 23, 23, 23, 24,
        25, 26, 27, 33),
    t_d=(0, 0, 0, 2, 2, 4, 5, 5, 7, 7, 8, 8, 9, 10, 11, 11, 12, 12, 13, 14, 14, 15, 16,
        16, 17, 17, 18, 18, 21, 22, 24, 24, 25, 28, 28, 30, 32, 32, 35, 35, 36, 37, 37,
        37, 39, 40, 40, 42),
    p_d=(6, 16, 21, 29, 29, 32, 37, 38, 42, 46, 50, 53),
    p_att=(65,),
    z_l=(23, 23, 28, 31, 35, 36, 37, 37, 39),
    a_k=(13, 17, 20, 26),
    a_k2=(0, 1, 3, 9),
    a_v=(13, 13, 14, 15, 16, 17, 18, 19),
    a_wo=(9, 18, 25, 36, 46),
    inner=(0, 3, 4, 6, 2, 1, 5),
    gorder=((0, 4), (0, 0), (1, 4), (1, 0), (1, 6), (0, 3), (1, 3), (0, 6), (0, 1), (1,
        1), (0, 2), (1, 2), (0, 5), (1, 5)),
    gorder0=((0, 4), (0, 0), (0, 3), (1, 0), (1, 4), (0, 6), (1, 6), (1, 3), (1, 1), (0,
        1), (0, 2), (0, 5), (1, 2), (1, 5)),
    f_g=(0, 0, 0, 0, 1, 1, 2, 2, 3, 3, 4, 5, 8, 9, 10, 11, 12, 13, 13, 14, 15, 16, 17,
        18, 20, 21, 21, 23, 24, 25, 27, 28, 30, 32, 32, 33, 33, 36, 37, 37, 39, 40, 41,
        45, 47, 49, 49, 52, 53, 58, 62, 65, 68, 73, 74, 74),
    t_l=(49, 50, 51, 53, 54, 55, 57, 57, 60),
    lorder=((1, 0), (1, 4), (0, 0), (0, 4), (0, 3), (0, 6), (1, 3), (1, 6), (0, 1), (1,
        1), (0, 2), (0, 5), (1, 2), (1, 5)),
    z_w=(1, 1, 3, 3, 5, 5, 6, 6, 8, 9, 17, 35),
    z_grp=1,
    f_grp=((1, 0), (4, 2), (3, 6), (5,)),
    t_w=(47, 49, 49, 50, 52, 54),
    torder=((0, 0), (0, 4), (1, 4), (1, 0), (0, 3), (1, 3), (1, 6), (0, 6), (0, 1), (1,
        1), (0, 2), (1, 2), (0, 5), (1, 5)),
)


def _run(A_x, A_wqkv, A_wo, B_w_gate, B_w_up, B_w_down, **kw):
    _, S, D = A_x.shape
    F = B_w_gate.shape[1]
    kernel, scratch = _make_kernel(S, D, F, 256, {**_CFG, **kw})
    hbm = pl.BlockSpec(memory_space=pl.ANY)
    out_t = pl.pallas_call(
        kernel,
        grid=(2,),
        in_specs=[hbm] * 6,
        out_specs=hbm,
        out_shape=jax.ShapeDtypeStruct((D, S), A_x.dtype),
        scratch_shapes=scratch,
        compiler_params=pltpu.CompilerParams(
            dimension_semantics=('arbitrary',), vmem_limit_bytes=110 * 1024 * 1024),
    )(A_x.reshape(S, D).T, A_wqkv, A_wo, B_w_gate, B_w_up, B_w_down.T)
    return out_t.T.reshape(A_x.shape)


@jax.jit
def pallas_interleave_layers__sliding_local_dilated__glu_gated_geglu__prompt_kernel(
    A_x: jax.Array,
    A_wqkv: jax.Array,
    A_wo: jax.Array,
    B_x: jax.Array,
    B_w_gate: jax.Array,
    B_w_up: jax.Array,
    B_w_down: jax.Array,
):
    del B_x
    return _run(A_x, A_wqkv, A_wo, B_w_gate, B_w_up, B_w_down)
```

```python
import jax
import jax.numpy as jnp
import jax.experimental.pallas as pl
import jax.experimental.pallas.tpu as pltpu
from jax import lax

H = 32
W = 8
DIL = 2
EPS = 1e-5
LANES = 128

F32 = jnp.float32
BF16 = jnp.bfloat16
U32 = jnp.uint32

_NT = (((1,), (1,)), ((), ()))


def _tree_sum(parts, op=jnp.add):
    while len(parts) > 1:
        nxt = [op(parts[i], parts[i + 1]) for i in range(0, len(parts) - 1, 2)]
        if len(parts) % 2:
            nxt.append(parts[-1])
        parts = nxt
    return parts[0]


def _ln_stats(slabs, d, anchors=()):
    n_acc = 4
    s1, s2, pilot = [None] * n_acc, [None] * n_acc, None
    for i, x in enumerate(slabs):
        if pilot is None:
            pilot = x[0:1, :]
            pil = jnp.broadcast_to(pilot, x.shape)
            pils = [_tie(pil, a) for a in anchors] or [pil]
        dx = x - pils[i * len(pils) // (d // 8)]
        j = i % n_acc
        s1[j] = dx if s1[j] is None else s1[j] + dx
        s2[j] = dx * dx if s2[j] is None else s2[j] + dx * dx
    e1 = jnp.sum(_tree_sum(s1), axis=0, keepdims=True) * (1.0 / d)
    e2 = jnp.sum(_tree_sum(s2), axis=0, keepdims=True) * (1.0 / d)
    var = jnp.maximum(e2 - e1 * e1, 0.0)
    return pilot + e1, lax.rsqrt(var + EPS)


def _zero_like_dep(v):
    return (lax.bitcast_convert_type(v, U32) >> 31) >> 1


def _tie(x, anchor):
    if anchor is None:
        return x
    z = lax.bitcast_convert_type(_zero_like_dep(anchor), F32)
    z = jnp.concatenate([z] * -(-x.shape[1] // LANES), axis=1)[:, :x.shape[1]]
    if x.shape[0] == 8:
        return x + z
    return jnp.concatenate([x[:8] + z, x[8:]], axis=0)


def _gelu_mul2(g, u):
    c0 = 0.7978845608028654
    c1 = c0 * 0.044715
    t = jnp.tanh(g * (c0 + c1 * (g * g)))
    return (g * u) * (1.0 + t)


def _lo(x):
    return lax.bitcast_convert_type(x << 16, F32)


def _hi(x):
    return lax.bitcast_convert_type(x & jnp.uint32(0xFFFF0000), F32)


def _pk(x):
    return pltpu.bitcast(x.astype(BF16), U32)


def _upk(x):
    return pltpu.bitcast(x, BF16)


def _dot(a, b):
    return jnp.dot(a, b, preferred_element_type=F32)


def _dot_nt(a, b):
    return lax.dot_general(a, b, _NT, preferred_element_type=F32)


def _x_ops(x1, x2):
    d = [a - b for a, b in zip(x1, x2)]
    return [x1[0] + x2[1], x2[0] + x2[1], x1[0] + x1[1],
            d[1] + x1[2], x1[1] + x1[2], d[1] + d[2],
            d[0] - x2[2], d[0] + d[2], x2[0] + x2[2],
            x1[0], d[0], x2[1], d[1], x1[2], x2[2]]


def _x_rem(x1, x2):
    a, b, c = 0, 1, 2
    cat = lambda u, v: jnp.concatenate([u, v], axis=0)
    return [cat(x1[c], x2[b]), cat(x1[a], x1[b] - x2[b]), cat(x2[a], x2[c] - x1[c])]


_W_TERMS = {0: ((0, 1, 1), (1, 0, 1)), 3: ((1, 2, 1), (2, 1, 1)), 6: ((0, 2, 1), (2, 0, 1)),
            9: ((0, 0, 1), (0, 2, 1), (1, 0, -1)), 10: ((2, 0, 1), (0, 0, -1), (0, 1, -1)),
            11: ((1, 1, 1), (1, 2, 1), (0, 1, -1)), 12: ((1, 0, 1), (1, 1, 1), (2, 1, -1)),
            13: ((2, 0, 1), (2, 2, 1), (1, 2, -1)), 14: ((2, 1, 1), (2, 2, 1), (0, 2, -1)),
            1: ((0, 1, 1),), 2: ((1, 0, 1),), 4: ((1, 2, 1),), 5: ((2, 1, 1),),
            7: ((2, 0, 1),), 8: ((0, 2, 1),)}


def _w_sums(w):
    return [_signed(_W_TERMS[i], lambda k, j: w[k][j]) for i in _W_SUM]


_W_SUM = {0: 0, 3: 1, 6: 2, 9: 3, 10: 4, 11: 5, 12: 6, 13: 7, 14: 8}
_W_RAW = {1: (0, 1), 2: (1, 0), 4: (1, 2), 5: (2, 1), 7: (2, 0), 8: (0, 2)}
_PAIR_ORDER = (1, 2, 4, 5, 7, 8, 0, 3, 6)
_DIAG = {(0, 0): 9, (2, 0): 10, (0, 1): 11, (1, 1): 12, (1, 2): 13, (2, 2): 14}
_PAIR = {(0, 0): ((6, -1), (8, -1)), (1, 0): ((2, 1), (7, 1)), (2, 0): ((0, 1), (1, -1)),
         (0, 1): ((3, 1), (4, -1)), (1, 1): ((0, 1), (2, -1)), (2, 1): ((1, 1), (5, -1)),
         (0, 2): ((4, 1), (8, 1)), (1, 2): ((6, 1), (7, -1)), (2, 2): ((5, 1), (3, -1))}


def _column(t, base, j, skew=False):
    s = []
    for k in range(3):
        v = base[k]
        for i, sg in _PAIR[k, j]:
            v = t[i] if v is None else (v + t[i] if sg > 0 else v - t[i])
        s.append(v)
    if skew:
        return s[1] + s[0], s[2] + 0.5 * (s[0] - s[1])
    return s[1] + s[0], s[2] + s[0]


_SA = (((0, 0, 1), (1, 1, 1)), ((1, 0, 1), (1, 1, 1)), ((0, 0, 1),), ((1, 1, 1),),
       ((0, 0, 1), (0, 1, 1)), ((1, 0, 1), (0, 0, -1)), ((0, 1, 1), (1, 1, -1)))
_SB = (((0, 0, 1), (1, 1, 1)), ((0, 0, 1),), ((0, 1, 1), (1, 1, -1)), ((1, 0, 1), (0, 0, -1)),
       ((1, 1, 1),), ((0, 0, 1), (0, 1, 1)), ((1, 0, 1), (1, 1, 1)))
_SCOL = {2: 1, 3: 0, 5: 1, 6: 0}
_SGRP = ((1, 4, 0), (3, 6), (2, 5))


def _signed(terms, f):
    v = None
    for a, b, sg in terms:
        v = f(a, b) if v is None else (v + f(a, b) if sg > 0 else v - f(a, b))
    return v


def _s_out(m):
    return [[m[0] + m[3] - m[4] + m[6], m[2] + m[4]],
            [m[1] + m[3], m[0] - m[1] + m[2] + m[5]]]


def _make_kernel(S, D, F, TM, cfg):
    NB = S // TM
    NT = TM // LANES
    DH = D // H
    DP = DH // 2
    RP = D // 2
    NG = H // 8
    scale = float(DH) ** -0.5
    NU = 2 * NB
    TH = TM // 2
    TQ = TM // 4
    D2 = D // 2
    D3 = D // 3
    Q3 = D3 // 2
    KU = D // 9
    KR = 3 * LANES
    NQ = 6
    QR = 3 * D // NQ
    WQ = (0, 640, 1152, 3 * D)
    PW = 4 * LANES
    NP = F // PW
    AOFF, fill = {}, [0, 0]
    for key in [(m1, m2) for m1 in range(7) for m2 in range(7)]:
        c = int(fill[1] < fill[0])
        AOFF[key] = (fill[c], slice(c * LANES, (c + 1) * LANES))
        fill[c] += 48 if key[0] in _SCOL and key[1] in _SCOL else 32
    scopes = cfg['scopes']
    assert NG == 4 and NB & (NB - 1) == 0
    SEM_P = 4

    def kernel(x_hbm, wqkv_hbm, wo_hbm, wg_hbm, wu_hbm, wdt_hbm, out_hbm,
               xio_s, wqkv_v, wo_v, wg_v, wu_v, wdt_v, wt_s, wl_s,
               gu_s, ds_s, xmid_s, a_s, qkv_s, o_s, acc_s, h3_s, r_s,
               sem_i, sem_o):

        def wait(name, cps):
            if scopes:
                with jax.named_scope(name):
                    for cp in cps:
                        cp.wait()
            else:
                for cp in cps:
                    cp.wait()

        def cols(lo, n):
            if not isinstance(lo, int):
                lo = pl.multiple_of(lo, LANES)
            return pl.ds(lo, n)

        def rows8(lo, n=8):
            if not isinstance(lo, int):
                lo = pl.multiple_of(lo, 8)
            return pl.ds(lo, n)

        def out_copy(b):
            return pltpu.make_async_copy(
                xio_s.at[b], out_hbm.at[:, cols(b * TM, TM)], sem_o.at[0])

        def x_cp(b, sem):
            return pltpu.make_async_copy(x_hbm.at[:, cols(b * TM, TM)], xio_s.at[b],
                                         sem_i.at[sem])

        def wq_cp(i):
            sl = cols(WQ[i], WQ[i + 1] - WQ[i])
            return pltpu.make_async_copy(wqkv_hbm.at[:, sl], wqkv_v.at[:, sl],
                                         sem_i.at[1 + i])

        def piece_cp(src, dst, p, sem, c0=0, n=PW):
            return pltpu.make_async_copy(src.at[:, cols(p * PW + c0, n)],
                                         dst.at[p, :, pl.ds(c0, n)], sem_i.at[sem])

        def group_cp(p):
            sem = SEM_P + p
            cps = []
            if not (isinstance(p, int) and p == NP):
                cps += [piece_cp(wg_hbm, wg_v, p, sem), piece_cp(wu_hbm, wu_v, p, sem)]
            if not (isinstance(p, int) and p == 0):
                cps.append(piece_cp(wdt_hbm, wdt_v, p - 1, sem, 0, KR))
            if isinstance(p, int) and p == NP:
                cps += [piece_cp(wdt_hbm, wdt_v, q, sem, KR, LANES) for q in range(NP)]
            return cps

        lane = lax.broadcasted_iota(jnp.int32, (8, LANES), 1)
        cat0 = lambda *v: jnp.concatenate(v, axis=0)
        cat1 = lambda *v: jnp.concatenate(v, axis=1)

        def spread_over(anchors, n, total):
            return anchors[n * len(anchors) // total] if anchors else None

        def slab_group(r):
            return (r % LANES) // 16 if r < KR else 8 + ((r - KR) % KU) // 16

        def ln1(blk, anchors1, anchors2=()):
            slabs = (xio_s[blk, r:r + 8, :].astype(F32) for r in range(0, D, 8))
            m, rs = _ln_stats(slabs, D, anchors1)
            if not anchors2:
                return (xio_s[blk].astype(F32) - m) * rs
            m8 = jnp.broadcast_to(m, (8, TM))
            ms = [_tie(m8, a) for a in anchors2]
            ms = [spread_over(ms, slab_group(r), 12) for r in range(0, D, 8)]
            return (xio_s[blk].astype(F32) - cat0(*ms)) * rs

        def dot_k(rows, x, anchors, even=False):
            y = None
            for n, k in enumerate(range(0, D, LANES)):
                ks = slice(k, min(k + LANES, D))
                if even and k + LANES >= D:
                    mid = (rows.start + rows.stop) // 2
                    v = cat0(_dot(_upk(wt_s[rows.start:mid, ks]), x[ks]),
                             _dot(_upk(wt_s[mid:rows.stop, ks]), x[ks]))
                else:
                    v = _dot(_upk(wt_s[rows, ks]), x[ks])
                anchors.extend(v[r:r + 8, :LANES] for r in ((0, 144) if n % 2 else (72, 216)))
                y = v if y is None else y + v
            return y

        def put_qkv(blk, rows, y):
            pk = _pk(y)
            for c in range(NT):
                qkv_s[1 + blk * NT + c, rows, :] = pk[:, c * LANES:(c + 1) * LANES]

        def qkv_mm(blk, xn, chunks, anchors, even=False):
            for r in chunks:
                rows = slice(r * QR // 2, (r + 1) * QR // 2)
                put_qkv(blk, rows, dot_k(rows, xn, anchors, even))

        def split_k(x):
            hs = (x[:, :TH], x[:, TH:])
            blocks = [[h[k * LANES:(k + 1) * LANES] for k in range(3)] for h in hs]
            units = [[h[KR + k * KU:KR + (k + 1) * KU] for k in range(3)] for h in hs]
            return blocks, units

        def prep_att(pat, anchor):
            assert Q3 == 96
            row0 = pat * 8
            src0 = row0 + ((pat * 43) >> 9) * (2 * Q3)
            w = [_upk(wt_s[rows8(src0 + j * Q3), :D]).astype(F32) for j in range(3)]
            w[0] = cat1(_tie(w[0][:, :LANES], anchor), w[0][:, LANES:])
            tiles = _w_sums([[w[j][:, k * LANES:(k + 1) * LANES] for j in range(3)]
                             for k in range(3)])
            for j in range(3):
                a, b, c = (w[j][:, KR + k * KU:KR + (k + 1) * KU] for k in range(3))
                tiles += [cat1(c, b), cat1(a, c)]
            wl_s[rows8(row0), :15 * LANES] = _pk(cat1(*tiles))

        def att_rhs(x, stash=None, anchors=()):
            half = 0.5
            if anchors:
                hs = [_tie(jnp.full((8, TH), 0.5, F32), a) for a in anchors]
                half = cat0(*[spread_over(hs, slab_group(r), 12) for r in range(0, D, 8)])
            blocks, units = split_k(cat1(x[:, :TH], x[:, TH:] + half * x[:, :TH]))
            ops = _x_ops(*blocks) + _x_rem(*units)
            if stash is None:
                return [v.astype(BF16) for v in ops]
            loc = lambda i, r0, n: (slice((i // 2) * 64 + r0, (i // 2) * 64 + r0 + n),
                                    slice((i % 2) * LANES, (i % 2 + 1) * LANES))
            for r in range(0, LANES, 16):
                for i, v in enumerate(ops):
                    r_s.at[0][loc(i, r // 2, 8)] = _pk(v[r:r + 16])
            return [_upk(r_s.at[stash][loc(i, 0, 64)]) for i in range(18)]

        def att_mm(sec, rhs, anchors):
            tl = lambda i: _upk(wl_s[sec * Q3:(sec + 1) * Q3, i * LANES:(i + 1) * LANES])
            raw = lambda k, j: _upk(wt_s[(3 * sec + j) * Q3:(3 * sec + j + 1) * Q3,
                                         k * LANES:(k + 1) * LANES])
            t = {}
            for i in _PAIR_ORDER:
                t[i] = _dot(raw(*_W_RAW[i]) if i in _W_RAW else tl(_W_SUM[i]), rhs[i])
                anchors.append(t[i][:8])
            out = []
            for j in range(3):
                base = []
                for s in range(3):
                    v = _dot(raw(3, j) if s == 1 else tl(9 + 2 * j + s // 2), rhs[15 + s])
                    if (s, j) in _DIAG:
                        i = _DIAG[s, j]
                        v = _dot(tl(_W_SUM[i]), rhs[i]) + v
                    base.append(v)
                    anchors.append(base[-1][:8])
                out.append(cat1(*_column(t, base, j, True)))
            return cat0(*out)

        def qkv_fast(blk, rhs, anchors):
            for sec in range(3):
                put_qkv(blk, slice(sec * RP, (sec + 1) * RP), att_mm(sec, rhs, anchors))

        def shifted(ln, cur, prev, w):
            if w == 0:
                return cur
            sh = DIL * w
            return pltpu.roll(jnp.where(ln < LANES - sh, cur, prev), sh, axis=1)

        def att_group(blk, c, hg, anchor):
            att_values(blk, c, hg, anchor)(None)

        def att_values(blk, c, hg, anchor):
            tile = blk * NT + c
            base = hg * 8 * DP
            if isinstance(hg, int):
                cur, prev, o_t = qkv_s.at[1 + tile], qkv_s.at[tile], o_s.at[c]
            else:
                n = 2 * RP + 8 * DP
                base = pl.multiple_of(base, 8)
                cur = qkv_s.at[1 + tile, pl.ds(base, n)]
                prev = qkv_s.at[tile, pl.ds(base, n)]
                o_t = o_s.at[c, pl.ds(base, RP + 8 * DP)]
                base = 0
            ln = lane + _zero_like_dep(anchor).astype(jnp.int32)
            logits = [None] * W
            for dd in range(DP):
                q = cur[pl.ds(base + dd, 8, stride=DP), :]
                kc = cur[pl.ds(RP + base + dd, 8, stride=DP), :]
                kp = prev[pl.ds(RP + base + dd, 8, stride=DP), :]
                q0, q1 = _lo(q), _hi(q)
                for w in range(W):
                    ks = shifted(ln, kc, kp, w)
                    t = q0 * _lo(ks) + q1 * _hi(ks)
                    logits[w] = t if logits[w] is None else logits[w] + t
            logits = [l * scale for l in logits]
            if not (isinstance(c, int) and c > 0):
                pos = lane + tile * LANES
                logits = [l if w == 0 else jnp.where(pos >= DIL * w, l, -1e9)
                          for w, l in enumerate(logits)]
            m = _tree_sum(logits, jnp.maximum)
            p = [jnp.exp(l - m) for l in logits]
            r = 1.0 / _tree_sum(p)

            def apply(anchor2):
                ln = lane + _zero_like_dep(_tie(m, anchor2)).astype(jnp.int32)
                for dd in range(DP):
                    vc = cur[pl.ds(2 * RP + base + dd, 8, stride=DP), :]
                    vp = prev[pl.ds(2 * RP + base + dd, 8, stride=DP), :]
                    o0 = o1 = None
                    for w in range(W):
                        vs = shifted(ln, vc, vp, w)
                        t0, t1 = p[w] * _lo(vs), p[w] * _hi(vs)
                        o0 = t0 if o0 is None else o0 + t0
                        o1 = t1 if o1 is None else o1 + t1
                    o0, o1 = o0 * r, o1 * r
                    o_t[pl.ds(base + dd, 8, stride=DP), :] = o0
                    o_t[pl.ds(RP + base + dd, 8, stride=DP), :] = o1

            return apply

        def attention(blk, anchors):
            for c in range(NT):
                for hg in range(NG):
                    att_group(blk, c, hg, anchors[c * NG + hg])

        def wo_mm(blk, anchors, fast, stash=None, anchors_in=()):
            o = cat1(*[o_s[c] for c in range(NT)])
            if fast:
                y = att_mm(3, att_rhs(o, stash, anchors_in), anchors)
            else:
                o = o.astype(BF16)
                q = D2 // 2
                y = cat0(*[dot_k(slice(h * q, (h + 1) * q), o, anchors) for h in (6, 7)])
            xm = xio_s[blk].astype(F32) + y
            xmid_s[blk] = xm
            return _ln_stats((xm[r:r + 8] for r in range(0, D, 8)), D)

        def ffn_lhs(blk, stats, anchors):
            m, rs = stats
            m8 = jnp.broadcast_to(m, (8, TM))
            xt = []
            for k in range(5):
                mt = cat0(*[_tie(m8, spread_over(anchors[:2], k, 5))] * (KU // 8 if k == 4 else 16))
                x = (xmid_s[blk, k * LANES:min((k + 1) * LANES, D), :] - mt) * rs
                xt.append((cat0(x, x) if k == 4 else x).T)
            lo = lax.broadcasted_iota(jnp.int32, (TQ // 2, LANES), 1) < KU
            for m1 in range(7):
                a = spread_over(anchors[2:], m1, 7)
                blk1 = lambda i2, k2: _signed(_SA[m1], lambda i1, k1: _tie(
                    xt[k2 if k2 == 4 else 2 * k1 + k2][(2 * i1 + i2) * TQ:(2 * i1 + i2 + 1) * TQ], a))
                l1 = {(i2, k2): blk1(i2, k2) for i2 in range(2)
                      for k2 in ((0, 1, 4) if m1 in _SCOL else (0, 1))}
                for m2 in range(7):
                    v = _signed(_SA[m2], lambda i2, k2: l1[i2, k2])
                    if m1 in _SCOL and m2 in _SCOL:
                        c = _signed(_SA[m2], lambda i2, k2: l1[i2, 4])
                        h = TQ // 2
                        vp, vq, cp, cq = v[:h], v[h:], c[:h], c[h:]
                        v = cat0(jnp.where(lo, cp, vq), jnp.where(lo, vp, vp - vq),
                                 jnp.where(lo, vq, cq - cp))
                    o, ac = AOFF[m1, m2]
                    a_s[o:o + v.shape[0] // 2, ac] = _pk(v)

        def in_triple(q):
            return q, lambda k: (q, k)

        def cross_triple(s):
            return NP + s, lambda k: (3 * s + k, 3)

        def wd_raw(tri, k, r0, n):
            q, c = tri[1](k)
            return wdt_v[q, r0:r0 + n, c * LANES:(c + 1) * LANES]

        def ds_loc(i, r0, n):
            return slice(r0, r0 + n), slice((i % 2) * LANES, (i % 2 + 1) * LANES)

        def prep_d(tri, anchors):
            PR = 16
            for n in range(D3 // PR):
                r = n * PR
                w = [[wd_raw(tri, k, j * D3 + r, PR).astype(F32) for j in range(3)]
                     for k in range(3)]
                w[0][1] = _tie(w[0][1], spread_over(anchors, n, D3 // PR))
                for i, v in enumerate(_w_sums(w)):
                    ds_s.at[tri[0], i // 2][ds_loc(i, r // 2, PR // 2)] = _pk(v)

        GU = (wg_v, wu_v)

        def prep_gu(p, gv, m, m1s, anchors):
            PR = 16
            cs = slice(m * LANES, (m + 1) * LANES)
            for n in range(LANES // PR):
                r = n * PR
                cache = {}

                def w(k, j1):
                    if (k, j1) not in cache:
                        v = GU[m][p, k * LANES + r:k * LANES + r + PR,
                                  2 * j1 * LANES:2 * (j1 + 1) * LANES].astype(F32)
                        if (k // 2, j1) in [_SB[m1][0][:2] for m1 in m1s[:2]]:
                            a = spread_over(anchors, n, LANES // PR)
                            c = (k % 2) * LANES
                            tied = _tie(v[:, c:c + LANES], a)
                            v = cat1(v[:, :LANES], tied) if c else cat1(tied, v[:, LANES:])
                        cache[k, j1] = v
                    return cache[k, j1]

                for m1 in m1s:
                    b1 = [_signed(_SB[m1], lambda k1, j1: w(2 * k1 + k2, j1)) for k2 in range(2)]
                    for m2 in range(7):
                        v = _signed(_SB[m2],
                                    lambda k2, j2: b1[k2][:, j2 * LANES:(j2 + 1) * LANES])
                        gv.at[7 * m1 + m2][r // 2:(r + PR) // 2, cs] = _pk(v)

        def prep_tail(p, gv, m, anchor):
            v = _tie(GU[m][p, 4 * LANES:, :].astype(F32), anchor)
            for j in range(4):
                gv.at[49 + j // 2][(j % 2) * 32:(j % 2 + 1) * 32,
                                        m * LANES:(m + 1) * LANES] = _pk(
                                            v[:, j * LANES:(j + 1) * LANES])

        def gu_outer(gv, m, m1, anchors, at=(0, 4)):
            cs = slice(m * LANES, (m + 1) * LANES)
            y = {}
            for m2 in cfg['inner']:
                i, (o, ac) = 7 * m1 + m2, AOFF[m1, m2]
                if m1 in _SCOL and m2 in _SCOL:
                    j = 2 * _SCOL[m1] + _SCOL[m2]
                    tail = lambda: gv[49 + j // 2, (j % 2) * 32:(j % 2 + 1) * 32, cs]
                    rhs = (cat0(tail(), gv[i, 32:, cs]), gv[i, :, cs],
                           cat0(gv[i, :32, cs], tail()))
                    r = [_dot(_upk(a_s[o + 16 * s:o + 16 * (s + 1), ac]), _upk(rhs[s]))
                         for s in range(3)]
                    y[m2] = cat0(r[1] + r[0], r[2] + r[0])
                else:
                    y[m2] = _dot(_upk(a_s[o:o + TQ // 2, ac]), _upk(gv[i, :, cs]))
            anchors.extend(y[cfg['inner'][k % 7]][(k // 7) * 32:(k // 7) * 32 + 8] for k in at)
            return _s_out(y)

        def gu_finish(t):
            gu = [{(i2, j2): _s_out([t[m][m1][i2][j2] for m1 in range(7)])
                   for i2 in range(2) for j2 in range(2)} for m in range(2)]
            return [[cat0(*[_gelu_mul2(*[gu[m][i2, j % 2][i1][j // 2] for m in range(2)])
                            for i2 in range(2)]) for i1 in range(2)] for j in range(4)]

        def gu_piece(gv, order, anchors, at=(0, 4)):
            t = ({}, {})
            for m, m1 in order:
                t[m][m1] = gu_outer(gv, m, m1, anchors, at)
            return gu_finish(t)

        def prep_piece(p, gv, anchors, group):
            if group in (0, 1):
                grp = _SGRP if group else [(m1,) for m1 in range(7)]
                k = len(anchors) // (2 * len(grp))
                for n in range(2 * len(grp)):
                    prep_gu(p, gv, n % 2, grp[n // 2], anchors[k * n:k * n + k])
            else:
                k, n = len(anchors) // 14, 0
                for g in group:
                    for m in range(2):
                        prep_gu(p, gv, m, g, anchors[n:n + k * len(g)])
                        n += k * len(g)
            for m in range(2):
                prep_tail(p, gv, m, anchors[m * len(anchors) // 2])

        def h_ops(h):
            return [v.astype(BF16) for v in _x_ops(*[[h[k][i] for k in range(3)]
                                                     for i in range(2)])]

        D_ORDER = _PAIR_ORDER + (9, 10, 11, 12, 13, 14)

        def down_mm(acc, work, anchors, which=D_ORDER):
            p = [None] * 15 if acc is None else list(acc)
            jobs = [(i, n) for i in which for n in range(len(work))]
            split = {0: (), 1: (4,), 2: (2, 2), 3: (2, 2, 4)}[len(jobs) % 4]
            split = dict(zip(jobs[len(jobs) - len(split):], split))
            for i in which:
                y = None
                for n, (tri, b) in enumerate(work):
                    ns = split.get((i, n), 1)
                    nr = D3 // ns
                    if i in _W_RAW:
                        k, j = _W_RAW[i]
                        lhs = lambda h: wd_raw(tri, k, j * D3 + h * nr, nr)
                    else:
                        s = _W_SUM[i]
                        lhs = lambda h: _upk(ds_s.at[tri[0], s // 2][ds_loc(s, h * nr // 2, nr // 2)])
                    v = cat0(*[_dot_nt(lhs(h), b[i]) for h in range(ns)])
                    y = v if y is None else y + v
                p[i] = y if p[i] is None else p[i] + y
                anchors.append(p[i][:8])
            return p

        def finish(blk, acc, after=None):
            y = [cat1(*_column(acc, [acc[_DIAG[s, j]] if (s, j) in _DIAG else None
                                     for s in range(3)], j)) for j in range(3)]
            if after is None:
                xio_s[blk] = (xmid_s[blk] + 0.5 * cat0(*y)).astype(BF16)
                return
            for j in range(3):
                rows = slice(j * D3, (j + 1) * D3)
                xio_s[blk, rows] = (xmid_s[blk, rows] + 0.5 * y[j]).astype(BF16)
                after(j)

        def load_acc(k):
            return [acc_s[k, i] for i in range(15)]

        def store_acc(k, acc):
            for i in range(15):
                acc_s[k, i] = acc[i]

        def early_gu(order):
            o, ac = AOFF[order[0][1], cfg['inner'][0]]
            return [a_s[o + 8 * k:o + 8 * k + 8, ac] for k in range(4)]

        def early_wt(row):
            return [wt_s[row + 16 * k:row + 16 * k + 8, :LANES] for k in range(4)]

        def pre_phase():
            first = [[x_cp(0, 0)], [wq_cp(0)], [x_cp(1, 2), wq_cp(1)],
                     [wq_cp(2), pltpu.make_async_copy(wo_hbm, wo_v, sem_i.at[3])]]
            order = sum(first, [])
            for p in range(NP + 1):
                order += group_cp(p)
            xr_cp = [x_cp(b, SEM_P + NP + 1) for b in range(2, NB)]
            order += xr_cp
            for cp in order:
                cp.start()
            get = lambda an, name: [an[min(i, len(an) - 1)] for i in cfg[name]]
            e_grp = lambda e: ((e >> 1) & 1, ((e >> 2) << 1) | (e & 1))
            if 'a' in cfg['sub']:
                pre_a(first, get, e_grp)
            if 'b' in cfg['sub']:
                pre_b(get, e_grp)
            if 'c' in cfg['sub']:
                pre_c(get)
            wait('WX', xr_cp)

        def pre_a(first, get, e_grp):
            def transpose_wq(i):
                wt_s[WQ[i] // 2:WQ[i + 1] // 2, :D] = _pk(wqkv_v[:, WQ[i]:WQ[i + 1]].T)

            def clear(i, carry):
                for k in range(2):
                    acc_s[k, i] = jnp.zeros((D3, TH), F32)
                r = jnp.minimum(i, 11) * (RP // 4)
                qkv_s[0, rows8(r, RP // 4)] = jnp.zeros((RP // 4, LANES), U32)
                return carry

            lax.fori_loop(0, 15, clear, 0)
            wait('WX0', first[0])
            xn0 = ln1(0, ()).astype(BF16)

            wait('WQ0', first[1])
            transpose_wq(0)
            qkv_mm(0, xn0, (0, 1), [])

            wait('WQ1', first[2])
            transpose_wq(1)
            an = []
            qkv_mm(0, xn0, (2, 3), an)
            xn1 = ln1(1, get(an, 'a_ln'), get(an, 'a_lnb')).astype(BF16)
            qkv_mm(1, xn1, (0,), an, True)
            for n, a in enumerate(get(an, 'a_w1')):
                prep_att(n, a)
            nk = len(cfg['a_k'])
            apply = [att_values(0, *e_grp(e), a) for e, a in enumerate(get(an, 'a_k'))]

            wait('WQ2', first[3])
            an = early_wt(QR)
            qkv_mm(1, xn1, (2,), an)
            transpose_wq(2)
            qkv_mm(0, xn0, (4, 5), an)
            qkv_mm(1, xn1, (4,), an)
            qkv_mm(1, xn1, (1,), an, True)
            apply += [att_values(0, *e_grp(nk + e), a)
                      for e, a in enumerate(get(an, 'a_k2')[:8 - nk])]
            for e, a in enumerate(get(an, 'a_v')):
                apply[e](a)
            wo = pltpu.bitcast(wo_v[...], U32)
            wo = cat0(_lo(wo), _hi(wo))
            wo = cat0(*[_tie(wo[n * LANES:(n + 1) * LANES], a)
                        for n, a in enumerate(get(an, 'a_wo'))])
            wt_s[3 * RP:, :D] = _pk(wo.astype(BF16).T)
            for n, a in enumerate(get(an, 'a_w2')):
                prep_att(len(cfg['a_w1']) + n, a)

            wait('WO', group_cp(0))
            an = early_wt(3 * RP)
            stats = wo_mm(0, an, False)
            qkv_mm(1, xn1, (3, 5), an)
            for n, a in enumerate(get(an, 'z_w')):
                prep_att(36 + n, a)
            prep_piece(0, gu_s.at[0], get(an, 'z_g'), cfg['z_grp'])
            ffn_lhs(0, stats, get(an, 'z_l'))

        def pre_b(get, e_grp):
            def piece(p, carry):
                wait('WP', group_cp(p))
                an = early_gu(cfg['gorder0'])
                win = gu_s.at[pl.ds(p - 1, 2)]
                h = gu_piece(win.at[0], cfg['gorder0'], an, (0, 7, 4, 11))
                h3_s[p - 1] = cat0(*h[3])
                tri = in_triple(p - 1)
                prep_d(tri, get(an, 'p_d'))
                store_acc(0, down_mm(load_acc(0), [(tri, h_ops(h[:3]))], an))
                prep_piece(p, win.at[1], get(an, 'f_g'), cfg['f_grp'])
                att_group(1, *e_grp(p - 1), an[cfg['p_att'][0]])
                return carry

            lax.fori_loop(1, NP, piece, 0)

        def pre_c(get):
            wait('WD', group_cp(NP))
            an = early_gu(cfg['torder'])
            h = gu_piece(gu_s.at[NP - 1], cfg['torder'], an)
            h3 = [[h3_s[q, :TH], h3_s[q, TH:]] for q in range(NP - 1)] + [h[3]]
            work = [(cross_triple(s), h_ops(h3[3 * s:3 * s + 3])) for s in range(3)]
            work.append((in_triple(NP - 1), h_ops(h[:3])))
            stats = wo_mm(1, an, True)
            td = get(an, 't_d')
            for n, (tri, _) in enumerate(work):
                prep_d(tri, td[n * len(td) // 4:(n + 1) * len(td) // 4])
            acc = down_mm(load_acc(0), work, an)
            nw = len(cfg['a_w1']) + len(cfg['a_w2'])
            for n, a in enumerate(get(an, 't_w')[:36 - nw]):
                prep_att(nw + n, a)
            ffn_lhs(1, stats, get(an, 't_l'))
            finish(0, acc)

        if 'pre' in cfg['phases']:
            pre_phase()

        def body(u, carry):
            bu = u & (NB - 1)
            ba = (u + 1) & (NB - 1)
            acc, stats, an, b, hh = None, None, {}, {}, {}
            get = lambda name: [an[k][i] for k, i in cfg[name]]
            for step in cfg['body']:
                an[step] = []
                if step == 'Q':
                    xn = ln1(ba, get('ln1'), get('ln1b'))
                    qkv_fast(ba, att_rhs(xn, u >> 8), an[step])
                elif step == 'W':
                    attention(ba, get('att'))
                    stats = wo_mm(ba, an[step], True, u >> 8, get('orhs'))
                elif step == 'L':
                    ffn_lhs(ba, stats, get('lhs'))
                elif step[0] == 'G':
                    q, go = int(step[1]), cfg['gorder']
                    t = b.setdefault(step[:2], ({}, {}))
                    for m, m1 in (go[:7] if step[2] == '0' else go[7:]):
                        t[m][m1] = gu_outer(gu_s.at[q], m, m1, an[step])
                    if len(t[0]) + len(t[1]) == 14:
                        hh[q] = gu_finish(t)
                else:
                    work = []
                    for c in step[1:]:
                        if c.isdigit():
                            work.append((in_triple(int(c)), h_ops(hh[int(c)][:3])))
                        else:
                            s = ord(c) - ord('a')
                            work.append((cross_triple(s),
                                         h_ops([hh[3 * s + k][3] for k in range(3)])))
                    acc = down_mm(acc, work, an[step])
            finish(bu, acc)

            @pl.when(u >= NB)
            def _():
                out_copy(bu).start()
            return carry

        if scopes:
            with jax.named_scope('LOOP'):
                lax.fori_loop(1, NU - 1, body, 0)
        elif 'main' in cfg['phases']:
            lax.fori_loop(1, NU - 1, body, 0)

        fin_cp = [pltpu.make_async_copy(
            xio_s.at[NB - 1, pl.ds(j * D3, D3)],
            out_hbm.at[pl.ds(j * D3, D3), cols((NB - 1) * TM, TM)], sem_o.at[0])
            for j in range(3)]

        def last(s, carry):
            h = [gu_piece(gu_s.at[3 * s + k], cfg['lorder'], []) for k in range(3)]
            work = [(in_triple(3 * s + k), h_ops(h[k][:3])) for k in range(3)]
            work.append((cross_triple(s), h_ops([h[k][3] for k in range(3)])))
            acc = down_mm(down_mm(load_acc(1), work[:2], []), work[2:], [], cfg['ldord'])
            store_acc(1, acc)
            finish(NB - 1, acc, lambda j: pl.when(s == NP // 3 - 1)(fin_cp[j].start))
            return carry

        if 'last' in cfg['phases']:
            lax.fori_loop(0, NP // 3, last, 0)
        if len(cfg['phases']) < 3:
            def keep(i, c):
                v = (gu_s[i, i, :8, :LANES] + ds_s[i, i, :8, :LANES]
                     + wl_s[rows8(i * 8), :LANES] + a_s[rows8(i * 8), :LANES] + qkv_s[i, :8]
                     + wt_s[rows8(i * 8), :LANES])
                acc_s[1, 0, :8] = (lax.bitcast_convert_type(v, F32) + o_s[i, :8]
                                   + acc_s[i, i, :8] + h3_s[i, :8])
                return c
            lax.fori_loop(0, 2, keep, 0)
            finish(NB - 1, load_acc(1))
        wait('WOUT', [out_copy(b) for b in range(NB - 1)] + fin_cp)

    scratch = [
        pltpu.VMEM((NB, D, TM), BF16),
        pltpu.VMEM((D, 3 * D), BF16),
        pltpu.VMEM((D, D), BF16),
        pltpu.VMEM((NP, D, PW), BF16),
        pltpu.VMEM((NP, D, PW), BF16),
        pltpu.VMEM((NP, D, PW), BF16),
        pltpu.VMEM((2 * D, 8 * LANES), U32),
        pltpu.VMEM((4 * Q3, 16 * LANES), U32),
        pltpu.VMEM((NP, 51, 64, 2 * LANES), U32),
        pltpu.VMEM((NP + 3, 5, Q3, 2 * LANES), U32),
        pltpu.VMEM((NB, D, TM), F32),
        pltpu.VMEM((max(fill), 2 * LANES), U32),
        pltpu.VMEM((S // LANES + 1, 3 * RP, LANES), U32),
        pltpu.VMEM((NT, D, LANES), F32),
        pltpu.VMEM((2, 15, D3, TH), F32),
        pltpu.VMEM((NP, TM, LANES), F32),
        pltpu.VMEM((1, 9 * 64, 2 * LANES), U32),
        pltpu.SemaphoreType.DMA((SEM_P + NP + 2,)),
        pltpu.SemaphoreType.DMA((1,)),
    ]

    def wrapped(*refs):
        @pl.when(pl.program_id(0) == 0)
        def _():
            kernel(*refs)

    return wrapped, scratch


_CFG = dict(
    scopes=False,
    ldord=(1, 2, 0, 7, 8, 6, 9, 10, 4, 5, 3, 11, 12, 13, 14),
    orhs=(('G80', 0), ('G80', 1), ('G80', 2), ('G80', 3), ('G80', 4), ('G80', 5),
        ('G80', 6), ('G80', 7), ('G80', 8), ('G80', 9), ('G80', 10), ('G80', 11)),
    sub='abc',
    phases=('pre', 'main', 'last'),
    body=('G20', 'G00', 'G01', 'G10', 'G11', 'Q', 'G30', 'G21', 'G40', 'G31', 'G50',
        'D012a', 'G41', 'G51', 'D345b', 'G70', 'G60', 'G71', 'G80', 'W', 'G61', 'G81',
        'D8c', 'D67', 'L'),
    ln1=(('G00', 0), ('G00', 1), ('G00', 2), ('G00', 3), ('G00', 4), ('G00', 5), ('G00',
        6), ('G00', 7), ('G00', 8)),
    ln1b=(('G10', 1), ('G10', 2), ('G10', 3), ('G10', 4), ('G10', 5), ('G10', 6),
        ('G10', 7), ('G10', 8), ('G10', 9), ('G10', 10), ('G10', 11), ('G10', 12)),
    att=(('D012a', 2), ('D012a', 4), ('D012a', 5), ('D012a', 8), ('D012a', 9), ('D345b',
        5), ('D345b', 6), ('D345b', 8)),
    lhs=(('D8c', 2), ('D8c', 3), ('D8c', 9), ('D8c', 11), ('D67', 5), ('D67', 8),
        ('D67', 10), ('D67', 11), ('D67', 14)),
    a_w1=(0, 0, 1, 1, 2, 2, 3, 3, 4, 5, 6, 11, 13, 15, 18, 20, 21, 21, 23, 24, 26, 27,
        28, 29),
    a_w2=(0, 3, 4, 13, 18, 23),
    a_ln=(3, 6, 7),
    a_lnb=(3, 11, 15),
    z_g=(0, 1, 2, 3, 4, 4, 5, 5, 6, 6, 7, 7, 8, 8, 9, 9, 10, 10, 11, 11, 12, 12, 13, 15,
        16, 16, 16, 17, 18, 18, 19, 19, 20, 20, 21, 22, 22, 23, 23, 24, 25, 25, 25, 26,
        27, 27, 28, 39),
    t_d=(4, 4, 4, 6, 6, 8, 9, 9, 11, 11, 12, 12, 13, 14, 15, 15, 16, 16, 17, 18, 18, 19,
        20, 20, 21, 21, 22, 22, 25, 26, 28, 28, 29, 32, 32, 34, 36, 36, 39, 39, 40, 41,
        41, 41, 43, 44, 44, 46),
    p_d=(6, 16, 21, 29, 29, 32, 37, 38, 42, 46, 50, 53),
    p_att=(65,),
    z_l=(27, 27, 32, 35, 40, 41, 41, 42, 43),
    a_k=(13, 17, 20, 26),
    a_k2=(5, 6, 7, 9),
    a_v=(11, 16, 17, 18, 20, 21, 22, 23),
    a_wo=(13, 22, 29, 40, 50),
    inner=(0, 3, 4, 6, 2, 1, 5),
    gorder=((0, 4), (0, 0), (1, 4), (1, 0), (1, 6), (0, 3), (1, 3), (0, 6), (0, 1), (1,
        1), (0, 2), (1, 2), (0, 5), (1, 5)),
    gorder0=((0, 4), (0, 0), (0, 3), (1, 0), (1, 4), (0, 6), (1, 6), (1, 3), (1, 1), (0,
        1), (0, 2), (0, 5), (1, 2), (1, 5)),
    f_g=(0, 0, 0, 0, 1, 1, 2, 2, 3, 3, 4, 5, 8, 9, 10, 11, 12, 13, 13, 14, 15, 16, 17,
        18, 20, 21, 21, 23, 24, 25, 27, 28, 30, 32, 32, 33, 33, 36, 37, 37, 39, 40, 41,
        45, 47, 49, 49, 52, 53, 58, 62, 65, 68, 73, 74, 74),
    t_l=(53, 54, 55, 57, 58, 59, 61, 61, 64),
    lorder=((1, 0), (1, 4), (0, 0), (0, 4), (0, 3), (0, 6), (1, 3), (1, 6), (0, 1), (1,
        1), (0, 2), (0, 5), (1, 2), (1, 5)),
    z_w=(0, 5, 7, 7, 9, 10, 10, 11, 12, 13, 39, 43),
    z_grp=1,
    f_grp=((1, 0), (4, 2), (3, 6), (5,)),
    t_w=(51, 53, 53, 54, 56, 58),
    torder=((0, 0), (0, 4), (1, 4), (1, 0), (0, 3), (1, 3), (1, 6), (0, 6), (0, 1), (1,
        1), (0, 2), (1, 2), (0, 5), (1, 5)),
)


def _run(A_x, A_wqkv, A_wo, B_w_gate, B_w_up, B_w_down, **kw):
    _, S, D = A_x.shape
    F = B_w_gate.shape[1]
    kernel, scratch = _make_kernel(S, D, F, 256, {**_CFG, **kw})
    hbm = pl.BlockSpec(memory_space=pl.ANY)
    out_t = pl.pallas_call(
        kernel,
        grid=(2,),
        in_specs=[hbm] * 6,
        out_specs=hbm,
        out_shape=jax.ShapeDtypeStruct((D, S), A_x.dtype),
        scratch_shapes=scratch,
        compiler_params=pltpu.CompilerParams(
            dimension_semantics=('arbitrary',), vmem_limit_bytes=110 * 1024 * 1024),
    )(A_x.reshape(S, D).T, A_wqkv, A_wo, B_w_gate, B_w_up, B_w_down.T)
    return out_t.T.reshape(A_x.shape)


@jax.jit
def pallas_interleave_layers__sliding_local_dilated__glu_gated_geglu__prompt_kernel(
    A_x: jax.Array,
    A_wqkv: jax.Array,
    A_wo: jax.Array,
    B_x: jax.Array,
    B_w_gate: jax.Array,
    B_w_up: jax.Array,
    B_w_down: jax.Array,
):
    del B_x
    return _run(A_x, A_wqkv, A_wo, B_w_gate, B_w_up, B_w_down)
```

```python
import jax
import jax.numpy as jnp
import jax.experimental.pallas as pl
import jax.experimental.pallas.tpu as pltpu
from jax import lax

H = 32
W = 8
DIL = 2
EPS = 1e-5
LANES = 128

F32 = jnp.float32
BF16 = jnp.bfloat16
U32 = jnp.uint32

_NT = (((1,), (1,)), ((), ()))


def _tree_sum(parts, op=jnp.add):
    while len(parts) > 1:
        nxt = [op(parts[i], parts[i + 1]) for i in range(0, len(parts) - 1, 2)]
        if len(parts) % 2:
            nxt.append(parts[-1])
        parts = nxt
    return parts[0]


def _ln_stats(slabs, d, anchors=()):
    n_acc = 4
    s1, s2, pilot = [None] * n_acc, [None] * n_acc, None
    for i, x in enumerate(slabs):
        if pilot is None:
            pilot = x[0:1, :]
            pil = jnp.broadcast_to(pilot, x.shape)
            pils = [_tie(pil, a) for a in anchors] or [pil]
        dx = x - pils[i * len(pils) // (d // 8)]
        j = i % n_acc
        s1[j] = dx if s1[j] is None else s1[j] + dx
        s2[j] = dx * dx if s2[j] is None else s2[j] + dx * dx
    e1 = jnp.sum(_tree_sum(s1), axis=0, keepdims=True) * (1.0 / d)
    e2 = jnp.sum(_tree_sum(s2), axis=0, keepdims=True) * (1.0 / d)
    var = jnp.maximum(e2 - e1 * e1, 0.0)
    return pilot + e1, lax.rsqrt(var + EPS)


def _zero_like_dep(v):
    return (lax.bitcast_convert_type(v, U32) >> 31) >> 1


def _tie(x, anchor):
    if anchor is None:
        return x
    z = lax.bitcast_convert_type(_zero_like_dep(anchor), F32)
    z = jnp.concatenate([z] * -(-x.shape[1] // LANES), axis=1)[:, :x.shape[1]]
    if x.shape[0] == 8:
        return x + z
    return jnp.concatenate([x[:8] + z, x[8:]], axis=0)


def _gelu_mul2(g, u):
    c0 = 0.7978845608028654
    c1 = c0 * 0.044715
    t = jnp.tanh(g * (c0 + c1 * (g * g)))
    return (g * u) * (1.0 + t)


def _lo(x):
    return lax.bitcast_convert_type(x << 16, F32)


def _hi(x):
    return lax.bitcast_convert_type(x & jnp.uint32(0xFFFF0000), F32)


def _pk(x):
    return pltpu.bitcast(x.astype(BF16), U32)


def _upk(x):
    return pltpu.bitcast(x, BF16)


def _dot(a, b):
    return jnp.dot(a, b, preferred_element_type=F32)


def _dot_nt(a, b):
    return lax.dot_general(a, b, _NT, preferred_element_type=F32)


def _x_ops(x1, x2):
    d = [a - b for a, b in zip(x1, x2)]
    return [x1[0] + x2[1], x2[0] + x2[1], x1[0] + x1[1],
            d[1] + x1[2], x1[1] + x1[2], d[1] + d[2],
            d[0] - x2[2], d[0] + d[2], x2[0] + x2[2],
            x1[0], d[0], x2[1], d[1], x1[2], x2[2]]


def _x_rem(x1, x2):
    a, b, c = 0, 1, 2
    cat = lambda u, v: jnp.concatenate([u, v], axis=0)
    return [cat(x1[c], x2[b]), cat(x1[a], x1[b] - x2[b]), cat(x2[a], x2[c] - x1[c])]


_W_TERMS = {0: ((0, 1, 1), (1, 0, 1)), 3: ((1, 2, 1), (2, 1, 1)), 6: ((0, 2, 1), (2, 0, 1)),
            9: ((0, 0, 1), (0, 2, 1), (1, 0, -1)), 10: ((2, 0, 1), (0, 0, -1), (0, 1, -1)),
            11: ((1, 1, 1), (1, 2, 1), (0, 1, -1)), 12: ((1, 0, 1), (1, 1, 1), (2, 1, -1)),
            13: ((2, 0, 1), (2, 2, 1), (1, 2, -1)), 14: ((2, 1, 1), (2, 2, 1), (0, 2, -1)),
            1: ((0, 1, 1),), 2: ((1, 0, 1),), 4: ((1, 2, 1),), 5: ((2, 1, 1),),
            7: ((2, 0, 1),), 8: ((0, 2, 1),)}


def _w_sums(w):
    return [_signed(_W_TERMS[i], lambda k, j: w[k][j]) for i in _W_SUM]


_W_SUM = {0: 0, 3: 1, 6: 2, 9: 3, 10: 4, 11: 5, 12: 6, 13: 7, 14: 8}
_W_RAW = {1: (0, 1), 2: (1, 0), 4: (1, 2), 5: (2, 1), 7: (2, 0), 8: (0, 2)}
_PAIR_ORDER = (1, 2, 4, 5, 7, 8, 0, 3, 6)
_DIAG = {(0, 0): 9, (2, 0): 10, (0, 1): 11, (1, 1): 12, (1, 2): 13, (2, 2): 14}
_PAIR = {(0, 0): ((6, -1), (8, -1)), (1, 0): ((2, 1), (7, 1)), (2, 0): ((0, 1), (1, -1)),
         (0, 1): ((3, 1), (4, -1)), (1, 1): ((0, 1), (2, -1)), (2, 1): ((1, 1), (5, -1)),
         (0, 2): ((4, 1), (8, 1)), (1, 2): ((6, 1), (7, -1)), (2, 2): ((5, 1), (3, -1))}


def _column(t, base, j, skew=False):
    s = []
    for k in range(3):
        v = base[k]
        for i, sg in _PAIR[k, j]:
            v = t[i] if v is None else (v + t[i] if sg > 0 else v - t[i])
        s.append(v)
    if skew:
        return s[1] + s[0], s[2] + 0.5 * (s[0] - s[1])
    return s[1] + s[0], s[2] + s[0]


_SA = (((0, 0, 1), (1, 1, 1)), ((1, 0, 1), (1, 1, 1)), ((0, 0, 1),), ((1, 1, 1),),
       ((0, 0, 1), (0, 1, 1)), ((1, 0, 1), (0, 0, -1)), ((0, 1, 1), (1, 1, -1)))
_SB = (((0, 0, 1), (1, 1, 1)), ((0, 0, 1),), ((0, 1, 1), (1, 1, -1)), ((1, 0, 1), (0, 0, -1)),
       ((1, 1, 1),), ((0, 0, 1), (0, 1, 1)), ((1, 0, 1), (1, 1, 1)))
_SCOL = {2: 1, 3: 0, 5: 1, 6: 0}
_SGRP = ((1, 4, 0), (3, 6), (2, 5))


def _signed(terms, f):
    v = None
    for a, b, sg in terms:
        v = f(a, b) if v is None else (v + f(a, b) if sg > 0 else v - f(a, b))
    return v


def _s_out(m):
    return [[m[0] + m[3] - m[4] + m[6], m[2] + m[4]],
            [m[1] + m[3], m[0] - m[1] + m[2] + m[5]]]


def _make_kernel(S, D, F, TM, cfg):
    NB = S // TM
    NT = TM // LANES
    DH = D // H
    DP = DH // 2
    RP = D // 2
    NG = H // 8
    scale = float(DH) ** -0.5
    NU = 2 * NB
    TH = TM // 2
    TQ = TM // 4
    D2 = D // 2
    D3 = D // 3
    Q3 = D3 // 2
    KU = D // 9
    KR = 3 * LANES
    NQ = 6
    QR = 3 * D // NQ
    WQ = (0, 640, 1152, 3 * D)
    PW = 4 * LANES
    NP = F // PW
    AOFF, fill = {}, [0, 0]
    for key in [(m1, m2) for m1 in range(7) for m2 in range(7)]:
        c = int(fill[1] < fill[0])
        AOFF[key] = (fill[c], slice(c * LANES, (c + 1) * LANES))
        fill[c] += 48 if key[0] in _SCOL and key[1] in _SCOL else 32
    scopes = cfg['scopes']
    assert NG == 4 and NB & (NB - 1) == 0
    SEM_P = 4

    def kernel(x_hbm, wqkv_hbm, wo_hbm, wg_hbm, wu_hbm, wdt_hbm, out_hbm,
               xio_s, wqkv_v, wo_v, wg_v, wu_v, wdt_v, wt_s, wl_s,
               gu_s, ds_s, xmid_s, a_s, qkv_s, o_s, acc_s, h3_s, r_s,
               sem_i, sem_o):

        def wait(name, cps):
            if scopes:
                with jax.named_scope(name):
                    for cp in cps:
                        cp.wait()
            else:
                for cp in cps:
                    cp.wait()

        def cols(lo, n):
            if not isinstance(lo, int):
                lo = pl.multiple_of(lo, LANES)
            return pl.ds(lo, n)

        def rows8(lo, n=8):
            if not isinstance(lo, int):
                lo = pl.multiple_of(lo, 8)
            return pl.ds(lo, n)

        def out_copy(b):
            return pltpu.make_async_copy(
                xio_s.at[b], out_hbm.at[:, cols(b * TM, TM)], sem_o.at[0])

        def x_cp(b, sem):
            return pltpu.make_async_copy(x_hbm.at[:, cols(b * TM, TM)], xio_s.at[b],
                                         sem_i.at[sem])

        def wq_cp(i):
            sl = cols(WQ[i], WQ[i + 1] - WQ[i])
            return pltpu.make_async_copy(wqkv_hbm.at[:, sl], wqkv_v.at[:, sl],
                                         sem_i.at[1 + i])

        def piece_cp(src, dst, p, sem, c0=0, n=PW):
            return pltpu.make_async_copy(src.at[:, cols(p * PW + c0, n)],
                                         dst.at[p, :, pl.ds(c0, n)], sem_i.at[sem])

        def group_cp(p):
            sem = SEM_P + p
            cps = []
            if not (isinstance(p, int) and p == NP):
                cps += [piece_cp(wg_hbm, wg_v, p, sem), piece_cp(wu_hbm, wu_v, p, sem)]
            if not (isinstance(p, int) and p == 0):
                cps.append(piece_cp(wdt_hbm, wdt_v, p - 1, sem, 0, KR))
            if isinstance(p, int) and p == NP:
                cps += [piece_cp(wdt_hbm, wdt_v, q, sem, KR, LANES) for q in range(NP)]
            return cps

        lane = lax.broadcasted_iota(jnp.int32, (8, LANES), 1)
        cat0 = lambda *v: jnp.concatenate(v, axis=0)
        cat1 = lambda *v: jnp.concatenate(v, axis=1)

        def spread_over(anchors, n, total):
            return anchors[n * len(anchors) // total] if anchors else None

        def slab_group(r):
            return (r % LANES) // 16 if r < KR else 8 + ((r - KR) % KU) // 16

        def ln1(blk, anchors1, anchors2=()):
            slabs = (xio_s[blk, r:r + 8, :].astype(F32) for r in range(0, D, 8))
            m, rs = _ln_stats(slabs, D, anchors1)
            if not anchors2:
                return (xio_s[blk].astype(F32) - m) * rs
            m8 = jnp.broadcast_to(m, (8, TM))
            ms = [_tie(m8, a) for a in anchors2]
            ms = [spread_over(ms, slab_group(r), 12) for r in range(0, D, 8)]
            return (xio_s[blk].astype(F32) - cat0(*ms)) * rs

        def dot_k(rows, x, anchors, even=False):
            y = None
            for n, k in enumerate(range(0, D, LANES)):
                ks = slice(k, min(k + LANES, D))
                if even and k + LANES >= D:
                    mid = (rows.start + rows.stop) // 2
                    v = cat0(_dot(_upk(wt_s[rows.start:mid, ks]), x[ks]),
                             _dot(_upk(wt_s[mid:rows.stop, ks]), x[ks]))
                else:
                    v = _dot(_upk(wt_s[rows, ks]), x[ks])
                anchors.extend(v[r:r + 8, :LANES] for r in ((0, 144) if n % 2 else (72, 216)))
                y = v if y is None else y + v
            return y

        def put_qkv(blk, rows, y):
            pk = _pk(y)
            for c in range(NT):
                qkv_s[1 + blk * NT + c, rows, :] = pk[:, c * LANES:(c + 1) * LANES]

        def qkv_mm(blk, xn, chunks, anchors, even=False):
            for r in chunks:
                rows = slice(r * QR // 2, (r + 1) * QR // 2)
                put_qkv(blk, rows, dot_k(rows, xn, anchors, even))

        def split_k(x):
            hs = (x[:, :TH], x[:, TH:])
            blocks = [[h[k * LANES:(k + 1) * LANES] for k in range(3)] for h in hs]
            units = [[h[KR + k * KU:KR + (k + 1) * KU] for k in range(3)] for h in hs]
            return blocks, units

        def prep_att(pat, anchor):
            assert Q3 == 96
            row0 = pat * 8
            src0 = row0 + ((pat * 43) >> 9) * (2 * Q3)
            w = [_upk(wt_s[rows8(src0 + j * Q3), :D]).astype(F32) for j in range(3)]
            w[0] = cat1(_tie(w[0][:, :LANES], anchor), w[0][:, LANES:])
            tiles = _w_sums([[w[j][:, k * LANES:(k + 1) * LANES] for j in range(3)]
                             for k in range(3)])
            for j in range(3):
                a, b, c = (w[j][:, KR + k * KU:KR + (k + 1) * KU] for k in range(3))
                tiles += [cat1(c, b), cat1(a, c)]
            wl_s[rows8(row0), :15 * LANES] = _pk(cat1(*tiles))

        def att_rhs(x, stash=None, anchors=()):
            half = 0.5
            if anchors:
                hs = [_tie(jnp.full((8, TH), 0.5, F32), a) for a in anchors]
                half = cat0(*[spread_over(hs, slab_group(r), 12) for r in range(0, D, 8)])
            blocks, units = split_k(cat1(x[:, :TH], x[:, TH:] + half * x[:, :TH]))
            ops = _x_ops(*blocks) + _x_rem(*units)
            if stash is None:
                return [v.astype(BF16) for v in ops]
            loc = lambda i, r0, n: (slice((i // 2) * 64 + r0, (i // 2) * 64 + r0 + n),
                                    slice((i % 2) * LANES, (i % 2 + 1) * LANES))
            for r in range(0, LANES, 16):
                for i, v in enumerate(ops):
                    r_s.at[0][loc(i, r // 2, 8)] = _pk(v[r:r + 16])
            return [_upk(r_s.at[stash][loc(i, 0, 64)]) for i in range(18)]

        def att_mm(sec, rhs, anchors):
            tl = lambda i: _upk(wl_s[sec * Q3:(sec + 1) * Q3, i * LANES:(i + 1) * LANES])
            raw = lambda k, j: _upk(wt_s[(3 * sec + j) * Q3:(3 * sec + j + 1) * Q3,
                                         k * LANES:(k + 1) * LANES])
            t = {}
            for i in _PAIR_ORDER:
                t[i] = _dot(raw(*_W_RAW[i]) if i in _W_RAW else tl(_W_SUM[i]), rhs[i])
                anchors.append(t[i][:8])
            out = []
            for j in range(3):
                base = []
                for s in range(3):
                    v = _dot(raw(3, j) if s == 1 else tl(9 + 2 * j + s // 2), rhs[15 + s])
                    if (s, j) in _DIAG:
                        i = _DIAG[s, j]
                        v = _dot(tl(_W_SUM[i]), rhs[i]) + v
                    base.append(v)
                    anchors.append(base[-1][:8])
                out.append(cat1(*_column(t, base, j, True)))
            return cat0(*out)

        def qkv_fast(blk, rhs, anchors):
            for sec in range(3):
                put_qkv(blk, slice(sec * RP, (sec + 1) * RP), att_mm(sec, rhs, anchors))

        def shifted(ln, cur, prev, w):
            if w == 0:
                return cur
            sh = DIL * w
            return pltpu.roll(jnp.where(ln < LANES - sh, cur, prev), sh, axis=1)

        def att_group(blk, c, hg, anchor):
            att_values(blk, c, hg, anchor)(None)

        def att_values(blk, c, hg, anchor):
            tile = blk * NT + c
            base = hg * 8 * DP
            if isinstance(hg, int):
                cur, prev, o_t = qkv_s.at[1 + tile], qkv_s.at[tile], o_s.at[c]
            else:
                n = 2 * RP + 8 * DP
                base = pl.multiple_of(base, 8)
                cur = qkv_s.at[1 + tile, pl.ds(base, n)]
                prev = qkv_s.at[tile, pl.ds(base, n)]
                o_t = o_s.at[c, pl.ds(base, RP + 8 * DP)]
                base = 0
            ln = lane + _zero_like_dep(anchor).astype(jnp.int32)
            logits = [None] * W
            for dd in range(DP):
                q = cur[pl.ds(base + dd, 8, stride=DP), :]
                kc = cur[pl.ds(RP + base + dd, 8, stride=DP), :]
                kp = prev[pl.ds(RP + base + dd, 8, stride=DP), :]
                q0, q1 = _lo(q), _hi(q)
                for w in range(W):
                    ks = shifted(ln, kc, kp, w)
                    t = q0 * _lo(ks) + q1 * _hi(ks)
                    logits[w] = t if logits[w] is None else logits[w] + t
            logits = [l * scale for l in logits]
            if not (isinstance(c, int) and c > 0):
                pos = lane + tile * LANES
                logits = [l if w == 0 else jnp.where(pos >= DIL * w, l, -1e9)
                          for w, l in enumerate(logits)]
            m = _tree_sum(logits, jnp.maximum)
            p = [jnp.exp(l - m) for l in logits]
            r = 1.0 / _tree_sum(p)

            def apply(anchor2):
                ln = lane + _zero_like_dep(_tie(m, anchor2)).astype(jnp.int32)
                for dd in range(DP):
                    vc = cur[pl.ds(2 * RP + base + dd, 8, stride=DP), :]
                    vp = prev[pl.ds(2 * RP + base + dd, 8, stride=DP), :]
                    o0 = o1 = None
                    for w in range(W):
                        vs = shifted(ln, vc, vp, w)
                        t0, t1 = p[w] * _lo(vs), p[w] * _hi(vs)
                        o0 = t0 if o0 is None else o0 + t0
                        o1 = t1 if o1 is None else o1 + t1
                    o0, o1 = o0 * r, o1 * r
                    o_t[pl.ds(base + dd, 8, stride=DP), :] = o0
                    o_t[pl.ds(RP + base + dd, 8, stride=DP), :] = o1

            return apply

        def attention(blk, anchors):
            for c in range(NT):
                for hg in range(NG):
                    att_group(blk, c, hg, anchors[c * NG + hg])

        def wo_mm(blk, anchors, fast, stash=None, anchors_in=()):
            o = cat1(*[o_s[c] for c in range(NT)])
            if fast:
                y = att_mm(3, att_rhs(o, stash, anchors_in), anchors)
            else:
                o = o.astype(BF16)
                q = D2 // 2
                y = cat0(*[dot_k(slice(h * q, (h + 1) * q), o, anchors) for h in (6, 7)])
            xm = xio_s[blk].astype(F32) + y
            xmid_s[blk] = xm
            return _ln_stats((xm[r:r + 8] for r in range(0, D, 8)), D)

        def ffn_lhs(blk, stats, anchors):
            m, rs = stats
            m8 = jnp.broadcast_to(m, (8, TM))
            xt = []
            for k in range(5):
                mt = cat0(*[_tie(m8, spread_over(anchors[:2], k, 5))] * (KU // 8 if k == 4 else 16))
                x = (xmid_s[blk, k * LANES:min((k + 1) * LANES, D), :] - mt) * rs
                xt.append((cat0(x, x) if k == 4 else x).T)
            lo = lax.broadcasted_iota(jnp.int32, (TQ // 2, LANES), 1) < KU
            for m1 in range(7):
                a = spread_over(anchors[2:], m1, 7)
                blk1 = lambda i2, k2: _signed(_SA[m1], lambda i1, k1: _tie(
                    xt[k2 if k2 == 4 else 2 * k1 + k2][(2 * i1 + i2) * TQ:(2 * i1 + i2 + 1) * TQ], a))
                l1 = {(i2, k2): blk1(i2, k2) for i2 in range(2)
                      for k2 in ((0, 1, 4) if m1 in _SCOL else (0, 1))}
                for m2 in range(7):
                    v = _signed(_SA[m2], lambda i2, k2: l1[i2, k2])
                    if m1 in _SCOL and m2 in _SCOL:
                        c = _signed(_SA[m2], lambda i2, k2: l1[i2, 4])
                        h = TQ // 2
                        vp, vq, cp, cq = v[:h], v[h:], c[:h], c[h:]
                        v = cat0(jnp.where(lo, cp, vq), jnp.where(lo, vp, vp - vq),
                                 jnp.where(lo, vq, cq - cp))
                    o, ac = AOFF[m1, m2]
                    a_s[o:o + v.shape[0] // 2, ac] = _pk(v)

        def in_triple(q):
            return q, lambda k: (q, k)

        def cross_triple(s):
            return NP + s, lambda k: (3 * s + k, 3)

        def wd_raw(tri, k, r0, n):
            q, c = tri[1](k)
            return wdt_v[q, r0:r0 + n, c * LANES:(c + 1) * LANES]

        def ds_loc(i, r0, n):
            return slice(r0, r0 + n), slice((i % 2) * LANES, (i % 2 + 1) * LANES)

        def prep_d(tri, anchors):
            PR = 16
            for n in range(D3 // PR):
                r = n * PR
                w = [[wd_raw(tri, k, j * D3 + r, PR).astype(F32) for j in range(3)]
                     for k in range(3)]
                w[0][1] = _tie(w[0][1], spread_over(anchors, n, D3 // PR))
                for i, v in enumerate(_w_sums(w)):
                    ds_s.at[tri[0], i // 2][ds_loc(i, r // 2, PR // 2)] = _pk(v)

        GU = (wg_v, wu_v)

        def prep_gu(p, gv, m, m1s, anchors):
            PR = 16
            cs = slice(m * LANES, (m + 1) * LANES)
            for n in range(LANES // PR):
                r = n * PR
                cache = {}

                def w(k, j1):
                    if (k, j1) not in cache:
                        v = GU[m][p, k * LANES + r:k * LANES + r + PR,
                                  2 * j1 * LANES:2 * (j1 + 1) * LANES].astype(F32)
                        if (k // 2, j1) in [_SB[m1][0][:2] for m1 in m1s[:2]]:
                            a = spread_over(anchors, n, LANES // PR)
                            c = (k % 2) * LANES
                            tied = _tie(v[:, c:c + LANES], a)
                            v = cat1(v[:, :LANES], tied) if c else cat1(tied, v[:, LANES:])
                        cache[k, j1] = v
                    return cache[k, j1]

                for m1 in m1s:
                    b1 = [_signed(_SB[m1], lambda k1, j1: w(2 * k1 + k2, j1)) for k2 in range(2)]
                    for m2 in range(7):
                        v = _signed(_SB[m2],
                                    lambda k2, j2: b1[k2][:, j2 * LANES:(j2 + 1) * LANES])
                        gv.at[7 * m1 + m2][r // 2:(r + PR) // 2, cs] = _pk(v)

        def prep_tail(p, gv, m, anchor):
            v = _tie(GU[m][p, 4 * LANES:, :].astype(F32), anchor)
            for j in range(4):
                gv.at[49 + j // 2][(j % 2) * 32:(j % 2 + 1) * 32,
                                        m * LANES:(m + 1) * LANES] = _pk(
                                            v[:, j * LANES:(j + 1) * LANES])

        def gu_outer(gv, m, m1, anchors, at=(0, 4)):
            cs = slice(m * LANES, (m + 1) * LANES)
            y = {}
            for m2 in cfg['inner']:
                i, (o, ac) = 7 * m1 + m2, AOFF[m1, m2]
                if m1 in _SCOL and m2 in _SCOL:
                    j = 2 * _SCOL[m1] + _SCOL[m2]
                    tail = lambda: gv[49 + j // 2, (j % 2) * 32:(j % 2 + 1) * 32, cs]
                    rhs = (cat0(tail(), gv[i, 32:, cs]), gv[i, :, cs],
                           cat0(gv[i, :32, cs], tail()))
                    r = [_dot(_upk(a_s[o + 16 * s:o + 16 * (s + 1), ac]), _upk(rhs[s]))
                         for s in range(3)]
                    y[m2] = cat0(r[1] + r[0], r[2] + r[0])
                else:
                    y[m2] = _dot(_upk(a_s[o:o + TQ // 2, ac]), _upk(gv[i, :, cs]))
            anchors.extend(y[cfg['inner'][k % 7]][(k // 7) * 32:(k // 7) * 32 + 8] for k in at)
            return _s_out(y)

        def gu_finish(t):
            gu = [{(i2, j2): _s_out([t[m][m1][i2][j2] for m1 in range(7)])
                   for i2 in range(2) for j2 in range(2)} for m in range(2)]
            return [[cat0(*[_gelu_mul2(*[gu[m][i2, j % 2][i1][j // 2] for m in range(2)])
                            for i2 in range(2)]) for i1 in range(2)] for j in range(4)]

        def gu_piece(gv, order, anchors, at=(0, 4)):
            t = ({}, {})
            for m, m1 in order:
                t[m][m1] = gu_outer(gv, m, m1, anchors, at)
            return gu_finish(t)

        def prep_piece(p, gv, anchors, group):
            if group in (0, 1):
                grp = _SGRP if group else [(m1,) for m1 in range(7)]
                k = len(anchors) // (2 * len(grp))
                for n in range(2 * len(grp)):
                    prep_gu(p, gv, n % 2, grp[n // 2], anchors[k * n:k * n + k])
            else:
                k, n = len(anchors) // 14, 0
                for g in group:
                    for m in range(2):
                        prep_gu(p, gv, m, g, anchors[n:n + k * len(g)])
                        n += k * len(g)
            for m in range(2):
                prep_tail(p, gv, m, anchors[m * len(anchors) // 2])

        def h_ops(h):
            return [v.astype(BF16) for v in _x_ops(*[[h[k][i] for k in range(3)]
                                                     for i in range(2)])]

        D_ORDER = _PAIR_ORDER + (9, 10, 11, 12, 13, 14)

        def down_mm(acc, work, anchors, which=D_ORDER):
            p = [None] * 15 if acc is None else list(acc)
            jobs = [(i, n) for i in which for n in range(len(work))]
            split = {0: (), 1: (4,), 2: (2, 2), 3: (2, 2, 4)}[len(jobs) % 4]
            split = dict(zip(jobs[len(jobs) - len(split):], split))
            for i in which:
                y = None
                for n, (tri, b) in enumerate(work):
                    ns = split.get((i, n), 1)
                    nr = D3 // ns
                    if i in _W_RAW:
                        k, j = _W_RAW[i]
                        lhs = lambda h: wd_raw(tri, k, j * D3 + h * nr, nr)
                    else:
                        s = _W_SUM[i]
                        lhs = lambda h: _upk(ds_s.at[tri[0], s // 2][ds_loc(s, h * nr // 2, nr // 2)])
                    v = cat0(*[_dot_nt(lhs(h), b[i]) for h in range(ns)])
                    y = v if y is None else y + v
                p[i] = y if p[i] is None else p[i] + y
                anchors.append(p[i][:8])
            return p

        def finish(blk, acc, after=None):
            y = [cat1(*_column(acc, [acc[_DIAG[s, j]] if (s, j) in _DIAG else None
                                     for s in range(3)], j)) for j in range(3)]
            if after is None:
                xio_s[blk] = (xmid_s[blk] + 0.5 * cat0(*y)).astype(BF16)
                return
            for j in range(3):
                rows = slice(j * D3, (j + 1) * D3)
                xio_s[blk, rows] = (xmid_s[blk, rows] + 0.5 * y[j]).astype(BF16)
                after(j)

        def load_acc(k):
            return [acc_s[k, i] for i in range(15)]

        def store_acc(k, acc):
            for i in range(15):
                acc_s[k, i] = acc[i]

        def early_gu(order):
            o, ac = AOFF[order[0][1], cfg['inner'][0]]
            return [a_s[o + 8 * k:o + 8 * k + 8, ac] for k in range(4)]

        def early_wt(row):
            return [wt_s[row + 16 * k:row + 16 * k + 8, :LANES] for k in range(4)]

        def pre_phase():
            first = [[x_cp(0, 0)], [wq_cp(0)], [x_cp(1, 2), wq_cp(1)],
                     [wq_cp(2), pltpu.make_async_copy(wo_hbm, wo_v, sem_i.at[3])]]
            order = sum(first, [])
            for p in range(NP + 1):
                order += group_cp(p)
            xr_cp = [x_cp(b, SEM_P + NP + 1) for b in range(2, NB)]
            order += xr_cp
            for cp in order:
                cp.start()
            get = lambda an, name: [an[min(i, len(an) - 1)] for i in cfg[name]]
            e_grp = lambda e: ((e >> 1) & 1, ((e >> 2) << 1) | (e & 1))
            if 'a' in cfg['sub']:
                pre_a(first, get, e_grp)
            if 'b' in cfg['sub']:
                pre_b(get, e_grp)
            if 'c' in cfg['sub']:
                pre_c(get)
            wait('WX', xr_cp)

        def pre_a(first, get, e_grp):
            def transpose_wq(i):
                wt_s[WQ[i] // 2:WQ[i + 1] // 2, :D] = _pk(wqkv_v[:, WQ[i]:WQ[i + 1]].T)

            def clear(i, carry):
                for k in range(2):
                    acc_s[k, i] = jnp.zeros((D3, TH), F32)
                r = jnp.minimum(i, 11) * (RP // 4)
                qkv_s[0, rows8(r, RP // 4)] = jnp.zeros((RP // 4, LANES), U32)
                return carry

            lax.fori_loop(0, 15, clear, 0)
            wait('WX0', first[0])
            xn0 = ln1(0, ()).astype(BF16)

            wait('WQ0', first[1])
            transpose_wq(0)
            qkv_mm(0, xn0, (0, 1), [])

            wait('WQ1', first[2])
            transpose_wq(1)
            an = []
            qkv_mm(0, xn0, (2, 3), an)
            xn1 = ln1(1, get(an, 'a_ln'), get(an, 'a_lnb')).astype(BF16)
            qkv_mm(1, xn1, (0,), an, True)
            for n, a in enumerate(get(an, 'a_w1')):
                prep_att(n, a)
            nk = len(cfg['a_k'])
            apply = [att_values(0, *e_grp(e), a) for e, a in enumerate(get(an, 'a_k'))]

            wait('WQ2', first[3])
            an = early_wt(QR)
            qkv_mm(1, xn1, (2,), an)
            transpose_wq(2)
            qkv_mm(0, xn0, (4, 5), an)
            qkv_mm(1, xn1, (4,), an)
            qkv_mm(1, xn1, (1,), an, True)
            apply += [att_values(0, *e_grp(nk + e), a)
                      for e, a in enumerate(get(an, 'a_k2')[:8 - nk])]
            for e, a in enumerate(get(an, 'a_v')):
                apply[e](a)
            wo = pltpu.bitcast(wo_v[...], U32)
            wo = cat0(_lo(wo), _hi(wo))
            wo = cat0(*[_tie(wo[n * LANES:(n + 1) * LANES], a)
                        for n, a in enumerate(get(an, 'a_wo'))])
            wt_s[3 * RP:, :D] = _pk(wo.astype(BF16).T)
            for n, a in enumerate(get(an, 'a_w2')):
                prep_att(len(cfg['a_w1']) + n, a)

            wait('WO', group_cp(0))
            an = early_wt(3 * RP)
            stats = wo_mm(0, an, False)
            qkv_mm(1, xn1, (3, 5), an)
            for n, a in enumerate(get(an, 'z_w')):
                prep_att(36 + n, a)
            prep_piece(0, gu_s.at[0], get(an, 'z_g'), cfg['z_grp'])
            ffn_lhs(0, stats, get(an, 'z_l'))

        def pre_b(get, e_grp):
            def piece(p, carry):
                wait('WP', group_cp(p))
                an = early_gu(cfg['gorder0'])
                win = gu_s.at[pl.ds(p - 1, 2)]
                h = gu_piece(win.at[0], cfg['gorder0'], an, (0, 7, 4, 11))
                h3_s[p - 1] = cat0(*h[3])
                tri = in_triple(p - 1)
                prep_d(tri, get(an, 'p_d'))
                store_acc(0, down_mm(load_acc(0), [(tri, h_ops(h[:3]))], an))
                prep_piece(p, win.at[1], get(an, 'f_g'), cfg['f_grp'])
                att_group(1, *e_grp(p - 1), an[cfg['p_att'][0]])
                return carry

            lax.fori_loop(1, NP, piece, 0)

        def pre_c(get):
            wait('WD', group_cp(NP))
            an = early_gu(cfg['torder'])
            h = gu_piece(gu_s.at[NP - 1], cfg['torder'], an)
            h3 = [[h3_s[q, :TH], h3_s[q, TH:]] for q in range(NP - 1)] + [h[3]]
            work = [(cross_triple(s), h_ops(h3[3 * s:3 * s + 3])) for s in range(3)]
            work.append((in_triple(NP - 1), h_ops(h[:3])))
            stats = wo_mm(1, an, True)
            td = get(an, 't_d')
            for n, (tri, _) in enumerate(work):
                prep_d(tri, td[n * len(td) // 4:(n + 1) * len(td) // 4])
            acc = down_mm(load_acc(0), work, an)
            nw = len(cfg['a_w1']) + len(cfg['a_w2'])
            for n, a in enumerate(get(an, 't_w')[:36 - nw]):
                prep_att(nw + n, a)
            ffn_lhs(1, stats, get(an, 't_l'))
            finish(0, acc)

        if 'pre' in cfg['phases']:
            pre_phase()

        def body(u, carry):
            bu = u & (NB - 1)
            ba = (u + 1) & (NB - 1)
            acc, stats, an, b, hh = None, None, {}, {}, {}
            get = lambda name: [an[k][i] for k, i in cfg[name]]
            for step in cfg['body']:
                an[step] = []
                if step == 'Q':
                    xn = ln1(ba, get('ln1'), get('ln1b'))
                    qkv_fast(ba, att_rhs(xn, u >> 8), an[step])
                elif step == 'W':
                    attention(ba, get('att'))
                    stats = wo_mm(ba, an[step], True, u >> 8, get('orhs'))
                elif step == 'L':
                    ffn_lhs(ba, stats, get('lhs'))
                elif step[0] == 'G':
                    q, go = int(step[1]), cfg['gorder']
                    t = b.setdefault(step[:2], ({}, {}))
                    for m, m1 in (go[:7] if step[2] == '0' else go[7:]):
                        t[m][m1] = gu_outer(gu_s.at[q], m, m1, an[step])
                    if len(t[0]) + len(t[1]) == 14:
                        hh[q] = gu_finish(t)
                else:
                    work = []
                    for c in step[1:]:
                        if c.isdigit():
                            work.append((in_triple(int(c)), h_ops(hh[int(c)][:3])))
                        else:
                            s = ord(c) - ord('a')
                            work.append((cross_triple(s),
                                         h_ops([hh[3 * s + k][3] for k in range(3)])))
                    acc = down_mm(acc, work, an[step])
            finish(bu, acc)

            @pl.when(u >= NB)
            def _():
                out_copy(bu).start()
            return carry

        if scopes:
            with jax.named_scope('LOOP'):
                lax.fori_loop(1, NU - 1, body, 0)
        elif 'main' in cfg['phases']:
            lax.fori_loop(1, NU - 1, body, 0)

        fin_cp = [pltpu.make_async_copy(
            xio_s.at[NB - 1, pl.ds(j * D3, D3)],
            out_hbm.at[pl.ds(j * D3, D3), cols((NB - 1) * TM, TM)], sem_o.at[0])
            for j in range(3)]

        def last(s, carry):
            h = [gu_piece(gu_s.at[3 * s + k], cfg['lorder'], []) for k in range(3)]
            work = [(in_triple(3 * s + k), h_ops(h[k][:3])) for k in range(3)]
            work.append((cross_triple(s), h_ops([h[k][3] for k in range(3)])))
            acc = down_mm(down_mm(load_acc(1), work[:2], []), work[2:], [], cfg['ldord'])
            store_acc(1, acc)
            finish(NB - 1, acc, lambda j: pl.when(s == NP // 3 - 1)(fin_cp[j].start))
            return carry

        if 'last' in cfg['phases']:
            lax.fori_loop(0, NP // 3, last, 0)
        if len(cfg['phases']) < 3:
            def keep(i, c):
                v = (gu_s[i, i, :8, :LANES] + ds_s[i, i, :8, :LANES]
                     + wl_s[rows8(i * 8), :LANES] + a_s[rows8(i * 8), :LANES] + qkv_s[i, :8]
                     + wt_s[rows8(i * 8), :LANES])
                acc_s[1, 0, :8] = (lax.bitcast_convert_type(v, F32) + o_s[i, :8]
                                   + acc_s[i, i, :8] + h3_s[i, :8])
                return c
            lax.fori_loop(0, 2, keep, 0)
            finish(NB - 1, load_acc(1))
            out_copy(0).start()
        wait('WOUT', [out_copy(b) for b in range(NB - 1)] + fin_cp)

    scratch = [
        pltpu.VMEM((NB, D, TM), BF16),
        pltpu.VMEM((D, 3 * D), BF16),
        pltpu.VMEM((D, D), BF16),
        pltpu.VMEM((NP, D, PW), BF16),
        pltpu.VMEM((NP, D, PW), BF16),
        pltpu.VMEM((NP, D, PW), BF16),
        pltpu.VMEM((2 * D, 8 * LANES), U32),
        pltpu.VMEM((4 * Q3, 16 * LANES), U32),
        pltpu.VMEM((NP, 51, 64, 2 * LANES), U32),
        pltpu.VMEM((NP + 3, 5, Q3, 2 * LANES), U32),
        pltpu.VMEM((NB, D, TM), F32),
        pltpu.VMEM((max(fill), 2 * LANES), U32),
        pltpu.VMEM((S // LANES + 1, 3 * RP, LANES), U32),
        pltpu.VMEM((NT, D, LANES), F32),
        pltpu.VMEM((2, 15, D3, TH), F32),
        pltpu.VMEM((NP, TM, LANES), F32),
        pltpu.VMEM((1, 9 * 64, 2 * LANES), U32),
        pltpu.SemaphoreType.DMA((SEM_P + NP + 2,)),
        pltpu.SemaphoreType.DMA((1,)),
    ]

    def wrapped(*refs):
        @pl.when(pl.program_id(0) == 0)
        def _():
            kernel(*refs)

    return wrapped, scratch


_CFG = dict(
    scopes=False,
    ldord=(1, 2, 0, 7, 8, 6, 9, 10, 4, 5, 3, 11, 12, 13, 14),
    orhs=(('G80', 0), ('G80', 1), ('G80', 2), ('G80', 3), ('G80', 4), ('G80', 5),
        ('G80', 6), ('G80', 7), ('G80', 8), ('G80', 9), ('G80', 10), ('G80', 11)),
    sub='abc',
    phases=('pre', 'main', 'last'),
    body=('G20', 'G00', 'G01', 'G10', 'G11', 'Q', 'G30', 'G21', 'G40', 'G31', 'G50',
        'D012a', 'G41', 'G51', 'D345b', 'G70', 'G60', 'G71', 'G80', 'W', 'G61', 'G81',
        'D8c', 'D67', 'L'),
    ln1=(('G00', 0), ('G00', 1), ('G00', 2), ('G00', 3), ('G00', 4), ('G00', 5), ('G00',
        6), ('G00', 7), ('G00', 8)),
    ln1b=(('G10', 1), ('G10', 2), ('G10', 3), ('G10', 4), ('G10', 5), ('G10', 6),
        ('G10', 7), ('G10', 8), ('G10', 9), ('G10', 10), ('G10', 11), ('G10', 12)),
    att=(('D012a', 2), ('D012a', 4), ('D012a', 5), ('D012a', 8), ('D012a', 9), ('D345b',
        5), ('D345b', 6), ('D345b', 8)),
    lhs=(('D8c', 2), ('D8c', 3), ('D8c', 9), ('D8c', 11), ('D67', 5), ('D67', 8),
        ('D67', 10), ('D67', 11), ('D67', 14)),
    a_w1=(0, 0, 1, 1, 2, 2, 3, 3, 4, 5, 6, 11, 13, 15, 18, 20, 21, 21, 23, 24, 26, 27,
        28, 29),
    a_w2=(0, 3, 4, 13, 18, 23),
    a_ln=(3, 6, 7),
    a_lnb=(3, 11, 15),
    z_g=(0, 1, 2, 3, 4, 4, 5, 5, 6, 6, 7, 7, 8, 8, 9, 9, 10, 10, 11, 11, 12, 12, 13, 15,
        16, 16, 16, 17, 18, 18, 19, 19, 20, 20, 21, 22, 22, 23, 23, 24, 25, 25, 25, 26,
        27, 27, 28, 39),
    t_d=(4, 4, 4, 6, 6, 7, 8, 9, 11, 11, 12, 12, 13, 14, 15, 15, 16, 16, 17, 18, 18, 19,
        20, 20, 21, 21, 22, 22, 25, 26, 28, 28, 29, 32, 32, 34, 36, 36, 39, 39, 40, 41,
        41, 41, 43, 44, 44, 46),
    p_d=(6, 16, 21, 29, 29, 32, 37, 38, 42, 46, 50, 53),
    p_att=(65,),
    z_l=(27, 27, 32, 35, 40, 41, 41, 42, 43),
    a_k=(13, 17, 20, 26),
    a_k2=(5, 6, 7, 9),
    a_v=(11, 16, 17, 18, 20, 21, 22, 23),
    a_wo=(13, 22, 29, 40, 50),
    inner=(0, 3, 4, 6, 2, 1, 5),
    gorder=((0, 4), (0, 0), (1, 4), (1, 0), (1, 6), (0, 3), (1, 3), (0, 6), (0, 1), (1,
        1), (0, 2), (1, 2), (0, 5), (1, 5)),
    gorder0=((0, 4), (0, 0), (0, 3), (1, 0), (1, 4), (0, 6), (1, 6), (1, 3), (1, 1), (0,
        1), (0, 2), (0, 5), (1, 2), (1, 5)),
    f_g=(0, 0, 0, 0, 1, 1, 2, 2, 3, 3, 4, 5, 8, 9, 10, 11, 12, 13, 13, 14, 15, 16, 17,
        18, 20, 21, 21, 23, 24, 25, 27, 28, 30, 32, 32, 33, 33, 36, 37, 37, 39, 40, 41,
        45, 47, 49, 49, 52, 53, 58, 62, 65, 68, 73, 74, 74),
    t_l=(53, 54, 55, 57, 58, 59, 61, 61, 64),
    lorder=((1, 0), (1, 4), (0, 0), (0, 4), (0, 3), (0, 6), (1, 3), (1, 6), (0, 1), (1,
        1), (0, 2), (0, 5), (1, 2), (1, 5)),
    z_w=(0, 5, 7, 7, 9, 10, 10, 11, 12, 13, 39, 43),
    z_grp=1,
    f_grp=((1, 0), (4, 2), (3, 6), (5,)),
    t_w=(2, 51, 51, 53, 56, 58),
    torder=((0, 0), (1, 4), (0, 4), (1, 3), (1, 6), (1, 0), (0, 3), (0, 6), (0, 1), (1,
        1), (0, 2), (1, 2), (1, 5), (0, 5)),
)


def _run(A_x, A_wqkv, A_wo, B_w_gate, B_w_up, B_w_down, **kw):
    _, S, D = A_x.shape
    F = B_w_gate.shape[1]
    kernel, scratch = _make_kernel(S, D, F, 256, {**_CFG, **kw})
    hbm = pl.BlockSpec(memory_space=pl.ANY)
    out_t = pl.pallas_call(
        kernel,
        grid=(2,),
        in_specs=[hbm] * 6,
        out_specs=hbm,
        out_shape=jax.ShapeDtypeStruct((D, S), A_x.dtype),
        scratch_shapes=scratch,
        compiler_params=pltpu.CompilerParams(
            dimension_semantics=('arbitrary',), vmem_limit_bytes=110 * 1024 * 1024),
    )(A_x.reshape(S, D).T, A_wqkv, A_wo, B_w_gate, B_w_up, B_w_down.T)
    return out_t.T.reshape(A_x.shape)


@jax.jit
def pallas_interleave_layers__sliding_local_dilated__glu_gated_geglu__prompt_kernel(
    A_x: jax.Array,
    A_wqkv: jax.Array,
    A_wo: jax.Array,
    B_x: jax.Array,
    B_w_gate: jax.Array,
    B_w_up: jax.Array,
    B_w_down: jax.Array,
):
    del B_x
    return _run(A_x, A_wqkv, A_wo, B_w_gate, B_w_up, B_w_down)
```
